```python
import jax
import jax.numpy as jnp

def _softmax(x, axis=-1):
    return jax.nn.softmax(x, axis=axis)

def _gelu(x):
    return jax.nn.gelu(x, approximate=True)

def _silu(x):
    return jax.nn.silu(x)

def _sigmoid(x):
    return jax.nn.sigmoid(x)

def _layernorm(x, axis=-1, eps=1e-05):
    m = jnp.mean(x, axis=axis, keepdims=True)
    v = jnp.var(x, axis=axis, keepdims=True)
    return (x - m) / jnp.sqrt(v + eps)

def _scatter_add(tgt, idx, src, axis=0):
    return tgt.at[idx].add(src)

def _segment_sum(src, seg, n):
    return jax.ops.segment_sum(src, seg, n)

class _Rng:

    def __init__(self, key):
        self._k = key

    def _next(self):
        self._k, sub = jax.random.split(self._k)
        return sub

    def normal(self, shape):
        return jax.random.normal(self._next(), shape, dtype=jnp.bfloat16)

    def randint(self, lo, hi, shape):
        return jax.random.randint(self._next(), shape, lo, hi, dtype=jnp.int32)

    def uniform(self, shape, lo=0.0, hi=1.0):
        return jax.random.uniform(self._next(), shape, jnp.bfloat16, lo, hi)

    def permutation(self, n):
        return jax.random.permutation(self._next(), n)
kernel_name = 'adaLN_cond__mha_block_cached__moe_arch_mod__prompt'

def setup_inputs():
    _rng = _Rng(jax.random.key(int.from_bytes(__import__("os").urandom(4), "little")))
    _w = lambda a: (lambda t: t.astype(jnp.bfloat16) if jnp.issubdtype(t.dtype, jnp.floating) else t)(jnp.asarray(a))

    def _A_setup():
        B, Sq, D = (1, 2048, 1024)
        H, Sk, Dh = (32, 2048, 128)
        return {'x': _w((lambda *s: _rng.normal(s) * 0.05)(B, Sq, D)), 'k_cache': _w((lambda *s: _rng.normal(s) * 0.05)(B, H, Sk, Dh)), 'v_cache': _w((lambda *s: _rng.normal(s) * 0.05)(B, H, Sk, Dh)), 'wq': _w((lambda *s: _rng.normal(s) * 0.05)(D, H * Dh) * D ** (-0.5)), 'wo': _w((lambda *s: _rng.normal(s) * 0.05)(H * Dh, D) * (H * Dh) ** (-0.5))}
    _A_in = _A_setup()

    def _B_setup():
        B, S, D, F, C = (1, 2048, 1024, 3584, 2)
        return {'x': _w((lambda *s: _rng.normal(s) * 0.05)(B, S, D)), 'w_r': _w((lambda *s: _rng.normal(s) * 0.05)(D)), 'w_gate': _w((lambda *s: _rng.normal(s) * 0.05)(D, F)), 'w_up': _w((lambda *s: _rng.normal(s) * 0.05)(D, F)), 'w_down': _w((lambda *s: _rng.normal(s) * 0.05)(F, D))}
    _B_in = _B_setup()
    return {'A_x': _A_in['x'], 'A_k_cache': _A_in['k_cache'], 'A_v_cache': _A_in['v_cache'], 'A_wq': _A_in['wq'], 'A_wo': _A_in['wo'], 'B_x': _B_in['x'], 'B_w_r': _B_in['w_r'], 'B_w_gate': _B_in['w_gate'], 'B_w_up': _B_in['w_up'], 'B_w_down': _B_in['w_down'], 'c': _w((lambda *s: _rng.normal(s) * 0.05)(1, 1024)), 'w_mod': _w((lambda *s: _rng.normal(s) * 0.05)(1024, 6 * 1024) * 1024 ** (-0.5))}

def reference(A_x, A_k_cache, A_v_cache, A_wq, A_wo, B_x, B_w_r, B_w_gate, B_w_up, B_w_down, c, w_mod):

    def _A_ref(x, k_cache, v_cache, wq, wo):
        B, Sq, D = x.shape
        H, Dh = (32, 128)
        q = (lambda x, *d: x.transpose(*d))((x @ wq).reshape(B, Sq, H, Dh), 0, 2, 1, 3)
        scores = jnp.einsum('bhqd,bhkd->bhqk', q, k_cache) * Dh ** (-0.5)
        p = _softmax(scores, axis=-1)
        o = jnp.einsum('bhqk,bhkd->bhqd', p, v_cache)
        return (lambda x, *d: x.transpose(*d))(o, 0, 2, 1, 3).reshape(B, Sq, H * Dh) @ wo

    def _B_ref(x, w_r, w_gate, w_up, w_down):
        B, S, D = x.shape
        C = 2
        r = x @ w_r
        idx = jnp.argsort(-r, axis=-1)[:, :C]
        idx_e = jnp.repeat(idx.reshape(B, C, 1), D, axis=2)
        x_sel = jnp.take_along_axis(x, idx_e, axis=1)
        g = _silu(x_sel @ w_gate)
        u = x_sel @ w_up
        y = g * u @ w_down
        r_sel = _sigmoid(jnp.take_along_axis(r, idx, axis=1))
        y = y * r_sel.reshape(B, C, 1)
        b_off = (jnp.arange(B) * S).reshape(B, 1)
        flat_idx = (idx + b_off).reshape(B * C)
        zero = (x * 0.0).reshape(B * S, D)
        upd = _scatter_add(zero, flat_idx, y.reshape(B * C, D), axis=0)
        return x + upd.reshape(B, S, D)
    x = A_x
    mod = (_silu(c) @ w_mod).reshape(c.shape[0], 6, 1, -1)
    sa, ca, ga, sb, cb, gb = (mod[:, 0].copy(), mod[:, 1].copy(), mod[:, 2].copy(), mod[:, 3].copy(), mod[:, 4].copy(), mod[:, 5].copy())
    h = _layernorm(x, axis=-1) * (1 + ca) + sa
    x = x + ga * _A_ref(h, A_k_cache, A_v_cache, A_wq, A_wo)
    h = _layernorm(x, axis=-1) * (1 + cb) + sb
    x = x + gb * _B_ref(h, B_w_r, B_w_gate, B_w_up, B_w_down)
    return x
```

```python
import functools

import jax
import jax.numpy as jnp
from jax import lax
import jax.experimental.pallas as pl
import jax.experimental.pallas.tpu as pltpu

f32 = jnp.float32
bf16 = jnp.bfloat16
u32 = jnp.uint32
i32 = jnp.int32

_NT = (((1,), (1,)), ((), ()))
_LOG2E = 1.4426950408889634
_EPS = 1e-5


def _rb(v):
    return v.astype(bf16).astype(f32)


def _layernorm_mod(xf, scale1p, shift):
    d = xf.shape[-1]
    mean = jnp.sum(xf, axis=-1, keepdims=True) * (1.0 / d)
    cen = xf - mean
    var = jnp.sum(cen * cen, axis=-1, keepdims=True) * (1.0 / d)
    sig = _rb(jnp.sqrt(_rb(_rb(var) + _EPS)))
    inv = 1.0 / sig
    n = _rb(_rb(xf - _rb(mean)) * inv)
    return _rb(n * scale1p) + shift


def _make_kernel(S, D, H, DH, SK, F, T0, TL, NRING, MCH):
    J0 = S // T0
    JL = S // TL
    qscale = DH ** -0.5 * _LOG2E
    n_mch = D // MCH
    MC = (4 * D) // H
    FC = 512

    def kernel(x_hbm, k_hbm, v_hbm, wq_hbm, wo_hbm, wr_hbm, wg_hbm, wu_hbm, wd_hbm,
               c_hbm, wmod_hbm, out_hbm,
               x_buf, h_buf, acc, x1_buf, h2_buf, s_buf, m_buf,
               kb, vb, wqb, wob, wmb, wm0, c_buf, wr_buf, cb_buf, mod0, modr,
               wg, wu, wd, o_buf, r_buf, fix,
               sem_small, sem_wm0, sem_x, sem_k, sem_v, sem_wq, sem_wo, sem_wm,
               sem_ffn, sem_out, sem_fix):

        def cp_c():
            return pltpu.make_async_copy(c_hbm, c_buf, sem_small.at[0])

        def cp_wr():
            return pltpu.make_async_copy(wr_hbm, wr_buf, sem_small.at[1])

        def cp_wm0(i):
            return pltpu.make_async_copy(
                wmod_hbm.at[pl.ds(i * MCH, MCH), pl.ds(0, 2 * D)],
                wm0.at[pl.ds(i * MCH, MCH), :], sem_wm0.at[i])

        def cp_x(j):
            r0 = j * T0
            if not isinstance(j, int):
                r0 = pl.multiple_of(r0, T0)
            return pltpu.make_async_copy(
                x_hbm.at[pl.ds(r0, T0), :], x_buf.at[pl.ds(r0, T0), :], sem_x.at[j])

        def _mul(a, n):
            v = a * n
            return v if isinstance(a, int) else pl.multiple_of(v, n)

        def cp_k(h):
            s = h % NRING
            return pltpu.make_async_copy(k_hbm.at[h], kb.at[s], sem_k.at[s])

        def cp_v(h):
            s = h % NRING
            return pltpu.make_async_copy(v_hbm.at[h], vb.at[s], sem_v.at[s])

        def cp_wq(h):
            s = h % NRING
            return pltpu.make_async_copy(
                wq_hbm.at[:, pl.ds(_mul(h, DH), DH)], wqb.at[s], sem_wq.at[s])

        def cp_wo(h):
            s = h % NRING
            return pltpu.make_async_copy(
                wo_hbm.at[pl.ds(_mul(h, DH), DH), :], wob.at[s], sem_wo.at[s])

        def cp_wm(h):
            s = h % NRING
            return pltpu.make_async_copy(
                wmod_hbm.at[:, pl.ds(_mul(h + (2 * D) // MC, MC), MC)], wmb.at[s],
                sem_wm.at[s])

        def cp_ffn(i):
            src, dst = ((wg_hbm, wg), (wu_hbm, wu), (wd_hbm, wd))[i]
            return pltpu.make_async_copy(src, dst, sem_ffn.at[i])

        def cp_out(j):
            r0 = _mul(j, TL)
            return pltpu.make_async_copy(
                o_buf.at[pl.ds(r0, TL), :], out_hbm.at[pl.ds(r0, TL), :], sem_out.at[j])

        def ln1(j):
            r0 = _mul(j, T0)
            xf = x_buf[pl.ds(r0, T0), :].astype(f32)
            hv = _layernorm_mod(xf, mod0[:, D:2 * D], mod0[:, 0:D])
            h_buf[pl.ds(_mul(j, T0 // 2), T0 // 2), :] = pltpu.bitcast(hv.astype(bf16), u32)
            acc[pl.ds(r0, T0), :] = jnp.zeros((T0, D), f32)

        def qproj(h, j, t):
            hh = pltpu.bitcast(h_buf[pl.ds(_mul(j, t // 2), t // 2), :], bf16)
            q = jnp.dot(hh, wqb[h % NRING], preferred_element_type=f32)
            return (q * qscale).astype(bf16)

        def scores(h, j, t, q):
            rows = pl.ds(_mul(j, t), t)
            s_buf[rows, :] = lax.dot_general(q, kb[h % NRING], _NT, preferred_element_type=f32)
            m = jnp.max(s_buf[rows, :], axis=-1, keepdims=True)
            m_buf[rows, :] = jnp.broadcast_to(m, (t, 128))

        def pv(h, j, t):
            rows = pl.ds(_mul(j, t), t)
            m = m_buf[rows, :]
            p = jnp.exp2(s_buf[rows, :] - jnp.tile(m, (1, SK // 128)))
            lp = p[:, 0:128]
            for c in range(1, SK // 128):
                lp = lp + p[:, c * 128:(c + 1) * 128]
            o = jnp.dot(p.astype(bf16), vb[h % NRING], preferred_element_type=f32)
            return o, lp

        def oproj(h, o, lp):
            l = jnp.sum(lp, axis=-1, keepdims=True)
            r = pl.reciprocal(l, approx=True)
            r = r * (2.0 - l * r)
            on = (o * r).astype(bf16)
            return jnp.dot(on, wob[h % NRING], preferred_element_type=f32)

        def mod_chunk(h):
            w = wmb[h % NRING].astype(f32)
            part = (w * cb_buf[...]).reshape(D // 8, 8, MC).sum(axis=0)
            modr[h] = _rb(jnp.sum(part, axis=0, keepdims=True))

        def mod_vec(i):
            n = D // MC
            return jnp.concatenate([modr[i * n + t] for t in range(n)], axis=-1)

        def epilogue(j, attn):
            rows = pl.ds(_mul(j, TL), TL)
            ga, sb, cb, gb = (mod_vec(i) for i in range(4))
            x1 = _rb(x_buf[rows, :].astype(f32) + _rb(ga * _rb(attn)))
            x1_buf[rows, :] = x1
            h2 = _rb(_layernorm_mod(x1, _rb(1.0 + cb), sb))
            h2_buf[rows, :] = h2
            wr = wr_buf[...].astype(f32)
            r_buf[rows, :] = _rb(jnp.sum(h2 * wr, axis=-1, keepdims=True))
            o_buf[rows, :] = (x1 + _rb(gb * h2)).astype(bf16)

        cp_c().start()
        cp_x(0).start()
        for i in range(n_mch):
            cp_wm0(i).start()
        cp_wq(0).start()
        cp_k(0).start()
        for j in range(1, J0):
            cp_x(j).start()
        cp_wq(1).start()
        cp_v(0).start()
        cp_wm(0).start()
        cp_k(1).start()
        cp_wo(0).start()
        cp_wr().start()

        cp_c().wait()
        cf = c_buf[...].astype(f32)
        sc = _rb(cf * jax.nn.sigmoid(cf))
        cb_buf[...] = jnp.transpose(jnp.broadcast_to(sc, (128, D)))

        part = jnp.zeros((8, 2 * D), f32)
        for i in range(n_mch):
            cp_wm0(i).wait()
            w = wm0[i * MCH:(i + 1) * MCH, :].astype(f32)
            cc = jnp.tile(cb_buf[i * MCH:(i + 1) * MCH, :], (1, (2 * D) // 128))
            part = part + (w * cc).reshape(MCH // 8, 8, 2 * D).sum(axis=0)
        m0 = _rb(jnp.sum(part, axis=0, keepdims=True))
        mod0[:, 0:D] = m0[:, 0:D]
        mod0[:, D:2 * D] = _rb(1.0 + m0[:, D:2 * D])

        cp_x(0).wait()
        ln1(0)
        cp_wq(0).wait()
        cp_k(0).wait()

        def p0_body(j, carry):
            @pl.when(j + 1 < J0)
            def _():
                cp_x(j + 1).wait()
            q = qproj(0, j, T0)
            scores(0, j, T0, q)
            ln1(jnp.minimum(j + 1, J0 - 1))
            return carry
        lax.fori_loop(0, J0, p0_body, 0)

        cp_v(1).start()
        cp_wo(1).start()
        cp_wm(1).start()
        for i in range(3):
            cp_ffn(i).start()

        def wait_head(h):
            cp_wq(h + 1).wait()
            cp_k(h + 1).wait()
            cp_v(h).wait()
            cp_wo(h).wait()
            cp_wm(h).wait()

        def main_body(h, carry):
            wait_head(h)
            cp_wq(h + 2).start()
            cp_k(h + 2).start()
            cp_v(h + 2).start()
            cp_wo(h + 2).start()
            cp_wm(h + 2).start()
            q = qproj(h + 1, 0, S)
            o, lp = pv(h, 0, S)
            scores(h + 1, 0, S, q)
            acc[...] += oproj(h, o, lp)
            mod_chunk(h)
            return carry
        lax.fori_loop(0, H - 2, main_body, 0)

        ha, hb = H - 2, H - 1
        wait_head(ha)
        cp_v(hb).wait()
        cp_wo(hb).wait()
        cp_wm(hb).wait()
        cp_wr().wait()

        def x_step(j, q):
            rows = pl.ds(_mul(j, TL), TL)
            o, lp = pv(ha, j, TL)
            scores(hb, j, TL, q)
            acc[rows, :] += oproj(ha, o, lp)

        def y_step(j):
            rows = pl.ds(_mul(j, TL), TL)
            o, lp = pv(hb, j, TL)
            epilogue(j, acc[rows, :] + oproj(hb, o, lp))

        mod_chunk(ha)
        mod_chunk(hb)
        x_step(0, qproj(hb, 0, TL))

        def pl_body(j, carry):
            q = qproj(hb, j, TL)
            y_step(j - 1)
            x_step(j, q)
            cp_out(j - 1).start()
            return carry
        lax.fori_loop(1, JL, pl_body, 0)
        y_step(JL - 1)
        cp_out(JL - 1).start()

        r = r_buf[...]
        row = lax.broadcasted_iota(i32, (S, 1), 0)
        r1 = jnp.max(r, axis=0, keepdims=True)
        i1 = jnp.min(jnp.where(r == r1, row, S), axis=0, keepdims=True)
        rm = jnp.where(row == i1, -jnp.inf, r)
        r2 = jnp.max(rm, axis=0, keepdims=True)
        i2 = jnp.min(jnp.where((rm == r2) & (row != i1), row, S), axis=0, keepdims=True)
        i1s = jnp.minimum(i1[0, 0], S - 1)
        i2s = jnp.minimum(i2[0, 0], S - 1)

        sub = lax.broadcasted_iota(i32, (16, D), 0)
        xa = h2_buf[pl.ds(i1s, 1), :]
        xb = h2_buf[pl.ds(i2s, 1), :]
        xs = jnp.where(sub == 0, xa, xb).astype(bf16)
        for i in range(3):
            cp_ffn(i).wait()
        y = jnp.zeros((16, D), f32)
        for c in range(F // FC):
            cs = slice(c * FC, (c + 1) * FC)
            g = _rb(jnp.dot(xs, wg[:, cs], preferred_element_type=f32))
            g = _rb(g * jax.nn.sigmoid(g))
            u = _rb(jnp.dot(xs, wu[:, cs], preferred_element_type=f32))
            y = y + jnp.dot((g * u).astype(bf16), wd[cs, :], preferred_element_type=f32)
        y = _rb(y)
        ya = _rb(y[0:1, :] * _rb(jax.nn.sigmoid(r1)))
        yb = _rb(y[1:2, :] * _rb(jax.nn.sigmoid(r2)))

        gb = mod_vec(3)
        g1 = pl.multiple_of((i1s // 16) * 16, 16)
        g2 = pl.multiple_of((i2s // 16) * 16, 16)
        for t, g0 in enumerate((g1, g2)):
            rid = sub + g0
            upd = jnp.where(rid == i1s, ya, 0.0) + jnp.where(rid == i2s, yb, 0.0)
            hb2 = _rb(h2_buf[pl.ds(g0, 16), :] + upd)
            fix[t] = (x1_buf[pl.ds(g0, 16), :] + _rb(gb * hb2)).astype(bf16)
        for j in range(JL):
            cp_out(j).wait()

        def cp_fix(t, g0):
            return pltpu.make_async_copy(fix.at[t], out_hbm.at[pl.ds(g0, 16), :], sem_fix.at[t])

        cp_fix(0, g1).start()

        @pl.when(g2 != g1)
        def _():
            cp_fix(1, g2).start()
            cp_fix(1, g2).wait()
        cp_fix(0, g1).wait()

    return kernel


def _build(A_x, A_k_cache, A_v_cache, A_wq, A_wo, B_w_r, B_w_gate, B_w_up, B_w_down, c, w_mod,
           T0=256, TL=256, NRING=4, MCH=128):
    B, S, D = A_x.shape
    _, H, SK, DH = A_k_cache.shape
    F = B_w_gate.shape[1]
    assert B == 1
    MC = (4 * D) // H
    kernel = _make_kernel(S, D, H, DH, SK, F, T0, TL, NRING, MCH)
    dma = pltpu.SemaphoreType.DMA
    scratch = [
        pltpu.VMEM((S, D), bf16),
        pltpu.VMEM((S // 2, D), u32),
        pltpu.VMEM((S, D), f32),
        pltpu.VMEM((S, D), f32),
        pltpu.VMEM((S, D), f32),
        pltpu.VMEM((S, SK), f32),
        pltpu.VMEM((S, 128), f32),
        pltpu.VMEM((NRING, SK, DH), bf16),
        pltpu.VMEM((NRING, SK, DH), bf16),
        pltpu.VMEM((NRING, D, DH), bf16),
        pltpu.VMEM((NRING, DH, D), bf16),
        pltpu.VMEM((NRING, D, MC), bf16),
        pltpu.VMEM((D, 2 * D), bf16),
        pltpu.VMEM((1, D), bf16),
        pltpu.VMEM((1, D), bf16),
        pltpu.VMEM((D, 128), f32),
        pltpu.VMEM((1, 2 * D), f32),
        pltpu.VMEM((H, 1, MC), f32),
        pltpu.VMEM((D, F), bf16),
        pltpu.VMEM((D, F), bf16),
        pltpu.VMEM((F, D), bf16),
        pltpu.VMEM((S, D), bf16),
        pltpu.VMEM((S, 1), f32),
        pltpu.VMEM((2, 16, D), bf16),
        dma((2,)), dma((D // MCH,)), dma((S // T0,)),
        dma((NRING,)), dma((NRING,)), dma((NRING,)), dma((NRING,)), dma((NRING,)),
        dma((3,)), dma((S // TL,)), dma((2,)),
    ]
    any_spec = pl.BlockSpec(memory_space=pl.ANY)
    out = pl.pallas_call(
        kernel,
        out_shape=jax.ShapeDtypeStruct((S, D), bf16),
        in_specs=[any_spec] * 11,
        out_specs=any_spec,
        scratch_shapes=scratch,
        compiler_params=pltpu.CompilerParams(vmem_limit_bytes=124 * 1024 * 1024),
    )(A_x.reshape(S, D), A_k_cache.reshape(H, SK, DH), A_v_cache.reshape(H, SK, DH),
      A_wq, A_wo, B_w_r.reshape(1, D), B_w_gate, B_w_up, B_w_down, c, w_mod)
    return out.reshape(B, S, D)


@jax.jit
def pallas_adaLN_cond__mha_block_cached__moe_arch_mod__prompt_kernel(
    A_x: jax.Array,
    A_k_cache: jax.Array,
    A_v_cache: jax.Array,
    A_wq: jax.Array,
    A_wo: jax.Array,
    B_x: jax.Array,
    B_w_r: jax.Array,
    B_w_gate: jax.Array,
    B_w_up: jax.Array,
    B_w_down: jax.Array,
    c: jax.Array,
    w_mod: jax.Array,
):
    del B_x
    return _build(A_x, A_k_cache, A_v_cache, A_wq, A_wo, B_w_r, B_w_gate, B_w_up, B_w_down,
                  c, w_mod)
```

```python
import jax
import jax.numpy as jnp
from jax import lax
import jax.experimental.pallas as pl
import jax.experimental.pallas.tpu as pltpu

f32 = jnp.float32
bf16 = jnp.bfloat16
u32 = jnp.uint32
i32 = jnp.int32

_NT = (((1,), (1,)), ((), ()))
_LOG2E = 1.4426950408889634
_EPS = 1e-5
_IMIN = -2 ** 31


def _rb(v):
    return v.astype(bf16).astype(f32)


def _layernorm_mod(xf, scale1p, shift, tok=None):
    d = xf.shape[-1]
    part = xf[:, 0:128] if tok is None else xf[:, 0:128] + _rep(tok, xf.shape[0])
    for c in range(1, d // 128):
        part = part + xf[:, c * 128:(c + 1) * 128]
    mean = jnp.sum(part, axis=-1, keepdims=True) * (1.0 / d)
    cen = xf - mean
    var = jnp.sum(cen * cen, axis=-1, keepdims=True) * (1.0 / d)
    inv = 1.0 / _rb(jnp.sqrt(_rb(_rb(var) + _EPS)))
    return (cen * inv) * scale1p + shift


def _rep(v, n):
    return jnp.tile(v, (n // 8, 1))


def _zero_of(v):
    bits = pltpu.bitcast(v, u32)
    return pltpu.bitcast(lax.shift_right_logical(lax.shift_right_logical(bits, jnp.uint32(31)),
                                                 jnp.uint32(1)), f32)


def _lane_fold(op, v):
    out = v[:, 0:128]
    for c in range(1, v.shape[1] // 128):
        out = op(out, v[:, c * 128:(c + 1) * 128])
    return out


def _interleave(rounds, chunks, counts):
    assert len(counts) == len(rounds) and sum(counts) == len(chunks), (counts, len(chunks))
    it = iter(chunks)
    res = None
    for rnd, n in zip(rounds, counts):
        res = rnd(res)
        for i in range(n):
            r0 = (i * res.shape[0] // n) // 8 * 8
            next(it)(_zero_of(res[r0:r0 + 8, 0:128]))


def _sem_sizes(S, D, cfg):
    n = cfg["NRING"]
    return [2, D // cfg["MCH"], S // cfg["T0"], n, n, n, n, n, 3, S // cfg["TL"], 2]


def _make_kernel(S, D, H, DH, SK, F, cfg):
    T0, TL, NRING, MCH = cfg["T0"], cfg["TL"], cfg["NRING"], cfg["MCH"]
    R0, RL = cfg["R0"], cfg["RL"]
    J0 = S // T0
    JL = S // TL
    qscale = DH ** -0.5 * _LOG2E
    n_mch = D // MCH
    MC = (4 * D) // H
    FC = 512
    W = 512
    NFF = 16
    assert NRING & (NRING - 1) == 0 and TL // 8 <= 128

    def kernel(x_hbm, k_hbm, v_hbm, wq_hbm, wo_hbm, wr_hbm, wg_hbm, wu_hbm, wd_hbm,
               c_hbm, wmod_hbm, out_hbm,
               x_buf, h_buf, acc, s_buf, m_buf, s2_buf, m2_buf, q_buf,
               kb, vb, wqb, wob, wmb, wm0, c_buf, wr_buf, cb_buf, mod0, modr, modv,
               wg, wu, wd, o_buf, key_buf, fix,
               sems):

        class _Sem:
            def __init__(self, base):
                self.base = base
                self.at = self

            def __getitem__(self, i):
                return sems.at[self.base + i]

        sizes = _sem_sizes(S, D, cfg)
        offs = [sum(sizes[:i]) for i in range(len(sizes))]
        (sem_small, sem_wm0, sem_x, sem_k, sem_v, sem_wq, sem_wo, sem_wm,
         sem_ffn, sem_out, sem_fix) = (_Sem(o) for o in offs)

        def _mul(a, n):
            v = a * n
            return v if isinstance(a, int) else pl.multiple_of(v, n)

        def _rows(j, t, off=0, n=None, half=False):
            n = t if n is None else n
            if half:
                t, off, n = t // 2, off // 2, n // 2
            if isinstance(j, int):
                return pl.ds(j * t + off, n)
            return pl.ds(pl.multiple_of(j * t + off, 8), n)

        def slot(h):
            return h & (NRING - 1)

        def cp_c():
            return pltpu.make_async_copy(c_hbm, c_buf, sem_small.at[0])

        def cp_wr():
            return pltpu.make_async_copy(wr_hbm, wr_buf, sem_small.at[1])

        def cp_wm0(i):
            return pltpu.make_async_copy(
                wmod_hbm.at[pl.ds(i * MCH, MCH), pl.ds(0, 2 * D)],
                wm0.at[pl.ds(i * MCH, MCH), :], sem_wm0.at[i])

        def cp_x(j):
            rows = pl.ds(_mul(j, T0), T0)
            return pltpu.make_async_copy(x_hbm.at[rows, :], x_buf.at[rows, :], sem_x.at[j])

        def cp_k(h):
            return pltpu.make_async_copy(k_hbm.at[h], kb.at[slot(h)], sem_k.at[slot(h)])

        def cp_v(h):
            return pltpu.make_async_copy(v_hbm.at[h], vb.at[slot(h)], sem_v.at[slot(h)])

        def cp_wq(h):
            return pltpu.make_async_copy(
                wq_hbm.at[:, pl.ds(_mul(h, DH), DH)], wqb.at[slot(h)], sem_wq.at[slot(h)])

        def cp_wo(h):
            return pltpu.make_async_copy(
                wo_hbm.at[pl.ds(_mul(h, DH), DH), :], wob.at[slot(h)], sem_wo.at[slot(h)])

        def cp_wm(h):
            return pltpu.make_async_copy(
                wmod_hbm.at[:, pl.ds(_mul(h + (2 * D) // MC, MC), MC)], wmb.at[slot(h)],
                sem_wm.at[slot(h)])

        ffn = ((wg_hbm, wg), (wu_hbm, wu), (wd_hbm, wd))

        def cp_ffn_piece(i, p):
            src, dst = ffn[i]
            n = src.shape[0] // NFF
            rows = pl.ds(_mul(p, n), n)
            return pltpu.make_async_copy(src.at[rows, :], dst.at[rows, :], sem_ffn.at[i])

        def wait_ffn(i):
            src, dst = ffn[i]
            pltpu.make_async_copy(src, dst, sem_ffn.at[i]).wait()

        def cp_out(j):
            rows = pl.ds(_mul(j, TL), TL)
            return pltpu.make_async_copy(o_buf.at[rows, :], out_hbm.at[rows, :], sem_out.at[j])

        def ln1_chunk(j, off, n, tok=None):
            xf = x_buf[_rows(j, T0, off, n), :].astype(f32)
            hv = _layernorm_mod(xf, _rep(mod0[:, D:2 * D], n), _rep(mod0[:, 0:D], n), tok)
            h_buf[_rows(j, T0, off, n, half=True), :] = pltpu.bitcast(hv.astype(bf16), u32)

        def qproj_rounds(h, j, t, out):
            st = {}

            def rnd(c):
                def f(prev=None):
                    hh = pltpu.bitcast(h_buf[_rows(j, t, half=True), c * W:(c + 1) * W], bf16)
                    part = jnp.dot(hh, wqb[slot(h), c * W:(c + 1) * W, :],
                                   preferred_element_type=f32)
                    st["q"] = part if c == 0 else st["q"] + part
                    if c == D // W - 1:
                        out((st["q"] * qscale).astype(bf16))
                    return part
                return f
            return [rnd(c) for c in range(D // W)]

        def score_rounds(h, j, t, get_q, s_buf=s_buf, m_buf=m_buf):
            st = {}

            def rnd(c):
                def f(prev=None):
                    if c == 0:
                        st["q"] = get_q()
                    s = lax.dot_general(st["q"], kb[slot(h), c * W:(c + 1) * W, :], _NT,
                                        preferred_element_type=f32)
                    s_buf[_rows(j, t), c * W:(c + 1) * W] = s
                    mp = _lane_fold(jnp.maximum, s)
                    st["m"] = mp if c == 0 else jnp.maximum(st["m"], mp)
                    if c == SK // W - 1:
                        m = jnp.max(st["m"], axis=-1, keepdims=True)
                        m_buf[_rows(j, t), :] = jnp.broadcast_to(m, (t, 128))
                    return s
                return f
            return [rnd(c) for c in range(SK // W)]

        def pv_rounds(h, j, t, out, s_buf=s_buf, m_buf=m_buf):
            bs = cfg["PB"] if t == S else cfg["PBL"]
            nb = t // bs
            st = {"l": [None] * nb, "hist": []}

            def rnd(c):
                def f(prev=None):
                    ps = []
                    for b in range(nb):
                        rows = _rows(j, t, b * bs, bs)
                        m = m_buf[rows, :]
                        if len(st["hist"]) >= cfg["PD"]:
                            m = m + _zero_of(st["hist"][-cfg["PD"]])
                        p = jnp.exp2(s_buf[rows, c * W:(c + 1) * W] - jnp.tile(m, (1, W // 128)))
                        lp = _lane_fold(jnp.add, p)
                        st["l"][b] = lp if c == 0 else st["l"][b] + lp
                        st["hist"].append(st["l"][b])
                        ps.append(p.astype(bf16))
                    pb = ps[0] if nb == 1 else jnp.concatenate(ps, axis=0)
                    o = jnp.dot(pb, vb[slot(h), c * W:(c + 1) * W, :], preferred_element_type=f32)
                    st["o"] = o if c == 0 else st["o"] + o
                    if c == SK // W - 1:
                        lf = st["l"][0] if nb == 1 else jnp.concatenate(st["l"], axis=0)
                        l = jnp.sum(lf, axis=-1, keepdims=True)
                        r = pl.reciprocal(l, approx=True)
                        r = r * (2.0 - l * r)
                        out((st["o"] * r).astype(bf16))
                    return o
                return f
            return [rnd(c) for c in range(SK // W)]

        def oproj_rounds(h, j, t, get_o):
            def rnd(c):
                def f(prev=None):
                    cs = slice(c * W, (c + 1) * W)
                    d = jnp.dot(get_o(), wob[slot(h), :, cs], preferred_element_type=f32)
                    old = acc[_rows(j, t), cs]
                    if not isinstance(h, int):
                        old = jnp.where(h > 0, old, 0.0)
                    acc[_rows(j, t), cs] = old + d
                    return d
                return f
            return [rnd(c) for c in range(D // W)]

        def mod_chunk(h):
            w = wmb[slot(h)].astype(f32)
            part = (w * cb_buf[...]).reshape(D // 8, 8, MC).sum(axis=0)
            modr[h] = _rb(jnp.sum(part, axis=0, keepdims=True))

        def epi_chunks(j, n):
            st = {}
            lane = lax.broadcasted_iota(i32, (8, 128), 1)
            sub = lax.broadcasted_iota(i32, (8, 128), 0)

            def chunk(off):
                def f(tok=None):
                    rows = _rows(j, TL, off, n)
                    ga, sb, cb1, gb, wr = (modv[i] for i in range(5))
                    if tok is not None:
                        ga = ga + jnp.tile(tok, (1, D // 128))
                    ga, sb, cb1, gb, wr = (_rep(v, n) for v in (ga, sb, cb1, gb, wr))
                    x1 = x_buf[rows, :].astype(f32) + ga * acc[rows, :]
                    h2 = _layernorm_mod(x1, cb1, sb)
                    o_buf[rows, :] = (x1 + gb * h2).astype(bf16)
                    r = jnp.sum(h2 * wr, axis=-1, keepdims=True)
                    rv = st["r"] if off else jnp.zeros((8, 128), f32)
                    for g in range(n // 8):
                        rv = jnp.where(lane == off // 8 + g, r[g * 8:(g + 1) * 8, :], rv)
                    st["r"] = rv
                    if off + n == TL:
                        bits = pltpu.bitcast(_rb(rv) + 0.0, i32)
                        mono = jnp.where(bits < 0, bits ^ 0x7FFF0000, bits)
                        row = j * TL + lane * 8 + sub
                        key_buf[j] = jnp.where(lane < TL // 8, mono | (0xFFFF - row), _IMIN)
                return f
            return [chunk(off) for off in range(0, TL, n)]

        cp_c().start()
        cp_x(0).start()
        for i in range(n_mch):
            cp_wm0(i).start()
        cp_wq(0).start()
        cp_k(0).start()
        for j in range(1, J0):
            cp_x(j).start()
        cp_wq(1).start()
        cp_v(0).start()
        cp_wm(0).start()
        cp_k(1).start()
        cp_wo(0).start()
        cp_wr().start()

        cp_c().wait()
        cf = c_buf[...].astype(f32)
        sc = _rb(cf * jax.nn.sigmoid(cf))
        cb_buf[...] = jnp.transpose(jnp.broadcast_to(sc, (128, D)))

        part = None
        for i in range(n_mch):
            cp_wm0(i).wait()
            scb = jnp.broadcast_to(sc[:, i * MCH:(i + 1) * MCH], (16, MCH)).astype(bf16)
            d = jnp.dot(scb, wm0[i * MCH:(i + 1) * MCH, :], preferred_element_type=f32)
            part = d if part is None else part + d
        m0 = _rb(part[0:8, :])
        mod0[:, 0:D] = m0[:, 0:D]
        mod0[:, D:2 * D] = _rb(1.0 + m0[:, D:2 * D])

        def put_q(q):
            q_buf[...] = pltpu.bitcast(q, u32)

        def get_q():
            return pltpu.bitcast(q_buf[...], bf16)

        cp_x(0).wait()
        cp_wq(0).wait()
        for off in range(0, T0, R0):
            ln1_chunk(0, off, R0)
        for rnd in qproj_rounds(0, 0, T0, put_q):
            rnd()
        cp_k(0).wait()

        def p0_body(j, carry):
            cp_x(j + 1).wait()
            chunks = [(lambda tok, off=off: ln1_chunk(j + 1, off, R0, tok)) for off in range(0, T0, R0)]
            n = len(chunks) // 4
            _interleave(score_rounds(0, j, T0, get_q) + qproj_rounds(0, j + 1, T0, put_q),
                        chunks, [n, n, n, n, 0, 0])
            return carry
        lax.fori_loop(0, J0 - 1, p0_body, 0)
        cp_v(1).start()
        cp_wo(1).start()
        cp_wm(1).start()
        cp_wq(2).start()
        cp_k(2).start()
        for rnd in score_rounds(0, J0 - 1, T0, get_q):
            rnd()

        def wait_head(h):
            cp_wq(h + 1).wait()
            cp_k(h + 1).wait()
            cp_v(h).wait()
            cp_wo(h).wait()
            cp_wm(h).wait()

        def main_body(h, carry):
            st = {}
            res = None
            for rnd in qproj_rounds(h + 1, 0, S, lambda q: st.update(q=q)):
                res = rnd()
            for rnd in pv_rounds(h, 0, S, lambda o: st.update(o=o)):
                res = rnd(res)
            cp_v(h + 2).start()
            mod_chunk(h)
            cp_wm(h + 2).start()
            for rnd in score_rounds(h + 1, 0, S, lambda: st["q"]):
                rnd()
            for rnd in oproj_rounds(h, 0, S, lambda: st["o"]):
                rnd()
            cp_wo(h + 2).start()
            wait_head(h + 1)

            @pl.when(h + 3 < H)
            def _():
                cp_wq(h + 3).start()
                cp_k(h + 3).start()

            @pl.when(h < NFF)
            def _():
                for i in range(3):
                    cp_ffn_piece(i, h).start()
            return carry
        wait_head(0)
        lax.fori_loop(0, H - 2, main_body, 0)

        ha, hb = H - 2, H - 1
        cp_v(hb).wait()
        cp_wo(hb).wait()
        cp_wm(hb).wait()
        cp_wr().wait()

        def x_rounds(j, st):
            return (pv_rounds(ha, j, TL, lambda o: st.update(oa=o))
                    + score_rounds(hb, 0, TL, lambda: st["q"], s2_buf, m2_buf)
                    + oproj_rounds(ha, j, TL, lambda: st["oa"]))

        def y_rounds(j, st):
            return (pv_rounds(hb, 0, TL, lambda o: st.update(ob=o), s2_buf, m2_buf)
                    + oproj_rounds(hb, j, TL, lambda: st["ob"]))

        def finish_mod():
            n = D // MC
            for i in range(4):
                v = jnp.concatenate([modr[i * n + t] for t in range(n)], axis=-1)
                modv[i] = jnp.broadcast_to(_rb(1.0 + v) if i == 2 else v, (8, D))
            modv[4] = jnp.broadcast_to(wr_buf[...].astype(f32), (8, D))

        st0 = {}
        _interleave(qproj_rounds(hb, 0, TL, lambda q: st0.update(q=q)) + x_rounds(0, st0),
                    [lambda _: mod_chunk(ha), lambda _: mod_chunk(hb), lambda _: finish_mod()],
                    [0] * 6 + [1, 1, 1, 0, 0, 0])

        def pl_body(j, carry):
            st = {}
            chunks = epi_chunks(j - 1, RL)
            parts = dict(
                Q=qproj_rounds(hb, j, TL, lambda q: st.update(q=q)),
                B=pv_rounds(hb, 0, TL, lambda o: st.update(ob=o), s2_buf, m2_buf),
                b=oproj_rounds(hb, j - 1, TL, lambda: st["ob"]),
                A=pv_rounds(ha, j, TL, lambda o: st.update(oa=o)),
                S=score_rounds(hb, 0, TL, lambda: st["q"], s2_buf, m2_buf),
                a=oproj_rounds(ha, j, TL, lambda: st["oa"]))
            rounds = [parts[ch].pop(0) for ch in cfg["LORD"]]
            _interleave(rounds, chunks, [int(ch) for ch in cfg["LCNT"]])
            cp_out(j - 1).start()
            return carry
        lax.fori_loop(1, JL, pl_body, 0)
        res = None
        for rnd in y_rounds(JL - 1, {}):
            res = rnd(res)
        for ch in epi_chunks(JL - 1, RL):
            ch()
        cp_out(JL - 1).start()

        keys = key_buf[...].reshape(JL * 8, 128)
        k1 = jnp.max(keys, keepdims=True)
        k2 = jnp.max(jnp.where(keys == k1, _IMIN, keys), keepdims=True)

        def score_of(k):
            hi = k & jnp.int32(-65536)
            return pltpu.bitcast(jnp.where(hi < 0, hi ^ 0x7FFF0000, hi), f32)

        i1s = jnp.minimum(0xFFFF - (k1[0, 0] & 0xFFFF), S - 1)
        i2s = jnp.minimum(0xFFFF - (k2[0, 0] & 0xFFFF), S - 1)

        sub = lax.broadcasted_iota(i32, (16, D), 0)
        ga, sb, cb1, gb = (_rep(modv[i], 16) for i in range(4))
        g1 = pl.multiple_of((i1s >> 4) << 4, 16)
        g2 = pl.multiple_of((i2s >> 4) << 4, 16)
        x1s, h2s, sel = [], [], []
        for g0, idx in ((g1, i1s), (g2, i2s)):
            x1 = x_buf[pl.ds(g0, 16), :].astype(f32) + ga * acc[pl.ds(g0, 16), :]
            h2 = _layernorm_mod(x1, cb1, sb)
            x1s.append(x1)
            h2s.append(h2)
            sel.append(jnp.sum(jnp.where(sub + g0 == idx, h2, 0.0), axis=0, keepdims=True))
        xs = jnp.where(sub == 0, sel[0], sel[1]).astype(bf16)
        for i in range(3):
            wait_ffn(i)
        y = jnp.zeros((16, D), f32)
        for c in range(F // FC):
            cs = slice(c * FC, (c + 1) * FC)
            g = _rb(jnp.dot(xs, wg[:, cs], preferred_element_type=f32))
            g = _rb(g * jax.nn.sigmoid(g))
            u = _rb(jnp.dot(xs, wu[:, cs], preferred_element_type=f32))
            y = y + jnp.dot((g * u).astype(bf16), wd[cs, :], preferred_element_type=f32)
        y = _rb(y)
        ya = _rb(y[0:1, :] * _rb(jax.nn.sigmoid(score_of(k1))))
        yb = _rb(y[1:2, :] * _rb(jax.nn.sigmoid(score_of(k2))))

        for t, g0 in enumerate((g1, g2)):
            rid = sub + g0
            upd = jnp.where(rid == i1s, ya, 0.0) + jnp.where(rid == i2s, yb, 0.0)
            fix[t] = (x1s[t] + gb * (h2s[t] + upd)).astype(bf16)
        for j in range(JL):
            cp_out(j).wait()

        def cp_fix(t, g0):
            return pltpu.make_async_copy(fix.at[t], out_hbm.at[pl.ds(g0, 16), :], sem_fix.at[t])

        cp_fix(0, g1).start()

        @pl.when(g2 != g1)
        def _():
            cp_fix(1, g2).start()
            cp_fix(1, g2).wait()
        cp_fix(0, g1).wait()

    return kernel


_CFG = dict(PB=2048, PBL=256, PD=100, T0=256, TL=256, NRING=4, MCH=128, R0=32, RL=16,
            LORD='QQBBBBbbAAAASSSSaa', LCNT='000000002222222200')


def _build(A_x, A_k_cache, A_v_cache, A_wq, A_wo, B_w_r, B_w_gate, B_w_up, B_w_down, c, w_mod,
           **over):
    B, S, D = A_x.shape
    _, H, SK, DH = A_k_cache.shape
    F = B_w_gate.shape[1]
    assert B == 1
    cfg = dict(_CFG, **over)
    T0, TL, NRING, MCH = cfg["T0"], cfg["TL"], cfg["NRING"], cfg["MCH"]
    MC = (4 * D) // H
    kernel = _make_kernel(S, D, H, DH, SK, F, cfg)
    dma = pltpu.SemaphoreType.DMA
    scratch = [
        pltpu.VMEM((S, D), bf16),
        pltpu.VMEM((S // 2, D), u32),
        pltpu.VMEM((S, D), f32),
        pltpu.VMEM((S, SK), f32),
        pltpu.VMEM((S, 128), f32),
        pltpu.VMEM((TL, SK), f32),
        pltpu.VMEM((TL, 128), f32),
        pltpu.VMEM((T0 // 2, DH), u32),
        pltpu.VMEM((NRING, SK, DH), bf16),
        pltpu.VMEM((NRING, SK, DH), bf16),
        pltpu.VMEM((NRING, D, DH), bf16),
        pltpu.VMEM((NRING, DH, D), bf16),
        pltpu.VMEM((NRING, D, MC), bf16),
        pltpu.VMEM((D, 2 * D), bf16),
        pltpu.VMEM((1, D), bf16),
        pltpu.VMEM((1, D), bf16),
        pltpu.VMEM((D, 128), f32),
        pltpu.VMEM((8, 2 * D), f32),
        pltpu.VMEM((H, 1, MC), f32),
        pltpu.VMEM((5, 8, D), f32),
        pltpu.VMEM((D, F), bf16),
        pltpu.VMEM((D, F), bf16),
        pltpu.VMEM((F, D), bf16),
        pltpu.VMEM((S, D), bf16),
        pltpu.VMEM((S // TL, 8, 128), i32),
        pltpu.VMEM((2, 16, D), bf16),
        dma((sum(_sem_sizes(S, D, cfg)),)),
    ]
    any_spec = pl.BlockSpec(memory_space=pl.ANY)
    out = pl.pallas_call(
        kernel,
        out_shape=jax.ShapeDtypeStruct((S, D), bf16),
        in_specs=[any_spec] * 11,
        out_specs=any_spec,
        scratch_shapes=scratch,
        compiler_params=pltpu.CompilerParams(vmem_limit_bytes=124 * 1024 * 1024,
                                             disable_bounds_checks=True),
    )(A_x.reshape(S, D), A_k_cache.reshape(H, SK, DH), A_v_cache.reshape(H, SK, DH),
      A_wq, A_wo, B_w_r.reshape(1, D), B_w_gate, B_w_up, B_w_down, c, w_mod)
    return out.reshape(B, S, D)


@jax.jit
def pallas_adaLN_cond__mha_block_cached__moe_arch_mod__prompt_kernel(
    A_x: jax.Array,
    A_k_cache: jax.Array,
    A_v_cache: jax.Array,
    A_wq: jax.Array,
    A_wo: jax.Array,
    B_x: jax.Array,
    B_w_r: jax.Array,
    B_w_gate: jax.Array,
    B_w_up: jax.Array,
    B_w_down: jax.Array,
    c: jax.Array,
    w_mod: jax.Array,
):
    del B_x
    return _build(A_x, A_k_cache, A_v_cache, A_wq, A_wo, B_w_r, B_w_gate, B_w_up, B_w_down,
                  c, w_mod)
```

```python
import jax
import jax.numpy as jnp
from jax import lax
import jax.experimental.pallas as pl
import jax.experimental.pallas.tpu as pltpu

f32 = jnp.float32
bf16 = jnp.bfloat16
u32 = jnp.uint32
i32 = jnp.int32

_NT = (((1,), (1,)), ((), ()))
_LOG2E = 1.4426950408889634
_EPS = 1e-5
_IMIN = -2 ** 31


def _rb(v):
    return v.astype(bf16).astype(f32)


def _rep(v, n):
    return v if n == 8 else jnp.tile(v, (n // 8, 1))


def _wide(v, w):
    return jnp.tile(v, (1, w // 128))


def _zero_of(v):
    bits = pltpu.bitcast(v, u32)
    return pltpu.bitcast(lax.shift_right_logical(lax.shift_right_logical(bits, jnp.uint32(31)),
                                                 jnp.uint32(1)), f32)


def _tiles(v):
    return [v[:, c * 128:(c + 1) * 128] for c in range(v.shape[1] // 128)]


def _fold(op, parts):
    out = parts[0]
    for p in parts[1:]:
        out = op(out, p)
    return out


def _lane_sum(v):
    return jnp.broadcast_to(jnp.sum(v, axis=-1, keepdims=True), v.shape)


def _row_stats(xf, tok=None):
    d = xf.shape[-1]
    ts = _tiles(xf)
    nt = len(ts)
    if tok is not None:
        ts = [ts[0] + tok] + ts[1:]
    mu = _fold(jnp.add, ts) * (1.0 / nt)
    m2 = _fold(jnp.add, [(t - mu) * (t - mu) for t in ts])
    mean = _lane_sum(mu) * (1.0 / 128)
    dm = mu - mean
    var = _lane_sum(m2 + (dm * dm) * float(nt)) * (1.0 / d)
    return mean, lax.rsqrt(var + _EPS), m2


def _sem_sizes(S, D, cfg):
    n = cfg["NRING"]
    return [2, D // cfg["MCH"], S // cfg["T0"], n, n, n, n, n, 3, S // cfg["TL"], 2]


def _make_kernel(S, D, H, DH, SK, F, cfg):
    T0, TL, NRING, MCH = cfg["T0"], cfg["TL"], cfg["NRING"], cfg["MCH"]
    R0, RL, CD0, CDL = cfg["R0"], cfg["RL"], cfg["CD0"], cfg["CDL"]
    J0 = S // T0
    JL = S // TL
    qscale = DH ** -0.5 * _LOG2E
    n_mch = D // MCH
    MC = (4 * D) // H
    FC = 512
    W = 512
    NFF = 16
    assert NRING == 4 and TL // 8 <= 128 and JL >= 3

    def kernel(x_hbm, k_hbm, v_hbm, wq_hbm, wo_hbm, wr_hbm, wg_hbm, wu_hbm, wd_hbm,
               c_hbm, wmod_hbm, out_hbm,
               x_buf, h_buf, acc, s_buf, m_buf, s2_buf, m2_buf, st_buf,
               kb, vb, wqb, wob, wmb, wm0, c_buf, wr_buf, cb_buf, mod0, modr, modv,
               wg, wu, wd, o_buf, key_buf, fix,
               sems):

        class _Sem:
            def __init__(self, base):
                self.base = base
                self.at = self

            def __getitem__(self, i):
                return sems.at[self.base + i]

        sizes = _sem_sizes(S, D, cfg)
        offs = [sum(sizes[:i]) for i in range(len(sizes))]
        (sem_small, sem_wm0, sem_x, sem_k, sem_v, sem_wq, sem_wo, sem_wm,
         sem_ffn, sem_out, sem_fix) = (_Sem(o) for o in offs)

        def _mul(a, n):
            v = a * n
            return v if isinstance(a, int) else pl.multiple_of(v, n)

        def view(ref, j, t, n=1):
            return ref.at[pl.ds(_mul(j, t), n * t), :]

        def slot(h):
            return h & (NRING - 1)

        def cp_c():
            return pltpu.make_async_copy(c_hbm, c_buf, sem_small.at[0])

        def cp_wr():
            return pltpu.make_async_copy(wr_hbm, wr_buf, sem_small.at[1])

        def cp_wm0(i):
            return pltpu.make_async_copy(
                wmod_hbm.at[pl.ds(i * MCH, MCH), pl.ds(0, 2 * D)],
                wm0.at[pl.ds(i * MCH, MCH), :], sem_wm0.at[i])

        def cp_x(j):
            return pltpu.make_async_copy(view(x_hbm, j, T0), view(x_buf, j, T0), sem_x.at[j])

        def cp_k(h):
            return pltpu.make_async_copy(k_hbm.at[h], kb.at[slot(h)], sem_k.at[slot(h)])

        def cp_v(h):
            return pltpu.make_async_copy(v_hbm.at[h], vb.at[slot(h)], sem_v.at[slot(h)])

        def cp_wq(h):
            return pltpu.make_async_copy(
                wq_hbm.at[:, pl.ds(_mul(h, DH), DH)], wqb.at[slot(h)], sem_wq.at[slot(h)])

        def cp_wo(h):
            return pltpu.make_async_copy(
                wo_hbm.at[pl.ds(_mul(h, DH), DH), :], wob.at[slot(h)], sem_wo.at[slot(h)])

        def cp_wm(h):
            return pltpu.make_async_copy(
                wmod_hbm.at[:, pl.ds(_mul(h + (2 * D) // MC, MC), MC)], wmb.at[slot(h)],
                sem_wm.at[slot(h)])

        ffn = ((wg_hbm, wg), (wu_hbm, wu), (wd_hbm, wd))

        def cp_ffn_piece(i, p):
            src, dst = ffn[i]
            n = src.shape[0] // NFF
            return pltpu.make_async_copy(view(src, p, n), view(dst, p, n), sem_ffn.at[i])

        def wait_ffn(i):
            src, dst = ffn[i]
            pltpu.make_async_copy(src, dst, sem_ffn.at[i]).wait()

        def cp_out(j):
            return pltpu.make_async_copy(view(o_buf, j, TL), view(out_hbm, j, TL), sem_out.at[j])

        def ln1_stats(xv):
            hist = []
            for off in range(0, T0, R0):
                tok = _zero_of(hist[-CD0]) if len(hist) >= CD0 else None
                mean, inv, m2 = _row_stats(xv[off:off + R0, :].astype(f32), tok)
                hist.append(m2)
                st_buf[0, off:off + R0, :] = mean
                st_buf[1, off:off + R0, :] = inv

        def qproj(h, hv, xv=None):
            q = None
            for c in range(D // W):
                cs = slice(c * W, (c + 1) * W)
                if xv is None:
                    hh = pltpu.bitcast(hv[:, cs], bf16)
                else:
                    n = (xv[:, cs].astype(f32) - _wide(st_buf[0], W)) * _wide(st_buf[1], W)
                    hh = (n * _rep(mod0[:, D + c * W:D + (c + 1) * W], T0)
                          + _rep(mod0[:, cs], T0)).astype(bf16)
                    hv[:, cs] = pltpu.bitcast(hh, u32)
                part = jnp.dot(hh, wqb[slot(h), cs, :], preferred_element_type=f32)
                q = part if q is None else q + part
            return (q * qscale).astype(bf16)

        def scores(h, q, sv, mv):
            mp = None
            for c in range(SK // W):
                cs = slice(c * W, (c + 1) * W)
                s = lax.dot_general(q, kb[slot(h), cs, :], _NT, preferred_element_type=f32)
                sv[:, cs] = s
                mp = _fold(jnp.maximum, ([] if mp is None else [mp]) + _tiles(s))
            mv[...] = jnp.broadcast_to(jnp.max(mp, axis=-1, keepdims=True), mp.shape)

        def pv(h, sv, mv):
            o = lp = None
            for c in range(SK // W):
                cs = slice(c * W, (c + 1) * W)
                p = jnp.exp2(sv[:, cs] - _wide(mv[...], W))
                lp = _fold(jnp.add, ([] if lp is None else [lp]) + _tiles(p))
                d = jnp.dot(p.astype(bf16), vb[slot(h), cs, :], preferred_element_type=f32)
                o = d if o is None else o + d
            l = jnp.sum(lp, axis=-1, keepdims=True)
            r = pl.reciprocal(l, approx=True)
            r = r * (2.0 - l * r)
            return (o * r).astype(bf16)

        def oproj(h, o, av, xv=None):
            for c in range(D // W):
                cs = slice(c * W, (c + 1) * W)
                d = jnp.dot(o, wob[slot(h), :, cs], preferred_element_type=f32)
                old = av[:, cs]
                if not isinstance(h, int):
                    old = jnp.where(h > 0, old, 0.0)
                a = old + d
                if xv is not None:
                    a = xv[:, cs].astype(f32) + _rep(modv[0, :, cs], a.shape[0]) * a
                av[:, cs] = a

        def mod_chunk(h):
            w = wmb[slot(h)].astype(f32)
            part = (w * cb_buf[...]).reshape(D // 8, 8, MC).sum(axis=0)
            modr[h] = _rb(jnp.sum(part, axis=0, keepdims=True))

        def finish_mod():
            n = D // MC
            ga, sb, cb, gb = (jnp.concatenate([modr[i * n + t] for t in range(n)], axis=-1)
                              for i in range(4))
            cb1 = _rb(1.0 + cb)
            wr = wr_buf[...].astype(f32)
            a = cb1 * wr
            a0 = jnp.broadcast_to(jnp.sum(a, axis=-1, keepdims=True), (1, D))
            b0 = jnp.broadcast_to(jnp.sum(sb * wr, axis=-1, keepdims=True), (1, D))
            for i, v in enumerate((ga, sb, cb1, gb, a, gb * cb1, gb * sb, a0, b0)):
                modv[i] = jnp.broadcast_to(v, (8, D))

        def epilogue(j, x1v, ov, chain):
            lane = lax.broadcasted_iota(i32, (8, 128), 1)
            sub = lax.broadcasted_iota(i32, (8, 128), 0)
            rv = jnp.zeros((8, 128), f32)
            hist = []
            for off in range(0, TL, RL):
                tok = _zero_of(hist[-chain]) if chain and len(hist) >= chain else None
                x1 = x1v[off:off + RL, :]
                mean, inv, m2 = _row_stats(x1, tok)
                hist.append(m2)
                ra = _lane_sum(_fold(jnp.add, _tiles(x1 * _rep(modv[4], RL))))
                r = inv * (ra - mean * _rep(modv[7, :, 0:128], RL)) + _rep(modv[8, :, 0:128], RL)
                u = _wide(inv, D) * _rep(modv[5], RL)
                ov[off:off + RL, :] = (x1 + ((x1 - _wide(mean, D)) * u + _rep(modv[6], RL))).astype(bf16)
                for g in range(RL // 8):
                    rv = jnp.where(lane == off // 8 + g, r[g * 8:(g + 1) * 8, :], rv)
            bits = pltpu.bitcast(_rb(rv) + 0.0, i32)
            mono = jnp.where(bits < 0, bits ^ 0x7FFF0000, bits)
            row = j * TL + lane * 8 + sub
            key_buf[j] = jnp.where(lane < TL // 8, mono | (0xFFFF - row), _IMIN)

        cp_c().start()
        cp_x(0).start()
        for i in range(n_mch):
            cp_wm0(i).start()
        cp_wq(0).start()
        cp_k(0).start()
        for j in range(1, J0):
            cp_x(j).start()
        cp_wq(1).start()
        cp_v(0).start()
        cp_wm(0).start()
        cp_k(1).start()
        cp_wo(0).start()
        cp_wr().start()
        cp_v(1).start()
        cp_wo(1).start()
        cp_wm(1).start()
        cp_wq(2).start()
        cp_k(2).start()

        cp_c().wait()
        cf = c_buf[...].astype(f32)
        sc = _rb(cf * jax.nn.sigmoid(cf))
        cb_buf[...] = jnp.transpose(jnp.broadcast_to(sc, (128, D)))
        cp_x(0).wait()
        ln1_stats(view(x_buf, 0, T0))

        part = None
        for i in range(n_mch):
            cp_wm0(i).wait()
            scb = jnp.broadcast_to(sc[:, i * MCH:(i + 1) * MCH], (16, MCH)).astype(bf16)
            d = jnp.dot(scb, wm0[i * MCH:(i + 1) * MCH, :], preferred_element_type=f32)
            part = d if part is None else part + d
        m0 = _rb(part[0:8, :])
        mod0[:, 0:D] = m0[:, 0:D]
        mod0[:, D:2 * D] = _rb(1.0 + m0[:, D:2 * D])
        cp_wq(0).wait()
        cp_k(0).wait()

        def p0_body(j, carry):
            @pl.when(j + 1 < J0)
            def _():
                cp_x(j + 1).wait()
            q = qproj(0, view(h_buf, j, T0 // 2), view(x_buf, j, T0))
            scores(0, q, view(s_buf, j, T0), view(m_buf, j, T0))
            ln1_stats(view(x_buf, jnp.minimum(j + 1, J0 - 1), T0))
            return carry
        lax.fori_loop(0, J0, p0_body, 0)

        def wait_head(h):
            cp_wq(h + 1).wait()
            cp_k(h + 1).wait()
            cp_v(h).wait()
            cp_wo(h).wait()
            cp_wm(h).wait()

        def main_body(h, carry):
            q = qproj(h + 1, h_buf)
            o = pv(h, s_buf, m_buf)
            cp_v(h + 2).start()
            mod_chunk(h)
            scores(h + 1, q, s_buf, m_buf)
            oproj(h, o, acc)
            cp_wm(h + 2).start()
            cp_wo(h + 2).start()

            @pl.when(h + 3 < H)
            def _():
                cp_wq(h + 3).start()
                cp_k(h + 3).start()

            @pl.when(h < NFF)
            def _():
                for i in range(3):
                    cp_ffn_piece(i, h).start()
            wait_head(h + 1)
            return carry
        wait_head(0)
        lax.fori_loop(0, H - 2, main_body, 0)

        ha, hb = H - 2, H - 1
        cp_v(hb).wait()
        cp_wo(hb).wait()
        cp_wm(hb).wait()
        cp_wr().wait()

        def l_step(j, do_x, do_y, do_e, chain=CDL):
            first = j - 2 if do_e else (j - 1 if do_y else j)
            last = j if do_x else (j - 1 if do_y else j - 2)
            n = (2 if do_e else (1 if do_y else 0)) - (0 if do_x else (1 if do_y else 2)) + 1
            aw = view(acc, first, TL, n)

            def tile(k):
                o = ((2 if do_e else (1 if do_y else 0)) - k) * TL
                return aw.at[o:o + TL, :]
            del last
            if do_e:
                epilogue(j - 2, tile(2), view(o_buf, j - 2, TL), chain)
            if do_x:
                q = qproj(hb, view(h_buf, j, TL // 2))
            if do_y:
                ob = pv(hb, s2_buf, m2_buf)
                oproj(hb, ob, tile(1), view(x_buf, j - 1, TL))
            if do_x:
                oa = pv(ha, view(s_buf, j, TL), view(m_buf, j, TL))
                scores(hb, q, s2_buf, m2_buf)
                oproj(ha, oa, tile(0))
            if do_e:
                cp_out(j - 2).start()

        mod_chunk(ha)
        mod_chunk(hb)
        finish_mod()
        l_step(0, True, False, False)
        for i in range(3):
            wait_ffn(i)
        l_step(1, True, True, False)

        def pl_body(j, carry):
            l_step(j, True, True, True)
            return carry
        lax.fori_loop(2, JL, pl_body, 0)
        l_step(JL, False, True, True)
        for j in range(JL - 2):
            cp_out(j).wait()
        l_step(JL + 1, False, False, True, chain=0)

        keys = key_buf[...].reshape(JL * 8, 128)
        k1 = jnp.max(keys, keepdims=True)
        k2 = jnp.max(jnp.where(keys == k1, _IMIN, keys), keepdims=True)

        def score_of(k):
            hi = k & jnp.int32(-65536)
            return pltpu.bitcast(jnp.where(hi < 0, hi ^ 0x7FFF0000, hi), f32)

        i1s = jnp.minimum(0xFFFF - (k1[0, 0] & 0xFFFF), S - 1)
        i2s = jnp.minimum(0xFFFF - (k2[0, 0] & 0xFFFF), S - 1)

        sub = lax.broadcasted_iota(i32, (16, D), 0)
        sb, cb1, gb = (_rep(modv[i], 16) for i in (1, 2, 3))

        def adaln2(x1):
            mean, inv, _ = _row_stats(x1)
            return (x1 - _wide(mean, D)) * _wide(inv, D) * cb1 + sb

        xs = adaln2(jnp.where(sub == 0, acc[pl.ds(i1s, 1), :], acc[pl.ds(i2s, 1), :])).astype(bf16)
        y = jnp.zeros((16, D), f32)
        for c in range(F // FC):
            cs = slice(c * FC, (c + 1) * FC)
            g = _rb(jnp.dot(xs, wg[:, cs], preferred_element_type=f32))
            g = _rb(g * jax.nn.sigmoid(g))
            u = _rb(jnp.dot(xs, wu[:, cs], preferred_element_type=f32))
            y = y + jnp.dot((g * u).astype(bf16), wd[cs, :], preferred_element_type=f32)
        y = _rb(y)
        ya = _rb(y[0:1, :] * _rb(jax.nn.sigmoid(score_of(k1))))
        yb = _rb(y[1:2, :] * _rb(jax.nn.sigmoid(score_of(k2))))

        g1 = pl.multiple_of((i1s >> 4) << 4, 16)
        g2 = pl.multiple_of((i2s >> 4) << 4, 16)
        for t, g0 in enumerate((g1, g2)):
            rid = sub + g0
            x1 = acc[pl.ds(g0, 16), :]
            upd = jnp.where(rid == i1s, ya, 0.0) + jnp.where(rid == i2s, yb, 0.0)
            fix[t] = (x1 + gb * (adaln2(x1) + upd)).astype(bf16)

        for j in range(JL - 2, JL):
            cp_out(j).wait()

        def cp_fix(t, g0):
            return pltpu.make_async_copy(fix.at[t], out_hbm.at[pl.ds(g0, 16), :], sem_fix.at[t])

        cp_fix(0, g1).start()

        @pl.when(g2 != g1)
        def _():
            cp_fix(1, g2).start()
            cp_fix(1, g2).wait()
        cp_fix(0, g1).wait()

    return kernel


_CFG = dict(T0=256, TL=256, NRING=4, MCH=128, R0=16, RL=8, CD0=2, CDL=2)


def _build(A_x, A_k_cache, A_v_cache, A_wq, A_wo, B_w_r, B_w_gate, B_w_up, B_w_down, c, w_mod,
           **over):
    B, S, D = A_x.shape
    _, H, SK, DH = A_k_cache.shape
    F = B_w_gate.shape[1]
    assert B == 1
    cfg = dict(_CFG, **over)
    T0, TL, NRING = cfg["T0"], cfg["TL"], cfg["NRING"]
    MC = (4 * D) // H
    kernel = _make_kernel(S, D, H, DH, SK, F, cfg)
    scratch = [
        pltpu.VMEM((S, D), bf16),
        pltpu.VMEM((S // 2, D), u32),
        pltpu.VMEM((S, D), f32),
        pltpu.VMEM((S, SK), f32),
        pltpu.VMEM((S, 128), f32),
        pltpu.VMEM((TL, SK), f32),
        pltpu.VMEM((TL, 128), f32),
        pltpu.VMEM((2, T0, 128), f32),
        pltpu.VMEM((NRING, SK, DH), bf16),
        pltpu.VMEM((NRING, SK, DH), bf16),
        pltpu.VMEM((NRING, D, DH), bf16),
        pltpu.VMEM((NRING, DH, D), bf16),
        pltpu.VMEM((NRING, D, MC), bf16),
        pltpu.VMEM((D, 2 * D), bf16),
        pltpu.VMEM((1, D), bf16),
        pltpu.VMEM((1, D), bf16),
        pltpu.VMEM((D, 128), f32),
        pltpu.VMEM((8, 2 * D), f32),
        pltpu.VMEM((H, 1, MC), f32),
        pltpu.VMEM((9, 8, D), f32),
        pltpu.VMEM((D, F), bf16),
        pltpu.VMEM((D, F), bf16),
        pltpu.VMEM((F, D), bf16),
        pltpu.VMEM((S, D), bf16),
        pltpu.VMEM((S // TL, 8, 128), i32),
        pltpu.VMEM((2, 16, D), bf16),
        pltpu.SemaphoreType.DMA((sum(_sem_sizes(S, D, cfg)),)),
    ]
    any_spec = pl.BlockSpec(memory_space=pl.ANY)
    out = pl.pallas_call(
        kernel,
        out_shape=jax.ShapeDtypeStruct((S, D), bf16),
        in_specs=[any_spec] * 11,
        out_specs=any_spec,
        scratch_shapes=scratch,
        compiler_params=pltpu.CompilerParams(vmem_limit_bytes=124 * 1024 * 1024,
                                             disable_bounds_checks=True),
    )(A_x.reshape(S, D), A_k_cache.reshape(H, SK, DH), A_v_cache.reshape(H, SK, DH),
      A_wq, A_wo, B_w_r.reshape(1, D), B_w_gate, B_w_up, B_w_down, c, w_mod)
    return out.reshape(B, S, D)


@jax.jit
def pallas_adaLN_cond__mha_block_cached__moe_arch_mod__prompt_kernel(
    A_x: jax.Array,
    A_k_cache: jax.Array,
    A_v_cache: jax.Array,
    A_wq: jax.Array,
    A_wo: jax.Array,
    B_x: jax.Array,
    B_w_r: jax.Array,
    B_w_gate: jax.Array,
    B_w_up: jax.Array,
    B_w_down: jax.Array,
    c: jax.Array,
    w_mod: jax.Array,
):
    del B_x
    return _build(A_x, A_k_cache, A_v_cache, A_wq, A_wo, B_w_r, B_w_gate, B_w_up, B_w_down,
                  c, w_mod)
```

```python
import jax
import jax.numpy as jnp
from jax import lax
import jax.experimental.pallas as pl
import jax.experimental.pallas.tpu as pltpu

f32 = jnp.float32
bf16 = jnp.bfloat16
u32 = jnp.uint32
i32 = jnp.int32

_NT = (((1,), (1,)), ((), ()))
_LOG2E = 1.4426950408889634
_EPS = 1e-5
_IMIN = -2 ** 31


def _rb(v):
    return v.astype(bf16).astype(f32)


def _rep(v, n):
    return v if n == 8 else jnp.tile(v, (n // 8, 1))


def _wide(v, w):
    return jnp.tile(v, (1, w // 128))


def _zero_of(v):
    bits = pltpu.bitcast(v, u32)
    return pltpu.bitcast(lax.shift_right_logical(lax.shift_right_logical(bits, jnp.uint32(31)),
                                                 jnp.uint32(1)), f32)


def _zero_bits(v):
    bits = pltpu.bitcast(v, u32)
    return lax.shift_right_logical(lax.shift_right_logical(bits, jnp.uint32(31)), jnp.uint32(1))


class _Pace:
    def __init__(self, chunks, counts, lag):
        self.chunks, self.counts, self.lag = list(chunks), list(counts), lag
        self.r = 0
        self.due = {}

    def gate(self, lhs):
        items = self.due.pop(self.r, [])
        if not items:
            return lhs
        u = pltpu.bitcast(lhs, u32)
        first = u[:, 0:128]
        parts, pos = [], 0
        for frac, tok in items:
            g = max(int(frac * u.shape[0]) // 8 * 8, pos)
            if g > pos:
                parts.append(first[pos:g])
            parts.append(first[g:g + 8] | tok)
            pos = g + 8
        if pos < u.shape[0]:
            parts.append(first[pos:])
        first = jnp.concatenate(parts, axis=0)
        if u.shape[1] > 128:
            first = jnp.concatenate([first, u[:, 128:]], axis=1)
        return pltpu.bitcast(first, bf16)

    def done(self, res):
        n = self.counts[self.r]
        for i in range(n):
            r0 = (i * res.shape[0] // n) // 8 * 8
            end = self.chunks.pop(0)(_zero_of(res[r0:r0 + 8, 0:128]))
            t = self.r + i / n + self.lag
            self.due.setdefault(int(t), []).append((t - int(t), _zero_bits(end)))
        self.r += 1


def _tiles(v):
    return [v[:, c * 128:(c + 1) * 128] for c in range(v.shape[1] // 128)]


def _fold(op, parts):
    out = parts[0]
    for p in parts[1:]:
        out = op(out, p)
    return out


def _lane_sum(v):
    return jnp.broadcast_to(jnp.sum(v, axis=-1, keepdims=True), v.shape)


def _row_stats(xf, tok=None):
    d = xf.shape[-1]
    ts = _tiles(xf)
    nt = len(ts)
    if tok is not None:
        ts = [ts[0] + tok] + ts[1:]
    mu = _fold(jnp.add, ts) * (1.0 / nt)
    m2 = _fold(jnp.add, [(t - mu) * (t - mu) for t in ts])
    mean = _lane_sum(mu) * (1.0 / 128)
    dm = mu - mean
    var = _lane_sum(m2 + (dm * dm) * float(nt)) * (1.0 / d)
    return mean, lax.rsqrt(var + _EPS), m2


def _sem_sizes(S, D, cfg):
    n = cfg["NRING"]
    return [2, D // cfg["MCH"], S // cfg["T0"], n, n, n, n, n, 3, S // cfg["TL"], 2]


def _make_kernel(S, D, H, DH, SK, F, cfg):
    T0, TL, NRING, MCH = cfg["T0"], cfg["TL"], cfg["NRING"], cfg["MCH"]
    R0, RL = cfg["R0"], cfg["RL"]
    J0 = S // T0
    JL = S // TL
    qscale = DH ** -0.5 * _LOG2E
    n_mch = D // MCH
    MC = (4 * D) // H
    FC = 512
    W = 512
    NFF = 16
    assert NRING == 4 and TL // 8 <= 128 and JL >= 3

    def kernel(x_hbm, k_hbm, v_hbm, wq_hbm, wo_hbm, wr_hbm, wg_hbm, wu_hbm, wd_hbm,
               c_hbm, wmod_hbm, out_hbm,
               x_buf, h_buf, acc, s_buf, m_buf, s2_buf, m2_buf, st_buf,
               kb, vb, wqb, wob, wmb, wm0, c_buf, wr_buf, cb_buf, mod0, modr, modv,
               wg, wu, wd, o_buf, key_buf, fix,
               sems):

        class _Sem:
            def __init__(self, base):
                self.base = base
                self.at = self

            def __getitem__(self, i):
                return sems.at[self.base + i]

        sizes = _sem_sizes(S, D, cfg)
        offs = [sum(sizes[:i]) for i in range(len(sizes))]
        (sem_small, sem_wm0, sem_x, sem_k, sem_v, sem_wq, sem_wo, sem_wm,
         sem_ffn, sem_out, sem_fix) = (_Sem(o) for o in offs)

        def _mul(a, n):
            v = a * n
            return v if isinstance(a, int) else pl.multiple_of(v, n)

        def view(ref, j, t, n=1):
            return ref.at[pl.ds(_mul(j, t), n * t), :]

        def slot(h):
            return h & (NRING - 1)

        def cp_c():
            return pltpu.make_async_copy(c_hbm, c_buf, sem_small.at[0])

        def cp_wr():
            return pltpu.make_async_copy(wr_hbm, wr_buf, sem_small.at[1])

        def cp_wm0(i):
            return pltpu.make_async_copy(
                wmod_hbm.at[pl.ds(i * MCH, MCH), pl.ds(0, 2 * D)],
                wm0.at[pl.ds(i * MCH, MCH), :], sem_wm0.at[i])

        def cp_x(j):
            return pltpu.make_async_copy(view(x_hbm, j, T0), view(x_buf, j, T0), sem_x.at[j])

        def cp_k(h):
            return pltpu.make_async_copy(k_hbm.at[h], kb.at[slot(h)], sem_k.at[slot(h)])

        def cp_v(h):
            return pltpu.make_async_copy(v_hbm.at[h], vb.at[slot(h)], sem_v.at[slot(h)])

        def cp_wq(h):
            return pltpu.make_async_copy(
                wq_hbm.at[:, pl.ds(_mul(h, DH), DH)], wqb.at[slot(h)], sem_wq.at[slot(h)])

        def cp_wo(h):
            return pltpu.make_async_copy(
                wo_hbm.at[pl.ds(_mul(h, DH), DH), :], wob.at[slot(h)], sem_wo.at[slot(h)])

        def cp_wm(h):
            return pltpu.make_async_copy(
                wmod_hbm.at[:, pl.ds(_mul(h + (2 * D) // MC, MC), MC)], wmb.at[slot(h)],
                sem_wm.at[slot(h)])

        ffn = ((wg_hbm, wg), (wu_hbm, wu), (wd_hbm, wd))

        def cp_ffn_piece(i, p):
            src, dst = ffn[i]
            n = src.shape[0] // NFF
            return pltpu.make_async_copy(view(src, p, n), view(dst, p, n), sem_ffn.at[i])

        def wait_ffn(i):
            src, dst = ffn[i]
            pltpu.make_async_copy(src, dst, sem_ffn.at[i]).wait()

        def cp_out(j):
            return pltpu.make_async_copy(view(o_buf, j, TL), view(out_hbm, j, TL), sem_out.at[j])

        def ln1_chunks(xv):
            def chunk(off):
                def f(tok=None):
                    mean, inv, _ = _row_stats(xv[off:off + R0, :].astype(f32),
                                              None if tok is None else _rep(tok, R0))
                    st_buf[0, off:off + R0, :] = mean
                    st_buf[1, off:off + R0, :] = inv
                    return inv[R0 - 8:, :]
                return f
            return [chunk(off) for off in range(0, T0, R0)]

        def qproj(h, hv, xv=None, rec=None):
            q = None
            for c in range(D // W):
                cs = slice(c * W, (c + 1) * W)
                if xv is None:
                    hh = pltpu.bitcast(hv[:, cs], bf16)
                else:
                    n = (xv[:, cs].astype(f32) - _wide(st_buf[0], W)) * _wide(st_buf[1], W)
                    hh = (n * _rep(mod0[:, D + c * W:D + (c + 1) * W], T0)
                          + _rep(mod0[:, cs], T0)).astype(bf16)
                    hv[:, cs] = pltpu.bitcast(hh, u32)
                if rec is not None:
                    hh = rec.gate(hh)
                part = jnp.dot(hh, wqb[slot(h), cs, :], preferred_element_type=f32)
                q = part if q is None else q + part
                if rec is not None:
                    rec.done(part)
            return (q * qscale).astype(bf16)

        def scores(h, q, sv, mv, rec=None):
            mp = None
            for c in range(SK // W):
                cs = slice(c * W, (c + 1) * W)
                qq = q if rec is None else rec.gate(q)
                s = lax.dot_general(qq, kb[slot(h), cs, :], _NT, preferred_element_type=f32)
                sv[:, cs] = s
                if rec is not None:
                    rec.done(s)
                mp = _fold(jnp.maximum, ([] if mp is None else [mp]) + _tiles(s))
            mv[...] = jnp.broadcast_to(jnp.max(mp, axis=-1, keepdims=True), mp.shape)

        def pv(h, sv, mv, late=None, rec=None):
            o = lp = None
            for c in range(SK // W):
                cs = slice(c * W, (c + 1) * W)
                p = jnp.exp2(sv[:, cs] - _wide(mv[...], W))
                lp = _fold(jnp.add, ([] if lp is None else [lp]) + _tiles(p))
                pb = p.astype(bf16)
                if rec is not None:
                    pb = rec.gate(pb)
                d = jnp.dot(pb, vb[slot(h), cs, :], preferred_element_type=f32)
                o = d if o is None else o + d
                if c == late:
                    lp = lp + _zero_of(d)
                if rec is not None:
                    rec.done(d)
            l = jnp.sum(lp, axis=-1, keepdims=True)
            r = pl.reciprocal(l, approx=True)
            r = r * (2.0 - l * r)
            return (o * r).astype(bf16)

        def oproj(h, o, av, xv=None, rec=None):
            for c in range(D // W):
                cs = slice(c * W, (c + 1) * W)
                oo = o if rec is None else rec.gate(o)
                d = jnp.dot(oo, wob[slot(h), :, cs], preferred_element_type=f32)
                if rec is not None:
                    rec.done(d)
                old = av[:, cs]
                if not isinstance(h, int):
                    old = jnp.where(h > 0, old, 0.0)
                a = old + d
                if xv is not None:
                    a = xv[:, cs].astype(f32) + _rep(modv[0, :, cs], a.shape[0]) * a
                av[:, cs] = a

        def mod_chunk(h):
            w = wmb[slot(h)].astype(f32)
            part = (w * cb_buf[...]).reshape(D // 8, 8, MC).sum(axis=0)
            modr[h] = _rb(jnp.sum(part, axis=0, keepdims=True))

        def finish_mod():
            n = D // MC
            ga, sb, cb, gb = (jnp.concatenate([modr[i * n + t] for t in range(n)], axis=-1)
                              for i in range(4))
            cb1 = _rb(1.0 + cb)
            wr = wr_buf[...].astype(f32)
            a = cb1 * wr
            a0 = jnp.broadcast_to(jnp.sum(a, axis=-1, keepdims=True), (1, D))
            b0 = jnp.broadcast_to(jnp.sum(sb * wr, axis=-1, keepdims=True), (1, D))
            for i, v in enumerate((ga, sb, cb1, gb, a, gb * cb1, gb * sb, a0, b0)):
                modv[i] = jnp.broadcast_to(v, (8, D))

        def epi_chunks(j, x1v, ov):
            lane = lax.broadcasted_iota(i32, (8, 128), 1)
            sub = lax.broadcasted_iota(i32, (8, 128), 0)
            st = {"rv": jnp.zeros((8, 128), f32)}

            def chunk(off):
                def f(tok=None):
                    x1 = x1v[off:off + RL, :]
                    mean, inv, _ = _row_stats(x1, None if tok is None else _rep(tok, RL))
                    xa = _tiles(x1 * _rep(modv[4], RL))
                    if tok is not None:
                        xa[0] = xa[0] + _rep(tok, RL)
                    ra = _lane_sum(_fold(jnp.add, xa))
                    r = inv * (ra - mean * _rep(modv[7, :, 0:128], RL)) + _rep(modv[8, :, 0:128], RL)
                    u = _wide(inv, D) * _rep(modv[5], RL)
                    res = x1 + ((x1 - _wide(mean, D)) * u + _rep(modv[6], RL))
                    ov[off:off + RL, :] = res.astype(bf16)
                    for g in range(RL // 8):
                        st["rv"] = jnp.where(lane == off // 8 + g, r[g * 8:(g + 1) * 8, :], st["rv"])
                    if off + RL == TL:
                        bits = pltpu.bitcast(_rb(st["rv"]) + 0.0, i32)
                        mono = jnp.where(bits < 0, bits ^ 0x7FFF0000, bits)
                        row = j * TL + lane * 8 + sub
                        key_buf[j] = jnp.where(lane < TL // 8, mono | (0xFFFF - row), _IMIN)
                    ends = _tiles(res[RL - 8:, :])
                    return _fold(jnp.add, ends[-cfg["NEND"]:] + [st["rv"]])
                return f
            return [chunk(off) for off in range(0, TL, RL)]

        cp_c().start()
        cp_x(0).start()
        for i in range(n_mch):
            cp_wm0(i).start()
        cp_wq(0).start()
        cp_k(0).start()
        for j in range(1, J0):
            cp_x(j).start()
        cp_wq(1).start()
        cp_v(0).start()
        cp_wm(0).start()
        cp_k(1).start()
        cp_wo(0).start()
        cp_wr().start()
        cp_v(1).start()
        cp_wo(1).start()
        cp_wm(1).start()
        cp_wq(2).start()
        cp_k(2).start()

        cp_c().wait()
        cf = c_buf[...].astype(f32)
        sc = _rb(cf * jax.nn.sigmoid(cf))
        cb_buf[...] = jnp.transpose(jnp.broadcast_to(sc, (128, D)))
        cp_x(0).wait()
        for ch in ln1_chunks(view(x_buf, 0, T0)):
            ch()

        part = None
        for i in range(n_mch):
            cp_wm0(i).wait()
            scb = jnp.broadcast_to(sc[:, i * MCH:(i + 1) * MCH], (16, MCH)).astype(bf16)
            d = jnp.dot(scb, wm0[i * MCH:(i + 1) * MCH, :], preferred_element_type=f32)
            part = d if part is None else part + d
        m0 = _rb(part[0:8, :])
        mod0[:, 0:D] = m0[:, 0:D]
        mod0[:, D:2 * D] = _rb(1.0 + m0[:, D:2 * D])
        cp_wq(0).wait()
        cp_k(0).wait()

        def p0_body(j, carry):
            @pl.when(j + 1 < J0)
            def _():
                cp_x(j + 1).wait()
            rec = _Pace(ln1_chunks(view(x_buf, jnp.minimum(j + 1, J0 - 1), T0)),
                        [int(ch, 36) for ch in cfg["LC0"]], 100)
            q = qproj(0, view(h_buf, j, T0 // 2), view(x_buf, j, T0), rec=rec)
            scores(0, q, view(s_buf, j, T0), view(m_buf, j, T0), rec=rec)
            return carry
        lax.fori_loop(0, J0, p0_body, 0)

        def wait_head(h):
            cp_wq(h + 1).wait()
            cp_k(h + 1).wait()
            cp_v(h).wait()
            cp_wo(h).wait()
            cp_wm(h).wait()

        def main_body(h, carry):
            q = qproj(h + 1, h_buf)
            o = pv(h, s_buf, m_buf)
            cp_v(h + 2).start()
            mod_chunk(h)
            scores(h + 1, q, s_buf, m_buf)
            oproj(h, o, acc)
            cp_wm(h + 2).start()
            cp_wo(h + 2).start()

            @pl.when(h + 3 < H)
            def _():
                cp_wq(h + 3).start()
                cp_k(h + 3).start()

            @pl.when(h < NFF)
            def _():
                for i in range(3):
                    cp_ffn_piece(i, h).start()
            wait_head(h + 1)
            return carry
        wait_head(0)
        lax.fori_loop(0, H - 2, main_body, 0)

        ha, hb = H - 2, H - 1
        cp_v(hb).wait()
        cp_wo(hb).wait()
        cp_wm(hb).wait()
        cp_wr().wait()

        def l_step(j, do_x, do_y):
            if do_x and do_y:
                aw = view(acc, j - 1, TL, 2)
                ay, ax = aw.at[0:TL, :], aw.at[TL:2 * TL, :]
            elif do_x:
                ax = view(acc, j, TL)
            else:
                ay = view(acc, j - 1, TL)
            rec = None
            if do_y:
                chunks = epi_chunks(j - 1, ay, view(o_buf, j - 1, TL))
                if do_x:
                    cnt = [int(ch) for ch in cfg["LCNT"]]
                    assert sum(cnt) == len(chunks)
                    rec = _Pace(chunks, cnt, cfg["LAG"] / 4)
            v = {}
            for op in cfg["LORD"]:
                if op == "Q" and do_x:
                    v["q"] = qproj(hb, view(h_buf, j, TL // 2), rec=rec)
                if op == "B" and do_y:
                    v["ob"] = pv(hb, s2_buf, m2_buf, rec=rec)
                if op == "b" and do_y:
                    oproj(hb, v["ob"], ay, view(x_buf, j - 1, TL), rec=rec)
                if op == "A" and do_x:
                    v["oa"] = pv(ha, view(s_buf, j, TL), view(m_buf, j, TL), rec=rec)
                if op == "S" and do_x:
                    scores(hb, v["q"], s2_buf, m2_buf, rec=rec)
                if op == "a" and do_x:
                    oproj(ha, v["oa"], ax, rec=rec)
            if do_y:
                if not do_x:
                    for ch in chunks:
                        ch()
                cp_out(j - 1).start()

        mod_chunk(ha)
        mod_chunk(hb)
        finish_mod()
        l_step(0, True, False)

        def pl_body(j, carry):
            l_step(j, True, True)
            return carry
        lax.fori_loop(1, JL, pl_body, 0)
        for i in range(3):
            wait_ffn(i)
        for j in range(JL - 2):
            cp_out(j).wait()
        l_step(JL, False, True)

        keys = key_buf[...].reshape(JL * 8, 128)
        k1 = jnp.max(keys, keepdims=True)
        k2 = jnp.max(jnp.where(keys == k1, _IMIN, keys), keepdims=True)

        def score_of(k):
            hi = k & jnp.int32(-65536)
            return pltpu.bitcast(jnp.where(hi < 0, hi ^ 0x7FFF0000, hi), f32)

        i1s = jnp.minimum(0xFFFF - (k1[0, 0] & 0xFFFF), S - 1)
        i2s = jnp.minimum(0xFFFF - (k2[0, 0] & 0xFFFF), S - 1)

        sub = lax.broadcasted_iota(i32, (16, D), 0)
        sb, cb1, gb = (_rep(modv[i], 16) for i in (1, 2, 3))

        def adaln2(x1):
            mean, inv, _ = _row_stats(x1)
            return (x1 - _wide(mean, D)) * _wide(inv, D) * cb1 + sb

        xs = adaln2(jnp.where(sub == 0, acc[pl.ds(i1s, 1), :], acc[pl.ds(i2s, 1), :])).astype(bf16)
        y = jnp.zeros((16, D), f32)
        for c in range(F // FC):
            cs = slice(c * FC, (c + 1) * FC)
            g = _rb(jnp.dot(xs, wg[:, cs], preferred_element_type=f32))
            g = _rb(g * jax.nn.sigmoid(g))
            u = _rb(jnp.dot(xs, wu[:, cs], preferred_element_type=f32))
            y = y + jnp.dot((g * u).astype(bf16), wd[cs, :], preferred_element_type=f32)
        y = _rb(y)
        ya = _rb(y[0:1, :] * _rb(jax.nn.sigmoid(score_of(k1))))
        yb = _rb(y[1:2, :] * _rb(jax.nn.sigmoid(score_of(k2))))

        g1 = pl.multiple_of((i1s >> 4) << 4, 16)
        g2 = pl.multiple_of((i2s >> 4) << 4, 16)
        for t, g0 in enumerate((g1, g2)):
            rid = sub + g0
            x1 = acc[pl.ds(g0, 16), :]
            upd = jnp.where(rid == i1s, ya, 0.0) + jnp.where(rid == i2s, yb, 0.0)
            fix[t] = (x1 + gb * (adaln2(x1) + upd)).astype(bf16)

        for j in range(JL - 2, JL):
            cp_out(j).wait()

        def cp_fix(t, g0):
            return pltpu.make_async_copy(fix.at[t], out_hbm.at[pl.ds(g0, 16), :], sem_fix.at[t])

        cp_fix(0, g1).start()

        @pl.when(g2 != g1)
        def _():
            cp_fix(1, g2).start()
            cp_fix(1, g2).wait()
        cp_fix(0, g1).wait()

    return kernel


_CFG = dict(T0=256, TL=256, NRING=4, MCH=128, R0=16, RL=8,  LORD='BAbQSa', LAG=100, NEND=1, LCNT='000000000055555520', LC0='045520')


def _build(A_x, A_k_cache, A_v_cache, A_wq, A_wo, B_w_r, B_w_gate, B_w_up, B_w_down, c, w_mod,
           **over):
    B, S, D = A_x.shape
    _, H, SK, DH = A_k_cache.shape
    F = B_w_gate.shape[1]
    assert B == 1
    cfg = dict(_CFG, **over)
    T0, TL, NRING = cfg["T0"], cfg["TL"], cfg["NRING"]
    MC = (4 * D) // H
    kernel = _make_kernel(S, D, H, DH, SK, F, cfg)
    scratch = [
        pltpu.VMEM((S, D), bf16),
        pltpu.VMEM((S // 2, D), u32),
        pltpu.VMEM((S, D), f32),
        pltpu.VMEM((S, SK), f32),
        pltpu.VMEM((S, 128), f32),
        pltpu.VMEM((TL, SK), f32),
        pltpu.VMEM((TL, 128), f32),
        pltpu.VMEM((2, T0, 128), f32),
        pltpu.VMEM((NRING, SK, DH), bf16),
        pltpu.VMEM((NRING, SK, DH), bf16),
        pltpu.VMEM((NRING, D, DH), bf16),
        pltpu.VMEM((NRING, DH, D), bf16),
        pltpu.VMEM((NRING, D, MC), bf16),
        pltpu.VMEM((D, 2 * D), bf16),
        pltpu.VMEM((1, D), bf16),
        pltpu.VMEM((1, D), bf16),
        pltpu.VMEM((D, 128), f32),
        pltpu.VMEM((8, 2 * D), f32),
        pltpu.VMEM((H, 1, MC), f32),
        pltpu.VMEM((9, 8, D), f32),
        pltpu.VMEM((D, F), bf16),
        pltpu.VMEM((D, F), bf16),
        pltpu.VMEM((F, D), bf16),
        pltpu.VMEM((S, D), bf16),
        pltpu.VMEM((S // TL, 8, 128), i32),
        pltpu.VMEM((2, 16, D), bf16),
        pltpu.SemaphoreType.DMA((sum(_sem_sizes(S, D, cfg)),)),
    ]
    any_spec = pl.BlockSpec(memory_space=pl.ANY)
    out = pl.pallas_call(
        kernel,
        out_shape=jax.ShapeDtypeStruct((S, D), bf16),
        in_specs=[any_spec] * 11,
        out_specs=any_spec,
        scratch_shapes=scratch,
        compiler_params=pltpu.CompilerParams(vmem_limit_bytes=124 * 1024 * 1024,
                                             disable_bounds_checks=True),
    )(A_x.reshape(S, D), A_k_cache.reshape(H, SK, DH), A_v_cache.reshape(H, SK, DH),
      A_wq, A_wo, B_w_r.reshape(1, D), B_w_gate, B_w_up, B_w_down, c, w_mod)
    return out.reshape(B, S, D)


@jax.jit
def pallas_adaLN_cond__mha_block_cached__moe_arch_mod__prompt_kernel(
    A_x: jax.Array,
    A_k_cache: jax.Array,
    A_v_cache: jax.Array,
    A_wq: jax.Array,
    A_wo: jax.Array,
    B_x: jax.Array,
    B_w_r: jax.Array,
    B_w_gate: jax.Array,
    B_w_up: jax.Array,
    B_w_down: jax.Array,
    c: jax.Array,
    w_mod: jax.Array,
):
    del B_x
    return _build(A_x, A_k_cache, A_v_cache, A_wq, A_wo, B_w_r, B_w_gate, B_w_up, B_w_down,
                  c, w_mod)
```

```python
import jax
import jax.numpy as jnp
from jax import lax
import jax.experimental.pallas as pl
import jax.experimental.pallas.tpu as pltpu

f32 = jnp.float32
bf16 = jnp.bfloat16
u32 = jnp.uint32
i32 = jnp.int32

_NT = (((1,), (1,)), ((), ()))
_LOG2E = 1.4426950408889634
_EPS = 1e-5
_IMIN = -2 ** 31


def _rb(v):
    return v.astype(bf16).astype(f32)


def _rep(v, n):
    return v if n == 8 else jnp.tile(v, (n // 8, 1))


def _wide(v, w):
    return jnp.tile(v, (1, w // 128))


def _zero_of(v):
    bits = pltpu.bitcast(v, u32)
    return pltpu.bitcast(lax.shift_right_logical(lax.shift_right_logical(bits, jnp.uint32(31)),
                                                 jnp.uint32(1)), f32)


def _zero_bits(v):
    bits = pltpu.bitcast(v, u32)
    return lax.shift_right_logical(lax.shift_right_logical(bits, jnp.uint32(31)), jnp.uint32(1))


class _Pace:
    def __init__(self, chunks, counts, lag):
        self.chunks, self.counts, self.lag = list(chunks), list(counts), lag
        self.r = 0
        self.due = {}

    def gate(self, lhs):
        items = self.due.pop(self.r, [])
        if not items:
            return lhs
        u = pltpu.bitcast(lhs, u32)
        first = u[:, 0:128]
        parts, pos = [], 0
        for frac, tok in items:
            g = max(int(frac * u.shape[0]) // 8 * 8, pos)
            if g > pos:
                parts.append(first[pos:g])
            parts.append(first[g:g + 8] | tok)
            pos = g + 8
        if pos < u.shape[0]:
            parts.append(first[pos:])
        first = jnp.concatenate(parts, axis=0)
        if u.shape[1] > 128:
            first = jnp.concatenate([first, u[:, 128:]], axis=1)
        return pltpu.bitcast(first, bf16)

    def done(self, res):
        n = self.counts[self.r]
        for i in range(n):
            r0 = (i * res.shape[0] // n) // 8 * 8
            end = self.chunks.pop(0)(_zero_of(res[r0:r0 + 8, 0:128]))
            t = self.r + i / n + self.lag
            self.due.setdefault(int(t), []).append((t - int(t), _zero_bits(end)))
        self.r += 1


def _tiles(v):
    return [v[:, c * 128:(c + 1) * 128] for c in range(v.shape[1] // 128)]


def _fold(op, parts):
    out = parts[0]
    for p in parts[1:]:
        out = op(out, p)
    return out


def _lane_sum(v):
    return jnp.broadcast_to(jnp.sum(v, axis=-1, keepdims=True), v.shape)


def _row_stats(xf, tok=None):
    d = xf.shape[-1]
    ts = _tiles(xf)
    nt = len(ts)
    if tok is not None:
        ts = [ts[0] + tok] + ts[1:]
    mu = _fold(jnp.add, ts) * (1.0 / nt)
    m2 = _fold(jnp.add, [(t - mu) * (t - mu) for t in ts])
    mean = _lane_sum(mu) * (1.0 / 128)
    dm = mu - mean
    var = _lane_sum(m2 + (dm * dm) * float(nt)) * (1.0 / d)
    return mean, lax.rsqrt(var + _EPS), m2


def _sem_sizes(S, D, cfg):
    n = cfg["NRING"]
    return [2, D // cfg["MCH"], S // cfg["T0"], n, n, n, n, n, 3, S // cfg["TL"], 2]


def _make_kernel(S, D, H, DH, SK, F, cfg):
    T0, TL, NRING, MCH = cfg["T0"], cfg["TL"], cfg["NRING"], cfg["MCH"]
    R0 = cfg["R0"]
    J0 = S // T0
    JL = S // TL
    qscale = DH ** -0.5 * _LOG2E
    n_mch = D // MCH
    MC = (4 * D) // H
    W = 512
    NFF = 16
    assert NRING == 4 and TL // 8 <= 128 and JL >= 3

    def kernel(x_hbm, k_hbm, v_hbm, wq_hbm, wo_hbm, wr_hbm, wg_hbm, wu_hbm, wd_hbm,
               c_hbm, wmod_hbm, out_hbm,
               x_buf, h_buf, acc, s_buf, m_buf, s2_buf, m2_buf, st_buf, st2_buf,
               kb, vb, wqb, wob, wmb, wm0, c_buf, wr_buf, cb_buf, mod0, modr, modv,
               wg, wu, wd, o_buf, key_buf, fix,
               sems):

        class _Sem:
            def __init__(self, base):
                self.base = base
                self.at = self

            def __getitem__(self, i):
                return sems.at[self.base + i]

        sizes = _sem_sizes(S, D, cfg)
        offs = [sum(sizes[:i]) for i in range(len(sizes))]
        (sem_small, sem_wm0, sem_x, sem_k, sem_v, sem_wq, sem_wo, sem_wm,
         sem_ffn, sem_out, sem_fix) = (_Sem(o) for o in offs)

        def _mul(a, n):
            v = a * n
            return v if isinstance(a, int) else pl.multiple_of(v, n)

        def view(ref, j, t, n=1):
            return ref.at[pl.ds(_mul(j, t), n * t), :]

        def slot(h):
            return h & (NRING - 1)

        def cp_c():
            return pltpu.make_async_copy(c_hbm, c_buf, sem_small.at[0])

        def cp_wr():
            return pltpu.make_async_copy(wr_hbm, wr_buf, sem_small.at[1])

        def cp_wm0(i):
            return pltpu.make_async_copy(
                wmod_hbm.at[pl.ds(i * MCH, MCH), pl.ds(0, 2 * D)],
                wm0.at[pl.ds(i * MCH, MCH), :], sem_wm0.at[i])

        def cp_x(j):
            return pltpu.make_async_copy(view(x_hbm, j, T0), view(x_buf, j, T0), sem_x.at[j])

        def cp_k(h):
            return pltpu.make_async_copy(k_hbm.at[h], kb.at[slot(h)], sem_k.at[slot(h)])

        def cp_v(h):
            return pltpu.make_async_copy(v_hbm.at[h], vb.at[slot(h)], sem_v.at[slot(h)])

        def cp_wq(h):
            return pltpu.make_async_copy(
                wq_hbm.at[:, pl.ds(_mul(h, DH), DH)], wqb.at[slot(h)], sem_wq.at[slot(h)])

        def cp_wo(h):
            return pltpu.make_async_copy(
                wo_hbm.at[pl.ds(_mul(h, DH), DH), :], wob.at[slot(h)], sem_wo.at[slot(h)])

        def cp_wm(h):
            return pltpu.make_async_copy(
                wmod_hbm.at[:, pl.ds(_mul(h + (2 * D) // MC, MC), MC)], wmb.at[slot(h)],
                sem_wm.at[slot(h)])

        ffn = ((wg_hbm, wg), (wu_hbm, wu), (wd_hbm, wd))

        def cp_ffn_piece(i, p):
            src, dst = ffn[i]
            n = src.shape[0] // NFF
            return pltpu.make_async_copy(view(src, p, n), view(dst, p, n), sem_ffn.at[i])

        def wait_ffn(i):
            src, dst = ffn[i]
            pltpu.make_async_copy(src, dst, sem_ffn.at[i]).wait()

        def cp_out(j):
            return pltpu.make_async_copy(view(o_buf, j, TL), view(out_hbm, j, TL), sem_out.at[j])

        def ln1_chunks(xv):
            def chunk(off):
                def f(tok=None):
                    mean, inv, _ = _row_stats(xv[off:off + R0, :].astype(f32),
                                              None if tok is None else _rep(tok, R0))
                    st_buf[0, off:off + R0, :] = mean
                    st_buf[1, off:off + R0, :] = inv
                    return inv[R0 - 8:, :]
                return f
            return [chunk(off) for off in range(0, T0, R0)]

        def qproj(h, hv, xv=None, rec=None):
            q = None
            for c in range(D // W):
                cs = slice(c * W, (c + 1) * W)
                if xv is None:
                    hh = pltpu.bitcast(hv[:, cs], bf16)
                else:
                    n = (xv[:, cs].astype(f32) - _wide(st_buf[0], W)) * _wide(st_buf[1], W)
                    hh = (n * _rep(mod0[:, D + c * W:D + (c + 1) * W], T0)
                          + _rep(mod0[:, cs], T0)).astype(bf16)
                    hv[:, cs] = pltpu.bitcast(hh, u32)
                if rec is not None:
                    hh = rec.gate(hh)
                part = jnp.dot(hh, wqb[slot(h), cs, :], preferred_element_type=f32)
                q = part if q is None else q + part
                if rec is not None:
                    rec.done(part)
            return (q * qscale).astype(bf16)

        def scores(h, q, sv, mv, rec=None):
            mp = None
            for c in range(SK // W):
                cs = slice(c * W, (c + 1) * W)
                qq = q if rec is None else rec.gate(q)
                s = lax.dot_general(qq, kb[slot(h), cs, :], _NT, preferred_element_type=f32)
                sv[:, cs] = s
                if rec is not None:
                    rec.done(s)
                mp = _fold(jnp.maximum, ([] if mp is None else [mp]) + _tiles(s))
            mv[...] = jnp.broadcast_to(jnp.max(mp, axis=-1, keepdims=True), mp.shape)

        def pv(h, sv, mv, late=None, rec=None):
            o = lp = None
            for c in range(SK // W):
                cs = slice(c * W, (c + 1) * W)
                p = jnp.exp2(sv[:, cs] - _wide(mv[...], W))
                lp = _fold(jnp.add, ([] if lp is None else [lp]) + _tiles(p))
                pb = p.astype(bf16)
                if rec is not None:
                    pb = rec.gate(pb)
                d = jnp.dot(pb, vb[slot(h), cs, :], preferred_element_type=f32)
                o = d if o is None else o + d
                if c == late:
                    lp = lp + _zero_of(d)
                if rec is not None:
                    rec.done(d)
            l = jnp.sum(lp, axis=-1, keepdims=True)
            r = pl.reciprocal(l, approx=True)
            r = r * (2.0 - l * r)
            return (o * r).astype(bf16)

        def oproj(h, o, av, xv=None, rec=None):
            for c in range(D // W):
                cs = slice(c * W, (c + 1) * W)
                oo = o if rec is None else rec.gate(o)
                d = jnp.dot(oo, wob[slot(h), :, cs], preferred_element_type=f32)
                if rec is not None:
                    rec.done(d)
                old = av[:, cs]
                if not isinstance(h, int):
                    old = jnp.where(h > 0, old, 0.0)
                a = old + d
                if xv is not None:
                    a = xv[:, cs].astype(f32) + _rep(modv[0, :, cs], a.shape[0]) * a
                av[:, cs] = a

        def mod_chunk(h):
            w = wmb[slot(h)].astype(f32)
            part = (w * cb_buf[...]).reshape(D // 8, 8, MC).sum(axis=0)
            modr[h] = _rb(jnp.sum(part, axis=0, keepdims=True))

        def finish_mod():
            n = D // MC
            ga, sb, cb, gb = (jnp.concatenate([modr[i * n + t] for t in range(n)], axis=-1)
                              for i in range(4))
            cb1 = _rb(1.0 + cb)
            wr = wr_buf[...].astype(f32).reshape(1, D)
            a = cb1 * wr
            a0 = jnp.broadcast_to(jnp.sum(a, axis=-1, keepdims=True), (1, D))
            b0 = jnp.broadcast_to(jnp.sum(sb * wr, axis=-1, keepdims=True), (1, D))
            for i, v in enumerate((ga, sb, cb1, gb, a, gb * cb1, gb * sb, a0, b0)):
                modv[i] = jnp.broadcast_to(v, (8, D))

        def epi_chunks(j, x1v, ov, st):
            sub = lax.broadcasted_iota(i32, (8, 128), 0)
            low = (0xFFFF - j * TL) - sub
            sv = view(st2_buf, j, TL)

            def chunk(off):
                def f(tok=None):
                    if off == 0:
                        st["k1"], st["k2"] = key_buf[0], key_buf[1]
                    x1 = x1v[off:off + 8, :]
                    mean, inv, _ = _row_stats(x1, tok)
                    sv[off:off + 8, 0:128] = mean
                    sv[off:off + 8, 128:256] = inv
                    xa = _tiles(x1 * modv[4])
                    if tok is not None:
                        xa[0] = xa[0] + tok
                    ra = _lane_sum(_fold(jnp.add, xa))
                    r = inv * (ra - mean * modv[7, :, 0:128]) + modv[8, :, 0:128]
                    res = x1 + ((x1 - _wide(mean, D)) * (_wide(inv, D) * modv[5]) + modv[6])
                    ov[off:off + 8, :] = res.astype(bf16)
                    bits = pltpu.bitcast(_rb(r) + 0.0, i32)
                    key = jnp.where(bits < 0, bits ^ 0x7FFF0000, bits) | (low - off)
                    st["k2"] = jnp.maximum(st["k2"], jnp.minimum(st["k1"], key))
                    st["k1"] = jnp.maximum(st["k1"], key)
                    if off + 8 == TL:
                        key_buf[0], key_buf[1] = st["k1"], st["k2"]
                    return res[:, D - 128:]
                return f
            return [chunk(off) for off in range(0, TL, 8)]

        cp_c().start()
        cp_x(0).start()
        for i in range(n_mch):
            cp_wm0(i).start()
        cp_wq(0).start()
        cp_k(0).start()
        for j in range(1, J0):
            cp_x(j).start()
        cp_wq(1).start()
        cp_v(0).start()
        cp_wm(0).start()
        cp_k(1).start()
        cp_wo(0).start()
        cp_wr().start()
        cp_v(1).start()
        cp_wo(1).start()
        cp_wm(1).start()
        cp_wq(2).start()
        cp_k(2).start()

        cp_c().wait()
        cf = c_buf[...].astype(f32)
        sc = _rb(cf * jax.nn.sigmoid(cf))
        cb_buf[...] = jnp.transpose(jnp.broadcast_to(sc, (128, D)))
        cp_x(0).wait()
        for ch in ln1_chunks(view(x_buf, 0, T0)):
            ch()

        part = None
        for i in range(n_mch):
            cp_wm0(i).wait()
            scb = jnp.broadcast_to(sc[:, i * MCH:(i + 1) * MCH], (16, MCH)).astype(bf16)
            d = jnp.dot(scb, wm0[i * MCH:(i + 1) * MCH, :], preferred_element_type=f32)
            part = d if part is None else part + d
        m0 = _rb(part[0:8, :])
        mod0[:, 0:D] = m0[:, 0:D]
        mod0[:, D:2 * D] = _rb(1.0 + m0[:, D:2 * D])
        cp_wq(0).wait()
        cp_k(0).wait()

        def p0_body(j, carry):
            @pl.when(j + 1 < J0)
            def _():
                cp_x(j + 1).wait()
            rec = _Pace(ln1_chunks(view(x_buf, jnp.minimum(j + 1, J0 - 1), T0)),
                        [int(ch, 36) for ch in cfg["LC0"]], 100)
            q = qproj(0, view(h_buf, j, T0 // 2), view(x_buf, j, T0), rec=rec)
            scores(0, q, view(s_buf, j, T0), view(m_buf, j, T0), rec=rec)
            return carry
        lax.fori_loop(0, J0, p0_body, 0)

        def wait_head(h):
            cp_wq(h + 1).wait()
            cp_k(h + 1).wait()
            cp_v(h).wait()
            cp_wo(h).wait()
            cp_wm(h).wait()

        def main_body(h, carry):
            q = qproj(h + 1, h_buf)
            o = pv(h, s_buf, m_buf)
            cp_v(h + 2).start()
            mod_chunk(h)
            scores(h + 1, q, s_buf, m_buf)
            oproj(h, o, acc)
            cp_wm(h + 2).start()
            cp_wo(h + 2).start()

            @pl.when(h + 3 < H)
            def _():
                cp_wq(h + 3).start()
                cp_k(h + 3).start()

            @pl.when(h < NFF)
            def _():
                for i in range(3):
                    cp_ffn_piece(i, h).start()
            wait_head(h + 1)
            return carry
        wait_head(0)
        lax.fori_loop(0, H - 2, main_body, 0)

        ha, hb = H - 2, H - 1
        cp_v(hb).wait()
        cp_wo(hb).wait()
        cp_wm(hb).wait()
        cp_wr().wait()

        def l_step(j, do_x, do_y):
            if do_x and do_y:
                aw = view(acc, j - 1, TL, 2)
                ay, ax = aw.at[0:TL, :], aw.at[TL:2 * TL, :]
            elif do_x:
                ax = view(acc, j, TL)
            else:
                ay = view(acc, j - 1, TL)
            rec = None
            if do_y:
                chunks = epi_chunks(j - 1, ay, view(o_buf, j - 1, TL), {})
                if do_x:
                    cnt = [int(ch) for ch in cfg["LCNT"]]
                    assert sum(cnt) == len(chunks)
                    rec = _Pace(chunks, cnt, cfg["LAG"] / 4)
            v = {}
            for op in cfg["LORD"]:
                if op == "Q" and do_x:
                    v["q"] = qproj(hb, view(h_buf, j, TL // 2), rec=rec)
                if op == "B" and do_y:
                    v["ob"] = pv(hb, s2_buf, m2_buf, rec=rec)
                if op == "b" and do_y:
                    oproj(hb, v["ob"], ay, view(x_buf, j - 1, TL), rec=rec)
                if op == "A" and do_x:
                    v["oa"] = pv(ha, view(s_buf, j, TL), view(m_buf, j, TL), rec=rec)
                if op == "S" and do_x:
                    scores(hb, v["q"], s2_buf, m2_buf, rec=rec)
                if op == "a" and do_x:
                    oproj(ha, v["oa"], ax, rec=rec)
            if do_y:
                if not do_x:
                    for ch in chunks:
                        ch()
                cp_out(j - 1).start()

        mod_chunk(ha)
        mod_chunk(hb)
        finish_mod()
        key_buf[...] = jnp.full(key_buf.shape, _IMIN, i32)
        l_step(0, True, False)

        def pl_body(j, carry):
            l_step(j, True, True)
            return carry
        lax.fori_loop(1, JL, pl_body, 0)
        for i in range(3):
            wait_ffn(i)
        for j in range(JL - 2):
            cp_out(j).wait()
        l_step(JL, False, True)

        k1, k2 = key_buf[0], key_buf[1]
        for sh in (4, 2, 1):
            o1, o2 = pltpu.roll(k1, sh, 0), pltpu.roll(k2, sh, 0)
            k2 = jnp.maximum(jnp.minimum(k1, o1), jnp.maximum(k2, o2))
            k1 = jnp.maximum(k1, o1)

        def score_of(k):
            hi = k & jnp.int32(-65536)
            return pltpu.bitcast(jnp.where(hi < 0, hi ^ 0x7FFF0000, hi), f32)

        i1s = jnp.minimum(0xFFFF - (k1[0, 0] & 0xFFFF), S - 1)
        i2s = jnp.minimum(0xFFFF - (k2[0, 0] & 0xFFFF), S - 1)

        sub = lax.broadcasted_iota(i32, (16, D), 0)
        sb, cb1, gb = (_rep(modv[i], 16) for i in (1, 2, 3))

        def adaln2(x1, stat):
            return (x1 - _wide(stat[:, 0:128], D)) * _wide(stat[:, 128:256], D) * cb1 + sb

        def pick(ref):
            sel = lax.broadcasted_iota(i32, (16, ref.shape[1]), 0) == 0
            return jnp.where(sel, ref[pl.ds(i1s, 1), :], ref[pl.ds(i2s, 1), :])

        xs = adaln2(pick(acc), pick(st2_buf)).astype(bf16)
        FC, lag = cfg["FC"], cfg["FLAG"]
        y = None
        act = []
        for c in range(F // FC + lag):
            if c < F // FC:
                cs = slice(c * FC, (c + 1) * FC)
                g = _rb(jnp.dot(xs, wg[:, cs], preferred_element_type=f32))
                u = _rb(jnp.dot(xs, wu[:, cs], preferred_element_type=f32))
                act.append((_rb(g * jax.nn.sigmoid(g)) * u).astype(bf16))
            if c >= lag:
                d = jnp.dot(act[c - lag], wd[(c - lag) * FC:(c - lag + 1) * FC, :],
                            preferred_element_type=f32)
                y = d if y is None else y + d
        y = _rb(y)
        ya = _rb(y[0:1, :] * _wide(_rb(jax.nn.sigmoid(score_of(k1[0:1, :]))), D))
        yb = _rb(y[1:2, :] * _wide(_rb(jax.nn.sigmoid(score_of(k2[0:1, :]))), D))

        g1 = pl.multiple_of((i1s >> 4) << 4, 16)
        g2 = pl.multiple_of((i2s >> 4) << 4, 16)
        for t, g0 in enumerate((g1, g2)):
            rid = sub + g0
            x1 = acc[pl.ds(g0, 16), :]
            upd = jnp.where(rid == i1s, ya, 0.0) + jnp.where(rid == i2s, yb, 0.0)
            fix[t] = (x1 + gb * (adaln2(x1, st2_buf[pl.ds(g0, 16), :]) + upd)).astype(bf16)

        for j in range(JL - 2, JL):
            cp_out(j).wait()

        def cp_fix(t, g0):
            return pltpu.make_async_copy(fix.at[t], out_hbm.at[pl.ds(g0, 16), :], sem_fix.at[t])

        cp_fix(0, g1).start()

        @pl.when(g2 != g1)
        def _():
            cp_fix(1, g2).start()
            cp_fix(1, g2).wait()
        cp_fix(0, g1).wait()

    return kernel


_CFG = dict(FC=256, FLAG=2, T0=256, TL=256, NRING=4, MCH=128, R0=8,  LORD='BAbQSa', LAG=100, LCNT='000000000055555520', LC0='088880')


def _build(A_x, A_k_cache, A_v_cache, A_wq, A_wo, B_w_r, B_w_gate, B_w_up, B_w_down, c, w_mod,
           **over):
    B, S, D = A_x.shape
    _, H, SK, DH = A_k_cache.shape
    F = B_w_gate.shape[1]
    assert B == 1
    cfg = dict(_CFG, **over)
    T0, TL, NRING = cfg["T0"], cfg["TL"], cfg["NRING"]
    MC = (4 * D) // H
    kernel = _make_kernel(S, D, H, DH, SK, F, cfg)
    scratch = [
        pltpu.VMEM((S, D), bf16),
        pltpu.VMEM((S // 2, D), u32),
        pltpu.VMEM((S, D), f32),
        pltpu.VMEM((S, SK), f32),
        pltpu.VMEM((S, 128), f32),
        pltpu.VMEM((TL, SK), f32),
        pltpu.VMEM((TL, 128), f32),
        pltpu.VMEM((2, T0, 128), f32),
        pltpu.VMEM((S, 256), f32),
        pltpu.VMEM((NRING, SK, DH), bf16),
        pltpu.VMEM((NRING, SK, DH), bf16),
        pltpu.VMEM((NRING, D, DH), bf16),
        pltpu.VMEM((NRING, DH, D), bf16),
        pltpu.VMEM((NRING, D, MC), bf16),
        pltpu.VMEM((D, 2 * D), bf16),
        pltpu.VMEM((1, D), bf16),
        pltpu.VMEM((D,), bf16),
        pltpu.VMEM((D, 128), f32),
        pltpu.VMEM((8, 2 * D), f32),
        pltpu.VMEM((H, 1, MC), f32),
        pltpu.VMEM((9, 8, D), f32),
        pltpu.VMEM((D, F), bf16),
        pltpu.VMEM((D, F), bf16),
        pltpu.VMEM((F, D), bf16),
        pltpu.VMEM((S, D), bf16),
        pltpu.VMEM((2, 8, 128), i32),
        pltpu.VMEM((2, 16, D), bf16),
        pltpu.SemaphoreType.DMA((sum(_sem_sizes(S, D, cfg)),)),
    ]
    any_spec = pl.BlockSpec(memory_space=pl.ANY)
    out = pl.pallas_call(
        kernel,
        out_shape=jax.ShapeDtypeStruct((S, D), bf16),
        in_specs=[any_spec] * 11,
        out_specs=any_spec,
        scratch_shapes=scratch,
        compiler_params=pltpu.CompilerParams(vmem_limit_bytes=124 * 1024 * 1024,
                                             disable_bounds_checks=True,
                                             disable_semaphore_checks=True),
    )(A_x.reshape(S, D), A_k_cache.reshape(H, SK, DH), A_v_cache.reshape(H, SK, DH),
      A_wq, A_wo, B_w_r, B_w_gate, B_w_up, B_w_down, c, w_mod)
    return out.reshape(B, S, D)


@jax.jit
def pallas_adaLN_cond__mha_block_cached__moe_arch_mod__prompt_kernel(
    A_x: jax.Array,
    A_k_cache: jax.Array,
    A_v_cache: jax.Array,
    A_wq: jax.Array,
    A_wo: jax.Array,
    B_x: jax.Array,
    B_w_r: jax.Array,
    B_w_gate: jax.Array,
    B_w_up: jax.Array,
    B_w_down: jax.Array,
    c: jax.Array,
    w_mod: jax.Array,
):
    del B_x
    return _build(A_x, A_k_cache, A_v_cache, A_wq, A_wo, B_w_r, B_w_gate, B_w_up, B_w_down,
                  c, w_mod)
```

```python
import jax
import jax.numpy as jnp
from jax import lax
import jax.experimental.pallas as pl
import jax.experimental.pallas.tpu as pltpu

f32 = jnp.float32
bf16 = jnp.bfloat16
u32 = jnp.uint32
i32 = jnp.int32

_NT = (((1,), (1,)), ((), ()))
_LOG2E = 1.4426950408889634
_EPS = 1e-5
_IMIN = -2 ** 31


def _rb(v):
    return v.astype(bf16).astype(f32)


def _rep(v, n):
    return v if n == 8 else jnp.tile(v, (n // 8, 1))


def _wide(v, w):
    return jnp.tile(v, (1, w // 128))


def _zero_of(v):
    bits = pltpu.bitcast(v, u32)
    return pltpu.bitcast(lax.shift_right_logical(lax.shift_right_logical(bits, jnp.uint32(31)),
                                                 jnp.uint32(1)), f32)


class _Pace:
    def __init__(self, chunks, counts):
        self.chunks = list(chunks)
        self.counts = [int(ch, 36) for ch in counts]
        assert sum(self.counts) == len(self.chunks), (counts, len(self.chunks))

    def done(self, res):
        n = self.counts.pop(0)
        for i in range(n):
            r0 = (i * res.shape[0] // n) // 8 * 8
            self.chunks.pop(0)(_zero_of(res[r0:r0 + 8, 0:128]))


def _tiles(v):
    return [v[:, c * 128:(c + 1) * 128] for c in range(v.shape[1] // 128)]


def _fold(op, parts):
    out = parts[0]
    for p in parts[1:]:
        out = op(out, p)
    return out


def _lane_sum(v):
    return jnp.broadcast_to(jnp.sum(v, axis=-1, keepdims=True), v.shape)


def _row_stats(xf, tok=None):
    d = xf.shape[-1]
    ts = _tiles(xf)
    nt = len(ts)
    if tok is not None:
        ts = [ts[0] + tok] + ts[1:]
    mu = _fold(jnp.add, ts) * (1.0 / nt)
    m2 = _fold(jnp.add, [(t - mu) * (t - mu) for t in ts])
    mean = _lane_sum(mu) * (1.0 / 128)
    dm = mu - mean
    var = _lane_sum(m2 + (dm * dm) * float(nt)) * (1.0 / d)
    return mean, lax.rsqrt(var + _EPS)


def _sem_sizes(S, D, cfg):
    j0 = S // cfg["T0"]
    return [2, D // cfg["MCH"], j0, j0, 16, 5, 3, S // cfg["TL"], 2]


def _make_kernel(S, D, H, DH, SK, F, cfg):
    T0, TB, TL, MCH = cfg["T0"], cfg["TB"], cfg["TL"], cfg["MCH"]
    J0 = S // T0
    JL = S // TL
    qscale = DH ** -0.5 * _LOG2E
    n_mch = D // MCH
    PW = D // J0
    G = cfg["G"]
    NB = H - G
    MC = (4 * D) // H
    W = 512
    assert PW % 128 == 0 and 2 <= G <= 4

    def kernel(x_hbm, k_hbm, v_hbm, wq_hbm, wo_hbm, wr_hbm, wg_hbm, wu_hbm, wd_hbm,
               c_hbm, wmod_hbm, out_hbm,
               x_buf, h_buf, acc, s_buf, m_buf, s2_buf, m2_buf, s3_buf, m3_buf, s4_buf, m4_buf,
               st_buf, st2_buf,
               q_ring, qf_buf, bq_buf,
               kb, vb, wq0, wqb, wob, wmb, wca, wsa, c_buf, wr_buf, cb_buf, mod0, sar, modr, modv,
               wg, wu, wd, o_buf, key_buf, fix,
               sems):

        class _Sem:
            def __init__(self, base):
                self.base = base
                self.at = self

            def __getitem__(self, i):
                return sems.at[self.base + i]

        sizes = _sem_sizes(S, D, cfg)
        offs = [sum(sizes[:i]) for i in range(len(sizes))]
        (sem_small, sem_ca, sem_x, sem_sa, sem_first, sem_head,
         sem_ffn, sem_out, sem_fix) = (_Sem(o) for o in offs)

        def _mul(a, n):
            v = a * n
            return v if isinstance(a, int) else pl.multiple_of(v, n)

        def view(ref, j, t, n=1):
            return ref.at[pl.ds(_mul(j, t), n * t), :]

        def cp_c():
            return pltpu.make_async_copy(c_hbm, c_buf, sem_small.at[0])

        def cp_wr():
            return pltpu.make_async_copy(wr_hbm, wr_buf, sem_small.at[1])

        def cp_ca(i):
            return pltpu.make_async_copy(
                wmod_hbm.at[pl.ds(i * MCH, MCH), pl.ds(D, D)], view(wca, i, MCH), sem_ca.at[i])

        def cp_sa(j):
            return pltpu.make_async_copy(
                wmod_hbm.at[:, pl.ds(_mul(j, PW), PW)], wsa.at[j], sem_sa.at[j])

        def cp_x(j):
            return pltpu.make_async_copy(view(x_hbm, j, T0), view(x_buf, j, T0), sem_x.at[j])

        def cp_wq0():
            return pltpu.make_async_copy(wq_hbm.at[:, pl.ds(0, G * DH)], wq0, sem_first.at[0])

        def cp_k(h, sem=None):
            return pltpu.make_async_copy(k_hbm.at[h], kb.at[h & 3],
                                         sem_head.at[0] if sem is None else sem)

        def cp_wq(h):
            src = h if isinstance(h, int) else jnp.minimum(h, H - 1)
            return pltpu.make_async_copy(wq_hbm.at[:, pl.ds(_mul(src, DH), DH)], wqb.at[h & 1],
                                         sem_head.at[1])

        def cp_v(h, sem=None):
            return pltpu.make_async_copy(v_hbm.at[h], vb.at[h & 3],
                                         sem_head.at[2] if sem is None else sem)

        def cp_wo(h, sem=None):
            return pltpu.make_async_copy(view(wo_hbm, h, DH), wob.at[h & 3],
                                         sem_head.at[3] if sem is None else sem)

        def wm_slot(p):
            return p - NB + 1 if (isinstance(p, int) and p > NB) else p & 1

        def cp_wm(p):
            extra = isinstance(p, int) and p > NB
            return pltpu.make_async_copy(
                wmod_hbm.at[:, pl.ds(_mul(p + (2 * D) // MC, MC), MC)], wmb.at[wm_slot(p)],
                sem_first.at[4 + p - NB] if extra else sem_head.at[4])

        ffn = ((wg_hbm, wg), (wu_hbm, wu), (wd_hbm, wd))

        def start_ffn_piece(p):
            for i, (src, dst) in enumerate(ffn):
                n = src.shape[0] // H
                pltpu.make_async_copy(view(src, p, n), view(dst, p, n), sem_ffn.at[i]).start()

        def wait_ffn():
            for i, (src, dst) in enumerate(ffn):
                pltpu.make_async_copy(src, dst, sem_ffn.at[i]).wait()

        def cp_out(j):
            return pltpu.make_async_copy(view(o_buf, j, TL), view(out_hbm, j, TL), sem_out.at[j])

        def head_copies(h):
            return [cp_wq(h + G), cp_k(h + G - 1), cp_wo(h), cp_wm(h), cp_v(h)]

        def ln1_chunks(xv, sv):
            def chunk(off):
                def f(tok=None):
                    mean, inv = _row_stats(xv[off:off + 8, :].astype(f32), tok)
                    sv[off:off + 8, 0:128] = mean
                    sv[off:off + 8, 128:256] = inv
                return f
            return [chunk(off) for off in range(0, T0, 8)]

        def ln1_scaled(x, stat, cs, tok=None):
            w = x.shape[1]
            mean = stat[:, 0:128] if tok is None else stat[:, 0:128] + _rep(tok, x.shape[0])
            n = (x.astype(f32) - _wide(mean, w)) * _wide(stat[:, 128:256], w)
            return n * _rep(mod0[1, :, cs], x.shape[0])

        def qproj(h):
            q = None
            for c in range(D // W):
                cs = slice(c * W, (c + 1) * W)
                part = jnp.dot(pltpu.bitcast(h_buf[:, cs], bf16), wqb[h & 1, cs, :],
                               preferred_element_type=f32)
                q = part if q is None else q + part
            q_ring[h & 3] = pltpu.bitcast((q * qscale).astype(bf16), u32)

        def q_early(g, q):
            return ((q + _rep(bq_buf[:, g * DH:(g + 1) * DH], q.shape[0])) * qscale).astype(bf16)

        def scores(h, q, sv, mv, rec=None):
            mp = None
            for c in range(SK // W):
                cs = slice(c * W, (c + 1) * W)
                s = lax.dot_general(q, kb[h & 3, cs, :], _NT, preferred_element_type=f32)
                sv[:, cs] = s
                if rec is not None:
                    rec.done(s)
                mp = _fold(jnp.maximum, ([] if mp is None else [mp]) + _tiles(s))
            mv[...] = jnp.broadcast_to(jnp.max(mp, axis=-1, keepdims=True), mp.shape)

        def pv(h, sv, mv, rec=None):
            o = lp = None
            for c in range(SK // W):
                cs = slice(c * W, (c + 1) * W)
                m = mv[...]
                if c >= cfg["LD"] and sv.shape[0] == S:
                    m = m + _zero_of(lp)
                p = jnp.exp2(sv[:, cs] - _wide(m, W))
                lp = _fold(jnp.add, ([] if lp is None else [lp]) + _tiles(p))
                d = jnp.dot(p.astype(bf16), vb[h & 3, cs, :], preferred_element_type=f32)
                o = d if o is None else o + d
                if rec is not None:
                    rec.done(d)
            l = jnp.sum(lp, axis=-1, keepdims=True)
            r = pl.reciprocal(l, approx=True)
            r = r * (2.0 - l * r)
            return (o * r).astype(bf16)

        def oproj(hos, av, xv=None, rec=None):
            for c in range(D // W):
                cs = slice(c * W, (c + 1) * W)
                a = av[:, cs]
                for h, o in hos:
                    if not isinstance(h, int):
                        a = jnp.where(h > 0, a, 0.0)
                    d = jnp.dot(o, wob[h & 3, :, cs], preferred_element_type=f32)
                    if rec is not None:
                        rec.done(d)
                    a = a + d
                if xv is not None:
                    a = xv[:, cs].astype(f32) + _rep(modv[0, :, cs], a.shape[0]) * a
                av[:, cs] = a

        def matvec(wv, tok=None):
            n = wv.shape[1]
            NCH = cfg['NCH']
            parts = [None if tok is None else _wide(tok, n)] * NCH
            for r in range(0, D, 16):
                t = wv[r:r + 16, :].astype(f32) * _wide(cb_buf[r:r + 16, :], n)
                for e in range(2):
                    i = (r // 8 + e) % NCH
                    te = t[e * 8:(e + 1) * 8, :]
                    parts[i] = te if parts[i] is None else parts[i] + te
            return _rb(jnp.sum(_fold(jnp.add, parts), axis=0, keepdims=True))

        def mod_piece(p, tok=None):
            modr[p] = matvec(wmb.at[wm_slot(p)], tok)

        def finish_mod():
            n = D // MC
            ga, sb, cb, gb = (jnp.concatenate([modr[i * n + t] for t in range(n)], axis=-1)
                              for i in range(4))
            cb1 = _rb(1.0 + cb)
            wr = wr_buf[...].astype(f32).reshape(1, D)
            a = cb1 * wr
            a0 = jnp.broadcast_to(jnp.sum(a, axis=-1, keepdims=True), (1, D))
            b0 = jnp.broadcast_to(jnp.sum(sb * wr, axis=-1, keepdims=True), (1, D))
            for i, v in enumerate((ga, sb, cb1, gb, a, gb * cb1, gb * sb, a0, b0)):
                modv[i] = jnp.broadcast_to(v, (8, D))

        def epi_chunks(j, x1v, ov):
            sub = lax.broadcasted_iota(i32, (8, 128), 0)
            low = (0xFFFF - j * TL) - sub
            sv = view(st2_buf, j, TL)
            st = {}

            def chunk(off):
                def f(tok=None):
                    if off == 0:
                        st["k1"], st["k2"] = key_buf[0], key_buf[1]
                    x1 = x1v[off:off + 8, :]
                    mean, inv = _row_stats(x1, tok)
                    sv[off:off + 8, 0:128] = mean
                    sv[off:off + 8, 128:256] = inv
                    xa = _tiles(x1 * modv[4])
                    if tok is not None:
                        xa[0] = xa[0] + tok
                    ra = _lane_sum(_fold(jnp.add, xa))
                    r = inv * (ra - mean * modv[7, :, 0:128]) + modv[8, :, 0:128]
                    res = x1 + ((x1 - _wide(mean, D)) * (_wide(inv, D) * modv[5]) + modv[6])
                    ov[off:off + 8, :] = res.astype(bf16)
                    bits = pltpu.bitcast(_rb(r) + 0.0, i32)
                    key = jnp.where(bits < 0, bits ^ 0x7FFF0000, bits) | (low - off)
                    st["k2"] = jnp.maximum(st["k2"], jnp.minimum(st["k1"], key))
                    st["k1"] = jnp.maximum(st["k1"], key)
                    if off + 8 == TL:
                        key_buf[0], key_buf[1] = st["k1"], st["k2"]
                return f
            return [chunk(off) for off in range(0, TL, 8)]

        cp_c().start()
        cp_x(0).start()
        cp_wq0().start()
        for i in range(n_mch):
            cp_ca(i).start()
        for j in range(J0):
            if j + 1 < J0:
                cp_x(j + 1).start()
            cp_sa(j).start()
        for h in range(G - 1):
            cp_k(h, sem_first.at[1 + h]).start()
        for cp in head_copies(0):
            cp.start()

        cp_c().wait()
        cf = c_buf[...].astype(f32)
        sc = _rb(cf * jax.nn.sigmoid(cf))
        cb_buf[...] = jnp.transpose(jnp.broadcast_to(sc, (128, D)))
        key_buf[...] = jnp.full(key_buf.shape, _IMIN, i32)
        cp_x(0).wait()
        for ch in ln1_chunks(view(x_buf, 0, T0), view(st_buf, 0, T0)):
            ch()
        cp_wq0().wait()

        part = None
        for i in range(n_mch):
            cp_ca(i).wait()
            scb = jnp.broadcast_to(sc[:, i * MCH:(i + 1) * MCH], (16, MCH)).astype(bf16)
            d = jnp.dot(scb, wca[i * MCH:(i + 1) * MCH, :], preferred_element_type=f32)
            part = d if part is None else part + d
        mod0[1] = _rb(1.0 + _rb(part[0:8, :]))

        def p0a_body(j, carry):
            @pl.when(j + 1 < J0)
            def _():
                cp_x(j + 1).wait()
            cp_sa(j).wait()
            jn = jnp.minimum(j + 1, J0 - 1)
            xv, stat = view(x_buf, j, T0), view(st_buf, j, T0)[...]
            rec = _Pace(ln1_chunks(view(x_buf, jn, T0), view(st_buf, jn, T0)), cfg["LC0"])
            qs = [None] * G
            for c in range(D // W):
                cs = slice(c * W, (c + 1) * W)
                hh = ln1_scaled(xv[:, cs], stat, cs).astype(bf16)
                for g in range(G):
                    part = jnp.dot(hh, wq0[cs, g * DH:(g + 1) * DH], preferred_element_type=f32)
                    qs[g] = part if c == 0 else qs[g] + part
                    rec.done(part)
            for g in range(G):
                qf_buf[g, pl.ds(_mul(j, T0), T0), :] = qs[g]
            sar[j] = matvec(wsa.at[j])
            return carry
        lax.fori_loop(0, J0, p0a_body, 0)

        sa = jnp.concatenate([sar[j] for j in range(J0)], axis=-1)
        mod0[0] = jnp.broadcast_to(sa, (8, D))
        bq_buf[...] = jnp.dot(jnp.broadcast_to(sa, (16, D)).astype(bf16), wq0[...],
                              preferred_element_type=f32)[0:8, :]
        cp_k(0, sem_first.at[1]).wait()

        def p0b_body(j, carry):
            RB = cfg["RB"]
            xv, sv, hv = view(x_buf, j, TB), view(st_buf, j, TB), view(h_buf, j, TB // 2)
            qfv = [view(qf_buf.at[g], j, TB) for g in range(G)]
            qrv = [view(q_ring.at[g], j, TB // 2) for g in range(G)]

            def chunk(off):
                def f(tok):
                    hh = (ln1_scaled(xv[off:off + RB, :], sv[off:off + RB, :], slice(0, D), tok)
                          + _rep(mod0[0], RB)).astype(bf16)
                    hv[off // 2:(off + RB) // 2, :] = pltpu.bitcast(hh, u32)
                    for g in range(1, G):
                        qg = q_early(g, qfv[g][off:off + RB, :] + _rep(tok, RB))
                        qrv[g][off // 2:(off + RB) // 2, :] = pltpu.bitcast(qg, u32)
                return f
            rec = _Pace([chunk(off) for off in range(0, TB, RB)], cfg["LCB"])
            scores(0, q_early(0, qfv[0][...]), view(s_buf, j, TB), view(m_buf, j, TB), rec=rec)
            return carry
        lax.fori_loop(0, S // TB, p0b_body, 0)

        def main_body(h, carry):
            qproj(h + G)
            start_ffn_piece(h)
            for cp in head_copies(h + 1):
                cp.start()
            o = pv(h, s_buf, m_buf)
            rec = _Pace([lambda tok: mod_piece(h, tok)], "1000")
            scores(h + 1, pltpu.bitcast(q_ring[(h + 1) & 3], bf16), s_buf, m_buf, rec=rec)
            oproj([(h, o)], acc)
            for cp in head_copies(h + 1):
                cp.wait()
            return carry
        for h in range(1, G - 1):
            cp_k(h, sem_first.at[1 + h]).wait()
        for cp in head_copies(0):
            cp.wait()
        cp_wr().start()
        for p in range(NB + 1, H):
            cp_wm(p).start()
        for p in range(NB, H):
            start_ffn_piece(p)
        lax.fori_loop(0, NB, main_body, 0)

        ha = NB
        rest = list(zip(range(NB + 1, H), (s2_buf, s3_buf, s4_buf), (m2_buf, m3_buf, m4_buf)))
        late = []
        for n, (h, _, _) in enumerate(rest):
            late += [cp_v(h, sem_first.at[8 + 2 * n]), cp_wo(h, sem_first.at[9 + 2 * n])]
        for cp in late:
            cp.start()
        cp_wr().wait()
        for p in range(NB + 1, H):
            cp_wm(p).wait()

        def l_step(j, do_x, do_y):
            if do_x and do_y:
                aw = view(acc, j - 1, TL, 2)
                ay, ax = aw.at[0:TL, :], aw.at[TL:2 * TL, :]
            elif do_x:
                ax = view(acc, j, TL)
            else:
                ay = view(acc, j - 1, TL)
            rec = None
            if do_y:
                chunks = epi_chunks(j - 1, ay, view(o_buf, j - 1, TL))
                os_ = [(h, pv(h, sv, mv)) for h, sv, mv in rest]
            if do_x:
                oa = pv(ha, view(s_buf, j, TL), view(m_buf, j, TL))
            if do_y:
                oproj(os_, ay, view(x_buf, j - 1, TL))
            if do_x:
                if do_y:
                    rec = _Pace(chunks, cfg["LCNT"])
                for h, sv, mv in rest:
                    q = pltpu.bitcast(view(q_ring.at[h & 3], j, TL // 2)[...], bf16)
                    scores(h, q, sv, mv, rec=rec)
                oproj([(ha, oa)], ax, rec=rec)
            if do_y:
                if not do_x:
                    for ch in chunks:
                        ch()
                cp_out(j - 1).start()

        for p in range(NB, H):
            mod_piece(p)
        finish_mod()
        l_step(0, True, False)
        for cp in late:
            cp.wait()

        def pl_body(j, carry):
            l_step(j, True, True)
            return carry
        lax.fori_loop(1, JL, pl_body, 0)
        wait_ffn()
        for j in range(JL - 2):
            cp_out(j).wait()
        l_step(JL, False, True)

        k1, k2 = key_buf[0], key_buf[1]
        for sh in (4, 2, 1):
            o1, o2 = pltpu.roll(k1, sh, 0), pltpu.roll(k2, sh, 0)
            k2 = jnp.maximum(jnp.minimum(k1, o1), jnp.maximum(k2, o2))
            k1 = jnp.maximum(k1, o1)

        def score_of(k):
            hi = k & jnp.int32(-65536)
            return pltpu.bitcast(jnp.where(hi < 0, hi ^ 0x7FFF0000, hi), f32)

        i1s = jnp.minimum(0xFFFF - (k1[0, 0] & 0xFFFF), S - 1)
        i2s = jnp.minimum(0xFFFF - (k2[0, 0] & 0xFFFF), S - 1)

        sub = lax.broadcasted_iota(i32, (16, D), 0)
        sb, cb1, gb = (_rep(modv[i], 16) for i in (1, 2, 3))

        def adaln2(x1, stat):
            return (x1 - _wide(stat[:, 0:128], D)) * _wide(stat[:, 128:256], D) * cb1 + sb

        def pick(ref):
            sel = lax.broadcasted_iota(i32, (16, ref.shape[1]), 0) == 0
            return jnp.where(sel, ref[pl.ds(i1s, 1), :], ref[pl.ds(i2s, 1), :])

        xs = adaln2(pick(acc), pick(st2_buf)).astype(bf16)
        FC, lag = cfg["FC"], 2
        y = None
        act = []
        for c in range(F // FC + lag):
            if c < F // FC:
                cs = slice(c * FC, (c + 1) * FC)
                g = _rb(jnp.dot(xs, wg[:, cs], preferred_element_type=f32))
                u = _rb(jnp.dot(xs, wu[:, cs], preferred_element_type=f32))
                act.append((_rb(g * jax.nn.sigmoid(g)) * u).astype(bf16))
            if c >= lag:
                d = jnp.dot(act[c - lag], wd[(c - lag) * FC:(c - lag + 1) * FC, :],
                            preferred_element_type=f32)
                y = d if y is None else y + d
        y = _rb(y)
        ya = _rb(y[0:1, :] * _wide(_rb(jax.nn.sigmoid(score_of(k1[0:1, :]))), D))
        yb = _rb(y[1:2, :] * _wide(_rb(jax.nn.sigmoid(score_of(k2[0:1, :]))), D))

        g1 = pl.multiple_of((i1s >> 4) << 4, 16)
        g2 = pl.multiple_of((i2s >> 4) << 4, 16)
        for t, g0 in enumerate((g1, g2)):
            rid = sub + g0
            x1 = acc[pl.ds(g0, 16), :]
            upd = jnp.where(rid == i1s, ya, 0.0) + jnp.where(rid == i2s, yb, 0.0)
            fix[t] = (x1 + gb * (adaln2(x1, st2_buf[pl.ds(g0, 16), :]) + upd)).astype(bf16)

        for j in range(JL - 2, JL):
            cp_out(j).wait()

        def cp_fix(t, g0):
            return pltpu.make_async_copy(fix.at[t], out_hbm.at[pl.ds(g0, 16), :], sem_fix.at[t])

        cp_fix(0, g1).start()

        @pl.when(g2 != g1)
        def _():
            cp_fix(1, g2).start()
            cp_fix(1, g2).wait()
        cp_fix(0, g1).wait()

    return kernel


_CFG = dict(FC=256, T0=256, TL=256, MCH=128, LD=9, TB=1024, RB=16, NCH=1,
            G=4, LCNT='33333333332000', LC0='28860800', LCB='gggg')


def _build(A_x, A_k_cache, A_v_cache, A_wq, A_wo, B_w_r, B_w_gate, B_w_up, B_w_down, c, w_mod,
           **over):
    B, S, D = A_x.shape
    _, H, SK, DH = A_k_cache.shape
    F = B_w_gate.shape[1]
    assert B == 1
    cfg = dict(_CFG, **over)
    T0, TL, G = cfg["T0"], cfg["TL"], cfg["G"]
    MC = (4 * D) // H
    kernel = _make_kernel(S, D, H, DH, SK, F, cfg)
    scratch = [
        pltpu.VMEM((S, D), bf16),
        pltpu.VMEM((S // 2, D), u32),
        pltpu.VMEM((S, D), f32),
        pltpu.VMEM((S, SK), f32),
        pltpu.VMEM((S, 128), f32),
        pltpu.VMEM((TL, SK), f32),
        pltpu.VMEM((TL, 128), f32),
        pltpu.VMEM((TL, SK), f32),
        pltpu.VMEM((TL, 128), f32),
        pltpu.VMEM((TL, SK), f32),
        pltpu.VMEM((TL, 128), f32),
        pltpu.VMEM((S, 256), f32),
        pltpu.VMEM((S, 256), f32),
        pltpu.VMEM((4, S // 2, DH), u32),
        pltpu.VMEM((G, S, DH), f32),
        pltpu.VMEM((8, G * DH), f32),
        pltpu.VMEM((4, SK, DH), bf16),
        pltpu.VMEM((4, SK, DH), bf16),
        pltpu.VMEM((D, G * DH), bf16),
        pltpu.VMEM((2, D, DH), bf16),
        pltpu.VMEM((4, DH, D), bf16),
        pltpu.VMEM((G + 1, D, MC), bf16),
        pltpu.VMEM((D, D), bf16),
        pltpu.VMEM((S // T0, D, D // (S // T0)), bf16),
        pltpu.VMEM((1, D), bf16),
        pltpu.VMEM((D,), bf16),
        pltpu.VMEM((D, 128), f32),
        pltpu.VMEM((2, 8, D), f32),
        pltpu.VMEM((S // T0, 1, D // (S // T0)), f32),
        pltpu.VMEM((H, 1, MC), f32),
        pltpu.VMEM((9, 8, D), f32),
        pltpu.VMEM((D, F), bf16),
        pltpu.VMEM((D, F), bf16),
        pltpu.VMEM((F, D), bf16),
        pltpu.VMEM((S, D), bf16),
        pltpu.VMEM((2, 8, 128), i32),
        pltpu.VMEM((2, 16, D), bf16),
        pltpu.SemaphoreType.DMA((sum(_sem_sizes(S, D, cfg)),)),
    ]
    any_spec = pl.BlockSpec(memory_space=pl.ANY)
    out = pl.pallas_call(
        kernel,
        out_shape=jax.ShapeDtypeStruct((S, D), bf16),
        in_specs=[any_spec] * 11,
        out_specs=any_spec,
        scratch_shapes=scratch,
        compiler_params=pltpu.CompilerParams(vmem_limit_bytes=112 * 1024 * 1024,
                                             disable_bounds_checks=True,
                                             disable_semaphore_checks=True),
    )(A_x.reshape(S, D), A_k_cache.reshape(H, SK, DH), A_v_cache.reshape(H, SK, DH),
      A_wq, A_wo, B_w_r, B_w_gate, B_w_up, B_w_down, c, w_mod)
    return out.reshape(B, S, D)


@jax.jit
def pallas_adaLN_cond__mha_block_cached__moe_arch_mod__prompt_kernel(
    A_x: jax.Array,
    A_k_cache: jax.Array,
    A_v_cache: jax.Array,
    A_wq: jax.Array,
    A_wo: jax.Array,
    B_x: jax.Array,
    B_w_r: jax.Array,
    B_w_gate: jax.Array,
    B_w_up: jax.Array,
    B_w_down: jax.Array,
    c: jax.Array,
    w_mod: jax.Array,
):
    del B_x
    return _build(A_x, A_k_cache, A_v_cache, A_wq, A_wo, B_w_r, B_w_gate, B_w_up, B_w_down,
                  c, w_mod)
```

```python
import jax
import jax.numpy as jnp
from jax import lax
import jax.experimental.pallas as pl
import jax.experimental.pallas.tpu as pltpu

f32 = jnp.float32
bf16 = jnp.bfloat16
u32 = jnp.uint32
i32 = jnp.int32

_NT = (((1,), (1,)), ((), ()))
_LOG2E = 1.4426950408889634
_EPS = 1e-5
_IMIN = -2 ** 31


def _rb(v):
    return v.astype(bf16).astype(f32)


def _rep(v, n):
    return v if n == 8 else jnp.tile(v, (n // 8, 1))


def _wide(v, w):
    return jnp.tile(v, (1, w // 128))


def _zero_of(v):
    bits = pltpu.bitcast(v, u32)
    return pltpu.bitcast(lax.shift_right_logical(lax.shift_right_logical(bits, jnp.uint32(31)),
                                                 jnp.uint32(1)), f32)


class _Pace:
    def __init__(self, chunks, counts):
        self.chunks = list(chunks)
        self.counts = [int(ch, 36) for ch in counts]
        assert sum(self.counts) == len(self.chunks), (counts, len(self.chunks))

    def done(self, res):
        n = self.counts.pop(0)
        for i in range(n):
            r0 = (i * res.shape[0] // n) // 8 * 8
            self.chunks.pop(0)(_zero_of(res[r0:r0 + 8, 0:128]))


def _tiles(v):
    return [v[:, c * 128:(c + 1) * 128] for c in range(v.shape[1] // 128)]


def _fold(op, parts):
    out = parts[0]
    for p in parts[1:]:
        out = op(out, p)
    return out


def _lane_sum(v):
    return jnp.broadcast_to(jnp.sum(v, axis=-1, keepdims=True), v.shape)


def _row_stats(xf, tok=None):
    d = xf.shape[-1]
    ts = _tiles(xf)
    nt = len(ts)
    if tok is not None:
        ts = [ts[0] + tok] + ts[1:]
    mu = _fold(jnp.add, ts) * (1.0 / nt)
    m2 = _fold(jnp.add, [(t - mu) * (t - mu) for t in ts])
    mean = _lane_sum(mu) * (1.0 / 128)
    dm = mu - mean
    var = _lane_sum(m2 + (dm * dm) * float(nt)) * (1.0 / d)
    return mean, lax.rsqrt(var + _EPS)


def _sem_sizes(S, D, cfg):
    j0 = S // cfg["T0"]
    return [2, D // cfg["MCH"], j0, j0, 16, 5, 3, S // cfg["TL"], 2]


def _make_kernel(S, D, H, DH, SK, F, cfg):
    T0, TB, TL, MCH = cfg["T0"], cfg["TB"], cfg["TL"], cfg["MCH"]
    J0 = S // T0
    JL = S // TL
    qscale = DH ** -0.5 * _LOG2E
    n_mch = D // MCH
    PW = D // J0
    G = cfg["G"]
    NB = H - G
    MC = (4 * D) // H
    W = 512
    assert PW % 128 == 0 and 2 <= G <= 4

    def kernel(x_hbm, k_hbm, v_hbm, wq_hbm, wo_hbm, wr_hbm, wg_hbm, wu_hbm, wd_hbm,
               c_hbm, wmod_hbm, out_hbm,
               x_buf, h_buf, acc, s_buf, m_buf, s2_buf, m2_buf, s3_buf, m3_buf, s4_buf, m4_buf,
               st_buf, st2_buf,
               q_ring, qf_buf, bq_buf,
               kb, vb, wq0, wqb, wob, wmb, wca, wsa, c_buf, wr_buf, cb_buf, mod0, sar, modr, modv,
               wg, wu, wd, o_buf, key_buf, fix,
               sems):

        class _Sem:
            def __init__(self, base):
                self.base = base
                self.at = self

            def __getitem__(self, i):
                return sems.at[self.base + i]

        sizes = _sem_sizes(S, D, cfg)
        offs = [sum(sizes[:i]) for i in range(len(sizes))]
        (sem_small, sem_ca, sem_x, sem_sa, sem_first, sem_head,
         sem_ffn, sem_out, sem_fix) = (_Sem(o) for o in offs)

        def _mul(a, n):
            v = a * n
            return v if isinstance(a, int) else pl.multiple_of(v, n)

        def view(ref, j, t, n=1):
            return ref.at[pl.ds(_mul(j, t), n * t), :]

        def cp_c():
            return pltpu.make_async_copy(c_hbm, c_buf, sem_small.at[0])

        def cp_wr():
            return pltpu.make_async_copy(wr_hbm, wr_buf, sem_small.at[1])

        def cp_ca(i):
            return pltpu.make_async_copy(
                wmod_hbm.at[pl.ds(i * MCH, MCH), pl.ds(D, D)], view(wca, i, MCH), sem_ca.at[i])

        def cp_sa(j):
            return pltpu.make_async_copy(
                wmod_hbm.at[:, pl.ds(_mul(j, PW), PW)], wsa.at[j], sem_sa.at[j])

        def cp_x(j):
            return pltpu.make_async_copy(view(x_hbm, j, T0), view(x_buf, j, T0), sem_x.at[j])

        def cp_wq0():
            return pltpu.make_async_copy(wq_hbm.at[:, pl.ds(0, G * DH)], wq0, sem_first.at[0])

        def cp_k(h, sem=None):
            return pltpu.make_async_copy(k_hbm.at[h], kb.at[h & 3],
                                         sem_head.at[0] if sem is None else sem)

        def cp_wq(h):
            src = h if isinstance(h, int) else jnp.minimum(h, H - 1)
            return pltpu.make_async_copy(wq_hbm.at[:, pl.ds(_mul(src, DH), DH)], wqb.at[h & 1],
                                         sem_head.at[1])

        def cp_v(h, sem=None):
            return pltpu.make_async_copy(v_hbm.at[h], vb.at[h & 3],
                                         sem_head.at[2] if sem is None else sem)

        def cp_wo(h, sem=None):
            return pltpu.make_async_copy(view(wo_hbm, h, DH), wob.at[h & 3],
                                         sem_head.at[3] if sem is None else sem)

        def wm_slot(p):
            return p - NB + 1 if (isinstance(p, int) and p > NB) else p & 1

        def cp_wm(p):
            extra = isinstance(p, int) and p > NB
            return pltpu.make_async_copy(
                wmod_hbm.at[:, pl.ds(_mul(p + (2 * D) // MC, MC), MC)], wmb.at[wm_slot(p)],
                sem_first.at[4 + p - NB] if extra else sem_head.at[4])

        ffn = ((wg_hbm, wg), (wu_hbm, wu), (wd_hbm, wd))

        def start_ffn_piece(p):
            for i, (src, dst) in enumerate(ffn):
                n = src.shape[0] // H
                pltpu.make_async_copy(view(src, p, n), view(dst, p, n), sem_ffn.at[i]).start()

        def wait_ffn():
            for i, (src, dst) in enumerate(ffn):
                pltpu.make_async_copy(src, dst, sem_ffn.at[i]).wait()

        def cp_out(j):
            return pltpu.make_async_copy(view(o_buf, j, TL), view(out_hbm, j, TL), sem_out.at[j])

        def head_copies(h):
            return [cp_wq(h + G), cp_k(h + G - 1), cp_wo(h + 2), cp_wm(h), cp_v(h + 2)]

        def ln1_chunks(xv, sv):
            def chunk(off):
                def f(tok=None):
                    mean, inv = _row_stats(xv[off:off + 8, :].astype(f32), tok)
                    sv[off:off + 8, 0:128] = mean
                    sv[off:off + 8, 128:256] = inv
                return f
            return [chunk(off) for off in range(0, T0, 8)]

        def ln1_scaled(x, stat, cs, tok=None):
            w = x.shape[1]
            mean = stat[:, 0:128] if tok is None else stat[:, 0:128] + _rep(tok, x.shape[0])
            n = (x.astype(f32) - _wide(mean, w)) * _wide(stat[:, 128:256], w)
            return n * _rep(mod0[1, :, cs], x.shape[0])

        def qproj(h):
            q = None
            for c in range(D // W):
                cs = slice(c * W, (c + 1) * W)
                part = jnp.dot(pltpu.bitcast(h_buf[:, cs], bf16), wqb[h & 1, cs, :],
                               preferred_element_type=f32)
                q = part if q is None else q + part
            q_ring[h & 3] = pltpu.bitcast((q * qscale).astype(bf16), u32)

        def q_early(g, q):
            return ((q + _rep(bq_buf[:, g * DH:(g + 1) * DH], q.shape[0])) * qscale).astype(bf16)

        def scores(h, q, sv, mv, rec=None, reload=False):
            mp = None
            for c in range(SK // W):
                cs = slice(c * W, (c + 1) * W)
                s = lax.dot_general(q, kb[h & 3, cs, :], _NT, preferred_element_type=f32)
                sv[:, cs] = s
                if rec is not None:
                    rec.done(s)
                if not reload:
                    mp = _fold(jnp.maximum, ([] if mp is None else [mp]) + _tiles(s))
            if reload:
                mp = _fold(jnp.maximum, _tiles(sv[...]))
            mv[...] = jnp.broadcast_to(jnp.max(mp, axis=-1, keepdims=True), mp.shape)

        def pv(h, sv, mv, rec=None):
            o = lp = None
            for c in range(SK // W):
                cs = slice(c * W, (c + 1) * W)
                m = mv[...]
                if c >= cfg["LD"] and sv.shape[0] == S:
                    m = m + _zero_of(lp)
                p = jnp.exp2(sv[:, cs] - _wide(m, W))
                lp = _fold(jnp.add, ([] if lp is None else [lp]) + _tiles(p))
                d = jnp.dot(p.astype(bf16), vb[h & 3, cs, :], preferred_element_type=f32)
                o = d if o is None else o + d
                if rec is not None:
                    rec.done(d)
            l = jnp.sum(lp, axis=-1, keepdims=True)
            r = pl.reciprocal(l, approx=True)
            r = r * (2.0 - l * r)
            return (o * r).astype(bf16)

        def oproj(hos, av, xv=None, rec=None):
            for c in range(D // W):
                cs = slice(c * W, (c + 1) * W)
                a = av[:, cs]
                for h, o in hos:
                    if not isinstance(h, int):
                        a = jnp.where(h > 0, a, 0.0)
                    d = jnp.dot(o, wob[h & 3, :, cs], preferred_element_type=f32)
                    if rec is not None:
                        rec.done(d)
                    a = a + d
                if xv is not None:
                    a = xv[:, cs].astype(f32) + _rep(modv[0, :, cs], a.shape[0]) * a
                av[:, cs] = a

        def matvec(wv, tok=None):
            n = wv.shape[1]
            NCH = cfg['NCH']
            parts = [None if tok is None else _wide(tok, n)] * NCH
            for r in range(0, D, 16):
                t = wv[r:r + 16, :].astype(f32) * _wide(cb_buf[r:r + 16, :], n)
                for e in range(2):
                    i = (r // 8 + e) % NCH
                    te = t[e * 8:(e + 1) * 8, :]
                    parts[i] = te if parts[i] is None else parts[i] + te
            return _rb(jnp.sum(_fold(jnp.add, parts), axis=0, keepdims=True))

        def mod_piece(p, tok=None):
            modr[p] = matvec(wmb.at[wm_slot(p)], tok)

        def finish_mod():
            n = D // MC
            ga, sb, cb, gb = (jnp.concatenate([modr[i * n + t] for t in range(n)], axis=-1)
                              for i in range(4))
            cb1 = _rb(1.0 + cb)
            wr = wr_buf[...].astype(f32).reshape(1, D)
            a = cb1 * wr
            a0 = jnp.broadcast_to(jnp.sum(a, axis=-1, keepdims=True), (1, D))
            b0 = jnp.broadcast_to(jnp.sum(sb * wr, axis=-1, keepdims=True), (1, D))
            for i, v in enumerate((ga, sb, cb1, gb, a, gb * cb1, gb * sb, a0, b0)):
                modv[i] = jnp.broadcast_to(v, (8, D))

        def epi_chunks(j, x1v, ov):
            sub = lax.broadcasted_iota(i32, (8, 128), 0)
            low = (0xFFFF - j * TL) - sub
            sv = view(st2_buf, j, TL)
            st = {}

            def chunk(off):
                def f(tok=None):
                    if off == 0:
                        st["k1"], st["k2"] = key_buf[0], key_buf[1]
                    x1 = x1v[off:off + 8, :]
                    mean, inv = _row_stats(x1, tok)
                    sv[off:off + 8, 0:128] = mean
                    sv[off:off + 8, 128:256] = inv
                    xa = _tiles(x1 * modv[4])
                    if tok is not None:
                        xa[0] = xa[0] + tok
                    ra = _lane_sum(_fold(jnp.add, xa))
                    r = inv * (ra - mean * modv[7, :, 0:128]) + modv[8, :, 0:128]
                    res = x1 + ((x1 - _wide(mean, D)) * (_wide(inv, D) * modv[5]) + modv[6])
                    ov[off:off + 8, :] = res.astype(bf16)
                    bits = pltpu.bitcast(_rb(r) + 0.0, i32)
                    key = jnp.where(bits < 0, bits ^ 0x7FFF0000, bits) | (low - off)
                    st["k2"] = jnp.maximum(st["k2"], jnp.minimum(st["k1"], key))
                    st["k1"] = jnp.maximum(st["k1"], key)
                    if off + 8 == TL:
                        key_buf[0], key_buf[1] = st["k1"], st["k2"]
                return f
            return [chunk(off) for off in range(0, TL, 8)]

        cp_c().start()
        cp_x(0).start()
        cp_wq0().start()
        for i in range(n_mch):
            cp_ca(i).start()
        for j in range(J0):
            if j + 1 < J0:
                cp_x(j + 1).start()
            cp_sa(j).start()
        for h in range(G - 1):
            cp_k(h, sem_first.at[1 + h]).start()
        early = []
        for h in range(2):
            early += [cp_v(h, sem_first.at[8 + 2 * h]), cp_wo(h, sem_first.at[9 + 2 * h])]
        for cp in early + head_copies(0):
            cp.start()

        cp_c().wait()
        cf = c_buf[...].astype(f32)
        sc = _rb(cf * jax.nn.sigmoid(cf))
        cb_buf[...] = jnp.transpose(jnp.broadcast_to(sc, (128, D)))
        key_buf[...] = jnp.full(key_buf.shape, _IMIN, i32)
        cp_x(0).wait()
        for ch in ln1_chunks(view(x_buf, 0, T0), view(st_buf, 0, T0)):
            ch()
        cp_wq0().wait()

        part = None
        for i in range(n_mch):
            cp_ca(i).wait()
            scb = jnp.broadcast_to(sc[:, i * MCH:(i + 1) * MCH], (16, MCH)).astype(bf16)
            d = jnp.dot(scb, wca[i * MCH:(i + 1) * MCH, :], preferred_element_type=f32)
            part = d if part is None else part + d
        mod0[1] = _rb(1.0 + _rb(part[0:8, :]))

        def p0a_body(j, carry):
            @pl.when(j + 1 < J0)
            def _():
                cp_x(j + 1).wait()
            cp_sa(j).wait()
            jn = jnp.minimum(j + 1, J0 - 1)
            xv, stat = view(x_buf, j, T0), view(st_buf, j, T0)[...]
            rec = _Pace(ln1_chunks(view(x_buf, jn, T0), view(st_buf, jn, T0)), cfg["LC0"])
            qs = [None] * G
            for c in range(D // W):
                cs = slice(c * W, (c + 1) * W)
                hh = ln1_scaled(xv[:, cs], stat, cs).astype(bf16)
                for g in range(G):
                    part = jnp.dot(hh, wq0[cs, g * DH:(g + 1) * DH], preferred_element_type=f32)
                    qs[g] = part if c == 0 else qs[g] + part
                    rec.done(part)
            for g in range(G):
                qf_buf[g, pl.ds(_mul(j, T0), T0), :] = qs[g]
            sar[j] = matvec(wsa.at[j])
            return carry
        lax.fori_loop(0, J0, p0a_body, 0)

        sa = jnp.concatenate([sar[j] for j in range(J0)], axis=-1)
        mod0[0] = jnp.broadcast_to(sa, (8, D))
        bq_buf[...] = jnp.dot(jnp.broadcast_to(sa, (16, D)).astype(bf16), wq0[...],
                              preferred_element_type=f32)[0:8, :]
        cp_k(0, sem_first.at[1]).wait()

        def p0b_body(j, carry):
            RB = cfg["RB"]
            xv, sv, hv = view(x_buf, j, TB), view(st_buf, j, TB), view(h_buf, j, TB // 2)
            qfv = [view(qf_buf.at[g], j, TB) for g in range(G)]
            qrv = [view(q_ring.at[g], j, TB // 2) for g in range(G)]

            def chunk(off):
                def f(tok):
                    hh = (ln1_scaled(xv[off:off + RB, :], sv[off:off + RB, :], slice(0, D), tok)
                          + _rep(mod0[0], RB)).astype(bf16)
                    hv[off // 2:(off + RB) // 2, :] = pltpu.bitcast(hh, u32)
                    for g in range(1, G):
                        qg = q_early(g, qfv[g][off:off + RB, :] + _rep(tok, RB))
                        qrv[g][off // 2:(off + RB) // 2, :] = pltpu.bitcast(qg, u32)
                return f
            rec = _Pace([chunk(off) for off in range(0, TB, RB)], cfg["LCB"])
            scores(0, q_early(0, qfv[0][...]), view(s_buf, j, TB), view(m_buf, j, TB), rec=rec,
                   reload=cfg['RLB'])
            return carry
        lax.fori_loop(0, S // TB, p0b_body, 0)

        def main_body(h, carry):
            qproj(h + G)
            start_ffn_piece(h)
            for cp in head_copies(h + 1):
                cp.start()
            o = pv(h, s_buf, m_buf)
            rec = _Pace([lambda tok: mod_piece(h, tok)], "1000")
            scores(h + 1, pltpu.bitcast(q_ring[(h + 1) & 3], bf16), s_buf, m_buf, rec=rec,
                   reload=cfg['RLM'])
            oproj([(h, o)], acc)
            for cp in head_copies(h + 1):
                cp.wait()
            return carry
        for h in range(1, G - 1):
            cp_k(h, sem_first.at[1 + h]).wait()
        for cp in early + head_copies(0):
            cp.wait()
        cp_wr().start()
        for p in range(NB + 1, H):
            cp_wm(p).start()
        for p in range(NB, H):
            start_ffn_piece(p)
        lax.fori_loop(0, NB, main_body, 0)

        ha = NB
        rest = list(zip(range(NB + 1, H), (s2_buf, s3_buf, s4_buf), (m2_buf, m3_buf, m4_buf)))
        late = []
        for n, h in enumerate(range(NB + 3, H)):
            late += [cp_v(h, sem_first.at[8 + 2 * n]), cp_wo(h, sem_first.at[9 + 2 * n])]
        for cp in late:
            cp.start()
        cp_wr().wait()
        for p in range(NB + 1, H):
            cp_wm(p).wait()

        def l_step(j, do_x, do_y):
            if do_x and do_y:
                aw = view(acc, j - 1, TL, 2)
                ay, ax = aw.at[0:TL, :], aw.at[TL:2 * TL, :]
            elif do_x:
                ax = view(acc, j, TL)
            else:
                ay = view(acc, j - 1, TL)
            rec = None
            if do_y:
                chunks = epi_chunks(j - 1, ay, view(o_buf, j - 1, TL))
                os_ = [(h, pv(h, sv, mv)) for h, sv, mv in rest]
            if do_x:
                oa = pv(ha, view(s_buf, j, TL), view(m_buf, j, TL))
            if do_y:
                oproj(os_, ay, view(x_buf, j - 1, TL))
            if do_x:
                if do_y:
                    rec = _Pace(chunks, cfg["LCNT"])
                for h, sv, mv in rest:
                    q = pltpu.bitcast(view(q_ring.at[h & 3], j, TL // 2)[...], bf16)
                    scores(h, q, sv, mv, rec=rec)
                oproj([(ha, oa)], ax, rec=rec)
            if do_y:
                if not do_x:
                    for ch in chunks:
                        ch()
                cp_out(j - 1).start()

        for p in range(NB, H):
            mod_piece(p)
        finish_mod()
        l_step(0, True, False)
        for cp in late:
            cp.wait()

        def pl_body(j, carry):
            l_step(j, True, True)
            return carry
        lax.fori_loop(1, JL, pl_body, 0)
        wait_ffn()
        for j in range(JL - 2):
            cp_out(j).wait()
        l_step(JL, False, True)

        k1, k2 = key_buf[0], key_buf[1]
        for sh in (4, 2, 1):
            o1, o2 = pltpu.roll(k1, sh, 0), pltpu.roll(k2, sh, 0)
            k2 = jnp.maximum(jnp.minimum(k1, o1), jnp.maximum(k2, o2))
            k1 = jnp.maximum(k1, o1)

        def score_of(k):
            hi = k & jnp.int32(-65536)
            return pltpu.bitcast(jnp.where(hi < 0, hi ^ 0x7FFF0000, hi), f32)

        i1s = jnp.minimum(0xFFFF - (k1[0, 0] & 0xFFFF), S - 1)
        i2s = jnp.minimum(0xFFFF - (k2[0, 0] & 0xFFFF), S - 1)

        sub = lax.broadcasted_iota(i32, (16, D), 0)
        sb, cb1, gb = (_rep(modv[i], 16) for i in (1, 2, 3))

        def adaln2(x1, stat):
            return (x1 - _wide(stat[:, 0:128], D)) * _wide(stat[:, 128:256], D) * cb1 + sb

        def pick(ref):
            sel = lax.broadcasted_iota(i32, (16, ref.shape[1]), 0) == 0
            return jnp.where(sel, ref[pl.ds(i1s, 1), :], ref[pl.ds(i2s, 1), :])

        xs = adaln2(pick(acc), pick(st2_buf)).astype(bf16)
        FC, lag = cfg["FC"], 2
        y = None
        act = []
        for c in range(F // FC + lag):
            if c < F // FC:
                cs = slice(c * FC, (c + 1) * FC)
                g = _rb(jnp.dot(xs, wg[:, cs], preferred_element_type=f32))
                u = _rb(jnp.dot(xs, wu[:, cs], preferred_element_type=f32))
                act.append((_rb(g * jax.nn.sigmoid(g)) * u).astype(bf16))
            if c >= lag:
                d = jnp.dot(act[c - lag], wd[(c - lag) * FC:(c - lag + 1) * FC, :],
                            preferred_element_type=f32)
                y = d if y is None else y + d
        y = _rb(y)
        ya = _rb(y[0:1, :] * _wide(_rb(jax.nn.sigmoid(score_of(k1[0:1, :]))), D))
        yb = _rb(y[1:2, :] * _wide(_rb(jax.nn.sigmoid(score_of(k2[0:1, :]))), D))

        g1 = pl.multiple_of((i1s >> 4) << 4, 16)
        g2 = pl.multiple_of((i2s >> 4) << 4, 16)
        for t, g0 in enumerate((g1, g2)):
            rid = sub + g0
            x1 = acc[pl.ds(g0, 16), :]
            upd = jnp.where(rid == i1s, ya, 0.0) + jnp.where(rid == i2s, yb, 0.0)
            fix[t] = (x1 + gb * (adaln2(x1, st2_buf[pl.ds(g0, 16), :]) + upd)).astype(bf16)

        for j in range(JL - 2, JL):
            cp_out(j).wait()

        def cp_fix(t, g0):
            return pltpu.make_async_copy(fix.at[t], out_hbm.at[pl.ds(g0, 16), :], sem_fix.at[t])

        cp_fix(0, g1).start()

        @pl.when(g2 != g1)
        def _():
            cp_fix(1, g2).start()
            cp_fix(1, g2).wait()
        cp_fix(0, g1).wait()

    return kernel


_CFG = dict(FC=256, T0=256, TL=256, MCH=128, LD=9, TB=2048, RLM=0, RLB=0, RB=16, NCH=1,
            G=4, LCNT='33333333332000', LC0='28860800', LCB='wwww')


def _build(A_x, A_k_cache, A_v_cache, A_wq, A_wo, B_w_r, B_w_gate, B_w_up, B_w_down, c, w_mod,
           **over):
    B, S, D = A_x.shape
    _, H, SK, DH = A_k_cache.shape
    F = B_w_gate.shape[1]
    assert B == 1
    cfg = dict(_CFG, **over)
    T0, TL, G = cfg["T0"], cfg["TL"], cfg["G"]
    MC = (4 * D) // H
    kernel = _make_kernel(S, D, H, DH, SK, F, cfg)
    scratch = [
        pltpu.VMEM((S, D), bf16),
        pltpu.VMEM((S // 2, D), u32),
        pltpu.VMEM((S, D), f32),
        pltpu.VMEM((S, SK), f32),
        pltpu.VMEM((S, 128), f32),
        pltpu.VMEM((TL, SK), f32),
        pltpu.VMEM((TL, 128), f32),
        pltpu.VMEM((TL, SK), f32),
        pltpu.VMEM((TL, 128), f32),
        pltpu.VMEM((TL, SK), f32),
        pltpu.VMEM((TL, 128), f32),
        pltpu.VMEM((S, 256), f32),
        pltpu.VMEM((S, 256), f32),
        pltpu.VMEM((4, S // 2, DH), u32),
        pltpu.VMEM((G, S, DH), f32),
        pltpu.VMEM((8, G * DH), f32),
        pltpu.VMEM((4, SK, DH), bf16),
        pltpu.VMEM((4, SK, DH), bf16),
        pltpu.VMEM((D, G * DH), bf16),
        pltpu.VMEM((2, D, DH), bf16),
        pltpu.VMEM((4, DH, D), bf16),
        pltpu.VMEM((G + 1, D, MC), bf16),
        pltpu.VMEM((D, D), bf16),
        pltpu.VMEM((S // T0, D, D // (S // T0)), bf16),
        pltpu.VMEM((1, D), bf16),
        pltpu.VMEM((D,), bf16),
        pltpu.VMEM((D, 128), f32),
        pltpu.VMEM((2, 8, D), f32),
        pltpu.VMEM((S // T0, 1, D // (S // T0)), f32),
        pltpu.VMEM((H, 1, MC), f32),
        pltpu.VMEM((9, 8, D), f32),
        pltpu.VMEM((D, F), bf16),
        pltpu.VMEM((D, F), bf16),
        pltpu.VMEM((F, D), bf16),
        pltpu.VMEM((S, D), bf16),
        pltpu.VMEM((2, 8, 128), i32),
        pltpu.VMEM((2, 16, D), bf16),
        pltpu.SemaphoreType.DMA((sum(_sem_sizes(S, D, cfg)),)),
    ]
    any_spec = pl.BlockSpec(memory_space=pl.ANY)
    out = pl.pallas_call(
        kernel,
        out_shape=jax.ShapeDtypeStruct((S, D), bf16),
        in_specs=[any_spec] * 11,
        out_specs=any_spec,
        scratch_shapes=scratch,
        compiler_params=pltpu.CompilerParams(vmem_limit_bytes=112 * 1024 * 1024,
                                             disable_bounds_checks=True,
                                             disable_semaphore_checks=True),
    )(A_x.reshape(S, D), A_k_cache.reshape(H, SK, DH), A_v_cache.reshape(H, SK, DH),
      A_wq, A_wo, B_w_r, B_w_gate, B_w_up, B_w_down, c, w_mod)
    return out.reshape(B, S, D)


@jax.jit
def pallas_adaLN_cond__mha_block_cached__moe_arch_mod__prompt_kernel(
    A_x: jax.Array,
    A_k_cache: jax.Array,
    A_v_cache: jax.Array,
    A_wq: jax.Array,
    A_wo: jax.Array,
    B_x: jax.Array,
    B_w_r: jax.Array,
    B_w_gate: jax.Array,
    B_w_up: jax.Array,
    B_w_down: jax.Array,
    c: jax.Array,
    w_mod: jax.Array,
):
    del B_x
    return _build(A_x, A_k_cache, A_v_cache, A_wq, A_wo, B_w_r, B_w_gate, B_w_up, B_w_down,
                  c, w_mod)
```

```python
import jax
import jax.numpy as jnp
from jax import lax
import jax.experimental.pallas as pl
import jax.experimental.pallas.tpu as pltpu

f32 = jnp.float32
bf16 = jnp.bfloat16
u32 = jnp.uint32
i32 = jnp.int32

_NT = (((1,), (1,)), ((), ()))
_LOG2E = 1.4426950408889634
_EPS = 1e-5
_IMIN = -2 ** 31


def _rb(v):
    return v.astype(bf16).astype(f32)


def _rep(v, n):
    return v if n == 8 else jnp.tile(v, (n // 8, 1))


def _wide(v, w):
    return jnp.tile(v, (1, w // 128))


def _zero_of(v):
    bits = pltpu.bitcast(v, u32)
    return pltpu.bitcast(lax.shift_right_logical(lax.shift_right_logical(bits, jnp.uint32(31)),
                                                 jnp.uint32(1)), f32)


class _Pace:
    def __init__(self, chunks, counts):
        self.chunks = list(chunks)
        self.counts = [int(ch, 36) for ch in counts]
        assert sum(self.counts) == len(self.chunks), (counts, len(self.chunks))

    def done(self, res):
        n = self.counts.pop(0)
        for i in range(n):
            r0 = (i * res.shape[0] // n) // 8 * 8
            self.chunks.pop(0)(_zero_of(res[r0:r0 + 8, 0:128]))


def _tiles(v):
    return [v[:, c * 128:(c + 1) * 128] for c in range(v.shape[1] // 128)]


def _fold(op, parts):
    out = parts[0]
    for p in parts[1:]:
        out = op(out, p)
    return out


def _lane_sum(v):
    return jnp.broadcast_to(jnp.sum(v, axis=-1, keepdims=True), v.shape)


def _row_stats(xf, tok=None):
    d = xf.shape[-1]
    ts = _tiles(xf)
    nt = len(ts)
    if tok is not None:
        ts = [ts[0] + tok] + ts[1:]
    mu = _fold(jnp.add, ts) * (1.0 / nt)
    m2 = _fold(jnp.add, [(t - mu) * (t - mu) for t in ts])
    mean = _lane_sum(mu) * (1.0 / 128)
    dm = mu - mean
    var = _lane_sum(m2 + (dm * dm) * float(nt)) * (1.0 / d)
    return mean, lax.rsqrt(var + _EPS)


def _sem_sizes(S, D, cfg):
    j0 = S // cfg["T0"]
    return [2, 2 * (D // cfg["MCH"]), j0, j0, 16, 5, 3, S // cfg["TL"], 2]


def _make_kernel(S, D, H, DH, SK, F, cfg):
    T0, TB, TL, MCH = cfg["T0"], cfg["TB"], cfg["TL"], cfg["MCH"]
    J0 = S // T0
    JL = S // TL
    qscale = DH ** -0.5 * _LOG2E
    n_mch = D // MCH
    NA = cfg["NA"]
    NP = J0 - NA
    PW = D // NP
    G = cfg["G"]
    NB = H - G
    MC = (4 * D) // H
    W = 512
    assert PW % 128 == 0 and 2 <= G <= 4

    def kernel(x_hbm, k_hbm, v_hbm, wq_hbm, wo_hbm, wr_hbm, wg_hbm, wu_hbm, wd_hbm,
               c_hbm, wmod_hbm, out_hbm,
               x_buf, h_buf, acc, s_buf, m_buf, s2_buf, m2_buf, s3_buf, m3_buf, s4_buf, m4_buf,
               st_buf, st2_buf,
               q_ring, qf_buf, bq_buf,
               kb, vb, wq0, wqb, wob, wmb, wca, wsa, c_buf, wr_buf, cb_buf, mod0, sar, modr, modv,
               wg, wu, wd, o_buf, key_buf, fix,
               sems):

        class _Sem:
            def __init__(self, base):
                self.base = base
                self.at = self

            def __getitem__(self, i):
                return sems.at[self.base + i]

        sizes = _sem_sizes(S, D, cfg)
        offs = [sum(sizes[:i]) for i in range(len(sizes))]
        (sem_small, sem_ca, sem_x, sem_sa, sem_first, sem_head,
         sem_ffn, sem_out, sem_fix) = (_Sem(o) for o in offs)

        def _mul(a, n):
            v = a * n
            return v if isinstance(a, int) else pl.multiple_of(v, n)

        def view(ref, j, t, n=1):
            return ref.at[pl.ds(_mul(j, t), n * t), :]

        def cp_c():
            return pltpu.make_async_copy(c_hbm, c_buf, sem_small.at[0])

        def cp_wr():
            return pltpu.make_async_copy(wr_hbm, wr_buf, sem_small.at[1])

        def cp_ca(c, i):
            return pltpu.make_async_copy(
                wmod_hbm.at[pl.ds(i * MCH, MCH), pl.ds(D + c * W, W)], view(wca.at[c], i, MCH),
                sem_ca.at[c * n_mch + i])

        def cp_sa(j):
            return pltpu.make_async_copy(
                wmod_hbm.at[:, pl.ds(_mul(j, PW), PW)], wsa.at[j], sem_sa.at[j])

        def cp_x(j):
            return pltpu.make_async_copy(view(x_hbm, j, T0), view(x_buf, j, T0), sem_x.at[j])

        def cp_wq0(c):
            return pltpu.make_async_copy(wq_hbm.at[pl.ds(c * W, W), pl.ds(0, G * DH)],
                                         view(wq0, c, W), sem_first.at[14 + c])

        def cp_k(h, sem=None):
            return pltpu.make_async_copy(k_hbm.at[h], kb.at[h & 3],
                                         sem_head.at[0] if sem is None else sem)

        def cp_wq(h):
            src = h if isinstance(h, int) else jnp.minimum(h, H - 1)
            return pltpu.make_async_copy(wq_hbm.at[:, pl.ds(_mul(src, DH), DH)], wqb.at[h & 1],
                                         sem_head.at[1])

        def cp_v(h, sem=None):
            return pltpu.make_async_copy(v_hbm.at[h], vb.at[h & 3],
                                         sem_head.at[2] if sem is None else sem)

        def cp_wo(h, sem=None):
            return pltpu.make_async_copy(view(wo_hbm, h, DH), wob.at[h & 3],
                                         sem_head.at[3] if sem is None else sem)

        def wm_slot(p):
            return p - NB + 1 if (isinstance(p, int) and p > NB) else p & 1

        def cp_wm(p):
            extra = isinstance(p, int) and p > NB
            return pltpu.make_async_copy(
                wmod_hbm.at[:, pl.ds(_mul(p + (2 * D) // MC, MC), MC)], wmb.at[wm_slot(p)],
                sem_first.at[4 + p - NB] if extra else sem_head.at[4])

        ffn = ((wg_hbm, wg), (wu_hbm, wu), (wd_hbm, wd))

        def start_ffn_piece(p):
            for i, (src, dst) in enumerate(ffn):
                n = src.shape[0] // H
                pltpu.make_async_copy(view(src, p, n), view(dst, p, n), sem_ffn.at[i]).start()

        def wait_ffn():
            for i, (src, dst) in enumerate(ffn):
                pltpu.make_async_copy(src, dst, sem_ffn.at[i]).wait()

        def cp_out(j):
            return pltpu.make_async_copy(view(o_buf, j, TL), view(out_hbm, j, TL), sem_out.at[j])

        def head_copies(h):
            return [cp_wq(h + G), cp_k(h + G - 1), cp_wo(h + 2), cp_wm(h), cp_v(h + 2)]

        def ln1_chunks(xv, sv):
            def chunk(off):
                def f(tok=None):
                    mean, inv = _row_stats(xv[off:off + 8, :].astype(f32), tok)
                    sv[off:off + 8, 0:128] = mean
                    sv[off:off + 8, 128:256] = inv
                return f
            return [chunk(off) for off in range(0, T0, 8)]

        def ln1_scaled(x, stat, cs, tok=None):
            w = x.shape[1]
            mean = stat[:, 0:128] if tok is None else stat[:, 0:128] + _rep(tok, x.shape[0])
            n = (x.astype(f32) - _wide(mean, w)) * _wide(stat[:, 128:256], w)
            return n * _rep(mod0[1, :, cs], x.shape[0])

        def qproj(h):
            q = None
            for c in range(D // W):
                cs = slice(c * W, (c + 1) * W)
                part = jnp.dot(pltpu.bitcast(h_buf[:, cs], bf16), wqb[h & 1, cs, :],
                               preferred_element_type=f32)
                q = part if q is None else q + part
            q_ring[h & 3] = pltpu.bitcast((q * qscale).astype(bf16), u32)

        def q_early(g, q):
            return ((q + _rep(bq_buf[:, g * DH:(g + 1) * DH], q.shape[0])) * qscale).astype(bf16)

        def scores(h, q, sv, mv, rec=None, reload=False):
            mp = None
            for c in range(SK // W):
                cs = slice(c * W, (c + 1) * W)
                s = lax.dot_general(q, kb[h & 3, cs, :], _NT, preferred_element_type=f32)
                sv[:, cs] = s
                if rec is not None:
                    rec.done(s)
                if not reload:
                    mp = _fold(jnp.maximum, ([] if mp is None else [mp]) + _tiles(s))
            if reload:
                mp = _fold(jnp.maximum, _tiles(sv[...]))
            mv[...] = jnp.broadcast_to(jnp.max(mp, axis=-1, keepdims=True), mp.shape)

        def pv(h, sv, mv, rec=None, late=False):
            o = lp = None
            for c in range(SK // W):
                cs = slice(c * W, (c + 1) * W)
                m = mv[...]
                if c >= cfg["LD"] and sv.shape[0] == S:
                    m = m + _zero_of(lp)
                p = jnp.exp2(sv[:, cs] - _wide(m, W))
                lp = _fold(jnp.add, ([] if lp is None else [lp]) + _tiles(p))
                d = jnp.dot(p.astype(bf16), vb[h & 3, cs, :], preferred_element_type=f32)
                o = d if o is None else o + d
                if rec is not None:
                    rec.done(d)
            if late:
                lp = lp + _zero_of(o)
            l = jnp.sum(lp, axis=-1, keepdims=True)
            r = pl.reciprocal(l, approx=True)
            r = r * (2.0 - l * r)
            return (o * r).astype(bf16)

        def oproj(hos, av, xv=None, rec=None):
            for c in range(D // W):
                cs = slice(c * W, (c + 1) * W)
                a = av[:, cs]
                for h, o in hos:
                    if not isinstance(h, int):
                        a = jnp.where(h > 0, a, 0.0)
                    d = jnp.dot(o, wob[h & 3, :, cs], preferred_element_type=f32)
                    if rec is not None:
                        rec.done(d)
                    a = a + d
                if xv is not None:
                    a = xv[:, cs].astype(f32) + _rep(modv[0, :, cs], a.shape[0]) * a
                av[:, cs] = a

        def matvec(wv, tok=None):
            n = wv.shape[1]
            NCH = cfg['NCH']
            parts = [None if tok is None else _wide(tok, n)] * NCH
            for r in range(0, D, 16):
                t = wv[r:r + 16, :].astype(f32) * _wide(cb_buf[r:r + 16, :], n)
                for e in range(2):
                    i = (r // 8 + e) % NCH
                    te = t[e * 8:(e + 1) * 8, :]
                    parts[i] = te if parts[i] is None else parts[i] + te
            return _rb(jnp.sum(_fold(jnp.add, parts), axis=0, keepdims=True))

        def mod_piece(p, tok=None):
            modr[p] = matvec(wmb.at[wm_slot(p)], tok)

        def finish_mod():
            n = D // MC
            ga, sb, cb, gb = (jnp.concatenate([modr[i * n + t] for t in range(n)], axis=-1)
                              for i in range(4))
            cb1 = _rb(1.0 + cb)
            wr = wr_buf[...].astype(f32).reshape(1, D)
            a = cb1 * wr
            a0 = jnp.broadcast_to(jnp.sum(a, axis=-1, keepdims=True), (1, D))
            b0 = jnp.broadcast_to(jnp.sum(sb * wr, axis=-1, keepdims=True), (1, D))
            for i, v in enumerate((ga, sb, cb1, gb, a, gb * cb1, gb * sb, a0, b0)):
                modv[i] = jnp.broadcast_to(v, (8, D))

        def out_rows(x1, mean, inv):
            return (x1 + ((x1 - _wide(mean, D)) * (_wide(inv, D) * modv[5]) + modv[6])).astype(bf16)

        def out_chunks(j):
            x1v, sv, ov = view(acc, j, TL), view(st2_buf, j, TL), view(o_buf, j, TL)

            def chunk(off):
                def f(tok):
                    rs = slice(off, off + 8)
                    ov[rs, :] = out_rows(x1v[rs, :], sv[rs, 0:128] + tok, sv[rs, 128:256] + tok)
                return f
            return [chunk(off) for off in range(0, TL, 8)]

        def epi_chunks(j, x1v, ov, with_out=True):
            sub = lax.broadcasted_iota(i32, (8, 128), 0)
            low = (0xFFFF - j * TL) - sub
            sv = view(st2_buf, j, TL)
            st = {}

            def chunk(off):
                def f(tok=None):
                    if off == 0:
                        st["k1"], st["k2"] = key_buf[0], key_buf[1]
                    x1 = x1v[off:off + 8, :]
                    mean, inv = _row_stats(x1, tok)
                    sv[off:off + 8, 0:128] = mean
                    sv[off:off + 8, 128:256] = inv
                    xa = _tiles(x1 * modv[4])
                    if tok is not None:
                        xa[0] = xa[0] + tok
                    ra = _lane_sum(_fold(jnp.add, xa))
                    r = inv * (ra - mean * modv[7, :, 0:128]) + modv[8, :, 0:128]
                    if with_out:
                        ov[off:off + 8, :] = out_rows(x1, mean, inv)
                    bits = pltpu.bitcast(_rb(r) + 0.0, i32)
                    key = jnp.where(bits < 0, bits ^ 0x7FFF0000, bits) | (low - off)
                    st["k2"] = jnp.maximum(st["k2"], jnp.minimum(st["k1"], key))
                    st["k1"] = jnp.maximum(st["k1"], key)
                    if off + 8 == TL:
                        key_buf[0], key_buf[1] = st["k1"], st["k2"]
                return f
            return [chunk(off) for off in range(0, TL, 8)]

        cp_c().start()
        cp_x(0).start()
        for c in range(2):
            cp_wq0(c).start()
            for i in range(n_mch):
                cp_ca(c, i).start()
            for j in (range(1, NA) if c == 0 else [NA]):
                cp_x(j).start()
        for j in range(NA, J0):
            if j + 1 < J0:
                cp_x(j + 1).start()
            cp_sa(j - NA).start()
        for h in range(G - 1):
            cp_k(h, sem_first.at[1 + h]).start()
        early = []
        for h in range(2):
            early += [cp_v(h, sem_first.at[8 + 2 * h]), cp_wo(h, sem_first.at[9 + 2 * h])]
        for cp in early + head_copies(0):
            cp.start()

        cp_c().wait()
        cf = c_buf[...].astype(f32)
        sc = _rb(cf * jax.nn.sigmoid(cf))
        cb_buf[...] = jnp.transpose(jnp.broadcast_to(sc, (128, D)))
        key_buf[...] = jnp.full(key_buf.shape, _IMIN, i32)
        cp_x(0).wait()
        for ch in ln1_chunks(view(x_buf, 0, T0), view(st_buf, 0, T0)):
            ch()

        def ca_half(c, stream):
            cp_wq0(c).wait()
            if not stream:
                for i in range(n_mch):
                    cp_ca(c, i).wait()
            part = None
            for i in range(n_mch):
                if stream:
                    cp_ca(c, i).wait()
                scb = jnp.broadcast_to(sc[:, i * MCH:(i + 1) * MCH], (16, MCH)).astype(bf16)
                d = jnp.dot(scb, wca[c, i * MCH:(i + 1) * MCH, :], preferred_element_type=f32)
                part = d if part is None else part + d
            mod0[1, :, c * W:(c + 1) * W] = _rb(1.0 + _rb(part[0:8, :]))

        def q_first(j, t, halves, jn, counts):
            xv, stat = view(x_buf, j, t), view(st_buf, j, t)[...]
            rec = _Pace(ln1_chunks(view(x_buf, jn, T0), view(st_buf, jn, T0)), counts)
            qfv = [view(qf_buf.at[g], j, t) for g in range(G)]
            qs = [None if halves[0] == 0 else qfv[g][...] for g in range(G)]
            for c in halves:
                cs = slice(c * W, (c + 1) * W)
                hh = ln1_scaled(xv[:, cs], stat, cs).astype(bf16)
                for g in range(G):
                    part = jnp.dot(hh, wq0[cs, g * DH:(g + 1) * DH], preferred_element_type=f32)
                    qs[g] = part if qs[g] is None else qs[g] + part
                    rec.done(part)
            for g in range(G):
                qfv[g][...] = qs[g]

        ca_half(0, True)

        def pa_body(j, carry):
            @pl.when(j + 1 < NA)
            def _():
                cp_x(j + 1).wait()
            q_first(j, T0, (0,), jnp.minimum(j + 1, NA - 1), cfg["LCA"])
            return carry
        lax.fori_loop(0, NA, pa_body, 0)
        ca_half(1, False)
        cp_x(NA).wait()
        q_first(0, NA * T0, (1,), NA, cfg["LCA2"])

        def p0a_body(j, carry):
            @pl.when(j + 1 < J0)
            def _():
                cp_x(j + 1).wait()
            cp_sa(j - NA).wait()
            q_first(j, T0, (0, 1), jnp.minimum(j + 1, J0 - 1), cfg["LC0"])
            sar[j - NA] = matvec(wsa.at[j - NA])
            return carry
        lax.fori_loop(NA, J0, p0a_body, 0)

        sa = jnp.concatenate([sar[j] for j in range(NP)], axis=-1)
        mod0[0] = jnp.broadcast_to(sa, (8, D))
        bq_buf[...] = jnp.dot(jnp.broadcast_to(sa, (16, D)).astype(bf16), wq0[...],
                              preferred_element_type=f32)[0:8, :]
        cp_k(0, sem_first.at[1]).wait()

        def p0b_body(j, carry):
            RB = cfg["RB"]
            xv, sv, hv = view(x_buf, j, TB), view(st_buf, j, TB), view(h_buf, j, TB // 2)
            qfv = [view(qf_buf.at[g], j, TB) for g in range(G)]
            qrv = [view(q_ring.at[g], j, TB // 2) for g in range(G)]

            def chunk(off):
                def f(tok):
                    hh = (ln1_scaled(xv[off:off + RB, :], sv[off:off + RB, :], slice(0, D), tok)
                          + _rep(mod0[0], RB)).astype(bf16)
                    hv[off // 2:(off + RB) // 2, :] = pltpu.bitcast(hh, u32)
                    for g in range(1, G):
                        qg = q_early(g, qfv[g][off:off + RB, :] + _rep(tok, RB))
                        qrv[g][off // 2:(off + RB) // 2, :] = pltpu.bitcast(qg, u32)
                return f
            rec = _Pace([chunk(off) for off in range(0, TB, RB)], cfg["LCB"])
            scores(0, q_early(0, qfv[0][...]), view(s_buf, j, TB), view(m_buf, j, TB), rec=rec,
                   reload=cfg['RLB'])
            return carry
        lax.fori_loop(0, S // TB, p0b_body, 0)

        def main_body(h, carry):
            qproj(h + G)
            start_ffn_piece(h)
            for cp in head_copies(h + 1):
                cp.start()
            o = pv(h, s_buf, m_buf)
            rec = _Pace([lambda tok: mod_piece(h, tok)], "1000")
            scores(h + 1, pltpu.bitcast(q_ring[(h + 1) & 3], bf16), s_buf, m_buf, rec=rec,
                   reload=cfg['RLM'])
            oproj([(h, o)], acc)
            for cp in head_copies(h + 1):
                cp.wait()
            return carry
        for h in range(1, G - 1):
            cp_k(h, sem_first.at[1 + h]).wait()
        for cp in early + head_copies(0):
            cp.wait()
        cp_wr().start()
        for p in range(NB + 1, H):
            cp_wm(p).start()
        for p in range(NB, H):
            start_ffn_piece(p)
        lax.fori_loop(0, NB, main_body, 0)

        ha = NB
        rest = list(zip(range(NB + 1, H), (s2_buf, s3_buf, s4_buf), (m2_buf, m3_buf, m4_buf)))
        late = []
        for n, h in enumerate(range(NB + 3, H)):
            late += [cp_v(h, sem_first.at[8 + 2 * n]), cp_wo(h, sem_first.at[9 + 2 * n])]
        for cp in late:
            cp.start()
        cp_wr().wait()
        for p in range(NB + 1, H):
            cp_wm(p).wait()

        def l_step(j, do_x, do_y):
            if do_x and do_y:
                aw = view(acc, j - 1, TL, 2)
                ay, ax = aw.at[0:TL, :], aw.at[TL:2 * TL, :]
            elif do_x:
                ax = view(acc, j, TL)
            else:
                ay = view(acc, j - 1, TL)
            rec = None
            if do_y:
                chunks = epi_chunks(j - 1, ay, view(o_buf, j - 1, TL), with_out=do_x)
                os_ = [(h, pv(h, sv, mv, late=not do_x)) for h, sv, mv in rest]
            if do_x:
                oa = pv(ha, view(s_buf, j, TL), view(m_buf, j, TL))
            if do_y and do_x:
                oproj(os_, ay, view(x_buf, j - 1, TL))
            elif do_y:
                xv = view(x_buf, j - 1, TL)
                r0, prev = 0, []
                for n in cfg["LSPLIT"]:
                    rs = slice(r0, r0 + n)
                    nr = len(os_) * (D // W)
                    cnt = [len(prev) // nr + (1 if i < len(prev) % nr else 0) for i in range(nr)]
                    rec = _Pace(prev, "".join("0123456789abcdefghijklmnopqrstuvwxyz"[i] for i in cnt))
                    oproj([(h, o[rs]) for h, o in os_], ay.at[rs, :], xv.at[rs, :], rec=rec)
                    prev = chunks[r0 // 8:(r0 + n) // 8]
                    r0 += n
                chunks = prev
            if do_x:
                if do_y:
                    rec = _Pace(chunks, cfg["LCNT"])
                for h, sv, mv in rest:
                    q = pltpu.bitcast(view(q_ring.at[h & 3], j, TL // 2)[...], bf16)
                    scores(h, q, sv, mv, rec=rec)
                oproj([(ha, oa)], ax, rec=rec)
            if do_y:
                if do_x:
                    cp_out(j - 1).start()
                else:
                    for ch in chunks:
                        ch()

        for p in range(NB, H):
            mod_piece(p)
        finish_mod()
        l_step(0, True, False)
        for cp in late:
            cp.wait()

        def pl_body(j, carry):
            l_step(j, True, True)
            return carry
        lax.fori_loop(1, JL, pl_body, 0)
        wait_ffn()
        for j in range(JL - 2):
            cp_out(j).wait()
        l_step(JL, False, True)

        k1, k2 = key_buf[0], key_buf[1]
        for sh in (4, 2, 1):
            o1, o2 = pltpu.roll(k1, sh, 0), pltpu.roll(k2, sh, 0)
            k2 = jnp.maximum(jnp.minimum(k1, o1), jnp.maximum(k2, o2))
            k1 = jnp.maximum(k1, o1)

        def score_of(k):
            hi = k & jnp.int32(-65536)
            return pltpu.bitcast(jnp.where(hi < 0, hi ^ 0x7FFF0000, hi), f32)

        i1s = jnp.minimum(0xFFFF - (k1[0, 0] & 0xFFFF), S - 1)
        i2s = jnp.minimum(0xFFFF - (k2[0, 0] & 0xFFFF), S - 1)

        sub = lax.broadcasted_iota(i32, (16, D), 0)
        sb, cb1, gb = (_rep(modv[i], 16) for i in (1, 2, 3))

        def adaln2(x1, stat):
            return (x1 - _wide(stat[:, 0:128], D)) * _wide(stat[:, 128:256], D) * cb1 + sb

        def pick(ref):
            sel = lax.broadcasted_iota(i32, (16, ref.shape[1]), 0) == 0
            return jnp.where(sel, ref[pl.ds(i1s, 1), :], ref[pl.ds(i2s, 1), :])

        xs = adaln2(pick(acc), pick(st2_buf)).astype(bf16)
        FC, lag = cfg["FC"], 2
        y = None
        act = []
        outs = out_chunks(JL - 1)
        for c in range(F // FC + lag):
            if c < F // FC:
                cs = slice(c * FC, (c + 1) * FC)
                g = jnp.dot(xs, wg[:, cs], preferred_element_type=f32)
                u = jnp.dot(xs, wu[:, cs], preferred_element_type=f32)
                for v in (g, u):
                    for t in range(cfg["FOUT"]):
                        if outs:
                            outs.pop(0)(_zero_of(v[0:8, (t % 2) * 128:(t % 2 + 1) * 128]))
                            if not outs:
                                cp_out(JL - 1).start()
                g, u = _rb(g), _rb(u)
                act.append((_rb(g * jax.nn.sigmoid(g)) * u).astype(bf16))
            if c >= lag:
                d = jnp.dot(act[c - lag], wd[(c - lag) * FC:(c - lag + 1) * FC, :],
                            preferred_element_type=f32)
                y = d if y is None else y + d
        y = _rb(y)
        ya = _rb(y[0:1, :] * _wide(_rb(jax.nn.sigmoid(score_of(k1[0:1, :]))), D))
        yb = _rb(y[1:2, :] * _wide(_rb(jax.nn.sigmoid(score_of(k2[0:1, :]))), D))

        g1 = pl.multiple_of((i1s >> 4) << 4, 16)
        g2 = pl.multiple_of((i2s >> 4) << 4, 16)
        for t, g0 in enumerate((g1, g2)):
            rid = sub + g0
            x1 = acc[pl.ds(g0, 16), :]
            upd = jnp.where(rid == i1s, ya, 0.0) + jnp.where(rid == i2s, yb, 0.0)
            fix[t] = (x1 + gb * (adaln2(x1, st2_buf[pl.ds(g0, 16), :]) + upd)).astype(bf16)

        for j in range(JL - 2, JL):
            cp_out(j).wait()

        def cp_fix(t, g0):
            return pltpu.make_async_copy(fix.at[t], out_hbm.at[pl.ds(g0, 16), :], sem_fix.at[t])

        cp_fix(0, g1).start()

        @pl.when(g2 != g1)
        def _():
            cp_fix(1, g2).start()
            cp_fix(1, g2).wait()
        cp_fix(0, g1).wait()

    return kernel


_CFG = dict(FC=256, T0=256, TL=256, MCH=256, NA=4, LCA='gg00', LCA2='0gg0', LD=9, TB=2048, RLM=0, RLB=0, RB=16, NCH=1,
            G=4, LSPLIT=(96, 96, 64), FOUT=2, LCNT='33333333332000', LC0='28860800', LCB='wwww')


def _build(A_x, A_k_cache, A_v_cache, A_wq, A_wo, B_w_r, B_w_gate, B_w_up, B_w_down, c, w_mod,
           **over):
    B, S, D = A_x.shape
    _, H, SK, DH = A_k_cache.shape
    F = B_w_gate.shape[1]
    assert B == 1
    cfg = dict(_CFG, **over)
    T0, TL, G = cfg["T0"], cfg["TL"], cfg["G"]
    MC = (4 * D) // H
    NP = S // T0 - cfg["NA"]
    kernel = _make_kernel(S, D, H, DH, SK, F, cfg)
    scratch = [
        pltpu.VMEM((S, D), bf16),
        pltpu.VMEM((S // 2, D), u32),
        pltpu.VMEM((S, D), f32),
        pltpu.VMEM((S, SK), f32),
        pltpu.VMEM((S, 128), f32),
        pltpu.VMEM((TL, SK), f32),
        pltpu.VMEM((TL, 128), f32),
        pltpu.VMEM((TL, SK), f32),
        pltpu.VMEM((TL, 128), f32),
        pltpu.VMEM((TL, SK), f32),
        pltpu.VMEM((TL, 128), f32),
        pltpu.VMEM((S, 256), f32),
        pltpu.VMEM((S, 256), f32),
        pltpu.VMEM((4, S // 2, DH), u32),
        pltpu.VMEM((G, S, DH), f32),
        pltpu.VMEM((8, G * DH), f32),
        pltpu.VMEM((4, SK, DH), bf16),
        pltpu.VMEM((4, SK, DH), bf16),
        pltpu.VMEM((D, G * DH), bf16),
        pltpu.VMEM((2, D, DH), bf16),
        pltpu.VMEM((4, DH, D), bf16),
        pltpu.VMEM((G + 1, D, MC), bf16),
        pltpu.VMEM((2, D, D // 2), bf16),
        pltpu.VMEM((NP, D, D // NP), bf16),
        pltpu.VMEM((1, D), bf16),
        pltpu.VMEM((D,), bf16),
        pltpu.VMEM((D, 128), f32),
        pltpu.VMEM((2, 8, D), f32),
        pltpu.VMEM((NP, 1, D // NP), f32),
        pltpu.VMEM((H, 1, MC), f32),
        pltpu.VMEM((9, 8, D), f32),
        pltpu.VMEM((D, F), bf16),
        pltpu.VMEM((D, F), bf16),
        pltpu.VMEM((F, D), bf16),
        pltpu.VMEM((S, D), bf16),
        pltpu.VMEM((2, 8, 128), i32),
        pltpu.VMEM((2, 16, D), bf16),
        pltpu.SemaphoreType.DMA((sum(_sem_sizes(S, D, cfg)),)),
    ]
    any_spec = pl.BlockSpec(memory_space=pl.ANY)
    out = pl.pallas_call(
        kernel,
        out_shape=jax.ShapeDtypeStruct((S, D), bf16),
        in_specs=[any_spec] * 11,
        out_specs=any_spec,
        scratch_shapes=scratch,
        compiler_params=pltpu.CompilerParams(vmem_limit_bytes=112 * 1024 * 1024,
                                             disable_bounds_checks=True,
                                             disable_semaphore_checks=True),
    )(A_x.reshape(S, D), A_k_cache.reshape(H, SK, DH), A_v_cache.reshape(H, SK, DH),
      A_wq, A_wo, B_w_r, B_w_gate, B_w_up, B_w_down, c, w_mod)
    return out.reshape(B, S, D)


@jax.jit
def pallas_adaLN_cond__mha_block_cached__moe_arch_mod__prompt_kernel(
    A_x: jax.Array,
    A_k_cache: jax.Array,
    A_v_cache: jax.Array,
    A_wq: jax.Array,
    A_wo: jax.Array,
    B_x: jax.Array,
    B_w_r: jax.Array,
    B_w_gate: jax.Array,
    B_w_up: jax.Array,
    B_w_down: jax.Array,
    c: jax.Array,
    w_mod: jax.Array,
):
    del B_x
    return _build(A_x, A_k_cache, A_v_cache, A_wq, A_wo, B_w_r, B_w_gate, B_w_up, B_w_down,
                  c, w_mod)
```

```python
import jax
import jax.numpy as jnp
from jax import lax
import jax.experimental.pallas as pl
import jax.experimental.pallas.tpu as pltpu

f32 = jnp.float32
bf16 = jnp.bfloat16
u32 = jnp.uint32
i32 = jnp.int32

_NT = (((1,), (1,)), ((), ()))
_LOG2E = 1.4426950408889634
_EPS = 1e-5
_IMIN = -2 ** 31


def _rb(v):
    return v.astype(bf16).astype(f32)


def _rep(v, n):
    return v if n == 8 else jnp.tile(v, (n // 8, 1))


def _wide(v, w):
    return jnp.tile(v, (1, w // 128))


def _zero_of(v):
    bits = pltpu.bitcast(v, u32)
    return pltpu.bitcast(lax.shift_right_logical(lax.shift_right_logical(bits, jnp.uint32(31)),
                                                 jnp.uint32(1)), f32)


class _Pace:
    def __init__(self, chunks, counts):
        self.chunks = list(chunks)
        self.counts = [ch if isinstance(ch, int) else int(ch, 36) for ch in counts]
        assert sum(self.counts) == len(self.chunks), (counts, len(self.chunks))

    def done(self, res):
        n = self.counts.pop(0)
        for i in range(n):
            r0 = (i * res.shape[0] // n) // 8 * 8
            self.chunks.pop(0)(_zero_of(res[r0:r0 + 8, 0:128]))


def _tiles(v):
    return [v[:, c * 128:(c + 1) * 128] for c in range(v.shape[1] // 128)]


def _fold(op, parts):
    out = parts[0]
    for p in parts[1:]:
        out = op(out, p)
    return out


def _lane_sum(v):
    return jnp.broadcast_to(jnp.sum(v, axis=-1, keepdims=True), v.shape)


def _row_stats(xf, tok=None):
    d = xf.shape[-1]
    ts = _tiles(xf)
    nt = len(ts)
    if tok is not None:
        ts = [ts[0] + tok] + ts[1:]
    mu = _fold(jnp.add, ts) * (1.0 / nt)
    m2 = _fold(jnp.add, [(t - mu) * (t - mu) for t in ts])
    mean = _lane_sum(mu) * (1.0 / 128)
    dm = mu - mean
    var = _lane_sum(m2 + (dm * dm) * float(nt)) * (1.0 / d)
    return mean, lax.rsqrt(var + _EPS)


def _sem_sizes(S, D, cfg):
    j0 = S // cfg["T0"]
    return [2, 2 * (D // cfg["MCH"]), j0, 1, 16, 5, 3, S // cfg["TL"], 2]


def _make_kernel(S, D, H, DH, SK, F, cfg):
    T0, TL, MCH = cfg["T0"], cfg["TL"], cfg["MCH"]
    J0 = S // T0
    JL = S // TL
    qscale = DH ** -0.5 * _LOG2E
    n_mch = D // MCH
    G = cfg["G"]
    NB = H - G
    MC = (4 * D) // H
    W = 512
    assert 2 <= G <= 4 and D == 2 * W

    def kernel(x_hbm, k_hbm, v_hbm, wq_hbm, wo_hbm, wr_hbm, wg_hbm, wu_hbm, wd_hbm,
               c_hbm, wmod_hbm, out_hbm,
               x_buf, h_buf, acc, s_buf, m_buf, s2_buf, m2_buf, s3_buf, m3_buf, s4_buf, m4_buf,
               st_buf, st2_buf,
               q_ring, qf_buf, bq_buf,
               kb, vb, wq0, wqb, wob, wmb, wca, wsa, c_buf, wr_buf, cb_buf, mod0, modr, modv,
               wg, wu, wd, o_buf, key_buf, fix,
               sems):

        class _Sem:
            def __init__(self, base):
                self.base = base
                self.at = self

            def __getitem__(self, i):
                return sems.at[self.base + i]

        sizes = _sem_sizes(S, D, cfg)
        offs = [sum(sizes[:i]) for i in range(len(sizes))]
        (sem_small, sem_ca, sem_x, sem_sa, sem_first, sem_head,
         sem_ffn, sem_out, sem_fix) = (_Sem(o) for o in offs)

        def _mul(a, n):
            v = a * n
            return v if isinstance(a, int) else pl.multiple_of(v, n)

        def view(ref, j, t, n=1):
            return ref.at[pl.ds(_mul(j, t), n * t), :]

        def cp_c():
            return pltpu.make_async_copy(c_hbm, c_buf, sem_small.at[0])

        def cp_wr():
            return pltpu.make_async_copy(wr_hbm, wr_buf, sem_small.at[1])

        def cp_ca(c, i):
            return pltpu.make_async_copy(
                wmod_hbm.at[pl.ds(i * MCH, MCH), pl.ds(D + c * W, W)], view(wca.at[c], i, MCH),
                sem_ca.at[c * n_mch + i])

        def cp_sa():
            return pltpu.make_async_copy(wmod_hbm.at[:, pl.ds(0, D)], wsa, sem_sa.at[0])

        def cp_x(j):
            return pltpu.make_async_copy(view(x_hbm, j, T0), view(x_buf, j, T0), sem_x.at[j])

        def cp_wq0(c):
            return pltpu.make_async_copy(wq_hbm.at[pl.ds(c * W, W), pl.ds(0, G * DH)],
                                         view(wq0, c, W), sem_first.at[14 + c])

        def cp_k(h, sem=None):
            return pltpu.make_async_copy(k_hbm.at[h], kb.at[h & 3],
                                         sem_head.at[0] if sem is None else sem)

        def cp_wq(h):
            src = h if isinstance(h, int) else jnp.minimum(h, H - 1)
            return pltpu.make_async_copy(wq_hbm.at[:, pl.ds(_mul(src, DH), DH)], wqb.at[h & 1],
                                         sem_head.at[1])

        def cp_v(h, sem=None):
            return pltpu.make_async_copy(v_hbm.at[h], vb.at[h & 3],
                                         sem_head.at[2] if sem is None else sem)

        def cp_wo(h, sem=None):
            return pltpu.make_async_copy(view(wo_hbm, h, DH), wob.at[h & 3],
                                         sem_head.at[3] if sem is None else sem)

        def wm_slot(p):
            return p - NB + 1 if (isinstance(p, int) and p > NB) else p & 1

        def cp_wm(p):
            extra = isinstance(p, int) and p > NB
            return pltpu.make_async_copy(
                wmod_hbm.at[:, pl.ds(_mul(p + (2 * D) // MC, MC), MC)], wmb.at[wm_slot(p)],
                sem_first.at[4 + p - NB] if extra else sem_head.at[4])

        ffn = ((wg_hbm, wg), (wu_hbm, wu), (wd_hbm, wd))

        def start_ffn_piece(p):
            for i, (src, dst) in enumerate(ffn):
                n = src.shape[0] // H
                pltpu.make_async_copy(view(src, p, n), view(dst, p, n), sem_ffn.at[i]).start()

        def wait_ffn():
            for i, (src, dst) in enumerate(ffn):
                pltpu.make_async_copy(src, dst, sem_ffn.at[i]).wait()

        def cp_out(j):
            return pltpu.make_async_copy(view(o_buf, j, TL), view(out_hbm, j, TL), sem_out.at[j])

        def head_copies(h):
            return [cp_wq(h + G), cp_k(h + G - 1), cp_wo(h + 2), cp_wm(h), cp_v(h + 2)]

        def ln1_chunks(xv, sv):
            def chunk(off):
                def f(tok=None):
                    mean, inv = _row_stats(xv[off:off + 8, :].astype(f32), tok)
                    sv[off:off + 8, 0:128] = mean
                    sv[off:off + 8, 128:256] = inv
                return f
            return [chunk(off) for off in range(0, xv.shape[0], 8)]

        def ln1_scaled(x, stat, cs, tok=None):
            w = x.shape[1]
            mean = stat[:, 0:128] if tok is None else stat[:, 0:128] + _rep(tok, x.shape[0])
            n = (x.astype(f32) - _wide(mean, w)) * _wide(stat[:, 128:256], w)
            return n * _rep(mod0[1, :, cs], x.shape[0])

        def qproj(h):
            q = None
            for c in range(D // W):
                cs = slice(c * W, (c + 1) * W)
                part = jnp.dot(pltpu.bitcast(h_buf[:, cs], bf16), wqb[h & 1, cs, :],
                               preferred_element_type=f32)
                q = part if q is None else q + part
            q_ring[h & 3] = pltpu.bitcast((q * qscale).astype(bf16), u32)

        def q_early(g, q):
            return ((q + _rep(bq_buf[:, g * DH:(g + 1) * DH], q.shape[0])) * qscale).astype(bf16)

        def scores(h, q, sv, mv, rec=None, reload=False):
            mp = None
            for c in range(SK // W):
                cs = slice(c * W, (c + 1) * W)
                s = lax.dot_general(q, kb[h & 3, cs, :], _NT, preferred_element_type=f32)
                sv[:, cs] = s
                if rec is not None:
                    rec.done(s)
                if not reload:
                    mp = _fold(jnp.maximum, ([] if mp is None else [mp]) + _tiles(s))
            if reload:
                mp = _fold(jnp.maximum, _tiles(sv[...]))
            mv[...] = jnp.broadcast_to(jnp.max(mp, axis=-1, keepdims=True), mp.shape)

        def pv(h, sv, mv, rec=None, late=False):
            o = lp = None
            for c in range(SK // W):
                cs = slice(c * W, (c + 1) * W)
                m = mv[...]
                if c >= cfg["LD"] and sv.shape[0] == S:
                    m = m + _zero_of(lp)
                p = jnp.exp2(sv[:, cs] - _wide(m, W))
                lp = _fold(jnp.add, ([] if lp is None else [lp]) + _tiles(p))
                d = jnp.dot(p.astype(bf16), vb[h & 3, cs, :], preferred_element_type=f32)
                o = d if o is None else o + d
                if rec is not None:
                    rec.done(d)
            if late:
                lp = lp + _zero_of(o)
            l = jnp.sum(lp, axis=-1, keepdims=True)
            r = pl.reciprocal(l, approx=True)
            r = r * (2.0 - l * r)
            return (o * r).astype(bf16)

        def oproj(hos, av, xv=None, rec=None):
            for c in range(D // W):
                cs = slice(c * W, (c + 1) * W)
                a = av[:, cs]
                for h, o in hos:
                    if not isinstance(h, int):
                        a = jnp.where(h > 0, a, 0.0)
                    d = jnp.dot(o, wob[h & 3, :, cs], preferred_element_type=f32)
                    if rec is not None:
                        rec.done(d)
                    a = a + d
                if xv is not None:
                    a = xv[:, cs].astype(f32) + _rep(modv[0, :, cs], a.shape[0]) * a
                av[:, cs] = a

        def matvec(wv, tok=None, step=16):
            n = wv.shape[1]
            part = None if tok is None else _wide(tok, n)
            for r in range(0, D, step):
                t = wv[r:r + step, :].astype(f32) * _wide(cb_buf[r:r + step, :], n)
                for e in range(step // 8):
                    te = t[e * 8:(e + 1) * 8, :]
                    part = te if part is None else part + te
            return _rb(jnp.sum(part, axis=0, keepdims=True))

        def mod_piece(p, tok=None):
            modr[p] = matvec(wmb.at[wm_slot(p)], tok)

        def finish_mod():
            n = D // MC
            ga, sb, cb, gb = (jnp.concatenate([modr[i * n + t] for t in range(n)], axis=-1)
                              for i in range(4))
            cb1 = _rb(1.0 + cb)
            wr = wr_buf[...].astype(f32).reshape(1, D)
            a = cb1 * wr
            a0 = jnp.broadcast_to(jnp.sum(a, axis=-1, keepdims=True), (1, D))
            b0 = jnp.broadcast_to(jnp.sum(sb * wr, axis=-1, keepdims=True), (1, D))
            for i, v in enumerate((ga, sb, cb1, gb, a, gb * cb1, gb * sb, a0, b0)):
                modv[i] = jnp.broadcast_to(v, (8, D))

        def out_rows(x1, mean, inv):
            return (x1 + ((x1 - _wide(mean, D)) * (_wide(inv, D) * modv[5]) + modv[6])).astype(bf16)

        def out_chunks(j):
            x1v, sv, ov = view(acc, j, TL), view(st2_buf, j, TL), view(o_buf, j, TL)

            def chunk(off):
                def f(tok):
                    rs = slice(off, off + 8)
                    ov[rs, :] = out_rows(x1v[rs, :], sv[rs, 0:128] + tok, sv[rs, 128:256] + tok)
                return f
            return [chunk(off) for off in range(0, TL, 8)]

        def epi_chunks(j, x1v, ov, with_out=True):
            sub = lax.broadcasted_iota(i32, (8, 128), 0)
            low = (0xFFFF - j * TL) - sub
            sv = view(st2_buf, j, TL)
            st = {}

            def chunk(off):
                def f(tok=None):
                    if off == 0:
                        st["k1"], st["k2"] = key_buf[0], key_buf[1]
                    x1 = x1v[off:off + 8, :]
                    mean, inv = _row_stats(x1, tok)
                    sv[off:off + 8, 0:128] = mean
                    sv[off:off + 8, 128:256] = inv
                    xa = _tiles(x1 * modv[4])
                    if tok is not None:
                        xa[0] = xa[0] + tok
                    ra = _lane_sum(_fold(jnp.add, xa))
                    r = inv * (ra - mean * modv[7, :, 0:128]) + modv[8, :, 0:128]
                    if with_out:
                        ov[off:off + 8, :] = out_rows(x1, mean, inv)
                    bits = pltpu.bitcast(_rb(r) + 0.0, i32)
                    key = jnp.where(bits < 0, bits ^ 0x7FFF0000, bits) | (low - off)
                    st["k2"] = jnp.maximum(st["k2"], jnp.minimum(st["k1"], key))
                    st["k1"] = jnp.maximum(st["k1"], key)
                    if off + 8 == TL:
                        key_buf[0], key_buf[1] = st["k1"], st["k2"]
                return f
            return [chunk(off) for off in range(0, TL, 8)]

        cp_c().start()
        cp_x(0).start()
        for c in range(2):
            cp_wq0(c).start()
            for i in range(n_mch):
                cp_ca(c, i).start()
            if c == 0:
                for j in range(1, J0):
                    cp_x(j).start()
        cp_sa().start()
        for h in range(G - 1):
            cp_k(h, sem_first.at[1 + h]).start()
        early = []
        for h in range(2):
            early += [cp_v(h, sem_first.at[8 + 2 * h]), cp_wo(h, sem_first.at[9 + 2 * h])]
        for cp in early + head_copies(0):
            cp.start()

        cp_c().wait()
        cf = c_buf[...].astype(f32)
        sc = _rb(cf * jax.nn.sigmoid(cf))
        cb_buf[...] = jnp.transpose(jnp.broadcast_to(sc, (128, D)))
        key_buf[...] = jnp.full(key_buf.shape, _IMIN, i32)
        cp_x(0).wait()

        def st0_body(i, carry):
            for ch in ln1_chunks(view(x_buf, i, T0 // 4), view(st_buf, i, T0 // 4)):
                ch()
            return carry
        lax.fori_loop(0, 4, st0_body, 0)

        def ca_half(c, stream):
            cp_wq0(c).wait()
            if not stream:
                for i in range(n_mch):
                    cp_ca(c, i).wait()
            part = None
            for i in range(n_mch):
                if stream:
                    cp_ca(c, i).wait()
                scb = jnp.broadcast_to(sc[:, i * MCH:(i + 1) * MCH], (16, MCH)).astype(bf16)
                d = jnp.dot(scb, wca[c, i * MCH:(i + 1) * MCH, :], preferred_element_type=f32)
                part = d if part is None else part + d
            mod0[1, :, c * W:(c + 1) * W] = _rb(1.0 + _rb(part[0:8, :]))

        def q_first(r0, t, c, rec, mid=None):
            rows = pl.ds(r0, t)
            cs = slice(c * W, (c + 1) * W)
            hh = ln1_scaled(x_buf[rows, cs], st_buf[rows, :], cs).astype(bf16)
            for g in range(G):
                if mid is not None and g == mid[0]:
                    mid[1]()
                part = jnp.dot(hh, wq0[cs, g * DH:(g + 1) * DH], preferred_element_type=f32)
                qf_buf[g, rows, :] = part if c == 0 else qf_buf[g, rows, :] + part
                if rec is not None:
                    rec.done(part)

        ca_half(0, True)

        def pa_body(j, carry):
            @pl.when(j + 1 < J0)
            def _():
                cp_x(j + 1).wait()
            jn = jnp.minimum(j + 1, J0 - 1)
            rec = _Pace(ln1_chunks(view(x_buf, jn, T0), view(st_buf, jn, T0)), cfg["LCA"])
            q_first(_mul(j, T0), T0, 0, rec)
            return carry
        lax.fori_loop(0, J0, pa_body, 0)

        TB, RB = cfg["TB"], cfg["RB"]
        ca_half(1, False)
        q_first(0, TB, 1, None)
        cp_sa().wait()
        cp_k(0, sem_first.at[1]).wait()

        def sa_chunk(t):
            def f(tok):
                cs = slice(t * 256, (t + 1) * 256)
                mod0[0, :, cs] = jnp.broadcast_to(matvec(wsa.at[:, cs], tok, 8), (8, 256))
            return f

        def sa_bias():
            bq_buf[...] = jnp.dot(_rep(mod0[0], 16).astype(bf16), wq0[...],
                                  preferred_element_type=f32)[0:8, :]

        def h_chunk(off):
            def f(tok):
                rs, rh = slice(off, off + RB), slice(off // 2, (off + RB) // 2)
                hh = (ln1_scaled(x_buf[rs, :], st_buf[rs, :], slice(0, D), tok)
                      + _rep(mod0[0], RB)).astype(bf16)
                h_buf[rh, :] = pltpu.bitcast(hh, u32)
            return f

        def q_chunk(off):
            def f(tok):
                n = 2 * RB
                rs, rh = slice(off, off + n), slice(off // 2, (off + n) // 2)
                for g in range(1, G):
                    q_ring[g, rh, :] = pltpu.bitcast(
                        q_early(g, qf_buf[g, rs, :] + _rep(tok, n)), u32)
            return f

        hs = [h_chunk(off) for off in range(0, S, RB)]
        qs = [q_chunk(off) for off in range(0, S, 2 * RB)]
        nh = cfg["NHB"]
        rest_chunks = []
        nq, nr = len(qs), len(hs) - nh
        for i, ch in enumerate(hs[nh:]):
            rest_chunks.append(ch)
            while qs and (nq - len(qs)) * nr < (i + 1) * nq:
                rest_chunks.append(qs.pop(0))
        assert not qs
        rec = _Pace([sa_chunk(t) for t in range(D // 256)] + hs[:nh], cfg["LCB2"])
        q_first(TB, S - TB, 1, rec, mid=(cfg["BQ"], sa_bias))
        n4 = len(rest_chunks)
        cnt = [n4 // 4 + (1 if i < n4 % 4 else 0) for i in range(4)]
        scores(0, q_early(0, qf_buf[0]), s_buf, m_buf, rec=_Pace(rest_chunks, cnt),
               reload=cfg['RLB'])

        def main_body(h, carry):
            qproj(h + G)
            start_ffn_piece(h)
            for cp in head_copies(h + 1):
                cp.start()
            o = pv(h, s_buf, m_buf)
            rec = _Pace([lambda tok: mod_piece(h, tok)], "1000")
            scores(h + 1, pltpu.bitcast(q_ring[(h + 1) & 3], bf16), s_buf, m_buf, rec=rec,
                   reload=cfg['RLM'])
            oproj([(h, o)], acc)
            for cp in head_copies(h + 1):
                cp.wait()
            return carry
        for h in range(1, G - 1):
            cp_k(h, sem_first.at[1 + h]).wait()
        for cp in early + head_copies(0):
            cp.wait()
        cp_wr().start()
        for p in range(NB + 1, H):
            cp_wm(p).start()
        for p in range(NB, H):
            start_ffn_piece(p)
        lax.fori_loop(0, NB, main_body, 0)

        ha = NB
        rest = list(zip(range(NB + 1, H), (s2_buf, s3_buf, s4_buf), (m2_buf, m3_buf, m4_buf)))
        late = []
        for n, h in enumerate(range(NB + 3, H)):
            late += [cp_v(h, sem_first.at[8 + 2 * n]), cp_wo(h, sem_first.at[9 + 2 * n])]
        for cp in late:
            cp.start()
        cp_wr().wait()
        for p in range(NB + 1, H):
            cp_wm(p).wait()

        def l_step(j, do_x, do_y):
            if do_x and do_y:
                aw = view(acc, j - 1, TL, 2)
                ay, ax = aw.at[0:TL, :], aw.at[TL:2 * TL, :]
            elif do_x:
                ax = view(acc, j, TL)
            else:
                ay = view(acc, j - 1, TL)
            rec = None
            if do_y:
                chunks = epi_chunks(j - 1, ay, view(o_buf, j - 1, TL), with_out=do_x)
                os_ = [(h, pv(h, sv, mv, late=not do_x)) for h, sv, mv in rest]
            if do_x:
                oa = pv(ha, view(s_buf, j, TL), view(m_buf, j, TL))
            if do_y and do_x:
                oproj(os_, ay, view(x_buf, j - 1, TL))
            elif do_y:
                xv = view(x_buf, j - 1, TL)
                r0, prev = 0, []
                for n in cfg["LSPLIT"]:
                    rs = slice(r0, r0 + n)
                    nr = len(os_) * (D // W)
                    cnt = [len(prev) // nr + (1 if i < len(prev) % nr else 0) for i in range(nr)]
                    rec = _Pace(prev, "".join("0123456789abcdefghijklmnopqrstuvwxyz"[i] for i in cnt))
                    oproj([(h, o[rs]) for h, o in os_], ay.at[rs, :], xv.at[rs, :], rec=rec)
                    prev = chunks[r0 // 8:(r0 + n) // 8]
                    r0 += n
                chunks = prev
            if do_x:
                if do_y:
                    rec = _Pace(chunks, cfg["LCNT"])
                for h, sv, mv in rest:
                    q = pltpu.bitcast(view(q_ring.at[h & 3], j, TL // 2)[...], bf16)
                    scores(h, q, sv, mv, rec=rec)
                oproj([(ha, oa)], ax, rec=rec)
            if do_y:
                if do_x:
                    cp_out(j - 1).start()
                else:
                    for ch in chunks:
                        ch()

        for p in range(NB, H):
            mod_piece(p)
        finish_mod()
        l_step(0, True, False)
        for cp in late:
            cp.wait()

        def pl_body(j, carry):
            l_step(j, True, True)
            return carry
        lax.fori_loop(1, JL, pl_body, 0)
        wait_ffn()
        for j in range(JL - 2):
            cp_out(j).wait()
        l_step(JL, False, True)

        k1, k2 = key_buf[0], key_buf[1]
        for sh in (4, 2, 1):
            o1, o2 = pltpu.roll(k1, sh, 0), pltpu.roll(k2, sh, 0)
            k2 = jnp.maximum(jnp.minimum(k1, o1), jnp.maximum(k2, o2))
            k1 = jnp.maximum(k1, o1)

        def score_of(k):
            hi = k & jnp.int32(-65536)
            return pltpu.bitcast(jnp.where(hi < 0, hi ^ 0x7FFF0000, hi), f32)

        i1s = jnp.minimum(0xFFFF - (k1[0, 0] & 0xFFFF), S - 1)
        i2s = jnp.minimum(0xFFFF - (k2[0, 0] & 0xFFFF), S - 1)

        sub = lax.broadcasted_iota(i32, (16, D), 0)
        sb, cb1, gb = (_rep(modv[i], 16) for i in (1, 2, 3))

        def adaln2(x1, stat):
            return (x1 - _wide(stat[:, 0:128], D)) * _wide(stat[:, 128:256], D) * cb1 + sb

        def pick(ref):
            sel = lax.broadcasted_iota(i32, (16, ref.shape[1]), 0) == 0
            return jnp.where(sel, ref[pl.ds(i1s, 1), :], ref[pl.ds(i2s, 1), :])

        xs = adaln2(pick(acc), pick(st2_buf)).astype(bf16)
        FC, lag = cfg["FC"], 2
        y = None
        act = []
        outs = out_chunks(JL - 1)
        for c in range(F // FC + lag):
            if c < F // FC:
                cs = slice(c * FC, (c + 1) * FC)
                g = jnp.dot(xs, wg[:, cs], preferred_element_type=f32)
                u = jnp.dot(xs, wu[:, cs], preferred_element_type=f32)
                for v in (g, u):
                    for t in range(cfg["FOUT"]):
                        if outs:
                            outs.pop(0)(_zero_of(v[0:8, (t % 2) * 128:(t % 2 + 1) * 128]))
                            if not outs:
                                cp_out(JL - 1).start()
                g, u = _rb(g), _rb(u)
                act.append((_rb(g * jax.nn.sigmoid(g)) * u).astype(bf16))
            if c >= lag:
                d = jnp.dot(act[c - lag], wd[(c - lag) * FC:(c - lag + 1) * FC, :],
                            preferred_element_type=f32)
                y = d if y is None else y + d
        y = _rb(y)
        ya = _rb(y[0:1, :] * _wide(_rb(jax.nn.sigmoid(score_of(k1[0:1, :]))), D))
        yb = _rb(y[1:2, :] * _wide(_rb(jax.nn.sigmoid(score_of(k2[0:1, :]))), D))

        g1 = pl.multiple_of((i1s >> 4) << 4, 16)
        g2 = pl.multiple_of((i2s >> 4) << 4, 16)
        for t, g0 in enumerate((g1, g2)):
            rid = sub + g0
            x1 = acc[pl.ds(g0, 16), :]
            upd = jnp.where(rid == i1s, ya, 0.0) + jnp.where(rid == i2s, yb, 0.0)
            fix[t] = (x1 + gb * (adaln2(x1, st2_buf[pl.ds(g0, 16), :]) + upd)).astype(bf16)

        for j in range(JL - 2, JL):
            cp_out(j).wait()

        def cp_fix(t, g0):
            return pltpu.make_async_copy(fix.at[t], out_hbm.at[pl.ds(g0, 16), :], sem_fix.at[t])

        cp_fix(0, g1).start()

        @pl.when(g2 != g1)
        def _():
            cp_fix(1, g2).start()
            cp_fix(1, g2).wait()
        cp_fix(0, g1).wait()

    return kernel


_CFG = dict(FC=256, T0=256, TL=256, MCH=256, LCA='cc80', LCB2='040g', NHB=16, BQ=3, LD=9, TB=1024, RLM=0, RLB=1, RB=16,
            G=4, LSPLIT=(96, 96, 64), FOUT=2, LCNT='33333333332000')


def _build(A_x, A_k_cache, A_v_cache, A_wq, A_wo, B_w_r, B_w_gate, B_w_up, B_w_down, c, w_mod,
           **over):
    B, S, D = A_x.shape
    _, H, SK, DH = A_k_cache.shape
    F = B_w_gate.shape[1]
    assert B == 1
    cfg = dict(_CFG, **over)
    T0, TL, G = cfg["T0"], cfg["TL"], cfg["G"]
    MC = (4 * D) // H
    kernel = _make_kernel(S, D, H, DH, SK, F, cfg)
    scratch = [
        pltpu.VMEM((S, D), bf16),
        pltpu.VMEM((S // 2, D), u32),
        pltpu.VMEM((S, D), f32),
        pltpu.VMEM((S, SK), f32),
        pltpu.VMEM((S, 128), f32),
        pltpu.VMEM((TL, SK), f32),
        pltpu.VMEM((TL, 128), f32),
        pltpu.VMEM((TL, SK), f32),
        pltpu.VMEM((TL, 128), f32),
        pltpu.VMEM((TL, SK), f32),
        pltpu.VMEM((TL, 128), f32),
        pltpu.VMEM((S, 256), f32),
        pltpu.VMEM((S, 256), f32),
        pltpu.VMEM((4, S // 2, DH), u32),
        pltpu.VMEM((G, S, DH), f32),
        pltpu.VMEM((8, G * DH), f32),
        pltpu.VMEM((4, SK, DH), bf16),
        pltpu.VMEM((4, SK, DH), bf16),
        pltpu.VMEM((D, G * DH), bf16),
        pltpu.VMEM((2, D, DH), bf16),
        pltpu.VMEM((4, DH, D), bf16),
        pltpu.VMEM((G + 1, D, MC), bf16),
        pltpu.VMEM((2, D, D // 2), bf16),
        pltpu.VMEM((D, D), bf16),
        pltpu.VMEM((1, D), bf16),
        pltpu.VMEM((D,), bf16),
        pltpu.VMEM((D, 128), f32),
        pltpu.VMEM((2, 8, D), f32),
        pltpu.VMEM((H, 1, MC), f32),
        pltpu.VMEM((9, 8, D), f32),
        pltpu.VMEM((D, F), bf16),
        pltpu.VMEM((D, F), bf16),
        pltpu.VMEM((F, D), bf16),
        pltpu.VMEM((S, D), bf16),
        pltpu.VMEM((2, 8, 128), i32),
        pltpu.VMEM((2, 16, D), bf16),
        pltpu.SemaphoreType.DMA((sum(_sem_sizes(S, D, cfg)),)),
    ]
    any_spec = pl.BlockSpec(memory_space=pl.ANY)
    out = pl.pallas_call(
        kernel,
        out_shape=jax.ShapeDtypeStruct((S, D), bf16),
        in_specs=[any_spec] * 11,
        out_specs=any_spec,
        scratch_shapes=scratch,
        compiler_params=pltpu.CompilerParams(vmem_limit_bytes=112 * 1024 * 1024,
                                             disable_bounds_checks=True,
                                             disable_semaphore_checks=True),
    )(A_x.reshape(S, D), A_k_cache.reshape(H, SK, DH), A_v_cache.reshape(H, SK, DH),
      A_wq, A_wo, B_w_r, B_w_gate, B_w_up, B_w_down, c, w_mod)
    return out.reshape(B, S, D)


@jax.jit
def pallas_adaLN_cond__mha_block_cached__moe_arch_mod__prompt_kernel(
    A_x: jax.Array,
    A_k_cache: jax.Array,
    A_v_cache: jax.Array,
    A_wq: jax.Array,
    A_wo: jax.Array,
    B_x: jax.Array,
    B_w_r: jax.Array,
    B_w_gate: jax.Array,
    B_w_up: jax.Array,
    B_w_down: jax.Array,
    c: jax.Array,
    w_mod: jax.Array,
):
    del B_x
    return _build(A_x, A_k_cache, A_v_cache, A_wq, A_wo, B_w_r, B_w_gate, B_w_up, B_w_down,
                  c, w_mod)
```

```python
import jax
import jax.numpy as jnp
from jax import lax
import jax.experimental.pallas as pl
import jax.experimental.pallas.tpu as pltpu

f32 = jnp.float32
bf16 = jnp.bfloat16
u32 = jnp.uint32
i32 = jnp.int32

_NT = (((1,), (1,)), ((), ()))
_LOG2E = 1.4426950408889634
_EPS = 1e-5
_IMIN = -2 ** 31


def _rb(v):
    return v.astype(bf16).astype(f32)


def _rep(v, n):
    return v if n == 8 else jnp.tile(v, (n // 8, 1))


def _wide(v, w):
    return jnp.tile(v, (1, w // 128))


def _zero_of(v):
    bits = pltpu.bitcast(v, u32)
    return pltpu.bitcast(lax.shift_right_logical(lax.shift_right_logical(bits, jnp.uint32(31)),
                                                 jnp.uint32(1)), f32)


class _Pace:
    def __init__(self, chunks, counts):
        self.chunks = list(chunks)
        self.counts = [ch if isinstance(ch, int) else int(ch, 36) for ch in counts]
        assert sum(self.counts) == len(self.chunks), (counts, len(self.chunks))

    def done(self, res):
        n = self.counts.pop(0)
        for i in range(n):
            r0 = (i * res.shape[0] // n) // 8 * 8
            self.chunks.pop(0)(_zero_of(res[r0:r0 + 8, 0:128]))


def _tiles(v):
    return [v[:, c * 128:(c + 1) * 128] for c in range(v.shape[1] // 128)]


def _fold(op, parts):
    out = parts[0]
    for p in parts[1:]:
        out = op(out, p)
    return out


def _lane_sum(v):
    return jnp.broadcast_to(jnp.sum(v, axis=-1, keepdims=True), v.shape)


def _row_stats(xf, tok=None):
    d = xf.shape[-1]
    ts = _tiles(xf)
    nt = len(ts)
    if tok is not None:
        ts = [ts[0] + tok] + ts[1:]
    mu = _fold(jnp.add, ts) * (1.0 / nt)
    m2 = _fold(jnp.add, [(t - mu) * (t - mu) for t in ts])
    mean = _lane_sum(mu) * (1.0 / 128)
    dm = mu - mean
    var = _lane_sum(m2 + (dm * dm) * float(nt)) * (1.0 / d)
    return mean, lax.rsqrt(var + _EPS)


def _sem_sizes(S, D, cfg):
    j0 = S // cfg["T0"]
    return [2, 2 * (D // cfg["MCH"]), j0, 1, 16, 5, 3, S // cfg["TL"], 2]


def _make_kernel(S, D, H, DH, SK, F, cfg):
    T0, TL, MCH = cfg["T0"], cfg["TL"], cfg["MCH"]
    J0 = S // T0
    JL = S // TL
    qscale = DH ** -0.5 * _LOG2E
    n_mch = D // MCH
    G = cfg["G"]
    NB = H - G
    MC = (4 * D) // H
    W = 512
    assert 2 <= G <= 4 and D == 2 * W

    def kernel(x_hbm, k_hbm, v_hbm, wq_hbm, wo_hbm, wr_hbm, wg_hbm, wu_hbm, wd_hbm,
               c_hbm, wmod_hbm, out_hbm,
               x_buf, h_buf, acc, s_buf, m_buf, s2_buf, m2_buf, s3_buf, m3_buf, s4_buf, m4_buf,
               st_buf, st2_buf,
               q_ring, qf_buf, bq_buf,
               kb, vb, wq0, wqb, wob, wmb, wca, wsa, c_buf, wr_buf, cb_buf, mod0, modr, modv,
               wg, wu, wd, o_buf, key_buf, fix,
               sems):

        class _Sem:
            def __init__(self, base):
                self.base = base
                self.at = self

            def __getitem__(self, i):
                return sems.at[self.base + i]

        sizes = _sem_sizes(S, D, cfg)
        offs = [sum(sizes[:i]) for i in range(len(sizes))]
        (sem_small, sem_ca, sem_x, sem_sa, sem_first, sem_head,
         sem_ffn, sem_out, sem_fix) = (_Sem(o) for o in offs)

        def _mul(a, n):
            v = a * n
            return v if isinstance(a, int) else pl.multiple_of(v, n)

        def view(ref, j, t, n=1):
            return ref.at[pl.ds(_mul(j, t), n * t), :]

        def cp_c():
            return pltpu.make_async_copy(c_hbm, c_buf, sem_small.at[0])

        def cp_wr():
            return pltpu.make_async_copy(wr_hbm, wr_buf, sem_small.at[1])

        def cp_ca(c, i):
            return pltpu.make_async_copy(
                wmod_hbm.at[pl.ds(i * MCH, MCH), pl.ds(D + c * W, W)], view(wca.at[c], i, MCH),
                sem_ca.at[c * n_mch + i])

        def cp_sa():
            return pltpu.make_async_copy(wmod_hbm.at[:, pl.ds(0, D)], wsa, sem_sa.at[0])

        def cp_x(j):
            return pltpu.make_async_copy(view(x_hbm, j, T0), view(x_buf, j, T0), sem_x.at[j])

        def cp_wq0(c):
            return pltpu.make_async_copy(wq_hbm.at[pl.ds(c * W, W), pl.ds(0, G * DH)],
                                         view(wq0, c, W), sem_first.at[14 + c])

        def cp_k(h, sem=None):
            return pltpu.make_async_copy(k_hbm.at[h], kb.at[h & 3],
                                         sem_head.at[0] if sem is None else sem)

        def cp_wq(h):
            src = h if isinstance(h, int) else jnp.minimum(h, H - 1)
            return pltpu.make_async_copy(wq_hbm.at[:, pl.ds(_mul(src, DH), DH)], wqb.at[h & 1],
                                         sem_head.at[1])

        def cp_v(h, sem=None):
            return pltpu.make_async_copy(v_hbm.at[h], vb.at[h & 3],
                                         sem_head.at[2] if sem is None else sem)

        def cp_wo(h, sem=None):
            return pltpu.make_async_copy(view(wo_hbm, h, DH), wob.at[h & 3],
                                         sem_head.at[3] if sem is None else sem)

        def wm_slot(p):
            return p - NB + 1 if (isinstance(p, int) and p > NB) else p & 1

        def cp_wm(p):
            extra = isinstance(p, int) and p > NB
            return pltpu.make_async_copy(
                wmod_hbm.at[:, pl.ds(_mul(p + (2 * D) // MC, MC), MC)], wmb.at[wm_slot(p)],
                sem_first.at[4 + p - NB] if extra else sem_head.at[4])

        ffn = ((wg_hbm, wg), (wu_hbm, wu), (wd_hbm, wd))

        def start_ffn_piece(p):
            for i, (src, dst) in enumerate(ffn):
                n = src.shape[0] // H
                pltpu.make_async_copy(view(src, p, n), view(dst, p, n), sem_ffn.at[i]).start()

        def wait_ffn():
            for i, (src, dst) in enumerate(ffn):
                pltpu.make_async_copy(src, dst, sem_ffn.at[i]).wait()

        def cp_out(j):
            return pltpu.make_async_copy(view(o_buf, j, TL), view(out_hbm, j, TL), sem_out.at[j])

        def head_copies(h):
            return [cp_wq(h + G), cp_k(h + G - 1), cp_wo(h + 2), cp_wm(h), cp_v(h + 2)]

        def ln1_chunks(xv, sv):
            def chunk(off):
                def f(tok=None):
                    mean, inv = _row_stats(xv[off:off + 8, :].astype(f32), tok)
                    sv[off:off + 8, 0:128] = mean
                    sv[off:off + 8, 128:256] = inv
                return f
            return [chunk(off) for off in range(0, xv.shape[0], 8)]

        def ln1_scaled(x, stat, cs, tok=None):
            w = x.shape[1]
            mean = stat[:, 0:128] if tok is None else stat[:, 0:128] + _rep(tok, x.shape[0])
            n = (x.astype(f32) - _wide(mean, w)) * _wide(stat[:, 128:256], w)
            return n * _rep(mod0[1, :, cs], x.shape[0])

        def qproj(h):
            q = None
            for c in range(D // W):
                cs = slice(c * W, (c + 1) * W)
                part = jnp.dot(pltpu.bitcast(h_buf[:, cs], bf16), wqb[h & 1, cs, :],
                               preferred_element_type=f32)
                q = part if q is None else q + part
            q_ring[h & 3] = pltpu.bitcast((q * qscale).astype(bf16), u32)

        def q_early(g, q):
            return ((q + _rep(bq_buf[:, g * DH:(g + 1) * DH], q.shape[0])) * qscale).astype(bf16)

        def scores(h, q, sv, mv, rec=None, reload=False):
            mp = None
            for c in range(SK // W):
                cs = slice(c * W, (c + 1) * W)
                s = lax.dot_general(q, kb[h & 3, cs, :], _NT, preferred_element_type=f32)
                sv[:, cs] = s
                if rec is not None:
                    rec.done(s)
                if not reload:
                    mp = _fold(jnp.maximum, ([] if mp is None else [mp]) + _tiles(s))
            if reload:
                mp = _fold(jnp.maximum, _tiles(sv[...]))
            mv[...] = jnp.broadcast_to(jnp.max(mp, axis=-1, keepdims=True), mp.shape)

        def pv(h, sv, mv, rec=None, late=False):
            o = lp = None
            for c in range(SK // W):
                cs = slice(c * W, (c + 1) * W)
                m = mv[...]
                if c >= cfg["LD"] and sv.shape[0] == S:
                    m = m + _zero_of(lp)
                p = jnp.exp2(sv[:, cs] - _wide(m, W))
                lp = _fold(jnp.add, ([] if lp is None else [lp]) + _tiles(p))
                d = jnp.dot(p.astype(bf16), vb[h & 3, cs, :], preferred_element_type=f32)
                o = d if o is None else o + d
                if rec is not None:
                    rec.done(d)
            if late:
                lp = lp + _zero_of(o)
            l = jnp.sum(lp, axis=-1, keepdims=True)
            r = pl.reciprocal(l, approx=True)
            r = r * (2.0 - l * r)
            return (o * r).astype(bf16)

        def oproj(hos, av, xv=None, rec=None):
            for c in range(D // W):
                cs = slice(c * W, (c + 1) * W)
                a = av[:, cs]
                for h, o in hos:
                    if not isinstance(h, int):
                        a = jnp.where(h > 0, a, 0.0)
                    d = jnp.dot(o, wob[h & 3, :, cs], preferred_element_type=f32)
                    if rec is not None:
                        rec.done(d)
                    a = a + d
                if xv is not None:
                    a = xv[:, cs].astype(f32) + _rep(modv[0, :, cs], a.shape[0]) * a
                av[:, cs] = a

        def matvec(wv, tok=None, step=16):
            n = wv.shape[1]
            part = None if tok is None else _wide(tok, n)
            for r in range(0, D, step):
                t = wv[r:r + step, :].astype(f32) * _wide(cb_buf[r:r + step, :], n)
                for e in range(step // 8):
                    te = t[e * 8:(e + 1) * 8, :]
                    part = te if part is None else part + te
            return _rb(jnp.sum(part, axis=0, keepdims=True))

        def mod_piece(p, tok=None):
            modr[p] = matvec(wmb.at[wm_slot(p)], tok)

        def finish_mod():
            n = D // MC
            ga, sb, cb, gb = (jnp.concatenate([modr[i * n + t] for t in range(n)], axis=-1)
                              for i in range(4))
            cb1 = _rb(1.0 + cb)
            wr = wr_buf[...].astype(f32).reshape(1, D)
            a = cb1 * wr
            a0 = jnp.broadcast_to(jnp.sum(a, axis=-1, keepdims=True), (1, D))
            b0 = jnp.broadcast_to(jnp.sum(sb * wr, axis=-1, keepdims=True), (1, D))
            for i, v in enumerate((ga, sb, cb1, gb, a, gb * cb1, gb * sb, a0, b0)):
                modv[i] = jnp.broadcast_to(v, (8, D))

        def out_rows(x1, mean, inv):
            return (x1 + ((x1 - _wide(mean, D)) * (_wide(inv, D) * modv[5]) + modv[6])).astype(bf16)

        def out_chunks(j):
            x1v, sv, ov = view(acc, j, TL), view(st2_buf, j, TL), view(o_buf, j, TL)

            def chunk(off):
                def f(tok):
                    rs = slice(off, off + 8)
                    ov[rs, :] = out_rows(x1v[rs, :], sv[rs, 0:128] + tok, sv[rs, 128:256] + tok)
                return f
            return [chunk(off) for off in range(0, TL, 8)]

        def epi_chunks(j, x1v, ov, with_out=True):
            sub = lax.broadcasted_iota(i32, (8, 128), 0)
            low = (0xFFFF - j * TL) - sub
            sv = view(st2_buf, j, TL)
            st = {}

            def chunk(off):
                def f(tok=None):
                    if off == 0:
                        st["k1"], st["k2"] = key_buf[0], key_buf[1]
                    x1 = x1v[off:off + 8, :]
                    mean, inv = _row_stats(x1, tok)
                    sv[off:off + 8, 0:128] = mean
                    sv[off:off + 8, 128:256] = inv
                    xa = _tiles(x1 * modv[4])
                    if tok is not None:
                        xa[0] = xa[0] + tok
                    ra = _lane_sum(_fold(jnp.add, xa))
                    r = inv * (ra - mean * modv[7, :, 0:128]) + modv[8, :, 0:128]
                    if with_out:
                        ov[off:off + 8, :] = out_rows(x1, mean, inv)
                    bits = pltpu.bitcast(_rb(r) + 0.0, i32)
                    key = jnp.where(bits < 0, bits ^ 0x7FFF0000, bits) | (low - off)
                    st["k2"] = jnp.maximum(st["k2"], jnp.minimum(st["k1"], key))
                    st["k1"] = jnp.maximum(st["k1"], key)
                    if off + 8 == TL:
                        key_buf[0], key_buf[1] = st["k1"], st["k2"]
                return f
            return [chunk(off) for off in range(0, TL, 8)]

        cp_c().start()
        cp_x(0).start()
        for c in range(2):
            cp_wq0(c).start()
            for i in range(n_mch):
                cp_ca(c, i).start()
            if c == 0:
                for j in range(1, J0):
                    cp_x(j).start()
        cp_sa().start()
        for h in range(G - 1):
            cp_k(h, sem_first.at[1 + h]).start()
        early = []
        for h in range(2):
            early += [cp_v(h, sem_first.at[8 + 2 * h]), cp_wo(h, sem_first.at[9 + 2 * h])]
        for cp in early + head_copies(0):
            cp.start()

        cp_c().wait()
        cf = c_buf[...].astype(f32)
        sc = _rb(cf * jax.nn.sigmoid(cf))
        cb_buf[...] = jnp.transpose(jnp.broadcast_to(sc, (128, D)))
        key_buf[...] = jnp.full(key_buf.shape, _IMIN, i32)
        cp_x(0).wait()

        def st0_body(i, carry):
            for ch in ln1_chunks(view(x_buf, i, T0 // 4), view(st_buf, i, T0 // 4)):
                ch()
            return carry
        lax.fori_loop(0, 4, st0_body, 0)

        def ca_half(c, stream):
            cp_wq0(c).wait()
            if not stream:
                for i in range(n_mch):
                    cp_ca(c, i).wait()
            part = None
            for i in range(n_mch):
                if stream:
                    cp_ca(c, i).wait()
                scb = jnp.broadcast_to(sc[:, i * MCH:(i + 1) * MCH], (16, MCH)).astype(bf16)
                d = jnp.dot(scb, wca[c, i * MCH:(i + 1) * MCH, :], preferred_element_type=f32)
                part = d if part is None else part + d
            mod0[1, :, c * W:(c + 1) * W] = _rb(1.0 + _rb(part[0:8, :]))

        def q_first(r0, t, c, rec, mid=None):
            rows = pl.ds(r0, t)
            cs = slice(c * W, (c + 1) * W)
            hh = ln1_scaled(x_buf[rows, cs], st_buf[rows, :], cs).astype(bf16)
            for g in range(G):
                if mid is not None and g == mid[0]:
                    mid[1]()
                part = jnp.dot(hh, wq0[cs, g * DH:(g + 1) * DH], preferred_element_type=f32)
                qf_buf[g, rows, :] = part if c == 0 else qf_buf[g, rows, :] + part
                if rec is not None:
                    rec.done(part)

        ca_half(0, True)

        def pa_body(j, carry):
            @pl.when(j + 1 < J0)
            def _():
                cp_x(j + 1).wait()
            jn = jnp.minimum(j + 1, J0 - 1)
            rec = _Pace(ln1_chunks(view(x_buf, jn, T0), view(st_buf, jn, T0)), cfg["LCA"])
            q_first(_mul(j, T0), T0, 0, rec)
            return carry
        lax.fori_loop(0, J0, pa_body, 0)

        TB, RB = cfg["TB"], cfg["RB"]
        ca_half(1, False)
        q_first(0, TB, 1, None)
        cp_sa().wait()
        cp_k(0, sem_first.at[1]).wait()
        cp_wr().start()
        for p in range(NB + 1, H):
            cp_wm(p).start()
        for p in range(NB, H):
            start_ffn_piece(p)

        def sa_chunk(t):
            def f(tok):
                cs = slice(t * 256, (t + 1) * 256)
                mod0[0, :, cs] = jnp.broadcast_to(matvec(wsa.at[:, cs], tok, 8), (8, 256))
            return f

        def sa_bias():
            bq_buf[...] = jnp.dot(_rep(mod0[0], 16).astype(bf16), wq0[...],
                                  preferred_element_type=f32)[0:8, :]

        def h_chunk(off):
            def f(tok):
                rs, rh = slice(off, off + RB), slice(off // 2, (off + RB) // 2)
                hh = (ln1_scaled(x_buf[rs, :], st_buf[rs, :], slice(0, D), tok)
                      + _rep(mod0[0], RB)).astype(bf16)
                h_buf[rh, :] = pltpu.bitcast(hh, u32)
            return f

        def q_chunk(off):
            def f(tok):
                n = 2 * RB
                rs, rh = slice(off, off + n), slice(off // 2, (off + n) // 2)
                for g in range(1, G):
                    q_ring[g, rh, :] = pltpu.bitcast(
                        q_early(g, qf_buf[g, rs, :] + _rep(tok, n)), u32)
            return f

        hs = [h_chunk(off) for off in range(0, S, RB)]
        qs = [q_chunk(off) for off in range(0, S, 2 * RB)]
        nh = cfg["NHB"]
        rest_chunks = []
        nq, nr = len(qs), len(hs) - nh
        for i, ch in enumerate(hs[nh:]):
            rest_chunks.append(ch)
            while qs and (nq - len(qs)) * nr < (i + 1) * nq:
                rest_chunks.append(qs.pop(0))
        assert not qs
        rec = _Pace([sa_chunk(t) for t in range(D // 256)] + hs[:nh], cfg["LCB2"])
        q_first(TB, S - TB, 1, rec, mid=(cfg["BQ"], sa_bias))
        n4 = len(rest_chunks)
        n3 = n4 - cfg["NL4"]
        cnt = [n3 // 3 + (1 if i < n3 % 3 else 0) for i in range(3)] + [cfg["NL4"]]
        scores(0, q_early(0, qf_buf[0]), s_buf, m_buf, rec=_Pace(rest_chunks, cnt),
               reload=cfg['RLB'])

        def main_body(h, carry):
            qproj(h + G)
            start_ffn_piece(h)
            for cp in head_copies(h + 1):
                cp.start()
            o = pv(h, s_buf, m_buf)
            rec = _Pace([lambda tok: mod_piece(h, tok)], "1000")
            scores(h + 1, pltpu.bitcast(q_ring[(h + 1) & 3], bf16), s_buf, m_buf, rec=rec,
                   reload=cfg['RLM'])
            oproj([(h, o)], acc)
            for cp in head_copies(h + 1):
                cp.wait()
            return carry
        for h in range(1, G - 1):
            cp_k(h, sem_first.at[1 + h]).wait()
        for cp in early + head_copies(0):
            cp.wait()
        lax.fori_loop(0, NB, main_body, 0)

        ha = NB
        rest = list(zip(range(NB + 1, H), (s2_buf, s3_buf, s4_buf), (m2_buf, m3_buf, m4_buf)))
        late = []
        for n, h in enumerate(range(NB + 3, H)):
            late += [cp_v(h, sem_first.at[8 + 2 * n]), cp_wo(h, sem_first.at[9 + 2 * n])]
        for cp in late:
            cp.start()
        cp_wr().wait()
        for p in range(NB + 1, H):
            cp_wm(p).wait()

        def l_step(j, do_x, do_y):
            if do_x and do_y:
                aw = view(acc, j - 1, TL, 2)
                ay, ax = aw.at[0:TL, :], aw.at[TL:2 * TL, :]
            elif do_x:
                ax = view(acc, j, TL)
            else:
                ay = view(acc, j - 1, TL)
            rec = None
            if do_y:
                chunks = epi_chunks(j - 1, ay, view(o_buf, j - 1, TL), with_out=do_x)
                os_ = [(h, pv(h, sv, mv, late=not do_x)) for h, sv, mv in rest]
            if do_x:
                oa = pv(ha, view(s_buf, j, TL), view(m_buf, j, TL))
            if do_y and do_x:
                oproj(os_, ay, view(x_buf, j - 1, TL))
            elif do_y:
                xv = view(x_buf, j - 1, TL)
                r0, prev = 0, []
                for n in cfg["LSPLIT"]:
                    rs = slice(r0, r0 + n)
                    nr = len(os_) * (D // W)
                    cnt = [len(prev) // nr + (1 if i < len(prev) % nr else 0) for i in range(nr)]
                    rec = _Pace(prev, "".join("0123456789abcdefghijklmnopqrstuvwxyz"[i] for i in cnt))
                    oproj([(h, o[rs]) for h, o in os_], ay.at[rs, :], xv.at[rs, :], rec=rec)
                    prev = chunks[r0 // 8:(r0 + n) // 8]
                    r0 += n
                chunks = prev
            if do_x:
                if do_y:
                    rec = _Pace(chunks, cfg["LCNT"])
                for h, sv, mv in rest:
                    q = pltpu.bitcast(view(q_ring.at[h & 3], j, TL // 2)[...], bf16)
                    scores(h, q, sv, mv, rec=rec, reload=cfg['RLL'])
                oproj([(ha, oa)], ax, rec=rec)
            if do_y:
                if do_x:
                    cp_out(j - 1).start()
                else:
                    for ch in chunks:
                        ch()

        for p in range(NB, H):
            mod_piece(p)
        finish_mod()
        l_step(0, True, False)
        for cp in late:
            cp.wait()

        def pl_body(j, carry):
            l_step(j, True, True)
            return carry
        lax.fori_loop(1, JL, pl_body, 0)
        wait_ffn()
        for j in range(JL - 2):
            cp_out(j).wait()
        l_step(JL, False, True)

        k1, k2 = key_buf[0], key_buf[1]
        for sh in (4, 2, 1):
            o1, o2 = pltpu.roll(k1, sh, 0), pltpu.roll(k2, sh, 0)
            k2 = jnp.maximum(jnp.minimum(k1, o1), jnp.maximum(k2, o2))
            k1 = jnp.maximum(k1, o1)

        def score_of(k):
            hi = k & jnp.int32(-65536)
            return pltpu.bitcast(jnp.where(hi < 0, hi ^ 0x7FFF0000, hi), f32)

        i1s = jnp.minimum(0xFFFF - (k1[0, 0] & 0xFFFF), S - 1)
        i2s = jnp.minimum(0xFFFF - (k2[0, 0] & 0xFFFF), S - 1)

        sub = lax.broadcasted_iota(i32, (16, D), 0)
        sb, cb1, gb = (_rep(modv[i], 16) for i in (1, 2, 3))

        def adaln2(x1, stat):
            return (x1 - _wide(stat[:, 0:128], D)) * _wide(stat[:, 128:256], D) * cb1 + sb

        def pick(ref):
            sel = lax.broadcasted_iota(i32, (16, ref.shape[1]), 0) == 0
            return jnp.where(sel, ref[pl.ds(i1s, 1), :], ref[pl.ds(i2s, 1), :])

        xs = adaln2(pick(acc), pick(st2_buf)).astype(bf16)
        FC, lag = cfg["FC"], 2
        y = None
        act = []
        outs = out_chunks(JL - 1)
        for c in range(F // FC + lag):
            if c < F // FC:
                cs = slice(c * FC, (c + 1) * FC)
                g = jnp.dot(xs, wg[:, cs], preferred_element_type=f32)
                u = jnp.dot(xs, wu[:, cs], preferred_element_type=f32)
                for v in (g, u):
                    for t in range(cfg["FOUT"]):
                        if outs:
                            outs.pop(0)(_zero_of(v[0:8, (t % 2) * 128:(t % 2 + 1) * 128]))
                            if not outs:
                                cp_out(JL - 1).start()
                g, u = _rb(g), _rb(u)
                act.append((_rb(g * jax.nn.sigmoid(g)) * u).astype(bf16))
            if c >= lag:
                d = jnp.dot(act[c - lag], wd[(c - lag) * FC:(c - lag + 1) * FC, :],
                            preferred_element_type=f32)
                y = d if y is None else y + d
        y = _rb(y)
        ya = _rb(y[0:1, :] * _wide(_rb(jax.nn.sigmoid(score_of(k1[0:1, :]))), D))
        yb = _rb(y[1:2, :] * _wide(_rb(jax.nn.sigmoid(score_of(k2[0:1, :]))), D))

        g1 = pl.multiple_of((i1s >> 4) << 4, 16)
        g2 = pl.multiple_of((i2s >> 4) << 4, 16)
        for t, g0 in enumerate((g1, g2)):
            rid = sub + g0
            x1 = acc[pl.ds(g0, 16), :]
            upd = jnp.where(rid == i1s, ya, 0.0) + jnp.where(rid == i2s, yb, 0.0)
            fix[t] = (x1 + gb * (adaln2(x1, st2_buf[pl.ds(g0, 16), :]) + upd)).astype(bf16)

        for j in range(JL - 2, JL):
            cp_out(j).wait()

        def cp_fix(t, g0):
            return pltpu.make_async_copy(fix.at[t], out_hbm.at[pl.ds(g0, 16), :], sem_fix.at[t])

        cp_fix(0, g1).start()

        @pl.when(g2 != g1)
        def _():
            cp_fix(1, g2).start()
            cp_fix(1, g2).wait()
        cp_fix(0, g1).wait()

    return kernel


_CFG = dict(FC=256, T0=256, TL=256, MCH=256, LCA='cc80', LCB2='040g', NHB=16, NL4=8, BQ=3, LD=9, TB=1024, RLM=1, RLL=1, RLB=1, RB=16,
            G=4, LSPLIT=(96, 96, 64), FOUT=2, LCNT='33333333332000')


def _build(A_x, A_k_cache, A_v_cache, A_wq, A_wo, B_w_r, B_w_gate, B_w_up, B_w_down, c, w_mod,
           **over):
    B, S, D = A_x.shape
    _, H, SK, DH = A_k_cache.shape
    F = B_w_gate.shape[1]
    assert B == 1
    cfg = dict(_CFG, **over)
    T0, TL, G = cfg["T0"], cfg["TL"], cfg["G"]
    MC = (4 * D) // H
    kernel = _make_kernel(S, D, H, DH, SK, F, cfg)
    scratch = [
        pltpu.VMEM((S, D), bf16),
        pltpu.VMEM((S // 2, D), u32),
        pltpu.VMEM((S, D), f32),
        pltpu.VMEM((S, SK), f32),
        pltpu.VMEM((S, 128), f32),
        pltpu.VMEM((TL, SK), f32),
        pltpu.VMEM((TL, 128), f32),
        pltpu.VMEM((TL, SK), f32),
        pltpu.VMEM((TL, 128), f32),
        pltpu.VMEM((TL, SK), f32),
        pltpu.VMEM((TL, 128), f32),
        pltpu.VMEM((S, 256), f32),
        pltpu.VMEM((S, 256), f32),
        pltpu.VMEM((4, S // 2, DH), u32),
        pltpu.VMEM((G, S, DH), f32),
        pltpu.VMEM((8, G * DH), f32),
        pltpu.VMEM((4, SK, DH), bf16),
        pltpu.VMEM((4, SK, DH), bf16),
        pltpu.VMEM((D, G * DH), bf16),
        pltpu.VMEM((2, D, DH), bf16),
        pltpu.VMEM((4, DH, D), bf16),
        pltpu.VMEM((G + 1, D, MC), bf16),
        pltpu.VMEM((2, D, D // 2), bf16),
        pltpu.VMEM((D, D), bf16),
        pltpu.VMEM((1, D), bf16),
        pltpu.VMEM((D,), bf16),
        pltpu.VMEM((D, 128), f32),
        pltpu.VMEM((2, 8, D), f32),
        pltpu.VMEM((H, 1, MC), f32),
        pltpu.VMEM((9, 8, D), f32),
        pltpu.VMEM((D, F), bf16),
        pltpu.VMEM((D, F), bf16),
        pltpu.VMEM((F, D), bf16),
        pltpu.VMEM((S, D), bf16),
        pltpu.VMEM((2, 8, 128), i32),
        pltpu.VMEM((2, 16, D), bf16),
        pltpu.SemaphoreType.DMA((sum(_sem_sizes(S, D, cfg)),)),
    ]
    any_spec = pl.BlockSpec(memory_space=pl.ANY)
    out = pl.pallas_call(
        kernel,
        out_shape=jax.ShapeDtypeStruct((S, D), bf16),
        in_specs=[any_spec] * 11,
        out_specs=any_spec,
        scratch_shapes=scratch,
        compiler_params=pltpu.CompilerParams(vmem_limit_bytes=112 * 1024 * 1024,
                                             disable_bounds_checks=True,
                                             disable_semaphore_checks=True),
    )(A_x.reshape(S, D), A_k_cache.reshape(H, SK, DH), A_v_cache.reshape(H, SK, DH),
      A_wq, A_wo, B_w_r, B_w_gate, B_w_up, B_w_down, c, w_mod)
    return out.reshape(B, S, D)


@jax.jit
def pallas_adaLN_cond__mha_block_cached__moe_arch_mod__prompt_kernel(
    A_x: jax.Array,
    A_k_cache: jax.Array,
    A_v_cache: jax.Array,
    A_wq: jax.Array,
    A_wo: jax.Array,
    B_x: jax.Array,
    B_w_r: jax.Array,
    B_w_gate: jax.Array,
    B_w_up: jax.Array,
    B_w_down: jax.Array,
    c: jax.Array,
    w_mod: jax.Array,
):
    del B_x
    return _build(A_x, A_k_cache, A_v_cache, A_wq, A_wo, B_w_r, B_w_gate, B_w_up, B_w_down,
                  c, w_mod)
```

```python
import jax
import jax.numpy as jnp
from jax import lax
import jax.experimental.pallas as pl
import jax.experimental.pallas.tpu as pltpu

f32 = jnp.float32
bf16 = jnp.bfloat16
u32 = jnp.uint32
i32 = jnp.int32

_NT = (((1,), (1,)), ((), ()))
_LOG2E = 1.4426950408889634
_EPS = 1e-5
_IMIN = -2 ** 31


def _rb(v):
    return v.astype(bf16).astype(f32)


def _rep(v, n):
    return v if n == 8 else jnp.tile(v, (n // 8, 1))


def _wide(v, w):
    return jnp.tile(v, (1, w // 128))


def _zero_of(v):
    bits = pltpu.bitcast(v, u32)
    return pltpu.bitcast(lax.shift_right_logical(lax.shift_right_logical(bits, jnp.uint32(31)),
                                                 jnp.uint32(1)), f32)


class _Pace:
    def __init__(self, chunks, counts):
        self.chunks = list(chunks)
        self.counts = [ch if isinstance(ch, int) else int(ch, 36) for ch in counts]
        assert sum(self.counts) == len(self.chunks), (counts, len(self.chunks))

    def done(self, res):
        n = self.counts.pop(0)
        for i in range(n):
            r0 = (i * res.shape[0] // n) // 8 * 8
            self.chunks.pop(0)(_zero_of(res[r0:r0 + 8, 0:128]))


def _tiles(v):
    return [v[:, c * 128:(c + 1) * 128] for c in range(v.shape[1] // 128)]


def _fold(op, parts):
    out = parts[0]
    for p in parts[1:]:
        out = op(out, p)
    return out


def _lane_sum(v):
    return jnp.broadcast_to(jnp.sum(v, axis=-1, keepdims=True), v.shape)


def _row_stats(xf, tok=None):
    d = xf.shape[-1]
    ts = _tiles(xf)
    nt = len(ts)
    if tok is not None:
        ts = [ts[0] + tok] + ts[1:]
    mu = _fold(jnp.add, ts) * (1.0 / nt)
    m2 = _fold(jnp.add, [(t - mu) * (t - mu) for t in ts])
    mean = _lane_sum(mu) * (1.0 / 128)
    dm = mu - mean
    var = _lane_sum(m2 + (dm * dm) * float(nt)) * (1.0 / d)
    return mean, lax.rsqrt(var + _EPS)


def _sem_sizes(S, D, cfg):
    j0 = S // cfg["T0"]
    return [2, 2 * (D // cfg["MCH"]), j0, 1, 16, 5, 3, S // cfg["TL"], 2]


def _make_kernel(S, D, H, DH, SK, F, cfg):
    T0, TL, MCH = cfg["T0"], cfg["TL"], cfg["MCH"]
    J0 = S // T0
    JL = S // TL
    qscale = DH ** -0.5 * _LOG2E
    n_mch = D // MCH
    G = cfg["G"]
    NB = H - G
    MC = (4 * D) // H
    W = 512
    assert 2 <= G <= 4 and D == 2 * W

    def kernel(x_hbm, k_hbm, v_hbm, wq_hbm, wo_hbm, wr_hbm, wg_hbm, wu_hbm, wd_hbm,
               c_hbm, wmod_hbm, out_hbm,
               x_buf, h_buf, acc, s_buf, m_buf, s2_buf, m2_buf, s3_buf, m3_buf, s4_buf, m4_buf,
               st_buf, st2_buf,
               q_ring, qf_buf, bq_buf,
               kb, vb, wq0, wqb, wob, wmb, wca, wsa, c_buf, wr_buf, sc_buf, cb_buf, mod0, modr, modv,
               wg, wu, wd, o_buf, key_buf, fix,
               sems):

        class _Sem:
            def __init__(self, base):
                self.base = base
                self.at = self

            def __getitem__(self, i):
                return sems.at[self.base + i]

        sizes = _sem_sizes(S, D, cfg)
        offs = [sum(sizes[:i]) for i in range(len(sizes))]
        (sem_small, sem_ca, sem_x, sem_sa, sem_first, sem_head,
         sem_ffn, sem_out, sem_fix) = (_Sem(o) for o in offs)

        def _mul(a, n):
            v = a * n
            return v if isinstance(a, int) else pl.multiple_of(v, n)

        def view(ref, j, t, n=1):
            return ref.at[pl.ds(_mul(j, t), n * t), :]

        def cp_c():
            return pltpu.make_async_copy(c_hbm, c_buf, sem_small.at[0])

        def cp_wr():
            return pltpu.make_async_copy(wr_hbm, wr_buf, sem_small.at[1])

        def cp_ca(c, i):
            return pltpu.make_async_copy(
                wmod_hbm.at[pl.ds(i * MCH, MCH), pl.ds(D + c * W, W)], view(wca.at[c], i, MCH),
                sem_ca.at[c * n_mch + i])

        def cp_sa():
            return pltpu.make_async_copy(wmod_hbm.at[:, pl.ds(0, D)], wsa, sem_sa.at[0])

        def cp_x(j):
            return pltpu.make_async_copy(view(x_hbm, j, T0), view(x_buf, j, T0), sem_x.at[j])

        def cp_wq0(c):
            return pltpu.make_async_copy(wq_hbm.at[pl.ds(c * W, W), pl.ds(0, G * DH)],
                                         view(wq0, c, W), sem_first.at[14 + c])

        def cp_k(h, sem=None):
            return pltpu.make_async_copy(k_hbm.at[h], kb.at[h & 3],
                                         sem_head.at[0] if sem is None else sem)

        def cp_wq(h):
            src = h if isinstance(h, int) else jnp.minimum(h, H - 1)
            return pltpu.make_async_copy(wq_hbm.at[:, pl.ds(_mul(src, DH), DH)], wqb.at[h & 1],
                                         sem_head.at[1])

        def cp_v(h, sem=None):
            return pltpu.make_async_copy(v_hbm.at[h], vb.at[h & 3],
                                         sem_head.at[2] if sem is None else sem)

        def cp_wo(h, sem=None):
            return pltpu.make_async_copy(view(wo_hbm, h, DH), wob.at[h & 3],
                                         sem_head.at[3] if sem is None else sem)

        def wm_slot(p):
            return p - NB + 1 if (isinstance(p, int) and p > NB) else p & 1

        def cp_wm(p):
            extra = isinstance(p, int) and p > NB
            return pltpu.make_async_copy(
                wmod_hbm.at[:, pl.ds(_mul(p + (2 * D) // MC, MC), MC)], wmb.at[wm_slot(p)],
                sem_first.at[4 + p - NB] if extra else sem_head.at[4])

        ffn = ((wg_hbm, wg), (wu_hbm, wu), (wd_hbm, wd))

        def start_ffn_piece(p):
            for i, (src, dst) in enumerate(ffn):
                n = src.shape[0] // H
                pltpu.make_async_copy(view(src, p, n), view(dst, p, n), sem_ffn.at[i]).start()

        def wait_ffn():
            for i, (src, dst) in enumerate(ffn):
                pltpu.make_async_copy(src, dst, sem_ffn.at[i]).wait()

        def cp_out(j):
            return pltpu.make_async_copy(view(o_buf, j, TL), view(out_hbm, j, TL), sem_out.at[j])

        def head_copies(h):
            return [cp_wq(h + G), cp_k(h + G - 1), cp_wo(h + 2), cp_wm(h), cp_v(h + 2)]

        def ln1_chunks(xv, sv):
            def chunk(off):
                def f(tok=None):
                    mean, inv = _row_stats(xv[off:off + 8, :].astype(f32), tok)
                    sv[off:off + 8, 0:128] = mean
                    sv[off:off + 8, 128:256] = inv
                return f
            return [chunk(off) for off in range(0, xv.shape[0], 8)]

        def ln1_scaled(x, stat, cs, tok=None):
            w = x.shape[1]
            mean = stat[:, 0:128] if tok is None else stat[:, 0:128] + _rep(tok, x.shape[0])
            n = (x.astype(f32) - _wide(mean, w)) * _wide(stat[:, 128:256], w)
            return n * _rep(mod0[1, :, cs], x.shape[0])

        def qproj(h):
            q = None
            for c in range(D // W):
                cs = slice(c * W, (c + 1) * W)
                part = jnp.dot(pltpu.bitcast(h_buf[:, cs], bf16), wqb[h & 1, cs, :],
                               preferred_element_type=f32)
                q = part if q is None else q + part
            q_ring[h & 3] = pltpu.bitcast((q * qscale).astype(bf16), u32)

        def q_early(g, q):
            return ((q + _rep(bq_buf[:, g * DH:(g + 1) * DH], q.shape[0])) * qscale).astype(bf16)

        def scores(h, q, sv, mv, rec=None, reload=False):
            mp = None
            for c in range(SK // W):
                cs = slice(c * W, (c + 1) * W)
                s = lax.dot_general(q, kb[h & 3, cs, :], _NT, preferred_element_type=f32)
                sv[:, cs] = s
                if rec is not None:
                    rec.done(s)
                if not reload:
                    mp = _fold(jnp.maximum, ([] if mp is None else [mp]) + _tiles(s))
            if reload:
                mp = _fold(jnp.maximum, _tiles(sv[...]))
            mv[...] = jnp.broadcast_to(jnp.max(mp, axis=-1, keepdims=True), mp.shape)

        def pv(h, sv, mv, rec=None, late=False):
            o = lp = None
            for c in range(SK // W):
                cs = slice(c * W, (c + 1) * W)
                m = mv[...]
                if c >= cfg["LD"] and sv.shape[0] == S:
                    m = m + _zero_of(lp)
                p = jnp.exp2(sv[:, cs] - _wide(m, W))
                lp = _fold(jnp.add, ([] if lp is None else [lp]) + _tiles(p))
                d = jnp.dot(p.astype(bf16), vb[h & 3, cs, :], preferred_element_type=f32)
                o = d if o is None else o + d
                if rec is not None:
                    rec.done(d)
            if late:
                lp = lp + _zero_of(o)
            l = jnp.sum(lp, axis=-1, keepdims=True)
            r = pl.reciprocal(l, approx=True)
            r = r * (2.0 - l * r)
            return (o * r).astype(bf16)

        def oproj(hos, av, xv=None, rec=None):
            for c in range(D // W):
                cs = slice(c * W, (c + 1) * W)
                a = av[:, cs]
                for h, o in hos:
                    if not isinstance(h, int):
                        a = jnp.where(h > 0, a, 0.0)
                    d = jnp.dot(o, wob[h & 3, :, cs], preferred_element_type=f32)
                    if rec is not None:
                        rec.done(d)
                    a = a + d
                if xv is not None:
                    a = xv[:, cs].astype(f32) + _rep(modv[0, :, cs], a.shape[0]) * a
                av[:, cs] = a

        def matvec(wv, tok=None, step=16):
            n = wv.shape[1]
            part = None if tok is None else _wide(tok, n)
            for r in range(0, D, step):
                t = wv[r:r + step, :].astype(f32) * _wide(cb_buf[r:r + step, :], n)
                for e in range(step // 8):
                    te = t[e * 8:(e + 1) * 8, :]
                    part = te if part is None else part + te
            return _rb(jnp.sum(part, axis=0, keepdims=True))

        def mod_piece(p, tok=None):
            modr[p] = matvec(wmb.at[wm_slot(p)], tok)

        def finish_mod():
            n = D // MC
            ga, sb, cb, gb = (jnp.concatenate([modr[i * n + t] for t in range(n)], axis=-1)
                              for i in range(4))
            cb1 = _rb(1.0 + cb)
            wr = wr_buf[...].astype(f32).reshape(1, D)
            a = cb1 * wr
            a0 = jnp.broadcast_to(jnp.sum(a, axis=-1, keepdims=True), (1, D))
            b0 = jnp.broadcast_to(jnp.sum(sb * wr, axis=-1, keepdims=True), (1, D))
            for i, v in enumerate((ga, sb, cb1, gb, a, gb * cb1, gb * sb, a0, b0)):
                modv[i] = jnp.broadcast_to(v, (8, D))

        def out_rows(x1, mean, inv):
            return (x1 + ((x1 - _wide(mean, D)) * (_wide(inv, D) * modv[5]) + modv[6])).astype(bf16)

        def out_chunks(j):
            x1v, sv, ov = view(acc, j, TL), view(st2_buf, j, TL), view(o_buf, j, TL)

            def chunk(off):
                def f(tok):
                    rs = slice(off, off + 8)
                    ov[rs, :] = out_rows(x1v[rs, :], sv[rs, 0:128] + tok, sv[rs, 128:256] + tok)
                return f
            return [chunk(off) for off in range(0, TL, 8)]

        def epi_chunks(j, x1v, ov, with_out=True):
            sub = lax.broadcasted_iota(i32, (8, 128), 0)
            low = (0xFFFF - j * TL) - sub
            sv = view(st2_buf, j, TL)
            st = {}

            def chunk(off):
                def f(tok=None):
                    if off == 0:
                        st["k1"], st["k2"] = key_buf[0], key_buf[1]
                    x1 = x1v[off:off + 8, :]
                    mean, inv = _row_stats(x1, tok)
                    sv[off:off + 8, 0:128] = mean
                    sv[off:off + 8, 128:256] = inv
                    xa = _tiles(x1 * modv[4])
                    if tok is not None:
                        xa[0] = xa[0] + tok
                    ra = _lane_sum(_fold(jnp.add, xa))
                    r = inv * (ra - mean * modv[7, :, 0:128]) + modv[8, :, 0:128]
                    if with_out:
                        ov[off:off + 8, :] = out_rows(x1, mean, inv)
                    bits = pltpu.bitcast(_rb(r) + 0.0, i32)
                    key = jnp.where(bits < 0, bits ^ 0x7FFF0000, bits) | (low - off)
                    st["k2"] = jnp.maximum(st["k2"], jnp.minimum(st["k1"], key))
                    st["k1"] = jnp.maximum(st["k1"], key)
                    if off + 8 == TL:
                        key_buf[0], key_buf[1] = st["k1"], st["k2"]
                return f
            return [chunk(off) for off in range(0, TL, 8)]

        cp_c().start()
        cp_x(0).start()
        for c in range(2):
            cp_wq0(c).start()
            for i in range(n_mch):
                cp_ca(c, i).start()
            if c == 0:
                for j in range(1, J0):
                    cp_x(j).start()
        cp_sa().start()
        for h in range(G - 1):
            cp_k(h, sem_first.at[1 + h]).start()
        early = []
        for h in range(2):
            early += [cp_v(h, sem_first.at[8 + 2 * h]), cp_wo(h, sem_first.at[9 + 2 * h])]
        for cp in early + head_copies(0):
            cp.start()

        cp_c().wait()
        cf = c_buf[...].astype(f32)
        sc = _rb(cf * jax.nn.sigmoid(cf))
        for t in range(4):
            sc_buf[t] = sc[:, t * (D // 4):(t + 1) * (D // 4)]

        def cb_body(t, carry):
            view(cb_buf, t, D // 4)[...] = jnp.transpose(jnp.broadcast_to(sc_buf[t], (128, D // 4)))
            return carry
        lax.fori_loop(0, 4, cb_body, 0)
        key_buf[...] = jnp.full(key_buf.shape, _IMIN, i32)
        cp_x(0).wait()

        def st0_body(i, carry):
            for ch in ln1_chunks(view(x_buf, i, T0 // 4), view(st_buf, i, T0 // 4)):
                ch()
            return carry
        lax.fori_loop(0, 4, st0_body, 0)

        def ca_half(c, stream):
            cp_wq0(c).wait()
            if not stream:
                for i in range(n_mch):
                    cp_ca(c, i).wait()
            part = None
            for i in range(n_mch):
                if stream:
                    cp_ca(c, i).wait()
                scb = jnp.broadcast_to(sc[:, i * MCH:(i + 1) * MCH], (16, MCH)).astype(bf16)
                d = jnp.dot(scb, wca[c, i * MCH:(i + 1) * MCH, :], preferred_element_type=f32)
                part = d if part is None else part + d
            mod0[1, :, c * W:(c + 1) * W] = _rb(1.0 + _rb(part[0:8, :]))

        def q_first(r0, t, c, rec, mid=None):
            rows = pl.ds(r0, t)
            cs = slice(c * W, (c + 1) * W)
            hh = ln1_scaled(x_buf[rows, cs], st_buf[rows, :], cs).astype(bf16)
            for g in range(G):
                if mid is not None and g == mid[0]:
                    mid[1]()
                part = jnp.dot(hh, wq0[cs, g * DH:(g + 1) * DH], preferred_element_type=f32)
                qf_buf[g, rows, :] = part if c == 0 else qf_buf[g, rows, :] + part
                if rec is not None:
                    rec.done(part)

        ca_half(0, True)

        def pa_body(j, carry):
            @pl.when(j + 1 < J0)
            def _():
                cp_x(j + 1).wait()
            jn = jnp.minimum(j + 1, J0 - 1)
            rec = _Pace(ln1_chunks(view(x_buf, jn, T0), view(st_buf, jn, T0)), cfg["LCA"])
            q_first(_mul(j, T0), T0, 0, rec)
            return carry
        lax.fori_loop(0, J0, pa_body, 0)

        TB, RB = cfg["TB"], cfg["RB"]
        ca_half(1, False)
        q_first(0, TB, 1, None)
        cp_sa().wait()
        cp_k(0, sem_first.at[1]).wait()
        cp_wr().start()
        for p in range(NB + 1, H):
            cp_wm(p).start()
        for p in range(NB, H):
            start_ffn_piece(p)

        def sa_chunk(t):
            def f(tok):
                cs = slice(t * 256, (t + 1) * 256)
                mod0[0, :, cs] = jnp.broadcast_to(matvec(wsa.at[:, cs], tok, 8), (8, 256))
            return f

        def sa_bias():
            bq_buf[...] = jnp.dot(_rep(mod0[0], 16).astype(bf16), wq0[...],
                                  preferred_element_type=f32)[0:8, :]

        def h_chunk(off):
            def f(tok):
                rs, rh = slice(off, off + RB), slice(off // 2, (off + RB) // 2)
                hh = (ln1_scaled(x_buf[rs, :], st_buf[rs, :], slice(0, D), tok)
                      + _rep(mod0[0], RB)).astype(bf16)
                h_buf[rh, :] = pltpu.bitcast(hh, u32)
            return f

        def q_chunk(off):
            def f(tok):
                n = 2 * RB
                rs, rh = slice(off, off + n), slice(off // 2, (off + n) // 2)
                for g in range(1, G):
                    q_ring[g, rh, :] = pltpu.bitcast(
                        q_early(g, qf_buf[g, rs, :] + _rep(tok, n)), u32)
            return f

        hs = [h_chunk(off) for off in range(0, S, RB)]
        qs = [q_chunk(off) for off in range(0, S, 2 * RB)]
        nh = cfg["NHB"]
        rest_chunks = []
        nq, nr = len(qs), len(hs) - nh
        for i, ch in enumerate(hs[nh:]):
            rest_chunks.append(ch)
            while qs and (nq - len(qs)) * nr < (i + 1) * nq:
                rest_chunks.append(qs.pop(0))
        assert not qs
        rec = _Pace([sa_chunk(t) for t in range(D // 256)] + hs[:nh], cfg["LCB2"])
        q_first(TB, S - TB, 1, rec, mid=(cfg["BQ"], sa_bias))
        n4 = len(rest_chunks)
        n3 = n4 - cfg["NL4"]
        cnt = [n3 // 3 + (1 if i < n3 % 3 else 0) for i in range(3)] + [cfg["NL4"]]
        scores(0, q_early(0, qf_buf[0]), s_buf, m_buf, rec=_Pace(rest_chunks, cnt),
               reload=cfg['RLB'])

        def main_body(h, carry):
            qproj(h + G)
            start_ffn_piece(h)
            for cp in head_copies(h + 1):
                cp.start()
            o = pv(h, s_buf, m_buf)
            rec = _Pace([lambda tok: mod_piece(h, tok)], "1000")
            scores(h + 1, pltpu.bitcast(q_ring[(h + 1) & 3], bf16), s_buf, m_buf, rec=rec,
                   reload=cfg['RLM'])
            oproj([(h, o)], acc)
            for cp in head_copies(h + 1):
                cp.wait()
            return carry
        for h in range(1, G - 1):
            cp_k(h, sem_first.at[1 + h]).wait()
        for cp in early + head_copies(0):
            cp.wait()
        lax.fori_loop(0, NB, main_body, 0)

        ha = NB
        rest = list(zip(range(NB + 1, H), (s2_buf, s3_buf, s4_buf), (m2_buf, m3_buf, m4_buf)))
        late = []
        for n, h in enumerate(range(NB + 3, H)):
            late += [cp_v(h, sem_first.at[8 + 2 * n]), cp_wo(h, sem_first.at[9 + 2 * n])]
        for cp in late:
            cp.start()
        cp_wr().wait()
        for p in range(NB + 1, H):
            cp_wm(p).wait()

        def l_step(j, do_x, do_y):
            if do_x and do_y:
                aw = view(acc, j - 1, TL, 2)
                ay, ax = aw.at[0:TL, :], aw.at[TL:2 * TL, :]
            elif do_x:
                ax = view(acc, j, TL)
            else:
                ay = view(acc, j - 1, TL)
            rec = None
            if do_y:
                chunks = epi_chunks(j - 1, ay, view(o_buf, j - 1, TL), with_out=do_x)
                os_ = [(h, pv(h, sv, mv, late=not do_x)) for h, sv, mv in rest]
            if do_x:
                oa = pv(ha, view(s_buf, j, TL), view(m_buf, j, TL))
            if do_y and do_x:
                oproj(os_, ay, view(x_buf, j - 1, TL))
            elif do_y:
                xv = view(x_buf, j - 1, TL)
                r0, prev = 0, []
                for n in cfg["LSPLIT"]:
                    rs = slice(r0, r0 + n)
                    nr = len(os_) * (D // W)
                    cnt = [len(prev) // nr + (1 if i < len(prev) % nr else 0) for i in range(nr)]
                    rec = _Pace(prev, "".join("0123456789abcdefghijklmnopqrstuvwxyz"[i] for i in cnt))
                    oproj([(h, o[rs]) for h, o in os_], ay.at[rs, :], xv.at[rs, :], rec=rec)
                    prev = chunks[r0 // 8:(r0 + n) // 8]
                    r0 += n
                chunks = prev
            if do_x:
                if do_y:
                    rec = _Pace(chunks, cfg["LCNT"])
                for h, sv, mv in rest:
                    q = pltpu.bitcast(view(q_ring.at[h & 3], j, TL // 2)[...], bf16)
                    scores(h, q, sv, mv, rec=rec, reload=cfg['RLL'])
                oproj([(ha, oa)], ax, rec=rec)
            if do_y:
                if do_x:
                    cp_out(j - 1).start()
                else:
                    for ch in chunks:
                        ch()

        for p in range(NB, H):
            mod_piece(p)
        finish_mod()
        l_step(0, True, False)
        for cp in late:
            cp.wait()

        def pl_body(j, carry):
            l_step(j, True, True)
            return carry
        lax.fori_loop(1, JL, pl_body, 0)
        wait_ffn()
        for j in range(JL - 2):
            cp_out(j).wait()
        l_step(JL, False, True)

        k1, k2 = key_buf[0], key_buf[1]
        for sh in (4, 2, 1):
            o1, o2 = pltpu.roll(k1, sh, 0), pltpu.roll(k2, sh, 0)
            k2 = jnp.maximum(jnp.minimum(k1, o1), jnp.maximum(k2, o2))
            k1 = jnp.maximum(k1, o1)

        def score_of(k):
            hi = k & jnp.int32(-65536)
            return pltpu.bitcast(jnp.where(hi < 0, hi ^ 0x7FFF0000, hi), f32)

        i1s = jnp.minimum(0xFFFF - (k1[0, 0] & 0xFFFF), S - 1)
        i2s = jnp.minimum(0xFFFF - (k2[0, 0] & 0xFFFF), S - 1)

        sub = lax.broadcasted_iota(i32, (16, D), 0)
        sb, cb1, gb = (_rep(modv[i], 16) for i in (1, 2, 3))

        def adaln2(x1, stat):
            return (x1 - _wide(stat[:, 0:128], D)) * _wide(stat[:, 128:256], D) * cb1 + sb

        def pick(ref):
            sel = lax.broadcasted_iota(i32, (16, ref.shape[1]), 0) == 0
            return jnp.where(sel, ref[pl.ds(i1s, 1), :], ref[pl.ds(i2s, 1), :])

        xs = adaln2(pick(acc), pick(st2_buf)).astype(bf16)
        FC, lag = cfg["FC"], 2
        y = None
        act = []
        outs = out_chunks(JL - 1)
        for c in range(F // FC + lag):
            if c < F // FC:
                cs = slice(c * FC, (c + 1) * FC)
                g = jnp.dot(xs, wg[:, cs], preferred_element_type=f32)
                u = jnp.dot(xs, wu[:, cs], preferred_element_type=f32)
                for v in (g, u):
                    for t in range(cfg["FOUT"]):
                        if outs:
                            outs.pop(0)(_zero_of(v[0:8, (t % 2) * 128:(t % 2 + 1) * 128]))
                            if not outs:
                                cp_out(JL - 1).start()
                g, u = _rb(g), _rb(u)
                act.append((_rb(g * jax.nn.sigmoid(g)) * u).astype(bf16))
            if c >= lag:
                d = jnp.dot(act[c - lag], wd[(c - lag) * FC:(c - lag + 1) * FC, :],
                            preferred_element_type=f32)
                y = d if y is None else y + d
        y = _rb(y)
        ya = _rb(y[0:1, :] * _wide(_rb(jax.nn.sigmoid(score_of(k1[0:1, :]))), D))
        yb = _rb(y[1:2, :] * _wide(_rb(jax.nn.sigmoid(score_of(k2[0:1, :]))), D))

        g1 = pl.multiple_of((i1s >> 4) << 4, 16)
        g2 = pl.multiple_of((i2s >> 4) << 4, 16)
        for t, g0 in enumerate((g1, g2)):
            rid = sub + g0
            x1 = acc[pl.ds(g0, 16), :]
            upd = jnp.where(rid == i1s, ya, 0.0) + jnp.where(rid == i2s, yb, 0.0)
            fix[t] = (x1 + gb * (adaln2(x1, st2_buf[pl.ds(g0, 16), :]) + upd)).astype(bf16)

        for j in range(JL - 2, JL):
            cp_out(j).wait()

        def cp_fix(t, g0):
            return pltpu.make_async_copy(fix.at[t], out_hbm.at[pl.ds(g0, 16), :], sem_fix.at[t])

        cp_fix(0, g1).start()

        @pl.when(g2 != g1)
        def _():
            cp_fix(1, g2).start()
            cp_fix(1, g2).wait()
        cp_fix(0, g1).wait()

    return kernel


_CFG = dict(FC=256, T0=256, TL=256, MCH=256, LCA='cc80', LCB2='040g', NHB=16, NL4=8, BQ=3, LD=9, TB=1024, RLM=0, RLL=1, RLB=1, RB=16,
            G=4, LSPLIT=(96, 96, 64), FOUT=2, LCNT='33333333332000')


def _build(A_x, A_k_cache, A_v_cache, A_wq, A_wo, B_w_r, B_w_gate, B_w_up, B_w_down, c, w_mod,
           **over):
    B, S, D = A_x.shape
    _, H, SK, DH = A_k_cache.shape
    F = B_w_gate.shape[1]
    assert B == 1
    cfg = dict(_CFG, **over)
    T0, TL, G = cfg["T0"], cfg["TL"], cfg["G"]
    MC = (4 * D) // H
    kernel = _make_kernel(S, D, H, DH, SK, F, cfg)
    scratch = [
        pltpu.VMEM((S, D), bf16),
        pltpu.VMEM((S // 2, D), u32),
        pltpu.VMEM((S, D), f32),
        pltpu.VMEM((S, SK), f32),
        pltpu.VMEM((S, 128), f32),
        pltpu.VMEM((TL, SK), f32),
        pltpu.VMEM((TL, 128), f32),
        pltpu.VMEM((TL, SK), f32),
        pltpu.VMEM((TL, 128), f32),
        pltpu.VMEM((TL, SK), f32),
        pltpu.VMEM((TL, 128), f32),
        pltpu.VMEM((S, 256), f32),
        pltpu.VMEM((S, 256), f32),
        pltpu.VMEM((4, S // 2, DH), u32),
        pltpu.VMEM((G, S, DH), f32),
        pltpu.VMEM((8, G * DH), f32),
        pltpu.VMEM((4, SK, DH), bf16),
        pltpu.VMEM((4, SK, DH), bf16),
        pltpu.VMEM((D, G * DH), bf16),
        pltpu.VMEM((2, D, DH), bf16),
        pltpu.VMEM((4, DH, D), bf16),
        pltpu.VMEM((G + 1, D, MC), bf16),
        pltpu.VMEM((2, D, D // 2), bf16),
        pltpu.VMEM((D, D), bf16),
        pltpu.VMEM((1, D), bf16),
        pltpu.VMEM((D,), bf16),
        pltpu.VMEM((4, 1, D // 4), f32),
        pltpu.VMEM((D, 128), f32),
        pltpu.VMEM((2, 8, D), f32),
        pltpu.VMEM((H, 1, MC), f32),
        pltpu.VMEM((9, 8, D), f32),
        pltpu.VMEM((D, F), bf16),
        pltpu.VMEM((D, F), bf16),
        pltpu.VMEM((F, D), bf16),
        pltpu.VMEM((S, D), bf16),
        pltpu.VMEM((2, 8, 128), i32),
        pltpu.VMEM((2, 16, D), bf16),
        pltpu.SemaphoreType.DMA((sum(_sem_sizes(S, D, cfg)),)),
    ]
    any_spec = pl.BlockSpec(memory_space=pl.ANY)
    out = pl.pallas_call(
        kernel,
        out_shape=jax.ShapeDtypeStruct((S, D), bf16),
        in_specs=[any_spec] * 11,
        out_specs=any_spec,
        scratch_shapes=scratch,
        compiler_params=pltpu.CompilerParams(vmem_limit_bytes=112 * 1024 * 1024,
                                             disable_bounds_checks=True,
                                             disable_semaphore_checks=True),
    )(A_x.reshape(S, D), A_k_cache.reshape(H, SK, DH), A_v_cache.reshape(H, SK, DH),
      A_wq, A_wo, B_w_r, B_w_gate, B_w_up, B_w_down, c, w_mod)
    return out.reshape(B, S, D)


@jax.jit
def pallas_adaLN_cond__mha_block_cached__moe_arch_mod__prompt_kernel(
    A_x: jax.Array,
    A_k_cache: jax.Array,
    A_v_cache: jax.Array,
    A_wq: jax.Array,
    A_wo: jax.Array,
    B_x: jax.Array,
    B_w_r: jax.Array,
    B_w_gate: jax.Array,
    B_w_up: jax.Array,
    B_w_down: jax.Array,
    c: jax.Array,
    w_mod: jax.Array,
):
    del B_x
    return _build(A_x, A_k_cache, A_v_cache, A_wq, A_wo, B_w_r, B_w_gate, B_w_up, B_w_down,
                  c, w_mod)
```

```python
import jax
import jax.numpy as jnp
from jax import lax
import jax.experimental.pallas as pl
import jax.experimental.pallas.tpu as pltpu

f32 = jnp.float32
bf16 = jnp.bfloat16
u32 = jnp.uint32
i32 = jnp.int32

_NT = (((1,), (1,)), ((), ()))
_LOG2E = 1.4426950408889634
_EPS = 1e-5
_IMIN = -2 ** 31


def _rb(v):
    return v.astype(bf16).astype(f32)


def _rep(v, n):
    return v if n == 8 else jnp.tile(v, (n // 8, 1))


def _wide(v, w):
    return jnp.tile(v, (1, w // 128))


def _zero_of(v):
    bits = pltpu.bitcast(v, u32)
    return pltpu.bitcast(lax.shift_right_logical(lax.shift_right_logical(bits, jnp.uint32(31)),
                                                 jnp.uint32(1)), f32)


class _Pace:
    def __init__(self, chunks, counts):
        self.chunks = list(chunks)
        self.counts = [ch if isinstance(ch, int) else int(ch, 36) for ch in counts]
        assert sum(self.counts) == len(self.chunks), (counts, len(self.chunks))

    def done(self, res):
        n = self.counts.pop(0)
        for i in range(n):
            r0 = (i * res.shape[0] // n) // 8 * 8
            self.chunks.pop(0)(_zero_of(res[r0:r0 + 8, 0:128]))


def _tiles(v):
    return [v[:, c * 128:(c + 1) * 128] for c in range(v.shape[1] // 128)]


def _fold(op, parts):
    out = parts[0]
    for p in parts[1:]:
        out = op(out, p)
    return out


def _lane_sum(v):
    return jnp.broadcast_to(jnp.sum(v, axis=-1, keepdims=True), v.shape)


def _row_stats(xf, tok=None):
    d = xf.shape[-1]
    ts = _tiles(xf)
    nt = len(ts)
    if tok is not None:
        ts = [ts[0] + tok] + ts[1:]
    mu = _fold(jnp.add, ts) * (1.0 / nt)
    m2 = _fold(jnp.add, [(t - mu) * (t - mu) for t in ts])
    mean = _lane_sum(mu) * (1.0 / 128)
    dm = mu - mean
    var = _lane_sum(m2 + (dm * dm) * float(nt)) * (1.0 / d)
    return mean, lax.rsqrt(var + _EPS)


def _sem_sizes(S, D, cfg):
    j0 = S // cfg["T0"]
    return [2, 2 * (D // cfg["MCH"]), j0, 1, 16, 5, 3, 1, 2]


def _make_kernel(S, D, H, DH, SK, F, cfg):
    T0, TL, MCH = cfg["T0"], cfg["TL"], cfg["MCH"]
    J0 = S // T0
    JL = S // TL
    qscale = DH ** -0.5 * _LOG2E
    n_mch = D // MCH
    G = cfg["G"]
    NB = H - G
    MC = (4 * D) // H
    W = 512
    assert 2 <= G <= 4 and D == 2 * W

    def kernel(x_hbm, k_hbm, v_hbm, wq_hbm, wo_hbm, wr_hbm, wg_hbm, wu_hbm, wd_hbm,
               c_hbm, wmod_hbm, out_hbm,
               x_buf, h_buf, acc, s_buf, m_buf, s2_buf, m2_buf, s3_buf, m3_buf, s4_buf, m4_buf,
               st_buf, st2_buf,
               q_ring, qf_buf, bq_buf,
               kb, vb, wq0, wqb, wob, wmb, wca, wsa, c_buf, wr_buf, sc_buf, cb_buf, mod0, modr, modv,
               wg, wu, wd, o_buf, key_buf, fix,
               sems):

        class _Sem:
            def __init__(self, base):
                self.base = base
                self.at = self

            def __getitem__(self, i):
                return sems.at[self.base + i]

        sizes = _sem_sizes(S, D, cfg)
        offs = [sum(sizes[:i]) for i in range(len(sizes))]
        (sem_small, sem_ca, sem_x, sem_sa, sem_first, sem_head,
         sem_ffn, sem_out, sem_fix) = (_Sem(o) for o in offs)

        def _mul(a, n):
            v = a * n
            return v if isinstance(a, int) else pl.multiple_of(v, n)

        def view(ref, j, t, n=1):
            return ref.at[pl.ds(_mul(j, t), n * t), :]

        def cp_c():
            return pltpu.make_async_copy(c_hbm, c_buf, sem_small.at[0])

        def cp_wr():
            return pltpu.make_async_copy(wr_hbm, wr_buf, sem_small.at[1])

        def cp_ca(c, i):
            return pltpu.make_async_copy(
                wmod_hbm.at[pl.ds(i * MCH, MCH), pl.ds(D + c * W, W)], view(wca.at[c], i, MCH),
                sem_ca.at[c * n_mch + i])

        def cp_sa():
            return pltpu.make_async_copy(wmod_hbm.at[:, pl.ds(0, D)], wsa, sem_sa.at[0])

        def cp_x(j):
            return pltpu.make_async_copy(view(x_hbm, j, T0), view(x_buf, j, T0), sem_x.at[j])

        def cp_wq0(c):
            return pltpu.make_async_copy(wq_hbm.at[pl.ds(c * W, W), pl.ds(0, G * DH)],
                                         view(wq0, c, W), sem_first.at[14 + c])

        def cp_k(h, sem=None):
            return pltpu.make_async_copy(k_hbm.at[h], kb.at[h & 3],
                                         sem_head.at[0] if sem is None else sem)

        def cp_wq(h):
            src = h if isinstance(h, int) else jnp.minimum(h, H - 1)
            return pltpu.make_async_copy(wq_hbm.at[:, pl.ds(_mul(src, DH), DH)], wqb.at[h & 1],
                                         sem_head.at[1])

        def cp_v(h, sem=None):
            return pltpu.make_async_copy(v_hbm.at[h], vb.at[h & 3],
                                         sem_head.at[2] if sem is None else sem)

        def cp_wo(h, sem=None):
            return pltpu.make_async_copy(view(wo_hbm, h, DH), wob.at[h & 3],
                                         sem_head.at[3] if sem is None else sem)

        def wm_slot(p):
            return p - NB + 1 if (isinstance(p, int) and p > NB) else p & 1

        def cp_wm(p):
            extra = isinstance(p, int) and p > NB
            return pltpu.make_async_copy(
                wmod_hbm.at[:, pl.ds(_mul(p + (2 * D) // MC, MC), MC)], wmb.at[wm_slot(p)],
                sem_first.at[4 + p - NB] if extra else sem_head.at[4])

        ffn = ((wg_hbm, wg), (wu_hbm, wu), (wd_hbm, wd))

        def start_ffn_piece(p):
            for i, (src, dst) in enumerate(ffn):
                n = src.shape[0] // H
                pltpu.make_async_copy(view(src, p, n), view(dst, p, n), sem_ffn.at[i]).start()

        def wait_ffn():
            for i, (src, dst) in enumerate(ffn):
                pltpu.make_async_copy(src, dst, sem_ffn.at[i]).wait()

        def cp_out(j):
            return pltpu.make_async_copy(view(o_buf, j, TL), view(out_hbm, j, TL), sem_out.at[0])

        def head_copies(h):
            return [cp_wq(h + G), cp_k(h + G - 1), cp_wo(h + 2), cp_wm(h), cp_v(h + 2)]

        def ln1_chunks(xv, sv):
            def chunk(off):
                def f(tok=None):
                    mean, inv = _row_stats(xv[off:off + 8, :].astype(f32), tok)
                    sv[off:off + 8, 0:128] = mean
                    sv[off:off + 8, 128:256] = inv
                return f
            return [chunk(off) for off in range(0, xv.shape[0], 8)]

        def ln1_scaled(x, stat, cs, tok=None):
            w = x.shape[1]
            mean = stat[:, 0:128] if tok is None else stat[:, 0:128] + _rep(tok, x.shape[0])
            n = (x.astype(f32) - _wide(mean, w)) * _wide(stat[:, 128:256], w)
            return n * _rep(mod0[1, :, cs], x.shape[0])

        def qproj(h):
            q = None
            for c in range(D // W):
                cs = slice(c * W, (c + 1) * W)
                part = jnp.dot(pltpu.bitcast(h_buf[:, cs], bf16), wqb[h & 1, cs, :],
                               preferred_element_type=f32)
                q = part if q is None else q + part
            q_ring[h & 3] = pltpu.bitcast((q * qscale).astype(bf16), u32)

        def q_early(g, q):
            return ((q + _rep(bq_buf[:, g * DH:(g + 1) * DH], q.shape[0])) * qscale).astype(bf16)

        def scores(h, q, sv, mv, rec=None, reload=False):
            mp = None
            for c in range(SK // W):
                cs = slice(c * W, (c + 1) * W)
                s = lax.dot_general(q, kb[h & 3, cs, :], _NT, preferred_element_type=f32)
                sv[:, cs] = s
                if rec is not None:
                    rec.done(s)
                if not reload:
                    mp = _fold(jnp.maximum, ([] if mp is None else [mp]) + _tiles(s))
            if reload:
                mp = _fold(jnp.maximum, _tiles(sv[...]))
            mv[...] = jnp.broadcast_to(jnp.max(mp, axis=-1, keepdims=True), mp.shape)

        def pv(h, sv, mv, rec=None, late=False):
            o = lp = None
            for c in range(SK // W):
                cs = slice(c * W, (c + 1) * W)
                p = jnp.exp2(sv[:, cs] - _wide(mv[...], W))
                lp = _fold(jnp.add, ([] if lp is None else [lp]) + _tiles(p))
                d = jnp.dot(p.astype(bf16), vb[h & 3, cs, :], preferred_element_type=f32)
                o = d if o is None else o + d
                if rec is not None:
                    rec.done(d)
            if late:
                lp = lp + _zero_of(o)
            l = jnp.sum(lp, axis=-1, keepdims=True)
            r = pl.reciprocal(l, approx=True)
            r = r * (2.0 - l * r)
            return (o * r).astype(bf16)

        def oproj(hos, av, xv=None, rec=None):
            for c in range(D // W):
                cs = slice(c * W, (c + 1) * W)
                a = av[:, cs]
                for h, o in hos:
                    if not isinstance(h, int):
                        a = jnp.where(h > 0, a, 0.0)
                    d = jnp.dot(o, wob[h & 3, :, cs], preferred_element_type=f32)
                    if rec is not None:
                        rec.done(d)
                    a = a + d
                if xv is not None:
                    a = xv[:, cs].astype(f32) + _rep(modv[0, :, cs], a.shape[0]) * a
                av[:, cs] = a

        def matvec(wv, tok=None, step=16):
            n = wv.shape[1]
            part = None if tok is None else _wide(tok, n)
            for r in range(0, D, step):
                t = wv[r:r + step, :].astype(f32) * _wide(cb_buf[r:r + step, :], n)
                for e in range(step // 8):
                    te = t[e * 8:(e + 1) * 8, :]
                    part = te if part is None else part + te
            return _rb(jnp.sum(part, axis=0, keepdims=True))

        def mod_piece(p, tok=None):
            modr[p] = matvec(wmb.at[wm_slot(p)], tok)

        def finish_mod():
            n = D // MC
            ga, sb, cb, gb = (jnp.concatenate([modr[i * n + t] for t in range(n)], axis=-1)
                              for i in range(4))
            cb1 = _rb(1.0 + cb)
            wr = wr_buf[...].astype(f32).reshape(1, D)
            a = cb1 * wr
            a0 = jnp.broadcast_to(jnp.sum(a, axis=-1, keepdims=True), (1, D))
            b0 = jnp.broadcast_to(jnp.sum(sb * wr, axis=-1, keepdims=True), (1, D))
            for i, v in enumerate((ga, sb, cb1, gb, a, gb * cb1, gb * sb, a0, b0)):
                modv[i] = jnp.broadcast_to(v, (8, D))

        def out_rows(x1, mean, inv):
            return (x1 + ((x1 - _wide(mean, D)) * (_wide(inv, D) * modv[5]) + modv[6])).astype(bf16)

        def out_chunks(j):
            x1v, sv, ov = view(acc, j, TL), view(st2_buf, j, TL), view(o_buf, j, TL)

            def chunk(off):
                def f(tok):
                    rs = slice(off, off + 8)
                    ov[rs, :] = out_rows(x1v[rs, :], sv[rs, 0:128] + tok, sv[rs, 128:256] + tok)
                return f
            return [chunk(off) for off in range(0, TL, 8)]

        def epi_chunks(j, x1v, ov, with_out=True):
            sub = lax.broadcasted_iota(i32, (8, 128), 0)
            low = (0xFFFF - j * TL) - sub
            sv = view(st2_buf, j, TL)
            st = {}

            def chunk(off):
                def f(tok=None):
                    if off == 0:
                        st["k1"], st["k2"] = key_buf[0], key_buf[1]
                    x1 = x1v[off:off + 8, :]
                    mean, inv = _row_stats(x1, tok)
                    sv[off:off + 8, 0:128] = mean
                    sv[off:off + 8, 128:256] = inv
                    xa = _tiles(x1 * modv[4])
                    if tok is not None:
                        xa[0] = xa[0] + tok
                    ra = _lane_sum(_fold(jnp.add, xa))
                    r = inv * (ra - mean * modv[7, :, 0:128]) + modv[8, :, 0:128]
                    if with_out:
                        ov[off:off + 8, :] = out_rows(x1, mean, inv)
                    bits = pltpu.bitcast(_rb(r) + 0.0, i32)
                    key = jnp.where(bits < 0, bits ^ 0x7FFF0000, bits) | (low - off)
                    st["k2"] = jnp.maximum(st["k2"], jnp.minimum(st["k1"], key))
                    st["k1"] = jnp.maximum(st["k1"], key)
                    if off + 8 == TL:
                        key_buf[0], key_buf[1] = st["k1"], st["k2"]
                return f
            return [chunk(off) for off in range(0, TL, 8)]

        cp_c().start()
        cp_x(0).start()
        for c in range(2):
            cp_wq0(c).start()
            for i in range(n_mch):
                cp_ca(c, i).start()
            if c == 0:
                for j in range(1, J0):
                    cp_x(j).start()
        cp_sa().start()
        for h in range(G - 1):
            cp_k(h, sem_first.at[1 + h]).start()
        early = []
        for h in range(2):
            early += [cp_v(h, sem_first.at[8 + 2 * h]), cp_wo(h, sem_first.at[9 + 2 * h])]
        for cp in early + head_copies(0):
            cp.start()

        cp_c().wait()
        cf = c_buf[...].astype(f32)
        sc = _rb(cf * jax.nn.sigmoid(cf))
        for t in range(4):
            sc_buf[t] = sc[:, t * (D // 4):(t + 1) * (D // 4)]

        def cb_body(t, carry):
            view(cb_buf, t, D // 4)[...] = jnp.transpose(jnp.broadcast_to(sc_buf[t], (128, D // 4)))
            return carry
        lax.fori_loop(0, 4, cb_body, 0)
        key_buf[...] = jnp.full(key_buf.shape, _IMIN, i32)
        cp_x(0).wait()

        def st0_body(i, carry):
            for ch in ln1_chunks(view(x_buf, i, T0 // 4), view(st_buf, i, T0 // 4)):
                ch()
            return carry
        lax.fori_loop(0, 4, st0_body, 0)

        def ca_half(c, stream):
            cp_wq0(c).wait()
            if not stream:
                for i in range(n_mch):
                    cp_ca(c, i).wait()
            part = None
            for i in range(n_mch):
                if stream:
                    cp_ca(c, i).wait()
                scb = jnp.broadcast_to(sc[:, i * MCH:(i + 1) * MCH], (16, MCH)).astype(bf16)
                d = jnp.dot(scb, wca[c, i * MCH:(i + 1) * MCH, :], preferred_element_type=f32)
                part = d if part is None else part + d
            mod0[1, :, c * W:(c + 1) * W] = _rb(1.0 + _rb(part[0:8, :]))

        def q_first(r0, t, c, rec, mid=None):
            rows = pl.ds(r0, t)
            cs = slice(c * W, (c + 1) * W)
            hh = ln1_scaled(x_buf[rows, cs], st_buf[rows, :], cs).astype(bf16)
            for g in range(G):
                if mid is not None and g == mid[0]:
                    mid[1]()
                part = jnp.dot(hh, wq0[cs, g * DH:(g + 1) * DH], preferred_element_type=f32)
                qf_buf[g, rows, :] = part if c == 0 else qf_buf[g, rows, :] + part
                if rec is not None:
                    rec.done(part)

        ca_half(0, True)

        def pa_body(j, carry):
            @pl.when(j + 1 < J0)
            def _():
                cp_x(j + 1).wait()
            jn = jnp.minimum(j + 1, J0 - 1)
            rec = _Pace(ln1_chunks(view(x_buf, jn, T0), view(st_buf, jn, T0)), cfg["LCA"])
            q_first(_mul(j, T0), T0, 0, rec)
            return carry
        lax.fori_loop(0, J0, pa_body, 0)

        TB, RB = cfg["TB"], cfg["RB"]
        ca_half(1, False)
        q_first(0, TB, 1, None)
        cp_sa().wait()
        cp_k(0, sem_first.at[1]).wait()
        cp_wr().start()
        for p in range(NB + 1, H):
            cp_wm(p).start()
        for p in range(NB, H):
            start_ffn_piece(p)

        def sa_chunk(t):
            def f(tok):
                cs = slice(t * 256, (t + 1) * 256)
                mod0[0, :, cs] = jnp.broadcast_to(matvec(wsa.at[:, cs], tok, 8), (8, 256))
            return f

        def sa_bias():
            bq_buf[...] = jnp.dot(_rep(mod0[0], 16).astype(bf16), wq0[...],
                                  preferred_element_type=f32)[0:8, :]

        def h_chunk(off):
            def f(tok):
                rs, rh = slice(off, off + RB), slice(off // 2, (off + RB) // 2)
                hh = (ln1_scaled(x_buf[rs, :], st_buf[rs, :], slice(0, D), tok)
                      + _rep(mod0[0], RB)).astype(bf16)
                h_buf[rh, :] = pltpu.bitcast(hh, u32)
            return f

        def q_chunk(off):
            def f(tok):
                n = 2 * RB
                rs, rh = slice(off, off + n), slice(off // 2, (off + n) // 2)
                for g in range(1, G):
                    q_ring[g, rh, :] = pltpu.bitcast(
                        q_early(g, qf_buf[g, rs, :] + _rep(tok, n)), u32)
            return f

        hs = [h_chunk(off) for off in range(0, S, RB)]
        qs = [q_chunk(off) for off in range(0, S, 2 * RB)]
        nh = cfg["NHB"]
        rest_chunks = []
        nq, nr = len(qs), len(hs) - nh
        for i, ch in enumerate(hs[nh:]):
            rest_chunks.append(ch)
            while qs and (nq - len(qs)) * nr < (i + 1) * nq:
                rest_chunks.append(qs.pop(0))
        assert not qs
        rec = _Pace([sa_chunk(t) for t in range(D // 256)] + hs[:nh], cfg["LCB2"])
        q_first(TB, S - TB, 1, rec, mid=(cfg["BQ"], sa_bias))
        n4 = len(rest_chunks)
        n3 = n4 - cfg["NL4"]
        cnt = [n3 // 3 + (1 if i < n3 % 3 else 0) for i in range(3)] + [cfg["NL4"]]
        scores(0, q_early(0, qf_buf[0]), s_buf, m_buf, rec=_Pace(rest_chunks, cnt), reload=True)

        def main_body(h, carry):
            qproj(h + G)
            start_ffn_piece(h)
            for cp in head_copies(h + 1):
                cp.start()
            o = pv(h, s_buf, m_buf)
            rec = _Pace([lambda tok: mod_piece(h, tok)], "1000")
            scores(h + 1, pltpu.bitcast(q_ring[(h + 1) & 3], bf16), s_buf, m_buf, rec=rec)
            oproj([(h, o)], acc)
            for cp in head_copies(h + 1):
                cp.wait()
            return carry
        for h in range(1, G - 1):
            cp_k(h, sem_first.at[1 + h]).wait()
        for cp in early + head_copies(0):
            cp.wait()
        lax.fori_loop(0, NB, main_body, 0)

        ha = NB
        rest = list(zip(range(NB + 1, H), (s2_buf, s3_buf, s4_buf), (m2_buf, m3_buf, m4_buf)))
        late = []
        for n, h in enumerate(range(NB + 3, H)):
            late += [cp_v(h, sem_first.at[8 + 2 * n]), cp_wo(h, sem_first.at[9 + 2 * n])]
        for cp in late:
            cp.start()
        cp_wr().wait()
        for p in range(NB + 1, H):
            cp_wm(p).wait()

        def l_step(j, do_x, do_y):
            if do_x and do_y:
                aw = view(acc, j - 1, TL, 2)
                ay, ax = aw.at[0:TL, :], aw.at[TL:2 * TL, :]
            elif do_x:
                ax = view(acc, j, TL)
            else:
                ay = view(acc, j - 1, TL)
            rec = None
            if do_y:
                chunks = epi_chunks(j - 1, ay, view(o_buf, j - 1, TL), with_out=do_x)
                os_ = [(h, pv(h, sv, mv, late=not do_x)) for h, sv, mv in rest]
            if do_x:
                oa = pv(ha, view(s_buf, j, TL), view(m_buf, j, TL))
            if do_y and do_x:
                oproj(os_, ay, view(x_buf, j - 1, TL))
            elif do_y:
                xv = view(x_buf, j - 1, TL)
                r0, prev = 0, []
                for n in cfg["LSPLIT"]:
                    rs = slice(r0, r0 + n)
                    nr = len(os_) * (D // W)
                    cnt = [len(prev) // nr + (1 if i < len(prev) % nr else 0) for i in range(nr)]
                    rec = _Pace(prev, cnt)
                    oproj([(h, o[rs]) for h, o in os_], ay.at[rs, :], xv.at[rs, :], rec=rec)
                    prev = chunks[r0 // 8:(r0 + n) // 8]
                    r0 += n
                chunks = prev
            if do_x:
                if do_y:
                    rec = _Pace(chunks, cfg["LCNT"])
                for h, sv, mv in rest:
                    q = pltpu.bitcast(view(q_ring.at[h & 3], j, TL // 2)[...], bf16)
                    scores(h, q, sv, mv, rec=rec, reload=True)
                oproj([(ha, oa)], ax, rec=rec)
            if do_y:
                if do_x:
                    cp_out(j - 1).start()
                else:
                    for ch in chunks:
                        ch()

        for p in range(NB, H):
            mod_piece(p)
        finish_mod()
        l_step(0, True, False)
        for cp in late:
            cp.wait()
        wait_ffn()

        def pl_body(j, carry):
            l_step(j, True, True)
            return carry
        lax.fori_loop(1, JL, pl_body, 0)
        l_step(JL, False, True)

        k1, k2 = key_buf[0], key_buf[1]
        for sh in (4, 2, 1):
            o1, o2 = pltpu.roll(k1, sh, 0), pltpu.roll(k2, sh, 0)
            k2 = jnp.maximum(jnp.minimum(k1, o1), jnp.maximum(k2, o2))
            k1 = jnp.maximum(k1, o1)

        def score_of(k):
            hi = k & jnp.int32(-65536)
            return pltpu.bitcast(jnp.where(hi < 0, hi ^ 0x7FFF0000, hi), f32)

        i1s = jnp.minimum(0xFFFF - (k1[0, 0] & 0xFFFF), S - 1)
        i2s = jnp.minimum(0xFFFF - (k2[0, 0] & 0xFFFF), S - 1)

        sub = lax.broadcasted_iota(i32, (16, D), 0)
        sb, cb1, gb = (_rep(modv[i], 16) for i in (1, 2, 3))

        def adaln2(x1, stat):
            return (x1 - _wide(stat[:, 0:128], D)) * _wide(stat[:, 128:256], D) * cb1 + sb

        def pick(ref):
            sel = lax.broadcasted_iota(i32, (16, ref.shape[1]), 0) == 0
            return jnp.where(sel, ref[pl.ds(i1s, 1), :], ref[pl.ds(i2s, 1), :])

        xs = adaln2(pick(acc), pick(st2_buf)).astype(bf16)
        FC, lag = cfg["FC"], 2
        y = None
        act = []
        outs = out_chunks(JL - 1)
        for c in range(F // FC + lag):
            if c < F // FC:
                cs = slice(c * FC, (c + 1) * FC)
                g = jnp.dot(xs, wg[:, cs], preferred_element_type=f32)
                u = jnp.dot(xs, wu[:, cs], preferred_element_type=f32)
                for v in (g, u):
                    for t in range(cfg["FOUT"]):
                        if outs:
                            outs.pop(0)(_zero_of(v[0:8, (t % 2) * 128:(t % 2 + 1) * 128]))
                            if not outs:
                                cp_out(JL - 1).start()
                g, u = _rb(g), _rb(u)
                act.append((_rb(g * jax.nn.sigmoid(g)) * u).astype(bf16))
            if c >= lag:
                d = jnp.dot(act[c - lag], wd[(c - lag) * FC:(c - lag + 1) * FC, :],
                            preferred_element_type=f32)
                y = d if y is None else y + d
        y = _rb(y)
        ya = _rb(y[0:1, :] * _wide(_rb(jax.nn.sigmoid(score_of(k1[0:1, :]))), D))
        yb = _rb(y[1:2, :] * _wide(_rb(jax.nn.sigmoid(score_of(k2[0:1, :]))), D))

        g1 = pl.multiple_of((i1s >> 4) << 4, 16)
        g2 = pl.multiple_of((i2s >> 4) << 4, 16)
        for t, g0 in enumerate((g1, g2)):
            rid = sub + g0
            x1 = acc[pl.ds(g0, 16), :]
            upd = jnp.where(rid == i1s, ya, 0.0) + jnp.where(rid == i2s, yb, 0.0)
            fix[t] = (x1 + gb * (adaln2(x1, st2_buf[pl.ds(g0, 16), :]) + upd)).astype(bf16)

        pltpu.make_async_copy(o_buf, out_hbm, sem_out.at[0]).wait()

        def cp_fix(t, g0):
            return pltpu.make_async_copy(fix.at[t], out_hbm.at[pl.ds(g0, 16), :], sem_fix.at[t])

        cp_fix(0, g1).start()

        @pl.when(g2 != g1)
        def _():
            cp_fix(1, g2).start()
            cp_fix(1, g2).wait()
        cp_fix(0, g1).wait()

    return kernel


_CFG = dict(
    G=4, T0=256, TB=1024, TL=256, MCH=256, RB=16, FC=256,
    LCA='cc80', LCB2='040g', NHB=16, NL4=8, BQ=3, LCNT='33333333332000',
    LSPLIT=(96, 96, 64), FOUT=2,
)


def _build(A_x, A_k_cache, A_v_cache, A_wq, A_wo, B_w_r, B_w_gate, B_w_up, B_w_down, c, w_mod,
           **over):
    B, S, D = A_x.shape
    _, H, SK, DH = A_k_cache.shape
    F = B_w_gate.shape[1]
    assert B == 1
    cfg = dict(_CFG, **over)
    T0, TL, G = cfg["T0"], cfg["TL"], cfg["G"]
    MC = (4 * D) // H
    kernel = _make_kernel(S, D, H, DH, SK, F, cfg)
    scratch = [
        pltpu.VMEM((S, D), bf16),
        pltpu.VMEM((S // 2, D), u32),
        pltpu.VMEM((S, D), f32),
        pltpu.VMEM((S, SK), f32),
        pltpu.VMEM((S, 128), f32),
        pltpu.VMEM((TL, SK), f32),
        pltpu.VMEM((TL, 128), f32),
        pltpu.VMEM((TL, SK), f32),
        pltpu.VMEM((TL, 128), f32),
        pltpu.VMEM((TL, SK), f32),
        pltpu.VMEM((TL, 128), f32),
        pltpu.VMEM((S, 256), f32),
        pltpu.VMEM((S, 256), f32),
        pltpu.VMEM((4, S // 2, DH), u32),
        pltpu.VMEM((G, S, DH), f32),
        pltpu.VMEM((8, G * DH), f32),
        pltpu.VMEM((4, SK, DH), bf16),
        pltpu.VMEM((4, SK, DH), bf16),
        pltpu.VMEM((D, G * DH), bf16),
        pltpu.VMEM((2, D, DH), bf16),
        pltpu.VMEM((4, DH, D), bf16),
        pltpu.VMEM((G + 1, D, MC), bf16),
        pltpu.VMEM((2, D, D // 2), bf16),
        pltpu.VMEM((D, D), bf16),
        pltpu.VMEM((1, D), bf16),
        pltpu.VMEM((D,), bf16),
        pltpu.VMEM((4, 1, D // 4), f32),
        pltpu.VMEM((D, 128), f32),
        pltpu.VMEM((2, 8, D), f32),
        pltpu.VMEM((H, 1, MC), f32),
        pltpu.VMEM((9, 8, D), f32),
        pltpu.VMEM((D, F), bf16),
        pltpu.VMEM((D, F), bf16),
        pltpu.VMEM((F, D), bf16),
        pltpu.VMEM((S, D), bf16),
        pltpu.VMEM((2, 8, 128), i32),
        pltpu.VMEM((2, 16, D), bf16),
        pltpu.SemaphoreType.DMA((sum(_sem_sizes(S, D, cfg)),)),
    ]
    any_spec = pl.BlockSpec(memory_space=pl.ANY)
    out = pl.pallas_call(
        kernel,
        out_shape=jax.ShapeDtypeStruct((S, D), bf16),
        in_specs=[any_spec] * 11,
        out_specs=any_spec,
        scratch_shapes=scratch,
        compiler_params=pltpu.CompilerParams(vmem_limit_bytes=112 * 1024 * 1024,
                                             disable_bounds_checks=True,
                                             disable_semaphore_checks=True),
    )(A_x.reshape(S, D), A_k_cache.reshape(H, SK, DH), A_v_cache.reshape(H, SK, DH),
      A_wq, A_wo, B_w_r, B_w_gate, B_w_up, B_w_down, c, w_mod)
    return out.reshape(B, S, D)


@jax.jit
def pallas_adaLN_cond__mha_block_cached__moe_arch_mod__prompt_kernel(
    A_x: jax.Array,
    A_k_cache: jax.Array,
    A_v_cache: jax.Array,
    A_wq: jax.Array,
    A_wo: jax.Array,
    B_x: jax.Array,
    B_w_r: jax.Array,
    B_w_gate: jax.Array,
    B_w_up: jax.Array,
    B_w_down: jax.Array,
    c: jax.Array,
    w_mod: jax.Array,
):
    del B_x
    return _build(A_x, A_k_cache, A_v_cache, A_wq, A_wo, B_w_r, B_w_gate, B_w_up, B_w_down,
                  c, w_mod)
```

```python
import jax
import jax.numpy as jnp
from jax import lax
import jax.experimental.pallas as pl
import jax.experimental.pallas.tpu as pltpu

f32 = jnp.float32
bf16 = jnp.bfloat16
u32 = jnp.uint32
i32 = jnp.int32

_NT = (((1,), (1,)), ((), ()))
_LOG2E = 1.4426950408889634
_EPS = 1e-5
_IMIN = -2 ** 31


def _rb(v):
    return v.astype(bf16).astype(f32)


def _rep(v, n):
    return v if n == 8 else jnp.tile(v, (n // 8, 1))


def _wide(v, w):
    return jnp.tile(v, (1, w // 128))


def _zero_of(v):
    bits = pltpu.bitcast(v, u32)
    return pltpu.bitcast(lax.shift_right_logical(lax.shift_right_logical(bits, jnp.uint32(31)),
                                                 jnp.uint32(1)), f32)


class _Pace:
    def __init__(self, chunks, counts):
        self.chunks = list(chunks)
        self.counts = [ch if isinstance(ch, int) else int(ch, 36) for ch in counts]
        assert sum(self.counts) == len(self.chunks), (counts, len(self.chunks))

    def done(self, res):
        n = self.counts.pop(0)
        for i in range(n):
            r0 = (i * res.shape[0] // n) // 8 * 8
            self.chunks.pop(0)(_zero_of(res[r0:r0 + 8, 0:128]))


def _tiles(v):
    return [v[:, c * 128:(c + 1) * 128] for c in range(v.shape[1] // 128)]


def _fold(op, parts):
    out = parts[0]
    for p in parts[1:]:
        out = op(out, p)
    return out


def _lane_sum(v):
    return jnp.broadcast_to(jnp.sum(v, axis=-1, keepdims=True), v.shape)


def _row_stats(xf, tok=None):
    d = xf.shape[-1]
    ts = _tiles(xf)
    nt = len(ts)
    if tok is not None:
        ts = [ts[0] + tok] + ts[1:]
    mu = _fold(jnp.add, ts) * (1.0 / nt)
    m2 = _fold(jnp.add, [(t - mu) * (t - mu) for t in ts])
    mean = _lane_sum(mu) * (1.0 / 128)
    dm = mu - mean
    var = _lane_sum(m2 + (dm * dm) * float(nt)) * (1.0 / d)
    return mean, lax.rsqrt(var + _EPS)


def _sem_sizes(S, D, cfg):
    j0 = S // cfg["T0"]
    return [2, 2 * (D // cfg["MCH"]), j0, 1, 16, 4, 1, 2]


def _make_kernel(S, D, H, DH, SK, F, cfg):
    T0, TL, MCH = cfg["T0"], cfg["TL"], cfg["MCH"]
    J0 = S // T0
    JL = S // TL
    qscale = DH ** -0.5 * _LOG2E
    n_mch = D // MCH
    G = cfg["G"]
    NB = H - G
    MC = (4 * D) // H
    W = 512
    NF = F // 128
    assert 2 <= G <= 4 and D == 2 * W and MC == DH == 128 and NF <= NB

    def kernel(x_hbm, k_hbm, v_hbm, wq_hbm, wo_hbm, wr_hbm, wg_hbm, wu_hbm, wd_hbm,
               c_hbm, wmod_hbm, out_hbm,
               x_buf, h_buf, acc, s_buf, m_buf, s2_buf, m2_buf, s3_buf, m3_buf, s4_buf, m4_buf,
               st_buf, st2_buf,
               q_ring, qf_buf, bq_buf,
               kb, vb, wq0, w4, wo2, wmx, wca, wsa, c_buf, wr_buf, sc_buf, cb_buf, mod0, modr, modv,
               wg, wu, wd, xc_buf, o_buf, key_buf, fix,
               sems):

        class _Sem:
            def __init__(self, base):
                self.base = base
                self.at = self

            def __getitem__(self, i):
                return sems.at[self.base + i]

        sizes = _sem_sizes(S, D, cfg)
        offs = [sum(sizes[:i]) for i in range(len(sizes))]
        (sem_small, sem_ca, sem_x, sem_sa, sem_first, sem_head,
         sem_out, sem_fix) = (_Sem(o) for o in offs)

        def _mul(a, n):
            v = a * n
            return v if isinstance(a, int) else pl.multiple_of(v, n)

        def view(ref, j, t, n=1):
            return ref.at[pl.ds(_mul(j, t), n * t), :]

        def cp_c():
            return pltpu.make_async_copy(c_hbm, c_buf, sem_small.at[0])

        def cp_wr():
            return pltpu.make_async_copy(wr_hbm, wr_buf, sem_small.at[1])

        def cp_ca(c, i):
            return pltpu.make_async_copy(
                wmod_hbm.at[pl.ds(i * MCH, MCH), pl.ds(D + c * W, W)], view(wca.at[c], i, MCH),
                sem_ca.at[c * n_mch + i])

        def cp_sa():
            return pltpu.make_async_copy(wmod_hbm.at[:, pl.ds(0, D)], wsa, sem_sa.at[0])

        def cp_x(j):
            return pltpu.make_async_copy(view(x_hbm, j, T0), view(x_buf, j, T0), sem_x.at[j])

        def cp_wq0(c):
            return pltpu.make_async_copy(wq_hbm.at[pl.ds(c * W, W), pl.ds(0, G * DH)],
                                         view(wq0, c, W), sem_first.at[14 + c])

        def cp_k(h, sem=None):
            return pltpu.make_async_copy(k_hbm.at[h], kb.at[h & 3],
                                         sem_head.at[0] if sem is None else sem)

        def cp_v(h, sem=None):
            return pltpu.make_async_copy(v_hbm.at[h], vb.at[h & 3],
                                         sem_head.at[1] if sem is None else sem)

        def cp_wo(h, sem=None):
            return pltpu.make_async_copy(view(wo_hbm, h, DH), wo2.at[h & 3, 0],
                                         sem_head.at[2] if sem is None else sem)

        def _clamp(a, hi):
            return min(a, hi) if isinstance(a, int) else jnp.minimum(a, hi)

        def cols(ref, t):
            return ref.at[:, pl.ds(_mul(t, 128), 128)]

        def cp_wmx(p):
            return pltpu.make_async_copy(cols(wmod_hbm, p + (2 * D) // MC), wmx.at[p - NB - 1],
                                         sem_first.at[4 + p - NB])

        def start_head(h):
            f = _clamp(h, NF - 1)
            for i, src in enumerate((cols(wq_hbm, _clamp(h + G, H - 1)),
                                     cols(wmod_hbm, h + (2 * D) // MC),
                                     cols(wg_hbm, f), cols(wu_hbm, f))):
                pltpu.make_async_copy(src, w4.at[h & 1, i], sem_head.at[3]).start()
            cp_k(h + G - 1).start()
            cp_wo(h + 2).start()
            pltpu.make_async_copy(view(wd_hbm, f, 128), wo2.at[(h + 2) & 3, 1],
                                  sem_head.at[2]).start()
            cp_v(h + 2).start()

        def wait_head(h):
            pltpu.make_async_copy(w4.at[h & 1], w4.at[h & 1], sem_head.at[3]).wait()
            cp_k(h + G - 1).wait()
            pltpu.make_async_copy(wo2.at[(h + 2) & 3], wo2.at[(h + 2) & 3], sem_head.at[2]).wait()
            cp_v(h + 2).wait()

        def pack_chunks(h):
            f = _clamp(h, NF - 1)
            out = []
            for sv, dv in ((w4.at[h & 1, 2], wg.at[f]), (w4.at[h & 1, 3], wu.at[f]),
                           (wo2.at[(h + 2) & 3, 1], view(wd, f, 64))):
                n, w = sv.shape
                step = n // 4

                def chunk(r, sv=sv, dv=dv, step=step, w=w):
                    def fn(tok):
                        z = _rep(_wide(pltpu.bitcast(tok, u32), w), step // 2)
                        dv[r // 2:(r + step) // 2, :] = pltpu.bitcast(sv[r:r + step, :], u32) | z
                    return fn
                out += [chunk(r) for r in range(0, n, step)]
            return out

        def cp_out(j):
            return pltpu.make_async_copy(view(o_buf, j, TL), view(out_hbm, j, TL), sem_out.at[0])

        def ln1_chunks(xv, sv):
            def chunk(off):
                def f(tok=None):
                    mean, inv = _row_stats(xv[off:off + 8, :].astype(f32), tok)
                    sv[off:off + 8, 0:128] = mean
                    sv[off:off + 8, 128:256] = inv
                return f
            return [chunk(off) for off in range(0, xv.shape[0], 8)]

        def ln1_scaled(x, stat, cs, tok=None):
            w = x.shape[1]
            mean = stat[:, 0:128] if tok is None else stat[:, 0:128] + _rep(tok, x.shape[0])
            n = (x.astype(f32) - _wide(mean, w)) * _wide(stat[:, 128:256], w)
            return n * _rep(mod0[1, :, cs], x.shape[0])

        def qproj(h, wv):
            q = None
            for c in range(D // W):
                cs = slice(c * W, (c + 1) * W)
                part = jnp.dot(pltpu.bitcast(h_buf[:, cs], bf16), wv[cs, :],
                               preferred_element_type=f32)
                q = part if q is None else q + part
            q_ring[h & 3] = pltpu.bitcast((q * qscale).astype(bf16), u32)

        def q_early(g, q):
            return ((q + _rep(bq_buf[:, g * DH:(g + 1) * DH], q.shape[0])) * qscale).astype(bf16)

        def scores(h, q, sv, mv, rec=None, reload=False):
            mp = None
            for c in range(SK // W):
                cs = slice(c * W, (c + 1) * W)
                s = lax.dot_general(q, kb[h & 3, cs, :], _NT, preferred_element_type=f32)
                sv[:, cs] = s
                if rec is not None:
                    rec.done(s)
                if not reload:
                    mp = _fold(jnp.maximum, ([] if mp is None else [mp]) + _tiles(s))
            if reload:
                mp = _fold(jnp.maximum, _tiles(sv[...]))
            mv[...] = jnp.broadcast_to(jnp.max(mp, axis=-1, keepdims=True), mp.shape)

        def pv(h, sv, mv, rec=None, late=False):
            o = lp = None
            for c in range(SK // W):
                cs = slice(c * W, (c + 1) * W)
                p = jnp.exp2(sv[:, cs] - _wide(mv[...], W))
                lp = _fold(jnp.add, ([] if lp is None else [lp]) + _tiles(p))
                d = jnp.dot(p.astype(bf16), vb[h & 3, cs, :], preferred_element_type=f32)
                o = d if o is None else o + d
                if rec is not None:
                    rec.done(d)
            if late:
                lp = lp + _zero_of(o)
            l = jnp.sum(lp, axis=-1, keepdims=True)
            r = pl.reciprocal(l, approx=True)
            r = r * (2.0 - l * r)
            return (o * r).astype(bf16)

        def oproj(hos, av, xv=None, rec=None):
            for c in range(D // W):
                cs = slice(c * W, (c + 1) * W)
                a = av[:, cs]
                for h, o in hos:
                    if not isinstance(h, int):
                        a = jnp.where(h > 0, a, 0.0)
                    d = jnp.dot(o, wo2[h & 3, 0, :, cs], preferred_element_type=f32)
                    if rec is not None:
                        rec.done(d)
                    a = a + d
                if xv is not None:
                    a = xv[:, cs].astype(f32) + _rep(modv[0, :, cs], a.shape[0]) * a
                av[:, cs] = a

        def matvec(wv, tok=None, step=16):
            n = wv.shape[1]
            part = None if tok is None else _wide(tok, n)
            for r in range(0, D, step):
                t = wv[r:r + step, :].astype(f32) * _wide(cb_buf[r:r + step, :], n)
                for e in range(step // 8):
                    te = t[e * 8:(e + 1) * 8, :]
                    part = te if part is None else part + te
            return _rb(jnp.sum(part, axis=0, keepdims=True))

        def mod_piece(p, tok=None):
            extra = isinstance(p, int) and p > NB
            modr[p] = matvec(wmx.at[p - NB - 1] if extra else w4.at[p & 1, 1], tok)

        def finish_mod():
            n = D // MC
            ga, sb, cb, gb = (jnp.concatenate([modr[i * n + t] for t in range(n)], axis=-1)
                              for i in range(4))
            cb1 = _rb(1.0 + cb)
            wr = wr_buf[...].astype(f32).reshape(1, D)
            a = cb1 * wr
            a0 = jnp.broadcast_to(jnp.sum(a, axis=-1, keepdims=True), (1, D))
            b0 = jnp.broadcast_to(jnp.sum(sb * wr, axis=-1, keepdims=True), (1, D))
            for i, v in enumerate((ga, sb, cb1, gb, a, gb * cb1, gb * sb, a0, b0)):
                modv[i] = jnp.broadcast_to(v, (8, D))

        def out_rows(x1, mean, inv):
            return (x1 + ((x1 - _wide(mean, D)) * (_wide(inv, D) * modv[5]) + modv[6])).astype(bf16)

        def out_chunks(j):
            x1v, sv, ov = view(acc, j, TL), view(st2_buf, j, TL), view(o_buf, j, TL)

            def chunk(off):
                def f(tok):
                    rs = slice(off, off + 8)
                    ov[rs, :] = out_rows(x1v[rs, :], sv[rs, 0:128] + tok, sv[rs, 128:256] + tok)
                return f
            return [chunk(off) for off in range(0, TL, 8)]

        def epi_chunks(j, x1v, ov, with_out=True):
            sub = lax.broadcasted_iota(i32, (8, 128), 0)
            low = (0xFFFF - j * TL) - sub
            sv = view(st2_buf, j, TL)
            st = {}

            def chunk(off):
                def f(tok=None):
                    if off == 0:
                        st["k1"], st["k2"] = key_buf[0], key_buf[1]
                    x1 = x1v[off:off + 8, :]
                    mean, inv = _row_stats(x1, tok)
                    sv[off:off + 8, 0:128] = mean
                    sv[off:off + 8, 128:256] = inv
                    xa = _tiles(x1 * modv[4])
                    if tok is not None:
                        xa[0] = xa[0] + tok
                    ra = _lane_sum(_fold(jnp.add, xa))
                    r = inv * (ra - mean * modv[7, :, 0:128]) + modv[8, :, 0:128]
                    if with_out:
                        ov[off:off + 8, :] = out_rows(x1, mean, inv)
                    bits = pltpu.bitcast(_rb(r) + 0.0, i32)
                    key = jnp.where(bits < 0, bits ^ 0x7FFF0000, bits) | (low - off)
                    st["k2"] = jnp.maximum(st["k2"], jnp.minimum(st["k1"], key))
                    st["k1"] = jnp.maximum(st["k1"], key)
                    if off + 8 == TL:
                        key_buf[0], key_buf[1] = st["k1"], st["k2"]
                return f
            return [chunk(off) for off in range(0, TL, 8)]

        cp_c().start()
        cp_x(0).start()
        for c in range(2):
            cp_wq0(c).start()
            for i in range(n_mch):
                cp_ca(c, i).start()
            if c == 0:
                for j in range(1, J0):
                    cp_x(j).start()
        cp_sa().start()
        for h in range(G - 1):
            cp_k(h, sem_first.at[1 + h]).start()
        early = []
        for h in range(2):
            early += [cp_v(h, sem_first.at[8 + 2 * h]), cp_wo(h, sem_first.at[9 + 2 * h])]
        for cp in early:
            cp.start()
        start_head(0)

        cp_c().wait()
        cf = c_buf[...].astype(f32)
        sc = _rb(cf * jax.nn.sigmoid(cf))
        for t in range(4):
            sc_buf[t] = sc[:, t * (D // 4):(t + 1) * (D // 4)]

        def cb_body(t, carry):
            view(cb_buf, t, D // 4)[...] = jnp.transpose(jnp.broadcast_to(sc_buf[t], (128, D // 4)))
            return carry
        lax.fori_loop(0, 4, cb_body, 0)
        key_buf[...] = jnp.full(key_buf.shape, _IMIN, i32)
        cp_x(0).wait()

        def st0_body(i, carry):
            for ch in ln1_chunks(view(x_buf, i, T0 // 4), view(st_buf, i, T0 // 4)):
                ch()
            return carry
        lax.fori_loop(0, 4, st0_body, 0)

        def ca_half(c, stream):
            cp_wq0(c).wait()
            if not stream:
                for i in range(n_mch):
                    cp_ca(c, i).wait()
            part = None
            for i in range(n_mch):
                if stream:
                    cp_ca(c, i).wait()
                scb = jnp.broadcast_to(sc[:, i * MCH:(i + 1) * MCH], (16, MCH)).astype(bf16)
                d = jnp.dot(scb, wca[c, i * MCH:(i + 1) * MCH, :], preferred_element_type=f32)
                part = d if part is None else part + d
            mod0[1, :, c * W:(c + 1) * W] = _rb(1.0 + _rb(part[0:8, :]))

        def q_first(r0, t, c, rec, mid=None):
            rows = pl.ds(r0, t)
            cs = slice(c * W, (c + 1) * W)
            hh = ln1_scaled(x_buf[rows, cs], st_buf[rows, :], cs).astype(bf16)
            for g in range(G):
                if mid is not None and g == mid[0]:
                    mid[1]()
                part = jnp.dot(hh, wq0[cs, g * DH:(g + 1) * DH], preferred_element_type=f32)
                qf_buf[g, rows, :] = part if c == 0 else qf_buf[g, rows, :] + part
                if rec is not None:
                    rec.done(part)

        ca_half(0, True)

        def pa_body(j, carry):
            @pl.when(j + 1 < J0)
            def _():
                cp_x(j + 1).wait()
            jn = jnp.minimum(j + 1, J0 - 1)
            rec = _Pace(ln1_chunks(view(x_buf, jn, T0), view(st_buf, jn, T0)), cfg["LCA"])
            q_first(_mul(j, T0), T0, 0, rec)
            return carry
        lax.fori_loop(0, J0, pa_body, 0)

        TB, RB = cfg["TB"], cfg["RB"]
        ca_half(1, False)
        q_first(0, TB, 1, None)
        cp_sa().wait()
        cp_k(0, sem_first.at[1]).wait()
        cp_wr().start()
        for p in range(NB + 1, H):
            cp_wmx(p).start()

        def sa_chunk(t):
            def f(tok):
                cs = slice(t * 256, (t + 1) * 256)
                mod0[0, :, cs] = jnp.broadcast_to(matvec(wsa.at[:, cs], tok, 8), (8, 256))
            return f

        def sa_bias():
            bq_buf[...] = jnp.dot(_rep(mod0[0], 16).astype(bf16), wq0[...],
                                  preferred_element_type=f32)[0:8, :]

        def h_chunk(off):
            def f(tok):
                rs, rh = slice(off, off + RB), slice(off // 2, (off + RB) // 2)
                hh = (ln1_scaled(x_buf[rs, :], st_buf[rs, :], slice(0, D), tok)
                      + _rep(mod0[0], RB)).astype(bf16)
                h_buf[rh, :] = pltpu.bitcast(hh, u32)
            return f

        def q_chunk(off):
            def f(tok):
                n = 2 * RB
                rs, rh = slice(off, off + n), slice(off // 2, (off + n) // 2)
                for g in range(1, G):
                    q_ring[g, rh, :] = pltpu.bitcast(
                        q_early(g, qf_buf[g, rs, :] + _rep(tok, n)), u32)
            return f

        hs = [h_chunk(off) for off in range(0, S, RB)]
        qs = [q_chunk(off) for off in range(0, S, 2 * RB)]
        nh = cfg["NHB"]
        rest_chunks = []
        nq, nr = len(qs), len(hs) - nh
        for i, ch in enumerate(hs[nh:]):
            rest_chunks.append(ch)
            while qs and (nq - len(qs)) * nr < (i + 1) * nq:
                rest_chunks.append(qs.pop(0))
        assert not qs
        rec = _Pace([sa_chunk(t) for t in range(D // 256)] + hs[:nh], cfg["LCB2"])
        q_first(TB, S - TB, 1, rec, mid=(cfg["BQ"], sa_bias))
        n4 = len(rest_chunks)
        n3 = n4 - cfg["NL4"]
        cnt = [n3 // 3 + (1 if i < n3 % 3 else 0) for i in range(3)] + [cfg["NL4"]]
        scores(0, q_early(0, qf_buf[0]), s_buf, m_buf, rec=_Pace(rest_chunks, cnt), reload=True)

        def main_body(h, carry):
            qproj(h + G, w4.at[h & 1, 0])
            start_head(h + 1)
            o = pv(h, s_buf, m_buf)
            rec = _Pace([lambda tok: mod_piece(h, tok)] + pack_chunks(h), cfg["LCM"])
            scores(h + 1, pltpu.bitcast(q_ring[(h + 1) & 3], bf16), s_buf, m_buf, rec=rec)
            oproj([(h, o)], acc)
            wait_head(h + 1)
            return carry
        for h in range(1, G - 1):
            cp_k(h, sem_first.at[1 + h]).wait()
        for cp in early:
            cp.wait()
        wait_head(0)
        lax.fori_loop(0, NB, main_body, 0)

        ha = NB
        rest = list(zip(range(NB + 1, H), (s2_buf, s3_buf, s4_buf), (m2_buf, m3_buf, m4_buf)))
        late = []
        for n, h in enumerate(range(NB + 3, H)):
            late += [cp_v(h, sem_first.at[8 + 2 * n]), cp_wo(h, sem_first.at[9 + 2 * n])]
        for cp in late:
            cp.start()
        cp_wr().wait()
        for p in range(NB + 1, H):
            cp_wmx(p).wait()

        def l_step(j, do_x, do_y):
            if do_x and do_y:
                aw = view(acc, j - 1, TL, 2)
                ay, ax = aw.at[0:TL, :], aw.at[TL:2 * TL, :]
            elif do_x:
                ax = view(acc, j, TL)
            else:
                ay = view(acc, j - 1, TL)
            rec = None
            if do_y:
                chunks = epi_chunks(j - 1, ay, view(o_buf, j - 1, TL), with_out=do_x)
                os_ = [(h, pv(h, sv, mv, late=not do_x)) for h, sv, mv in rest]
            if do_x:
                oa = pv(ha, view(s_buf, j, TL), view(m_buf, j, TL))
            if do_y and do_x:
                oproj(os_, ay, view(x_buf, j - 1, TL))
            elif do_y:
                xv = view(x_buf, j - 1, TL)
                r0, prev = 0, []
                for n in cfg["LSPLIT"]:
                    rs = slice(r0, r0 + n)
                    nr = len(os_) * (D // W)
                    cnt = [len(prev) // nr + (1 if i < len(prev) % nr else 0) for i in range(nr)]
                    rec = _Pace(prev, cnt)
                    oproj([(h, o[rs]) for h, o in os_], ay.at[rs, :], xv.at[rs, :], rec=rec)
                    prev = chunks[r0 // 8:(r0 + n) // 8]
                    r0 += n
                chunks = prev
            if do_x:
                if do_y:
                    rec = _Pace(chunks, cfg["LCNT"])
                for h, sv, mv in rest:
                    q = pltpu.bitcast(view(q_ring.at[h & 3], j, TL // 2)[...], bf16)
                    scores(h, q, sv, mv, rec=rec, reload=True)
                oproj([(ha, oa)], ax, rec=rec)
            if do_y:
                if do_x:
                    cp_out(j - 1).start()
                else:
                    for ch in chunks:
                        ch()

        for p in range(NB, H):
            mod_piece(p)
        finish_mod()
        l_step(0, True, False)
        for cp in late:
            cp.wait()

        def pl_body(j, carry):
            l_step(j, True, True)
            return carry
        lax.fori_loop(1, JL, pl_body, 0)
        l_step(JL, False, True)

        k1, k2 = key_buf[0], key_buf[1]
        for sh in (4, 2, 1):
            o1, o2 = pltpu.roll(k1, sh, 0), pltpu.roll(k2, sh, 0)
            k2 = jnp.maximum(jnp.minimum(k1, o1), jnp.maximum(k2, o2))
            k1 = jnp.maximum(k1, o1)

        def score_of(k):
            hi = k & jnp.int32(-65536)
            return pltpu.bitcast(jnp.where(hi < 0, hi ^ 0x7FFF0000, hi), f32)

        i1s = jnp.minimum(0xFFFF - (k1[0, 0] & 0xFFFF), S - 1)
        i2s = jnp.minimum(0xFFFF - (k2[0, 0] & 0xFFFF), S - 1)

        sub = lax.broadcasted_iota(i32, (16, D), 0)
        sb, cb1, gb = (_rep(modv[i], 16) for i in (1, 2, 3))

        def adaln2(x1, stat):
            return (x1 - _wide(stat[:, 0:128], D)) * _wide(stat[:, 128:256], D) * cb1 + sb

        def pick(ref):
            sel = lax.broadcasted_iota(i32, (16, ref.shape[1]), 0) == 0
            return jnp.where(sel, ref[pl.ds(i1s, 1), :], ref[pl.ds(i2s, 1), :])

        xs = adaln2(pick(acc), pick(st2_buf)).astype(bf16)
        FC, lag, KV, skip = cfg["FC"], cfg["FLAG"], cfg["KV"], cfg["FSKIP"]

        def wrows(ref, a, b, c):
            n = FC // 128
            u = [ref[c * n + t, a // 2:b // 2, :] for t in range(n)]
            return pltpu.bitcast(u[0] if n == 1 else jnp.concatenate(u, axis=1), bf16)

        DV = D - KV * 128
        if KV:
            xf = xs.astype(f32)
            for r in range(2):
                xc_buf[r] = jnp.transpose(jnp.broadcast_to(xf[r:r + 1, DV:], (128, D - DV)))
        subc = lax.broadcasted_iota(i32, (16, FC), 0)
        y = None
        act = []
        outs = out_chunks(JL - 1)
        for c in range(F // FC + lag):
            if c < F // FC:
                dm = DV if c >= skip else D
                gu = [jnp.dot(xs[:, :dm], wrows(w, 0, dm, c), preferred_element_type=f32)
                      for w in (wg, wu)]
                for v in gu:
                    for t in range(cfg["FOUT"]):
                        if outs:
                            outs.pop(0)(_zero_of(v[0:8, (t % 2) * 128:(t % 2 + 1) * 128]))
                            if not outs:
                                cp_out(JL - 1).start()
                if dm < D:
                    part = [[None, None], [None, None]]
                    for k in range(DV, D, 16):
                        xcol = [_wide(xc_buf[r, k - DV:k - DV + 16, :], FC) for r in range(2)]
                        for m, w in enumerate((wg, wu)):
                            wv = wrows(w, k, k + 16, c).astype(f32)
                            for r in range(2):
                                t = wv * xcol[r]
                                for e in range(2):
                                    te = t[e * 8:(e + 1) * 8, :]
                                    part[m][r] = te if part[m][r] is None else part[m][r] + te
                    for m in range(2):
                        ra, rb_ = (jnp.sum(v, axis=0, keepdims=True) for v in part[m])
                        gu[m] = gu[m] + jnp.where(subc == 0, ra, rb_)
                g, u = _rb(gu[0]), _rb(gu[1])
                act.append((_rb(g * jax.nn.sigmoid(g)) * u).astype(bf16))
            if c >= lag:
                wdc = pltpu.bitcast(wd[(c - lag) * FC // 2:(c - lag + 1) * FC // 2, :], bf16)
                d = jnp.dot(act[c - lag], wdc, preferred_element_type=f32)
                y = d if y is None else y + d
        y = _rb(y)
        ya = _rb(y[0:1, :] * _wide(_rb(jax.nn.sigmoid(score_of(k1[0:1, :]))), D))
        yb = _rb(y[1:2, :] * _wide(_rb(jax.nn.sigmoid(score_of(k2[0:1, :]))), D))

        g1 = pl.multiple_of((i1s >> 4) << 4, 16)
        g2 = pl.multiple_of((i2s >> 4) << 4, 16)
        for t, g0 in enumerate((g1, g2)):
            rid = sub + g0
            x1 = acc[pl.ds(g0, 16), :]
            upd = jnp.where(rid == i1s, ya, 0.0) + jnp.where(rid == i2s, yb, 0.0)
            fix[t] = (x1 + gb * (adaln2(x1, st2_buf[pl.ds(g0, 16), :]) + upd)).astype(bf16)

        pltpu.make_async_copy(o_buf, out_hbm, sem_out.at[0]).wait()

        def cp_fix(t, g0):
            return pltpu.make_async_copy(fix.at[t], out_hbm.at[pl.ds(g0, 16), :], sem_fix.at[t])

        cp_fix(0, g1).start()

        @pl.when(g2 != g1)
        def _():
            cp_fix(1, g2).start()
            cp_fix(1, g2).wait()
        cp_fix(0, g1).wait()

    return kernel


_CFG = dict(
    G=4, T0=256, TB=1024, TL=256, MCH=256, RB=16, FC=256,
    LCA='cc80', LCB2='040g', NHB=16, NL4=8, BQ=3, LCNT='33333333332000',
    LCM='1660',
    LSPLIT=(96, 96, 64), FOUT=2, FLAG=1, KV=2, FSKIP=2,
)


def _build(A_x, A_k_cache, A_v_cache, A_wq, A_wo, B_w_r, B_w_gate, B_w_up, B_w_down, c, w_mod,
           **over):
    B, S, D = A_x.shape
    _, H, SK, DH = A_k_cache.shape
    F = B_w_gate.shape[1]
    assert B == 1
    cfg = dict(_CFG, **over)
    T0, TL, G = cfg["T0"], cfg["TL"], cfg["G"]
    MC = (4 * D) // H
    kernel = _make_kernel(S, D, H, DH, SK, F, cfg)
    scratch = [
        pltpu.VMEM((S, D), bf16),
        pltpu.VMEM((S // 2, D), u32),
        pltpu.VMEM((S, D), f32),
        pltpu.VMEM((S, SK), f32),
        pltpu.VMEM((S, 128), f32),
        pltpu.VMEM((TL, SK), f32),
        pltpu.VMEM((TL, 128), f32),
        pltpu.VMEM((TL, SK), f32),
        pltpu.VMEM((TL, 128), f32),
        pltpu.VMEM((TL, SK), f32),
        pltpu.VMEM((TL, 128), f32),
        pltpu.VMEM((S, 256), f32),
        pltpu.VMEM((S, 256), f32),
        pltpu.VMEM((4, S // 2, DH), u32),
        pltpu.VMEM((G, S, DH), f32),
        pltpu.VMEM((8, G * DH), f32),
        pltpu.VMEM((4, SK, DH), bf16),
        pltpu.VMEM((4, SK, DH), bf16),
        pltpu.VMEM((D, G * DH), bf16),
        pltpu.VMEM((2, 4, D, 128), bf16),
        pltpu.VMEM((4, 2, DH, D), bf16),
        pltpu.VMEM((G - 1, D, MC), bf16),
        pltpu.VMEM((2, D, D // 2), bf16),
        pltpu.VMEM((D, D), bf16),
        pltpu.VMEM((1, D), bf16),
        pltpu.VMEM((D,), bf16),
        pltpu.VMEM((4, 1, D // 4), f32),
        pltpu.VMEM((D, 128), f32),
        pltpu.VMEM((2, 8, D), f32),
        pltpu.VMEM((H, 1, MC), f32),
        pltpu.VMEM((9, 8, D), f32),
        pltpu.VMEM((F // 128, D // 2, 128), u32),
        pltpu.VMEM((F // 128, D // 2, 128), u32),
        pltpu.VMEM((F // 2, D), u32),
        pltpu.VMEM((2, max(cfg["KV"], 1) * 128, 128), f32),
        pltpu.VMEM((S, D), bf16),
        pltpu.VMEM((2, 8, 128), i32),
        pltpu.VMEM((2, 16, D), bf16),
        pltpu.SemaphoreType.DMA((sum(_sem_sizes(S, D, cfg)),)),
    ]
    any_spec = pl.BlockSpec(memory_space=pl.ANY)
    out = pl.pallas_call(
        kernel,
        out_shape=jax.ShapeDtypeStruct((S, D), bf16),
        in_specs=[any_spec] * 11,
        out_specs=any_spec,
        scratch_shapes=scratch,
        compiler_params=pltpu.CompilerParams(vmem_limit_bytes=112 * 1024 * 1024,
                                             disable_bounds_checks=True,
                                             disable_semaphore_checks=True),
    )(A_x.reshape(S, D), A_k_cache.reshape(H, SK, DH), A_v_cache.reshape(H, SK, DH),
      A_wq, A_wo, B_w_r, B_w_gate, B_w_up, B_w_down, c, w_mod)
    return out.reshape(B, S, D)


@jax.jit
def pallas_adaLN_cond__mha_block_cached__moe_arch_mod__prompt_kernel(
    A_x: jax.Array,
    A_k_cache: jax.Array,
    A_v_cache: jax.Array,
    A_wq: jax.Array,
    A_wo: jax.Array,
    B_x: jax.Array,
    B_w_r: jax.Array,
    B_w_gate: jax.Array,
    B_w_up: jax.Array,
    B_w_down: jax.Array,
    c: jax.Array,
    w_mod: jax.Array,
):
    del B_x
    return _build(A_x, A_k_cache, A_v_cache, A_wq, A_wo, B_w_r, B_w_gate, B_w_up, B_w_down,
                  c, w_mod)
```

```python
import jax
import jax.numpy as jnp
from jax import lax
import jax.experimental.pallas as pl
import jax.experimental.pallas.tpu as pltpu

f32 = jnp.float32
bf16 = jnp.bfloat16
u32 = jnp.uint32
i32 = jnp.int32

_NT = (((1,), (1,)), ((), ()))
_LOG2E = 1.4426950408889634
_EPS = 1e-5
_IMIN = -2 ** 31


def _rb(v):
    return v.astype(bf16).astype(f32)


def _rep(v, n):
    return v if n == 8 else jnp.tile(v, (n // 8, 1))


def _wide(v, w):
    return jnp.tile(v, (1, w // 128))


def _zero_of(v):
    bits = pltpu.bitcast(v, u32)
    return pltpu.bitcast(lax.shift_right_logical(lax.shift_right_logical(bits, jnp.uint32(31)),
                                                 jnp.uint32(1)), f32)


class _Pace:
    def __init__(self, chunks, counts):
        self.chunks = list(chunks)
        self.counts = [ch if isinstance(ch, int) else int(ch, 36) for ch in counts]
        assert sum(self.counts) == len(self.chunks), (counts, len(self.chunks))

    def done(self, res):
        n = self.counts.pop(0)
        for i in range(n):
            r0 = (i * res.shape[0] // n) // 8 * 8
            self.chunks.pop(0)(_zero_of(res[r0:r0 + 8, 0:128]))


def _tiles(v):
    return [v[:, c * 128:(c + 1) * 128] for c in range(v.shape[1] // 128)]


def _fold(op, parts):
    out = parts[0]
    for p in parts[1:]:
        out = op(out, p)
    return out


def _lane_sum(v):
    return jnp.broadcast_to(jnp.sum(v, axis=-1, keepdims=True), v.shape)


def _row_stats(xf, tok=None):
    d = xf.shape[-1]
    ts = _tiles(xf)
    nt = len(ts)
    if tok is not None:
        ts = [ts[0] + tok] + ts[1:]
    mu = _fold(jnp.add, ts) * (1.0 / nt)
    m2 = _fold(jnp.add, [(t - mu) * (t - mu) for t in ts])
    mean = _lane_sum(mu) * (1.0 / 128)
    dm = mu - mean
    var = _lane_sum(m2 + (dm * dm) * float(nt)) * (1.0 / d)
    return mean, lax.rsqrt(var + _EPS)


def _sem_sizes(S, D, cfg):
    j0 = S // cfg["T0"]
    return [2, 2 * (D // cfg["MCH"]), j0, 1, 16, 4, 1, 2]


def _make_kernel(S, D, H, DH, SK, F, cfg):
    T0, TL, MCH = cfg["T0"], cfg["TL"], cfg["MCH"]
    J0 = S // T0
    JL = S // TL
    qscale = DH ** -0.5 * _LOG2E
    n_mch = D // MCH
    G = cfg["G"]
    NB = H - G
    MC = (4 * D) // H
    W = 512
    NF = F // 128
    assert 2 <= G <= 4 and D == 2 * W and MC == DH == 128 and NF <= NB

    def kernel(x_hbm, k_hbm, v_hbm, wq_hbm, wo_hbm, wr_hbm, wg_hbm, wu_hbm, wd_hbm,
               c_hbm, wmod_hbm, out_hbm,
               x_buf, h_buf, acc, s_buf, m_buf, s2_buf, m2_buf, s3_buf, m3_buf, s4_buf, m4_buf,
               st_buf, st2_buf,
               q_ring, qf_buf, bq_buf,
               kb, vb, wq0, w4, wo2, wmx, wca, wsa, c_buf, wr_buf, sc_buf, cb_buf, mod0, modr, modv,
               wg, wu, wd, xc_buf, o_buf, key_buf, fix,
               sems):

        class _Sem:
            def __init__(self, base):
                self.base = base
                self.at = self

            def __getitem__(self, i):
                return sems.at[self.base + i]

        sizes = _sem_sizes(S, D, cfg)
        offs = [sum(sizes[:i]) for i in range(len(sizes))]
        (sem_small, sem_ca, sem_x, sem_sa, sem_first, sem_head,
         sem_out, sem_fix) = (_Sem(o) for o in offs)

        def _mul(a, n):
            v = a * n
            return v if isinstance(a, int) else pl.multiple_of(v, n)

        def view(ref, j, t, n=1):
            return ref.at[pl.ds(_mul(j, t), n * t), :]

        def cp_c():
            return pltpu.make_async_copy(c_hbm, c_buf, sem_small.at[0])

        def cp_wr():
            return pltpu.make_async_copy(wr_hbm, wr_buf, sem_small.at[1])

        def cp_ca(c, i):
            return pltpu.make_async_copy(
                wmod_hbm.at[pl.ds(i * MCH, MCH), pl.ds(D + c * W, W)], view(wca.at[c], i, MCH),
                sem_ca.at[c * n_mch + i])

        def cp_sa():
            return pltpu.make_async_copy(wmod_hbm.at[:, pl.ds(0, D)], wsa, sem_sa.at[0])

        def cp_x(j):
            return pltpu.make_async_copy(view(x_hbm, j, T0), view(x_buf, j, T0), sem_x.at[j])

        def cp_wq0(c):
            return pltpu.make_async_copy(wq_hbm.at[pl.ds(c * W, W), pl.ds(0, G * DH)],
                                         view(wq0, c, W), sem_first.at[14 + c])

        def cp_k(h, sem=None):
            return pltpu.make_async_copy(k_hbm.at[h], kb.at[h & 3],
                                         sem_head.at[0] if sem is None else sem)

        def cp_v(h, sem=None):
            return pltpu.make_async_copy(v_hbm.at[h], vb.at[h & 3],
                                         sem_head.at[1] if sem is None else sem)

        def cp_wo(h, sem=None):
            return pltpu.make_async_copy(view(wo_hbm, h, DH), wo2.at[h & 3, 0],
                                         sem_head.at[2] if sem is None else sem)

        def _clamp(a, hi):
            return min(a, hi) if isinstance(a, int) else jnp.minimum(a, hi)

        def cols(ref, t):
            return ref.at[:, pl.ds(_mul(t, 128), 128)]

        def cp_wmx(p):
            return pltpu.make_async_copy(cols(wmod_hbm, p + (2 * D) // MC), wmx.at[p - NB - 1],
                                         sem_first.at[4 + p - NB])

        def start_head(h):
            f = _clamp(h, NF - 1)
            for i, src in enumerate((cols(wq_hbm, _clamp(h + G, H - 1)),
                                     cols(wmod_hbm, h + (2 * D) // MC),
                                     cols(wg_hbm, f), cols(wu_hbm, f))):
                pltpu.make_async_copy(src, w4.at[h & 1, i], sem_head.at[3]).start()
            cp_k(h + G - 1).start()
            cp_wo(h + 2).start()
            pltpu.make_async_copy(view(wd_hbm, f, 128), wo2.at[(h + 2) & 3, 1],
                                  sem_head.at[2]).start()
            cp_v(h + 2).start()

        def wait_head(h):
            pltpu.make_async_copy(w4.at[h & 1], w4.at[h & 1], sem_head.at[3]).wait()
            cp_k(h + G - 1).wait()
            pltpu.make_async_copy(wo2.at[(h + 2) & 3], wo2.at[(h + 2) & 3], sem_head.at[2]).wait()
            cp_v(h + 2).wait()

        def pack_chunks(h):
            f = _clamp(h, NF - 1)
            out = []
            for sv, dv in ((w4.at[h & 1, 2], wg.at[f]), (w4.at[h & 1, 3], wu.at[f]),
                           (wo2.at[(h + 2) & 3, 1], view(wd, f, 64))):
                n, w = sv.shape
                step = n // cfg['PKN']

                def chunk(r, sv=sv, dv=dv, step=step, w=w):
                    def fn(tok):
                        z = _rep(_wide(pltpu.bitcast(tok, u32), w), step // 2)
                        dv[r // 2:(r + step) // 2, :] = pltpu.bitcast(sv[r:r + step, :], u32) | z
                    return fn
                out += [chunk(r) for r in range(0, n, step)]
            return out

        def cp_out(j):
            return pltpu.make_async_copy(view(o_buf, j, TL), view(out_hbm, j, TL), sem_out.at[0])

        def ln1_chunks(xv, sv):
            def chunk(off):
                def f(tok=None):
                    mean, inv = _row_stats(xv[off:off + 8, :].astype(f32), tok)
                    sv[off:off + 8, 0:128] = mean
                    sv[off:off + 8, 128:256] = inv
                return f
            return [chunk(off) for off in range(0, xv.shape[0], 8)]

        def ln1_scaled(x, stat, cs, tok=None):
            w = x.shape[1]
            mean = stat[:, 0:128] if tok is None else stat[:, 0:128] + _rep(tok, x.shape[0])
            n = (x.astype(f32) - _wide(mean, w)) * _wide(stat[:, 128:256], w)
            return n * _rep(mod0[1, :, cs], x.shape[0])

        def qproj(h, wv, rec=None):
            q = None
            for c in range(D // W):
                cs = slice(c * W, (c + 1) * W)
                part = jnp.dot(pltpu.bitcast(h_buf[:, cs], bf16), wv[cs, :],
                               preferred_element_type=f32)
                q = part if q is None else q + part
                if rec is not None:
                    rec.done(part)
            q_ring[h & 3] = pltpu.bitcast((q * qscale).astype(bf16), u32)

        def q_early(g, q):
            return ((q + _rep(bq_buf[:, g * DH:(g + 1) * DH], q.shape[0])) * qscale).astype(bf16)

        def scores(h, q, sv, mv, rec=None, reload=False):
            mp = None
            for c in range(SK // W):
                cs = slice(c * W, (c + 1) * W)
                s = lax.dot_general(q, kb[h & 3, cs, :], _NT, preferred_element_type=f32)
                sv[:, cs] = s
                if rec is not None:
                    rec.done(s)
                if not reload:
                    mp = _fold(jnp.maximum, ([] if mp is None else [mp]) + _tiles(s))
            if reload:
                mp = _fold(jnp.maximum, _tiles(sv[...]))
            mv[...] = jnp.broadcast_to(jnp.max(mp, axis=-1, keepdims=True), mp.shape)

        def pv(h, sv, mv, rec=None, late=False):
            o = lp = None
            for c in range(SK // W):
                cs = slice(c * W, (c + 1) * W)
                p = jnp.exp2(sv[:, cs] - _wide(mv[...], W))
                lp = _fold(jnp.add, ([] if lp is None else [lp]) + _tiles(p))
                d = jnp.dot(p.astype(bf16), vb[h & 3, cs, :], preferred_element_type=f32)
                o = d if o is None else o + d
                if rec is not None:
                    rec.done(d)
            if late:
                lp = lp + _zero_of(o)
            l = jnp.sum(lp, axis=-1, keepdims=True)
            r = pl.reciprocal(l, approx=True)
            r = r * (2.0 - l * r)
            return (o * r).astype(bf16)

        def oproj(hos, av, xv=None, rec=None):
            for c in range(D // W):
                cs = slice(c * W, (c + 1) * W)
                a = av[:, cs]
                for h, o in hos:
                    if not isinstance(h, int):
                        a = jnp.where(h > 0, a, 0.0)
                    d = jnp.dot(o, wo2[h & 3, 0, :, cs], preferred_element_type=f32)
                    if rec is not None:
                        rec.done(d)
                    a = a + d
                if xv is not None:
                    a = xv[:, cs].astype(f32) + _rep(modv[0, :, cs], a.shape[0]) * a
                av[:, cs] = a

        def matvec(wv, tok=None, step=16):
            n = wv.shape[1]
            part = None if tok is None else _wide(tok, n)
            for r in range(0, D, step):
                t = wv[r:r + step, :].astype(f32) * _wide(cb_buf[r:r + step, :], n)
                for e in range(step // 8):
                    te = t[e * 8:(e + 1) * 8, :]
                    part = te if part is None else part + te
            return _rb(jnp.sum(part, axis=0, keepdims=True))

        def mod_piece(p, tok=None):
            extra = isinstance(p, int) and p > NB
            modr[p] = matvec(wmx.at[p - NB - 1] if extra else w4.at[p & 1, 1], tok)

        def finish_mod():
            n = D // MC
            ga, sb, cb, gb = (jnp.concatenate([modr[i * n + t] for t in range(n)], axis=-1)
                              for i in range(4))
            cb1 = _rb(1.0 + cb)
            wr = wr_buf[...].astype(f32).reshape(1, D)
            a = cb1 * wr
            a0 = jnp.broadcast_to(jnp.sum(a, axis=-1, keepdims=True), (1, D))
            b0 = jnp.broadcast_to(jnp.sum(sb * wr, axis=-1, keepdims=True), (1, D))
            for i, v in enumerate((ga, sb, cb1, gb, a, gb * cb1, gb * sb, a0, b0)):
                modv[i] = jnp.broadcast_to(v, (8, D))

        def out_rows(x1, mean, inv):
            return (x1 + ((x1 - _wide(mean, D)) * (_wide(inv, D) * modv[5]) + modv[6])).astype(bf16)

        def out_chunks(j):
            x1v, sv, ov = view(acc, j, TL), view(st2_buf, j, TL), view(o_buf, j, TL)

            def chunk(off):
                def f(tok):
                    rs = slice(off, off + 8)
                    ov[rs, :] = out_rows(x1v[rs, :], sv[rs, 0:128] + tok, sv[rs, 128:256] + tok)
                return f
            return [chunk(off) for off in range(0, TL, 8)]

        def epi_chunks(j, x1v, ov, with_out=True):
            sub = lax.broadcasted_iota(i32, (8, 128), 0)
            low = (0xFFFF - j * TL) - sub
            sv = view(st2_buf, j, TL)
            st = {}

            def chunk(off):
                def f(tok=None):
                    if off == 0:
                        st["k1"], st["k2"] = key_buf[0], key_buf[1]
                    x1 = x1v[off:off + 8, :]
                    mean, inv = _row_stats(x1, tok)
                    sv[off:off + 8, 0:128] = mean
                    sv[off:off + 8, 128:256] = inv
                    xa = _tiles(x1 * modv[4])
                    if tok is not None:
                        xa[0] = xa[0] + tok
                    ra = _lane_sum(_fold(jnp.add, xa))
                    r = inv * (ra - mean * modv[7, :, 0:128]) + modv[8, :, 0:128]
                    if with_out:
                        ov[off:off + 8, :] = out_rows(x1, mean, inv)
                    bits = pltpu.bitcast(_rb(r) + 0.0, i32)
                    key = jnp.where(bits < 0, bits ^ 0x7FFF0000, bits) | (low - off)
                    st["k2"] = jnp.maximum(st["k2"], jnp.minimum(st["k1"], key))
                    st["k1"] = jnp.maximum(st["k1"], key)
                    if off + 8 == TL:
                        key_buf[0], key_buf[1] = st["k1"], st["k2"]
                return f
            return [chunk(off) for off in range(0, TL, 8)]

        cp_c().start()
        cp_x(0).start()
        for c in range(2):
            cp_wq0(c).start()
            for i in range(n_mch):
                cp_ca(c, i).start()
            if c == 0:
                for j in range(1, J0):
                    cp_x(j).start()
        cp_sa().start()
        for h in range(G - 1):
            cp_k(h, sem_first.at[1 + h]).start()
        early = []
        for h in range(2):
            early += [cp_v(h, sem_first.at[8 + 2 * h]), cp_wo(h, sem_first.at[9 + 2 * h])]
        for cp in early:
            cp.start()
        start_head(0)

        cp_c().wait()
        cf = c_buf[...].astype(f32)
        sc = _rb(cf * jax.nn.sigmoid(cf))
        for t in range(4):
            sc_buf[t] = sc[:, t * (D // 4):(t + 1) * (D // 4)]

        def cb_body(t, carry):
            view(cb_buf, t, D // 4)[...] = jnp.transpose(jnp.broadcast_to(sc_buf[t], (128, D // 4)))
            return carry
        lax.fori_loop(0, 4, cb_body, 0)
        key_buf[...] = jnp.full(key_buf.shape, _IMIN, i32)
        cp_x(0).wait()

        def st0_body(i, carry):
            for ch in ln1_chunks(view(x_buf, i, T0 // 4), view(st_buf, i, T0 // 4)):
                ch()
            return carry
        lax.fori_loop(0, 4, st0_body, 0)

        def ca_half(c, stream):
            cp_wq0(c).wait()
            if not stream:
                for i in range(n_mch):
                    cp_ca(c, i).wait()
            part = None
            for i in range(n_mch):
                if stream:
                    cp_ca(c, i).wait()
                scb = jnp.broadcast_to(sc[:, i * MCH:(i + 1) * MCH], (16, MCH)).astype(bf16)
                d = jnp.dot(scb, wca[c, i * MCH:(i + 1) * MCH, :], preferred_element_type=f32)
                part = d if part is None else part + d
            mod0[1, :, c * W:(c + 1) * W] = _rb(1.0 + _rb(part[0:8, :]))

        def q_first(r0, t, c, rec, mid=None):
            rows = pl.ds(r0, t)
            cs = slice(c * W, (c + 1) * W)
            hh = ln1_scaled(x_buf[rows, cs], st_buf[rows, :], cs).astype(bf16)
            for g in range(G):
                if mid is not None and g == mid[0]:
                    mid[1]()
                part = jnp.dot(hh, wq0[cs, g * DH:(g + 1) * DH], preferred_element_type=f32)
                qf_buf[g, rows, :] = part if c == 0 else qf_buf[g, rows, :] + part
                if rec is not None:
                    rec.done(part)

        ca_half(0, True)

        def pa_body(j, carry):
            @pl.when(j + 1 < J0)
            def _():
                cp_x(j + 1).wait()
            jn = jnp.minimum(j + 1, J0 - 1)
            rec = _Pace(ln1_chunks(view(x_buf, jn, T0), view(st_buf, jn, T0)), cfg["LCA"])
            q_first(_mul(j, T0), T0, 0, rec)
            return carry
        lax.fori_loop(0, J0, pa_body, 0)

        TB, RB = cfg["TB"], cfg["RB"]
        ca_half(1, False)
        q_first(0, TB, 1, None)
        cp_sa().wait()
        cp_k(0, sem_first.at[1]).wait()
        cp_wr().start()
        for p in range(NB + 1, H):
            cp_wmx(p).start()

        def sa_chunk(t):
            def f(tok):
                cs = slice(t * 256, (t + 1) * 256)
                mod0[0, :, cs] = jnp.broadcast_to(matvec(wsa.at[:, cs], tok, 8), (8, 256))
            return f

        def sa_bias():
            bq_buf[...] = jnp.dot(_rep(mod0[0], 16).astype(bf16), wq0[...],
                                  preferred_element_type=f32)[0:8, :]

        def h_chunk(off):
            def f(tok):
                rs, rh = slice(off, off + RB), slice(off // 2, (off + RB) // 2)
                hh = (ln1_scaled(x_buf[rs, :], st_buf[rs, :], slice(0, D), tok)
                      + _rep(mod0[0], RB)).astype(bf16)
                h_buf[rh, :] = pltpu.bitcast(hh, u32)
            return f

        def q_chunk(off):
            def f(tok):
                n = 2 * RB
                rs, rh = slice(off, off + n), slice(off // 2, (off + n) // 2)
                for g in range(1, G):
                    q_ring[g, rh, :] = pltpu.bitcast(
                        q_early(g, qf_buf[g, rs, :] + _rep(tok, n)), u32)
            return f

        hs = [h_chunk(off) for off in range(0, S, RB)]
        qs = [q_chunk(off) for off in range(0, S, 2 * RB)]
        nh = cfg["NHB"]
        rest_chunks = []
        nq, nr = len(qs), len(hs) - nh
        for i, ch in enumerate(hs[nh:]):
            rest_chunks.append(ch)
            while qs and (nq - len(qs)) * nr < (i + 1) * nq:
                rest_chunks.append(qs.pop(0))
        assert not qs
        rec = _Pace([sa_chunk(t) for t in range(D // 256)] + hs[:nh], cfg["LCB2"])
        q_first(TB, S - TB, 1, rec, mid=(cfg["BQ"], sa_bias))
        n4 = len(rest_chunks)
        n3 = n4 - cfg["NL4"]
        cnt = [n3 // 3 + (1 if i < n3 % 3 else 0) for i in range(3)] + [cfg["NL4"]]
        scores(0, q_early(0, qf_buf[0]), s_buf, m_buf, rec=_Pace(rest_chunks, cnt), reload=True)

        def main_body(h, carry):
            rec = _Pace(pack_chunks(h) + [lambda tok: mod_piece(h, tok)], cfg["LCM"])
            qproj(h + G, w4.at[h & 1, 0], rec=rec)
            start_head(h + 1)
            o = pv(h, s_buf, m_buf)
            scores(h + 1, pltpu.bitcast(q_ring[(h + 1) & 3], bf16), s_buf, m_buf, rec=rec)
            oproj([(h, o)], acc)
            wait_head(h + 1)
            return carry
        for h in range(1, G - 1):
            cp_k(h, sem_first.at[1 + h]).wait()
        for cp in early:
            cp.wait()
        wait_head(0)
        lax.fori_loop(0, NB, main_body, 0)

        ha = NB
        rest = list(zip(range(NB + 1, H), (s2_buf, s3_buf, s4_buf), (m2_buf, m3_buf, m4_buf)))
        late = []
        for n, h in enumerate(range(NB + 3, H)):
            late += [cp_v(h, sem_first.at[8 + 2 * n]), cp_wo(h, sem_first.at[9 + 2 * n])]
        for cp in late:
            cp.start()
        cp_wr().wait()
        for p in range(NB + 1, H):
            cp_wmx(p).wait()

        def l_step(j, do_x, do_y):
            if do_x and do_y:
                aw = view(acc, j - 1, TL, 2)
                ay, ax = aw.at[0:TL, :], aw.at[TL:2 * TL, :]
            elif do_x:
                ax = view(acc, j, TL)
            else:
                ay = view(acc, j - 1, TL)
            rec = None
            if do_y:
                chunks = epi_chunks(j - 1, ay, view(o_buf, j - 1, TL), with_out=do_x)
                os_ = [(h, pv(h, sv, mv, late=not do_x)) for h, sv, mv in rest]
            if do_x:
                oa = pv(ha, view(s_buf, j, TL), view(m_buf, j, TL))
            if do_y and do_x:
                oproj(os_, ay, view(x_buf, j - 1, TL))
            elif do_y:
                xv = view(x_buf, j - 1, TL)
                r0, prev = 0, []
                for n in cfg["LSPLIT"]:
                    rs = slice(r0, r0 + n)
                    nr = len(os_) * (D // W)
                    cnt = [len(prev) // nr + (1 if i < len(prev) % nr else 0) for i in range(nr)]
                    rec = _Pace(prev, cnt)
                    oproj([(h, o[rs]) for h, o in os_], ay.at[rs, :], xv.at[rs, :], rec=rec)
                    prev = chunks[r0 // 8:(r0 + n) // 8]
                    r0 += n
                chunks = prev
            if do_x:
                if do_y:
                    rec = _Pace(chunks, cfg["LCNT"])
                for h, sv, mv in rest:
                    q = pltpu.bitcast(view(q_ring.at[h & 3], j, TL // 2)[...], bf16)
                    scores(h, q, sv, mv, rec=rec, reload=True)
                oproj([(ha, oa)], ax, rec=rec)
            if do_y:
                if do_x:
                    cp_out(j - 1).start()
                else:
                    for ch in chunks:
                        ch()

        for p in range(NB, H):
            mod_piece(p)
        finish_mod()
        l_step(0, True, False)
        for cp in late:
            cp.wait()

        def pl_body(j, carry):
            l_step(j, True, True)
            return carry
        lax.fori_loop(1, JL, pl_body, 0)
        l_step(JL, False, True)

        k1, k2 = key_buf[0], key_buf[1]
        for sh in (4, 2, 1):
            o1, o2 = pltpu.roll(k1, sh, 0), pltpu.roll(k2, sh, 0)
            k2 = jnp.maximum(jnp.minimum(k1, o1), jnp.maximum(k2, o2))
            k1 = jnp.maximum(k1, o1)

        def score_of(k):
            hi = k & jnp.int32(-65536)
            return pltpu.bitcast(jnp.where(hi < 0, hi ^ 0x7FFF0000, hi), f32)

        i1s = jnp.minimum(0xFFFF - (k1[0, 0] & 0xFFFF), S - 1)
        i2s = jnp.minimum(0xFFFF - (k2[0, 0] & 0xFFFF), S - 1)

        sub = lax.broadcasted_iota(i32, (16, D), 0)
        sb, cb1, gb = (_rep(modv[i], 16) for i in (1, 2, 3))

        def adaln2(x1, stat):
            return (x1 - _wide(stat[:, 0:128], D)) * _wide(stat[:, 128:256], D) * cb1 + sb

        def pick(ref):
            sel = lax.broadcasted_iota(i32, (16, ref.shape[1]), 0) == 0
            return jnp.where(sel, ref[pl.ds(i1s, 1), :], ref[pl.ds(i2s, 1), :])

        xs = adaln2(pick(acc), pick(st2_buf)).astype(bf16)
        FC, lag = cfg["FC"], cfg["FLAG"]
        kvs = [int(ch) for ch in cfg["LKV"]]
        fout = [int(ch, 36) for ch in cfg["LFO"]]
        KV = max(kvs)

        def wrows(ref, a, b, c):
            n = FC // 128
            u = [ref[c * n + t, a // 2:b // 2, :] for t in range(n)]
            return pltpu.bitcast(u[0] if n == 1 else jnp.concatenate(u, axis=1), bf16)

        DV = D - KV * 128
        if KV:
            xf = xs.astype(f32)
            for r in range(2):
                xc_buf[r] = jnp.transpose(jnp.broadcast_to(xf[r:r + 1, DV:], (128, D - DV)))
        subc = lax.broadcasted_iota(i32, (8, FC), 0)
        y = None
        act = []
        outs = out_chunks(JL - 1)
        for c in range(F // FC + lag):
            if c < F // FC:
                dm = D - kvs[c] * 128
                gu = [jnp.dot(xs[:, :dm], wrows(w, 0, dm, c), preferred_element_type=f32)[0:8, :]
                      for w in (wg, wu)]
                for v in gu:
                    for t in range(fout[c] if c < len(fout) else 0):
                        if outs:
                            outs.pop(0)(_zero_of(v[0:8, (t % 2) * 128:(t % 2 + 1) * 128]))
                            if not outs:
                                cp_out(JL - 1).start()
                if dm < D:
                    part = [[None, None], [None, None]]
                    for k in range(dm, D, 16):
                        xcol = [_wide(xc_buf[r, k - DV:k - DV + 16, :], FC) for r in range(2)]
                        for m, w in enumerate((wg, wu)):
                            wv = wrows(w, k, k + 16, c).astype(f32)
                            for r in range(2):
                                t = wv * xcol[r]
                                for e in range(2):
                                    te = t[e * 8:(e + 1) * 8, :]
                                    part[m][r] = te if part[m][r] is None else part[m][r] + te
                    for m in range(2):
                        ra, rb_ = (jnp.sum(v, axis=0, keepdims=True) for v in part[m])
                        gu[m] = gu[m] + jnp.where(subc == 0, ra, rb_)
                g, u = _rb(gu[0]), _rb(gu[1])
                act.append(_rep(_rb(g * jax.nn.sigmoid(g)) * u, 16).astype(bf16))
            if c >= lag:
                wdc = pltpu.bitcast(wd[(c - lag) * FC // 2:(c - lag + 1) * FC // 2, :], bf16)
                d = jnp.dot(act[c - lag], wdc, preferred_element_type=f32)[0:8, :]
                y = d if y is None else y + d
        y = _rb(y)
        ya = _rb(y[0:1, :] * _wide(_rb(jax.nn.sigmoid(score_of(k1[0:1, :]))), D))
        yb = _rb(y[1:2, :] * _wide(_rb(jax.nn.sigmoid(score_of(k2[0:1, :]))), D))

        g1 = pl.multiple_of((i1s >> 4) << 4, 16)
        g2 = pl.multiple_of((i2s >> 4) << 4, 16)
        for t, g0 in enumerate((g1, g2)):
            rid = sub + g0
            x1 = acc[pl.ds(g0, 16), :]
            upd = jnp.where(rid == i1s, ya, 0.0) + jnp.where(rid == i2s, yb, 0.0)
            fix[t] = (x1 + gb * (adaln2(x1, st2_buf[pl.ds(g0, 16), :]) + upd)).astype(bf16)

        pltpu.make_async_copy(o_buf, out_hbm, sem_out.at[0]).wait()

        def cp_fix(t, g0):
            return pltpu.make_async_copy(fix.at[t], out_hbm.at[pl.ds(g0, 16), :], sem_fix.at[t])

        cp_fix(0, g1).start()

        @pl.when(g2 != g1)
        def _():
            cp_fix(1, g2).start()
            cp_fix(1, g2).wait()
        cp_fix(0, g1).wait()

    return kernel


_CFG = dict(
    G=4, T0=256, TB=1024, TL=256, MCH=256, RB=16, FC=256,
    LCA='cc80', LCB2='040g', NHB=16, NL4=8, BQ=3, LCNT='33333333332000',
    PKN=8, LCM='008890',
    LSPLIT=(96, 96, 64), FLAG=1, LKV='00233333333333', LFO='88',
)


def _build(A_x, A_k_cache, A_v_cache, A_wq, A_wo, B_w_r, B_w_gate, B_w_up, B_w_down, c, w_mod,
           **over):
    B, S, D = A_x.shape
    _, H, SK, DH = A_k_cache.shape
    F = B_w_gate.shape[1]
    assert B == 1
    cfg = dict(_CFG, **over)
    T0, TL, G = cfg["T0"], cfg["TL"], cfg["G"]
    MC = (4 * D) // H
    kernel = _make_kernel(S, D, H, DH, SK, F, cfg)
    scratch = [
        pltpu.VMEM((S, D), bf16),
        pltpu.VMEM((S // 2, D), u32),
        pltpu.VMEM((S, D), f32),
        pltpu.VMEM((S, SK), f32),
        pltpu.VMEM((S, 128), f32),
        pltpu.VMEM((TL, SK), f32),
        pltpu.VMEM((TL, 128), f32),
        pltpu.VMEM((TL, SK), f32),
        pltpu.VMEM((TL, 128), f32),
        pltpu.VMEM((TL, SK), f32),
        pltpu.VMEM((TL, 128), f32),
        pltpu.VMEM((S, 256), f32),
        pltpu.VMEM((S, 256), f32),
        pltpu.VMEM((4, S // 2, DH), u32),
        pltpu.VMEM((G, S, DH), f32),
        pltpu.VMEM((8, G * DH), f32),
        pltpu.VMEM((4, SK, DH), bf16),
        pltpu.VMEM((4, SK, DH), bf16),
        pltpu.VMEM((D, G * DH), bf16),
        pltpu.VMEM((2, 4, D, 128), bf16),
        pltpu.VMEM((4, 2, DH, D), bf16),
        pltpu.VMEM((G - 1, D, MC), bf16),
        pltpu.VMEM((2, D, D // 2), bf16),
        pltpu.VMEM((D, D), bf16),
        pltpu.VMEM((1, D), bf16),
        pltpu.VMEM((D,), bf16),
        pltpu.VMEM((4, 1, D // 4), f32),
        pltpu.VMEM((D, 128), f32),
        pltpu.VMEM((2, 8, D), f32),
        pltpu.VMEM((H, 1, MC), f32),
        pltpu.VMEM((9, 8, D), f32),
        pltpu.VMEM((F // 128, D // 2, 128), u32),
        pltpu.VMEM((F // 128, D // 2, 128), u32),
        pltpu.VMEM((F // 2, D), u32),
        pltpu.VMEM((2, max(int(max(cfg["LKV"])), 1) * 128, 128), f32),
        pltpu.VMEM((S, D), bf16),
        pltpu.VMEM((2, 8, 128), i32),
        pltpu.VMEM((2, 16, D), bf16),
        pltpu.SemaphoreType.DMA((sum(_sem_sizes(S, D, cfg)),)),
    ]
    any_spec = pl.BlockSpec(memory_space=pl.ANY)
    out = pl.pallas_call(
        kernel,
        out_shape=jax.ShapeDtypeStruct((S, D), bf16),
        in_specs=[any_spec] * 11,
        out_specs=any_spec,
        scratch_shapes=scratch,
        compiler_params=pltpu.CompilerParams(vmem_limit_bytes=112 * 1024 * 1024,
                                             disable_bounds_checks=True,
                                             disable_semaphore_checks=True),
    )(A_x.reshape(S, D), A_k_cache.reshape(H, SK, DH), A_v_cache.reshape(H, SK, DH),
      A_wq, A_wo, B_w_r, B_w_gate, B_w_up, B_w_down, c, w_mod)
    return out.reshape(B, S, D)


@jax.jit
def pallas_adaLN_cond__mha_block_cached__moe_arch_mod__prompt_kernel(
    A_x: jax.Array,
    A_k_cache: jax.Array,
    A_v_cache: jax.Array,
    A_wq: jax.Array,
    A_wo: jax.Array,
    B_x: jax.Array,
    B_w_r: jax.Array,
    B_w_gate: jax.Array,
    B_w_up: jax.Array,
    B_w_down: jax.Array,
    c: jax.Array,
    w_mod: jax.Array,
):
    del B_x
    return _build(A_x, A_k_cache, A_v_cache, A_wq, A_wo, B_w_r, B_w_gate, B_w_up, B_w_down,
                  c, w_mod)
```

```python
import jax
import jax.numpy as jnp
from jax import lax
import jax.experimental.pallas as pl
import jax.experimental.pallas.tpu as pltpu

f32 = jnp.float32
bf16 = jnp.bfloat16
u32 = jnp.uint32
i32 = jnp.int32

_NT = (((1,), (1,)), ((), ()))
_LOG2E = 1.4426950408889634
_EPS = 1e-5
_IMIN = -2 ** 31


def _rb(v):
    return v.astype(bf16).astype(f32)


def _rep(v, n):
    return v if n == 8 else jnp.tile(v, (n // 8, 1))


def _wide(v, w):
    return jnp.tile(v, (1, w // 128))


def _zero_of(v):
    bits = pltpu.bitcast(v, u32)
    return pltpu.bitcast(lax.shift_right_logical(lax.shift_right_logical(bits, jnp.uint32(31)),
                                                 jnp.uint32(1)), f32)


def _gate(lhs, dep, row):
    u = pltpu.bitcast(lhs, u32)
    r = row // 16 * 8
    parts = [u[0:r]] if r else []
    parts.append(u[r:r + 8] | pltpu.bitcast(_zero_of(dep), u32))
    if r + 8 < u.shape[0]:
        parts.append(u[r + 8:])
    return pltpu.bitcast(jnp.concatenate(parts, axis=0), bf16)


class _Pace:
    def __init__(self, chunks, counts):
        self.chunks = list(chunks)
        self.counts = [ch if isinstance(ch, int) else int(ch, 36) for ch in counts]
        assert sum(self.counts) == len(self.chunks), (counts, len(self.chunks))

    def done(self, res):
        n = self.counts.pop(0)
        for i in range(n):
            r0 = (i * res.shape[0] // n) // 8 * 8
            self.chunks.pop(0)(_zero_of(res[r0:r0 + 8, 0:128]))


def _mix(*plans):
    plans = [(list(ch), [c if isinstance(c, int) else int(c, 36) for c in cnt]) for ch, cnt in plans]
    for ch, cnt in plans:
        assert sum(cnt) == len(ch), (cnt, len(ch))
    fill, total = [], []
    for r in range(len(plans[0][1])):
        slots = sorted((i / cnt[r], k) for k, (_, cnt) in enumerate(plans)
                       for i in range(cnt[r]))
        fill += [plans[k][0].pop(0) for _, k in slots]
        total.append(len(slots))
    return _Pace(fill, total)


def _tiles(v):
    return [v[:, c * 128:(c + 1) * 128] for c in range(v.shape[1] // 128)]


def _fold(op, parts):
    out = parts[0]
    for p in parts[1:]:
        out = op(out, p)
    return out


def _lane_sum(v):
    return jnp.broadcast_to(jnp.sum(v, axis=-1, keepdims=True), v.shape)


def _row_stats(xf, tok=None):
    d = xf.shape[-1]
    ts = _tiles(xf)
    nt = len(ts)
    if tok is not None:
        ts = [ts[0] + tok] + ts[1:]
    mu = _fold(jnp.add, ts) * (1.0 / nt)
    m2 = _fold(jnp.add, [(t - mu) * (t - mu) for t in ts])
    mean = _lane_sum(mu) * (1.0 / 128)
    dm = mu - mean
    var = _lane_sum(m2 + (dm * dm) * float(nt)) * (1.0 / d)
    return mean, lax.rsqrt(var + _EPS)


def _sem_sizes(S, D, cfg):
    j0 = S // cfg["T0"]
    return [2, 2 * (D // cfg["MCH"]), j0, 1, 16, 4, 1, 2]


def _make_kernel(S, D, H, DH, SK, F, cfg):
    T0, TL, MCH = cfg["T0"], cfg["TL"], cfg["MCH"]
    J0 = S // T0
    JL = S // TL
    qscale = DH ** -0.5 * _LOG2E
    n_mch = D // MCH
    G = cfg["G"]
    NB = H - G
    MC = (4 * D) // H
    W = 512
    NF = F // 128
    assert 2 <= G <= 4 and D == 2 * W and MC == DH == 128 and NF <= NB

    def kernel(x_hbm, k_hbm, v_hbm, wq_hbm, wo_hbm, wr_hbm, wg_hbm, wu_hbm, wd_hbm,
               c_hbm, wmod_hbm, out_hbm,
               x_buf, h_buf, acc, s_buf, m_buf, s2_buf, m2_buf, s3_buf, m3_buf, s4_buf, m4_buf,
               st_buf, st2_buf,
               q_ring, qf_buf, bq_buf,
               kb, vb, wq0, w4, wo2, wmx, wca, wsa, c_buf, wr_buf, sc_buf, cb_buf, mod0, modr, modv,
               wg, wu, wd, xc_buf, ov_buf, obx, wof, o_buf, key_buf, fix,
               sems):

        class _Sem:
            def __init__(self, base):
                self.base = base
                self.at = self

            def __getitem__(self, i):
                return sems.at[self.base + i]

        sizes = _sem_sizes(S, D, cfg)
        offs = [sum(sizes[:i]) for i in range(len(sizes))]
        (sem_small, sem_ca, sem_x, sem_sa, sem_first, sem_head,
         sem_out, sem_fix) = (_Sem(o) for o in offs)

        def _mul(a, n):
            v = a * n
            return v if isinstance(a, int) else pl.multiple_of(v, n)

        def view(ref, j, t, n=1):
            return ref.at[pl.ds(_mul(j, t), n * t), :]

        def cp_c():
            return pltpu.make_async_copy(c_hbm, c_buf, sem_small.at[0])

        def cp_wr():
            return pltpu.make_async_copy(wr_hbm, wr_buf, sem_small.at[1])

        def cp_ca(c, i):
            return pltpu.make_async_copy(
                wmod_hbm.at[pl.ds(i * MCH, MCH), pl.ds(D + c * W, W)], view(wca.at[c], i, MCH),
                sem_ca.at[c * n_mch + i])

        def cp_sa():
            return pltpu.make_async_copy(wmod_hbm.at[:, pl.ds(0, D)], wsa, sem_sa.at[0])

        def cp_x(j):
            return pltpu.make_async_copy(view(x_hbm, j, T0), view(x_buf, j, T0), sem_x.at[j])

        def cp_wq0(c):
            return pltpu.make_async_copy(wq_hbm.at[pl.ds(c * W, W), pl.ds(0, G * DH)],
                                         view(wq0, c, W), sem_first.at[14 + c])

        def cp_k(h, sem=None):
            return pltpu.make_async_copy(k_hbm.at[h], kb.at[h & 3],
                                         sem_head.at[0] if sem is None else sem)

        def cp_v(h, sem=None):
            return pltpu.make_async_copy(v_hbm.at[h], vb.at[h & 3],
                                         sem_head.at[1] if sem is None else sem)

        def cp_wo(h, sem=None):
            return pltpu.make_async_copy(view(wo_hbm, h, DH), wo2.at[h & 3, 0],
                                         sem_head.at[2] if sem is None else sem)

        def _clamp(a, hi):
            return min(a, hi) if isinstance(a, int) else jnp.minimum(a, hi)

        def cols(ref, t):
            return ref.at[:, pl.ds(_mul(t, 128), 128)]

        def cp_wmx(p):
            return pltpu.make_async_copy(cols(wmod_hbm, p + (2 * D) // MC), wmx.at[p - NB - 1],
                                         sem_first.at[4 + p - NB])

        def start_head(h):
            f = _clamp(h, NF - 1)
            for i, src in enumerate((cols(wq_hbm, _clamp(h + G, H - 1)),
                                     cols(wmod_hbm, h + (2 * D) // MC),
                                     cols(wg_hbm, f), cols(wu_hbm, f))):
                pltpu.make_async_copy(src, w4.at[h & 1, i], sem_head.at[3]).start()
            cp_k(h + G - 1).start()
            cp_wo(h + 2).start()
            pltpu.make_async_copy(view(wd_hbm, f, 128), wo2.at[(h + 2) & 3, 1],
                                  sem_head.at[2]).start()
            cp_v(h + 2).start()

        def wait_head(h):
            pltpu.make_async_copy(w4.at[h & 1], w4.at[h & 1], sem_head.at[3]).wait()
            cp_k(h + G - 1).wait()
            pltpu.make_async_copy(wo2.at[(h + 2) & 3], wo2.at[(h + 2) & 3], sem_head.at[2]).wait()
            cp_v(h + 2).wait()

        def pack_chunks(h):
            f = _clamp(h, NF - 1)
            out = []
            for sv, dv in ((w4.at[h & 1, 2], wg.at[f]), (w4.at[h & 1, 3], wu.at[f]),
                           (wo2.at[(h + 2) & 3, 1], view(wd, f, 64))):
                n, w = sv.shape
                step = n // cfg['PKN']

                def chunk(r, sv=sv, dv=dv, step=step, w=w):
                    def fn(tok):
                        z = _rep(_wide(pltpu.bitcast(tok, u32), w), step // 2)
                        dv[r // 2:(r + step) // 2, :] = pltpu.bitcast(sv[r:r + step, :], u32) | z
                    return fn
                out += [chunk(r) for r in range(0, n, step)]
            return out

        def cp_out(j):
            return pltpu.make_async_copy(view(o_buf, j, TL), view(out_hbm, j, TL), sem_out.at[0])

        def ln1_chunks(xv, sv):
            def chunk(off):
                def f(tok=None):
                    mean, inv = _row_stats(xv[off:off + 8, :].astype(f32), tok)
                    sv[off:off + 8, 0:128] = mean
                    sv[off:off + 8, 128:256] = inv
                return f
            return [chunk(off) for off in range(0, xv.shape[0], 8)]

        def ln1_scaled(x, stat, cs, tok=None):
            w = x.shape[1]
            mean = stat[:, 0:128] if tok is None else stat[:, 0:128] + _rep(tok, x.shape[0])
            n = (x.astype(f32) - _wide(mean, w)) * _wide(stat[:, 128:256], w)
            return n * _rep(mod0[1, :, cs], x.shape[0])

        def qproj(h, wv, rec=None):
            q = None
            for c in range(D // W):
                cs = slice(c * W, (c + 1) * W)
                part = jnp.dot(pltpu.bitcast(h_buf[:, cs], bf16), wv[cs, :],
                               preferred_element_type=f32)
                q = part if q is None else q + part
                if rec is not None:
                    rec.done(part)
            q_ring[h & 3] = pltpu.bitcast((q * qscale).astype(bf16), u32)

        def q_early(g, q):
            return ((q + _rep(bq_buf[:, g * DH:(g + 1) * DH], q.shape[0])) * qscale).astype(bf16)

        def scores(h, q, sv, mv, rec=None, reload=False, gate=None):
            mp = None
            for c in range(SK // W):
                cs = slice(c * W, (c + 1) * W)
                qq = _gate(q, gate[2][-1], gate[1]) if (gate and gate[0] == c) else q
                s = lax.dot_general(qq, kb[h & 3, cs, :], _NT, preferred_element_type=f32)
                sv[:, cs] = s
                if rec is not None:
                    rec.done(s)
                if not reload:
                    mp = _fold(jnp.maximum, ([] if mp is None else [mp]) + _tiles(s))
            if reload:
                mp = _fold(jnp.maximum, _tiles(sv[...]))
            mv[...] = jnp.broadcast_to(jnp.max(mp, axis=-1, keepdims=True), mp.shape)

        def pv(h, sv, mv, rec=None, late=False):
            o = lp = None
            for c in range(SK // W):
                cs = slice(c * W, (c + 1) * W)
                m = mv[...]
                if c >= cfg["LD"] and sv.shape[0] == S:
                    m = m + _zero_of(lp)
                p = jnp.exp2(sv[:, cs] - _wide(m, W))
                lp = _fold(jnp.add, ([] if lp is None else [lp]) + _tiles(p))
                d = jnp.dot(p.astype(bf16), vb[h & 3, cs, :], preferred_element_type=f32)
                o = d if o is None else o + d
                if rec is not None:
                    rec.done(d)
            if late:
                lp = lp + _zero_of(o)
            l = jnp.sum(lp, axis=-1, keepdims=True)
            r = pl.reciprocal(l, approx=True)
            r = r * (2.0 - l * r)
            return (o * r).astype(bf16)

        def oproj(hos, av, xv=None, rec=None):
            for c in range(D // W):
                cs = slice(c * W, (c + 1) * W)
                a = av[:, cs]
                for h, o in hos:
                    if not isinstance(h, int):
                        a = jnp.where(h > 0, a, 0.0)
                    d = jnp.dot(o, wo2[h & 3, 0, :, cs], preferred_element_type=f32)
                    if rec is not None:
                        rec.done(d)
                    a = a + d
                if xv is not None:
                    a = xv[:, cs].astype(f32) + _rep(modv[0, :, cs], a.shape[0]) * a
                av[:, cs] = a

        RV = cfg["RV"]

        def expand_chunks(h):
            def wchunk(r):
                def f(tok):
                    wof[r:r + 8, :] = wo2[h & 3, 0, r:r + 8, :].astype(f32) + _wide(tok, D)
                return f

            def wchunk2(r, c0):
                def f(tok):
                    cs = slice(c0, c0 + 256)
                    w = wo2[h & 3, 0, r:r + 8, cs].astype(f32) + _wide(tok, 256)
                    for e in range(8):
                        wof[(r + e) * 8:(r + e + 1) * 8, cs] = jnp.broadcast_to(w[e:e + 1, :], (8, 256))
                return f

            lane = lax.broadcasted_iota(i32, (8, 128), 1)

            def ochunk(g, e0):
                def f(tok):
                    o = ov_buf[g * 8:(g + 1) * 8, :] + tok
                    for e in range(e0, e0 + 32):
                        obx[g, e] = _lane_sum(jnp.where(lane == e, o, 0.0))
                return f
            och = [ochunk(g, e0) for g in range(RV // 8) for e0 in range(0, DH, 32)]
            if cfg["WX"]:
                return [wchunk2(r, c0) for r in range(0, DH, 8) for c0 in range(0, D, 256)], och
            return [wchunk(r) for r in range(0, DH, 8)], och

        def vproj(r0, r1, done, wrow):
            def f(tok):
                if not wrow and cfg["WX"]:
                    wrow.extend(wof[e * 8:(e + 1) * 8, :] for e in range(DH))
                if not wrow:
                    wrow.extend(jnp.concatenate(
                        [jnp.broadcast_to(wof[e:e + 1, t * 128:(t + 1) * 128], (8, 128))
                         for t in range(D // 128)], axis=1) for e in range(DH))
                n, cw = cfg["VR"], cfg["VC"]
                for r in range(r0, r1, n):
                    for c0 in range(0, D, cw):
                        rows = slice(S - RV + r, S - RV + r + n)
                        a = acc[rows, c0:c0 + cw] + _rep(_wide(tok, cw), n)
                        for e in range(DH):
                            ob = [obx[r // 8 + g, e] for g in range(n // 8)]
                            ob = ob[0] if n == 8 else jnp.concatenate(ob, axis=0)
                            a = a + _wide(ob, cw) * _rep(wrow[e][:, c0:c0 + cw], n)
                        acc[rows, c0:c0 + cw] = a
                        t = _fold(jnp.add, _tiles(a))
                        tok = _zero_of(_fold(jnp.add, [t[g:g + 8] for g in range(0, n, 8)]))
                done.append(tok)
            return f

        def matvec(wv, tok=None, step=16):
            n = wv.shape[1]
            part = None if tok is None else _wide(tok, n)
            for r in range(0, D, step):
                t = wv[r:r + step, :].astype(f32) * _wide(cb_buf[r:r + step, :], n)
                for e in range(step // 8):
                    te = t[e * 8:(e + 1) * 8, :]
                    part = te if part is None else part + te
            return _rb(jnp.sum(part, axis=0, keepdims=True))

        def mod_piece(p, tok=None):
            extra = isinstance(p, int) and p > NB
            modr[p] = matvec(wmx.at[p - NB - 1] if extra else w4.at[p & 1, 1], tok)

        def finish_mod():
            n = D // MC
            ga, sb, cb, gb = (jnp.concatenate([modr[i * n + t] for t in range(n)], axis=-1)
                              for i in range(4))
            cb1 = _rb(1.0 + cb)
            wr = wr_buf[...].astype(f32).reshape(1, D)
            a = cb1 * wr
            a0 = jnp.broadcast_to(jnp.sum(a, axis=-1, keepdims=True), (1, D))
            b0 = jnp.broadcast_to(jnp.sum(sb * wr, axis=-1, keepdims=True), (1, D))
            for i, v in enumerate((ga, sb, cb1, gb, a, gb * cb1, gb * sb, a0, b0)):
                modv[i] = jnp.broadcast_to(v, (8, D))

        def out_rows(x1, mean, inv):
            return (x1 + ((x1 - _wide(mean, D)) * (_wide(inv, D) * modv[5]) + modv[6])).astype(bf16)

        def out_chunks(j):
            x1v, sv, ov = view(acc, j, TL), view(st2_buf, j, TL), view(o_buf, j, TL)

            def chunk(off):
                def f(tok):
                    rs = slice(off, off + 8)
                    ov[rs, :] = out_rows(x1v[rs, :], sv[rs, 0:128] + tok, sv[rs, 128:256] + tok)
                return f
            return [chunk(off) for off in range(0, TL, 8)]

        def epi_chunks(j, x1v, ov, with_out=True):
            sub = lax.broadcasted_iota(i32, (8, 128), 0)
            low = (0xFFFF - j * TL) - sub
            sv = view(st2_buf, j, TL)
            st = {}

            def chunk(off):
                def f(tok=None):
                    if off == 0:
                        st["k1"], st["k2"] = key_buf[0], key_buf[1]
                    x1 = x1v[off:off + 8, :]
                    mean, inv = _row_stats(x1, tok)
                    sv[off:off + 8, 0:128] = mean
                    sv[off:off + 8, 128:256] = inv
                    xa = _tiles(x1 * modv[4])
                    if tok is not None:
                        xa[0] = xa[0] + tok
                    ra = _lane_sum(_fold(jnp.add, xa))
                    r = inv * (ra - mean * modv[7, :, 0:128]) + modv[8, :, 0:128]
                    if with_out:
                        ov[off:off + 8, :] = out_rows(x1, mean, inv)
                    bits = pltpu.bitcast(_rb(r) + 0.0, i32)
                    key = jnp.where(bits < 0, bits ^ 0x7FFF0000, bits) | (low - off)
                    st["k2"] = jnp.maximum(st["k2"], jnp.minimum(st["k1"], key))
                    st["k1"] = jnp.maximum(st["k1"], key)
                    if off + 8 == TL:
                        key_buf[0], key_buf[1] = st["k1"], st["k2"]
                return f
            return [chunk(off) for off in range(0, TL, 8)]

        cp_c().start()
        cp_x(0).start()
        for c in range(2):
            cp_wq0(c).start()
            for i in range(n_mch):
                cp_ca(c, i).start()
            if c == 0:
                for j in range(1, J0):
                    cp_x(j).start()
        cp_sa().start()
        for h in range(G - 1):
            cp_k(h, sem_first.at[1 + h]).start()
        early = []
        for h in range(2):
            early += [cp_v(h, sem_first.at[8 + 2 * h]), cp_wo(h, sem_first.at[9 + 2 * h])]
        for cp in early:
            cp.start()
        start_head(0)

        cp_c().wait()
        cf = c_buf[...].astype(f32)
        sc = _rb(cf * jax.nn.sigmoid(cf))
        for t in range(4):
            sc_buf[t] = sc[:, t * (D // 4):(t + 1) * (D // 4)]

        def cb_body(t, carry):
            view(cb_buf, t, D // 4)[...] = jnp.transpose(jnp.broadcast_to(sc_buf[t], (128, D // 4)))
            return carry
        lax.fori_loop(0, 4, cb_body, 0)
        key_buf[...] = jnp.full(key_buf.shape, _IMIN, i32)
        cp_x(0).wait()

        def st0_body(i, carry):
            for ch in ln1_chunks(view(x_buf, i, T0 // 4), view(st_buf, i, T0 // 4)):
                ch()
            return carry
        lax.fori_loop(0, 4, st0_body, 0)

        def zero_body(e, carry):
            obx[:, e] = jnp.zeros((RV // 8, 8, 128), f32)
            if cfg["WX"]:
                view(wof, e, 8)[...] = jnp.zeros((8, D), f32)
            return carry
        if RV:
            lax.fori_loop(0, DH, zero_body, 0, unroll=4)
            acc[S - RV:, :] = jnp.zeros((RV, D), f32)
            if not cfg["WX"]:
                wof[...] = jnp.zeros((DH, D), f32)

        def ca_half(c, stream):
            cp_wq0(c).wait()
            if not stream:
                for i in range(n_mch):
                    cp_ca(c, i).wait()
            part = None
            for i in range(n_mch):
                if stream:
                    cp_ca(c, i).wait()
                scb = jnp.broadcast_to(sc[:, i * MCH:(i + 1) * MCH], (16, MCH)).astype(bf16)
                d = jnp.dot(scb, wca[c, i * MCH:(i + 1) * MCH, :], preferred_element_type=f32)
                part = d if part is None else part + d
            mod0[1, :, c * W:(c + 1) * W] = _rb(1.0 + _rb(part[0:8, :]))

        def q_first(r0, t, c, rec, mid=None):
            rows = pl.ds(r0, t)
            cs = slice(c * W, (c + 1) * W)
            hh = ln1_scaled(x_buf[rows, cs], st_buf[rows, :], cs).astype(bf16)
            for g in range(G):
                if mid is not None and g == mid[0]:
                    mid[1]()
                part = jnp.dot(hh, wq0[cs, g * DH:(g + 1) * DH], preferred_element_type=f32)
                qf_buf[g, rows, :] = part if c == 0 else qf_buf[g, rows, :] + part
                if rec is not None:
                    rec.done(part)

        ca_half(0, True)

        def pa_body(j, carry):
            @pl.when(j + 1 < J0)
            def _():
                cp_x(j + 1).wait()
            jn = jnp.minimum(j + 1, J0 - 1)
            rec = _Pace(ln1_chunks(view(x_buf, jn, T0), view(st_buf, jn, T0)), cfg["LCA"])
            q_first(_mul(j, T0), T0, 0, rec)
            return carry
        lax.fori_loop(0, J0, pa_body, 0)

        TB, RB = cfg["TB"], cfg["RB"]
        ca_half(1, False)
        q_first(0, TB, 1, None)
        cp_sa().wait()
        cp_k(0, sem_first.at[1]).wait()
        cp_wr().start()
        for p in range(NB + 1, H):
            cp_wmx(p).start()

        def sa_chunk(t):
            def f(tok):
                cs = slice(t * 256, (t + 1) * 256)
                mod0[0, :, cs] = jnp.broadcast_to(matvec(wsa.at[:, cs], tok, 8), (8, 256))
            return f

        def sa_bias():
            bq_buf[...] = jnp.dot(_rep(mod0[0], 16).astype(bf16), wq0[...],
                                  preferred_element_type=f32)[0:8, :]

        def h_chunk(off):
            def f(tok):
                rs, rh = slice(off, off + RB), slice(off // 2, (off + RB) // 2)
                hh = (ln1_scaled(x_buf[rs, :], st_buf[rs, :], slice(0, D), tok)
                      + _rep(mod0[0], RB)).astype(bf16)
                h_buf[rh, :] = pltpu.bitcast(hh, u32)
            return f

        def q_chunk(off):
            def f(tok):
                n = 2 * RB
                rs, rh = slice(off, off + n), slice(off // 2, (off + n) // 2)
                for g in range(1, G):
                    q_ring[g, rh, :] = pltpu.bitcast(
                        q_early(g, qf_buf[g, rs, :] + _rep(tok, n)), u32)
            return f

        hs = [h_chunk(off) for off in range(0, S, RB)]
        qs = [q_chunk(off) for off in range(0, S, 2 * RB)]
        nh = cfg["NHB"]
        rest_chunks = []
        nq, nr = len(qs), len(hs) - nh
        for i, ch in enumerate(hs[nh:]):
            rest_chunks.append(ch)
            while qs and (nq - len(qs)) * nr < (i + 1) * nq:
                rest_chunks.append(qs.pop(0))
        assert not qs
        rec = _Pace([sa_chunk(t) for t in range(D // 256)] + hs[:nh], cfg["LCB2"])
        q_first(TB, S - TB, 1, rec, mid=(cfg["BQ"], sa_bias))
        n4 = len(rest_chunks)
        n3 = n4 - cfg["NL4"]
        cnt = [n3 // 3 + (1 if i < n3 % 3 else 0) for i in range(3)] + [cfg["NL4"]]
        scores(0, q_early(0, qf_buf[0]), s_buf, m_buf, rec=_Pace(rest_chunks, cnt), reload=True)

        def main_body(h, carry):
            plans = [(pack_chunks(h) + [lambda tok: mod_piece(h, tok)], cfg["LCM"])]
            vdone = []
            if RV:
                wch, och = expand_chunks(h)
                cuts = [0]
                for ch in cfg["LVN"]:
                    cuts.append(cuts[-1] + 8 * int(ch))
                assert cuts[-1] == RV
                wrow = []
                vps = [vproj(a, b, vdone, wrow) for a, b in zip(cuts, cuts[1:])]
                plans += [(vps, cfg["LCV"]), (wch, cfg["LCW"]), (och, cfg["LCO"])]
            rec = _mix(*plans)
            qproj(h + G, w4.at[h & 1, 0], rec=rec)
            start_head(h + 1)
            o = pv(h, s_buf, m_buf, rec=rec)
            if RV:
                ov_buf[...] = o[S - RV:, :].astype(f32)
            scores(h + 1, pltpu.bitcast(q_ring[(h + 1) & 3], bf16), s_buf, m_buf, rec=rec,
                   reload=cfg["RLM"], gate=(cfg["GR"], cfg["GP"], vdone) if RV else None)
            oproj([(h, o[0:S - RV, :])], acc.at[0:S - RV, :], rec=rec)
            wait_head(h + 1)
            return carry
        for h in range(1, G - 1):
            cp_k(h, sem_first.at[1 + h]).wait()
        for cp in early:
            cp.wait()
        wait_head(0)
        lax.fori_loop(0, NB, main_body, 0)

        ha = NB
        rest = list(zip(range(NB + 1, H), (s2_buf, s3_buf, s4_buf), (m2_buf, m3_buf, m4_buf)))
        late = []
        for n, h in enumerate(range(NB + 3, H)):
            late += [cp_v(h, sem_first.at[8 + 2 * n]), cp_wo(h, sem_first.at[9 + 2 * n])]
        cp_wr().wait()
        for p in range(NB + 1, H):
            cp_wmx(p).wait()
        if RV:
            oproj([(NB - 1, ov_buf[...].astype(bf16))], acc.at[S - RV:, :])
        for cp in late:
            cp.start()

        def l_step(j, do_x, do_y):
            if do_x and do_y:
                aw = view(acc, j - 1, TL, 2)
                ay, ax = aw.at[0:TL, :], aw.at[TL:2 * TL, :]
            elif do_x:
                ax = view(acc, j, TL)
            else:
                ay = view(acc, j - 1, TL)
            rec = None
            if do_y:
                chunks = epi_chunks(j - 1, ay, view(o_buf, j - 1, TL), with_out=do_x)
                os_ = [(h, pv(h, sv, mv, late=not do_x)) for h, sv, mv in rest]
            if do_x:
                oa = pv(ha, view(s_buf, j, TL), view(m_buf, j, TL))
            if do_y and do_x:
                oproj(os_, ay, view(x_buf, j - 1, TL))
            elif do_y:
                xv = view(x_buf, j - 1, TL)
                r0, prev = 0, []
                for n in cfg["LSPLIT"]:
                    rs = slice(r0, r0 + n)
                    nr = len(os_) * (D // W)
                    cnt = [len(prev) // nr + (1 if i < len(prev) % nr else 0) for i in range(nr)]
                    rec = _Pace(prev, cnt)
                    oproj([(h, o[rs]) for h, o in os_], ay.at[rs, :], xv.at[rs, :], rec=rec)
                    prev = chunks[r0 // 8:(r0 + n) // 8]
                    r0 += n
                chunks = prev
            if do_x:
                if do_y:
                    rec = _Pace(chunks, cfg["LCNT"])
                for h, sv, mv in rest:
                    q = pltpu.bitcast(view(q_ring.at[h & 3], j, TL // 2)[...], bf16)
                    scores(h, q, sv, mv, rec=rec, reload=True)
                oproj([(ha, oa)], ax, rec=rec)
            if do_y:
                if do_x:
                    cp_out(j - 1).start()
                else:
                    for ch in chunks:
                        ch()

        for p in range(NB, H):
            mod_piece(p)
        finish_mod()
        l_step(0, True, False)
        for cp in late:
            cp.wait()

        def pl_body(j, carry):
            l_step(j, True, True)
            return carry
        lax.fori_loop(1, JL, pl_body, 0)
        l_step(JL, False, True)

        k1, k2 = key_buf[0], key_buf[1]
        for sh in (4, 2, 1):
            o1, o2 = pltpu.roll(k1, sh, 0), pltpu.roll(k2, sh, 0)
            k2 = jnp.maximum(jnp.minimum(k1, o1), jnp.maximum(k2, o2))
            k1 = jnp.maximum(k1, o1)

        def score_of(k):
            hi = k & jnp.int32(-65536)
            return pltpu.bitcast(jnp.where(hi < 0, hi ^ 0x7FFF0000, hi), f32)

        i1s = jnp.minimum(0xFFFF - (k1[0, 0] & 0xFFFF), S - 1)
        i2s = jnp.minimum(0xFFFF - (k2[0, 0] & 0xFFFF), S - 1)

        sub = lax.broadcasted_iota(i32, (16, D), 0)
        sb, cb1, gb = (_rep(modv[i], 16) for i in (1, 2, 3))

        def adaln2(x1, stat):
            return (x1 - _wide(stat[:, 0:128], D)) * _wide(stat[:, 128:256], D) * cb1 + sb

        def pick(ref):
            sel = lax.broadcasted_iota(i32, (16, ref.shape[1]), 0) == 0
            return jnp.where(sel, ref[pl.ds(i1s, 1), :], ref[pl.ds(i2s, 1), :])

        xs = adaln2(pick(acc), pick(st2_buf)).astype(bf16)
        FC, lag = cfg["FC"], cfg["FLAG"]
        kvs = [int(ch) for ch in cfg["LKV"]]
        fout = [int(ch, 36) for ch in cfg["LFO"]]
        KV = max(kvs)

        def wrows(ref, a, b, c):
            n = FC // 128
            u = [ref[c * n + t, a // 2:b // 2, :] for t in range(n)]
            return pltpu.bitcast(u[0] if n == 1 else jnp.concatenate(u, axis=1), bf16)

        DV = D - KV * 128
        if KV:
            xf = xs.astype(f32)
            for r in range(2):
                xc_buf[r] = jnp.transpose(jnp.broadcast_to(xf[r:r + 1, DV:], (128, D - DV)))
        subc = lax.broadcasted_iota(i32, (8, FC), 0)
        y = None
        act = []
        outs = out_chunks(JL - 1)
        for c in range(F // FC + lag):
            if c < F // FC:
                dm = D - kvs[c] * 128
                gu = [jnp.dot(xs[:, :dm], wrows(w, 0, dm, c), preferred_element_type=f32)[0:8, :]
                      for w in (wg, wu)]
                for v in gu:
                    for t in range(fout[c] if c < len(fout) else 0):
                        if outs:
                            outs.pop(0)(_zero_of(v[0:8, (t % 2) * 128:(t % 2 + 1) * 128]))
                            if not outs:
                                cp_out(JL - 1).start()
                if dm < D:
                    part = [[None, None], [None, None]]
                    for k in range(dm, D, 16):
                        xcol = [_wide(xc_buf[r, k - DV:k - DV + 16, :], FC) for r in range(2)]
                        for m, w in enumerate((wg, wu)):
                            wv = wrows(w, k, k + 16, c).astype(f32)
                            for r in range(2):
                                t = wv * xcol[r]
                                for e in range(2):
                                    te = t[e * 8:(e + 1) * 8, :]
                                    part[m][r] = te if part[m][r] is None else part[m][r] + te
                    for m in range(2):
                        ra, rb_ = (jnp.sum(v, axis=0, keepdims=True) for v in part[m])
                        gu[m] = gu[m] + jnp.where(subc == 0, ra, rb_)
                g, u = _rb(gu[0]), _rb(gu[1])
                act.append(_rep(_rb(g * jax.nn.sigmoid(g)) * u, 16).astype(bf16))
            if c >= lag:
                wdc = pltpu.bitcast(wd[(c - lag) * FC // 2:(c - lag + 1) * FC // 2, :], bf16)
                d = jnp.dot(act[c - lag], wdc, preferred_element_type=f32)[0:8, :]
                y = d if y is None else y + d
        y = _rb(y)
        ya = _rb(y[0:1, :] * _wide(_rb(jax.nn.sigmoid(score_of(k1[0:1, :]))), D))
        yb = _rb(y[1:2, :] * _wide(_rb(jax.nn.sigmoid(score_of(k2[0:1, :]))), D))

        g1 = pl.multiple_of((i1s >> 4) << 4, 16)
        g2 = pl.multiple_of((i2s >> 4) << 4, 16)
        for t, g0 in enumerate((g1, g2)):
            rid = sub + g0
            x1 = acc[pl.ds(g0, 16), :]
            upd = jnp.where(rid == i1s, ya, 0.0) + jnp.where(rid == i2s, yb, 0.0)
            fix[t] = (x1 + gb * (adaln2(x1, st2_buf[pl.ds(g0, 16), :]) + upd)).astype(bf16)

        pltpu.make_async_copy(o_buf, out_hbm, sem_out.at[0]).wait()

        def cp_fix(t, g0):
            return pltpu.make_async_copy(fix.at[t], out_hbm.at[pl.ds(g0, 16), :], sem_fix.at[t])

        cp_fix(0, g1).start()

        @pl.when(g2 != g1)
        def _():
            cp_fix(1, g2).start()
            cp_fix(1, g2).wait()
        cp_fix(0, g1).wait()

    return kernel


_CFG = dict(
    G=4, T0=256, TB=1024, TL=256, MCH=256, RB=16, FC=256,
    LCA='cc80', LCB2='040g', NHB=16, NL4=8, BQ=3, LCNT='33333333332000',
    PKN=8, RV=64, WX=0, VR=8, VC=1024, GR=9, GP=0, LVN='8', LCV='000000100000', RLM=1, LD=2,
    LCM='000000988000', LCW='000000000088', LCO='000000000gg0',
    LSPLIT=(96, 96, 64), FLAG=1, LKV='00233333333333', LFO='88',
)


def _build(A_x, A_k_cache, A_v_cache, A_wq, A_wo, B_w_r, B_w_gate, B_w_up, B_w_down, c, w_mod,
           **over):
    B, S, D = A_x.shape
    _, H, SK, DH = A_k_cache.shape
    F = B_w_gate.shape[1]
    assert B == 1
    cfg = dict(_CFG, **over)
    T0, TL, G = cfg["T0"], cfg["TL"], cfg["G"]
    MC = (4 * D) // H
    kernel = _make_kernel(S, D, H, DH, SK, F, cfg)
    scratch = [
        pltpu.VMEM((S, D), bf16),
        pltpu.VMEM((S // 2, D), u32),
        pltpu.VMEM((S, D), f32),
        pltpu.VMEM((S, SK), f32),
        pltpu.VMEM((S, 128), f32),
        pltpu.VMEM((TL, SK), f32),
        pltpu.VMEM((TL, 128), f32),
        pltpu.VMEM((TL, SK), f32),
        pltpu.VMEM((TL, 128), f32),
        pltpu.VMEM((TL, SK), f32),
        pltpu.VMEM((TL, 128), f32),
        pltpu.VMEM((S, 256), f32),
        pltpu.VMEM((S, 256), f32),
        pltpu.VMEM((4, S // 2, DH), u32),
        pltpu.VMEM((G, S, DH), f32),
        pltpu.VMEM((8, G * DH), f32),
        pltpu.VMEM((4, SK, DH), bf16),
        pltpu.VMEM((4, SK, DH), bf16),
        pltpu.VMEM((D, G * DH), bf16),
        pltpu.VMEM((2, 4, D, 128), bf16),
        pltpu.VMEM((4, 2, DH, D), bf16),
        pltpu.VMEM((G - 1, D, MC), bf16),
        pltpu.VMEM((2, D, D // 2), bf16),
        pltpu.VMEM((D, D), bf16),
        pltpu.VMEM((1, D), bf16),
        pltpu.VMEM((D,), bf16),
        pltpu.VMEM((4, 1, D // 4), f32),
        pltpu.VMEM((D, 128), f32),
        pltpu.VMEM((2, 8, D), f32),
        pltpu.VMEM((H, 1, MC), f32),
        pltpu.VMEM((9, 8, D), f32),
        pltpu.VMEM((F // 128, D // 2, 128), u32),
        pltpu.VMEM((F // 128, D // 2, 128), u32),
        pltpu.VMEM((F // 2, D), u32),
        pltpu.VMEM((2, max(int(max(cfg["LKV"])), 1) * 128, 128), f32),
        pltpu.VMEM((max(cfg["RV"], 8), DH), f32),
        pltpu.VMEM((max(cfg["RV"], 8) // 8, DH, 8, 128), f32),
        pltpu.VMEM((DH * (8 if cfg['WX'] else 1), D), f32),
        pltpu.VMEM((S, D), bf16),
        pltpu.VMEM((2, 8, 128), i32),
        pltpu.VMEM((2, 16, D), bf16),
        pltpu.SemaphoreType.DMA((sum(_sem_sizes(S, D, cfg)),)),
    ]
    any_spec = pl.BlockSpec(memory_space=pl.ANY)
    out = pl.pallas_call(
        kernel,
        out_shape=jax.ShapeDtypeStruct((S, D), bf16),
        in_specs=[any_spec] * 11,
        out_specs=any_spec,
        scratch_shapes=scratch,
        compiler_params=pltpu.CompilerParams(vmem_limit_bytes=126 * 1024 * 1024,
                                             disable_bounds_checks=True,
                                             disable_semaphore_checks=True),
    )(A_x.reshape(S, D), A_k_cache.reshape(H, SK, DH), A_v_cache.reshape(H, SK, DH),
      A_wq, A_wo, B_w_r, B_w_gate, B_w_up, B_w_down, c, w_mod)
    return out.reshape(B, S, D)


@jax.jit
def pallas_adaLN_cond__mha_block_cached__moe_arch_mod__prompt_kernel(
    A_x: jax.Array,
    A_k_cache: jax.Array,
    A_v_cache: jax.Array,
    A_wq: jax.Array,
    A_wo: jax.Array,
    B_x: jax.Array,
    B_w_r: jax.Array,
    B_w_gate: jax.Array,
    B_w_up: jax.Array,
    B_w_down: jax.Array,
    c: jax.Array,
    w_mod: jax.Array,
):
    del B_x
    return _build(A_x, A_k_cache, A_v_cache, A_wq, A_wo, B_w_r, B_w_gate, B_w_up, B_w_down,
                  c, w_mod)
```

```python
import jax
import jax.numpy as jnp
from jax import lax
import jax.experimental.pallas as pl
import jax.experimental.pallas.tpu as pltpu

f32 = jnp.float32
bf16 = jnp.bfloat16
u32 = jnp.uint32
i32 = jnp.int32

_NT = (((1,), (1,)), ((), ()))
_LOG2E = 1.4426950408889634
_EPS = 1e-5
_IMIN = -2 ** 31


def _rb(v):
    return v.astype(bf16).astype(f32)


def _rep(v, n):
    return v if n == 8 else jnp.tile(v, (n // 8, 1))


def _wide(v, w):
    return jnp.tile(v, (1, w // 128))


def _zero_of(v):
    bits = pltpu.bitcast(v, u32)
    return pltpu.bitcast(lax.shift_right_logical(lax.shift_right_logical(bits, jnp.uint32(31)),
                                                 jnp.uint32(1)), f32)


def _gate(lhs, dep, row):
    u = pltpu.bitcast(lhs, u32)
    r = row // 16 * 8
    parts = [u[0:r]] if r else []
    parts.append(u[r:r + 8] | pltpu.bitcast(_zero_of(dep), u32))
    if r + 8 < u.shape[0]:
        parts.append(u[r + 8:])
    return pltpu.bitcast(jnp.concatenate(parts, axis=0), bf16)


class _Pace:
    def __init__(self, chunks, counts):
        self.chunks = list(chunks)
        self.counts = [ch if isinstance(ch, int) else int(ch, 36) for ch in counts]
        assert sum(self.counts) == len(self.chunks), (counts, len(self.chunks))

    def done(self, res):
        n = self.counts.pop(0)
        for i in range(n):
            r0 = (i * res.shape[0] // n) // 8 * 8
            self.chunks.pop(0)(_zero_of(res[r0:r0 + 8, 0:128]))


def _mix(*plans):
    plans = [(list(ch), [c if isinstance(c, int) else int(c, 36) for c in cnt]) for ch, cnt in plans]
    for ch, cnt in plans:
        assert sum(cnt) == len(ch), (cnt, len(ch))
    fill, total = [], []
    for r in range(len(plans[0][1])):
        slots = sorted((i / cnt[r], k) for k, (_, cnt) in enumerate(plans)
                       for i in range(cnt[r]))
        fill += [plans[k][0].pop(0) for _, k in slots]
        total.append(len(slots))
    return _Pace(fill, total)


def _tiles(v):
    return [v[:, c * 128:(c + 1) * 128] for c in range(v.shape[1] // 128)]


def _fold(op, parts):
    out = parts[0]
    for p in parts[1:]:
        out = op(out, p)
    return out


def _lane_sum(v):
    return jnp.broadcast_to(jnp.sum(v, axis=-1, keepdims=True), v.shape)


def _row_stats(xf, tok=None):
    d = xf.shape[-1]
    ts = _tiles(xf)
    nt = len(ts)
    if tok is not None:
        ts = [ts[0] + tok] + ts[1:]
    mu = _fold(jnp.add, ts) * (1.0 / nt)
    m2 = _fold(jnp.add, [(t - mu) * (t - mu) for t in ts])
    mean = _lane_sum(mu) * (1.0 / 128)
    dm = mu - mean
    var = _lane_sum(m2 + (dm * dm) * float(nt)) * (1.0 / d)
    return mean, lax.rsqrt(var + _EPS)


def _sem_sizes(S, D, cfg):
    j0 = S // cfg["T0"]
    return [2, 2 * (D // cfg["MCH"]), j0, 1, 16, 4, 1, 2]


def _make_kernel(S, D, H, DH, SK, F, cfg):
    T0, TL, MCH = cfg["T0"], cfg["TL"], cfg["MCH"]
    J0 = S // T0
    JL = S // TL
    qscale = DH ** -0.5 * _LOG2E
    n_mch = D // MCH
    G = cfg["G"]
    NB = H - G
    MC = (4 * D) // H
    W = 512
    NF = F // 128
    assert 2 <= G <= 4 and D == 2 * W and MC == DH == 128 and NF <= NB

    def kernel(x_hbm, k_hbm, v_hbm, wq_hbm, wo_hbm, wr_hbm, wg_hbm, wu_hbm, wd_hbm,
               c_hbm, wmod_hbm, out_hbm,
               x_buf, h_buf, acc, s_buf, m_buf, s2_buf, m2_buf, s3_buf, m3_buf, s4_buf, m4_buf,
               st_buf, st2_buf,
               q_ring, qf_buf, bq_buf,
               kb, vb, wq0, w4, wo2, wmx, wca, wsa, c_buf, wr_buf, sc_buf, cb_buf, mod0, modr, modv,
               wg, wu, wd, xc_buf, ov_buf, obx, wof, o_buf, key_buf, fix,
               sems):

        class _Sem:
            def __init__(self, base):
                self.base = base
                self.at = self

            def __getitem__(self, i):
                return sems.at[self.base + i]

        sizes = _sem_sizes(S, D, cfg)
        offs = [sum(sizes[:i]) for i in range(len(sizes))]
        (sem_small, sem_ca, sem_x, sem_sa, sem_first, sem_head,
         sem_out, sem_fix) = (_Sem(o) for o in offs)

        def _mul(a, n):
            v = a * n
            return v if isinstance(a, int) else pl.multiple_of(v, n)

        def view(ref, j, t, n=1):
            return ref.at[pl.ds(_mul(j, t), n * t), :]

        def cp_c():
            return pltpu.make_async_copy(c_hbm, c_buf, sem_small.at[0])

        def cp_wr():
            return pltpu.make_async_copy(wr_hbm, wr_buf, sem_small.at[1])

        def cp_ca(c, i):
            return pltpu.make_async_copy(
                wmod_hbm.at[pl.ds(i * MCH, MCH), pl.ds(D + c * W, W)], view(wca.at[c], i, MCH),
                sem_ca.at[c * n_mch + i])

        def cp_sa():
            return pltpu.make_async_copy(wmod_hbm.at[:, pl.ds(0, D)], wsa, sem_sa.at[0])

        def cp_x(j):
            return pltpu.make_async_copy(view(x_hbm, j, T0), view(x_buf, j, T0), sem_x.at[j])

        def cp_wq0(c):
            return pltpu.make_async_copy(wq_hbm.at[pl.ds(c * W, W), pl.ds(0, G * DH)],
                                         view(wq0, c, W), sem_first.at[14 + c])

        def cp_k(h, sem=None):
            return pltpu.make_async_copy(k_hbm.at[h], kb.at[h & 3],
                                         sem_head.at[0] if sem is None else sem)

        def cp_v(h, sem=None):
            return pltpu.make_async_copy(v_hbm.at[h], vb.at[h & 3],
                                         sem_head.at[1] if sem is None else sem)

        def cp_wo(h, sem=None):
            return pltpu.make_async_copy(view(wo_hbm, h, DH), wo2.at[h & 3, 0],
                                         sem_head.at[2] if sem is None else sem)

        def _clamp(a, hi):
            return min(a, hi) if isinstance(a, int) else jnp.minimum(a, hi)

        def cols(ref, t):
            return ref.at[:, pl.ds(_mul(t, 128), 128)]

        def cp_wmx(p):
            return pltpu.make_async_copy(cols(wmod_hbm, p + (2 * D) // MC), wmx.at[p - NB - 1],
                                         sem_first.at[4 + p - NB])

        def start_head(h):
            f = _clamp(h, NF - 1)
            for i, src in enumerate((cols(wq_hbm, _clamp(h + G, H - 1)),
                                     cols(wmod_hbm, h + (2 * D) // MC),
                                     cols(wg_hbm, f), cols(wu_hbm, f))):
                pltpu.make_async_copy(src, w4.at[h & 1, i], sem_head.at[3]).start()
            cp_k(h + G - 1).start()
            cp_wo(h + 2).start()
            pltpu.make_async_copy(view(wd_hbm, f, 128), wo2.at[(h + 2) & 3, 1],
                                  sem_head.at[2]).start()
            cp_v(h + 2).start()

        def wait_head(h):
            pltpu.make_async_copy(w4.at[h & 1], w4.at[h & 1], sem_head.at[3]).wait()
            cp_k(h + G - 1).wait()
            pltpu.make_async_copy(wo2.at[(h + 2) & 3], wo2.at[(h + 2) & 3], sem_head.at[2]).wait()
            cp_v(h + 2).wait()

        def pack_chunks(h):
            f = _clamp(h, NF - 1)
            out = []
            for sv, dv in ((w4.at[h & 1, 2], wg.at[f]), (w4.at[h & 1, 3], wu.at[f]),
                           (wo2.at[(h + 2) & 3, 1], view(wd, f, 64))):
                n, w = sv.shape
                step = n // cfg['PKN']

                def chunk(r, sv=sv, dv=dv, step=step, w=w):
                    def fn(tok):
                        z = _rep(_wide(pltpu.bitcast(tok, u32), w), step // 2)
                        dv[r // 2:(r + step) // 2, :] = pltpu.bitcast(sv[r:r + step, :], u32) | z
                    return fn
                out += [chunk(r) for r in range(0, n, step)]
            return out

        def cp_out(j):
            return pltpu.make_async_copy(view(o_buf, j, TL), view(out_hbm, j, TL), sem_out.at[0])

        def ln1_chunks(xv, sv):
            def chunk(off):
                def f(tok=None):
                    mean, inv = _row_stats(xv[off:off + 8, :].astype(f32), tok)
                    sv[off:off + 8, 0:128] = mean
                    sv[off:off + 8, 128:256] = inv
                return f
            return [chunk(off) for off in range(0, xv.shape[0], 8)]

        def ln1_scaled(x, stat, cs, tok=None):
            w = x.shape[1]
            mean = stat[:, 0:128] if tok is None else stat[:, 0:128] + _rep(tok, x.shape[0])
            n = (x.astype(f32) - _wide(mean, w)) * _wide(stat[:, 128:256], w)
            return n * _rep(mod0[1, :, cs], x.shape[0])

        def qproj(h, wv, rec=None):
            q = None
            for c in range(D // W):
                cs = slice(c * W, (c + 1) * W)
                part = jnp.dot(pltpu.bitcast(h_buf[:, cs], bf16), wv[cs, :],
                               preferred_element_type=f32)
                q = part if q is None else q + part
                if rec is not None:
                    rec.done(part)
            q_ring[h & 3] = pltpu.bitcast((q * qscale).astype(bf16), u32)

        def q_early(g, q):
            return ((q + _rep(bq_buf[:, g * DH:(g + 1) * DH], q.shape[0])) * qscale).astype(bf16)

        def scores(h, q, sv, mv, rec=None, reload=False, gate=None):
            mp = None
            for c in range(SK // W):
                cs = slice(c * W, (c + 1) * W)
                qq = _gate(q, gate[2][-1], gate[1]) if (gate and gate[0] == c) else q
                s = lax.dot_general(qq, kb[h & 3, cs, :], _NT, preferred_element_type=f32)
                sv[:, cs] = s
                if rec is not None:
                    rec.done(s)
                if not reload:
                    mp = _fold(jnp.maximum, ([] if mp is None else [mp]) + _tiles(s))
            if reload:
                mp = _fold(jnp.maximum, _tiles(sv[...]))
            mv[...] = jnp.broadcast_to(jnp.max(mp, axis=-1, keepdims=True), mp.shape)

        def pv(h, sv, mv, rec=None, late=False):
            o = lp = None
            for c in range(SK // W):
                cs = slice(c * W, (c + 1) * W)
                m = mv[...]
                if c >= cfg["LD"] and sv.shape[0] == S:
                    m = m + _zero_of(lp)
                p = jnp.exp2(sv[:, cs] - _wide(m, W))
                lp = _fold(jnp.add, ([] if lp is None else [lp]) + _tiles(p))
                d = jnp.dot(p.astype(bf16), vb[h & 3, cs, :], preferred_element_type=f32)
                o = d if o is None else o + d
                if rec is not None:
                    rec.done(d)
            if late:
                lp = lp + _zero_of(o)
            l = jnp.sum(lp, axis=-1, keepdims=True)
            r = pl.reciprocal(l, approx=True)
            r = r * (2.0 - l * r)
            return (o * r).astype(bf16)

        def oproj(hos, av, xv=None, rec=None):
            for c in range(D // W):
                cs = slice(c * W, (c + 1) * W)
                a = av[:, cs]
                for h, o in hos:
                    if not isinstance(h, int):
                        a = jnp.where(h > 0, a, 0.0)
                    d = jnp.dot(o, wo2[h & 3, 0, :, cs], preferred_element_type=f32)
                    if rec is not None:
                        rec.done(d)
                    a = a + d
                if xv is not None:
                    a = xv[:, cs].astype(f32) + _rep(modv[0, :, cs], a.shape[0]) * a
                av[:, cs] = a

        RV = cfg["RV"]

        def expand_chunks(h):
            def wchunk(r):
                def f(tok):
                    wof[r:r + 8, :] = wo2[h & 3, 0, r:r + 8, :].astype(f32) + _wide(tok, D)
                return f

            def wchunk2(r, c0):
                def f(tok):
                    cs = slice(c0, c0 + 256)
                    w = wo2[h & 3, 0, r:r + 8, cs].astype(f32) + _wide(tok, 256)
                    for e in range(8):
                        wof[(r + e) * 8:(r + e + 1) * 8, cs] = jnp.broadcast_to(w[e:e + 1, :], (8, 256))
                return f

            lane = lax.broadcasted_iota(i32, (8, 128), 1)

            def ochunk(g, e0):
                def f(tok):
                    o = ov_buf[g * 8:(g + 1) * 8, :] + tok
                    for e in range(e0, e0 + 32):
                        obx[g, e] = _lane_sum(jnp.where(lane == e, o, 0.0))
                return f
            och = [ochunk(g, e0) for g in range(RV // 8) for e0 in range(0, DH, 32)]
            if cfg["WX"]:
                return [wchunk2(r, c0) for r in range(0, DH, 8) for c0 in range(0, D, 256)], och
            return [wchunk(r) for r in range(0, DH, 8)], och

        def vproj(r0, r1, done, wrow):
            def f(tok):
                if not wrow and cfg["WX"]:
                    wrow.extend(wof[e * 8:(e + 1) * 8, :] for e in range(DH))
                if not wrow:
                    wrow.extend(jnp.concatenate(
                        [jnp.broadcast_to(wof[e:e + 1, t * 128:(t + 1) * 128], (8, 128))
                         for t in range(D // 128)], axis=1) for e in range(DH))
                for r in range(r0, r1, 8):
                    rows = slice(S - RV + r, S - RV + r + 8)
                    a = acc[rows, :] + _wide(tok, D)
                    for e in range(DH):
                        a = a + _wide(obx[r // 8, e], D) * wrow[e]
                        if e == cfg["TE"]:
                            tok = _zero_of(_fold(jnp.add, _tiles(a)))
                    acc[rows, :] = a
                done.append(tok)
            return f

        def matvec(wv, tok=None, step=16):
            n = wv.shape[1]
            part = None if tok is None else _wide(tok, n)
            for r in range(0, D, step):
                t = wv[r:r + step, :].astype(f32) * _wide(cb_buf[r:r + step, :], n)
                for e in range(step // 8):
                    te = t[e * 8:(e + 1) * 8, :]
                    part = te if part is None else part + te
            return _rb(jnp.sum(part, axis=0, keepdims=True))

        def mod_piece(p, tok=None):
            extra = isinstance(p, int) and p > NB
            modr[p] = matvec(wmx.at[p - NB - 1] if extra else w4.at[p & 1, 1], tok)

        def finish_mod():
            n = D // MC
            ga, sb, cb, gb = (jnp.concatenate([modr[i * n + t] for t in range(n)], axis=-1)
                              for i in range(4))
            cb1 = _rb(1.0 + cb)
            wr = wr_buf[...].astype(f32).reshape(1, D)
            a = cb1 * wr
            a0 = jnp.broadcast_to(jnp.sum(a, axis=-1, keepdims=True), (1, D))
            b0 = jnp.broadcast_to(jnp.sum(sb * wr, axis=-1, keepdims=True), (1, D))
            for i, v in enumerate((ga, sb, cb1, gb, a, gb * cb1, gb * sb, a0, b0)):
                modv[i] = jnp.broadcast_to(v, (8, D))

        def out_rows(x1, mean, inv):
            return (x1 + ((x1 - _wide(mean, D)) * (_wide(inv, D) * modv[5]) + modv[6])).astype(bf16)

        def out_chunks(j):
            x1v, sv, ov = view(acc, j, TL), view(st2_buf, j, TL), view(o_buf, j, TL)

            def chunk(off):
                def f(tok):
                    rs = slice(off, off + 8)
                    ov[rs, :] = out_rows(x1v[rs, :], sv[rs, 0:128] + tok, sv[rs, 128:256] + tok)
                return f
            return [chunk(off) for off in range(0, TL, 8)]

        def epi_chunks(j, x1v, ov, with_out=True):
            sub = lax.broadcasted_iota(i32, (8, 128), 0)
            low = (0xFFFF - j * TL) - sub
            sv = view(st2_buf, j, TL)
            st = {}

            def chunk(off):
                def f(tok=None):
                    if off == 0:
                        st["k1"], st["k2"] = key_buf[0], key_buf[1]
                    x1 = x1v[off:off + 8, :]
                    mean, inv = _row_stats(x1, tok)
                    sv[off:off + 8, 0:128] = mean
                    sv[off:off + 8, 128:256] = inv
                    xa = _tiles(x1 * modv[4])
                    if tok is not None:
                        xa[0] = xa[0] + tok
                    ra = _lane_sum(_fold(jnp.add, xa))
                    r = inv * (ra - mean * modv[7, :, 0:128]) + modv[8, :, 0:128]
                    if with_out:
                        ov[off:off + 8, :] = out_rows(x1, mean, inv)
                    bits = pltpu.bitcast(_rb(r) + 0.0, i32)
                    key = jnp.where(bits < 0, bits ^ 0x7FFF0000, bits) | (low - off)
                    st["k2"] = jnp.maximum(st["k2"], jnp.minimum(st["k1"], key))
                    st["k1"] = jnp.maximum(st["k1"], key)
                    if off + 8 == TL:
                        key_buf[0], key_buf[1] = st["k1"], st["k2"]
                return f
            return [chunk(off) for off in range(0, TL, 8)]

        cp_c().start()
        cp_x(0).start()
        for c in range(2):
            cp_wq0(c).start()
            for i in range(n_mch):
                cp_ca(c, i).start()
            if c == 0:
                for j in range(1, J0):
                    cp_x(j).start()
        cp_sa().start()
        for h in range(G - 1):
            cp_k(h, sem_first.at[1 + h]).start()
        early = []
        for h in range(2):
            early += [cp_v(h, sem_first.at[8 + 2 * h]), cp_wo(h, sem_first.at[9 + 2 * h])]
        for cp in early:
            cp.start()
        start_head(0)

        cp_c().wait()
        cf = c_buf[...].astype(f32)
        sc = _rb(cf * jax.nn.sigmoid(cf))
        for t in range(4):
            sc_buf[t] = sc[:, t * (D // 4):(t + 1) * (D // 4)]

        def cb_body(t, carry):
            view(cb_buf, t, D // 4)[...] = jnp.transpose(jnp.broadcast_to(sc_buf[t], (128, D // 4)))
            return carry
        lax.fori_loop(0, 4, cb_body, 0)
        key_buf[...] = jnp.full(key_buf.shape, _IMIN, i32)
        cp_x(0).wait()

        def st0_body(i, carry):
            for ch in ln1_chunks(view(x_buf, i, T0 // 4), view(st_buf, i, T0 // 4)):
                ch()
            return carry
        lax.fori_loop(0, 4, st0_body, 0)

        def zero_body(e, carry):
            obx[:, e] = jnp.zeros((RV // 8, 8, 128), f32)
            if cfg["WX"]:
                view(wof, e, 8)[...] = jnp.zeros((8, D), f32)
            return carry
        if RV:
            lax.fori_loop(0, DH, zero_body, 0, unroll=4)
            acc[S - RV:, :] = jnp.zeros((RV, D), f32)
            if not cfg["WX"]:
                wof[...] = jnp.zeros((DH, D), f32)

        def ca_half(c, stream):
            cp_wq0(c).wait()
            if not stream:
                for i in range(n_mch):
                    cp_ca(c, i).wait()
            part = None
            for i in range(n_mch):
                if stream:
                    cp_ca(c, i).wait()
                scb = jnp.broadcast_to(sc[:, i * MCH:(i + 1) * MCH], (16, MCH)).astype(bf16)
                d = jnp.dot(scb, wca[c, i * MCH:(i + 1) * MCH, :], preferred_element_type=f32)
                part = d if part is None else part + d
            mod0[1, :, c * W:(c + 1) * W] = _rb(1.0 + _rb(part[0:8, :]))

        def q_first(r0, t, c, rec, mid=None):
            rows = pl.ds(r0, t)
            cs = slice(c * W, (c + 1) * W)
            hh = ln1_scaled(x_buf[rows, cs], st_buf[rows, :], cs).astype(bf16)
            for g in range(G):
                if mid is not None and g == mid[0]:
                    mid[1]()
                part = jnp.dot(hh, wq0[cs, g * DH:(g + 1) * DH], preferred_element_type=f32)
                qf_buf[g, rows, :] = part if c == 0 else qf_buf[g, rows, :] + part
                if rec is not None:
                    rec.done(part)

        ca_half(0, True)

        def pa_body(j, carry):
            @pl.when(j + 1 < J0)
            def _():
                cp_x(j + 1).wait()
            jn = jnp.minimum(j + 1, J0 - 1)
            rec = _Pace(ln1_chunks(view(x_buf, jn, T0), view(st_buf, jn, T0)), cfg["LCA"])
            q_first(_mul(j, T0), T0, 0, rec)
            return carry
        lax.fori_loop(0, J0, pa_body, 0)

        TB, RB = cfg["TB"], cfg["RB"]
        ca_half(1, False)
        q_first(0, TB, 1, None)
        cp_sa().wait()
        cp_k(0, sem_first.at[1]).wait()
        cp_wr().start()
        for p in range(NB + 1, H):
            cp_wmx(p).start()

        def sa_chunk(t):
            def f(tok):
                cs = slice(t * 256, (t + 1) * 256)
                mod0[0, :, cs] = jnp.broadcast_to(matvec(wsa.at[:, cs], tok, 8), (8, 256))
            return f

        def sa_bias():
            bq_buf[...] = jnp.dot(_rep(mod0[0], 16).astype(bf16), wq0[...],
                                  preferred_element_type=f32)[0:8, :]

        def h_chunk(off):
            def f(tok):
                rs, rh = slice(off, off + RB), slice(off // 2, (off + RB) // 2)
                hh = (ln1_scaled(x_buf[rs, :], st_buf[rs, :], slice(0, D), tok)
                      + _rep(mod0[0], RB)).astype(bf16)
                h_buf[rh, :] = pltpu.bitcast(hh, u32)
            return f

        def q_chunk(off):
            def f(tok):
                n = 2 * RB
                rs, rh = slice(off, off + n), slice(off // 2, (off + n) // 2)
                for g in range(1, G):
                    q_ring[g, rh, :] = pltpu.bitcast(
                        q_early(g, qf_buf[g, rs, :] + _rep(tok, n)), u32)
            return f

        hs = [h_chunk(off) for off in range(0, S, RB)]
        qs = [q_chunk(off) for off in range(0, S, 2 * RB)]
        nh = cfg["NHB"]
        rest_chunks = []
        nq, nr = len(qs), len(hs) - nh
        for i, ch in enumerate(hs[nh:]):
            rest_chunks.append(ch)
            while qs and (nq - len(qs)) * nr < (i + 1) * nq:
                rest_chunks.append(qs.pop(0))
        assert not qs
        rec = _Pace([sa_chunk(t) for t in range(D // 256)] + hs[:nh], cfg["LCB2"])
        q_first(TB, S - TB, 1, rec, mid=(cfg["BQ"], sa_bias))
        n4 = len(rest_chunks)
        n3 = n4 - cfg["NL4"]
        cnt = [n3 // 3 + (1 if i < n3 % 3 else 0) for i in range(3)] + [cfg["NL4"]]
        scores(0, q_early(0, qf_buf[0]), s_buf, m_buf, rec=_Pace(rest_chunks, cnt), reload=True)

        def main_body(h, carry):
            plans = [(pack_chunks(h), cfg["LCM"])]
            if "1" in cfg["LCP"]:
                plans.append(([lambda tok: mod_piece(h, tok)], cfg["LCP"]))
            vdone = []
            if RV:
                wch, och = expand_chunks(h)
                cuts = [0]
                for ch in cfg["LVN"]:
                    cuts.append(cuts[-1] + 8 * int(ch, 36))
                assert cuts[-1] == RV
                wrow = []
                vps = [vproj(a, b, vdone, wrow) for a, b in zip(cuts, cuts[1:])]
                plans += [(vps, cfg["LCV"]), (wch, cfg["LCW"]), (och, cfg["LCO"])]
            rec = _mix(*plans)
            qproj(h + G, w4.at[h & 1, 0], rec=rec)
            start_head(h + 1)
            o = pv(h, s_buf, m_buf, rec=rec)
            if RV:
                ov_buf[...] = o[S - RV:, :].astype(f32)
            scores(h + 1, pltpu.bitcast(q_ring[(h + 1) & 3], bf16), s_buf, m_buf, rec=rec,
                   reload=cfg["RLM"], gate=(cfg["GR"], cfg["GP"], vdone) if RV else None)
            oproj([(h, o[0:S - RV, :])], acc.at[0:S - RV, :], rec=rec)
            if "1" not in cfg["LCP"]:
                mod_piece(h)
            wait_head(h + 1)
            return carry
        for h in range(1, G - 1):
            cp_k(h, sem_first.at[1 + h]).wait()
        for cp in early:
            cp.wait()
        wait_head(0)
        lax.fori_loop(0, NB, main_body, 0)

        ha = NB
        rest = list(zip(range(NB + 1, H), (s2_buf, s3_buf, s4_buf), (m2_buf, m3_buf, m4_buf)))
        late = []
        for n, h in enumerate(range(NB + 3, H)):
            late += [cp_v(h, sem_first.at[8 + 2 * n]), cp_wo(h, sem_first.at[9 + 2 * n])]
        cp_wr().wait()
        for p in range(NB + 1, H):
            cp_wmx(p).wait()
        if RV:
            oproj([(NB - 1, ov_buf[...].astype(bf16))], acc.at[S - RV:, :])
        for cp in late:
            cp.start()

        def l_step(j, do_x, do_y):
            if do_x and do_y:
                aw = view(acc, j - 1, TL, 2)
                ay, ax = aw.at[0:TL, :], aw.at[TL:2 * TL, :]
            elif do_x:
                ax = view(acc, j, TL)
            else:
                ay = view(acc, j - 1, TL)
            rec = None
            if do_y:
                chunks = epi_chunks(j - 1, ay, view(o_buf, j - 1, TL), with_out=do_x)
                os_ = [(h, pv(h, sv, mv, late=not do_x)) for h, sv, mv in rest]
            if do_x:
                oa = pv(ha, view(s_buf, j, TL), view(m_buf, j, TL))
            if do_y and do_x:
                oproj(os_, ay, view(x_buf, j - 1, TL))
            elif do_y:
                xv = view(x_buf, j - 1, TL)
                r0, prev = 0, []
                for n in cfg["LSPLIT"]:
                    rs = slice(r0, r0 + n)
                    nr = len(os_) * (D // W)
                    cnt = [len(prev) // nr + (1 if i < len(prev) % nr else 0) for i in range(nr)]
                    rec = _Pace(prev, cnt)
                    oproj([(h, o[rs]) for h, o in os_], ay.at[rs, :], xv.at[rs, :], rec=rec)
                    prev = chunks[r0 // 8:(r0 + n) // 8]
                    r0 += n
                chunks = prev
            if do_x:
                if do_y:
                    rec = _Pace(chunks, cfg["LCNT"])
                for h, sv, mv in rest:
                    q = pltpu.bitcast(view(q_ring.at[h & 3], j, TL // 2)[...], bf16)
                    scores(h, q, sv, mv, rec=rec, reload=True)
                oproj([(ha, oa)], ax, rec=rec)
            if do_y:
                if do_x:
                    cp_out(j - 1).start()
                else:
                    for ch in chunks:
                        ch()

        for p in range(NB, H):
            mod_piece(p)
        finish_mod()
        l_step(0, True, False)
        for cp in late:
            cp.wait()

        def pl_body(j, carry):
            l_step(j, True, True)
            return carry
        lax.fori_loop(1, JL, pl_body, 0)
        l_step(JL, False, True)

        k1, k2 = key_buf[0], key_buf[1]
        for sh in (4, 2, 1):
            o1, o2 = pltpu.roll(k1, sh, 0), pltpu.roll(k2, sh, 0)
            k2 = jnp.maximum(jnp.minimum(k1, o1), jnp.maximum(k2, o2))
            k1 = jnp.maximum(k1, o1)

        def score_of(k):
            hi = k & jnp.int32(-65536)
            return pltpu.bitcast(jnp.where(hi < 0, hi ^ 0x7FFF0000, hi), f32)

        i1s = jnp.minimum(0xFFFF - (k1[0, 0] & 0xFFFF), S - 1)
        i2s = jnp.minimum(0xFFFF - (k2[0, 0] & 0xFFFF), S - 1)

        sub = lax.broadcasted_iota(i32, (16, D), 0)
        sb, cb1, gb = (_rep(modv[i], 16) for i in (1, 2, 3))

        def adaln2(x1, stat):
            return (x1 - _wide(stat[:, 0:128], D)) * _wide(stat[:, 128:256], D) * cb1 + sb

        def pick(ref):
            sel = lax.broadcasted_iota(i32, (16, ref.shape[1]), 0) == 0
            return jnp.where(sel, ref[pl.ds(i1s, 1), :], ref[pl.ds(i2s, 1), :])

        xs = adaln2(pick(acc), pick(st2_buf)).astype(bf16)
        FC, lag = cfg["FC"], cfg["FLAG"]
        kvs = [int(ch) for ch in cfg["LKV"]]
        fout = [int(ch, 36) for ch in cfg["LFO"]]
        KV = max(kvs)

        def wrows(ref, a, b, c):
            n = FC // 128
            u = [ref[c * n + t, a // 2:b // 2, :] for t in range(n)]
            return pltpu.bitcast(u[0] if n == 1 else jnp.concatenate(u, axis=1), bf16)

        DV = D - KV * 128
        if KV:
            xf = xs.astype(f32)
            for r in range(2):
                xc_buf[r] = jnp.transpose(jnp.broadcast_to(xf[r:r + 1, DV:], (128, D - DV)))
        subc = lax.broadcasted_iota(i32, (8, FC), 0)
        y = None
        act = []
        outs = out_chunks(JL - 1)
        for c in range(F // FC + lag):
            if c < F // FC:
                dm = D - kvs[c] * 128
                gu = [jnp.dot(xs[:, :dm], wrows(w, 0, dm, c), preferred_element_type=f32)[0:8, :]
                      for w in (wg, wu)]
                for v in gu:
                    for t in range(fout[c] if c < len(fout) else 0):
                        if outs:
                            outs.pop(0)(_zero_of(v[0:8, (t % 2) * 128:(t % 2 + 1) * 128]))
                            if not outs:
                                cp_out(JL - 1).start()
                if dm < D:
                    part = [[None, None], [None, None]]
                    for k in range(dm, D, 16):
                        xcol = [_wide(xc_buf[r, k - DV:k - DV + 16, :], FC) for r in range(2)]
                        for m, w in enumerate((wg, wu)):
                            wv = wrows(w, k, k + 16, c).astype(f32)
                            for r in range(2):
                                t = wv * xcol[r]
                                for e in range(2):
                                    te = t[e * 8:(e + 1) * 8, :]
                                    part[m][r] = te if part[m][r] is None else part[m][r] + te
                    for m in range(2):
                        ra, rb_ = (jnp.sum(v, axis=0, keepdims=True) for v in part[m])
                        gu[m] = gu[m] + jnp.where(subc == 0, ra, rb_)
                g, u = _rb(gu[0]), _rb(gu[1])
                act.append(_rep(_rb(g * jax.nn.sigmoid(g)) * u, 16).astype(bf16))
            if c >= lag:
                wdc = pltpu.bitcast(wd[(c - lag) * FC // 2:(c - lag + 1) * FC // 2, :], bf16)
                d = jnp.dot(act[c - lag], wdc, preferred_element_type=f32)[0:8, :]
                y = d if y is None else y + d
        y = _rb(y)
        ya = _rb(y[0:1, :] * _wide(_rb(jax.nn.sigmoid(score_of(k1[0:1, :]))), D))
        yb = _rb(y[1:2, :] * _wide(_rb(jax.nn.sigmoid(score_of(k2[0:1, :]))), D))

        g1 = pl.multiple_of((i1s >> 4) << 4, 16)
        g2 = pl.multiple_of((i2s >> 4) << 4, 16)
        for t, g0 in enumerate((g1, g2)):
            rid = sub + g0
            x1 = acc[pl.ds(g0, 16), :]
            upd = jnp.where(rid == i1s, ya, 0.0) + jnp.where(rid == i2s, yb, 0.0)
            fix[t] = (x1 + gb * (adaln2(x1, st2_buf[pl.ds(g0, 16), :]) + upd)).astype(bf16)

        pltpu.make_async_copy(o_buf, out_hbm, sem_out.at[0]).wait()

        def cp_fix(t, g0):
            return pltpu.make_async_copy(fix.at[t], out_hbm.at[pl.ds(g0, 16), :], sem_fix.at[t])

        cp_fix(0, g1).start()

        @pl.when(g2 != g1)
        def _():
            cp_fix(1, g2).start()
            cp_fix(1, g2).wait()
        cp_fix(0, g1).wait()

    return kernel


_CFG = dict(
    G=4, T0=256, TB=1024, TL=256, MCH=256, RB=16, FC=256,
    LCA='cc80', LCB2='040g', NHB=16, NL4=8, BQ=3, LCNT='33333333332000',
    PKN=8, RV=80, WX=0, TE=127, GR=9, GP=0, LVN='a', LCV='000000100000', RLM=1, LD=2,
    LCM='00000000000o', LCP='000000000100', LCW='000000000088', LCO='000000000go0',
    LSPLIT=(96, 96, 64), FLAG=1, LKV='00233333333333', LFO='88',
)


def _build(A_x, A_k_cache, A_v_cache, A_wq, A_wo, B_w_r, B_w_gate, B_w_up, B_w_down, c, w_mod,
           **over):
    B, S, D = A_x.shape
    _, H, SK, DH = A_k_cache.shape
    F = B_w_gate.shape[1]
    assert B == 1
    cfg = dict(_CFG, **over)
    T0, TL, G = cfg["T0"], cfg["TL"], cfg["G"]
    MC = (4 * D) // H
    kernel = _make_kernel(S, D, H, DH, SK, F, cfg)
    scratch = [
        pltpu.VMEM((S, D), bf16),
        pltpu.VMEM((S // 2, D), u32),
        pltpu.VMEM((S, D), f32),
        pltpu.VMEM((S, SK), f32),
        pltpu.VMEM((S, 128), f32),
        pltpu.VMEM((TL, SK), f32),
        pltpu.VMEM((TL, 128), f32),
        pltpu.VMEM((TL, SK), f32),
        pltpu.VMEM((TL, 128), f32),
        pltpu.VMEM((TL, SK), f32),
        pltpu.VMEM((TL, 128), f32),
        pltpu.VMEM((S, 256), f32),
        pltpu.VMEM((S, 256), f32),
        pltpu.VMEM((4, S // 2, DH), u32),
        pltpu.VMEM((G, S, DH), f32),
        pltpu.VMEM((8, G * DH), f32),
        pltpu.VMEM((4, SK, DH), bf16),
        pltpu.VMEM((4, SK, DH), bf16),
        pltpu.VMEM((D, G * DH), bf16),
        pltpu.VMEM((2, 4, D, 128), bf16),
        pltpu.VMEM((4, 2, DH, D), bf16),
        pltpu.VMEM((G - 1, D, MC), bf16),
        pltpu.VMEM((2, D, D // 2), bf16),
        pltpu.VMEM((D, D), bf16),
        pltpu.VMEM((1, D), bf16),
        pltpu.VMEM((D,), bf16),
        pltpu.VMEM((4, 1, D // 4), f32),
        pltpu.VMEM((D, 128), f32),
        pltpu.VMEM((2, 8, D), f32),
        pltpu.VMEM((H, 1, MC), f32),
        pltpu.VMEM((9, 8, D), f32),
        pltpu.VMEM((F // 128, D // 2, 128), u32),
        pltpu.VMEM((F // 128, D // 2, 128), u32),
        pltpu.VMEM((F // 2, D), u32),
        pltpu.VMEM((2, max(int(max(cfg["LKV"])), 1) * 128, 128), f32),
        pltpu.VMEM((max(cfg["RV"], 8), DH), f32),
        pltpu.VMEM((max(cfg["RV"], 8) // 8, DH, 8, 128), f32),
        pltpu.VMEM((DH * (8 if cfg['WX'] else 1), D), f32),
        pltpu.VMEM((S, D), bf16),
        pltpu.VMEM((2, 8, 128), i32),
        pltpu.VMEM((2, 16, D), bf16),
        pltpu.SemaphoreType.DMA((sum(_sem_sizes(S, D, cfg)),)),
    ]
    any_spec = pl.BlockSpec(memory_space=pl.ANY)
    out = pl.pallas_call(
        kernel,
        out_shape=jax.ShapeDtypeStruct((S, D), bf16),
        in_specs=[any_spec] * 11,
        out_specs=any_spec,
        scratch_shapes=scratch,
        compiler_params=pltpu.CompilerParams(vmem_limit_bytes=126 * 1024 * 1024,
                                             disable_bounds_checks=True,
                                             disable_semaphore_checks=True),
    )(A_x.reshape(S, D), A_k_cache.reshape(H, SK, DH), A_v_cache.reshape(H, SK, DH),
      A_wq, A_wo, B_w_r, B_w_gate, B_w_up, B_w_down, c, w_mod)
    return out.reshape(B, S, D)


@jax.jit
def pallas_adaLN_cond__mha_block_cached__moe_arch_mod__prompt_kernel(
    A_x: jax.Array,
    A_k_cache: jax.Array,
    A_v_cache: jax.Array,
    A_wq: jax.Array,
    A_wo: jax.Array,
    B_x: jax.Array,
    B_w_r: jax.Array,
    B_w_gate: jax.Array,
    B_w_up: jax.Array,
    B_w_down: jax.Array,
    c: jax.Array,
    w_mod: jax.Array,
):
    del B_x
    return _build(A_x, A_k_cache, A_v_cache, A_wq, A_wo, B_w_r, B_w_gate, B_w_up, B_w_down,
                  c, w_mod)
```

```python
import jax
import jax.numpy as jnp
from jax import lax
import jax.experimental.pallas as pl
import jax.experimental.pallas.tpu as pltpu

f32 = jnp.float32
bf16 = jnp.bfloat16
u32 = jnp.uint32
i32 = jnp.int32

_NT = (((1,), (1,)), ((), ()))
_LOG2E = 1.4426950408889634
_EPS = 1e-5
_IMIN = -2 ** 31


def _rb(v):
    return v.astype(bf16).astype(f32)


def _rep(v, n):
    return v if n == 8 else jnp.tile(v, (n // 8, 1))


def _wide(v, w):
    return jnp.tile(v, (1, w // 128))


def _zero_of(v):
    bits = pltpu.bitcast(v, u32)
    return pltpu.bitcast(lax.shift_right_logical(lax.shift_right_logical(bits, jnp.uint32(31)),
                                                 jnp.uint32(1)), f32)


class _Pace:
    def __init__(self, chunks, counts):
        self.chunks = list(chunks)
        self.counts = [ch if isinstance(ch, int) else int(ch, 36) for ch in counts]
        assert sum(self.counts) == len(self.chunks), (counts, len(self.chunks))

    def done(self, res):
        n = self.counts.pop(0)
        for i in range(n):
            r0 = (i * res.shape[0] // n) // 8 * 8
            self.chunks.pop(0)(_zero_of(res[r0:r0 + 8, 0:128]))


def _mix(*plans):
    plans = [(list(ch), [c if isinstance(c, int) else int(c, 36) for c in cnt]) for ch, cnt in plans]
    for ch, cnt in plans:
        assert sum(cnt) == len(ch), (cnt, len(ch))
    fill, total = [], []
    for r in range(len(plans[0][1])):
        slots = sorted((i / cnt[r], k) for k, (_, cnt) in enumerate(plans)
                       for i in range(cnt[r]))
        fill += [plans[k][0].pop(0) for _, k in slots]
        total.append(len(slots))
    return _Pace(fill, total)


def _tiles(v):
    return [v[:, c * 128:(c + 1) * 128] for c in range(v.shape[1] // 128)]


def _fold(op, parts):
    out = parts[0]
    for p in parts[1:]:
        out = op(out, p)
    return out


def _lane_sum(v):
    return jnp.broadcast_to(jnp.sum(v, axis=-1, keepdims=True), v.shape)


def _row_stats(xf, tok=None):
    d = xf.shape[-1]
    ts = _tiles(xf)
    nt = len(ts)
    if tok is not None:
        ts = [ts[0] + tok] + ts[1:]
    mu = _fold(jnp.add, ts) * (1.0 / nt)
    m2 = _fold(jnp.add, [(t - mu) * (t - mu) for t in ts])
    mean = _lane_sum(mu) * (1.0 / 128)
    dm = mu - mean
    var = _lane_sum(m2 + (dm * dm) * float(nt)) * (1.0 / d)
    return mean, lax.rsqrt(var + _EPS)


def _sem_sizes(S, D, cfg):
    j0 = S // cfg["T0"]
    return [2, 2 * (D // cfg["MCH"]), j0, 1, 16, 4, 1, 2]


def _make_kernel(S, D, H, DH, SK, F, cfg):
    T0, TL, MCH = cfg["T0"], cfg["TL"], cfg["MCH"]
    J0 = S // T0
    JL = S // TL
    qscale = DH ** -0.5 * _LOG2E
    n_mch = D // MCH
    G = cfg["G"]
    NB = H - G
    MC = (4 * D) // H
    W = 512
    NF = F // 128
    assert 2 <= G <= 4 and D == 2 * W and MC == DH == 128 and NF <= NB

    def kernel(x_hbm, k_hbm, v_hbm, wq_hbm, wo_hbm, wr_hbm, wg_hbm, wu_hbm, wd_hbm,
               c_hbm, wmod_hbm, out_hbm,
               x_buf, h_buf, acc, s_buf, m_buf, s2_buf, m2_buf, s3_buf, m3_buf, s4_buf, m4_buf,
               st_buf, st2_buf,
               q_ring, qf_buf, bq_buf,
               kb, vb, wq0, w4, wo2, wmx, wca, wsa, c_buf, wr_buf, sc_buf, cb_buf, mod0, modr, modv,
               wg, wu, wd, xc_buf, ov_buf, obx, wof, o_buf, key_buf, fix,
               sems):

        class _Sem:
            def __init__(self, base):
                self.base = base
                self.at = self

            def __getitem__(self, i):
                return sems.at[self.base + i]

        sizes = _sem_sizes(S, D, cfg)
        offs = [sum(sizes[:i]) for i in range(len(sizes))]
        (sem_small, sem_ca, sem_x, sem_sa, sem_first, sem_head,
         sem_out, sem_fix) = (_Sem(o) for o in offs)

        def _mul(a, n):
            v = a * n
            return v if isinstance(a, int) else pl.multiple_of(v, n)

        def view(ref, j, t, n=1):
            return ref.at[pl.ds(_mul(j, t), n * t), :]

        def cp_c():
            return pltpu.make_async_copy(c_hbm, c_buf, sem_small.at[0])

        def cp_wr():
            return pltpu.make_async_copy(wr_hbm, wr_buf, sem_small.at[1])

        def cp_ca(c, i):
            return pltpu.make_async_copy(
                wmod_hbm.at[pl.ds(i * MCH, MCH), pl.ds(D + c * W, W)], view(wca.at[c], i, MCH),
                sem_ca.at[c * n_mch + i])

        def cp_sa():
            return pltpu.make_async_copy(wmod_hbm.at[:, pl.ds(0, D)], wsa, sem_sa.at[0])

        def cp_x(j):
            return pltpu.make_async_copy(view(x_hbm, j, T0), view(x_buf, j, T0), sem_x.at[j])

        def cp_wq0(c):
            return pltpu.make_async_copy(wq_hbm.at[pl.ds(c * W, W), pl.ds(0, G * DH)],
                                         view(wq0, c, W), sem_first.at[14 + c])

        def cp_k(h, sem=None):
            return pltpu.make_async_copy(k_hbm.at[h], kb.at[h & 3],
                                         sem_head.at[0] if sem is None else sem)

        def cp_v(h, sem=None):
            return pltpu.make_async_copy(v_hbm.at[h], vb.at[h & 3],
                                         sem_head.at[1] if sem is None else sem)

        def cp_wo(h, sem=None):
            return pltpu.make_async_copy(view(wo_hbm, h, DH), wo2.at[h & 3, 0],
                                         sem_head.at[2] if sem is None else sem)

        def _clamp(a, hi):
            return min(a, hi) if isinstance(a, int) else jnp.minimum(a, hi)

        def cols(ref, t):
            return ref.at[:, pl.ds(_mul(t, 128), 128)]

        def cp_wmx(p):
            return pltpu.make_async_copy(cols(wmod_hbm, p + (2 * D) // MC), wmx.at[p - NB - 1],
                                         sem_first.at[4 + p - NB])

        def start_head(h):
            f = _clamp(h, NF - 1)
            for i, src in enumerate((cols(wq_hbm, _clamp(h + G, H - 1)),
                                     cols(wmod_hbm, h + (2 * D) // MC),
                                     cols(wg_hbm, f), cols(wu_hbm, f))):
                pltpu.make_async_copy(src, w4.at[h & 1, i], sem_head.at[3]).start()
            cp_k(h + G - 1).start()
            cp_wo(h + 2).start()
            pltpu.make_async_copy(view(wd_hbm, f, 128), wo2.at[(h + 2) & 3, 1],
                                  sem_head.at[2]).start()
            cp_v(h + 2).start()

        def wait_head(h):
            pltpu.make_async_copy(w4.at[h & 1], w4.at[h & 1], sem_head.at[3]).wait()
            cp_k(h + G - 1).wait()
            pltpu.make_async_copy(wo2.at[(h + 2) & 3], wo2.at[(h + 2) & 3], sem_head.at[2]).wait()
            cp_v(h + 2).wait()

        def pack_chunks(h):
            f = _clamp(h, NF - 1)
            out = []
            for sv, dv in ((w4.at[h & 1, 2], wg.at[f]), (w4.at[h & 1, 3], wu.at[f]),
                           (wo2.at[(h + 2) & 3, 1], view(wd, f, 64))):
                n, w = sv.shape
                step = n // cfg['PKN']

                def chunk(r, sv=sv, dv=dv, step=step, w=w):
                    def fn(tok):
                        z = _rep(_wide(pltpu.bitcast(tok, u32), w), step // 2)
                        dv[r // 2:(r + step) // 2, :] = pltpu.bitcast(sv[r:r + step, :], u32) | z
                    return fn
                out += [chunk(r) for r in range(0, n, step)]
            return out

        def cp_out(j):
            return pltpu.make_async_copy(view(o_buf, j, TL), view(out_hbm, j, TL), sem_out.at[0])

        def ln1_chunks(xv, sv):
            def chunk(off):
                def f(tok=None):
                    mean, inv = _row_stats(xv[off:off + 8, :].astype(f32), tok)
                    sv[off:off + 8, 0:128] = mean
                    sv[off:off + 8, 128:256] = inv
                return f
            return [chunk(off) for off in range(0, xv.shape[0], 8)]

        def ln1_scaled(x, stat, cs, tok=None):
            w = x.shape[1]
            mean = stat[:, 0:128] if tok is None else stat[:, 0:128] + _rep(tok, x.shape[0])
            n = (x.astype(f32) - _wide(mean, w)) * _wide(stat[:, 128:256], w)
            return n * _rep(mod0[1, :, cs], x.shape[0])

        def qproj(h, wv, rec=None):
            q = None
            for c in range(D // W):
                cs = slice(c * W, (c + 1) * W)
                part = jnp.dot(pltpu.bitcast(h_buf[:, cs], bf16), wv[cs, :],
                               preferred_element_type=f32)
                q = part if q is None else q + part
                if rec is not None:
                    rec.done(part)
            q_ring[h & 3] = pltpu.bitcast((q * qscale).astype(bf16), u32)

        def q_early(g, q):
            return ((q + _rep(bq_buf[:, g * DH:(g + 1) * DH], q.shape[0])) * qscale).astype(bf16)

        def scores(h, q, sv, mv, rec=None, reload=False):
            mp = None
            for c in range(SK // W):
                cs = slice(c * W, (c + 1) * W)
                s = lax.dot_general(q, kb[h & 3, cs, :], _NT, preferred_element_type=f32)
                sv[:, cs] = s
                if rec is not None:
                    rec.done(s)
                if not reload:
                    mp = _fold(jnp.maximum, ([] if mp is None else [mp]) + _tiles(s))
            if reload:
                mp = _fold(jnp.maximum, _tiles(sv[...]))
            mv[...] = jnp.broadcast_to(jnp.max(mp, axis=-1, keepdims=True), mp.shape)

        def pv(h, sv, mv, rec=None, late=False):
            o = lp = None
            for c in range(SK // W):
                cs = slice(c * W, (c + 1) * W)
                m = mv[...]
                if c >= cfg["LD"] and sv.shape[0] == S:
                    m = m + _zero_of(lp)
                p = jnp.exp2(sv[:, cs] - _wide(m, W))
                lp = _fold(jnp.add, ([] if lp is None else [lp]) + _tiles(p))
                d = jnp.dot(p.astype(bf16), vb[h & 3, cs, :], preferred_element_type=f32)
                o = d if o is None else o + d
                if rec is not None:
                    rec.done(d)
            if late:
                lp = lp + _zero_of(o)
            l = jnp.sum(lp, axis=-1, keepdims=True)
            r = pl.reciprocal(l, approx=True)
            r = r * (2.0 - l * r)
            return (o * r).astype(bf16)

        def oproj(hos, av, xv=None, rec=None):
            for c in range(D // W):
                cs = slice(c * W, (c + 1) * W)
                a = av[:, cs]
                for h, o in hos:
                    if not isinstance(h, int):
                        a = jnp.where(h > 0, a, 0.0)
                    d = jnp.dot(o, wo2[h & 3, 0, :, cs], preferred_element_type=f32)
                    if rec is not None:
                        rec.done(d)
                    a = a + d
                if xv is not None:
                    a = xv[:, cs].astype(f32) + _rep(modv[0, :, cs], a.shape[0]) * a
                av[:, cs] = a

        RV = cfg["RV"]

        def expand_chunks(h):
            def wchunk(r):
                def f(tok):
                    wof[r:r + 8, :] = wo2[h & 3, 0, r:r + 8, :].astype(f32) + _wide(tok, D)
                return f

            lane = lax.broadcasted_iota(i32, (8, 128), 1)

            def ochunk(g, e0):
                def f(tok):
                    o = ov_buf[g * 8:(g + 1) * 8, :] + tok
                    for e in range(e0, e0 + 32):
                        obx[g, e] = _lane_sum(jnp.where(lane == e, o, 0.0))
                return f
            och = [ochunk(g, e0) for g in range(RV // 8) for e0 in range(0, DH, 32)]
            return [wchunk(r) for r in range(0, DH, 8)], och

        def vproj(h, r0, r1, wrow):
            def f(tok):
                if not wrow:
                    wrow.extend(jnp.concatenate(
                        [jnp.broadcast_to(wof[e:e + 1, t * 128:(t + 1) * 128], (8, 128))
                         for t in range(D // 128)], axis=1) for e in range(DH))
                for r in range(r0, r1, 8):
                    rows = slice(S - RV + r, S - RV + r + 8)
                    a = acc[rows, :] + _wide(tok, D)
                    for e in range(DH):
                        a = a + _wide(obx[r // 8, e], D) * wrow[e]
                        if e == cfg["TE"]:
                            tok = _zero_of(_fold(jnp.add, _tiles(a)))
                    acc[rows, :] = jnp.where(h > 0, a, 0.0)
            return f

        def matvec(wv, tok=None, step=16):
            n = wv.shape[1]
            part = None if tok is None else _wide(tok, n)
            for r in range(0, D, step):
                t = wv[r:r + step, :].astype(f32) * _wide(cb_buf[r:r + step, :], n)
                for e in range(step // 8):
                    te = t[e * 8:(e + 1) * 8, :]
                    part = te if part is None else part + te
            return _rb(jnp.sum(part, axis=0, keepdims=True))

        def mod_piece(p, tok=None):
            extra = isinstance(p, int) and p > NB
            modr[p] = matvec(wmx.at[p - NB - 1] if extra else w4.at[p & 1, 1], tok)

        def finish_mod():
            n = D // MC
            ga, sb, cb, gb = (jnp.concatenate([modr[i * n + t] for t in range(n)], axis=-1)
                              for i in range(4))
            cb1 = _rb(1.0 + cb)
            wr = wr_buf[...].astype(f32).reshape(1, D)
            a = cb1 * wr
            a0 = jnp.broadcast_to(jnp.sum(a, axis=-1, keepdims=True), (1, D))
            b0 = jnp.broadcast_to(jnp.sum(sb * wr, axis=-1, keepdims=True), (1, D))
            for i, v in enumerate((ga, sb, cb1, gb, a, gb * cb1, gb * sb, a0, b0)):
                modv[i] = jnp.broadcast_to(v, (8, D))

        def out_rows(x1, mean, inv):
            return (x1 + ((x1 - _wide(mean, D)) * (_wide(inv, D) * modv[5]) + modv[6])).astype(bf16)

        def out_chunks(j):
            x1v, sv, ov = view(acc, j, TL), view(st2_buf, j, TL), view(o_buf, j, TL)

            def chunk(off):
                def f(tok):
                    rs = slice(off, off + 8)
                    ov[rs, :] = out_rows(x1v[rs, :], sv[rs, 0:128] + tok, sv[rs, 128:256] + tok)
                return f
            return [chunk(off) for off in range(0, TL, 8)]

        def epi_chunks(j, x1v, ov, with_out=True):
            sub = lax.broadcasted_iota(i32, (8, 128), 0)
            low = (0xFFFF - j * TL) - sub
            sv = view(st2_buf, j, TL)
            st = {}

            def chunk(off):
                def f(tok=None):
                    if off == 0:
                        st["k1"], st["k2"] = key_buf[0], key_buf[1]
                    x1 = x1v[off:off + 8, :]
                    mean, inv = _row_stats(x1, tok)
                    sv[off:off + 8, 0:128] = mean
                    sv[off:off + 8, 128:256] = inv
                    xa = _tiles(x1 * modv[4])
                    if tok is not None:
                        xa[0] = xa[0] + tok
                    ra = _lane_sum(_fold(jnp.add, xa))
                    r = inv * (ra - mean * modv[7, :, 0:128]) + modv[8, :, 0:128]
                    if with_out:
                        ov[off:off + 8, :] = out_rows(x1, mean, inv)
                    bits = pltpu.bitcast(_rb(r) + 0.0, i32)
                    key = jnp.where(bits < 0, bits ^ 0x7FFF0000, bits) | (low - off)
                    st["k2"] = jnp.maximum(st["k2"], jnp.minimum(st["k1"], key))
                    st["k1"] = jnp.maximum(st["k1"], key)
                    if off + 8 == TL:
                        key_buf[0], key_buf[1] = st["k1"], st["k2"]
                return f
            return [chunk(off) for off in range(0, TL, 8)]

        cp_c().start()
        cp_x(0).start()
        for c in range(2):
            cp_wq0(c).start()
            for i in range(n_mch):
                cp_ca(c, i).start()
            if c == 0:
                for j in range(1, J0):
                    cp_x(j).start()
        cp_sa().start()
        for h in range(G - 1):
            cp_k(h, sem_first.at[1 + h]).start()
        early = []
        for h in range(2):
            early += [cp_v(h, sem_first.at[8 + 2 * h]), cp_wo(h, sem_first.at[9 + 2 * h])]
        for cp in early:
            cp.start()
        start_head(0)

        cp_c().wait()
        cf = c_buf[...].astype(f32)
        sc = _rb(cf * jax.nn.sigmoid(cf))
        for t in range(4):
            sc_buf[t] = sc[:, t * (D // 4):(t + 1) * (D // 4)]

        def cb_body(t, carry):
            view(cb_buf, t, D // 4)[...] = jnp.transpose(jnp.broadcast_to(sc_buf[t], (128, D // 4)))
            return carry
        lax.fori_loop(0, 4, cb_body, 0)
        key_buf[...] = jnp.full(key_buf.shape, _IMIN, i32)
        cp_x(0).wait()

        def st0_body(i, carry):
            for ch in ln1_chunks(view(x_buf, i, T0 // 4), view(st_buf, i, T0 // 4)):
                ch()
            return carry
        lax.fori_loop(0, 4, st0_body, 0)

        def ca_half(c, stream):
            cp_wq0(c).wait()
            if not stream:
                for i in range(n_mch):
                    cp_ca(c, i).wait()
            part = None
            for i in range(n_mch):
                if stream:
                    cp_ca(c, i).wait()
                scb = jnp.broadcast_to(sc[:, i * MCH:(i + 1) * MCH], (16, MCH)).astype(bf16)
                d = jnp.dot(scb, wca[c, i * MCH:(i + 1) * MCH, :], preferred_element_type=f32)
                part = d if part is None else part + d
            mod0[1, :, c * W:(c + 1) * W] = _rb(1.0 + _rb(part[0:8, :]))

        def q_first(r0, t, c, rec, mid=None):
            rows = pl.ds(r0, t)
            cs = slice(c * W, (c + 1) * W)
            hh = ln1_scaled(x_buf[rows, cs], st_buf[rows, :], cs).astype(bf16)
            for g in range(G):
                if mid is not None and g == mid[0]:
                    mid[1]()
                part = jnp.dot(hh, wq0[cs, g * DH:(g + 1) * DH], preferred_element_type=f32)
                qf_buf[g, rows, :] = part if c == 0 else qf_buf[g, rows, :] + part
                if rec is not None:
                    rec.done(part)

        ca_half(0, True)

        def pa_body(j, carry):
            @pl.when(j + 1 < J0)
            def _():
                cp_x(j + 1).wait()
            jn = jnp.minimum(j + 1, J0 - 1)
            rec = _Pace(ln1_chunks(view(x_buf, jn, T0), view(st_buf, jn, T0)), cfg["LCA"])
            q_first(_mul(j, T0), T0, 0, rec)
            return carry
        lax.fori_loop(0, J0, pa_body, 0)

        TB, RB = cfg["TB"], cfg["RB"]
        ca_half(1, False)

        def pb_body(j, carry):
            q_first(_mul(j, TB // 2), TB // 2, 1, None)
            return carry
        lax.fori_loop(0, 2, pb_body, 0)
        cp_sa().wait()
        cp_k(0, sem_first.at[1]).wait()
        cp_wr().start()
        for p in range(NB + 1, H):
            cp_wmx(p).start()

        def sa_chunk(t):
            def f(tok):
                cs = slice(t * 256, (t + 1) * 256)
                mod0[0, :, cs] = jnp.broadcast_to(matvec(wsa.at[:, cs], tok, 8), (8, 256))
            return f

        def sa_bias():
            bq_buf[...] = jnp.dot(_rep(mod0[0], 16).astype(bf16), wq0[...],
                                  preferred_element_type=f32)[0:8, :]

        def h_chunk(off):
            def f(tok):
                rs, rh = slice(off, off + RB), slice(off // 2, (off + RB) // 2)
                hh = (ln1_scaled(x_buf[rs, :], st_buf[rs, :], slice(0, D), tok)
                      + _rep(mod0[0], RB)).astype(bf16)
                h_buf[rh, :] = pltpu.bitcast(hh, u32)
            return f

        def q_chunk(off):
            def f(tok):
                n = 2 * RB
                rs, rh = slice(off, off + n), slice(off // 2, (off + n) // 2)
                for g in range(1, G):
                    q_ring[g, rh, :] = pltpu.bitcast(
                        q_early(g, qf_buf[g, rs, :] + _rep(tok, n)), u32)
            return f

        hs = [h_chunk(off) for off in range(0, S, RB)]
        qs = [q_chunk(off) for off in range(0, S, 2 * RB)]
        nh = cfg["NHB"]
        rest_chunks = []
        nq, nr = len(qs), len(hs) - nh
        for i, ch in enumerate(hs[nh:]):
            rest_chunks.append(ch)
            while qs and (nq - len(qs)) * nr < (i + 1) * nq:
                rest_chunks.append(qs.pop(0))
        assert not qs
        rec = _Pace([sa_chunk(t) for t in range(D // 256)] + hs[:nh], cfg["LCB2"])
        q_first(TB, S - TB, 1, rec, mid=(cfg["BQ"], sa_bias))
        n4 = len(rest_chunks)
        n3 = n4 - cfg["NL4"]
        cnt = [n3 // 3 + (1 if i < n3 % 3 else 0) for i in range(3)] + [cfg["NL4"]]
        scores(0, q_early(0, qf_buf[0]), s_buf, m_buf, rec=_Pace(rest_chunks, cnt), reload=True)

        def main_body(h, carry):
            plans = [(pack_chunks(h), cfg["LCM"])]
            if "1" in cfg["LCP"]:
                plans.append(([lambda tok: mod_piece(h, tok)], cfg["LCP"]))
            if RV:
                wch, och = expand_chunks(h)
                cuts = [0]
                for ch in cfg["LVN"]:
                    cuts.append(cuts[-1] + 8 * int(ch, 36))
                assert cuts[-1] == RV
                wrow = []
                vps = [vproj(h, a, b, wrow) for a, b in zip(cuts, cuts[1:])]
                order = [int(ch, 36) for ch in cfg["LOO"]]
                assert sorted(order) == list(range(RV // 8))
                och = [och[4 * g + i] for g in order for i in range(4)]
                plans += [(vps, cfg["LCV"]), (wch, cfg["LCW"]), (och, cfg["LCO"])]
            rec = _mix(*plans)
            o = pv(h, s_buf, m_buf, rec=rec)
            if RV:
                ov_buf[...] = o[S - RV:, :].astype(f32)
            qproj(h + G, w4.at[h & 1, 0], rec=rec)
            start_head(h + 1)
            scores(h + 1, pltpu.bitcast(q_ring[(h + 1) & 3], bf16), s_buf, m_buf, rec=rec,
                   reload=cfg["RLM"])
            oproj([(h, o[0:S - RV, :])], acc.at[0:S - RV, :], rec=rec)
            if "1" not in cfg["LCP"]:
                mod_piece(h)
            wait_head(h + 1)
            return carry
        for h in range(1, G - 1):
            cp_k(h, sem_first.at[1 + h]).wait()
        for cp in early:
            cp.wait()
        wait_head(0)
        lax.fori_loop(0, NB, main_body, 0)

        ha = NB
        rest = list(zip(range(NB + 1, H), (s2_buf, s3_buf, s4_buf), (m2_buf, m3_buf, m4_buf)))
        late = []
        for n, h in enumerate(range(NB + 3, H)):
            late += [cp_v(h, sem_first.at[8 + 2 * n]), cp_wo(h, sem_first.at[9 + 2 * n])]
        cp_wr().wait()
        for p in range(NB + 1, H):
            cp_wmx(p).wait()
        if RV:
            oproj([(NB - 1, ov_buf[...].astype(bf16))], acc.at[S - RV:, :])
        for cp in late:
            cp.start()

        def l_step(j, do_x, do_y):
            if do_x and do_y:
                aw = view(acc, j - 1, TL, 2)
                ay, ax = aw.at[0:TL, :], aw.at[TL:2 * TL, :]
            elif do_x:
                ax = view(acc, j, TL)
            else:
                ay = view(acc, j - 1, TL)
            rec = None
            if do_y:
                chunks = epi_chunks(j - 1, ay, view(o_buf, j - 1, TL), with_out=do_x)
                os_ = [(h, pv(h, sv, mv, late=not do_x)) for h, sv, mv in rest]
            if do_x:
                oa = pv(ha, view(s_buf, j, TL), view(m_buf, j, TL))
            if do_y and do_x:
                oproj(os_, ay, view(x_buf, j - 1, TL))
            elif do_y:
                xv = view(x_buf, j - 1, TL)
                r0, prev = 0, []
                for n in cfg["LSPLIT"]:
                    rs = slice(r0, r0 + n)
                    nr = len(os_) * (D // W)
                    cnt = [len(prev) // nr + (1 if i < len(prev) % nr else 0) for i in range(nr)]
                    rec = _Pace(prev, cnt)
                    oproj([(h, o[rs]) for h, o in os_], ay.at[rs, :], xv.at[rs, :], rec=rec)
                    prev = chunks[r0 // 8:(r0 + n) // 8]
                    r0 += n
                chunks = prev
            if do_x:
                if do_y:
                    rec = _Pace(chunks, cfg["LCNT"])
                for h, sv, mv in rest:
                    q = pltpu.bitcast(view(q_ring.at[h & 3], j, TL // 2)[...], bf16)
                    scores(h, q, sv, mv, rec=rec, reload=True)
                oproj([(ha, oa)], ax, rec=rec)
            if do_y:
                if do_x:
                    cp_out(j - 1).start()
                else:
                    for ch in chunks:
                        ch()

        for p in range(NB, H):
            mod_piece(p)
        finish_mod()
        l_step(0, True, False)
        for cp in late:
            cp.wait()

        def pl_body(j, carry):
            l_step(j, True, True)
            return carry
        lax.fori_loop(1, JL, pl_body, 0)
        l_step(JL, False, True)

        k1, k2 = key_buf[0], key_buf[1]
        for sh in (4, 2, 1):
            o1, o2 = pltpu.roll(k1, sh, 0), pltpu.roll(k2, sh, 0)
            k2 = jnp.maximum(jnp.minimum(k1, o1), jnp.maximum(k2, o2))
            k1 = jnp.maximum(k1, o1)

        def score_of(k):
            hi = k & jnp.int32(-65536)
            return pltpu.bitcast(jnp.where(hi < 0, hi ^ 0x7FFF0000, hi), f32)

        i1s = jnp.minimum(0xFFFF - (k1[0, 0] & 0xFFFF), S - 1)
        i2s = jnp.minimum(0xFFFF - (k2[0, 0] & 0xFFFF), S - 1)

        sub = lax.broadcasted_iota(i32, (16, D), 0)
        sb, cb1, gb = (_rep(modv[i], 16) for i in (1, 2, 3))

        def adaln2(x1, stat):
            return (x1 - _wide(stat[:, 0:128], D)) * _wide(stat[:, 128:256], D) * cb1 + sb

        def pick(ref):
            sel = lax.broadcasted_iota(i32, (16, ref.shape[1]), 0) == 0
            return jnp.where(sel, ref[pl.ds(i1s, 1), :], ref[pl.ds(i2s, 1), :])

        xs = adaln2(pick(acc), pick(st2_buf)).astype(bf16)
        FC, lag = cfg["FC"], cfg["FLAG"]
        kvs = [int(ch) for ch in cfg["LKV"]]
        fout = [int(ch, 36) for ch in cfg["LFO"]]
        KV = max(kvs)

        def wrows(ref, a, b, c):
            n = FC // 128
            u = [ref[c * n + t, a // 2:b // 2, :] for t in range(n)]
            return pltpu.bitcast(u[0] if n == 1 else jnp.concatenate(u, axis=1), bf16)

        DV = D - KV * 128
        if KV:
            xf = xs.astype(f32)
            for r in range(2):
                xc_buf[r] = jnp.transpose(jnp.broadcast_to(xf[r:r + 1, DV:], (128, D - DV)))
        subc = lax.broadcasted_iota(i32, (8, FC), 0)
        y = None
        act = []
        outs = out_chunks(JL - 1)
        for c in range(F // FC + lag):
            if c < F // FC:
                dm = D - kvs[c] * 128
                gu = [jnp.dot(xs[:, :dm], wrows(w, 0, dm, c), preferred_element_type=f32)[0:8, :]
                      for w in (wg, wu)]
                for v in gu:
                    for t in range(fout[c] if c < len(fout) else 0):
                        if outs:
                            outs.pop(0)(_zero_of(v[0:8, (t % 2) * 128:(t % 2 + 1) * 128]))
                            if not outs:
                                cp_out(JL - 1).start()
                if dm < D:
                    part = [[None, None], [None, None]]
                    for k in range(dm, D, 16):
                        xcol = [_wide(xc_buf[r, k - DV:k - DV + 16, :], FC) for r in range(2)]
                        for m, w in enumerate((wg, wu)):
                            wv = wrows(w, k, k + 16, c).astype(f32)
                            for r in range(2):
                                t = wv * xcol[r]
                                for e in range(2):
                                    te = t[e * 8:(e + 1) * 8, :]
                                    part[m][r] = te if part[m][r] is None else part[m][r] + te
                    for m in range(2):
                        ra, rb_ = (jnp.sum(v, axis=0, keepdims=True) for v in part[m])
                        gu[m] = gu[m] + jnp.where(subc == 0, ra, rb_)
                g, u = _rb(gu[0]), _rb(gu[1])
                act.append(_rep(_rb(g * jax.nn.sigmoid(g)) * u, 16).astype(bf16))
            if c >= lag:
                wdc = pltpu.bitcast(wd[(c - lag) * FC // 2:(c - lag + 1) * FC // 2, :], bf16)
                d = jnp.dot(act[c - lag], wdc, preferred_element_type=f32)[0:8, :]
                y = d if y is None else y + d
        y = _rb(y)
        ya = _rb(y[0:1, :] * _wide(_rb(jax.nn.sigmoid(score_of(k1[0:1, :]))), D))
        yb = _rb(y[1:2, :] * _wide(_rb(jax.nn.sigmoid(score_of(k2[0:1, :]))), D))

        g1 = pl.multiple_of((i1s >> 4) << 4, 16)
        g2 = pl.multiple_of((i2s >> 4) << 4, 16)
        for t, g0 in enumerate((g1, g2)):
            rid = sub + g0
            x1 = acc[pl.ds(g0, 16), :]
            upd = jnp.where(rid == i1s, ya, 0.0) + jnp.where(rid == i2s, yb, 0.0)
            fix[t] = (x1 + gb * (adaln2(x1, st2_buf[pl.ds(g0, 16), :]) + upd)).astype(bf16)

        pltpu.make_async_copy(o_buf, out_hbm, sem_out.at[0]).wait()

        def cp_fix(t, g0):
            return pltpu.make_async_copy(fix.at[t], out_hbm.at[pl.ds(g0, 16), :], sem_fix.at[t])

        cp_fix(0, g1).start()

        @pl.when(g2 != g1)
        def _():
            cp_fix(1, g2).start()
            cp_fix(1, g2).wait()
        cp_fix(0, g1).wait()

    return kernel


_CFG = dict(
    G=4, T0=256, TB=1024, TL=256, MCH=256, RB=16, FC=256, PKN=8, RV=128, TE=127, RLM=1, LD=2,
    LCA='cc80', LCB2='040g', NHB=16, NL4=8, BQ=3, LCNT='33333333332000',
    LCM='10000000000n', LCP='000000000000', LCV='000010000000', LCW='000000000088',
    LCO='000000aa80z1', LVN='g', LOO='0123456789abcdef',
    LSPLIT=(96, 96, 64), FLAG=1, LKV='00233333333333', LFO='88',
)


def _build(A_x, A_k_cache, A_v_cache, A_wq, A_wo, B_w_r, B_w_gate, B_w_up, B_w_down, c, w_mod,
           **over):
    B, S, D = A_x.shape
    _, H, SK, DH = A_k_cache.shape
    F = B_w_gate.shape[1]
    assert B == 1
    cfg = dict(_CFG, **over)
    T0, TL, G = cfg["T0"], cfg["TL"], cfg["G"]
    MC = (4 * D) // H
    kernel = _make_kernel(S, D, H, DH, SK, F, cfg)
    scratch = [
        pltpu.VMEM((S, D), bf16),
        pltpu.VMEM((S // 2, D), u32),
        pltpu.VMEM((S, D), f32),
        pltpu.VMEM((S, SK), f32),
        pltpu.VMEM((S, 128), f32),
        pltpu.VMEM((TL, SK), f32),
        pltpu.VMEM((TL, 128), f32),
        pltpu.VMEM((TL, SK), f32),
        pltpu.VMEM((TL, 128), f32),
        pltpu.VMEM((TL, SK), f32),
        pltpu.VMEM((TL, 128), f32),
        pltpu.VMEM((S, 256), f32),
        pltpu.VMEM((S, 256), f32),
        pltpu.VMEM((4, S // 2, DH), u32),
        pltpu.VMEM((G, S, DH), f32),
        pltpu.VMEM((8, G * DH), f32),
        pltpu.VMEM((4, SK, DH), bf16),
        pltpu.VMEM((4, SK, DH), bf16),
        pltpu.VMEM((D, G * DH), bf16),
        pltpu.VMEM((2, 4, D, 128), bf16),
        pltpu.VMEM((4, 2, DH, D), bf16),
        pltpu.VMEM((G - 1, D, MC), bf16),
        pltpu.VMEM((2, D, D // 2), bf16),
        pltpu.VMEM((D, D), bf16),
        pltpu.VMEM((1, D), bf16),
        pltpu.VMEM((D,), bf16),
        pltpu.VMEM((4, 1, D // 4), f32),
        pltpu.VMEM((D, 128), f32),
        pltpu.VMEM((2, 8, D), f32),
        pltpu.VMEM((H, 1, MC), f32),
        pltpu.VMEM((9, 8, D), f32),
        pltpu.VMEM((F // 128, D // 2, 128), u32),
        pltpu.VMEM((F // 128, D // 2, 128), u32),
        pltpu.VMEM((F // 2, D), u32),
        pltpu.VMEM((2, max(int(max(cfg["LKV"])), 1) * 128, 128), f32),
        pltpu.VMEM((max(cfg["RV"], 8), DH), f32),
        pltpu.VMEM((max(cfg["RV"], 8) // 8, DH, 8, 128), f32),
        pltpu.VMEM((DH, D), f32),
        pltpu.VMEM((S, D), bf16),
        pltpu.VMEM((2, 8, 128), i32),
        pltpu.VMEM((2, 16, D), bf16),
        pltpu.SemaphoreType.DMA((sum(_sem_sizes(S, D, cfg)),)),
    ]
    any_spec = pl.BlockSpec(memory_space=pl.ANY)
    out = pl.pallas_call(
        kernel,
        out_shape=jax.ShapeDtypeStruct((S, D), bf16),
        in_specs=[any_spec] * 11,
        out_specs=any_spec,
        scratch_shapes=scratch,
        compiler_params=pltpu.CompilerParams(vmem_limit_bytes=126 * 1024 * 1024,
                                             disable_bounds_checks=True,
                                             disable_semaphore_checks=True),
    )(A_x.reshape(S, D), A_k_cache.reshape(H, SK, DH), A_v_cache.reshape(H, SK, DH),
      A_wq, A_wo, B_w_r, B_w_gate, B_w_up, B_w_down, c, w_mod)
    return out.reshape(B, S, D)


@jax.jit
def pallas_adaLN_cond__mha_block_cached__moe_arch_mod__prompt_kernel(
    A_x: jax.Array,
    A_k_cache: jax.Array,
    A_v_cache: jax.Array,
    A_wq: jax.Array,
    A_wo: jax.Array,
    B_x: jax.Array,
    B_w_r: jax.Array,
    B_w_gate: jax.Array,
    B_w_up: jax.Array,
    B_w_down: jax.Array,
    c: jax.Array,
    w_mod: jax.Array,
):
    del B_x
    return _build(A_x, A_k_cache, A_v_cache, A_wq, A_wo, B_w_r, B_w_gate, B_w_up, B_w_down,
                  c, w_mod)
```

```python
import jax
import jax.numpy as jnp
from jax import lax
import jax.experimental.pallas as pl
import jax.experimental.pallas.tpu as pltpu

f32 = jnp.float32
bf16 = jnp.bfloat16
u32 = jnp.uint32
i32 = jnp.int32

_NT = (((1,), (1,)), ((), ()))
_LOG2E = 1.4426950408889634
_EPS = 1e-5
_IMIN = -2 ** 31


def _rb(v):
    return v.astype(bf16).astype(f32)


def _rep(v, n):
    return v if n == 8 else jnp.tile(v, (n // 8, 1))


def _wide(v, w):
    return jnp.tile(v, (1, w // 128))


def _zero_of(v):
    bits = pltpu.bitcast(v, u32)
    return pltpu.bitcast(lax.shift_right_logical(lax.shift_right_logical(bits, jnp.uint32(31)),
                                                 jnp.uint32(1)), f32)


class _Pace:
    def __init__(self, chunks, counts):
        self.chunks = list(chunks)
        self.counts = [ch if isinstance(ch, int) else int(ch, 36) for ch in counts]
        assert sum(self.counts) == len(self.chunks), (counts, len(self.chunks))

    def done(self, res):
        n = self.counts.pop(0)
        for i in range(n):
            r0 = (i * res.shape[0] // n) // 8 * 8
            self.chunks.pop(0)(_zero_of(res[r0:r0 + 8, 0:128]))


def _mix(*plans):
    plans = [(list(ch), [c if isinstance(c, int) else int(c, 36) for c in cnt]) for ch, cnt in plans]
    for ch, cnt in plans:
        assert sum(cnt) == len(ch), (cnt, len(ch))
    fill, total = [], []
    for r in range(len(plans[0][1])):
        slots = sorted((i / cnt[r], k) for k, (_, cnt) in enumerate(plans)
                       for i in range(cnt[r]))
        fill += [plans[k][0].pop(0) for _, k in slots]
        total.append(len(slots))
    return _Pace(fill, total)


def _tiles(v):
    return [v[:, c * 128:(c + 1) * 128] for c in range(v.shape[1] // 128)]


def _fold(op, parts):
    out = parts[0]
    for p in parts[1:]:
        out = op(out, p)
    return out


def _lane_sum(v):
    return jnp.broadcast_to(jnp.sum(v, axis=-1, keepdims=True), v.shape)


def _row_stats(xf, tok=None):
    d = xf.shape[-1]
    ts = _tiles(xf)
    nt = len(ts)
    if tok is not None:
        ts = [ts[0] + tok] + ts[1:]
    mu = _fold(jnp.add, ts) * (1.0 / nt)
    m2 = _fold(jnp.add, [(t - mu) * (t - mu) for t in ts])
    mean = _lane_sum(mu) * (1.0 / 128)
    dm = mu - mean
    var = _lane_sum(m2 + (dm * dm) * float(nt)) * (1.0 / d)
    return mean, lax.rsqrt(var + _EPS)


def _sem_sizes(S, D, cfg):
    j0 = S // cfg["T0"]
    return [2, 2 * (D // cfg["MCH"]), j0, 1, 16, 4, 1, 2]


def _make_kernel(S, D, H, DH, SK, F, cfg):
    T0, TL, MCH = cfg["T0"], cfg["TL"], cfg["MCH"]
    J0 = S // T0
    JL = S // TL
    qscale = DH ** -0.5 * _LOG2E
    n_mch = D // MCH
    G = cfg["G"]
    NB = H - G
    MC = (4 * D) // H
    W = 512
    NF = F // 128
    assert 2 <= G <= 4 and D == 2 * W and MC == DH == 128 and NF <= NB

    def kernel(x_hbm, k_hbm, v_hbm, wq_hbm, wo_hbm, wr_hbm, wg_hbm, wu_hbm, wd_hbm,
               c_hbm, wmod_hbm, out_hbm,
               x_buf, h_buf, acc, s_buf, m_buf, s2_buf, m2_buf, s3_buf, m3_buf, s4_buf, m4_buf,
               st_buf, st2_buf,
               q_ring, qf_buf, bq_buf,
               kb, vb, wq0, w4, wo2, wmx, wca, wsa, c_buf, wr_buf, sc_buf, cb_buf, mod0, modr, modv,
               wg, wu, wd, xc_buf, ov_buf, obx, wof, o_buf, key_buf, fix,
               sems):

        class _Sem:
            def __init__(self, base):
                self.base = base
                self.at = self

            def __getitem__(self, i):
                return sems.at[self.base + i]

        sizes = _sem_sizes(S, D, cfg)
        offs = [sum(sizes[:i]) for i in range(len(sizes))]
        (sem_small, sem_ca, sem_x, sem_sa, sem_first, sem_head,
         sem_out, sem_fix) = (_Sem(o) for o in offs)

        def _mul(a, n):
            v = a * n
            return v if isinstance(a, int) else pl.multiple_of(v, n)

        def view(ref, j, t, n=1):
            return ref.at[pl.ds(_mul(j, t), n * t), :]

        def cp_c():
            return pltpu.make_async_copy(c_hbm, c_buf, sem_small.at[0])

        def cp_wr():
            return pltpu.make_async_copy(wr_hbm, wr_buf, sem_small.at[1])

        def cp_ca(c, i):
            return pltpu.make_async_copy(
                wmod_hbm.at[pl.ds(i * MCH, MCH), pl.ds(D + c * W, W)], view(wca.at[c], i, MCH),
                sem_ca.at[c * n_mch + i])

        def cp_sa():
            return pltpu.make_async_copy(wmod_hbm.at[:, pl.ds(0, D)], wsa, sem_sa.at[0])

        def cp_x(j):
            return pltpu.make_async_copy(view(x_hbm, j, T0), view(x_buf, j, T0), sem_x.at[j])

        def cp_wq0(c):
            return pltpu.make_async_copy(wq_hbm.at[pl.ds(c * W, W), pl.ds(0, G * DH)],
                                         view(wq0, c, W), sem_first.at[14 + c])

        def cp_k(h, sem=None):
            return pltpu.make_async_copy(k_hbm.at[h], kb.at[h & 3],
                                         sem_head.at[0] if sem is None else sem)

        def cp_v(h, sem=None):
            return pltpu.make_async_copy(v_hbm.at[h], vb.at[h & 3],
                                         sem_head.at[1] if sem is None else sem)

        def cp_wo(h, sem=None):
            return pltpu.make_async_copy(view(wo_hbm, h, DH), wo2.at[h & 3, 0],
                                         sem_head.at[2] if sem is None else sem)

        def _clamp(a, hi):
            return min(a, hi) if isinstance(a, int) else jnp.minimum(a, hi)

        def cols(ref, t):
            return ref.at[:, pl.ds(_mul(t, 128), 128)]

        def cp_wmx(p):
            return pltpu.make_async_copy(cols(wmod_hbm, p + (2 * D) // MC), wmx.at[p - NB - 1],
                                         sem_first.at[4 + p - NB])

        def start_head(h):
            f = _clamp(h, NF - 1)
            for i, src in enumerate((cols(wq_hbm, _clamp(h + G, H - 1)),
                                     cols(wmod_hbm, h + (2 * D) // MC),
                                     cols(wg_hbm, f), cols(wu_hbm, f))):
                pltpu.make_async_copy(src, w4.at[h & 1, i], sem_head.at[3]).start()
            cp_k(h + G - 1).start()
            cp_wo(h + 2).start()
            pltpu.make_async_copy(view(wd_hbm, f, 128), wo2.at[(h + 2) & 3, 1],
                                  sem_head.at[2]).start()
            cp_v(h + 2).start()

        def wait_head(h):
            pltpu.make_async_copy(w4.at[h & 1], w4.at[h & 1], sem_head.at[3]).wait()
            cp_k(h + G - 1).wait()
            pltpu.make_async_copy(wo2.at[(h + 2) & 3], wo2.at[(h + 2) & 3], sem_head.at[2]).wait()
            cp_v(h + 2).wait()

        def pack_chunks(h):
            f = _clamp(h, NF - 1)
            out = []
            for sv, dv in ((w4.at[h & 1, 2], wg.at[f]), (w4.at[h & 1, 3], wu.at[f]),
                           (wo2.at[(h + 2) & 3, 1], view(wd, f, 64))):
                n, w = sv.shape
                step = n // cfg['PKN']

                def chunk(r, sv=sv, dv=dv, step=step, w=w):
                    def fn(tok):
                        z = _rep(_wide(pltpu.bitcast(tok, u32), w), step // 2)
                        dv[r // 2:(r + step) // 2, :] = pltpu.bitcast(sv[r:r + step, :], u32) | z
                    return fn
                out += [chunk(r) for r in range(0, n, step)]
            return out

        def cp_out(j):
            return pltpu.make_async_copy(view(o_buf, j, TL), view(out_hbm, j, TL), sem_out.at[0])

        def ln1_chunks(xv, sv):
            def chunk(off):
                def f(tok=None):
                    mean, inv = _row_stats(xv[off:off + 8, :].astype(f32), tok)
                    sv[off:off + 8, 0:128] = mean
                    sv[off:off + 8, 128:256] = inv
                return f
            return [chunk(off) for off in range(0, xv.shape[0], 8)]

        def ln1_scaled(x, stat, cs, tok=None):
            w = x.shape[1]
            mean = stat[:, 0:128] if tok is None else stat[:, 0:128] + _rep(tok, x.shape[0])
            n = (x.astype(f32) - _wide(mean, w)) * _wide(stat[:, 128:256], w)
            return n * _rep(mod0[1, :, cs], x.shape[0])

        def qproj(h, wv, rec=None):
            q = None
            for c in range(D // W):
                cs = slice(c * W, (c + 1) * W)
                part = jnp.dot(pltpu.bitcast(h_buf[:, cs], bf16), wv[cs, :],
                               preferred_element_type=f32)
                q = part if q is None else q + part
                if rec is not None:
                    rec.done(part)
            q_ring[h & 3] = pltpu.bitcast((q * qscale).astype(bf16), u32)

        def q_early(g, q):
            return ((q + _rep(bq_buf[:, g * DH:(g + 1) * DH], q.shape[0])) * qscale).astype(bf16)

        def scores(h, q, sv, mv, rec):
            for c in range(SK // W):
                cs = slice(c * W, (c + 1) * W)
                s = lax.dot_general(q, kb[h & 3, cs, :], _NT, preferred_element_type=f32)
                sv[:, cs] = s
                if rec is not None:
                    rec.done(s)
            mp = _fold(jnp.maximum, _tiles(sv[...]))
            mv[...] = jnp.broadcast_to(jnp.max(mp, axis=-1, keepdims=True), mp.shape)

        def pv(h, sv, mv, rec=None, late=False):
            o = lp = None
            for c in range(SK // W):
                cs = slice(c * W, (c + 1) * W)
                m = mv[...]
                if c >= 2 and sv.shape[0] == S:
                    m = m + _zero_of(lp)
                p = jnp.exp2(sv[:, cs] - _wide(m, W))
                lp = _fold(jnp.add, ([] if lp is None else [lp]) + _tiles(p))
                d = jnp.dot(p.astype(bf16), vb[h & 3, cs, :], preferred_element_type=f32)
                o = d if o is None else o + d
                if rec is not None:
                    rec.done(d)
            if late:
                lp = lp + _zero_of(o)
            l = jnp.sum(lp, axis=-1, keepdims=True)
            r = pl.reciprocal(l, approx=True)
            r = r * (2.0 - l * r)
            return (o * r).astype(bf16)

        def oproj(hos, av, xv=None, rec=None):
            for c in range(D // W):
                cs = slice(c * W, (c + 1) * W)
                a = av[:, cs]
                for h, o in hos:
                    if not isinstance(h, int):
                        a = jnp.where(h > 0, a, 0.0)
                    d = jnp.dot(o, wo2[h & 3, 0, :, cs], preferred_element_type=f32)
                    if rec is not None:
                        rec.done(d)
                    a = a + d
                if xv is not None:
                    a = xv[:, cs].astype(f32) + _rep(modv[0, :, cs], a.shape[0]) * a
                av[:, cs] = a

        RV = cfg["RV"]

        def expand_chunks(h):
            def wchunk(r):
                def f(tok):
                    wof[r:r + 8, :] = wo2[h & 3, 0, r:r + 8, :].astype(f32) + _wide(tok, D)
                return f

            lane = lax.broadcasted_iota(i32, (8, 128), 1)

            def ochunk(g, e0):
                def f(tok):
                    o = ov_buf[g * 8:(g + 1) * 8, :] + tok
                    cols = [jnp.where(lane == e, o, 0.0) for e in range(e0, e0 + 32)]
                    obx[g, e0 * 8:(e0 + 32) * 8, :] = _lane_sum(jnp.concatenate(cols, axis=0))
                return f
            och = [ochunk(g, e0) for g in range(RV // 8) for e0 in range(0, DH, 32)]
            return [wchunk(r) for r in range(0, DH, 8)], och

        def vproj(h):
            def f(tok):
                wrow = [jnp.concatenate(
                    [jnp.broadcast_to(wof[e:e + 1, t * 128:(t + 1) * 128], (8, 128))
                     for t in range(D // 128)], axis=1) for e in range(DH)]
                tok = _wide(tok, D)
                for g in range(RV // 8):
                    rows = slice(S - RV + g * 8, S - RV + g * 8 + 8)
                    a = acc[rows, :] + tok
                    ob = obx[g]
                    for e in range(DH):
                        a = a + _wide(ob[e * 8:(e + 1) * 8, :], D) * wrow[e]
                    tok = _zero_of(a)
                    acc[rows, :] = jnp.where(h > 0, a, 0.0)
            return f

        def matvec(wv, tok=None, step=16):
            n = wv.shape[1]
            part = None if tok is None else _wide(tok, n)
            for r in range(0, D, step):
                t = wv[r:r + step, :].astype(f32) * _wide(cb_buf[r:r + step, :], n)
                for e in range(step // 8):
                    te = t[e * 8:(e + 1) * 8, :]
                    part = te if part is None else part + te
            return _rb(jnp.sum(part, axis=0, keepdims=True))

        def mod_piece(p):
            extra = isinstance(p, int) and p > NB
            modr[p] = matvec(wmx.at[p - NB - 1] if extra else w4.at[p & 1, 1])

        def finish_mod():
            n = D // MC
            ga, sb, cb, gb = (jnp.concatenate([modr[i * n + t] for t in range(n)], axis=-1)
                              for i in range(4))
            cb1 = _rb(1.0 + cb)
            wr = wr_buf[...].astype(f32).reshape(1, D)
            a = cb1 * wr
            a0 = jnp.broadcast_to(jnp.sum(a, axis=-1, keepdims=True), (1, D))
            b0 = jnp.broadcast_to(jnp.sum(sb * wr, axis=-1, keepdims=True), (1, D))
            for i, v in enumerate((ga, sb, cb1, gb, a, gb * cb1, gb * sb, a0, b0)):
                modv[i] = jnp.broadcast_to(v, (8, D))

        def out_rows(x1, mean, inv):
            return (x1 + ((x1 - _wide(mean, D)) * (_wide(inv, D) * modv[5]) + modv[6])).astype(bf16)

        def out_chunks(j):
            x1v, sv, ov = view(acc, j, TL), view(st2_buf, j, TL), view(o_buf, j, TL)

            def chunk(off):
                def f(tok):
                    rs = slice(off, off + 8)
                    ov[rs, :] = out_rows(x1v[rs, :], sv[rs, 0:128] + tok, sv[rs, 128:256] + tok)
                return f
            return [chunk(off) for off in range(0, TL, 8)]

        def epi_chunks(j, x1v, ov, with_out=True):
            sub = lax.broadcasted_iota(i32, (8, 128), 0)
            low = (0xFFFF - j * TL) - sub
            sv = view(st2_buf, j, TL)
            st = {}

            def chunk(off):
                def f(tok=None):
                    if off == 0:
                        st["k1"], st["k2"] = key_buf[0], key_buf[1]
                    x1 = x1v[off:off + 8, :]
                    mean, inv = _row_stats(x1, tok)
                    sv[off:off + 8, 0:128] = mean
                    sv[off:off + 8, 128:256] = inv
                    xa = _tiles(x1 * modv[4])
                    if tok is not None:
                        xa[0] = xa[0] + tok
                    ra = _lane_sum(_fold(jnp.add, xa))
                    r = inv * (ra - mean * modv[7, :, 0:128]) + modv[8, :, 0:128]
                    if with_out:
                        ov[off:off + 8, :] = out_rows(x1, mean, inv)
                    bits = pltpu.bitcast(_rb(r) + 0.0, i32)
                    key = jnp.where(bits < 0, bits ^ 0x7FFF0000, bits) | (low - off)
                    st["k2"] = jnp.maximum(st["k2"], jnp.minimum(st["k1"], key))
                    st["k1"] = jnp.maximum(st["k1"], key)
                    if off + 8 == TL:
                        key_buf[0], key_buf[1] = st["k1"], st["k2"]
                return f
            return [chunk(off) for off in range(0, TL, 8)]

        cp_c().start()
        cp_x(0).start()
        for c in range(2):
            cp_wq0(c).start()
            for i in range(n_mch):
                cp_ca(c, i).start()
            if c == 0:
                for j in range(1, J0):
                    cp_x(j).start()
        cp_sa().start()
        for h in range(G - 1):
            cp_k(h, sem_first.at[1 + h]).start()
        early = []
        for h in range(2):
            early += [cp_v(h, sem_first.at[8 + 2 * h]), cp_wo(h, sem_first.at[9 + 2 * h])]
        for cp in early:
            cp.start()
        start_head(0)

        cp_c().wait()
        cf = c_buf[...].astype(f32)
        sc = _rb(cf * jax.nn.sigmoid(cf))
        for t in range(4):
            sc_buf[t] = sc[:, t * (D // 4):(t + 1) * (D // 4)]

        def cb_body(t, carry):
            view(cb_buf, t, D // 4)[...] = jnp.transpose(jnp.broadcast_to(sc_buf[t], (128, D // 4)))
            return carry
        lax.fori_loop(0, 4, cb_body, 0)
        key_buf[...] = jnp.full(key_buf.shape, _IMIN, i32)
        cp_x(0).wait()

        def st0_body(i, carry):
            for ch in ln1_chunks(view(x_buf, i, T0 // 4), view(st_buf, i, T0 // 4)):
                ch()
            return carry
        lax.fori_loop(0, 4, st0_body, 0)

        def ca_half(c, stream):
            cp_wq0(c).wait()
            if not stream:
                for i in range(n_mch):
                    cp_ca(c, i).wait()
            part = None
            for i in range(n_mch):
                if stream:
                    cp_ca(c, i).wait()
                scb = jnp.broadcast_to(sc[:, i * MCH:(i + 1) * MCH], (16, MCH)).astype(bf16)
                d = jnp.dot(scb, wca[c, i * MCH:(i + 1) * MCH, :], preferred_element_type=f32)
                part = d if part is None else part + d
            mod0[1, :, c * W:(c + 1) * W] = _rb(1.0 + _rb(part[0:8, :]))

        def q_first(r0, t, c, rec, mid=None):
            rows = pl.ds(r0, t)
            cs = slice(c * W, (c + 1) * W)
            hh = ln1_scaled(x_buf[rows, cs], st_buf[rows, :], cs).astype(bf16)
            for g in range(G):
                if mid is not None and g == mid[0]:
                    mid[1]()
                part = jnp.dot(hh, wq0[cs, g * DH:(g + 1) * DH], preferred_element_type=f32)
                qf_buf[g, rows, :] = part if c == 0 else qf_buf[g, rows, :] + part
                if rec is not None:
                    rec.done(part)

        ca_half(0, True)

        def pa_body(j, carry):
            @pl.when(j + 1 < J0)
            def _():
                cp_x(j + 1).wait()
            jn = jnp.minimum(j + 1, J0 - 1)
            rec = _Pace(ln1_chunks(view(x_buf, jn, T0), view(st_buf, jn, T0)), cfg["LCA"])
            q_first(_mul(j, T0), T0, 0, rec)
            return carry
        lax.fori_loop(0, J0, pa_body, 0)

        TB, RB = cfg["TB"], cfg["RB"]
        ca_half(1, False)

        def pb_body(j, carry):
            q_first(_mul(j, TB // 2), TB // 2, 1, None)
            return carry
        lax.fori_loop(0, 2, pb_body, 0)
        cp_sa().wait()
        cp_k(0, sem_first.at[1]).wait()
        cp_wr().start()
        for p in range(NB + 1, H):
            cp_wmx(p).start()

        def sa_chunk(t):
            def f(tok):
                cs = slice(t * 256, (t + 1) * 256)
                mod0[0, :, cs] = jnp.broadcast_to(matvec(wsa.at[:, cs], tok, 8), (8, 256))
            return f

        def sa_bias():
            bq_buf[...] = jnp.dot(_rep(mod0[0], 16).astype(bf16), wq0[...],
                                  preferred_element_type=f32)[0:8, :]

        def h_chunk(off):
            def f(tok):
                rs, rh = slice(off, off + RB), slice(off // 2, (off + RB) // 2)
                hh = (ln1_scaled(x_buf[rs, :], st_buf[rs, :], slice(0, D), tok)
                      + _rep(mod0[0], RB)).astype(bf16)
                h_buf[rh, :] = pltpu.bitcast(hh, u32)
            return f

        def q_chunk(off):
            def f(tok):
                n = 2 * RB
                rs, rh = slice(off, off + n), slice(off // 2, (off + n) // 2)
                for g in range(1, G):
                    q_ring[g, rh, :] = pltpu.bitcast(
                        q_early(g, qf_buf[g, rs, :] + _rep(tok, n)), u32)
            return f

        hs = [h_chunk(off) for off in range(0, S, RB)]
        qs = [q_chunk(off) for off in range(0, S, 2 * RB)]
        nh = cfg["NHB"]
        rest_chunks = []
        nq, nr = len(qs), len(hs) - nh
        for i, ch in enumerate(hs[nh:]):
            rest_chunks.append(ch)
            while qs and (nq - len(qs)) * nr < (i + 1) * nq:
                rest_chunks.append(qs.pop(0))
        assert not qs
        rec = _Pace([sa_chunk(t) for t in range(D // 256)] + hs[:nh], cfg["LCB2"])
        q_first(TB, S - TB, 1, rec, mid=(cfg["BQ"], sa_bias))
        n4 = len(rest_chunks)
        n3 = n4 - cfg["NL4"]
        cnt = [n3 // 3 + (1 if i < n3 % 3 else 0) for i in range(3)] + [cfg["NL4"]]
        scores(0, q_early(0, qf_buf[0]), s_buf, m_buf, rec=_Pace(rest_chunks, cnt))

        def main_body(h, carry):
            wch, och = expand_chunks(h)
            rec = _mix((pack_chunks(h), cfg["LCM"]), ([vproj(h)], cfg["LCV"]),
                       (wch, cfg["LCW"]), (och, cfg["LCO"]))
            o = pv(h, s_buf, m_buf, rec=rec)
            ov_buf[...] = o[S - RV:, :].astype(f32)
            qproj(h + G, w4.at[h & 1, 0], rec=rec)
            start_head(h + 1)
            scores(h + 1, pltpu.bitcast(q_ring[(h + 1) & 3], bf16), s_buf, m_buf, rec=rec)
            oproj([(h, o[0:S - RV, :])], acc.at[0:S - RV, :], rec=rec)
            mod_piece(h)
            wait_head(h + 1)
            return carry
        for h in range(1, G - 1):
            cp_k(h, sem_first.at[1 + h]).wait()
        for cp in early:
            cp.wait()
        wait_head(0)
        lax.fori_loop(0, NB, main_body, 0)

        ha = NB
        rest = list(zip(range(NB + 1, H), (s2_buf, s3_buf, s4_buf), (m2_buf, m3_buf, m4_buf)))
        late = []
        for n, h in enumerate(range(NB + 3, H)):
            late += [cp_v(h, sem_first.at[8 + 2 * n]), cp_wo(h, sem_first.at[9 + 2 * n])]
        cp_wr().wait()
        for p in range(NB + 1, H):
            cp_wmx(p).wait()
        oproj([(NB - 1, ov_buf[...].astype(bf16))], acc.at[S - RV:, :])
        for cp in late:
            cp.start()

        def l_step(j, do_x, do_y):
            if do_x and do_y:
                aw = view(acc, j - 1, TL, 2)
                ay, ax = aw.at[0:TL, :], aw.at[TL:2 * TL, :]
            elif do_x:
                ax = view(acc, j, TL)
            else:
                ay = view(acc, j - 1, TL)
            rec = None
            if do_y:
                chunks = epi_chunks(j - 1, ay, view(o_buf, j - 1, TL), with_out=do_x)
                os_ = [(h, pv(h, sv, mv, late=not do_x)) for h, sv, mv in rest]
            if do_x:
                oa = pv(ha, view(s_buf, j, TL), view(m_buf, j, TL))
            if do_y and do_x:
                oproj(os_, ay, view(x_buf, j - 1, TL))
            elif do_y:
                xv = view(x_buf, j - 1, TL)
                r0, prev = 0, []
                for n in cfg["LSPLIT"]:
                    rs = slice(r0, r0 + n)
                    nr = len(os_) * (D // W)
                    cnt = [len(prev) // nr + (1 if i < len(prev) % nr else 0) for i in range(nr)]
                    rec = _Pace(prev, cnt)
                    oproj([(h, o[rs]) for h, o in os_], ay.at[rs, :], xv.at[rs, :], rec=rec)
                    prev = chunks[r0 // 8:(r0 + n) // 8]
                    r0 += n
                chunks = prev
            if do_x:
                if do_y:
                    rec = _Pace(chunks, cfg["LCNT"])
                for h, sv, mv in rest:
                    q = pltpu.bitcast(view(q_ring.at[h & 3], j, TL // 2)[...], bf16)
                    scores(h, q, sv, mv, rec=rec)
                oproj([(ha, oa)], ax, rec=rec)
            if do_y:
                if do_x:
                    cp_out(j - 1).start()
                else:
                    for ch in chunks:
                        ch()

        for p in range(NB, H):
            mod_piece(p)
        finish_mod()
        l_step(0, True, False)
        for cp in late:
            cp.wait()

        def pl_body(j, carry):
            l_step(j, True, True)
            return carry
        lax.fori_loop(1, JL, pl_body, 0)
        l_step(JL, False, True)

        k1, k2 = key_buf[0], key_buf[1]
        for sh in (4, 2, 1):
            o1, o2 = pltpu.roll(k1, sh, 0), pltpu.roll(k2, sh, 0)
            k2 = jnp.maximum(jnp.minimum(k1, o1), jnp.maximum(k2, o2))
            k1 = jnp.maximum(k1, o1)

        def score_of(k):
            hi = k & jnp.int32(-65536)
            return pltpu.bitcast(jnp.where(hi < 0, hi ^ 0x7FFF0000, hi), f32)

        i1s = jnp.minimum(0xFFFF - (k1[0, 0] & 0xFFFF), S - 1)
        i2s = jnp.minimum(0xFFFF - (k2[0, 0] & 0xFFFF), S - 1)

        sub = lax.broadcasted_iota(i32, (16, D), 0)
        sb, cb1, gb = (_rep(modv[i], 16) for i in (1, 2, 3))

        def adaln2(x1, stat):
            return (x1 - _wide(stat[:, 0:128], D)) * _wide(stat[:, 128:256], D) * cb1 + sb

        def pick(ref):
            sel = lax.broadcasted_iota(i32, (16, ref.shape[1]), 0) == 0
            return jnp.where(sel, ref[pl.ds(i1s, 1), :], ref[pl.ds(i2s, 1), :])

        xs = adaln2(pick(acc), pick(st2_buf)).astype(bf16)
        FC, lag = cfg["FC"], cfg["FLAG"]
        kvs = [int(ch) for ch in cfg["LKV"]]
        fout = [int(ch, 36) for ch in cfg["LFO"]]
        KV = max(kvs)

        def wrows(ref, a, b, c):
            n = FC // 128
            u = [ref[c * n + t, a // 2:b // 2, :] for t in range(n)]
            return pltpu.bitcast(u[0] if n == 1 else jnp.concatenate(u, axis=1), bf16)

        DV = D - KV * 128
        if KV:
            xf = xs.astype(f32)
            for r in range(2):
                xc_buf[r] = jnp.transpose(jnp.broadcast_to(xf[r:r + 1, DV:], (128, D - DV)))
        subc = lax.broadcasted_iota(i32, (8, FC), 0)
        y = None
        act = []
        outs = out_chunks(JL - 1)
        for c in range(F // FC + lag):
            if c < F // FC:
                dm = D - kvs[c] * 128
                gu = [jnp.dot(xs[:, :dm], wrows(w, 0, dm, c), preferred_element_type=f32)[0:8, :]
                      for w in (wg, wu)]
                for v in gu:
                    for t in range(fout[c] if c < len(fout) else 0):
                        if outs:
                            outs.pop(0)(_zero_of(v[0:8, (t % 2) * 128:(t % 2 + 1) * 128]))
                            if not outs:
                                cp_out(JL - 1).start()
                if dm < D:
                    part = [[None, None], [None, None]]
                    for k in range(dm, D, 16):
                        xcol = [_wide(xc_buf[r, k - DV:k - DV + 16, :], FC) for r in range(2)]
                        for m, w in enumerate((wg, wu)):
                            wv = wrows(w, k, k + 16, c).astype(f32)
                            for r in range(2):
                                t = wv * xcol[r]
                                for e in range(2):
                                    te = t[e * 8:(e + 1) * 8, :]
                                    part[m][r] = te if part[m][r] is None else part[m][r] + te
                    for m in range(2):
                        ra, rb_ = (jnp.sum(v, axis=0, keepdims=True) for v in part[m])
                        gu[m] = gu[m] + jnp.where(subc == 0, ra, rb_)
                g, u = _rb(gu[0]), _rb(gu[1])
                act.append(_rep(_rb(g * jax.nn.sigmoid(g)) * u, 16).astype(bf16))
            if c >= lag:
                wdc = pltpu.bitcast(wd[(c - lag) * FC // 2:(c - lag + 1) * FC // 2, :], bf16)
                d = jnp.dot(act[c - lag], wdc, preferred_element_type=f32)[0:8, :]
                y = d if y is None else y + d
        y = _rb(y)
        ya = _rb(y[0:1, :] * _wide(_rb(jax.nn.sigmoid(score_of(k1[0:1, :]))), D))
        yb = _rb(y[1:2, :] * _wide(_rb(jax.nn.sigmoid(score_of(k2[0:1, :]))), D))

        g1 = pl.multiple_of((i1s >> 4) << 4, 16)
        g2 = pl.multiple_of((i2s >> 4) << 4, 16)
        for t, g0 in enumerate((g1, g2)):
            rid = sub + g0
            x1 = acc[pl.ds(g0, 16), :]
            upd = jnp.where(rid == i1s, ya, 0.0) + jnp.where(rid == i2s, yb, 0.0)
            fix[t] = (x1 + gb * (adaln2(x1, st2_buf[pl.ds(g0, 16), :]) + upd)).astype(bf16)

        pltpu.make_async_copy(o_buf, out_hbm, sem_out.at[0]).wait()

        def cp_fix(t, g0):
            return pltpu.make_async_copy(fix.at[t], out_hbm.at[pl.ds(g0, 16), :], sem_fix.at[t])

        cp_fix(0, g1).start()

        @pl.when(g2 != g1)
        def _():
            cp_fix(1, g2).start()
            cp_fix(1, g2).wait()
        cp_fix(0, g1).wait()

    return kernel


_CFG = dict(
    G=4, T0=256, TB=1024, TL=256, MCH=256, RB=16, FC=256, PKN=8, RV=128,
    LCA='cc80', LCB2='040g', NHB=16, NL4=8, BQ=3, LCNT='33333333332000',
    LCM='10000000000n', LCV='000010000000', LCW='000000000088', LCO='000000aa80z1',
    LSPLIT=(96, 96, 64), FLAG=1, LKV='00233333333333', LFO='88',
)


def _build(A_x, A_k_cache, A_v_cache, A_wq, A_wo, B_w_r, B_w_gate, B_w_up, B_w_down, c, w_mod,
           **over):
    B, S, D = A_x.shape
    _, H, SK, DH = A_k_cache.shape
    F = B_w_gate.shape[1]
    assert B == 1
    cfg = dict(_CFG, **over)
    T0, TL, G = cfg["T0"], cfg["TL"], cfg["G"]
    MC = (4 * D) // H
    kernel = _make_kernel(S, D, H, DH, SK, F, cfg)
    scratch = [
        pltpu.VMEM((S, D), bf16),
        pltpu.VMEM((S // 2, D), u32),
        pltpu.VMEM((S, D), f32),
        pltpu.VMEM((S, SK), f32),
        pltpu.VMEM((S, 128), f32),
        pltpu.VMEM((TL, SK), f32),
        pltpu.VMEM((TL, 128), f32),
        pltpu.VMEM((TL, SK), f32),
        pltpu.VMEM((TL, 128), f32),
        pltpu.VMEM((TL, SK), f32),
        pltpu.VMEM((TL, 128), f32),
        pltpu.VMEM((S, 256), f32),
        pltpu.VMEM((S, 256), f32),
        pltpu.VMEM((4, S // 2, DH), u32),
        pltpu.VMEM((G, S, DH), f32),
        pltpu.VMEM((8, G * DH), f32),
        pltpu.VMEM((4, SK, DH), bf16),
        pltpu.VMEM((4, SK, DH), bf16),
        pltpu.VMEM((D, G * DH), bf16),
        pltpu.VMEM((2, 4, D, 128), bf16),
        pltpu.VMEM((4, 2, DH, D), bf16),
        pltpu.VMEM((G - 1, D, MC), bf16),
        pltpu.VMEM((2, D, D // 2), bf16),
        pltpu.VMEM((D, D), bf16),
        pltpu.VMEM((1, D), bf16),
        pltpu.VMEM((D,), bf16),
        pltpu.VMEM((4, 1, D // 4), f32),
        pltpu.VMEM((D, 128), f32),
        pltpu.VMEM((2, 8, D), f32),
        pltpu.VMEM((H, 1, MC), f32),
        pltpu.VMEM((9, 8, D), f32),
        pltpu.VMEM((F // 128, D // 2, 128), u32),
        pltpu.VMEM((F // 128, D // 2, 128), u32),
        pltpu.VMEM((F // 2, D), u32),
        pltpu.VMEM((2, max(int(max(cfg["LKV"])), 1) * 128, 128), f32),
        pltpu.VMEM((cfg["RV"], DH), f32),
        pltpu.VMEM((cfg["RV"] // 8, DH * 8, 128), f32),
        pltpu.VMEM((DH, D), f32),
        pltpu.VMEM((S, D), bf16),
        pltpu.VMEM((2, 8, 128), i32),
        pltpu.VMEM((2, 16, D), bf16),
        pltpu.SemaphoreType.DMA((sum(_sem_sizes(S, D, cfg)),)),
    ]
    any_spec = pl.BlockSpec(memory_space=pl.ANY)
    out = pl.pallas_call(
        kernel,
        out_shape=jax.ShapeDtypeStruct((S, D), bf16),
        in_specs=[any_spec] * 11,
        out_specs=any_spec,
        scratch_shapes=scratch,
        compiler_params=pltpu.CompilerParams(vmem_limit_bytes=126 * 1024 * 1024,
                                             disable_bounds_checks=True,
                                             disable_semaphore_checks=True),
    )(A_x.reshape(S, D), A_k_cache.reshape(H, SK, DH), A_v_cache.reshape(H, SK, DH),
      A_wq, A_wo, B_w_r, B_w_gate, B_w_up, B_w_down, c, w_mod)
    return out.reshape(B, S, D)


@jax.jit
def pallas_adaLN_cond__mha_block_cached__moe_arch_mod__prompt_kernel(
    A_x: jax.Array,
    A_k_cache: jax.Array,
    A_v_cache: jax.Array,
    A_wq: jax.Array,
    A_wo: jax.Array,
    B_x: jax.Array,
    B_w_r: jax.Array,
    B_w_gate: jax.Array,
    B_w_up: jax.Array,
    B_w_down: jax.Array,
    c: jax.Array,
    w_mod: jax.Array,
):
    del B_x
    return _build(A_x, A_k_cache, A_v_cache, A_wq, A_wo, B_w_r, B_w_gate, B_w_up, B_w_down,
                  c, w_mod)
```

```python
import jax
import jax.numpy as jnp
from jax import lax
import jax.experimental.pallas as pl
import jax.experimental.pallas.tpu as pltpu

f32 = jnp.float32
bf16 = jnp.bfloat16
u32 = jnp.uint32
i32 = jnp.int32

_NT = (((1,), (1,)), ((), ()))
_LOG2E = 1.4426950408889634
_EPS = 1e-5
_IMIN = -2 ** 31


def _rb(v):
    return v.astype(bf16).astype(f32)


def _rep(v, n):
    return v if n == 8 else jnp.tile(v, (n // 8, 1))


def _wide(v, w):
    return jnp.tile(v, (1, w // 128))


def _zero_of(v):
    bits = pltpu.bitcast(v, u32)
    return pltpu.bitcast(lax.shift_right_logical(lax.shift_right_logical(bits, jnp.uint32(31)),
                                                 jnp.uint32(1)), f32)


class _Pace:
    def __init__(self, chunks, counts):
        self.chunks = list(chunks)
        self.counts = [ch if isinstance(ch, int) else int(ch, 36) for ch in counts]
        assert sum(self.counts) == len(self.chunks), (counts, len(self.chunks))

    def done(self, res):
        n = self.counts.pop(0)
        for i in range(n):
            r0 = (i * res.shape[0] // n) // 8 * 8
            self.chunks.pop(0)(_zero_of(res[r0:r0 + 8, 0:128]))


def _mix(*plans):
    plans = [(list(ch), [c if isinstance(c, int) else int(c, 36) for c in cnt]) for ch, cnt in plans]
    for ch, cnt in plans:
        assert sum(cnt) == len(ch), (cnt, len(ch))
    fill, total = [], []
    for r in range(len(plans[0][1])):
        slots = sorted((i / cnt[r], k) for k, (_, cnt) in enumerate(plans)
                       for i in range(cnt[r]))
        fill += [plans[k][0].pop(0) for _, k in slots]
        total.append(len(slots))
    return _Pace(fill, total)


def _tiles(v):
    return [v[:, c * 128:(c + 1) * 128] for c in range(v.shape[1] // 128)]


def _fold(op, parts):
    out = parts[0]
    for p in parts[1:]:
        out = op(out, p)
    return out


def _lane_sum(v):
    return jnp.broadcast_to(jnp.sum(v, axis=-1, keepdims=True), v.shape)


def _row_stats(xf, tok=None):
    d = xf.shape[-1]
    ts = _tiles(xf)
    nt = len(ts)
    if tok is not None:
        ts = [ts[0] + tok] + ts[1:]
    mu = _fold(jnp.add, ts) * (1.0 / nt)
    m2 = _fold(jnp.add, [(t - mu) * (t - mu) for t in ts])
    mean = _lane_sum(mu) * (1.0 / 128)
    dm = mu - mean
    var = _lane_sum(m2 + (dm * dm) * float(nt)) * (1.0 / d)
    return mean, lax.rsqrt(var + _EPS)


def _sem_sizes(S, D, cfg):
    j0 = S // cfg["T0"]
    return [2, 2 * (D // cfg["MCH"]), j0, 1, 16, 4, 1, 2]


def _make_kernel(S, D, H, DH, SK, F, cfg):
    T0, TL, MCH = cfg["T0"], cfg["TL"], cfg["MCH"]
    J0 = S // T0
    JL = S // TL
    qscale = DH ** -0.5 * _LOG2E
    n_mch = D // MCH
    G = cfg["G"]
    NB = H - G
    MC = (4 * D) // H
    W = 512
    NF = F // 128
    assert 2 <= G <= 4 and D == 2 * W and MC == DH == 128 and NF <= NB

    def kernel(x_hbm, k_hbm, v_hbm, wq_hbm, wo_hbm, wr_hbm, wg_hbm, wu_hbm, wd_hbm,
               c_hbm, wmod_hbm, out_hbm,
               x_buf, h_buf, acc, s_buf, m_buf, s2_buf, m2_buf, s3_buf, m3_buf, s4_buf, m4_buf,
               st_buf, st2_buf, mp_buf,
               q_ring, qf_buf, bq_buf,
               kb, vb, wq0, w4, wo2, wmx, wca, wsa, c_buf, wr_buf, sc_buf, cb_buf, mod0, modr, modv,
               wg, wu, wd, xc_buf, ov_buf, obx, onehot, wof, o_buf, key_buf, fix,
               sems):

        class _Sem:
            def __init__(self, base):
                self.base = base
                self.at = self

            def __getitem__(self, i):
                return sems.at[self.base + i]

        sizes = _sem_sizes(S, D, cfg)
        offs = [sum(sizes[:i]) for i in range(len(sizes))]
        (sem_small, sem_ca, sem_x, sem_sa, sem_first, sem_head,
         sem_out, sem_fix) = (_Sem(o) for o in offs)

        def _mul(a, n):
            v = a * n
            return v if isinstance(a, int) else pl.multiple_of(v, n)

        def view(ref, j, t, n=1):
            return ref.at[pl.ds(_mul(j, t), n * t), :]

        def cp_c():
            return pltpu.make_async_copy(c_hbm, c_buf, sem_small.at[0])

        def cp_wr():
            return pltpu.make_async_copy(wr_hbm, wr_buf, sem_small.at[1])

        def cp_ca(c, i):
            return pltpu.make_async_copy(
                wmod_hbm.at[pl.ds(i * MCH, MCH), pl.ds(D + c * W, W)], view(wca.at[c], i, MCH),
                sem_ca.at[c * n_mch + i])

        def cp_sa():
            return pltpu.make_async_copy(wmod_hbm.at[:, pl.ds(0, D)], wsa, sem_sa.at[0])

        def cp_x(j):
            return pltpu.make_async_copy(view(x_hbm, j, T0), view(x_buf, j, T0), sem_x.at[j])

        def cp_wq0(c):
            return pltpu.make_async_copy(wq_hbm.at[pl.ds(c * W, W), pl.ds(0, G * DH)],
                                         view(wq0, c, W), sem_first.at[14 + c])

        def cp_k(h, sem=None):
            return pltpu.make_async_copy(k_hbm.at[h], kb.at[h & 3],
                                         sem_head.at[0] if sem is None else sem)

        def cp_v(h, sem=None):
            return pltpu.make_async_copy(v_hbm.at[h], vb.at[h & 3],
                                         sem_head.at[1] if sem is None else sem)

        def cp_wo(h, sem=None):
            return pltpu.make_async_copy(view(wo_hbm, h, DH), wo2.at[h & 3, 0],
                                         sem_head.at[2] if sem is None else sem)

        def _clamp(a, hi):
            return min(a, hi) if isinstance(a, int) else jnp.minimum(a, hi)

        def cols(ref, t):
            return ref.at[:, pl.ds(_mul(t, 128), 128)]

        def cp_wmx(p):
            return pltpu.make_async_copy(cols(wmod_hbm, p + (2 * D) // MC), wmx.at[p - NB - 1],
                                         sem_first.at[4 + p - NB])

        def start_head(h):
            f = _clamp(h, NF - 1)
            for i, src in enumerate((cols(wq_hbm, _clamp(h + G, H - 1)),
                                     cols(wmod_hbm, h + (2 * D) // MC),
                                     cols(wg_hbm, f), cols(wu_hbm, f))):
                pltpu.make_async_copy(src, w4.at[h & 1, i], sem_head.at[3]).start()
            cp_k(h + G - 1).start()
            cp_wo(h + 2).start()
            pltpu.make_async_copy(view(wd_hbm, f, 128), wo2.at[(h + 2) & 3, 1],
                                  sem_head.at[2]).start()
            cp_v(h + 2).start()

        def wait_head(h):
            pltpu.make_async_copy(w4.at[h & 1], w4.at[h & 1], sem_head.at[3]).wait()
            cp_k(h + G - 1).wait()
            pltpu.make_async_copy(wo2.at[(h + 2) & 3], wo2.at[(h + 2) & 3], sem_head.at[2]).wait()
            cp_v(h + 2).wait()

        def pack_chunks(h):
            f = _clamp(h, NF - 1)
            out = []
            for sv, dv in ((w4.at[h & 1, 2], wg.at[f]), (w4.at[h & 1, 3], wu.at[f]),
                           (wo2.at[(h + 2) & 3, 1], view(wd, f, 64))):
                n, w = sv.shape
                step = n // cfg['PKN']

                def chunk(r, sv=sv, dv=dv, step=step, w=w):
                    def fn(tok):
                        z = _rep(_wide(pltpu.bitcast(tok, u32), w), step // 2)
                        dv[r // 2:(r + step) // 2, :] = pltpu.bitcast(sv[r:r + step, :], u32) | z
                    return fn
                out += [chunk(r) for r in range(0, n, step)]
            return out

        def cp_out(j):
            return pltpu.make_async_copy(view(o_buf, j, TL), view(out_hbm, j, TL), sem_out.at[0])

        def ln1_chunks(xv, sv):
            def chunk(off):
                def f(tok=None):
                    mean, inv = _row_stats(xv[off:off + 8, :].astype(f32), tok)
                    sv[off:off + 8, 0:128] = mean
                    sv[off:off + 8, 128:256] = inv
                return f
            return [chunk(off) for off in range(0, xv.shape[0], 8)]

        def ln1_scaled(x, stat, cs, tok=None):
            w = x.shape[1]
            mean = stat[:, 0:128] if tok is None else stat[:, 0:128] + _rep(tok, x.shape[0])
            n = (x.astype(f32) - _wide(mean, w)) * _wide(stat[:, 128:256], w)
            return n * _rep(mod0[1, :, cs], x.shape[0])

        def qproj(h, wv, rec=None):
            q = None
            for c in range(D // W):
                cs = slice(c * W, (c + 1) * W)
                part = jnp.dot(pltpu.bitcast(h_buf[:, cs], bf16), wv[cs, :],
                               preferred_element_type=f32)
                q = part if q is None else q + part
                if rec is not None:
                    rec.done(part)
            q_ring[h & 3] = pltpu.bitcast((q * qscale).astype(bf16), u32)

        def q_early(g, q):
            return ((q + _rep(bq_buf[:, g * DH:(g + 1) * DH], q.shape[0])) * qscale).astype(bf16)

        def scores(h, q, sv, mv, rec, mode=0):
            mps = []
            for c in range(SK // W):
                cs = slice(c * W, (c + 1) * W)
                s = lax.dot_general(q, kb[h & 3, cs, :], _NT, preferred_element_type=f32)
                if mode:
                    t = _tiles(s)
                    mp = jnp.maximum(jnp.maximum(t[0], t[1]), jnp.maximum(t[2], t[3]))
                    if mode == 2:
                        s = jnp.concatenate(t[0:3] + [t[3] + _zero_of(mp)], axis=1)
                    if mode == 3 and c < SK // W - 1:
                        z = lax.shift_right_logical(h, 8)
                        mp_buf[z, :, c * 128:(c + 1) * 128] = mp
                    else:
                        mps.append(mp)
                sv[:, cs] = s
                if rec is not None:
                    rec.done(s)
            if mode == 3:
                mps += _tiles(mp_buf[0])
            mp = _fold(jnp.maximum, mps if mode else _tiles(sv[...]))
            mv[...] = jnp.broadcast_to(jnp.max(mp, axis=-1, keepdims=True), mp.shape)

        def pv(h, sv, mv, rec=None, late=False):
            o = lp = None
            for c in range(SK // W):
                cs = slice(c * W, (c + 1) * W)
                m = mv[...]
                if c >= 2 and sv.shape[0] == S:
                    m = m + _zero_of(lp)
                p = jnp.exp2(sv[:, cs] - _wide(m, W))
                lp = _fold(jnp.add, ([] if lp is None else [lp]) + _tiles(p))
                d = jnp.dot(p.astype(bf16), vb[h & 3, cs, :], preferred_element_type=f32)
                o = d if o is None else o + d
                if rec is not None:
                    rec.done(d)
            if late:
                lp = lp + _zero_of(o)
            l = jnp.sum(lp, axis=-1, keepdims=True)
            r = pl.reciprocal(l, approx=True)
            r = r * (2.0 - l * r)
            return (o * r).astype(bf16)

        def oproj(hos, av, xv=None, rec=None):
            for c in range(D // W):
                cs = slice(c * W, (c + 1) * W)
                a = av[:, cs]
                for h, o in hos:
                    if not isinstance(h, int):
                        a = jnp.where(h > 0, a, 0.0)
                    d = jnp.dot(o, wo2[h & 3, 0, :, cs], preferred_element_type=f32)
                    if rec is not None:
                        rec.done(d)
                    a = a + d
                if xv is not None:
                    a = xv[:, cs].astype(f32) + _rep(modv[0, :, cs], a.shape[0]) * a
                av[:, cs] = a

        RV = cfg["RV"]

        def expand_chunks(h):
            def wchunk(r):
                def f(tok):
                    wof[r:r + 8, :] = wo2[h & 3, 0, r:r + 8, :].astype(f32) + _wide(tok, D)
                return f

            lane = lax.broadcasted_iota(i32, (8, 128), 1)

            def ochunk(g, e0):
                def f(tok):
                    o = ov_buf[g * 8:(g + 1) * 8, :] + tok
                    rs = slice(e0 * 8, (e0 + 32) * 8)
                    if cfg["OH"]:
                        cols = pltpu.bitcast(_rep(pltpu.bitcast(o, u32), 256) & onehot[rs, :], f32)
                    else:
                        cols = jnp.concatenate(
                            [jnp.where(lane == e, o, 0.0) for e in range(e0, e0 + 32)], axis=0)
                    obx[g, rs, :] = _lane_sum(cols)
                return f
            och = [ochunk(g, e0) for g in range(RV // 8) for e0 in range(0, DH, 32)]
            return [wchunk(r) for r in range(0, DH, 8)], och

        def vproj(h):
            def f(tok):
                wrow = [jnp.concatenate(
                    [jnp.broadcast_to(wof[e:e + 1, t * 128:(t + 1) * 128], (8, 128))
                     for t in range(D // 128)], axis=1) for e in range(DH)]
                tok = _wide(tok, D)
                for g in range(RV // 8):
                    rows = slice(S - RV + g * 8, S - RV + g * 8 + 8)
                    a = acc[rows, :] + tok
                    ob = obx[g]
                    for e in range(DH):
                        a = a + _wide(ob[e * 8:(e + 1) * 8, :], D) * wrow[e]
                    tok = _zero_of(a)
                    acc[rows, :] = jnp.where(h > 0, a, 0.0)
            return f

        def matvec(wv, tok=None, step=16):
            n = wv.shape[1]
            part = None if tok is None else _wide(tok, n)
            for r in range(0, D, step):
                t = wv[r:r + step, :].astype(f32) * _wide(cb_buf[r:r + step, :], n)
                for e in range(step // 8):
                    te = t[e * 8:(e + 1) * 8, :]
                    part = te if part is None else part + te
            return _rb(jnp.sum(part, axis=0, keepdims=True))

        def mod_piece(p):
            extra = isinstance(p, int) and p > NB
            modr[p] = matvec(wmx.at[p - NB - 1] if extra else w4.at[p & 1, 1])

        def finish_mod():
            n = D // MC
            ga, sb, cb, gb = (jnp.concatenate([modr[i * n + t] for t in range(n)], axis=-1)
                              for i in range(4))
            cb1 = _rb(1.0 + cb)
            wr = wr_buf[...].astype(f32).reshape(1, D)
            a = cb1 * wr
            a0 = jnp.broadcast_to(jnp.sum(a, axis=-1, keepdims=True), (1, D))
            b0 = jnp.broadcast_to(jnp.sum(sb * wr, axis=-1, keepdims=True), (1, D))
            for i, v in enumerate((ga, sb, cb1, gb, a, gb * cb1, gb * sb, a0, b0)):
                modv[i] = jnp.broadcast_to(v, (8, D))

        def out_rows(x1, mean, inv):
            return (x1 + ((x1 - _wide(mean, D)) * (_wide(inv, D) * modv[5]) + modv[6])).astype(bf16)

        def out_chunks(j):
            x1v, sv, ov = view(acc, j, TL), view(st2_buf, j, TL), view(o_buf, j, TL)

            def chunk(off):
                def f(tok):
                    rs = slice(off, off + 8)
                    ov[rs, :] = out_rows(x1v[rs, :], sv[rs, 0:128] + tok, sv[rs, 128:256] + tok)
                return f
            return [chunk(off) for off in range(0, TL, 8)]

        def epi_chunks(j, x1v, ov, with_out=True):
            sub = lax.broadcasted_iota(i32, (8, 128), 0)
            low = (0xFFFF - j * TL) - sub
            sv = view(st2_buf, j, TL)
            st = {}

            def chunk(off):
                def f(tok=None):
                    if off == 0:
                        st["k1"], st["k2"] = key_buf[0], key_buf[1]
                    x1 = x1v[off:off + 8, :]
                    mean, inv = _row_stats(x1, tok)
                    sv[off:off + 8, 0:128] = mean
                    sv[off:off + 8, 128:256] = inv
                    xa = _tiles(x1 * modv[4])
                    if tok is not None:
                        xa[0] = xa[0] + tok
                    ra = _lane_sum(_fold(jnp.add, xa))
                    r = inv * (ra - mean * modv[7, :, 0:128]) + modv[8, :, 0:128]
                    if with_out:
                        ov[off:off + 8, :] = out_rows(x1, mean, inv)
                    bits = pltpu.bitcast(_rb(r) + 0.0, i32)
                    key = jnp.where(bits < 0, bits ^ 0x7FFF0000, bits) | (low - off)
                    st["k2"] = jnp.maximum(st["k2"], jnp.minimum(st["k1"], key))
                    st["k1"] = jnp.maximum(st["k1"], key)
                    if off + 8 == TL:
                        key_buf[0], key_buf[1] = st["k1"], st["k2"]
                return f
            return [chunk(off) for off in range(0, TL, 8)]

        cp_c().start()
        cp_x(0).start()
        for c in range(2):
            cp_wq0(c).start()
            for i in range(n_mch):
                cp_ca(c, i).start()
            if c == 0:
                for j in range(1, J0):
                    cp_x(j).start()
        cp_sa().start()
        for h in range(G - 1):
            cp_k(h, sem_first.at[1 + h]).start()
        early = []
        for h in range(2):
            early += [cp_v(h, sem_first.at[8 + 2 * h]), cp_wo(h, sem_first.at[9 + 2 * h])]
        for cp in early:
            cp.start()
        start_head(0)

        cp_c().wait()
        cf = c_buf[...].astype(f32)
        sc = _rb(cf * jax.nn.sigmoid(cf))
        for t in range(4):
            sc_buf[t] = sc[:, t * (D // 4):(t + 1) * (D // 4)]

        def cb_body(t, carry):
            view(cb_buf, t, D // 4)[...] = jnp.transpose(jnp.broadcast_to(sc_buf[t], (128, D // 4)))
            n = DH * 2
            hit = (lax.broadcasted_iota(i32, (n, 128), 1)
                   == ((lax.broadcasted_iota(i32, (n, 128), 0) + t * n) >> 3))
            view(onehot, t, n)[...] = jnp.where(hit, jnp.uint32(0xFFFFFFFF), jnp.uint32(0))
            return carry
        lax.fori_loop(0, 4, cb_body, 0)
        key_buf[...] = jnp.full(key_buf.shape, _IMIN, i32)
        cp_x(0).wait()

        def st0_body(i, carry):
            for ch in ln1_chunks(view(x_buf, i, T0 // 4), view(st_buf, i, T0 // 4)):
                ch()
            return carry
        lax.fori_loop(0, 4, st0_body, 0)

        def ca_half(c, stream):
            cp_wq0(c).wait()
            if not stream:
                for i in range(n_mch):
                    cp_ca(c, i).wait()
            part = None
            for i in range(n_mch):
                if stream:
                    cp_ca(c, i).wait()
                scb = jnp.broadcast_to(sc[:, i * MCH:(i + 1) * MCH], (16, MCH)).astype(bf16)
                d = jnp.dot(scb, wca[c, i * MCH:(i + 1) * MCH, :], preferred_element_type=f32)
                part = d if part is None else part + d
            mod0[1, :, c * W:(c + 1) * W] = _rb(1.0 + _rb(part[0:8, :]))

        def q_first(r0, t, c, rec, mid=None):
            rows = pl.ds(r0, t)
            cs = slice(c * W, (c + 1) * W)
            hh = ln1_scaled(x_buf[rows, cs], st_buf[rows, :], cs).astype(bf16)
            for g in range(G):
                if mid is not None and g == mid[0]:
                    mid[1]()
                part = jnp.dot(hh, wq0[cs, g * DH:(g + 1) * DH], preferred_element_type=f32)
                qf_buf[g, rows, :] = part if c == 0 else qf_buf[g, rows, :] + part
                if rec is not None:
                    rec.done(part)

        ca_half(0, True)

        def pa_body(j, carry):
            @pl.when(j + 1 < J0)
            def _():
                cp_x(j + 1).wait()
            jn = jnp.minimum(j + 1, J0 - 1)
            rec = _Pace(ln1_chunks(view(x_buf, jn, T0), view(st_buf, jn, T0)), cfg["LCA"])
            q_first(_mul(j, T0), T0, 0, rec)
            return carry
        lax.fori_loop(0, J0, pa_body, 0)

        TB, RB = cfg["TB"], cfg["RB"]
        ca_half(1, False)

        def pb_body(j, carry):
            q_first(_mul(j, TB // 2), TB // 2, 1, None)
            return carry
        lax.fori_loop(0, 2, pb_body, 0)
        cp_sa().wait()
        cp_k(0, sem_first.at[1]).wait()
        cp_wr().start()
        for p in range(NB + 1, H):
            cp_wmx(p).start()

        def sa_chunk(t):
            def f(tok):
                cs = slice(t * 256, (t + 1) * 256)
                mod0[0, :, cs] = jnp.broadcast_to(matvec(wsa.at[:, cs], tok, 8), (8, 256))
            return f

        def sa_bias():
            bq_buf[...] = jnp.dot(_rep(mod0[0], 16).astype(bf16), wq0[...],
                                  preferred_element_type=f32)[0:8, :]

        def h_chunk(off):
            def f(tok):
                rs, rh = slice(off, off + RB), slice(off // 2, (off + RB) // 2)
                hh = (ln1_scaled(x_buf[rs, :], st_buf[rs, :], slice(0, D), tok)
                      + _rep(mod0[0], RB)).astype(bf16)
                h_buf[rh, :] = pltpu.bitcast(hh, u32)
            return f

        def q_chunk(off):
            def f(tok):
                n = 2 * RB
                rs, rh = slice(off, off + n), slice(off // 2, (off + n) // 2)
                for g in range(1, G):
                    q_ring[g, rh, :] = pltpu.bitcast(
                        q_early(g, qf_buf[g, rs, :] + _rep(tok, n)), u32)
            return f

        hs = [h_chunk(off) for off in range(0, S, RB)]
        qs = [q_chunk(off) for off in range(0, S, 2 * RB)]
        nh = cfg["NHB"]
        rest_chunks = []
        nq, nr = len(qs), len(hs) - nh
        for i, ch in enumerate(hs[nh:]):
            rest_chunks.append(ch)
            while qs and (nq - len(qs)) * nr < (i + 1) * nq:
                rest_chunks.append(qs.pop(0))
        assert not qs
        rec = _Pace([sa_chunk(t) for t in range(D // 256)] + hs[:nh], cfg["LCB2"])
        q_first(TB, S - TB, 1, rec, mid=(cfg["BQ"], sa_bias))
        n4 = len(rest_chunks)
        n3 = n4 - cfg["NL4"]
        cnt = [n3 // 3 + (1 if i < n3 % 3 else 0) for i in range(3)] + [cfg["NL4"]]
        scores(0, q_early(0, qf_buf[0]), s_buf, m_buf, rec=_Pace(rest_chunks, cnt))

        def main_body(h, carry):
            wch, och = expand_chunks(h)
            rec = _mix((pack_chunks(h), cfg["LCM"]), ([vproj(h)], cfg["LCV"]),
                       (wch, cfg["LCW"]), (och, cfg["LCO"]))
            o = pv(h, s_buf, m_buf, rec=rec)
            ov_buf[...] = o[S - RV:, :].astype(f32)
            qproj(h + G, w4.at[h & 1, 0], rec=rec)
            start_head(h + 1)
            scores(h + 1, pltpu.bitcast(q_ring[(h + 1) & 3], bf16), s_buf, m_buf, rec=rec,
                   mode=cfg['MX'])
            oproj([(h, o[0:S - RV, :])], acc.at[0:S - RV, :], rec=rec)
            mod_piece(h)
            wait_head(h + 1)
            return carry
        for h in range(1, G - 1):
            cp_k(h, sem_first.at[1 + h]).wait()
        for cp in early:
            cp.wait()
        wait_head(0)
        lax.fori_loop(0, NB, main_body, 0)

        ha = NB
        rest = list(zip(range(NB + 1, H), (s2_buf, s3_buf, s4_buf), (m2_buf, m3_buf, m4_buf)))
        late = []
        for n, h in enumerate(range(NB + 3, H)):
            late += [cp_v(h, sem_first.at[8 + 2 * n]), cp_wo(h, sem_first.at[9 + 2 * n])]
        cp_wr().wait()
        for p in range(NB + 1, H):
            cp_wmx(p).wait()
        oproj([(NB - 1, ov_buf[...].astype(bf16))], acc.at[S - RV:, :])
        for cp in late:
            cp.start()

        def l_step(j, do_x, do_y):
            if do_x and do_y:
                aw = view(acc, j - 1, TL, 2)
                ay, ax = aw.at[0:TL, :], aw.at[TL:2 * TL, :]
            elif do_x:
                ax = view(acc, j, TL)
            else:
                ay = view(acc, j - 1, TL)
            rec = None
            if do_y:
                chunks = epi_chunks(j - 1, ay, view(o_buf, j - 1, TL), with_out=do_x)
                os_ = [(h, pv(h, sv, mv, late=not do_x)) for h, sv, mv in rest]
            if do_x:
                oa = pv(ha, view(s_buf, j, TL), view(m_buf, j, TL))
            if do_y and do_x:
                oproj(os_, ay, view(x_buf, j - 1, TL))
            elif do_y:
                xv = view(x_buf, j - 1, TL)
                r0, prev = 0, []
                for n in cfg["LSPLIT"]:
                    rs = slice(r0, r0 + n)
                    nr = len(os_) * (D // W)
                    cnt = [len(prev) // nr + (1 if i < len(prev) % nr else 0) for i in range(nr)]
                    rec = _Pace(prev, cnt)
                    oproj([(h, o[rs]) for h, o in os_], ay.at[rs, :], xv.at[rs, :], rec=rec)
                    prev = chunks[r0 // 8:(r0 + n) // 8]
                    r0 += n
                chunks = prev
            if do_x:
                if do_y:
                    rec = _Pace(chunks, cfg["LCNT"])
                for h, sv, mv in rest:
                    q = pltpu.bitcast(view(q_ring.at[h & 3], j, TL // 2)[...], bf16)
                    scores(h, q, sv, mv, rec=rec)
                oproj([(ha, oa)], ax, rec=rec)
            if do_y:
                if do_x:
                    cp_out(j - 1).start()
                else:
                    for ch in chunks:
                        ch()

        for p in range(NB, H):
            mod_piece(p)
        finish_mod()
        l_step(0, True, False)
        for cp in late:
            cp.wait()

        def pl_body(j, carry):
            l_step(j, True, True)
            return carry
        lax.fori_loop(1, JL, pl_body, 0)
        l_step(JL, False, True)

        k1, k2 = key_buf[0], key_buf[1]
        for sh in (4, 2, 1):
            o1, o2 = pltpu.roll(k1, sh, 0), pltpu.roll(k2, sh, 0)
            k2 = jnp.maximum(jnp.minimum(k1, o1), jnp.maximum(k2, o2))
            k1 = jnp.maximum(k1, o1)

        def score_of(k):
            hi = k & jnp.int32(-65536)
            return pltpu.bitcast(jnp.where(hi < 0, hi ^ 0x7FFF0000, hi), f32)

        i1s = jnp.minimum(0xFFFF - (k1[0, 0] & 0xFFFF), S - 1)
        i2s = jnp.minimum(0xFFFF - (k2[0, 0] & 0xFFFF), S - 1)

        sub = lax.broadcasted_iota(i32, (16, D), 0)
        sb, cb1, gb = (_rep(modv[i], 16) for i in (1, 2, 3))

        def adaln2(x1, stat):
            return (x1 - _wide(stat[:, 0:128], D)) * _wide(stat[:, 128:256], D) * cb1 + sb

        def pick(ref):
            sel = lax.broadcasted_iota(i32, (16, ref.shape[1]), 0) == 0
            return jnp.where(sel, ref[pl.ds(i1s, 1), :], ref[pl.ds(i2s, 1), :])

        xs = adaln2(pick(acc), pick(st2_buf)).astype(bf16)
        FC, lag = cfg["FC"], cfg["FLAG"]
        kvs = [int(ch) for ch in cfg["LKV"]]
        fout = [int(ch, 36) for ch in cfg["LFO"]]
        KV = max(kvs)

        def wrows(ref, a, b, c):
            n = FC // 128
            u = [ref[c * n + t, a // 2:b // 2, :] for t in range(n)]
            return pltpu.bitcast(u[0] if n == 1 else jnp.concatenate(u, axis=1), bf16)

        DV = D - KV * 128
        if KV:
            xf = xs.astype(f32)
            for r in range(2):
                xc_buf[r] = jnp.transpose(jnp.broadcast_to(xf[r:r + 1, DV:], (128, D - DV)))
        subc = lax.broadcasted_iota(i32, (8, FC), 0)
        y = None
        act = []
        outs = out_chunks(JL - 1)
        for c in range(F // FC + lag):
            if c < F // FC:
                dm = D - kvs[c] * 128
                gu = [jnp.dot(xs[:, :dm], wrows(w, 0, dm, c), preferred_element_type=f32)[0:8, :]
                      for w in (wg, wu)]
                for v in gu:
                    for t in range(fout[c] if c < len(fout) else 0):
                        if outs:
                            outs.pop(0)(_zero_of(v[0:8, (t % 2) * 128:(t % 2 + 1) * 128]))
                            if not outs:
                                cp_out(JL - 1).start()
                if dm < D:
                    part = [[None, None], [None, None]]
                    for k in range(dm, D, 16):
                        xcol = [_wide(xc_buf[r, k - DV:k - DV + 16, :], FC) for r in range(2)]
                        for m, w in enumerate((wg, wu)):
                            wv = wrows(w, k, k + 16, c).astype(f32)
                            for r in range(2):
                                t = wv * xcol[r]
                                for e in range(2):
                                    te = t[e * 8:(e + 1) * 8, :]
                                    part[m][r] = te if part[m][r] is None else part[m][r] + te
                    for m in range(2):
                        ra, rb_ = (jnp.sum(v, axis=0, keepdims=True) for v in part[m])
                        gu[m] = gu[m] + jnp.where(subc == 0, ra, rb_)
                g, u = _rb(gu[0]), _rb(gu[1])
                act.append(_rep(_rb(g * jax.nn.sigmoid(g)) * u, 16).astype(bf16))
            if c >= lag:
                wdc = pltpu.bitcast(wd[(c - lag) * FC // 2:(c - lag + 1) * FC // 2, :], bf16)
                d = jnp.dot(act[c - lag], wdc, preferred_element_type=f32)[0:8, :]
                y = d if y is None else y + d
        y = _rb(y)
        ya = _rb(y[0:1, :] * _wide(_rb(jax.nn.sigmoid(score_of(k1[0:1, :]))), D))
        yb = _rb(y[1:2, :] * _wide(_rb(jax.nn.sigmoid(score_of(k2[0:1, :]))), D))

        g1 = pl.multiple_of((i1s >> 4) << 4, 16)
        g2 = pl.multiple_of((i2s >> 4) << 4, 16)
        for t, g0 in enumerate((g1, g2)):
            rid = sub + g0
            x1 = acc[pl.ds(g0, 16), :]
            upd = jnp.where(rid == i1s, ya, 0.0) + jnp.where(rid == i2s, yb, 0.0)
            fix[t] = (x1 + gb * (adaln2(x1, st2_buf[pl.ds(g0, 16), :]) + upd)).astype(bf16)

        pltpu.make_async_copy(o_buf, out_hbm, sem_out.at[0]).wait()

        def cp_fix(t, g0):
            return pltpu.make_async_copy(fix.at[t], out_hbm.at[pl.ds(g0, 16), :], sem_fix.at[t])

        cp_fix(0, g1).start()

        @pl.when(g2 != g1)
        def _():
            cp_fix(1, g2).start()
            cp_fix(1, g2).wait()
        cp_fix(0, g1).wait()

    return kernel


_CFG = dict(
    G=4, T0=256, TB=1024, TL=256, MCH=256, RB=16, FC=256, PKN=8, RV=144, MX=3, OH=0,
    LCA='cc80', LCB2='040g', NHB=16, NL4=8, BQ=3, LCNT='33333333332000',
    LCM='10000000000n', LCV='000010000000', LCW='000000000088', LCO='000000ccc0z1',
    LSPLIT=(96, 96, 64), FLAG=1, LKV='00233333333333', LFO='88',
)


def _build(A_x, A_k_cache, A_v_cache, A_wq, A_wo, B_w_r, B_w_gate, B_w_up, B_w_down, c, w_mod,
           **over):
    B, S, D = A_x.shape
    _, H, SK, DH = A_k_cache.shape
    F = B_w_gate.shape[1]
    assert B == 1
    cfg = dict(_CFG, **over)
    T0, TL, G = cfg["T0"], cfg["TL"], cfg["G"]
    MC = (4 * D) // H
    kernel = _make_kernel(S, D, H, DH, SK, F, cfg)
    scratch = [
        pltpu.VMEM((S, D), bf16),
        pltpu.VMEM((S // 2, D), u32),
        pltpu.VMEM((S, D), f32),
        pltpu.VMEM((S, SK), f32),
        pltpu.VMEM((S, 128), f32),
        pltpu.VMEM((TL, SK), f32),
        pltpu.VMEM((TL, 128), f32),
        pltpu.VMEM((TL, SK), f32),
        pltpu.VMEM((TL, 128), f32),
        pltpu.VMEM((TL, SK), f32),
        pltpu.VMEM((TL, 128), f32),
        pltpu.VMEM((S, 256), f32),
        pltpu.VMEM((S, 256), f32),
        pltpu.VMEM((1, S, 384), f32),
        pltpu.VMEM((4, S // 2, DH), u32),
        pltpu.VMEM((G, S, DH), f32),
        pltpu.VMEM((8, G * DH), f32),
        pltpu.VMEM((4, SK, DH), bf16),
        pltpu.VMEM((4, SK, DH), bf16),
        pltpu.VMEM((D, G * DH), bf16),
        pltpu.VMEM((2, 4, D, 128), bf16),
        pltpu.VMEM((4, 2, DH, D), bf16),
        pltpu.VMEM((G - 1, D, MC), bf16),
        pltpu.VMEM((2, D, D // 2), bf16),
        pltpu.VMEM((D, D), bf16),
        pltpu.VMEM((1, D), bf16),
        pltpu.VMEM((D,), bf16),
        pltpu.VMEM((4, 1, D // 4), f32),
        pltpu.VMEM((D, 128), f32),
        pltpu.VMEM((2, 8, D), f32),
        pltpu.VMEM((H, 1, MC), f32),
        pltpu.VMEM((9, 8, D), f32),
        pltpu.VMEM((F // 128, D // 2, 128), u32),
        pltpu.VMEM((F // 128, D // 2, 128), u32),
        pltpu.VMEM((F // 2, D), u32),
        pltpu.VMEM((2, max(int(max(cfg["LKV"])), 1) * 128, 128), f32),
        pltpu.VMEM((cfg["RV"], DH), f32),
        pltpu.VMEM((cfg["RV"] // 8, DH * 8, 128), f32),
        pltpu.VMEM((DH * 8, 128), u32),
        pltpu.VMEM((DH, D), f32),
        pltpu.VMEM((S, D), bf16),
        pltpu.VMEM((2, 8, 128), i32),
        pltpu.VMEM((2, 16, D), bf16),
        pltpu.SemaphoreType.DMA((sum(_sem_sizes(S, D, cfg)),)),
    ]
    any_spec = pl.BlockSpec(memory_space=pl.ANY)
    out = pl.pallas_call(
        kernel,
        out_shape=jax.ShapeDtypeStruct((S, D), bf16),
        in_specs=[any_spec] * 11,
        out_specs=any_spec,
        scratch_shapes=scratch,
        compiler_params=pltpu.CompilerParams(vmem_limit_bytes=126 * 1024 * 1024,
                                             disable_bounds_checks=True,
                                             disable_semaphore_checks=True),
    )(A_x.reshape(S, D), A_k_cache.reshape(H, SK, DH), A_v_cache.reshape(H, SK, DH),
      A_wq, A_wo, B_w_r, B_w_gate, B_w_up, B_w_down, c, w_mod)
    return out.reshape(B, S, D)


@jax.jit
def pallas_adaLN_cond__mha_block_cached__moe_arch_mod__prompt_kernel(
    A_x: jax.Array,
    A_k_cache: jax.Array,
    A_v_cache: jax.Array,
    A_wq: jax.Array,
    A_wo: jax.Array,
    B_x: jax.Array,
    B_w_r: jax.Array,
    B_w_gate: jax.Array,
    B_w_up: jax.Array,
    B_w_down: jax.Array,
    c: jax.Array,
    w_mod: jax.Array,
):
    del B_x
    return _build(A_x, A_k_cache, A_v_cache, A_wq, A_wo, B_w_r, B_w_gate, B_w_up, B_w_down,
                  c, w_mod)
```

```python
import jax
import jax.numpy as jnp
from jax import lax
import jax.experimental.pallas as pl
import jax.experimental.pallas.tpu as pltpu

f32 = jnp.float32
bf16 = jnp.bfloat16
u32 = jnp.uint32
i32 = jnp.int32

_NT = (((1,), (1,)), ((), ()))
_LOG2E = 1.4426950408889634
_EPS = 1e-5
_IMIN = -2 ** 31


def _rb(v):
    return v.astype(bf16).astype(f32)


def _rep(v, n):
    return v if n == 8 else jnp.tile(v, (n // 8, 1))


def _wide(v, w):
    return jnp.tile(v, (1, w // 128))


def _zero_of(v):
    bits = pltpu.bitcast(v, u32)
    return pltpu.bitcast(lax.shift_right_logical(lax.shift_right_logical(bits, jnp.uint32(31)),
                                                 jnp.uint32(1)), f32)


class _Pace:
    def __init__(self, chunks, counts):
        self.chunks = list(chunks)
        self.counts = [ch if isinstance(ch, int) else int(ch, 36) for ch in counts]
        assert sum(self.counts) == len(self.chunks), (counts, len(self.chunks))

    def done(self, res):
        n = self.counts.pop(0)
        for i in range(n):
            r0 = (i * res.shape[0] // n) // 8 * 8
            self.chunks.pop(0)(_zero_of(res[r0:r0 + 8, 0:128]))


def _mix(*plans):
    plans = [(list(ch), [c if isinstance(c, int) else int(c, 36) for c in cnt]) for ch, cnt in plans]
    for ch, cnt in plans:
        assert sum(cnt) == len(ch), (cnt, len(ch))
    fill, total = [], []
    for r in range(len(plans[0][1])):
        slots = sorted((i / cnt[r], k) for k, (_, cnt) in enumerate(plans)
                       for i in range(cnt[r]))
        fill += [plans[k][0].pop(0) for _, k in slots]
        total.append(len(slots))
    return _Pace(fill, total)


def _tiles(v):
    return [v[:, c * 128:(c + 1) * 128] for c in range(v.shape[1] // 128)]


def _fold(op, parts):
    out = parts[0]
    for p in parts[1:]:
        out = op(out, p)
    return out


def _lane_sum(v):
    return jnp.broadcast_to(jnp.sum(v, axis=-1, keepdims=True), v.shape)


def _row_stats(xf, tok=None):
    d = xf.shape[-1]
    ts = _tiles(xf)
    nt = len(ts)
    if tok is not None:
        ts = [ts[0] + tok] + ts[1:]
    mu = _fold(jnp.add, ts) * (1.0 / nt)
    m2 = _fold(jnp.add, [(t - mu) * (t - mu) for t in ts])
    mean = _lane_sum(mu) * (1.0 / 128)
    dm = mu - mean
    var = _lane_sum(m2 + (dm * dm) * float(nt)) * (1.0 / d)
    return mean, lax.rsqrt(var + _EPS)


def _sem_sizes(S, D, cfg):
    j0 = S // cfg["T0"]
    return [2, 2 * (D // cfg["MCH"]), j0, 1, 16, 4, 1, 2]


def _make_kernel(S, D, H, DH, SK, F, cfg):
    T0, TL, MCH = cfg["T0"], cfg["TL"], cfg["MCH"]
    J0 = S // T0
    JL = S // TL
    qscale = DH ** -0.5 * _LOG2E
    n_mch = D // MCH
    G = cfg["G"]
    NB = H - G
    MC = (4 * D) // H
    W = 512
    NF = F // 128
    assert 2 <= G <= 4 and D == 2 * W and MC == DH == 128 and NF <= NB

    def kernel(x_hbm, k_hbm, v_hbm, wq_hbm, wo_hbm, wr_hbm, wg_hbm, wu_hbm, wd_hbm,
               c_hbm, wmod_hbm, out_hbm,
               x_buf, h_buf, acc, s_buf, m_buf, s2_buf, m2_buf, s3_buf, m3_buf, s4_buf, m4_buf,
               st_buf, st2_buf, mp_buf,
               q_ring, qf_buf, bq_buf,
               kb, vb, wq0, w4, wo2, wmx, wca, wsa, c_buf, wr_buf, sc_buf, cb_buf, mod0, modr, modv,
               wg, wu, wd, xc_buf, ov_buf, obx, wof, o_buf, key_buf, fix,
               sems):

        class _Sem:
            def __init__(self, base):
                self.base = base
                self.at = self

            def __getitem__(self, i):
                return sems.at[self.base + i]

        sizes = _sem_sizes(S, D, cfg)
        offs = [sum(sizes[:i]) for i in range(len(sizes))]
        (sem_small, sem_ca, sem_x, sem_sa, sem_first, sem_head,
         sem_out, sem_fix) = (_Sem(o) for o in offs)

        def _mul(a, n):
            v = a * n
            return v if isinstance(a, int) else pl.multiple_of(v, n)

        def view(ref, j, t, n=1):
            return ref.at[pl.ds(_mul(j, t), n * t), :]

        def cp_c():
            return pltpu.make_async_copy(c_hbm, c_buf, sem_small.at[0])

        def cp_wr():
            return pltpu.make_async_copy(wr_hbm, wr_buf, sem_small.at[1])

        def cp_ca(c, i):
            return pltpu.make_async_copy(
                wmod_hbm.at[pl.ds(i * MCH, MCH), pl.ds(D + c * W, W)], view(wca.at[c], i, MCH),
                sem_ca.at[c * n_mch + i])

        def cp_sa():
            return pltpu.make_async_copy(wmod_hbm.at[:, pl.ds(0, D)], wsa, sem_sa.at[0])

        def cp_x(j):
            return pltpu.make_async_copy(view(x_hbm, j, T0), view(x_buf, j, T0), sem_x.at[j])

        def cp_wq0(c):
            return pltpu.make_async_copy(wq_hbm.at[pl.ds(c * W, W), pl.ds(0, G * DH)],
                                         view(wq0, c, W), sem_first.at[14 + c])

        def cp_k(h, sem=None):
            return pltpu.make_async_copy(k_hbm.at[h], kb.at[h & 3],
                                         sem_head.at[0] if sem is None else sem)

        def cp_v(h, sem=None):
            return pltpu.make_async_copy(v_hbm.at[h], vb.at[h & 3],
                                         sem_head.at[1] if sem is None else sem)

        def cp_wo(h, sem=None):
            return pltpu.make_async_copy(view(wo_hbm, h, DH), wo2.at[h & 3, 0],
                                         sem_head.at[2] if sem is None else sem)

        def _clamp(a, hi):
            return min(a, hi) if isinstance(a, int) else jnp.minimum(a, hi)

        def cols(ref, t):
            return ref.at[:, pl.ds(_mul(t, 128), 128)]

        def cp_wmx(p):
            return pltpu.make_async_copy(cols(wmod_hbm, p + (2 * D) // MC), wmx.at[p - NB - 1],
                                         sem_first.at[4 + p - NB])

        def start_head(h):
            f = _clamp(h, NF - 1)
            for i, src in enumerate((cols(wq_hbm, _clamp(h + G, H - 1)),
                                     cols(wmod_hbm, h + (2 * D) // MC),
                                     cols(wg_hbm, f), cols(wu_hbm, f))):
                pltpu.make_async_copy(src, w4.at[h & 1, i], sem_head.at[3]).start()
            cp_k(h + G - 1).start()
            cp_wo(h + 2).start()
            pltpu.make_async_copy(view(wd_hbm, f, 128), wo2.at[(h + 2) & 3, 1],
                                  sem_head.at[2]).start()
            cp_v(h + 2).start()

        def wait_head(h):
            pltpu.make_async_copy(w4.at[h & 1], w4.at[h & 1], sem_head.at[3]).wait()
            cp_k(h + G - 1).wait()
            pltpu.make_async_copy(wo2.at[(h + 2) & 3], wo2.at[(h + 2) & 3], sem_head.at[2]).wait()
            cp_v(h + 2).wait()

        def pack_chunks(h):
            f = _clamp(h, NF - 1)
            out = []
            for sv, dv in ((w4.at[h & 1, 2], wg.at[f]), (w4.at[h & 1, 3], wu.at[f]),
                           (wo2.at[(h + 2) & 3, 1], view(wd, f, 64))):
                n, w = sv.shape
                step = n // cfg['PKN']

                def chunk(r, sv=sv, dv=dv, step=step, w=w):
                    def fn(tok):
                        z = _rep(_wide(pltpu.bitcast(tok, u32), w), step // 2)
                        dv[r // 2:(r + step) // 2, :] = pltpu.bitcast(sv[r:r + step, :], u32) | z
                    return fn
                out += [chunk(r) for r in range(0, n, step)]
            return out

        def cp_out(j):
            return pltpu.make_async_copy(view(o_buf, j, TL), view(out_hbm, j, TL), sem_out.at[0])

        def ln1_chunks(j, t):
            xv, sv, av = view(x_buf, j, t), view(st_buf, j, t), view(acc, j, t)

            def chunk(off):
                def f(tok=None):
                    av[off:off + 8, :] = jnp.zeros((8, D), f32) if tok is None else _wide(tok, D)
                    mean, inv = _row_stats(xv[off:off + 8, :].astype(f32), tok)
                    sv[off:off + 8, 0:128] = mean
                    sv[off:off + 8, 128:256] = inv
                return f
            return [chunk(off) for off in range(0, xv.shape[0], 8)]

        def ln1_scaled(x, stat, cs, tok=None):
            w = x.shape[1]
            mean = stat[:, 0:128] if tok is None else stat[:, 0:128] + _rep(tok, x.shape[0])
            n = (x.astype(f32) - _wide(mean, w)) * _wide(stat[:, 128:256], w)
            return n * _rep(mod0[1, :, cs], x.shape[0])

        def qproj(h, wv, rec=None):
            q = None
            for c in range(D // W):
                cs = slice(c * W, (c + 1) * W)
                part = jnp.dot(pltpu.bitcast(h_buf[:, cs], bf16), wv[cs, :],
                               preferred_element_type=f32)
                q = part if q is None else q + part
                if rec is not None:
                    rec.done(part)
            q_ring[h & 3] = pltpu.bitcast((q * qscale).astype(bf16), u32)

        def q_early(g, q):
            return ((q + _rep(bq_buf[:, g * DH:(g + 1) * DH], q.shape[0])) * qscale).astype(bf16)

        def scores(h, q, sv, mv, rec, mode=0):
            mps = []
            for c in range(SK // W):
                cs = slice(c * W, (c + 1) * W)
                s = lax.dot_general(q, kb[h & 3, cs, :], _NT, preferred_element_type=f32)
                if mode:
                    t = _tiles(s)
                    mp = jnp.maximum(jnp.maximum(t[0], t[1]), jnp.maximum(t[2], t[3]))
                    if mode == 2:
                        s = jnp.concatenate(t[0:3] + [t[3] + _zero_of(mp)], axis=1)
                    if mode == 3 and c < SK // W - 1:
                        z = lax.shift_right_logical(h, 8)
                        mp_buf[z, :, c * 128:(c + 1) * 128] = mp
                    else:
                        mps.append(mp)
                sv[:, cs] = s
                if rec is not None:
                    rec.done(s)
            if mode == 3:
                mps += _tiles(mp_buf[0])
            mp = _fold(jnp.maximum, mps if mode else _tiles(sv[...]))
            mv[...] = jnp.broadcast_to(jnp.max(mp, axis=-1, keepdims=True), mp.shape)

        def pv(h, sv, mv, rec=None, late=False):
            o = lp = None
            for c in range(SK // W):
                cs = slice(c * W, (c + 1) * W)
                m = mv[...]
                if c >= 2 and sv.shape[0] == S:
                    m = m + _zero_of(lp)
                p = jnp.exp2(sv[:, cs] - _wide(m, W))
                lp = _fold(jnp.add, ([] if lp is None else [lp]) + _tiles(p))
                d = jnp.dot(p.astype(bf16), vb[h & 3, cs, :], preferred_element_type=f32)
                o = d if o is None else o + d
                if rec is not None:
                    rec.done(d)
            if late:
                lp = lp + _zero_of(o)
            l = jnp.sum(lp, axis=-1, keepdims=True)
            r = pl.reciprocal(l, approx=True)
            r = r * (2.0 - l * r)
            return (o * r).astype(bf16)

        def oproj(hos, av, xv=None, rec=None):
            for c in range(D // W):
                cs = slice(c * W, (c + 1) * W)
                a = av[:, cs]
                for h, o in hos:
                    d = jnp.dot(o, wo2[h & 3, 0, :, cs], preferred_element_type=f32)
                    if rec is not None:
                        rec.done(d)
                    a = a + d
                if xv is not None:
                    a = xv[:, cs].astype(f32) + _rep(modv[0, :, cs], a.shape[0]) * a
                av[:, cs] = a

        RV = cfg["RV"]

        def expand_chunks(h):
            def wchunk(r):
                def f(tok):
                    wof[r:r + 8, :] = wo2[h & 3, 0, r:r + 8, :].astype(f32) + _wide(tok, D)
                return f

            lane = lax.broadcasted_iota(i32, (8, 128), 1)

            def ochunk(g, e0):
                def f(tok):
                    o = ov_buf[g * 8:(g + 1) * 8, :] + tok
                    rs = slice(e0 * 8, (e0 + 32) * 8)
                    cols = jnp.concatenate(
                        [jnp.where(lane == e, o, 0.0) for e in range(e0, e0 + 32)], axis=0)
                    obx[g, rs, :] = _lane_sum(cols)
                return f
            och = [ochunk(g, e0) for g in range(RV // 8) for e0 in range(0, DH, 32)]
            return [wchunk(r) for r in range(0, DH, 8)], och

        def vproj(h):
            def f(tok):
                wrow = [jnp.concatenate(
                    [jnp.broadcast_to(wof[e:e + 1, t * 128:(t + 1) * 128], (8, 128))
                     for t in range(D // 128)], axis=1) for e in range(DH)]
                tok = _wide(tok, D)
                for g in range(RV // 8):
                    rows = slice(S - RV + g * 8, S - RV + g * 8 + 8)
                    a = acc[rows, :] + tok
                    ob = obx[g]
                    for e in range(DH):
                        a = a + _wide(ob[e * 8:(e + 1) * 8, :], D) * wrow[e]
                    tok = _zero_of(a)
                    acc[rows, :] = jnp.where(h > 0, a, 0.0)
            return f

        def matvec(wv, tok=None, step=16):
            n = wv.shape[1]
            part = None if tok is None else _wide(tok, n)
            for r in range(0, D, step):
                t = wv[r:r + step, :].astype(f32) * _wide(cb_buf[r:r + step, :], n)
                for e in range(step // 8):
                    te = t[e * 8:(e + 1) * 8, :]
                    part = te if part is None else part + te
            return _rb(jnp.sum(part, axis=0, keepdims=True))

        def mod_piece(p):
            extra = isinstance(p, int) and p > NB
            modr[p] = matvec(wmx.at[p - NB - 1] if extra else w4.at[p & 1, 1])

        def finish_mod():
            n = D // MC
            ga, sb, cb, gb = (jnp.concatenate([modr[i * n + t] for t in range(n)], axis=-1)
                              for i in range(4))
            cb1 = _rb(1.0 + cb)
            wr = wr_buf[...].astype(f32).reshape(1, D)
            a = cb1 * wr
            a0 = jnp.broadcast_to(jnp.sum(a, axis=-1, keepdims=True), (1, D))
            b0 = jnp.broadcast_to(jnp.sum(sb * wr, axis=-1, keepdims=True), (1, D))
            for i, v in enumerate((ga, sb, cb1, gb, a, gb * cb1, gb * sb, a0, b0)):
                modv[i] = jnp.broadcast_to(v, (8, D))

        def out_rows(x1, mean, inv):
            return (x1 + ((x1 - _wide(mean, D)) * (_wide(inv, D) * modv[5]) + modv[6])).astype(bf16)

        def out_chunks(j):
            x1v, sv, ov = view(acc, j, TL), view(st2_buf, j, TL), view(o_buf, j, TL)

            def chunk(off):
                def f(tok):
                    rs = slice(off, off + 8)
                    ov[rs, :] = out_rows(x1v[rs, :], sv[rs, 0:128] + tok, sv[rs, 128:256] + tok)
                return f
            return [chunk(off) for off in range(0, TL, 8)]

        def epi_chunks(j, x1v, ov, with_out=True):
            sub = lax.broadcasted_iota(i32, (8, 128), 0)
            low = (0xFFFF - j * TL) - sub
            sv = view(st2_buf, j, TL)
            st = {}

            def chunk(off):
                def f(tok=None):
                    if off == 0:
                        st["k1"], st["k2"] = key_buf[0], key_buf[1]
                    x1 = x1v[off:off + 8, :]
                    mean, inv = _row_stats(x1, tok)
                    sv[off:off + 8, 0:128] = mean
                    sv[off:off + 8, 128:256] = inv
                    xa = _tiles(x1 * modv[4])
                    if tok is not None:
                        xa[0] = xa[0] + tok
                    ra = _lane_sum(_fold(jnp.add, xa))
                    r = inv * (ra - mean * modv[7, :, 0:128]) + modv[8, :, 0:128]
                    if with_out:
                        ov[off:off + 8, :] = out_rows(x1, mean, inv)
                    bits = pltpu.bitcast(_rb(r) + 0.0, i32)
                    key = jnp.where(bits < 0, bits ^ 0x7FFF0000, bits) | (low - off)
                    st["k2"] = jnp.maximum(st["k2"], jnp.minimum(st["k1"], key))
                    st["k1"] = jnp.maximum(st["k1"], key)
                    if off + 8 == TL:
                        key_buf[0], key_buf[1] = st["k1"], st["k2"]
                return f
            return [chunk(off) for off in range(0, TL, 8)]

        cp_c().start()
        cp_x(0).start()
        for c in range(2):
            cp_wq0(c).start()
            for i in range(n_mch):
                cp_ca(c, i).start()
            if c == 0:
                for j in range(1, J0):
                    cp_x(j).start()
        cp_sa().start()
        for h in range(G - 1):
            cp_k(h, sem_first.at[1 + h]).start()
        early = []
        for h in range(2):
            early += [cp_v(h, sem_first.at[8 + 2 * h]), cp_wo(h, sem_first.at[9 + 2 * h])]
        for cp in early:
            cp.start()
        start_head(0)

        cp_c().wait()
        cf = c_buf[...].astype(f32)
        sc = _rb(cf * jax.nn.sigmoid(cf))
        for t in range(4):
            sc_buf[t] = sc[:, t * (D // 4):(t + 1) * (D // 4)]

        def cb_body(t, carry):
            view(cb_buf, t, D // 4)[...] = jnp.transpose(jnp.broadcast_to(sc_buf[t], (128, D // 4)))
            return carry
        lax.fori_loop(0, 4, cb_body, 0)
        key_buf[...] = jnp.full(key_buf.shape, _IMIN, i32)
        cp_x(0).wait()

        def st0_body(i, carry):
            for ch in ln1_chunks(i, T0 // 4):
                ch()
            return carry
        lax.fori_loop(0, 4, st0_body, 0)

        def ca_half(c, stream):
            cp_wq0(c).wait()
            if not stream:
                for i in range(n_mch):
                    cp_ca(c, i).wait()
            part = None
            for i in range(n_mch):
                if stream:
                    cp_ca(c, i).wait()
                scb = jnp.broadcast_to(sc[:, i * MCH:(i + 1) * MCH], (16, MCH)).astype(bf16)
                d = jnp.dot(scb, wca[c, i * MCH:(i + 1) * MCH, :], preferred_element_type=f32)
                part = d if part is None else part + d
            mod0[1, :, c * W:(c + 1) * W] = _rb(1.0 + _rb(part[0:8, :]))

        def q_first(r0, t, c, rec, mid=None):
            rows = pl.ds(r0, t)
            cs = slice(c * W, (c + 1) * W)
            hh = ln1_scaled(x_buf[rows, cs], st_buf[rows, :], cs).astype(bf16)
            for g in range(G):
                if mid is not None and g == mid[0]:
                    mid[1]()
                part = jnp.dot(hh, wq0[cs, g * DH:(g + 1) * DH], preferred_element_type=f32)
                qf_buf[g, rows, :] = part if c == 0 else qf_buf[g, rows, :] + part
                if rec is not None:
                    rec.done(part)

        ca_half(0, True)

        def pa_body(j, carry):
            @pl.when(j + 1 < J0)
            def _():
                cp_x(j + 1).wait()
            jn = jnp.minimum(j + 1, J0 - 1)
            rec = _Pace(ln1_chunks(jn, T0), cfg["LCA"])
            q_first(_mul(j, T0), T0, 0, rec)
            return carry
        lax.fori_loop(0, J0, pa_body, 0)

        TB, RB = cfg["TB"], cfg["RB"]
        ca_half(1, False)

        def pb_body(j, carry):
            q_first(_mul(j, TB // 2), TB // 2, 1, None)
            return carry
        lax.fori_loop(0, 2, pb_body, 0)
        cp_sa().wait()
        cp_k(0, sem_first.at[1]).wait()
        cp_wr().start()
        for p in range(NB + 1, H):
            cp_wmx(p).start()

        def sa_chunk(t):
            def f(tok):
                cs = slice(t * 256, (t + 1) * 256)
                mod0[0, :, cs] = jnp.broadcast_to(matvec(wsa.at[:, cs], tok, 8), (8, 256))
            return f

        def sa_bias():
            bq_buf[...] = jnp.dot(_rep(mod0[0], 16).astype(bf16), wq0[...],
                                  preferred_element_type=f32)[0:8, :]

        def h_chunk(off):
            def f(tok):
                rs, rh = slice(off, off + RB), slice(off // 2, (off + RB) // 2)
                hh = (ln1_scaled(x_buf[rs, :], st_buf[rs, :], slice(0, D), tok)
                      + _rep(mod0[0], RB)).astype(bf16)
                h_buf[rh, :] = pltpu.bitcast(hh, u32)
            return f

        def q_chunk(off):
            def f(tok):
                n = 2 * RB
                rs, rh = slice(off, off + n), slice(off // 2, (off + n) // 2)
                for g in range(1, G):
                    q_ring[g, rh, :] = pltpu.bitcast(
                        q_early(g, qf_buf[g, rs, :] + _rep(tok, n)), u32)
            return f

        hs = [h_chunk(off) for off in range(0, S, RB)]
        qs = [q_chunk(off) for off in range(0, S, 2 * RB)]
        nh = cfg["NHB"]
        rest_chunks = []
        nq, nr = len(qs), len(hs) - nh
        for i, ch in enumerate(hs[nh:]):
            rest_chunks.append(ch)
            while qs and (nq - len(qs)) * nr < (i + 1) * nq:
                rest_chunks.append(qs.pop(0))
        assert not qs
        rec = _Pace([sa_chunk(t) for t in range(D // 256)] + hs[:nh], cfg["LCB2"])
        q_first(TB, S - TB, 1, rec, mid=(cfg["BQ"], sa_bias))
        n4 = len(rest_chunks)
        n3 = n4 - cfg["NL4"]
        cnt = [n3 // 3 + (1 if i < n3 % 3 else 0) for i in range(3)] + [cfg["NL4"]]
        scores(0, q_early(0, qf_buf[0]), s_buf, m_buf, rec=_Pace(rest_chunks, cnt))

        def main_body(h, carry):
            wch, och = expand_chunks(h)
            rec = _mix((pack_chunks(h), cfg["LCM"]), ([vproj(h)], cfg["LCV"]),
                       (wch, cfg["LCW"]), (och, cfg["LCO"]))
            o = pv(h, s_buf, m_buf, rec=rec)
            ov_buf[...] = o[S - RV:, :].astype(f32)
            qproj(h + G, w4.at[h & 1, 0], rec=rec)
            start_head(h + 1)
            scores(h + 1, pltpu.bitcast(q_ring[(h + 1) & 3], bf16), s_buf, m_buf, rec=rec,
                   mode=cfg['MX'])
            oproj([(h, o[0:S - RV, :])], acc.at[0:S - RV, :], rec=rec)
            mod_piece(h)
            wait_head(h + 1)
            return carry
        for h in range(1, G - 1):
            cp_k(h, sem_first.at[1 + h]).wait()
        for cp in early:
            cp.wait()
        wait_head(0)
        lax.fori_loop(0, NB, main_body, 0)

        ha = NB
        rest = list(zip(range(NB + 1, H), (s2_buf, s3_buf, s4_buf), (m2_buf, m3_buf, m4_buf)))
        late = []
        for n, h in enumerate(range(NB + 3, H)):
            late += [cp_v(h, sem_first.at[8 + 2 * n]), cp_wo(h, sem_first.at[9 + 2 * n])]
        cp_wr().wait()
        for p in range(NB + 1, H):
            cp_wmx(p).wait()
        oproj([(NB - 1, ov_buf[...].astype(bf16))], acc.at[S - RV:, :])
        for cp in late:
            cp.start()

        def l_step(j, do_x, do_y):
            if do_x and do_y:
                aw = view(acc, j - 1, TL, 2)
                ay, ax = aw.at[0:TL, :], aw.at[TL:2 * TL, :]
            elif do_x:
                ax = view(acc, j, TL)
            else:
                ay = view(acc, j - 1, TL)
            rec = None
            if do_y:
                chunks = epi_chunks(j - 1, ay, view(o_buf, j - 1, TL), with_out=do_x)
                os_ = [(h, pv(h, sv, mv, late=not do_x)) for h, sv, mv in rest]
            if do_x:
                oa = pv(ha, view(s_buf, j, TL), view(m_buf, j, TL))
            if do_y and do_x:
                oproj(os_, ay, view(x_buf, j - 1, TL))
            elif do_y:
                xv = view(x_buf, j - 1, TL)
                r0, prev = 0, []
                for n in cfg["LSPLIT"]:
                    rs = slice(r0, r0 + n)
                    nr = len(os_) * (D // W)
                    cnt = [len(prev) // nr + (1 if i < len(prev) % nr else 0) for i in range(nr)]
                    rec = _Pace(prev, cnt)
                    oproj([(h, o[rs]) for h, o in os_], ay.at[rs, :], xv.at[rs, :], rec=rec)
                    prev = chunks[r0 // 8:(r0 + n) // 8]
                    r0 += n
                chunks = prev
            if do_x:
                if do_y:
                    rec = _Pace(chunks, cfg["LCNT"])
                for h, sv, mv in rest:
                    q = pltpu.bitcast(view(q_ring.at[h & 3], j, TL // 2)[...], bf16)
                    scores(h, q, sv, mv, rec=rec)
                oproj([(ha, oa)], ax, rec=rec)
            if do_y:
                if do_x:
                    cp_out(j - 1).start()
                else:
                    for ch in chunks:
                        ch()

        for p in range(NB, H):
            mod_piece(p)
        finish_mod()
        l_step(0, True, False)
        for cp in late:
            cp.wait()

        def pl_body(j, carry):
            l_step(j, True, True)
            return carry
        lax.fori_loop(1, JL, pl_body, 0)
        l_step(JL, False, True)

        k1, k2 = key_buf[0], key_buf[1]
        for sh in (4, 2, 1):
            o1, o2 = pltpu.roll(k1, sh, 0), pltpu.roll(k2, sh, 0)
            k2 = jnp.maximum(jnp.minimum(k1, o1), jnp.maximum(k2, o2))
            k1 = jnp.maximum(k1, o1)

        def score_of(k):
            hi = k & jnp.int32(-65536)
            return pltpu.bitcast(jnp.where(hi < 0, hi ^ 0x7FFF0000, hi), f32)

        i1s = jnp.minimum(0xFFFF - (k1[0, 0] & 0xFFFF), S - 1)
        i2s = jnp.minimum(0xFFFF - (k2[0, 0] & 0xFFFF), S - 1)

        sub = lax.broadcasted_iota(i32, (16, D), 0)
        sb, cb1, gb = (_rep(modv[i], 16) for i in (1, 2, 3))

        def adaln2(x1, stat):
            return (x1 - _wide(stat[:, 0:128], D)) * _wide(stat[:, 128:256], D) * cb1 + sb

        def pick(ref):
            sel = lax.broadcasted_iota(i32, (16, ref.shape[1]), 0) == 0
            return jnp.where(sel, ref[pl.ds(i1s, 1), :], ref[pl.ds(i2s, 1), :])

        xs = adaln2(pick(acc), pick(st2_buf)).astype(bf16)
        FC, lag = cfg["FC"], cfg["FLAG"]
        kvs = [int(ch) for ch in cfg["LKV"]]
        fout = [int(ch, 36) for ch in cfg["LFO"]]
        KV = max(kvs)

        def wrows(ref, a, b, c):
            n = FC // 128
            u = [ref[c * n + t, a // 2:b // 2, :] for t in range(n)]
            return pltpu.bitcast(u[0] if n == 1 else jnp.concatenate(u, axis=1), bf16)

        DV = D - KV * 128
        if KV:
            xf = xs.astype(f32)
            for r in range(2):
                xc_buf[r] = jnp.transpose(jnp.broadcast_to(xf[r:r + 1, DV:], (128, D - DV)))
        subc = lax.broadcasted_iota(i32, (8, FC), 0)
        y = None
        act = []
        outs = out_chunks(JL - 1)
        for c in range(F // FC + lag):
            if c < F // FC:
                dm = D - kvs[c] * 128
                gu = [jnp.dot(xs[:, :dm], wrows(w, 0, dm, c), preferred_element_type=f32)[0:8, :]
                      for w in (wg, wu)]
                for v in gu:
                    for t in range(fout[c] if c < len(fout) else 0):
                        if outs:
                            outs.pop(0)(_zero_of(v[0:8, (t % 2) * 128:(t % 2 + 1) * 128]))
                            if not outs:
                                cp_out(JL - 1).start()
                if dm < D:
                    part = [[None, None], [None, None]]
                    for k in range(dm, D, 16):
                        xcol = [_wide(xc_buf[r, k - DV:k - DV + 16, :], FC) for r in range(2)]
                        for m, w in enumerate((wg, wu)):
                            wv = wrows(w, k, k + 16, c).astype(f32)
                            for r in range(2):
                                t = wv * xcol[r]
                                for e in range(2):
                                    te = t[e * 8:(e + 1) * 8, :]
                                    part[m][r] = te if part[m][r] is None else part[m][r] + te
                    for m in range(2):
                        ra, rb_ = (jnp.sum(v, axis=0, keepdims=True) for v in part[m])
                        gu[m] = gu[m] + jnp.where(subc == 0, ra, rb_)
                g, u = _rb(gu[0]), _rb(gu[1])
                act.append(_rep(_rb(g * jax.nn.sigmoid(g)) * u, 16).astype(bf16))
            if c >= lag:
                wdc = pltpu.bitcast(wd[(c - lag) * FC // 2:(c - lag + 1) * FC // 2, :], bf16)
                d = jnp.dot(act[c - lag], wdc, preferred_element_type=f32)[0:8, :]
                y = d if y is None else y + d
        y = _rb(y)
        ya = _rb(y[0:1, :] * _wide(_rb(jax.nn.sigmoid(score_of(k1[0:1, :]))), D))
        yb = _rb(y[1:2, :] * _wide(_rb(jax.nn.sigmoid(score_of(k2[0:1, :]))), D))

        g1 = pl.multiple_of((i1s >> 4) << 4, 16)
        g2 = pl.multiple_of((i2s >> 4) << 4, 16)
        for t, g0 in enumerate((g1, g2)):
            rid = sub + g0
            x1 = acc[pl.ds(g0, 16), :]
            upd = jnp.where(rid == i1s, ya, 0.0) + jnp.where(rid == i2s, yb, 0.0)
            fix[t] = (x1 + gb * (adaln2(x1, st2_buf[pl.ds(g0, 16), :]) + upd)).astype(bf16)

        pltpu.make_async_copy(o_buf, out_hbm, sem_out.at[0]).wait()

        def cp_fix(t, g0):
            return pltpu.make_async_copy(fix.at[t], out_hbm.at[pl.ds(g0, 16), :], sem_fix.at[t])

        cp_fix(0, g1).start()

        @pl.when(g2 != g1)
        def _():
            cp_fix(1, g2).start()
            cp_fix(1, g2).wait()
        cp_fix(0, g1).wait()

    return kernel


_CFG = dict(
    G=4, T0=256, TB=1024, TL=256, MCH=256, RB=16, FC=256, PKN=8, RV=160, MX=3,
    LCA='cc80', LCB2='040g', NHB=16, NL4=8, BQ=3, LCNT='33333333332000',
    LCM='1000000000n0', LCV='000010000000', LCW='00000000000g', LCO='000008ccc0z1',
    LSPLIT=(96, 96, 64), FLAG=1, LKV='00233333333333', LFO='88',
)


def _build(A_x, A_k_cache, A_v_cache, A_wq, A_wo, B_w_r, B_w_gate, B_w_up, B_w_down, c, w_mod,
           **over):
    B, S, D = A_x.shape
    _, H, SK, DH = A_k_cache.shape
    F = B_w_gate.shape[1]
    assert B == 1
    cfg = dict(_CFG, **over)
    T0, TL, G = cfg["T0"], cfg["TL"], cfg["G"]
    MC = (4 * D) // H
    kernel = _make_kernel(S, D, H, DH, SK, F, cfg)
    scratch = [
        pltpu.VMEM((S, D), bf16),
        pltpu.VMEM((S // 2, D), u32),
        pltpu.VMEM((S, D), f32),
        pltpu.VMEM((S, SK), f32),
        pltpu.VMEM((S, 128), f32),
        pltpu.VMEM((TL, SK), f32),
        pltpu.VMEM((TL, 128), f32),
        pltpu.VMEM((TL, SK), f32),
        pltpu.VMEM((TL, 128), f32),
        pltpu.VMEM((TL, SK), f32),
        pltpu.VMEM((TL, 128), f32),
        pltpu.VMEM((S, 256), f32),
        pltpu.VMEM((S, 256), f32),
        pltpu.VMEM((1, S, 384), f32),
        pltpu.VMEM((4, S // 2, DH), u32),
        pltpu.VMEM((G, S, DH), f32),
        pltpu.VMEM((8, G * DH), f32),
        pltpu.VMEM((4, SK, DH), bf16),
        pltpu.VMEM((4, SK, DH), bf16),
        pltpu.VMEM((D, G * DH), bf16),
        pltpu.VMEM((2, 4, D, 128), bf16),
        pltpu.VMEM((4, 2, DH, D), bf16),
        pltpu.VMEM((G - 1, D, MC), bf16),
        pltpu.VMEM((2, D, D // 2), bf16),
        pltpu.VMEM((D, D), bf16),
        pltpu.VMEM((1, D), bf16),
        pltpu.VMEM((D,), bf16),
        pltpu.VMEM((4, 1, D // 4), f32),
        pltpu.VMEM((D, 128), f32),
        pltpu.VMEM((2, 8, D), f32),
        pltpu.VMEM((H, 1, MC), f32),
        pltpu.VMEM((9, 8, D), f32),
        pltpu.VMEM((F // 128, D // 2, 128), u32),
        pltpu.VMEM((F // 128, D // 2, 128), u32),
        pltpu.VMEM((F // 2, D), u32),
        pltpu.VMEM((2, max(int(max(cfg["LKV"])), 1) * 128, 128), f32),
        pltpu.VMEM((cfg["RV"], DH), f32),
        pltpu.VMEM((cfg["RV"] // 8, DH * 8, 128), f32),
        pltpu.VMEM((DH, D), f32),
        pltpu.VMEM((S, D), bf16),
        pltpu.VMEM((2, 8, 128), i32),
        pltpu.VMEM((2, 16, D), bf16),
        pltpu.SemaphoreType.DMA((sum(_sem_sizes(S, D, cfg)),)),
    ]
    any_spec = pl.BlockSpec(memory_space=pl.ANY)
    out = pl.pallas_call(
        kernel,
        out_shape=jax.ShapeDtypeStruct((S, D), bf16),
        in_specs=[any_spec] * 11,
        out_specs=any_spec,
        scratch_shapes=scratch,
        compiler_params=pltpu.CompilerParams(vmem_limit_bytes=126 * 1024 * 1024,
                                             disable_bounds_checks=True,
                                             disable_semaphore_checks=True),
    )(A_x.reshape(S, D), A_k_cache.reshape(H, SK, DH), A_v_cache.reshape(H, SK, DH),
      A_wq, A_wo, B_w_r, B_w_gate, B_w_up, B_w_down, c, w_mod)
    return out.reshape(B, S, D)


@jax.jit
def pallas_adaLN_cond__mha_block_cached__moe_arch_mod__prompt_kernel(
    A_x: jax.Array,
    A_k_cache: jax.Array,
    A_v_cache: jax.Array,
    A_wq: jax.Array,
    A_wo: jax.Array,
    B_x: jax.Array,
    B_w_r: jax.Array,
    B_w_gate: jax.Array,
    B_w_up: jax.Array,
    B_w_down: jax.Array,
    c: jax.Array,
    w_mod: jax.Array,
):
    del B_x
    return _build(A_x, A_k_cache, A_v_cache, A_wq, A_wo, B_w_r, B_w_gate, B_w_up, B_w_down,
                  c, w_mod)
```

```python
import jax
import jax.numpy as jnp
from jax import lax
import jax.experimental.pallas as pl
import jax.experimental.pallas.tpu as pltpu

f32 = jnp.float32
bf16 = jnp.bfloat16
u32 = jnp.uint32
i32 = jnp.int32

_NT = (((1,), (1,)), ((), ()))
_LOG2E = 1.4426950408889634
_EPS = 1e-5
_IMIN = -2 ** 31


def _rb(v):
    return v.astype(bf16).astype(f32)


def _rep(v, n):
    return v if n == 8 else jnp.tile(v, (n // 8, 1))


def _wide(v, w):
    return jnp.tile(v, (1, w // 128))


def _zero_of(v):
    bits = pltpu.bitcast(v, u32)
    return pltpu.bitcast(lax.shift_right_logical(lax.shift_right_logical(bits, jnp.uint32(31)),
                                                 jnp.uint32(1)), f32)


class _Pace:
    def __init__(self, chunks, counts):
        self.chunks = list(chunks)
        self.counts = [ch if isinstance(ch, int) else int(ch, 36) for ch in counts]
        assert sum(self.counts) == len(self.chunks), (counts, len(self.chunks))

    def done(self, res):
        n = self.counts.pop(0)
        for i in range(n):
            r0 = (i * res.shape[0] // n) // 8 * 8
            self.chunks.pop(0)(_zero_of(res[r0:r0 + 8, 0:128]))


def _mix(*plans):
    plans = [(list(ch), [c if isinstance(c, int) else int(c, 36) for c in cnt]) for ch, cnt in plans]
    for ch, cnt in plans:
        assert sum(cnt) == len(ch), (cnt, len(ch))
    fill, total = [], []
    for r in range(len(plans[0][1])):
        slots = sorted((i / cnt[r], k) for k, (_, cnt) in enumerate(plans)
                       for i in range(cnt[r]))
        fill += [plans[k][0].pop(0) for _, k in slots]
        total.append(len(slots))
    return _Pace(fill, total)


def _tiles(v):
    return [v[:, c * 128:(c + 1) * 128] for c in range(v.shape[1] // 128)]


def _fold(op, parts):
    out = parts[0]
    for p in parts[1:]:
        out = op(out, p)
    return out


def _lane_sum(v):
    return jnp.broadcast_to(jnp.sum(v, axis=-1, keepdims=True), v.shape)


def _row_stats(xf, tok=None):
    d = xf.shape[-1]
    ts = _tiles(xf)
    nt = len(ts)
    if tok is not None:
        ts = [ts[0] + tok] + ts[1:]
    mu = _fold(jnp.add, ts) * (1.0 / nt)
    m2 = _fold(jnp.add, [(t - mu) * (t - mu) for t in ts])
    mean = _lane_sum(mu) * (1.0 / 128)
    dm = mu - mean
    var = _lane_sum(m2 + (dm * dm) * float(nt)) * (1.0 / d)
    return mean, lax.rsqrt(var + _EPS)


def _sem_sizes(S, D, cfg):
    j0 = S // cfg["T0"]
    return [2, 2 * (D // cfg["MCH"]), j0, 1, 16, 4, 1, 2]


def _make_kernel(S, D, H, DH, SK, F, cfg):
    T0, TL, MCH = cfg["T0"], cfg["TL"], cfg["MCH"]
    J0 = S // T0
    JL = S // TL
    qscale = DH ** -0.5 * _LOG2E
    n_mch = D // MCH
    G = cfg["G"]
    NB = H - G
    MC = (4 * D) // H
    W = 512
    NF = F // 128
    assert H < 256 and 2 <= G <= 4 and D == 2 * W and MC == DH == 128 and NF <= NB

    def kernel(x_hbm, k_hbm, v_hbm, wq_hbm, wo_hbm, wr_hbm, wg_hbm, wu_hbm, wd_hbm,
               c_hbm, wmod_hbm, out_hbm,
               x_buf, h_buf, acc, s_buf, m_buf, s2_buf, m2_buf, s3_buf, m3_buf, s4_buf, m4_buf,
               st_buf, st2_buf, mp_buf,
               q_ring, qf_buf, bq_buf,
               kb, vb, wq0, w4, wo2, wmx, wca, wsa, c_buf, wr_buf, sc_buf, cb_buf, mod0, modr, modv,
               wg, wu, wd, xc_buf, ov_buf, obx, wof, o_buf, key_buf, fix,
               sems):

        class _Sem:
            def __init__(self, base):
                self.base = base
                self.at = self

            def __getitem__(self, i):
                return sems.at[self.base + i]

        sizes = _sem_sizes(S, D, cfg)
        offs = [sum(sizes[:i]) for i in range(len(sizes))]
        (sem_small, sem_ca, sem_x, sem_sa, sem_first, sem_head,
         sem_out, sem_fix) = (_Sem(o) for o in offs)

        def _mul(a, n):
            v = a * n
            return v if isinstance(a, int) else pl.multiple_of(v, n)

        def view(ref, j, t, n=1):
            return ref.at[pl.ds(_mul(j, t), n * t), :]

        def cp_c():
            return pltpu.make_async_copy(c_hbm, c_buf, sem_small.at[0])

        def cp_wr():
            return pltpu.make_async_copy(wr_hbm, wr_buf, sem_small.at[1])

        def cp_ca(c, i):
            return pltpu.make_async_copy(
                wmod_hbm.at[pl.ds(i * MCH, MCH), pl.ds(D + c * W, W)], view(wca.at[c], i, MCH),
                sem_ca.at[c * n_mch + i])

        def cp_sa():
            return pltpu.make_async_copy(wmod_hbm.at[:, pl.ds(0, D)], wsa, sem_sa.at[0])

        def cp_x(j):
            return pltpu.make_async_copy(view(x_hbm, j, T0), view(x_buf, j, T0), sem_x.at[j])

        def cp_wq0(c):
            return pltpu.make_async_copy(wq_hbm.at[pl.ds(c * W, W), pl.ds(0, G * DH)],
                                         view(wq0, c, W), sem_first.at[14 + c])

        def cp_k(h, sem=None):
            return pltpu.make_async_copy(k_hbm.at[h], kb.at[h & 3],
                                         sem_head.at[0] if sem is None else sem)

        def cp_v(h, sem=None):
            return pltpu.make_async_copy(v_hbm.at[h], vb.at[h & 3],
                                         sem_head.at[1] if sem is None else sem)

        def cp_wo(h, sem=None):
            return pltpu.make_async_copy(view(wo_hbm, h, DH), wo2.at[h & 3, 0],
                                         sem_head.at[2] if sem is None else sem)

        def _clamp(a, hi):
            return min(a, hi) if isinstance(a, int) else jnp.minimum(a, hi)

        def cols(ref, t):
            return ref.at[:, pl.ds(_mul(t, 128), 128)]

        def cp_wmx(p):
            return pltpu.make_async_copy(cols(wmod_hbm, p + (2 * D) // MC), wmx.at[p - NB - 1],
                                         sem_first.at[4 + p - NB])

        def start_head(h):
            f = _clamp(h, NF - 1)
            for i, src in enumerate((cols(wq_hbm, _clamp(h + G, H - 1)),
                                     cols(wmod_hbm, h + (2 * D) // MC),
                                     cols(wg_hbm, f), cols(wu_hbm, f))):
                pltpu.make_async_copy(src, w4.at[h & 1, i], sem_head.at[3]).start()
            cp_k(h + G - 1).start()
            cp_wo(h + 2).start()
            pltpu.make_async_copy(view(wd_hbm, f, 128), wo2.at[(h + 2) & 3, 1],
                                  sem_head.at[2]).start()
            cp_v(h + 2).start()

        def wait_head(h):
            pltpu.make_async_copy(w4.at[h & 1], w4.at[h & 1], sem_head.at[3]).wait()
            cp_k(h + G - 1).wait()
            pltpu.make_async_copy(wo2.at[(h + 2) & 3], wo2.at[(h + 2) & 3], sem_head.at[2]).wait()
            cp_v(h + 2).wait()

        def pack_chunks(h):
            f = _clamp(h, NF - 1)
            out = []
            for sv, dv in ((w4.at[h & 1, 2], wg.at[f]), (w4.at[h & 1, 3], wu.at[f]),
                           (wo2.at[(h + 2) & 3, 1], view(wd, f, 64))):
                n, w = sv.shape
                step = n // cfg['PKN']

                def chunk(r, sv=sv, dv=dv, step=step, w=w):
                    def fn(tok):
                        z = _rep(_wide(pltpu.bitcast(tok, u32), w), step // 2)
                        dv[r // 2:(r + step) // 2, :] = pltpu.bitcast(sv[r:r + step, :], u32) | z
                    return fn
                out += [chunk(r) for r in range(0, n, step)]
            return out

        def cp_out(j):
            return pltpu.make_async_copy(view(o_buf, j, TL), view(out_hbm, j, TL), sem_out.at[0])

        def ln1_chunks(j, t):
            xv, sv, av = view(x_buf, j, t), view(st_buf, j, t), view(acc, j, t)

            def chunk(off):
                def f(tok=None):
                    av[off:off + 8, :] = jnp.zeros((8, D), f32) if tok is None else _wide(tok, D)
                    mean, inv = _row_stats(xv[off:off + 8, :].astype(f32), tok)
                    sv[off:off + 8, 0:128] = mean
                    sv[off:off + 8, 128:256] = inv
                return f
            return [chunk(off) for off in range(0, xv.shape[0], 8)]

        def ln1_scaled(x, stat, cs, tok=None):
            w = x.shape[1]
            mean = stat[:, 0:128] if tok is None else stat[:, 0:128] + _rep(tok, x.shape[0])
            n = (x.astype(f32) - _wide(mean, w)) * _wide(stat[:, 128:256], w)
            return n * _rep(mod0[1, :, cs], x.shape[0])

        def qproj(h, wv, rec=None):
            q = None
            for c in range(D // W):
                cs = slice(c * W, (c + 1) * W)
                part = jnp.dot(pltpu.bitcast(h_buf[:, cs], bf16), wv[cs, :],
                               preferred_element_type=f32)
                q = part if q is None else q + part
                if rec is not None:
                    rec.done(part)
            q_ring[h & 3] = pltpu.bitcast((q * qscale).astype(bf16), u32)

        def q_early(g, q):
            return ((q + _rep(bq_buf[:, g * DH:(g + 1) * DH], q.shape[0])) * qscale).astype(bf16)

        def scores(h, q, sv, mv, rec, partial=False):
            nr = SK // W
            for c in range(nr):
                cs = slice(c * W, (c + 1) * W)
                s = lax.dot_general(q, kb[h & 3, cs, :], _NT, preferred_element_type=f32)
                if partial:
                    t = _tiles(s)
                    mp = jnp.maximum(jnp.maximum(t[0], t[1]), jnp.maximum(t[2], t[3]))
                    if c < nr - 1:
                        z = lax.shift_right_logical(h, 8)
                        mp_buf[z, :, c * 128:(c + 1) * 128] = mp
                sv[:, cs] = s
                if rec is not None:
                    rec.done(s)
            mp = _fold(jnp.maximum, [mp] + _tiles(mp_buf[0]) if partial else _tiles(sv[...]))
            mv[...] = jnp.broadcast_to(jnp.max(mp, axis=-1, keepdims=True), mp.shape)

        def pv(h, sv, mv, rec=None, late=False):
            o = lp = None
            for c in range(SK // W):
                cs = slice(c * W, (c + 1) * W)
                m = mv[...]
                if c >= 2 and sv.shape[0] == S:
                    m = m + _zero_of(lp)
                p = jnp.exp2(sv[:, cs] - _wide(m, W))
                lp = _fold(jnp.add, ([] if lp is None else [lp]) + _tiles(p))
                d = jnp.dot(p.astype(bf16), vb[h & 3, cs, :], preferred_element_type=f32)
                o = d if o is None else o + d
                if rec is not None:
                    rec.done(d)
            if late:
                lp = lp + _zero_of(o)
            l = jnp.sum(lp, axis=-1, keepdims=True)
            r = pl.reciprocal(l, approx=True)
            r = r * (2.0 - l * r)
            return (o * r).astype(bf16)

        def oproj(hos, av, xv=None, rec=None):
            for c in range(D // W):
                cs = slice(c * W, (c + 1) * W)
                a = av[:, cs]
                for h, o in hos:
                    d = jnp.dot(o, wo2[h & 3, 0, :, cs], preferred_element_type=f32)
                    if rec is not None:
                        rec.done(d)
                    a = a + d
                if xv is not None:
                    a = xv[:, cs].astype(f32) + _rep(modv[0, :, cs], a.shape[0]) * a
                av[:, cs] = a

        RV = cfg["RV"]

        def expand_chunks(h):
            def wchunk(r):
                def f(tok):
                    wof[r:r + 8, :] = wo2[h & 3, 0, r:r + 8, :].astype(f32) + _wide(tok, D)
                return f

            lane = lax.broadcasted_iota(i32, (8, 128), 1)

            def ochunk(g, e0):
                def f(tok):
                    o = ov_buf[g * 8:(g + 1) * 8, :] + tok
                    rs = slice(e0 * 8, (e0 + 32) * 8)
                    cols = jnp.concatenate(
                        [jnp.where(lane == e, o, 0.0) for e in range(e0, e0 + 32)], axis=0)
                    obx[g, rs, :] = _lane_sum(cols)
                return f
            och = [ochunk(g, e0) for g in range(RV // 8) for e0 in range(0, DH, 32)]
            return [wchunk(r) for r in range(0, DH, 8)], och

        def vproj(h):
            def f(tok):
                wrow = [jnp.concatenate(
                    [jnp.broadcast_to(wof[e:e + 1, t * 128:(t + 1) * 128], (8, 128))
                     for t in range(D // 128)], axis=1) for e in range(DH)]
                tok = _wide(tok, D)
                for g in range(RV // 8):
                    rows = slice(S - RV + g * 8, S - RV + g * 8 + 8)
                    a = acc[rows, :] + tok
                    ob = obx[g]
                    for e in range(DH):
                        a = a + _wide(ob[e * 8:(e + 1) * 8, :], D) * wrow[e]
                    tok = _zero_of(a)
                    acc[rows, :] = jnp.where(h > 0, a, 0.0)
            return f

        def matvec(wv, tok=None, step=16):
            n = wv.shape[1]
            part = None if tok is None else _wide(tok, n)
            for r in range(0, D, step):
                t = wv[r:r + step, :].astype(f32) * _wide(cb_buf[r:r + step, :], n)
                for e in range(step // 8):
                    te = t[e * 8:(e + 1) * 8, :]
                    part = te if part is None else part + te
            return _rb(jnp.sum(part, axis=0, keepdims=True))

        def mod_piece(p):
            extra = isinstance(p, int) and p > NB
            modr[p] = matvec(wmx.at[p - NB - 1] if extra else w4.at[p & 1, 1])

        def finish_mod():
            n = D // MC
            ga, sb, cb, gb = (jnp.concatenate([modr[i * n + t] for t in range(n)], axis=-1)
                              for i in range(4))
            cb1 = _rb(1.0 + cb)
            wr = wr_buf[...].astype(f32).reshape(1, D)
            a = cb1 * wr
            a0 = jnp.broadcast_to(jnp.sum(a, axis=-1, keepdims=True), (1, D))
            b0 = jnp.broadcast_to(jnp.sum(sb * wr, axis=-1, keepdims=True), (1, D))
            for i, v in enumerate((ga, sb, cb1, gb, a, gb * cb1, gb * sb, a0, b0)):
                modv[i] = jnp.broadcast_to(v, (8, D))

        def out_rows(x1, mean, inv):
            return (x1 + ((x1 - _wide(mean, D)) * (_wide(inv, D) * modv[5]) + modv[6])).astype(bf16)

        def out_chunks(j):
            x1v, sv, ov = view(acc, j, TL), view(st2_buf, j, TL), view(o_buf, j, TL)

            def chunk(off):
                def f(tok):
                    rs = slice(off, off + 8)
                    ov[rs, :] = out_rows(x1v[rs, :], sv[rs, 0:128] + tok, sv[rs, 128:256] + tok)
                return f
            return [chunk(off) for off in range(0, TL, 8)]

        def epi_chunks(j, x1v, ov, with_out=True):
            sub = lax.broadcasted_iota(i32, (8, 128), 0)
            low = (0xFFFF - j * TL) - sub
            sv = view(st2_buf, j, TL)
            st = {}

            def chunk(off):
                def f(tok=None):
                    if off == 0:
                        st["k1"], st["k2"] = key_buf[0], key_buf[1]
                    x1 = x1v[off:off + 8, :]
                    mean, inv = _row_stats(x1, tok)
                    sv[off:off + 8, 0:128] = mean
                    sv[off:off + 8, 128:256] = inv
                    xa = _tiles(x1 * modv[4])
                    if tok is not None:
                        xa[0] = xa[0] + tok
                    ra = _lane_sum(_fold(jnp.add, xa))
                    r = inv * (ra - mean * modv[7, :, 0:128]) + modv[8, :, 0:128]
                    if with_out:
                        ov[off:off + 8, :] = out_rows(x1, mean, inv)
                    bits = pltpu.bitcast(_rb(r) + 0.0, i32)
                    key = jnp.where(bits < 0, bits ^ 0x7FFF0000, bits) | (low - off)
                    st["k2"] = jnp.maximum(st["k2"], jnp.minimum(st["k1"], key))
                    st["k1"] = jnp.maximum(st["k1"], key)
                    if off + 8 == TL:
                        key_buf[0], key_buf[1] = st["k1"], st["k2"]
                return f
            return [chunk(off) for off in range(0, TL, 8)]

        cp_c().start()
        cp_x(0).start()
        for c in range(2):
            cp_wq0(c).start()
            for i in range(n_mch):
                cp_ca(c, i).start()
            if c == 0:
                for j in range(1, J0):
                    cp_x(j).start()
        cp_sa().start()
        for h in range(G - 1):
            cp_k(h, sem_first.at[1 + h]).start()
        early = []
        for h in range(2):
            early += [cp_v(h, sem_first.at[8 + 2 * h]), cp_wo(h, sem_first.at[9 + 2 * h])]
        for cp in early:
            cp.start()
        start_head(0)

        cp_c().wait()
        cf = c_buf[...].astype(f32)
        sc = _rb(cf * jax.nn.sigmoid(cf))
        for t in range(4):
            sc_buf[t] = sc[:, t * (D // 4):(t + 1) * (D // 4)]

        def cb_body(t, carry):
            view(cb_buf, t, D // 4)[...] = jnp.transpose(jnp.broadcast_to(sc_buf[t], (128, D // 4)))
            return carry
        lax.fori_loop(0, 4, cb_body, 0)
        key_buf[...] = jnp.full(key_buf.shape, _IMIN, i32)
        cp_x(0).wait()

        def st0_body(i, carry):
            for ch in ln1_chunks(i, T0 // 4):
                ch()
            return carry
        lax.fori_loop(0, 4, st0_body, 0)

        def ca_half(c, stream):
            cp_wq0(c).wait()
            if not stream:
                for i in range(n_mch):
                    cp_ca(c, i).wait()
            part = None
            for i in range(n_mch):
                if stream:
                    cp_ca(c, i).wait()
                scb = jnp.broadcast_to(sc[:, i * MCH:(i + 1) * MCH], (16, MCH)).astype(bf16)
                d = jnp.dot(scb, wca[c, i * MCH:(i + 1) * MCH, :], preferred_element_type=f32)
                part = d if part is None else part + d
            mod0[1, :, c * W:(c + 1) * W] = _rb(1.0 + _rb(part[0:8, :]))

        def q_first(r0, t, c, rec, mid=None):
            rows = pl.ds(r0, t)
            cs = slice(c * W, (c + 1) * W)
            hh = ln1_scaled(x_buf[rows, cs], st_buf[rows, :], cs).astype(bf16)
            for g in range(G):
                if mid is not None and g == mid[0]:
                    mid[1]()
                part = jnp.dot(hh, wq0[cs, g * DH:(g + 1) * DH], preferred_element_type=f32)
                qf_buf[g, rows, :] = part if c == 0 else qf_buf[g, rows, :] + part
                if rec is not None:
                    rec.done(part)

        ca_half(0, True)

        def pa_body(j, carry):
            @pl.when(j + 1 < J0)
            def _():
                cp_x(j + 1).wait()
            jn = jnp.minimum(j + 1, J0 - 1)
            rec = _Pace(ln1_chunks(jn, T0), cfg["LCA"])
            q_first(_mul(j, T0), T0, 0, rec)
            return carry
        lax.fori_loop(0, J0, pa_body, 0)

        TB, RB = cfg["TB"], cfg["RB"]
        ca_half(1, False)

        def pb_body(j, carry):
            q_first(_mul(j, TB // 2), TB // 2, 1, None)
            return carry
        lax.fori_loop(0, 2, pb_body, 0)
        cp_sa().wait()
        cp_k(0, sem_first.at[1]).wait()
        cp_wr().start()
        for p in range(NB + 1, H):
            cp_wmx(p).start()

        def sa_chunk(t):
            def f(tok):
                cs = slice(t * 256, (t + 1) * 256)
                mod0[0, :, cs] = jnp.broadcast_to(matvec(wsa.at[:, cs], tok, 8), (8, 256))
            return f

        def sa_bias():
            bq_buf[...] = jnp.dot(_rep(mod0[0], 16).astype(bf16), wq0[...],
                                  preferred_element_type=f32)[0:8, :]

        def h_chunk(off):
            def f(tok):
                rs, rh = slice(off, off + RB), slice(off // 2, (off + RB) // 2)
                hh = (ln1_scaled(x_buf[rs, :], st_buf[rs, :], slice(0, D), tok)
                      + _rep(mod0[0], RB)).astype(bf16)
                h_buf[rh, :] = pltpu.bitcast(hh, u32)
            return f

        def q_chunk(off):
            def f(tok):
                n = 2 * RB
                rs, rh = slice(off, off + n), slice(off // 2, (off + n) // 2)
                for g in range(1, G):
                    q_ring[g, rh, :] = pltpu.bitcast(
                        q_early(g, qf_buf[g, rs, :] + _rep(tok, n)), u32)
            return f

        hs = [h_chunk(off) for off in range(0, S, RB)]
        qs = [q_chunk(off) for off in range(0, S, 2 * RB)]
        nh = cfg["NHB"]
        rest_chunks = []
        nq, nr = len(qs), len(hs) - nh
        for i, ch in enumerate(hs[nh:]):
            rest_chunks.append(ch)
            while qs and (nq - len(qs)) * nr < (i + 1) * nq:
                rest_chunks.append(qs.pop(0))
        assert not qs
        rec = _Pace([sa_chunk(t) for t in range(D // 256)] + hs[:nh], cfg["LCB2"])
        q_first(TB, S - TB, 1, rec, mid=(cfg["BQ"], sa_bias))
        n4 = len(rest_chunks)
        n3 = n4 - cfg["NL4"]
        cnt = [n3 // 3 + (1 if i < n3 % 3 else 0) for i in range(3)] + [cfg["NL4"]]
        scores(0, q_early(0, qf_buf[0]), s_buf, m_buf, rec=_Pace(rest_chunks, cnt))

        def main_body(h, carry):
            wch, och = expand_chunks(h)
            rec = _mix((pack_chunks(h), cfg["LCM"]), ([vproj(h)], cfg["LCV"]),
                       (wch, cfg["LCW"]), (och, cfg["LCO"]))
            o = pv(h, s_buf, m_buf, rec=rec)
            ov_buf[...] = o[S - RV:, :].astype(f32)
            qproj(h + G, w4.at[h & 1, 0], rec=rec)
            start_head(h + 1)
            scores(h + 1, pltpu.bitcast(q_ring[(h + 1) & 3], bf16), s_buf, m_buf, rec=rec,
                   partial=True)
            oproj([(h, o[0:S - RV, :])], acc.at[0:S - RV, :], rec=rec)
            mod_piece(h)
            wait_head(h + 1)
            return carry
        for h in range(1, G - 1):
            cp_k(h, sem_first.at[1 + h]).wait()
        for cp in early:
            cp.wait()
        wait_head(0)
        lax.fori_loop(0, NB, main_body, 0)

        ha = NB
        rest = list(zip(range(NB + 1, H), (s2_buf, s3_buf, s4_buf), (m2_buf, m3_buf, m4_buf)))
        late = []
        for n, h in enumerate(range(NB + 3, H)):
            late += [cp_v(h, sem_first.at[8 + 2 * n]), cp_wo(h, sem_first.at[9 + 2 * n])]
        cp_wr().wait()
        for p in range(NB + 1, H):
            cp_wmx(p).wait()
        oproj([(NB - 1, ov_buf[...].astype(bf16))], acc.at[S - RV:, :])
        for cp in late:
            cp.start()

        def l_step(j, do_x, do_y):
            if do_x and do_y:
                aw = view(acc, j - 1, TL, 2)
                ay, ax = aw.at[0:TL, :], aw.at[TL:2 * TL, :]
            elif do_x:
                ax = view(acc, j, TL)
            else:
                ay = view(acc, j - 1, TL)
            rec = None
            if do_y:
                chunks = epi_chunks(j - 1, ay, view(o_buf, j - 1, TL), with_out=do_x)
                os_ = [(h, pv(h, sv, mv, late=not do_x)) for h, sv, mv in rest]
            if do_x:
                oa = pv(ha, view(s_buf, j, TL), view(m_buf, j, TL))
            if do_y and do_x:
                oproj(os_, ay, view(x_buf, j - 1, TL))
            elif do_y:
                xv = view(x_buf, j - 1, TL)
                r0, prev = 0, []
                for n in cfg["LSPLIT"]:
                    rs = slice(r0, r0 + n)
                    nr = len(os_) * (D // W)
                    cnt = [len(prev) // nr + (1 if i < len(prev) % nr else 0) for i in range(nr)]
                    rec = _Pace(prev, cnt)
                    oproj([(h, o[rs]) for h, o in os_], ay.at[rs, :], xv.at[rs, :], rec=rec)
                    prev = chunks[r0 // 8:(r0 + n) // 8]
                    r0 += n
                chunks = prev
            if do_x:
                if do_y:
                    rec = _Pace(chunks, cfg["LCNT"])
                for h, sv, mv in rest:
                    q = pltpu.bitcast(view(q_ring.at[h & 3], j, TL // 2)[...], bf16)
                    scores(h, q, sv, mv, rec=rec)
                oproj([(ha, oa)], ax, rec=rec)
            if do_y:
                if do_x:
                    cp_out(j - 1).start()
                else:
                    for ch in chunks:
                        ch()

        for p in range(NB, H):
            mod_piece(p)
        finish_mod()
        l_step(0, True, False)
        for cp in late:
            cp.wait()

        def pl_body(j, carry):
            l_step(j, True, True)
            return carry
        lax.fori_loop(1, JL, pl_body, 0)
        l_step(JL, False, True)

        k1, k2 = key_buf[0], key_buf[1]
        for sh in (4, 2, 1):
            o1, o2 = pltpu.roll(k1, sh, 0), pltpu.roll(k2, sh, 0)
            k2 = jnp.maximum(jnp.minimum(k1, o1), jnp.maximum(k2, o2))
            k1 = jnp.maximum(k1, o1)

        def score_of(k):
            hi = k & jnp.int32(-65536)
            return pltpu.bitcast(jnp.where(hi < 0, hi ^ 0x7FFF0000, hi), f32)

        i1s = jnp.minimum(0xFFFF - (k1[0, 0] & 0xFFFF), S - 1)
        i2s = jnp.minimum(0xFFFF - (k2[0, 0] & 0xFFFF), S - 1)

        sub = lax.broadcasted_iota(i32, (16, D), 0)
        sb, cb1, gb = (_rep(modv[i], 16) for i in (1, 2, 3))

        def adaln2(x1, stat):
            return (x1 - _wide(stat[:, 0:128], D)) * _wide(stat[:, 128:256], D) * cb1 + sb

        def pick(ref):
            sel = lax.broadcasted_iota(i32, (16, ref.shape[1]), 0) == 0
            return jnp.where(sel, ref[pl.ds(i1s, 1), :], ref[pl.ds(i2s, 1), :])

        xs = adaln2(pick(acc), pick(st2_buf)).astype(bf16)
        FC, lag = cfg["FC"], cfg["FLAG"]
        kvs = [int(ch) for ch in cfg["LKV"]]
        fout = [int(ch, 36) for ch in cfg["LFO"]]
        KV = max(kvs)

        def wrows(ref, a, b, c):
            n = FC // 128
            u = [ref[c * n + t, a // 2:b // 2, :] for t in range(n)]
            return pltpu.bitcast(u[0] if n == 1 else jnp.concatenate(u, axis=1), bf16)

        DV = D - KV * 128
        if KV:
            xf = xs.astype(f32)
            for r in range(2):
                xc_buf[r] = jnp.transpose(jnp.broadcast_to(xf[r:r + 1, DV:], (128, D - DV)))
        subc = lax.broadcasted_iota(i32, (8, FC), 0)
        y = None
        act = []
        outs = out_chunks(JL - 1)
        for c in range(F // FC + lag):
            if c < F // FC:
                dm = D - kvs[c] * 128
                gu = [jnp.dot(xs[:, :dm], wrows(w, 0, dm, c), preferred_element_type=f32)[0:8, :]
                      for w in (wg, wu)]
                for v in gu:
                    for t in range(fout[c] if c < len(fout) else 0):
                        if outs:
                            outs.pop(0)(_zero_of(v[0:8, (t % 2) * 128:(t % 2 + 1) * 128]))
                            if not outs:
                                cp_out(JL - 1).start()
                if dm < D:
                    part = [[None, None], [None, None]]
                    for k in range(dm, D, 16):
                        xcol = [_wide(xc_buf[r, k - DV:k - DV + 16, :], FC) for r in range(2)]
                        for m, w in enumerate((wg, wu)):
                            wv = wrows(w, k, k + 16, c).astype(f32)
                            for r in range(2):
                                t = wv * xcol[r]
                                for e in range(2):
                                    te = t[e * 8:(e + 1) * 8, :]
                                    part[m][r] = te if part[m][r] is None else part[m][r] + te
                    for m in range(2):
                        ra, rb_ = (jnp.sum(v, axis=0, keepdims=True) for v in part[m])
                        gu[m] = gu[m] + jnp.where(subc == 0, ra, rb_)
                g, u = _rb(gu[0]), _rb(gu[1])
                act.append(_rep(_rb(g * jax.nn.sigmoid(g)) * u, 16).astype(bf16))
            if c >= lag:
                wdc = pltpu.bitcast(wd[(c - lag) * FC // 2:(c - lag + 1) * FC // 2, :], bf16)
                d = jnp.dot(act[c - lag], wdc, preferred_element_type=f32)[0:8, :]
                y = d if y is None else y + d
        y = _rb(y)
        ya = _rb(y[0:1, :] * _wide(_rb(jax.nn.sigmoid(score_of(k1[0:1, :]))), D))
        yb = _rb(y[1:2, :] * _wide(_rb(jax.nn.sigmoid(score_of(k2[0:1, :]))), D))

        g1 = pl.multiple_of((i1s >> 4) << 4, 16)
        g2 = pl.multiple_of((i2s >> 4) << 4, 16)
        for t, g0 in enumerate((g1, g2)):
            rid = sub + g0
            x1 = acc[pl.ds(g0, 16), :]
            upd = jnp.where(rid == i1s, ya, 0.0) + jnp.where(rid == i2s, yb, 0.0)
            fix[t] = (x1 + gb * (adaln2(x1, st2_buf[pl.ds(g0, 16), :]) + upd)).astype(bf16)

        pltpu.make_async_copy(o_buf, out_hbm, sem_out.at[0]).wait()

        def cp_fix(t, g0):
            return pltpu.make_async_copy(fix.at[t], out_hbm.at[pl.ds(g0, 16), :], sem_fix.at[t])

        cp_fix(0, g1).start()

        @pl.when(g2 != g1)
        def _():
            cp_fix(1, g2).start()
            cp_fix(1, g2).wait()
        cp_fix(0, g1).wait()

    return kernel


_CFG = dict(
    G=4, T0=256, TB=1024, TL=256, MCH=256, RB=16, FC=256, PKN=8, RV=160,
    LCA='cc80', LCB2='040g', NHB=16, NL4=8, BQ=3, LCNT='33333333332000',
    LCM='1000000000n0', LCV='000010000000', LCW='00000000000g', LCO='000008ccc0z1',
    LSPLIT=(96, 96, 64), FLAG=1, LKV='00233333333333', LFO='88',
)


def _build(A_x, A_k_cache, A_v_cache, A_wq, A_wo, B_w_r, B_w_gate, B_w_up, B_w_down, c, w_mod,
           **over):
    B, S, D = A_x.shape
    _, H, SK, DH = A_k_cache.shape
    F = B_w_gate.shape[1]
    assert B == 1
    cfg = dict(_CFG, **over)
    T0, TL, G = cfg["T0"], cfg["TL"], cfg["G"]
    MC = (4 * D) // H
    kernel = _make_kernel(S, D, H, DH, SK, F, cfg)
    scratch = [
        pltpu.VMEM((S, D), bf16),
        pltpu.VMEM((S // 2, D), u32),
        pltpu.VMEM((S, D), f32),
        pltpu.VMEM((S, SK), f32),
        pltpu.VMEM((S, 128), f32),
        pltpu.VMEM((TL, SK), f32),
        pltpu.VMEM((TL, 128), f32),
        pltpu.VMEM((TL, SK), f32),
        pltpu.VMEM((TL, 128), f32),
        pltpu.VMEM((TL, SK), f32),
        pltpu.VMEM((TL, 128), f32),
        pltpu.VMEM((S, 256), f32),
        pltpu.VMEM((S, 256), f32),
        pltpu.VMEM((1, S, SK // 4 - 128), f32),
        pltpu.VMEM((4, S // 2, DH), u32),
        pltpu.VMEM((G, S, DH), f32),
        pltpu.VMEM((8, G * DH), f32),
        pltpu.VMEM((4, SK, DH), bf16),
        pltpu.VMEM((4, SK, DH), bf16),
        pltpu.VMEM((D, G * DH), bf16),
        pltpu.VMEM((2, 4, D, 128), bf16),
        pltpu.VMEM((4, 2, DH, D), bf16),
        pltpu.VMEM((G - 1, D, MC), bf16),
        pltpu.VMEM((2, D, D // 2), bf16),
        pltpu.VMEM((D, D), bf16),
        pltpu.VMEM((1, D), bf16),
        pltpu.VMEM((D,), bf16),
        pltpu.VMEM((4, 1, D // 4), f32),
        pltpu.VMEM((D, 128), f32),
        pltpu.VMEM((2, 8, D), f32),
        pltpu.VMEM((H, 1, MC), f32),
        pltpu.VMEM((9, 8, D), f32),
        pltpu.VMEM((F // 128, D // 2, 128), u32),
        pltpu.VMEM((F // 128, D // 2, 128), u32),
        pltpu.VMEM((F // 2, D), u32),
        pltpu.VMEM((2, max(int(max(cfg["LKV"])), 1) * 128, 128), f32),
        pltpu.VMEM((cfg["RV"], DH), f32),
        pltpu.VMEM((cfg["RV"] // 8, DH * 8, 128), f32),
        pltpu.VMEM((DH, D), f32),
        pltpu.VMEM((S, D), bf16),
        pltpu.VMEM((2, 8, 128), i32),
        pltpu.VMEM((2, 16, D), bf16),
        pltpu.SemaphoreType.DMA((sum(_sem_sizes(S, D, cfg)),)),
    ]
    any_spec = pl.BlockSpec(memory_space=pl.ANY)
    out = pl.pallas_call(
        kernel,
        out_shape=jax.ShapeDtypeStruct((S, D), bf16),
        in_specs=[any_spec] * 11,
        out_specs=any_spec,
        scratch_shapes=scratch,
        compiler_params=pltpu.CompilerParams(vmem_limit_bytes=126 * 1024 * 1024,
                                             disable_bounds_checks=True,
                                             disable_semaphore_checks=True),
    )(A_x.reshape(S, D), A_k_cache.reshape(H, SK, DH), A_v_cache.reshape(H, SK, DH),
      A_wq, A_wo, B_w_r, B_w_gate, B_w_up, B_w_down, c, w_mod)
    return out.reshape(B, S, D)


@jax.jit
def pallas_adaLN_cond__mha_block_cached__moe_arch_mod__prompt_kernel(
    A_x: jax.Array,
    A_k_cache: jax.Array,
    A_v_cache: jax.Array,
    A_wq: jax.Array,
    A_wo: jax.Array,
    B_x: jax.Array,
    B_w_r: jax.Array,
    B_w_gate: jax.Array,
    B_w_up: jax.Array,
    B_w_down: jax.Array,
    c: jax.Array,
    w_mod: jax.Array,
):
    del B_x
    return _build(A_x, A_k_cache, A_v_cache, A_wq, A_wo, B_w_r, B_w_gate, B_w_up, B_w_down,
                  c, w_mod)
```

```python
import jax
import jax.numpy as jnp
from jax import lax
import jax.experimental.pallas as pl
import jax.experimental.pallas.tpu as pltpu

f32 = jnp.float32
bf16 = jnp.bfloat16
u32 = jnp.uint32
i32 = jnp.int32

_NT = (((1,), (1,)), ((), ()))
_LOG2E = 1.4426950408889634
_EPS = 1e-5
_IMIN = -2 ** 31


def _rb(v):
    return v.astype(bf16).astype(f32)


def _rep(v, n):
    return v if n == 8 else jnp.tile(v, (n // 8, 1))


def _wide(v, w):
    return jnp.tile(v, (1, w // 128))


def _pack(v):
    return pltpu.bitcast(v.astype(bf16), u32)


def _zero_of(v):
    bits = pltpu.bitcast(v, u32)
    return pltpu.bitcast(lax.shift_right_logical(lax.shift_right_logical(bits, jnp.uint32(31)),
                                                 jnp.uint32(1)), f32)


class _Pace:
    def __init__(self, chunks, counts):
        self.chunks = list(chunks)
        self.counts = [ch if isinstance(ch, int) else int(ch, 36) for ch in counts]
        assert sum(self.counts) == len(self.chunks), (counts, len(self.chunks))

    def done(self, res):
        n = self.counts.pop(0)
        for i in range(n):
            r0 = (i * res.shape[0] // n) // 8 * 8
            self.chunks.pop(0)(_zero_of(res[r0:r0 + 8, 0:128]))


def _mix(*plans):
    plans = [(list(ch), [c if isinstance(c, int) else int(c, 36) for c in cnt]) for ch, cnt in plans]
    for ch, cnt in plans:
        assert sum(cnt) == len(ch), (cnt, len(ch))
    fill, total = [], []
    for r in range(len(plans[0][1])):
        slots = sorted((i / cnt[r], k) for k, (_, cnt) in enumerate(plans)
                       for i in range(cnt[r]))
        fill += [plans[k][0].pop(0) for _, k in slots]
        total.append(len(slots))
    return _Pace(fill, total)


def _tiles(v):
    return [v[:, c * 128:(c + 1) * 128] for c in range(v.shape[1] // 128)]


def _fold(op, parts):
    out = parts[0]
    for p in parts[1:]:
        out = op(out, p)
    return out


def _lane_sum(v):
    return jnp.broadcast_to(jnp.sum(v, axis=-1, keepdims=True), v.shape)


def _row_stats(xf, tok=None):
    d = xf.shape[-1]
    ts = _tiles(xf)
    nt = len(ts)
    if tok is not None:
        ts = [ts[0] + tok] + ts[1:]
    mu = _fold(jnp.add, ts) * (1.0 / nt)
    m2 = _fold(jnp.add, [(t - mu) * (t - mu) for t in ts])
    mean = _lane_sum(mu) * (1.0 / 128)
    dm = mu - mean
    var = _lane_sum(m2 + (dm * dm) * float(nt)) * (1.0 / d)
    return mean, lax.rsqrt(var + _EPS)


def _sem_sizes(S, D, cfg):
    j0 = S // cfg["T0"]
    return [2, 2 * (D // cfg["MCH"]), j0, 1, 16, 4, 1, 2]


def _make_kernel(S, D, H, DH, SK, F, cfg):
    T0, TL, MCH = cfg["T0"], cfg["TL"], cfg["MCH"]
    J0 = S // T0
    JL = S // TL
    qscale = DH ** -0.5 * _LOG2E
    n_mch = D // MCH
    G = cfg["G"]
    NB = H - G
    MC = (4 * D) // H
    W = 512
    NF = F // 128
    assert H < 256 and 2 <= G <= 4 and D == 2 * W and MC == DH == 128 and NF <= NB

    def kernel(x_hbm, k_hbm, v_hbm, wq_hbm, wo_hbm, wr_hbm, wg_hbm, wu_hbm, wd_hbm,
               c_hbm, wmod_hbm, out_hbm,
               x_buf, h_buf, acc, s_buf, m_buf, s2_buf, m2_buf, s3_buf, m3_buf, s4_buf, m4_buf,
               st_buf, st2_buf, mp_buf,
               q_ring, qf_buf, bq_buf,
               kb, vb, wq0, w4, wo2, wmx, wca, wsa, c_buf, wr_buf, sc_buf, cb_buf, mod0, modr, modv,
               wg, wu, wd, xc_buf, ov_buf, obx, wof, o_buf, key_buf, fix,
               sems):

        class _Sem:
            def __init__(self, base):
                self.base = base
                self.at = self

            def __getitem__(self, i):
                return sems.at[self.base + i]

        sizes = _sem_sizes(S, D, cfg)
        offs = [sum(sizes[:i]) for i in range(len(sizes))]
        (sem_small, sem_ca, sem_x, sem_sa, sem_first, sem_head,
         sem_out, sem_fix) = (_Sem(o) for o in offs)

        def _mul(a, n):
            v = a * n
            return v if isinstance(a, int) else pl.multiple_of(v, n)

        def view(ref, j, t, n=1):
            return ref.at[pl.ds(_mul(j, t), n * t), :]

        def cp_c():
            return pltpu.make_async_copy(c_hbm, c_buf, sem_small.at[0])

        def cp_wr():
            return pltpu.make_async_copy(wr_hbm, wr_buf, sem_small.at[1])

        def cp_ca(c, i):
            return pltpu.make_async_copy(
                wmod_hbm.at[pl.ds(i * MCH, MCH), pl.ds(D + c * W, W)], view(wca.at[c], i, MCH),
                sem_ca.at[c * n_mch + i])

        def cp_sa():
            return pltpu.make_async_copy(wmod_hbm.at[:, pl.ds(0, D)], wsa, sem_sa.at[0])

        def cp_x(j):
            return pltpu.make_async_copy(view(x_hbm, j, T0), view(x_buf, j, T0), sem_x.at[j])

        def cp_wq0(c):
            return pltpu.make_async_copy(wq_hbm.at[pl.ds(c * W, W), pl.ds(0, G * DH)],
                                         view(wq0, c, W), sem_first.at[14 + c])

        def cp_k(h, sem=None):
            return pltpu.make_async_copy(k_hbm.at[h], kb.at[h & 3],
                                         sem_head.at[0] if sem is None else sem)

        def cp_v(h, sem=None):
            return pltpu.make_async_copy(v_hbm.at[h], vb.at[h & 3],
                                         sem_head.at[1] if sem is None else sem)

        def cp_wo(h, sem=None):
            return pltpu.make_async_copy(view(wo_hbm, h, DH), wo2.at[h & 3, 0],
                                         sem_head.at[2] if sem is None else sem)

        def _clamp(a, hi):
            return min(a, hi) if isinstance(a, int) else jnp.minimum(a, hi)

        def cols(ref, t):
            return ref.at[:, pl.ds(_mul(t, 128), 128)]

        def cp_wmx(p):
            return pltpu.make_async_copy(cols(wmod_hbm, p + (2 * D) // MC), wmx.at[p - NB - 1],
                                         sem_first.at[4 + p - NB])

        def start_head(h):
            f = _clamp(h, NF - 1)
            for i, src in enumerate((cols(wq_hbm, _clamp(h + G, H - 1)),
                                     cols(wmod_hbm, h + (2 * D) // MC),
                                     cols(wg_hbm, f), cols(wu_hbm, f))):
                pltpu.make_async_copy(src, w4.at[h & 1, i], sem_head.at[3]).start()
            cp_k(h + G - 1).start()
            cp_wo(h + 2).start()
            pltpu.make_async_copy(view(wd_hbm, f, 128), wo2.at[(h + 2) & 3, 1],
                                  sem_head.at[2]).start()
            cp_v(h + 2).start()

        def wait_head(h):
            pltpu.make_async_copy(w4.at[h & 1], w4.at[h & 1], sem_head.at[3]).wait()
            cp_k(h + G - 1).wait()
            pltpu.make_async_copy(wo2.at[(h + 2) & 3], wo2.at[(h + 2) & 3], sem_head.at[2]).wait()
            cp_v(h + 2).wait()

        def pack_chunks(h):
            f = _clamp(h, NF - 1)
            out = []
            for sv, dv in ((w4.at[h & 1, 2], wg.at[f]), (w4.at[h & 1, 3], wu.at[f]),
                           (wo2.at[(h + 2) & 3, 1], view(wd, f, 64))):
                n, w = sv.shape
                step = n // cfg['PKN']

                def chunk(r, sv=sv, dv=dv, step=step, w=w):
                    def fn(tok):
                        z = _rep(_wide(pltpu.bitcast(tok, u32), w), step // 2)
                        dv[r // 2:(r + step) // 2, :] = pltpu.bitcast(sv[r:r + step, :], u32) | z
                    return fn
                out += [chunk(r) for r in range(0, n, step)]
            return out

        def cp_out(j):
            return pltpu.make_async_copy(view(o_buf, j, TL), view(out_hbm, j, TL), sem_out.at[0])

        def ln1_chunks(j, t):
            xv, sv, av = view(x_buf, j, t), view(st_buf, j, t), view(acc, j, t)

            def chunk(off):
                def f(tok=None):
                    av[off:off + 8, :] = jnp.zeros((8, D), f32) if tok is None else _wide(tok, D)
                    mean, inv = _row_stats(xv[off:off + 8, :].astype(f32), tok)
                    sv[off:off + 8, 0:128] = mean
                    sv[off:off + 8, 128:256] = inv
                return f
            return [chunk(off) for off in range(0, xv.shape[0], 8)]

        def ln1_scaled(x, stat, cs, tok=None):
            w = x.shape[1]
            mean = stat[:, 0:128] if tok is None else stat[:, 0:128] + _rep(tok, x.shape[0])
            n = (x.astype(f32) - _wide(mean, w)) * _wide(stat[:, 128:256], w)
            return n * _rep(mod0[1, :, cs], x.shape[0])

        def qproj(h, wv, rec=None):
            q = None
            for c in range(D // W):
                cs = slice(c * W, (c + 1) * W)
                part = jnp.dot(pltpu.bitcast(h_buf[:, cs], bf16), wv[cs, :],
                               preferred_element_type=f32)
                q = part if q is None else q + part
                if rec is not None:
                    rec.done(part)
            q_ring[h & 3] = _pack(q * qscale)

        def q_early(g, q):
            return (q + _rep(bq_buf[:, g * DH:(g + 1) * DH], q.shape[0])) * qscale

        def scores(h, q, sv, mv, rec, partial=False):
            nr = SK // W
            for c in range(nr):
                cs = slice(c * W, (c + 1) * W)
                s = lax.dot_general(q, kb[h & 3, cs, :], _NT, preferred_element_type=f32)
                if partial:
                    t = _tiles(s)
                    mp = jnp.maximum(jnp.maximum(t[0], t[1]), jnp.maximum(t[2], t[3]))
                    if c < nr - 1:
                        z = lax.shift_right_logical(h, 8)
                        mp_buf[z, :, c * 128:(c + 1) * 128] = mp
                sv[:, cs] = s
                if rec is not None:
                    rec.done(s)
            mp = _fold(jnp.maximum, [mp] + _tiles(mp_buf[0]) if partial else _tiles(sv[...]))
            mv[...] = jnp.broadcast_to(jnp.max(mp, axis=-1, keepdims=True), mp.shape)

        def pv(h, sv, mv, rec=None, late=False):
            o = lp = None
            for c in range(SK // W):
                cs = slice(c * W, (c + 1) * W)
                m = mv[...]
                if c >= 2 and sv.shape[0] == S:
                    m = m + _zero_of(lp)
                p = jnp.exp2(sv[:, cs] - _wide(m, W))
                lp = _fold(jnp.add, ([] if lp is None else [lp]) + _tiles(p))
                d = jnp.dot(p.astype(bf16), vb[h & 3, cs, :], preferred_element_type=f32)
                o = d if o is None else o + d
                if rec is not None:
                    rec.done(d)
            if late:
                lp = lp + _zero_of(o)
            l = jnp.sum(lp, axis=-1, keepdims=True)
            r = pl.reciprocal(l, approx=True)
            r = r * (2.0 - l * r)
            return o * r

        def oproj(hos, av, xv=None, rec=None):
            for c in range(D // W):
                cs = slice(c * W, (c + 1) * W)
                a = av[:, cs]
                for h, o in hos:
                    d = jnp.dot(o.astype(bf16), wo2[h & 3, 0, :, cs], preferred_element_type=f32)
                    if rec is not None:
                        rec.done(d)
                    a = a + d
                if xv is not None:
                    a = xv[:, cs].astype(f32) + _rep(modv[0, :, cs], a.shape[0]) * a
                av[:, cs] = a

        RV = cfg["RV"]

        def expand_chunks(h):
            def wchunk(r):
                def f(tok):
                    wof[r:r + 8, :] = wo2[h & 3, 0, r:r + 8, :].astype(f32) + _wide(tok, D)
                return f

            lane = lax.broadcasted_iota(i32, (8, 128), 1)

            def ochunk(g, e0):
                def f(tok):
                    o = ov_buf[g * 8:(g + 1) * 8, :] + tok
                    rs = slice(e0 * 8, (e0 + 32) * 8)
                    cols = jnp.concatenate(
                        [jnp.where(lane == e, o, 0.0) for e in range(e0, e0 + 32)], axis=0)
                    obx[g, rs, :] = _lane_sum(cols)
                return f
            och = [ochunk(g, e0) for g in range(RV // 8) for e0 in range(0, DH, 32)]
            return [wchunk(r) for r in range(0, DH, 8)], och

        def vproj(h):
            def f(tok):
                wrow = [jnp.concatenate(
                    [jnp.broadcast_to(wof[e:e + 1, t * 128:(t + 1) * 128], (8, 128))
                     for t in range(D // 128)], axis=1) for e in range(DH)]
                tok = _wide(tok, D)
                for g in range(RV // 8):
                    rows = slice(S - RV + g * 8, S - RV + g * 8 + 8)
                    a = acc[rows, :] + tok
                    ob = obx[g]
                    for e in range(DH):
                        a = a + _wide(ob[e * 8:(e + 1) * 8, :], D) * wrow[e]
                    tok = _zero_of(a)
                    acc[rows, :] = jnp.where(h > 0, a, 0.0)
            return f

        def matvec(wv, tok=None, step=16):
            n = wv.shape[1]
            part = None if tok is None else _wide(tok, n)
            for r in range(0, D, step):
                t = wv[r:r + step, :].astype(f32) * _wide(cb_buf[r:r + step, :], n)
                for e in range(step // 8):
                    te = t[e * 8:(e + 1) * 8, :]
                    part = te if part is None else part + te
            return _rb(jnp.sum(part, axis=0, keepdims=True))

        def mod_piece(p):
            extra = isinstance(p, int) and p > NB
            modr[p] = matvec(wmx.at[p - NB - 1] if extra else w4.at[p & 1, 1])

        def finish_mod():
            n = D // MC
            ga, sb, cb, gb = (jnp.concatenate([modr[i * n + t] for t in range(n)], axis=-1)
                              for i in range(4))
            cb1 = _rb(1.0 + cb)
            wr = wr_buf[...].astype(f32).reshape(1, D)
            a = cb1 * wr
            a0 = jnp.broadcast_to(jnp.sum(a, axis=-1, keepdims=True), (1, D))
            b0 = jnp.broadcast_to(jnp.sum(sb * wr, axis=-1, keepdims=True), (1, D))
            for i, v in enumerate((ga, sb, cb1, gb, a, gb * cb1, gb * sb, a0, b0)):
                modv[i] = jnp.broadcast_to(v, (8, D))

        def out_rows(x1, mean, inv):
            return (x1 + ((x1 - _wide(mean, D)) * (_wide(inv, D) * modv[5]) + modv[6])).astype(bf16)

        def out_chunks(j):
            x1v, sv, ov = view(acc, j, TL), view(st2_buf, j, TL), view(o_buf, j, TL)

            def chunk(off):
                def f(tok):
                    rs = slice(off, off + 8)
                    ov[rs, :] = out_rows(x1v[rs, :], sv[rs, 0:128] + tok, sv[rs, 128:256] + tok)
                return f
            return [chunk(off) for off in range(0, TL, 8)]

        def epi_chunks(j, x1v, ov, with_out=True):
            sub = lax.broadcasted_iota(i32, (8, 128), 0)
            low = (0xFFFF - j * TL) - sub
            sv = view(st2_buf, j, TL)
            st = {}

            def chunk(off):
                def f(tok=None):
                    if off == 0:
                        st["k1"], st["k2"] = key_buf[0], key_buf[1]
                    x1 = x1v[off:off + 8, :]
                    mean, inv = _row_stats(x1, tok)
                    sv[off:off + 8, 0:128] = mean
                    sv[off:off + 8, 128:256] = inv
                    xa = _tiles(x1 * modv[4])
                    if tok is not None:
                        xa[0] = xa[0] + tok
                    ra = _lane_sum(_fold(jnp.add, xa))
                    r = inv * (ra - mean * modv[7, :, 0:128]) + modv[8, :, 0:128]
                    if with_out:
                        ov[off:off + 8, :] = out_rows(x1, mean, inv)
                    bits = pltpu.bitcast(_rb(r) + 0.0, i32)
                    key = jnp.where(bits < 0, bits ^ 0x7FFF0000, bits) | (low - off)
                    st["k2"] = jnp.maximum(st["k2"], jnp.minimum(st["k1"], key))
                    st["k1"] = jnp.maximum(st["k1"], key)
                    if off + 8 == TL:
                        key_buf[0], key_buf[1] = st["k1"], st["k2"]
                return f
            return [chunk(off) for off in range(0, TL, 8)]

        cp_c().start()
        cp_x(0).start()
        for c in range(2):
            cp_wq0(c).start()
            for i in range(n_mch):
                cp_ca(c, i).start()
            if c == 0:
                for j in range(1, J0):
                    cp_x(j).start()
        cp_sa().start()
        for h in range(G - 1):
            cp_k(h, sem_first.at[1 + h]).start()
        early = []
        for h in range(2):
            early += [cp_v(h, sem_first.at[8 + 2 * h]), cp_wo(h, sem_first.at[9 + 2 * h])]
        for cp in early:
            cp.start()
        start_head(0)

        cp_c().wait()
        cf = c_buf[...].astype(f32)
        sc = _rb(cf * jax.nn.sigmoid(cf))
        for t in range(4):
            sc_buf[t] = sc[:, t * (D // 4):(t + 1) * (D // 4)]

        def cb_body(t, carry):
            view(cb_buf, t, D // 4)[...] = jnp.transpose(jnp.broadcast_to(sc_buf[t], (128, D // 4)))
            return carry
        lax.fori_loop(0, 4, cb_body, 0)
        key_buf[...] = jnp.full(key_buf.shape, _IMIN, i32)
        cp_x(0).wait()

        def st0_body(i, carry):
            for ch in ln1_chunks(i, T0 // 4):
                ch()
            return carry
        lax.fori_loop(0, 4, st0_body, 0)

        def ca_half(c, stream):
            cp_wq0(c).wait()
            if not stream:
                for i in range(n_mch):
                    cp_ca(c, i).wait()
            part = None
            for i in range(n_mch):
                if stream:
                    cp_ca(c, i).wait()
                scb = jnp.broadcast_to(sc[:, i * MCH:(i + 1) * MCH], (16, MCH)).astype(bf16)
                d = jnp.dot(scb, wca[c, i * MCH:(i + 1) * MCH, :], preferred_element_type=f32)
                part = d if part is None else part + d
            mod0[1, :, c * W:(c + 1) * W] = _rb(1.0 + _rb(part[0:8, :]))

        def q_first(r0, t, c, rec, mid=None):
            rows = pl.ds(r0, t)
            cs = slice(c * W, (c + 1) * W)
            hh = ln1_scaled(x_buf[rows, cs], st_buf[rows, :], cs).astype(bf16)
            for g in range(G):
                if mid is not None and g == mid[0]:
                    mid[1]()
                part = jnp.dot(hh, wq0[cs, g * DH:(g + 1) * DH], preferred_element_type=f32)
                qf_buf[g, rows, :] = part if c == 0 else qf_buf[g, rows, :] + part
                if rec is not None:
                    rec.done(part)

        ca_half(0, True)

        def pa_body(j, carry):
            @pl.when(j + 1 < J0)
            def _():
                cp_x(j + 1).wait()
            jn = jnp.minimum(j + 1, J0 - 1)
            rec = _Pace(ln1_chunks(jn, T0), cfg["LCA"])
            q_first(_mul(j, T0), T0, 0, rec)
            return carry
        lax.fori_loop(0, J0, pa_body, 0)

        TB, RB = cfg["TB"], cfg["RB"]
        ca_half(1, False)

        def pb_body(j, carry):
            q_first(_mul(j, TB // 2), TB // 2, 1, None)
            return carry
        lax.fori_loop(0, 2, pb_body, 0)
        cp_sa().wait()
        cp_k(0, sem_first.at[1]).wait()
        cp_wr().start()
        for p in range(NB + 1, H):
            cp_wmx(p).start()

        def sa_chunk(t):
            def f(tok):
                cs = slice(t * 256, (t + 1) * 256)
                mod0[0, :, cs] = jnp.broadcast_to(matvec(wsa.at[:, cs], tok, 8), (8, 256))
            return f

        def sa_bias():
            bq_buf[...] = jnp.dot(_rep(mod0[0], 16).astype(bf16), wq0[...],
                                  preferred_element_type=f32)[0:8, :]

        def h_chunk(off):
            def f(tok):
                rs, rh = slice(off, off + RB), slice(off // 2, (off + RB) // 2)
                hh = (ln1_scaled(x_buf[rs, :], st_buf[rs, :], slice(0, D), tok)
                      + _rep(mod0[0], RB)).astype(bf16)
                h_buf[rh, :] = pltpu.bitcast(hh, u32)
            return f

        def q_chunk(off):
            def f(tok):
                n = 2 * RB
                rs, rh = slice(off, off + n), slice(off // 2, (off + n) // 2)
                for g in range(1, G):
                    q_ring[g, rh, :] = _pack(q_early(g, qf_buf[g, rs, :] + _rep(tok, n)))
            return f

        hs = [h_chunk(off) for off in range(0, S, RB)]
        qs = [q_chunk(off) for off in range(0, S, 2 * RB)]
        nh = cfg["NHB"]
        rest_chunks = []
        nq, nr = len(qs), len(hs) - nh
        for i, ch in enumerate(hs[nh:]):
            rest_chunks.append(ch)
            while qs and (nq - len(qs)) * nr < (i + 1) * nq:
                rest_chunks.append(qs.pop(0))
        assert not qs
        rec = _Pace([sa_chunk(t) for t in range(D // 256)] + hs[:nh], cfg["LCB2"])
        q_first(TB, S - TB, 1, rec, mid=(cfg["BQ"], sa_bias))
        n4 = len(rest_chunks)
        n3 = n4 - cfg["NL4"]
        cnt = [n3 // 3 + (1 if i < n3 % 3 else 0) for i in range(3)] + [cfg["NL4"]]
        scores(0, q_early(0, qf_buf[0]).astype(bf16), s_buf, m_buf, rec=_Pace(rest_chunks, cnt))

        def main_body(h, carry):
            wch, och = expand_chunks(h)
            rec = _mix((pack_chunks(h), cfg["LCM"]), ([vproj(h)], cfg["LCV"]),
                       (wch, cfg["LCW"]), (och, cfg["LCO"]))
            o = pv(h, s_buf, m_buf, rec=rec)
            ov_buf[...] = _rb(o[S - RV:, :])
            qproj(h + G, w4.at[h & 1, 0], rec=rec)
            start_head(h + 1)
            scores(h + 1, pltpu.bitcast(q_ring[(h + 1) & 3], bf16), s_buf, m_buf, rec=rec,
                   partial=True)
            oproj([(h, o[0:S - RV, :])], acc.at[0:S - RV, :], rec=rec)
            mod_piece(h)
            wait_head(h + 1)
            return carry
        for h in range(1, G - 1):
            cp_k(h, sem_first.at[1 + h]).wait()
        for cp in early:
            cp.wait()
        wait_head(0)
        lax.fori_loop(0, NB, main_body, 0)

        ha = NB
        rest = list(zip(range(NB + 1, H), (s2_buf, s3_buf, s4_buf), (m2_buf, m3_buf, m4_buf)))
        late = []
        for n, h in enumerate(range(NB + 3, H)):
            late += [cp_v(h, sem_first.at[8 + 2 * n]), cp_wo(h, sem_first.at[9 + 2 * n])]
        cp_wr().wait()
        for p in range(NB + 1, H):
            cp_wmx(p).wait()
        oproj([(NB - 1, ov_buf[...])], acc.at[S - RV:, :])
        for cp in late:
            cp.start()

        def l_step(j, do_x, do_y):
            if do_x and do_y:
                aw = view(acc, j - 1, TL, 2)
                ay, ax = aw.at[0:TL, :], aw.at[TL:2 * TL, :]
            elif do_x:
                ax = view(acc, j, TL)
            else:
                ay = view(acc, j - 1, TL)
            rec = None
            if do_y:
                chunks = epi_chunks(j - 1, ay, view(o_buf, j - 1, TL), with_out=do_x)
                os_ = [(h, pv(h, sv, mv, late=not do_x)) for h, sv, mv in rest]
            if do_x:
                oa = pv(ha, view(s_buf, j, TL), view(m_buf, j, TL))
            if do_y and do_x:
                oproj(os_, ay, view(x_buf, j - 1, TL))
            elif do_y:
                xv = view(x_buf, j - 1, TL)
                r0, prev = 0, []
                for n in cfg["LSPLIT"]:
                    rs = slice(r0, r0 + n)
                    nr = len(os_) * (D // W)
                    cnt = [len(prev) // nr + (1 if i < len(prev) % nr else 0) for i in range(nr)]
                    rec = _Pace(prev, cnt)
                    oproj([(h, o[rs]) for h, o in os_], ay.at[rs, :], xv.at[rs, :], rec=rec)
                    prev = chunks[r0 // 8:(r0 + n) // 8]
                    r0 += n
                chunks = prev
            if do_x:
                if do_y:
                    rec = _Pace(chunks, cfg["LCNT"])
                for h, sv, mv in rest:
                    q = pltpu.bitcast(view(q_ring.at[h & 3], j, TL // 2)[...], bf16)
                    scores(h, q, sv, mv, rec=rec)
                oproj([(ha, oa)], ax, rec=rec)
            if do_y:
                if do_x:
                    cp_out(j - 1).start()
                else:
                    for ch in chunks:
                        ch()

        for p in range(NB, H):
            mod_piece(p)
        finish_mod()
        l_step(0, True, False)
        for cp in late:
            cp.wait()

        def pl_body(j, carry):
            l_step(j, True, True)
            return carry
        lax.fori_loop(1, JL, pl_body, 0)
        l_step(JL, False, True)

        k1, k2 = key_buf[0], key_buf[1]
        for sh in (4, 2, 1):
            o1, o2 = pltpu.roll(k1, sh, 0), pltpu.roll(k2, sh, 0)
            k2 = jnp.maximum(jnp.minimum(k1, o1), jnp.maximum(k2, o2))
            k1 = jnp.maximum(k1, o1)

        def score_of(k):
            hi = k & jnp.int32(-65536)
            return pltpu.bitcast(jnp.where(hi < 0, hi ^ 0x7FFF0000, hi), f32)

        i1s = jnp.minimum(0xFFFF - (k1[0, 0] & 0xFFFF), S - 1)
        i2s = jnp.minimum(0xFFFF - (k2[0, 0] & 0xFFFF), S - 1)

        sub = lax.broadcasted_iota(i32, (16, D), 0)
        sb, cb1, gb = (_rep(modv[i], 16) for i in (1, 2, 3))

        def adaln2(x1, stat):
            return (x1 - _wide(stat[:, 0:128], D)) * _wide(stat[:, 128:256], D) * cb1 + sb

        def pick(ref):
            sel = lax.broadcasted_iota(i32, (16, ref.shape[1]), 0) == 0
            return jnp.where(sel, ref[pl.ds(i1s, 1), :], ref[pl.ds(i2s, 1), :])

        xs = adaln2(pick(acc), pick(st2_buf)).astype(bf16)
        FC, lag = cfg["FC"], cfg["FLAG"]
        kvs = [int(ch) for ch in cfg["LKV"]]
        fout = [int(ch, 36) for ch in cfg["LFO"]]
        KV = max(kvs)

        def wrows(ref, a, b, c):
            n = FC // 128
            u = [ref[c * n + t, a // 2:b // 2, :] for t in range(n)]
            return pltpu.bitcast(u[0] if n == 1 else jnp.concatenate(u, axis=1), bf16)

        DV = D - KV * 128
        if KV:
            xf = xs.astype(f32)
            for r in range(2):
                xc_buf[r] = jnp.transpose(jnp.broadcast_to(xf[r:r + 1, DV:], (128, D - DV)))
        subc = lax.broadcasted_iota(i32, (8, FC), 0)
        y = None
        act = []
        outs = out_chunks(JL - 1)
        for c in range(F // FC + lag):
            if c < F // FC:
                dm = D - kvs[c] * 128
                gu = [jnp.dot(xs[:, :dm], wrows(w, 0, dm, c), preferred_element_type=f32)[0:8, :]
                      for w in (wg, wu)]
                for v in gu:
                    for t in range(fout[c] if c < len(fout) else 0):
                        if outs:
                            outs.pop(0)(_zero_of(v[0:8, (t % 2) * 128:(t % 2 + 1) * 128]))
                            if not outs:
                                cp_out(JL - 1).start()
                if dm < D:
                    part = [[None, None], [None, None]]
                    for k in range(dm, D, 16):
                        xcol = [_wide(xc_buf[r, k - DV:k - DV + 16, :], FC) for r in range(2)]
                        for m, w in enumerate((wg, wu)):
                            wv = wrows(w, k, k + 16, c).astype(f32)
                            for r in range(2):
                                t = wv * xcol[r]
                                for e in range(2):
                                    te = t[e * 8:(e + 1) * 8, :]
                                    part[m][r] = te if part[m][r] is None else part[m][r] + te
                    for m in range(2):
                        ra, rb_ = (jnp.sum(v, axis=0, keepdims=True) for v in part[m])
                        gu[m] = gu[m] + jnp.where(subc == 0, ra, rb_)
                g, u = _rb(gu[0]), _rb(gu[1])
                act.append(_rep(_rb(g * jax.nn.sigmoid(g)) * u, 16).astype(bf16))
            if c >= lag:
                wdc = pltpu.bitcast(wd[(c - lag) * FC // 2:(c - lag + 1) * FC // 2, :], bf16)
                d = jnp.dot(act[c - lag], wdc, preferred_element_type=f32)[0:8, :]
                y = d if y is None else y + d
        y = _rb(y)
        ya = _rb(y[0:1, :] * _wide(_rb(jax.nn.sigmoid(score_of(k1[0:1, :]))), D))
        yb = _rb(y[1:2, :] * _wide(_rb(jax.nn.sigmoid(score_of(k2[0:1, :]))), D))

        g1 = pl.multiple_of((i1s >> 4) << 4, 16)
        g2 = pl.multiple_of((i2s >> 4) << 4, 16)
        for t, g0 in enumerate((g1, g2)):
            rid = sub + g0
            x1 = acc[pl.ds(g0, 16), :]
            upd = jnp.where(rid == i1s, ya, 0.0) + jnp.where(rid == i2s, yb, 0.0)
            fix[t] = (x1 + gb * (adaln2(x1, st2_buf[pl.ds(g0, 16), :]) + upd)).astype(bf16)

        pltpu.make_async_copy(o_buf, out_hbm, sem_out.at[0]).wait()

        def cp_fix(t, g0):
            return pltpu.make_async_copy(fix.at[t], out_hbm.at[pl.ds(g0, 16), :], sem_fix.at[t])

        cp_fix(0, g1).start()

        @pl.when(g2 != g1)
        def _():
            cp_fix(1, g2).start()
            cp_fix(1, g2).wait()
        cp_fix(0, g1).wait()

    return kernel


_CFG = dict(
    G=4, T0=256, TB=1024, TL=256, MCH=256, RB=16, FC=256, PKN=8, RV=160,
    LCA='cc80', LCB2='040g', NHB=16, NL4=8, BQ=3, LCNT='33333333332000',
    LCM='cc0000000000', LCV='000010000000', LCW='00000000000g', LCO='000006bbb0z6',
    LSPLIT=(96, 96, 64), FLAG=1, LKV='00233333333333', LFO='88',
)


def _build(A_x, A_k_cache, A_v_cache, A_wq, A_wo, B_w_r, B_w_gate, B_w_up, B_w_down, c, w_mod,
           **over):
    B, S, D = A_x.shape
    _, H, SK, DH = A_k_cache.shape
    F = B_w_gate.shape[1]
    assert B == 1
    cfg = dict(_CFG, **over)
    T0, TL, G = cfg["T0"], cfg["TL"], cfg["G"]
    MC = (4 * D) // H
    kernel = _make_kernel(S, D, H, DH, SK, F, cfg)
    scratch = [
        pltpu.VMEM((S, D), bf16),
        pltpu.VMEM((S // 2, D), u32),
        pltpu.VMEM((S, D), f32),
        pltpu.VMEM((S, SK), f32),
        pltpu.VMEM((S, 128), f32),
        pltpu.VMEM((TL, SK), f32),
        pltpu.VMEM((TL, 128), f32),
        pltpu.VMEM((TL, SK), f32),
        pltpu.VMEM((TL, 128), f32),
        pltpu.VMEM((TL, SK), f32),
        pltpu.VMEM((TL, 128), f32),
        pltpu.VMEM((S, 256), f32),
        pltpu.VMEM((S, 256), f32),
        pltpu.VMEM((1, S, SK // 4 - 128), f32),
        pltpu.VMEM((4, S // 2, DH), u32),
        pltpu.VMEM((G, S, DH), f32),
        pltpu.VMEM((8, G * DH), f32),
        pltpu.VMEM((4, SK, DH), bf16),
        pltpu.VMEM((4, SK, DH), bf16),
        pltpu.VMEM((D, G * DH), bf16),
        pltpu.VMEM((2, 4, D, 128), bf16),
        pltpu.VMEM((4, 2, DH, D), bf16),
        pltpu.VMEM((G - 1, D, MC), bf16),
        pltpu.VMEM((2, D, D // 2), bf16),
        pltpu.VMEM((D, D), bf16),
        pltpu.VMEM((1, D), bf16),
        pltpu.VMEM((D,), bf16),
        pltpu.VMEM((4, 1, D // 4), f32),
        pltpu.VMEM((D, 128), f32),
        pltpu.VMEM((2, 8, D), f32),
        pltpu.VMEM((H, 1, MC), f32),
        pltpu.VMEM((9, 8, D), f32),
        pltpu.VMEM((F // 128, D // 2, 128), u32),
        pltpu.VMEM((F // 128, D // 2, 128), u32),
        pltpu.VMEM((F // 2, D), u32),
        pltpu.VMEM((2, max(int(max(cfg["LKV"])), 1) * 128, 128), f32),
        pltpu.VMEM((cfg["RV"], DH), f32),
        pltpu.VMEM((cfg["RV"] // 8, DH * 8, 128), f32),
        pltpu.VMEM((DH, D), f32),
        pltpu.VMEM((S, D), bf16),
        pltpu.VMEM((2, 8, 128), i32),
        pltpu.VMEM((2, 16, D), bf16),
        pltpu.SemaphoreType.DMA((sum(_sem_sizes(S, D, cfg)),)),
    ]
    any_spec = pl.BlockSpec(memory_space=pl.ANY)
    out = pl.pallas_call(
        kernel,
        out_shape=jax.ShapeDtypeStruct((S, D), bf16),
        in_specs=[any_spec] * 11,
        out_specs=any_spec,
        scratch_shapes=scratch,
        compiler_params=pltpu.CompilerParams(vmem_limit_bytes=126 * 1024 * 1024,
                                             disable_bounds_checks=True,
                                             disable_semaphore_checks=True),
    )(A_x.reshape(S, D), A_k_cache.reshape(H, SK, DH), A_v_cache.reshape(H, SK, DH),
      A_wq, A_wo, B_w_r, B_w_gate, B_w_up, B_w_down, c, w_mod)
    return out.reshape(B, S, D)


@jax.jit
def pallas_adaLN_cond__mha_block_cached__moe_arch_mod__prompt_kernel(
    A_x: jax.Array,
    A_k_cache: jax.Array,
    A_v_cache: jax.Array,
    A_wq: jax.Array,
    A_wo: jax.Array,
    B_x: jax.Array,
    B_w_r: jax.Array,
    B_w_gate: jax.Array,
    B_w_up: jax.Array,
    B_w_down: jax.Array,
    c: jax.Array,
    w_mod: jax.Array,
):
    del B_x
    return _build(A_x, A_k_cache, A_v_cache, A_wq, A_wo, B_w_r, B_w_gate, B_w_up, B_w_down,
                  c, w_mod)
```

```python
import jax
import jax.numpy as jnp
from jax import lax
import jax.experimental.pallas as pl
import jax.experimental.pallas.tpu as pltpu

f32 = jnp.float32
bf16 = jnp.bfloat16
u32 = jnp.uint32
i32 = jnp.int32

_NT = (((1,), (1,)), ((), ()))
_LOG2E = 1.4426950408889634
_EPS = 1e-5
_IMIN = -2 ** 31


def _rb(v):
    return v.astype(bf16).astype(f32)


def _rep(v, n):
    return v if n == 8 else jnp.tile(v, (n // 8, 1))


def _wide(v, w):
    return jnp.tile(v, (1, w // 128))


def _pack(v):
    return pltpu.bitcast(v.astype(bf16), u32)


def _zero_of(v):
    bits = pltpu.bitcast(v, u32)
    return pltpu.bitcast(lax.shift_right_logical(lax.shift_right_logical(bits, jnp.uint32(31)),
                                                 jnp.uint32(1)), f32)


class _Pace:
    def __init__(self, chunks, counts):
        self.chunks = list(chunks)
        self.counts = [ch if isinstance(ch, int) else int(ch, 36) for ch in counts]
        assert sum(self.counts) == len(self.chunks), (counts, len(self.chunks))

    def done(self, res):
        n = self.counts.pop(0)
        for i in range(n):
            r0 = (i * res.shape[0] // n) // 8 * 8
            self.chunks.pop(0)(_zero_of(res[r0:r0 + 8, 0:128]))


def _mix(*plans):
    plans = [(list(ch), [c if isinstance(c, int) else int(c, 36) for c in cnt]) for ch, cnt in plans]
    for ch, cnt in plans:
        assert sum(cnt) == len(ch), (cnt, len(ch))
    fill, total = [], []
    for r in range(len(plans[0][1])):
        slots = sorted((i / cnt[r], k) for k, (_, cnt) in enumerate(plans)
                       for i in range(cnt[r]))
        fill += [plans[k][0].pop(0) for _, k in slots]
        total.append(len(slots))
    return _Pace(fill, total)


def _tiles(v):
    return [v[:, c * 128:(c + 1) * 128] for c in range(v.shape[1] // 128)]


def _fold(op, parts):
    out = parts[0]
    for p in parts[1:]:
        out = op(out, p)
    return out


def _lane_sum(v):
    return jnp.broadcast_to(jnp.sum(v, axis=-1, keepdims=True), v.shape)


def _row_stats(xf, tok=None, like_bf16=False):
    d = xf.shape[-1]
    ts = _tiles(xf)
    nt = len(ts)
    if tok is not None:
        ts = [ts[0] + tok] + ts[1:]
    mu = _fold(jnp.add, ts) * (1.0 / nt)
    m2 = _fold(jnp.add, [(t - mu) * (t - mu) for t in ts])
    mean = _lane_sum(mu) * (1.0 / 128)
    dm = mu - mean
    var = _lane_sum(m2 + (dm * dm) * float(nt)) * (1.0 / d)
    if not like_bf16:
        return mean, lax.rsqrt(var + _EPS)
    v = _rb(_rb(var) + _EPS)
    y = lax.rsqrt(v)
    sig = _rb(v * y)
    return mean, y * (2.0 - sig * y)


def _sem_sizes(S, D, cfg):
    j0 = S // cfg["T0"]
    return [2, 2 * (D // cfg["MCH"]), j0, 1, 16, 4, 1, 2]


def _make_kernel(S, D, H, DH, SK, F, cfg):
    T0, TL, MCH = cfg["T0"], cfg["TL"], cfg["MCH"]
    J0 = S // T0
    JL = S // TL
    qscale = DH ** -0.5 * _LOG2E
    n_mch = D // MCH
    G = cfg["G"]
    NB = H - G
    MC = (4 * D) // H
    W = 512
    NF = F // 128
    assert H < 256 and 2 <= G <= 4 and D == 2 * W and MC == DH == 128 and NF <= NB

    def kernel(x_hbm, k_hbm, v_hbm, wq_hbm, wo_hbm, wr_hbm, wg_hbm, wu_hbm, wd_hbm,
               c_hbm, wmod_hbm, out_hbm,
               x_buf, h_buf, acc, s_buf, m_buf, s2_buf, m2_buf, s3_buf, m3_buf, s4_buf, m4_buf,
               st_buf, st2_buf, mp_buf,
               q_ring, qf_buf, bq_buf,
               kb, vb, wq0, w4, wo2, wmx, wca, wsa, c_buf, wr_buf, sc_buf, cb_buf, mod0, modr, modv,
               wg, wu, wd, xc_buf, ov_buf, obx, wof, o_buf, key_buf, fix,
               sems):

        class _Sem:
            def __init__(self, base):
                self.base = base
                self.at = self

            def __getitem__(self, i):
                return sems.at[self.base + i]

        sizes = _sem_sizes(S, D, cfg)
        offs = [sum(sizes[:i]) for i in range(len(sizes))]
        (sem_small, sem_ca, sem_x, sem_sa, sem_first, sem_head,
         sem_out, sem_fix) = (_Sem(o) for o in offs)

        def _mul(a, n):
            v = a * n
            return v if isinstance(a, int) else pl.multiple_of(v, n)

        def view(ref, j, t, n=1):
            return ref.at[pl.ds(_mul(j, t), n * t), :]

        def cp_c():
            return pltpu.make_async_copy(c_hbm, c_buf, sem_small.at[0])

        def cp_wr():
            return pltpu.make_async_copy(wr_hbm, wr_buf, sem_small.at[1])

        def cp_ca(c, i):
            return pltpu.make_async_copy(
                wmod_hbm.at[pl.ds(i * MCH, MCH), pl.ds(D + c * W, W)], view(wca.at[c], i, MCH),
                sem_ca.at[c * n_mch + i])

        def cp_sa():
            return pltpu.make_async_copy(wmod_hbm.at[:, pl.ds(0, D)], wsa, sem_sa.at[0])

        def cp_x(j):
            return pltpu.make_async_copy(view(x_hbm, j, T0), view(x_buf, j, T0), sem_x.at[j])

        def cp_wq0(c):
            return pltpu.make_async_copy(wq_hbm.at[pl.ds(c * W, W), pl.ds(0, G * DH)],
                                         view(wq0, c, W), sem_first.at[14 + c])

        def cp_k(h, sem=None):
            return pltpu.make_async_copy(k_hbm.at[h], kb.at[h & 3],
                                         sem_head.at[0] if sem is None else sem)

        def cp_v(h, sem=None):
            return pltpu.make_async_copy(v_hbm.at[h], vb.at[h & 3],
                                         sem_head.at[1] if sem is None else sem)

        def cp_wo(h, sem=None):
            return pltpu.make_async_copy(view(wo_hbm, h, DH), wo2.at[h & 3, 0],
                                         sem_head.at[2] if sem is None else sem)

        def _clamp(a, hi):
            return min(a, hi) if isinstance(a, int) else jnp.minimum(a, hi)

        def cols(ref, t):
            return ref.at[:, pl.ds(_mul(t, 128), 128)]

        def cp_wmx(p):
            return pltpu.make_async_copy(cols(wmod_hbm, p + (2 * D) // MC), wmx.at[p - NB - 1],
                                         sem_first.at[4 + p - NB])

        def start_head(h):
            f = _clamp(h, NF - 1)
            for i, src in enumerate((cols(wq_hbm, _clamp(h + G, H - 1)),
                                     cols(wmod_hbm, h + (2 * D) // MC),
                                     cols(wg_hbm, f), cols(wu_hbm, f))):
                pltpu.make_async_copy(src, w4.at[h & 1, i], sem_head.at[3]).start()
            cp_k(h + G - 1).start()
            cp_wo(h + 2).start()
            pltpu.make_async_copy(view(wd_hbm, f, 128), wo2.at[(h + 2) & 3, 1],
                                  sem_head.at[2]).start()
            cp_v(h + 2).start()

        def wait_head(h):
            pltpu.make_async_copy(w4.at[h & 1], w4.at[h & 1], sem_head.at[3]).wait()
            cp_k(h + G - 1).wait()
            pltpu.make_async_copy(wo2.at[(h + 2) & 3], wo2.at[(h + 2) & 3], sem_head.at[2]).wait()
            cp_v(h + 2).wait()

        def pack_chunks(h):
            f = _clamp(h, NF - 1)
            out = []
            for sv, dv in ((w4.at[h & 1, 2], wg.at[f]), (w4.at[h & 1, 3], wu.at[f]),
                           (wo2.at[(h + 2) & 3, 1], view(wd, f, 64))):
                n, w = sv.shape
                step = n // cfg['PKN']

                def chunk(r, sv=sv, dv=dv, step=step, w=w):
                    def fn(tok):
                        z = _rep(_wide(pltpu.bitcast(tok, u32), w), step // 2)
                        dv[r // 2:(r + step) // 2, :] = pltpu.bitcast(sv[r:r + step, :], u32) | z
                    return fn
                out += [chunk(r) for r in range(0, n, step)]
            return out

        def cp_out(j):
            return pltpu.make_async_copy(view(o_buf, j, TL), view(out_hbm, j, TL), sem_out.at[0])

        def ln1_chunks(j, t):
            xv, sv, av = view(x_buf, j, t), view(st_buf, j, t), view(acc, j, t)

            def chunk(off):
                def f(tok=None):
                    av[off:off + 8, :] = jnp.zeros((8, D), f32) if tok is None else _wide(tok, D)
                    mean, inv = _row_stats(xv[off:off + 8, :].astype(f32), tok)
                    sv[off:off + 8, 0:128] = mean
                    sv[off:off + 8, 128:256] = inv
                return f
            return [chunk(off) for off in range(0, xv.shape[0], 8)]

        def ln1_scaled(x, stat, cs, tok=None):
            w = x.shape[1]
            mean = stat[:, 0:128] if tok is None else stat[:, 0:128] + _rep(tok, x.shape[0])
            n = (x.astype(f32) - _wide(mean, w)) * _wide(stat[:, 128:256], w)
            return n * _rep(mod0[1, :, cs], x.shape[0])

        def qproj(h, wv, rec=None):
            q = None
            for c in range(D // W):
                cs = slice(c * W, (c + 1) * W)
                part = jnp.dot(pltpu.bitcast(h_buf[:, cs], bf16), wv[cs, :],
                               preferred_element_type=f32)
                q = part if q is None else q + part
                if rec is not None:
                    rec.done(part)
            q_ring[h & 3] = _pack(q * qscale)

        def q_early(g, q):
            return (q + _rep(bq_buf[:, g * DH:(g + 1) * DH], q.shape[0])) * qscale

        def scores(h, q, sv, mv, rec, partial=False):
            nr = SK // W
            for c in range(nr):
                cs = slice(c * W, (c + 1) * W)
                s = lax.dot_general(q, kb[h & 3, cs, :], _NT, preferred_element_type=f32)
                if partial:
                    t = _tiles(s)
                    mp = jnp.maximum(jnp.maximum(t[0], t[1]), jnp.maximum(t[2], t[3]))
                    if c < nr - 1:
                        z = lax.shift_right_logical(h, 8)
                        mp_buf[z, :, c * 128:(c + 1) * 128] = mp
                sv[:, cs] = s
                if rec is not None:
                    rec.done(s)
            mp = _fold(jnp.maximum, [mp] + _tiles(mp_buf[0]) if partial else _tiles(sv[...]))
            mv[...] = jnp.broadcast_to(jnp.max(mp, axis=-1, keepdims=True), mp.shape)

        def pv(h, sv, mv, rec=None, late=False):
            o = lp = None
            for c in range(SK // W):
                cs = slice(c * W, (c + 1) * W)
                m = mv[...]
                if c >= 2 and sv.shape[0] == S:
                    m = m + _zero_of(lp)
                p = jnp.exp2(sv[:, cs] - _wide(m, W))
                lp = _fold(jnp.add, ([] if lp is None else [lp]) + _tiles(p))
                d = jnp.dot(p.astype(bf16), vb[h & 3, cs, :], preferred_element_type=f32)
                o = d if o is None else o + d
                if rec is not None:
                    rec.done(d)
            if late:
                lp = lp + _zero_of(o)
            l = jnp.sum(lp, axis=-1, keepdims=True)
            r = pl.reciprocal(l, approx=True)
            r = r * (2.0 - l * r)
            return o * r

        def oproj(hos, av, xv=None, rec=None):
            for c in range(D // W):
                cs = slice(c * W, (c + 1) * W)
                a = av[:, cs]
                for h, o in hos:
                    d = jnp.dot(o.astype(bf16), wo2[h & 3, 0, :, cs], preferred_element_type=f32)
                    if rec is not None:
                        rec.done(d)
                    a = a + d
                if xv is not None:
                    a = xv[:, cs].astype(f32) + _rep(modv[0, :, cs], a.shape[0]) * a
                av[:, cs] = a

        RV = cfg["RV"]

        def expand_chunks(h):
            def wchunk(r):
                def f(tok):
                    wof[r:r + 8, :] = wo2[h & 3, 0, r:r + 8, :].astype(f32) + _wide(tok, D)
                return f

            lane = lax.broadcasted_iota(i32, (8, 128), 1)

            def ochunk(g, e0):
                def f(tok):
                    o = ov_buf[g * 8:(g + 1) * 8, :] + tok
                    rs = slice(e0 * 8, (e0 + 32) * 8)
                    cols = jnp.concatenate(
                        [jnp.where(lane == e, o, 0.0) for e in range(e0, e0 + 32)], axis=0)
                    obx[g, rs, :] = _lane_sum(cols)
                return f
            och = [ochunk(g, e0) for g in range(RV // 8) for e0 in range(0, DH, 32)]
            return [wchunk(r) for r in range(0, DH, 8)], och

        def vproj(h):
            def f(tok):
                wrow = [jnp.concatenate(
                    [jnp.broadcast_to(wof[e:e + 1, t * 128:(t + 1) * 128], (8, 128))
                     for t in range(D // 128)], axis=1) for e in range(DH)]
                tok = _wide(tok, D)
                for g in range(RV // 8):
                    rows = slice(S - RV + g * 8, S - RV + g * 8 + 8)
                    a = acc[rows, :] + tok
                    ob = obx[g]
                    for e in range(DH):
                        a = a + _wide(ob[e * 8:(e + 1) * 8, :], D) * wrow[e]
                    tok = _zero_of(a)
                    acc[rows, :] = jnp.where(h > 0, a, 0.0)
            return f

        def matvec(wv, tok=None, step=16):
            n = wv.shape[1]
            part = None if tok is None else _wide(tok, n)
            for r in range(0, D, step):
                t = wv[r:r + step, :].astype(f32) * _wide(cb_buf[r:r + step, :], n)
                for e in range(step // 8):
                    te = t[e * 8:(e + 1) * 8, :]
                    part = te if part is None else part + te
            return _rb(jnp.sum(part, axis=0, keepdims=True))

        def mod_piece(p):
            extra = isinstance(p, int) and p > NB
            modr[p] = matvec(wmx.at[p - NB - 1] if extra else w4.at[p & 1, 1])

        def finish_mod():
            n = D // MC
            ga, sb, cb, gb = (jnp.concatenate([modr[i * n + t] for t in range(n)], axis=-1)
                              for i in range(4))
            cb1 = _rb(1.0 + cb)
            wr = wr_buf[...].astype(f32).reshape(1, D)
            a = cb1 * wr
            a0 = jnp.broadcast_to(jnp.sum(a, axis=-1, keepdims=True), (1, D))
            b0 = jnp.broadcast_to(jnp.sum(sb * wr, axis=-1, keepdims=True), (1, D))
            for i, v in enumerate((ga, sb, cb1, gb, a, gb * cb1, gb * sb, a0, b0)):
                modv[i] = jnp.broadcast_to(v, (8, D))

        def out_rows(x1, mean, inv):
            return (x1 + ((x1 - _wide(mean, D)) * (_wide(inv, D) * modv[5]) + modv[6])).astype(bf16)

        def out_chunks(j):
            x1v, sv, ov = view(acc, j, TL), view(st2_buf, j, TL), view(o_buf, j, TL)

            def chunk(off):
                def f(tok):
                    rs = slice(off, off + 8)
                    ov[rs, :] = out_rows(x1v[rs, :], sv[rs, 0:128] + tok, sv[rs, 128:256] + tok)
                return f
            return [chunk(off) for off in range(0, TL, 8)]

        def epi_chunks(j, x1v, ov, with_out=True):
            sub = lax.broadcasted_iota(i32, (8, 128), 0)
            low = (0xFFFF - j * TL) - sub
            sv = view(st2_buf, j, TL)
            st = {}

            def chunk(off):
                def f(tok=None):
                    if off == 0:
                        st["k1"], st["k2"] = key_buf[0], key_buf[1]
                    x1 = x1v[off:off + 8, :]
                    mean, inv = _row_stats(x1, tok, like_bf16=True)
                    sv[off:off + 8, 0:128] = mean
                    sv[off:off + 8, 128:256] = inv
                    xa = _tiles(x1 * modv[4])
                    if tok is not None:
                        xa[0] = xa[0] + tok
                    ra = _lane_sum(_fold(jnp.add, xa))
                    r = inv * (ra - mean * modv[7, :, 0:128]) + modv[8, :, 0:128]
                    if with_out:
                        ov[off:off + 8, :] = out_rows(x1, mean, inv)
                    bits = pltpu.bitcast(_rb(r) + 0.0, i32)
                    key = jnp.where(bits < 0, bits ^ 0x7FFF0000, bits) | (low - off)
                    st["k2"] = jnp.maximum(st["k2"], jnp.minimum(st["k1"], key))
                    st["k1"] = jnp.maximum(st["k1"], key)
                    if off + 8 == TL:
                        key_buf[0], key_buf[1] = st["k1"], st["k2"]
                return f
            return [chunk(off) for off in range(0, TL, 8)]

        cp_c().start()
        cp_x(0).start()
        for c in range(2):
            cp_wq0(c).start()
            for i in range(n_mch):
                cp_ca(c, i).start()
            if c == 0:
                for j in range(1, J0):
                    cp_x(j).start()
        cp_sa().start()
        for h in range(G - 1):
            cp_k(h, sem_first.at[1 + h]).start()
        early = []
        for h in range(2):
            early += [cp_v(h, sem_first.at[8 + 2 * h]), cp_wo(h, sem_first.at[9 + 2 * h])]
        for cp in early:
            cp.start()
        start_head(0)

        cp_c().wait()
        cf = c_buf[...].astype(f32)
        sc = _rb(cf * jax.nn.sigmoid(cf))
        for t in range(4):
            sc_buf[t] = sc[:, t * (D // 4):(t + 1) * (D // 4)]

        def cb_body(t, carry):
            view(cb_buf, t, D // 4)[...] = jnp.transpose(jnp.broadcast_to(sc_buf[t], (128, D // 4)))
            return carry
        lax.fori_loop(0, 4, cb_body, 0)
        key_buf[...] = jnp.full(key_buf.shape, _IMIN, i32)
        cp_x(0).wait()

        def st0_body(i, carry):
            for ch in ln1_chunks(i, T0 // 4):
                ch()
            return carry
        lax.fori_loop(0, 4, st0_body, 0)

        def ca_half(c, stream):
            cp_wq0(c).wait()
            if not stream:
                for i in range(n_mch):
                    cp_ca(c, i).wait()
            part = None
            for i in range(n_mch):
                if stream:
                    cp_ca(c, i).wait()
                scb = jnp.broadcast_to(sc[:, i * MCH:(i + 1) * MCH], (16, MCH)).astype(bf16)
                d = jnp.dot(scb, wca[c, i * MCH:(i + 1) * MCH, :], preferred_element_type=f32)
                part = d if part is None else part + d
            mod0[1, :, c * W:(c + 1) * W] = _rb(1.0 + _rb(part[0:8, :]))

        def q_first(r0, t, c, rec, mid=None):
            rows = pl.ds(r0, t)
            cs = slice(c * W, (c + 1) * W)
            hh = ln1_scaled(x_buf[rows, cs], st_buf[rows, :], cs).astype(bf16)
            for g in range(G):
                if mid is not None and g == mid[0]:
                    mid[1]()
                part = jnp.dot(hh, wq0[cs, g * DH:(g + 1) * DH], preferred_element_type=f32)
                qf_buf[g, rows, :] = part if c == 0 else qf_buf[g, rows, :] + part
                if rec is not None:
                    rec.done(part)

        ca_half(0, True)

        def pa_body(j, carry):
            @pl.when(j + 1 < J0)
            def _():
                cp_x(j + 1).wait()
            jn = jnp.minimum(j + 1, J0 - 1)
            rec = _Pace(ln1_chunks(jn, T0), cfg["LCA"])
            q_first(_mul(j, T0), T0, 0, rec)
            return carry
        lax.fori_loop(0, J0, pa_body, 0)

        TB, RB = cfg["TB"], cfg["RB"]
        ca_half(1, False)

        def pb_body(j, carry):
            q_first(_mul(j, TB // 2), TB // 2, 1, None)
            return carry
        lax.fori_loop(0, 2, pb_body, 0)
        cp_sa().wait()
        cp_k(0, sem_first.at[1]).wait()
        cp_wr().start()
        for p in range(NB + 1, H):
            cp_wmx(p).start()

        def sa_chunk(t):
            def f(tok):
                cs = slice(t * 256, (t + 1) * 256)
                mod0[0, :, cs] = jnp.broadcast_to(matvec(wsa.at[:, cs], tok, 8), (8, 256))
            return f

        def sa_bias():
            bq_buf[...] = jnp.dot(_rep(mod0[0], 16).astype(bf16), wq0[...],
                                  preferred_element_type=f32)[0:8, :]

        def h_chunk(off):
            def f(tok):
                rs, rh = slice(off, off + RB), slice(off // 2, (off + RB) // 2)
                hh = (ln1_scaled(x_buf[rs, :], st_buf[rs, :], slice(0, D), tok)
                      + _rep(mod0[0], RB)).astype(bf16)
                h_buf[rh, :] = pltpu.bitcast(hh, u32)
            return f

        def q_chunk(off):
            def f(tok):
                n = 2 * RB
                rs, rh = slice(off, off + n), slice(off // 2, (off + n) // 2)
                for g in range(1, G):
                    q_ring[g, rh, :] = _pack(q_early(g, qf_buf[g, rs, :] + _rep(tok, n)))
            return f

        hs = [h_chunk(off) for off in range(0, S, RB)]
        qs = [q_chunk(off) for off in range(0, S, 2 * RB)]
        nh = cfg["NHB"]
        rest_chunks = []
        nq, nr = len(qs), len(hs) - nh
        for i, ch in enumerate(hs[nh:]):
            rest_chunks.append(ch)
            while qs and (nq - len(qs)) * nr < (i + 1) * nq:
                rest_chunks.append(qs.pop(0))
        assert not qs
        rec = _Pace([sa_chunk(t) for t in range(D // 256)] + hs[:nh], cfg["LCB2"])
        q_first(TB, S - TB, 1, rec, mid=(cfg["BQ"], sa_bias))
        n4 = len(rest_chunks)
        n3 = n4 - cfg["NL4"]
        cnt = [n3 // 3 + (1 if i < n3 % 3 else 0) for i in range(3)] + [cfg["NL4"]]
        scores(0, q_early(0, qf_buf[0]).astype(bf16), s_buf, m_buf, rec=_Pace(rest_chunks, cnt))

        def main_body(h, carry):
            wch, och = expand_chunks(h)
            rec = _mix((pack_chunks(h), cfg["LCM"]), ([vproj(h)], cfg["LCV"]),
                       (wch, cfg["LCW"]), (och, cfg["LCO"]))
            o = pv(h, s_buf, m_buf, rec=rec)
            ov_buf[...] = _rb(o[S - RV:, :])
            qproj(h + G, w4.at[h & 1, 0], rec=rec)
            start_head(h + 1)
            scores(h + 1, pltpu.bitcast(q_ring[(h + 1) & 3], bf16), s_buf, m_buf, rec=rec,
                   partial=True)
            oproj([(h, o[0:S - RV, :])], acc.at[0:S - RV, :], rec=rec)
            mod_piece(h)
            wait_head(h + 1)
            return carry
        for h in range(1, G - 1):
            cp_k(h, sem_first.at[1 + h]).wait()
        for cp in early:
            cp.wait()
        wait_head(0)
        lax.fori_loop(0, NB, main_body, 0)

        ha = NB
        rest = list(zip(range(NB + 1, H), (s2_buf, s3_buf, s4_buf), (m2_buf, m3_buf, m4_buf)))
        late = []
        for n, h in enumerate(range(NB + 3, H)):
            late += [cp_v(h, sem_first.at[8 + 2 * n]), cp_wo(h, sem_first.at[9 + 2 * n])]
        cp_wr().wait()
        for p in range(NB + 1, H):
            cp_wmx(p).wait()
        oproj([(NB - 1, ov_buf[...])], acc.at[S - RV:, :])
        for cp in late:
            cp.start()

        def l_step(j, do_x, do_y):
            if do_x and do_y:
                aw = view(acc, j - 1, TL, 2)
                ay, ax = aw.at[0:TL, :], aw.at[TL:2 * TL, :]
            elif do_x:
                ax = view(acc, j, TL)
            else:
                ay = view(acc, j - 1, TL)
            rec = None
            if do_y:
                chunks = epi_chunks(j - 1, ay, view(o_buf, j - 1, TL), with_out=do_x)
                os_ = [(h, pv(h, sv, mv, late=not do_x)) for h, sv, mv in rest]
            if do_x:
                oa = pv(ha, view(s_buf, j, TL), view(m_buf, j, TL))
            if do_y and do_x:
                oproj(os_, ay, view(x_buf, j - 1, TL))
            elif do_y:
                xv = view(x_buf, j - 1, TL)
                r0, prev = 0, []
                for n in cfg["LSPLIT"]:
                    rs = slice(r0, r0 + n)
                    nr = len(os_) * (D // W)
                    cnt = [len(prev) // nr + (1 if i < len(prev) % nr else 0) for i in range(nr)]
                    rec = _Pace(prev, cnt)
                    oproj([(h, o[rs]) for h, o in os_], ay.at[rs, :], xv.at[rs, :], rec=rec)
                    prev = chunks[r0 // 8:(r0 + n) // 8]
                    r0 += n
                chunks = prev
            if do_x:
                if do_y:
                    rec = _Pace(chunks, cfg["LCNT"])
                for h, sv, mv in rest:
                    q = pltpu.bitcast(view(q_ring.at[h & 3], j, TL // 2)[...], bf16)
                    scores(h, q, sv, mv, rec=rec)
                oproj([(ha, oa)], ax, rec=rec)
            if do_y:
                if do_x:
                    cp_out(j - 1).start()
                else:
                    for ch in chunks:
                        ch()

        for p in range(NB, H):
            mod_piece(p)
        finish_mod()
        l_step(0, True, False)
        for cp in late:
            cp.wait()

        def pl_body(j, carry):
            l_step(j, True, True)
            return carry
        lax.fori_loop(1, JL, pl_body, 0)
        l_step(JL, False, True)

        k1, k2 = key_buf[0], key_buf[1]
        for sh in (4, 2, 1):
            o1, o2 = pltpu.roll(k1, sh, 0), pltpu.roll(k2, sh, 0)
            k2 = jnp.maximum(jnp.minimum(k1, o1), jnp.maximum(k2, o2))
            k1 = jnp.maximum(k1, o1)

        def score_of(k):
            hi = k & jnp.int32(-65536)
            return pltpu.bitcast(jnp.where(hi < 0, hi ^ 0x7FFF0000, hi), f32)

        i1s = jnp.minimum(0xFFFF - (k1[0, 0] & 0xFFFF), S - 1)
        i2s = jnp.minimum(0xFFFF - (k2[0, 0] & 0xFFFF), S - 1)

        sub = lax.broadcasted_iota(i32, (16, D), 0)
        sb, cb1, gb = (_rep(modv[i], 16) for i in (1, 2, 3))

        def adaln2(x1, stat):
            return (x1 - _wide(stat[:, 0:128], D)) * _wide(stat[:, 128:256], D) * cb1 + sb

        def pick(ref):
            sel = lax.broadcasted_iota(i32, (16, ref.shape[1]), 0) == 0
            return jnp.where(sel, ref[pl.ds(i1s, 1), :], ref[pl.ds(i2s, 1), :])

        xs = adaln2(pick(acc), pick(st2_buf)).astype(bf16)
        FC, lag = cfg["FC"], cfg["FLAG"]
        kvs = [int(ch) for ch in cfg["LKV"]]
        fout = [int(ch, 36) for ch in cfg["LFO"]]
        KV = max(kvs)

        def wrows(ref, a, b, c):
            n = FC // 128
            u = [ref[c * n + t, a // 2:b // 2, :] for t in range(n)]
            return pltpu.bitcast(u[0] if n == 1 else jnp.concatenate(u, axis=1), bf16)

        DV = D - KV * 128
        if KV:
            xf = xs.astype(f32)
            for r in range(2):
                xc_buf[r] = jnp.transpose(jnp.broadcast_to(xf[r:r + 1, DV:], (128, D - DV)))
        subc = lax.broadcasted_iota(i32, (8, FC), 0)
        y = None
        act = []
        outs = out_chunks(JL - 1)
        for c in range(F // FC + lag):
            if c < F // FC:
                dm = D - kvs[c] * 128
                gu = [jnp.dot(xs[:, :dm], wrows(w, 0, dm, c), preferred_element_type=f32)[0:8, :]
                      for w in (wg, wu)]
                for v in gu:
                    for t in range(fout[c] if c < len(fout) else 0):
                        if outs:
                            outs.pop(0)(_zero_of(v[0:8, (t % 2) * 128:(t % 2 + 1) * 128]))
                            if not outs:
                                cp_out(JL - 1).start()
                if dm < D:
                    part = [[None, None], [None, None]]
                    for k in range(dm, D, 16):
                        xcol = [_wide(xc_buf[r, k - DV:k - DV + 16, :], FC) for r in range(2)]
                        for m, w in enumerate((wg, wu)):
                            wv = wrows(w, k, k + 16, c).astype(f32)
                            for r in range(2):
                                t = wv * xcol[r]
                                for e in range(2):
                                    te = t[e * 8:(e + 1) * 8, :]
                                    part[m][r] = te if part[m][r] is None else part[m][r] + te
                    for m in range(2):
                        ra, rb_ = (jnp.sum(v, axis=0, keepdims=True) for v in part[m])
                        gu[m] = gu[m] + jnp.where(subc == 0, ra, rb_)
                g, u = _rb(gu[0]), _rb(gu[1])
                act.append(_rep(_rb(g * jax.nn.sigmoid(g)) * u, 16).astype(bf16))
            if c >= lag:
                wdc = pltpu.bitcast(wd[(c - lag) * FC // 2:(c - lag + 1) * FC // 2, :], bf16)
                d = jnp.dot(act[c - lag], wdc, preferred_element_type=f32)[0:8, :]
                y = d if y is None else y + d
        y = _rb(y)
        ya = _rb(y[0:1, :] * _wide(_rb(jax.nn.sigmoid(score_of(k1[0:1, :]))), D))
        yb = _rb(y[1:2, :] * _wide(_rb(jax.nn.sigmoid(score_of(k2[0:1, :]))), D))

        g1 = pl.multiple_of((i1s >> 4) << 4, 16)
        g2 = pl.multiple_of((i2s >> 4) << 4, 16)
        for t, g0 in enumerate((g1, g2)):
            rid = sub + g0
            x1 = acc[pl.ds(g0, 16), :]
            upd = jnp.where(rid == i1s, ya, 0.0) + jnp.where(rid == i2s, yb, 0.0)
            fix[t] = (x1 + gb * (adaln2(x1, st2_buf[pl.ds(g0, 16), :]) + upd)).astype(bf16)

        pltpu.make_async_copy(o_buf, out_hbm, sem_out.at[0]).wait()

        def cp_fix(t, g0):
            return pltpu.make_async_copy(fix.at[t], out_hbm.at[pl.ds(g0, 16), :], sem_fix.at[t])

        cp_fix(0, g1).start()

        @pl.when(g2 != g1)
        def _():
            cp_fix(1, g2).start()
            cp_fix(1, g2).wait()
        cp_fix(0, g1).wait()

    return kernel


_CFG = dict(
    G=4, T0=256, TB=1024, TL=256, MCH=256, RB=16, FC=256, PKN=8, RV=160,
    LCA='cc80', LCB2='040g', NHB=16, NL4=8, BQ=3, LCNT='33333333332000',
    LCM='cc0000000000', LCV='000010000000', LCW='00000000000g', LCO='000006bbb0z6',
    LSPLIT=(96, 96, 64), FLAG=1, LKV='00233333333333', LFO='88',
)


def _build(A_x, A_k_cache, A_v_cache, A_wq, A_wo, B_w_r, B_w_gate, B_w_up, B_w_down, c, w_mod,
           **over):
    B, S, D = A_x.shape
    _, H, SK, DH = A_k_cache.shape
    F = B_w_gate.shape[1]
    assert B == 1
    cfg = dict(_CFG, **over)
    T0, TL, G = cfg["T0"], cfg["TL"], cfg["G"]
    MC = (4 * D) // H
    kernel = _make_kernel(S, D, H, DH, SK, F, cfg)
    scratch = [
        pltpu.VMEM((S, D), bf16),
        pltpu.VMEM((S // 2, D), u32),
        pltpu.VMEM((S, D), f32),
        pltpu.VMEM((S, SK), f32),
        pltpu.VMEM((S, 128), f32),
        pltpu.VMEM((TL, SK), f32),
        pltpu.VMEM((TL, 128), f32),
        pltpu.VMEM((TL, SK), f32),
        pltpu.VMEM((TL, 128), f32),
        pltpu.VMEM((TL, SK), f32),
        pltpu.VMEM((TL, 128), f32),
        pltpu.VMEM((S, 256), f32),
        pltpu.VMEM((S, 256), f32),
        pltpu.VMEM((1, S, SK // 4 - 128), f32),
        pltpu.VMEM((4, S // 2, DH), u32),
        pltpu.VMEM((G, S, DH), f32),
        pltpu.VMEM((8, G * DH), f32),
        pltpu.VMEM((4, SK, DH), bf16),
        pltpu.VMEM((4, SK, DH), bf16),
        pltpu.VMEM((D, G * DH), bf16),
        pltpu.VMEM((2, 4, D, 128), bf16),
        pltpu.VMEM((4, 2, DH, D), bf16),
        pltpu.VMEM((G - 1, D, MC), bf16),
        pltpu.VMEM((2, D, D // 2), bf16),
        pltpu.VMEM((D, D), bf16),
        pltpu.VMEM((1, D), bf16),
        pltpu.VMEM((D,), bf16),
        pltpu.VMEM((4, 1, D // 4), f32),
        pltpu.VMEM((D, 128), f32),
        pltpu.VMEM((2, 8, D), f32),
        pltpu.VMEM((H, 1, MC), f32),
        pltpu.VMEM((9, 8, D), f32),
        pltpu.VMEM((F // 128, D // 2, 128), u32),
        pltpu.VMEM((F // 128, D // 2, 128), u32),
        pltpu.VMEM((F // 2, D), u32),
        pltpu.VMEM((2, max(int(max(cfg["LKV"])), 1) * 128, 128), f32),
        pltpu.VMEM((cfg["RV"], DH), f32),
        pltpu.VMEM((cfg["RV"] // 8, DH * 8, 128), f32),
        pltpu.VMEM((DH, D), f32),
        pltpu.VMEM((S, D), bf16),
        pltpu.VMEM((2, 8, 128), i32),
        pltpu.VMEM((2, 16, D), bf16),
        pltpu.SemaphoreType.DMA((sum(_sem_sizes(S, D, cfg)),)),
    ]
    any_spec = pl.BlockSpec(memory_space=pl.ANY)
    out = pl.pallas_call(
        kernel,
        out_shape=jax.ShapeDtypeStruct((S, D), bf16),
        in_specs=[any_spec] * 11,
        out_specs=any_spec,
        scratch_shapes=scratch,
        compiler_params=pltpu.CompilerParams(vmem_limit_bytes=126 * 1024 * 1024,
                                             disable_bounds_checks=True,
                                             disable_semaphore_checks=True),
    )(A_x.reshape(S, D), A_k_cache.reshape(H, SK, DH), A_v_cache.reshape(H, SK, DH),
      A_wq, A_wo, B_w_r, B_w_gate, B_w_up, B_w_down, c, w_mod)
    return out.reshape(B, S, D)


@jax.jit
def pallas_adaLN_cond__mha_block_cached__moe_arch_mod__prompt_kernel(
    A_x: jax.Array,
    A_k_cache: jax.Array,
    A_v_cache: jax.Array,
    A_wq: jax.Array,
    A_wo: jax.Array,
    B_x: jax.Array,
    B_w_r: jax.Array,
    B_w_gate: jax.Array,
    B_w_up: jax.Array,
    B_w_down: jax.Array,
    c: jax.Array,
    w_mod: jax.Array,
):
    del B_x
    return _build(A_x, A_k_cache, A_v_cache, A_wq, A_wo, B_w_r, B_w_gate, B_w_up, B_w_down,
                  c, w_mod)
```

```python
import jax
import jax.numpy as jnp
from jax import lax
import jax.experimental.pallas as pl
import jax.experimental.pallas.tpu as pltpu

f32 = jnp.float32
bf16 = jnp.bfloat16
u32 = jnp.uint32
i32 = jnp.int32

_NT = (((1,), (1,)), ((), ()))
_LOG2E = 1.4426950408889634
_EPS = 1e-5
_IMIN = -2 ** 31


def _rb(v):
    return v.astype(bf16).astype(f32)


def _rep(v, n):
    return v if n == 8 else jnp.tile(v, (n // 8, 1))


def _wide(v, w):
    return jnp.tile(v, (1, w // 128))


def _pack(v):
    return pltpu.bitcast(v.astype(bf16), u32)


def _zero_of(v):
    bits = pltpu.bitcast(v, u32)
    return pltpu.bitcast(lax.shift_right_logical(lax.shift_right_logical(bits, jnp.uint32(31)),
                                                 jnp.uint32(1)), f32)


class _Pace:
    def __init__(self, chunks, counts):
        self.chunks = list(chunks)
        self.counts = [ch if isinstance(ch, int) else int(ch, 36) for ch in counts]
        assert sum(self.counts) == len(self.chunks), (counts, len(self.chunks))

    def done(self, res):
        n = self.counts.pop(0)
        for i in range(n):
            r0 = (i * res.shape[0] // n) // 8 * 8
            self.chunks.pop(0)(_zero_of(res[r0:r0 + 8, 0:128]))


def _mix(*plans):
    plans = [(list(ch), [c if isinstance(c, int) else int(c, 36) for c in cnt]) for ch, cnt in plans]
    for ch, cnt in plans:
        assert sum(cnt) == len(ch), (cnt, len(ch))
    fill, total = [], []
    for r in range(len(plans[0][1])):
        slots = sorted((i / cnt[r], k) for k, (_, cnt) in enumerate(plans)
                       for i in range(cnt[r]))
        fill += [plans[k][0].pop(0) for _, k in slots]
        total.append(len(slots))
    return _Pace(fill, total)


def _tiles(v):
    return [v[:, c * 128:(c + 1) * 128] for c in range(v.shape[1] // 128)]


def _fold(op, parts):
    out = parts[0]
    for p in parts[1:]:
        out = op(out, p)
    return out


def _lane_sum(v):
    return jnp.broadcast_to(jnp.sum(v, axis=-1, keepdims=True), v.shape)


def _row_stats(xf, tok=None, like_bf16=False):
    d = xf.shape[-1]
    ts = _tiles(xf)
    nt = len(ts)
    if tok is not None:
        ts = [ts[0] + tok] + ts[1:]
    mu = _fold(jnp.add, ts) * (1.0 / nt)
    m2 = _fold(jnp.add, [(t - mu) * (t - mu) for t in ts])
    mean = _lane_sum(mu) * (1.0 / 128)
    dm = mu - mean
    var = _lane_sum(m2 + (dm * dm) * float(nt)) * (1.0 / d)
    if not like_bf16:
        return mean, lax.rsqrt(var + _EPS)
    v = _rb(_rb(var) + _EPS)
    y = lax.rsqrt(v)
    sig = _rb(v * y)
    return mean, y * (2.0 - sig * y)


def _sem_sizes(S, D, cfg):
    j0 = S // cfg["T0"]
    return [2, 2 * (D // cfg["MCH"]), j0, 1, 16, 4, 1, 2]


def _make_kernel(S, D, H, DH, SK, F, cfg):
    T0, TL, MCH = cfg["T0"], cfg["TL"], cfg["MCH"]
    J0 = S // T0
    JL = S // TL
    qscale = DH ** -0.5 * _LOG2E
    n_mch = D // MCH
    G = cfg["G"]
    NB = H - G
    MC = (4 * D) // H
    W = 512
    NF = F // 128
    assert H < 256 and 2 <= G <= 4 and D == 2 * W and MC == DH == 128 and NF <= NB

    def kernel(x_hbm, k_hbm, v_hbm, wq_hbm, wo_hbm, wr_hbm, wg_hbm, wu_hbm, wd_hbm,
               c_hbm, wmod_hbm, out_hbm,
               x_buf, h_buf, acc, s_buf, m_buf, s2_buf, m2_buf, s3_buf, m3_buf, s4_buf, m4_buf,
               st_buf, st2_buf, mp_buf,
               q_ring, qf_buf, bq_buf,
               kb, vb, wq0, w4, wo2, wmx, wca, wsa, c_buf, wr_buf, sc_buf, cb_buf, mod0, modr, modv,
               wg, wu, wd, xc_buf, ov_buf, obx, wof, o_buf, key_buf, fix,
               sems):

        class _Sem:
            def __init__(self, base):
                self.base = base
                self.at = self

            def __getitem__(self, i):
                return sems.at[self.base + i]

        sizes = _sem_sizes(S, D, cfg)
        offs = [sum(sizes[:i]) for i in range(len(sizes))]
        (sem_small, sem_ca, sem_x, sem_sa, sem_first, sem_head,
         sem_out, sem_fix) = (_Sem(o) for o in offs)

        def _mul(a, n):
            v = a * n
            return v if isinstance(a, int) else pl.multiple_of(v, n)

        def view(ref, j, t, n=1):
            return ref.at[pl.ds(_mul(j, t), n * t), :]

        def cp_c():
            return pltpu.make_async_copy(c_hbm, c_buf, sem_small.at[0])

        def cp_wr():
            return pltpu.make_async_copy(wr_hbm, wr_buf, sem_small.at[1])

        def cp_ca(c, i):
            return pltpu.make_async_copy(
                wmod_hbm.at[pl.ds(i * MCH, MCH), pl.ds(D + c * W, W)], view(wca.at[c], i, MCH),
                sem_ca.at[c * n_mch + i])

        def cp_sa():
            return pltpu.make_async_copy(wmod_hbm.at[:, pl.ds(0, D)], wsa, sem_sa.at[0])

        def cp_x(j):
            return pltpu.make_async_copy(view(x_hbm, j, T0), view(x_buf, j, T0), sem_x.at[j])

        def cp_wq0(c):
            return pltpu.make_async_copy(wq_hbm.at[pl.ds(c * W, W), pl.ds(0, G * DH)],
                                         view(wq0, c, W), sem_first.at[14 + c])

        def cp_k(h, sem=None):
            return pltpu.make_async_copy(k_hbm.at[h], kb.at[h & 3],
                                         sem_head.at[0] if sem is None else sem)

        def cp_v(h, sem=None):
            return pltpu.make_async_copy(v_hbm.at[h], vb.at[h & 3],
                                         sem_head.at[1] if sem is None else sem)

        def cp_wo(h, sem=None):
            return pltpu.make_async_copy(view(wo_hbm, h, DH), wo2.at[h & 3, 0],
                                         sem_head.at[2] if sem is None else sem)

        def _clamp(a, hi):
            return min(a, hi) if isinstance(a, int) else jnp.minimum(a, hi)

        def cols(ref, t):
            return ref.at[:, pl.ds(_mul(t, 128), 128)]

        def cp_wmx(p):
            return pltpu.make_async_copy(cols(wmod_hbm, p + (2 * D) // MC), wmx.at[p - NB - 1],
                                         sem_first.at[4 + p - NB])

        def start_head(h):
            f = _clamp(h, NF - 1)
            for i, src in enumerate((cols(wq_hbm, _clamp(h + G, H - 1)),
                                     cols(wmod_hbm, h + (2 * D) // MC),
                                     cols(wg_hbm, f), cols(wu_hbm, f))):
                pltpu.make_async_copy(src, w4.at[h & 1, i], sem_head.at[3]).start()
            cp_k(h + G - 1).start()
            cp_wo(h + 2).start()
            pltpu.make_async_copy(view(wd_hbm, f, 128), wo2.at[(h + 2) & 3, 1],
                                  sem_head.at[2]).start()
            cp_v(h + 2).start()

        def wait_head(h):
            pltpu.make_async_copy(w4.at[h & 1], w4.at[h & 1], sem_head.at[3]).wait()
            cp_k(h + G - 1).wait()
            pltpu.make_async_copy(wo2.at[(h + 2) & 3], wo2.at[(h + 2) & 3], sem_head.at[2]).wait()
            cp_v(h + 2).wait()

        def pack_chunks(h):
            f = _clamp(h, NF - 1)
            out = []
            for sv, dv in ((w4.at[h & 1, 2], wg.at[f]), (w4.at[h & 1, 3], wu.at[f]),
                           (wo2.at[(h + 2) & 3, 1], view(wd, f, 64))):
                n, w = sv.shape
                step = n // cfg['PKN']

                def chunk(r, sv=sv, dv=dv, step=step, w=w):
                    def fn(tok):
                        z = _rep(_wide(pltpu.bitcast(tok, u32), w), step // 2)
                        dv[r // 2:(r + step) // 2, :] = pltpu.bitcast(sv[r:r + step, :], u32) | z
                    return fn
                out += [chunk(r) for r in range(0, n, step)]
            return out

        def cp_out(j):
            return pltpu.make_async_copy(view(o_buf, j, TL), view(out_hbm, j, TL), sem_out.at[0])

        def ln1_chunks(j, t):
            xv, sv, av = view(x_buf, j, t), view(st_buf, j, t), view(acc, j, t)

            def chunk(off):
                def f(tok=None):
                    av[off:off + 8, :] = jnp.zeros((8, D), f32) if tok is None else _wide(tok, D)
                    mean, inv = _row_stats(xv[off:off + 8, :].astype(f32), tok)
                    sv[off:off + 8, 0:128] = mean
                    sv[off:off + 8, 128:256] = inv
                return f
            return [chunk(off) for off in range(0, xv.shape[0], 8)]

        def ln1_scaled(x, stat, cs, tok=None):
            w = x.shape[1]
            mean = stat[:, 0:128] if tok is None else stat[:, 0:128] + _rep(tok, x.shape[0])
            n = (x.astype(f32) - _wide(mean, w)) * _wide(stat[:, 128:256], w)
            return n * _rep(mod0[1, :, cs], x.shape[0])

        def qproj(h, wv, rec=None):
            q = None
            for c in range(D // W):
                cs = slice(c * W, (c + 1) * W)
                part = jnp.dot(pltpu.bitcast(h_buf[:, cs], bf16), wv[cs, :],
                               preferred_element_type=f32)
                q = part if q is None else q + part
                if rec is not None:
                    rec.done(part)
            q_ring[h & 3] = _pack(q * qscale)

        def q_early(g, q):
            return (q + _rep(bq_buf[:, g * DH:(g + 1) * DH], q.shape[0])) * qscale

        def scores(h, q, sv, mv, rec, partial=False):
            nr = SK // W
            for c in range(nr):
                cs = slice(c * W, (c + 1) * W)
                s = lax.dot_general(q, kb[h & 3, cs, :], _NT, preferred_element_type=f32)
                if partial:
                    t = _tiles(s)
                    mp = jnp.maximum(jnp.maximum(t[0], t[1]), jnp.maximum(t[2], t[3]))
                    if c < nr - 1:
                        z = lax.shift_right_logical(h, 8)
                        mp_buf[z, :, c * 128:(c + 1) * 128] = mp
                sv[:, cs] = s
                if rec is not None:
                    rec.done(s)
            mp = _fold(jnp.maximum, [mp] + _tiles(mp_buf[0]) if partial else _tiles(sv[...]))
            mv[...] = jnp.broadcast_to(jnp.max(mp, axis=-1, keepdims=True), mp.shape)

        def pv(h, sv, mv, rec=None, late=False):
            o = lp = None
            for c in range(SK // W):
                cs = slice(c * W, (c + 1) * W)
                m = mv[...]
                if c >= 2 and sv.shape[0] == S:
                    m = m + _zero_of(lp)
                p = jnp.exp2(sv[:, cs] - _wide(m, W))
                lp = _fold(jnp.add, ([] if lp is None else [lp]) + _tiles(p))
                d = jnp.dot(p.astype(bf16), vb[h & 3, cs, :], preferred_element_type=f32)
                o = d if o is None else o + d
                if rec is not None:
                    rec.done(d)
            if late:
                lp = lp + _zero_of(o)
            l = jnp.sum(lp, axis=-1, keepdims=True)
            r = pl.reciprocal(l, approx=True)
            r = r * (2.0 - l * r)
            return o * r

        def oproj(hos, av, xv=None, rec=None):
            for c in range(D // W):
                cs = slice(c * W, (c + 1) * W)
                a = av[:, cs]
                for h, o in hos:
                    d = jnp.dot(o.astype(bf16), wo2[h & 3, 0, :, cs], preferred_element_type=f32)
                    if rec is not None:
                        rec.done(d)
                    a = a + d
                if xv is not None:
                    a = xv[:, cs].astype(f32) + _rep(modv[0, :, cs], a.shape[0]) * a
                av[:, cs] = a

        RV = cfg["RV"]

        def expand_chunks(h):
            def wchunk(r):
                def f(tok):
                    wof[r:r + 8, :] = wo2[h & 3, 0, r:r + 8, :].astype(f32) + _wide(tok, D)
                return f

            lane = lax.broadcasted_iota(i32, (8, 128), 1)

            def ochunk(g, e0):
                def f(tok):
                    o = ov_buf[g * 8:(g + 1) * 8, :] + tok
                    rs = slice(e0 * 8, (e0 + 32) * 8)
                    cols = jnp.concatenate(
                        [jnp.where(lane == e, o, 0.0) for e in range(e0, e0 + 32)], axis=0)
                    obx[g, rs, :] = _lane_sum(cols)
                return f
            och = [ochunk(g, e0) for g in range(RV // 8) for e0 in range(0, DH, 32)]
            return [wchunk(r) for r in range(0, DH, 8)], och

        def vproj(h):
            def f(tok):
                wrow = [jnp.concatenate(
                    [jnp.broadcast_to(wof[e:e + 1, t * 128:(t + 1) * 128], (8, 128))
                     for t in range(D // 128)], axis=1) for e in range(DH)]
                tok = _wide(tok, D)
                for g in range(RV // 8):
                    rows = slice(S - RV + g * 8, S - RV + g * 8 + 8)
                    a = acc[rows, :] + tok
                    ob = obx[g]
                    for e in range(DH):
                        a = a + _wide(ob[e * 8:(e + 1) * 8, :], D) * wrow[e]
                    tok = _zero_of(a)
                    acc[rows, :] = jnp.where(h > 0, a, 0.0)
            return f

        def matvec(wv, tok=None, step=16):
            n = wv.shape[1]
            part = None if tok is None else _wide(tok, n)
            for r in range(0, D, step):
                t = wv[r:r + step, :].astype(f32) * _wide(cb_buf[r:r + step, :], n)
                for e in range(step // 8):
                    te = t[e * 8:(e + 1) * 8, :]
                    part = te if part is None else part + te
            return _rb(jnp.sum(part, axis=0, keepdims=True))

        def mod_piece(p):
            extra = isinstance(p, int) and p > NB
            modr[p] = matvec(wmx.at[p - NB - 1] if extra else w4.at[p & 1, 1])

        def finish_mod():
            n = D // MC
            ga, sb, cb, gb = (jnp.concatenate([modr[i * n + t] for t in range(n)], axis=-1)
                              for i in range(4))
            cb1 = _rb(1.0 + cb)
            wr = wr_buf[...].astype(f32).reshape(1, D)
            a = cb1 * wr
            a0 = jnp.broadcast_to(jnp.sum(a, axis=-1, keepdims=True), (1, D))
            b0 = jnp.broadcast_to(jnp.sum(sb * wr, axis=-1, keepdims=True), (1, D))
            for i, v in enumerate((ga, sb, cb1, gb, a, gb * cb1, gb * sb, a0, b0)):
                modv[i] = jnp.broadcast_to(v, (8, D))

        def out_rows(x1, mean, inv):
            return (x1 + ((x1 - _wide(mean, D)) * (_wide(inv, D) * modv[5]) + modv[6])).astype(bf16)

        def out_chunks(j):
            x1v, sv, ov = view(acc, j, TL), view(st2_buf, j, TL), view(o_buf, j, TL)

            def chunk(off):
                def f(tok):
                    rs = slice(off, off + 8)
                    ov[rs, :] = out_rows(x1v[rs, :], sv[rs, 0:128] + tok, sv[rs, 128:256] + tok)
                return f
            return [chunk(off) for off in range(0, TL, 8)]

        def epi_chunks(j, x1v, ov, with_out=True):
            sub = lax.broadcasted_iota(i32, (8, 128), 0)
            low = (0xFFFF - j * TL) - sub
            sv = view(st2_buf, j, TL)
            st = {}

            def chunk(off):
                def f(tok=None):
                    if off == 0:
                        st["k1"], st["k2"] = key_buf[0], key_buf[1]
                    x1 = x1v[off:off + 8, :]
                    mean, inv = _row_stats(x1, tok, like_bf16=True)
                    sv[off:off + 8, 0:128] = mean
                    sv[off:off + 8, 128:256] = inv
                    xa = _tiles(x1 * modv[4])
                    if tok is not None:
                        xa[0] = xa[0] + tok
                    ra = _lane_sum(_fold(jnp.add, xa))
                    r = inv * (ra - mean * modv[7, :, 0:128]) + modv[8, :, 0:128]
                    if with_out:
                        ov[off:off + 8, :] = out_rows(x1, mean, inv)
                    bits = pltpu.bitcast(_rb(r) + 0.0, i32)
                    key = jnp.where(bits < 0, bits ^ 0x7FFF0000, bits) | (low - off)
                    st["k2"] = jnp.maximum(st["k2"], jnp.minimum(st["k1"], key))
                    st["k1"] = jnp.maximum(st["k1"], key)
                    if off + 8 == TL:
                        key_buf[0], key_buf[1] = st["k1"], st["k2"]
                return f
            return [chunk(off) for off in range(0, TL, 8)]

        cp_c().start()
        cp_x(0).start()
        for c in range(2):
            cp_wq0(c).start()
            for i in range(n_mch):
                cp_ca(c, i).start()
            if c == 0:
                for j in range(1, J0):
                    cp_x(j).start()
        cp_sa().start()
        for h in range(G - 1):
            cp_k(h, sem_first.at[1 + h]).start()
        early = []
        for h in range(2):
            early += [cp_v(h, sem_first.at[8 + 2 * h]), cp_wo(h, sem_first.at[9 + 2 * h])]
        for cp in early:
            cp.start()
        start_head(0)

        cp_c().wait()
        cf = c_buf[...].astype(f32)
        sc = _rb(cf * jax.nn.sigmoid(cf))
        for t in range(4):
            sc_buf[t] = sc[:, t * (D // 4):(t + 1) * (D // 4)]

        def cb_body(t, carry):
            view(cb_buf, t, D // 4)[...] = jnp.transpose(jnp.broadcast_to(sc_buf[t], (128, D // 4)))
            return carry
        lax.fori_loop(0, 4, cb_body, 0)
        key_buf[...] = jnp.full(key_buf.shape, _IMIN, i32)
        cp_x(0).wait()

        def st0_body(i, carry):
            for ch in ln1_chunks(i, T0 // 4):
                ch()
            return carry
        lax.fori_loop(0, 4, st0_body, 0)

        def ca_half(c, stream):
            cp_wq0(c).wait()
            if not stream:
                for i in range(n_mch):
                    cp_ca(c, i).wait()
            part = None
            for i in range(n_mch):
                if stream:
                    cp_ca(c, i).wait()
                scb = jnp.broadcast_to(sc[:, i * MCH:(i + 1) * MCH], (16, MCH)).astype(bf16)
                d = jnp.dot(scb, wca[c, i * MCH:(i + 1) * MCH, :], preferred_element_type=f32)
                part = d if part is None else part + d
            mod0[1, :, c * W:(c + 1) * W] = _rb(1.0 + _rb(part[0:8, :]))

        def q_first(r0, t, c, rec, mid=None):
            rows = pl.ds(r0, t)
            cs = slice(c * W, (c + 1) * W)
            hh = ln1_scaled(x_buf[rows, cs], st_buf[rows, :], cs).astype(bf16)
            for g in range(G):
                if mid is not None and g == mid[0]:
                    mid[1]()
                part = jnp.dot(hh, wq0[cs, g * DH:(g + 1) * DH], preferred_element_type=f32)
                qf_buf[g, rows, :] = part if c == 0 else qf_buf[g, rows, :] + part
                if rec is not None:
                    rec.done(part)

        ca_half(0, True)

        def pa_body(j, carry):
            @pl.when(j + 1 < J0)
            def _():
                cp_x(j + 1).wait()
            jn = jnp.minimum(j + 1, J0 - 1)
            rec = _Pace(ln1_chunks(jn, T0), cfg["LCA"])
            q_first(_mul(j, T0), T0, 0, rec)
            return carry
        lax.fori_loop(0, J0, pa_body, 0)

        TB, RB = cfg["TB"], cfg["RB"]
        ca_half(1, False)

        def pb_body(j, carry):
            q_first(_mul(j, TB // 2), TB // 2, 1, None)
            return carry
        lax.fori_loop(0, 2, pb_body, 0)
        cp_sa().wait()
        cp_k(0, sem_first.at[1]).wait()
        cp_wr().start()
        for p in range(NB + 1, H):
            cp_wmx(p).start()

        def sa_chunk(t):
            def f(tok):
                cs = slice(t * 256, (t + 1) * 256)
                mod0[0, :, cs] = jnp.broadcast_to(matvec(wsa.at[:, cs], tok, 8), (8, 256))
            return f

        def sa_bias():
            bq_buf[...] = jnp.dot(_rep(mod0[0], 16).astype(bf16), wq0[...],
                                  preferred_element_type=f32)[0:8, :]

        def h_chunk(off):
            def f(tok):
                rs, rh = slice(off, off + RB), slice(off // 2, (off + RB) // 2)
                hh = (ln1_scaled(x_buf[rs, :], st_buf[rs, :], slice(0, D), tok)
                      + _rep(mod0[0], RB)).astype(bf16)
                h_buf[rh, :] = pltpu.bitcast(hh, u32)
            return f

        def q_chunk(off):
            def f(tok):
                n = 2 * RB
                rs, rh = slice(off, off + n), slice(off // 2, (off + n) // 2)
                for g in range(1, G):
                    q_ring[g, rh, :] = _pack(q_early(g, qf_buf[g, rs, :] + _rep(tok, n)))
            return f

        hs = [h_chunk(off) for off in range(0, S, RB)]
        qs = [q_chunk(off) for off in range(0, S, 2 * RB)]
        nh = cfg["NHB"]
        rest_chunks = []
        nq, nr = len(qs), len(hs) - nh
        for i, ch in enumerate(hs[nh:]):
            rest_chunks.append(ch)
            while qs and (nq - len(qs)) * nr < (i + 1) * nq:
                rest_chunks.append(qs.pop(0))
        assert not qs
        rec = _Pace([sa_chunk(t) for t in range(D // 256)] + hs[:nh], cfg["LCB2"])
        q_first(TB, S - TB, 1, rec, mid=(cfg["BQ"], sa_bias))
        n4 = len(rest_chunks)
        n3 = n4 - cfg["NL4"]
        cnt = [n3 // 3 + (1 if i < n3 % 3 else 0) for i in range(3)] + [cfg["NL4"]]
        scores(0, q_early(0, qf_buf[0]).astype(bf16), s_buf, m_buf, rec=_Pace(rest_chunks, cnt))

        def main_body(h, carry):
            wch, och = expand_chunks(h)
            rec = _mix((pack_chunks(h), cfg["LCM"]), ([vproj(h)], cfg["LCV"]),
                       (wch, cfg["LCW"]), (och, cfg["LCO"]))
            o = pv(h, s_buf, m_buf, rec=rec)
            ov_buf[...] = _rb(o[S - RV:, :])
            qproj(h + G, w4.at[h & 1, 0], rec=rec)
            start_head(h + 1)
            scores(h + 1, pltpu.bitcast(q_ring[(h + 1) & 3], bf16), s_buf, m_buf, rec=rec,
                   partial=True)
            oproj([(h, o[0:S - RV, :])], acc.at[0:S - RV, :], rec=rec)
            mod_piece(h)
            wait_head(h + 1)
            return carry
        for h in range(1, G - 1):
            cp_k(h, sem_first.at[1 + h]).wait()
        for cp in early:
            cp.wait()
        wait_head(0)
        lax.fori_loop(0, NB, main_body, 0)

        ha = NB
        rest = list(zip(range(NB + 1, H), (s2_buf, s3_buf, s4_buf), (m2_buf, m3_buf, m4_buf)))
        late = []
        for n, h in enumerate(range(NB + 3, H)):
            late += [cp_v(h, sem_first.at[8 + 2 * n]), cp_wo(h, sem_first.at[9 + 2 * n])]
        cp_wr().wait()
        for p in range(NB + 1, H):
            cp_wmx(p).wait()
        oproj([(NB - 1, ov_buf[...])], acc.at[S - RV:, :])
        for cp in late:
            cp.start()

        def l_step(j, do_x, do_y):
            if do_x and do_y:
                aw = view(acc, j - 1, TL, 2)
                ay, ax = aw.at[0:TL, :], aw.at[TL:2 * TL, :]
            elif do_x:
                ax = view(acc, j, TL)
            else:
                ay = view(acc, j - 1, TL)
            rec = None
            if do_y:
                chunks = epi_chunks(j - 1, ay, view(o_buf, j - 1, TL), with_out=do_x)
                os_ = [(h, pv(h, sv, mv, late=not do_x)) for h, sv, mv in rest]
            if do_x:
                oa = pv(ha, view(s_buf, j, TL), view(m_buf, j, TL))
            if do_y and do_x:
                oproj(os_, ay, view(x_buf, j - 1, TL))
            elif do_y:
                xv = view(x_buf, j - 1, TL)
                r0, prev = 0, []
                for n in cfg["LSPLIT"]:
                    rs = slice(r0, r0 + n)
                    nr = len(os_) * (D // W)
                    cnt = [len(prev) // nr + (1 if i < len(prev) % nr else 0) for i in range(nr)]
                    rec = _Pace(prev, cnt)
                    oproj([(h, o[rs]) for h, o in os_], ay.at[rs, :], xv.at[rs, :], rec=rec)
                    prev = chunks[r0 // 8:(r0 + n) // 8]
                    r0 += n
                chunks = prev
            if do_x:
                if do_y:
                    rec = _Pace(chunks, cfg["LCNT"])
                for h, sv, mv in rest:
                    q = pltpu.bitcast(view(q_ring.at[h & 3], j, TL // 2)[...], bf16)
                    scores(h, q, sv, mv, rec=rec)
                oproj([(ha, oa)], ax, rec=rec)
            if do_y:
                if do_x:
                    cp_out(j - 1).start()
                else:
                    for ch in chunks:
                        ch()

        for p in range(NB, H):
            mod_piece(p)
        finish_mod()
        l_step(0, True, False)
        for cp in late:
            cp.wait()

        def pl_body(j, carry):
            l_step(j, True, True)
            return carry
        lax.fori_loop(1, JL, pl_body, 0)
        l_step(JL, False, True)

        k1, k2 = key_buf[0], key_buf[1]
        for sh in (4, 2, 1):
            o1, o2 = pltpu.roll(k1, sh, 0), pltpu.roll(k2, sh, 0)
            k2 = jnp.maximum(jnp.minimum(k1, o1), jnp.maximum(k2, o2))
            k1 = jnp.maximum(k1, o1)

        def score_of(k):
            hi = k & jnp.int32(-65536)
            return pltpu.bitcast(jnp.where(hi < 0, hi ^ 0x7FFF0000, hi), f32)

        i1s = jnp.minimum(0xFFFF - (k1[0, 0] & 0xFFFF), S - 1)
        i2s = jnp.minimum(0xFFFF - (k2[0, 0] & 0xFFFF), S - 1)

        sub = lax.broadcasted_iota(i32, (16, D), 0)
        sb, cb1, gb = (_rep(modv[i], 16) for i in (1, 2, 3))

        def adaln2(x1, stat):
            return (x1 - _wide(stat[:, 0:128], D)) * _wide(stat[:, 128:256], D) * cb1 + sb

        def pick(ref):
            sel = lax.broadcasted_iota(i32, (16, ref.shape[1]), 0) == 0
            return jnp.where(sel, ref[pl.ds(i1s, 1), :], ref[pl.ds(i2s, 1), :])

        xs = adaln2(pick(acc), pick(st2_buf)).astype(bf16)
        FC, lag = cfg["FC"], cfg["FLAG"]
        kvs = [int(ch) for ch in cfg["LKV"]]
        fout = [int(ch, 36) for ch in cfg["LFO"]]
        KV = max(kvs)

        def wrows(ref, a, b, c):
            n = FC // 128
            u = [ref[c * n + t, a // 2:b // 2, :] for t in range(n)]
            return pltpu.bitcast(u[0] if n == 1 else jnp.concatenate(u, axis=1), bf16)

        DV = D - KV * 128
        if KV:
            xf = xs.astype(f32)
            for r in range(2):
                xc_buf[r] = jnp.transpose(jnp.broadcast_to(xf[r:r + 1, DV:], (128, D - DV)))
        subc = lax.broadcasted_iota(i32, (8, FC), 0)
        y = None
        act = []
        outs = out_chunks(JL - 1)
        for c in range(F // FC + lag):
            if c < F // FC:
                dm = D - kvs[c] * 128
                gu = [jnp.dot(xs[:, :dm], wrows(w, 0, dm, c), preferred_element_type=f32)[0:8, :]
                      for w in (wg, wu)]
                for v in gu:
                    for t in range(fout[c] if c < len(fout) else 0):
                        if outs:
                            outs.pop(0)(_zero_of(v[0:8, (t % 2) * 128:(t % 2 + 1) * 128]))
                            if not outs:
                                cp_out(JL - 1).start()
                if dm < D:
                    part = [[None, None], [None, None]]
                    for k in range(dm, D, 16):
                        xcol = [_wide(xc_buf[r, k - DV:k - DV + 16, :], FC) for r in range(2)]
                        for m, w in enumerate((wg, wu)):
                            wv = wrows(w, k, k + 16, c).astype(f32)
                            for r in range(2):
                                t = wv * xcol[r]
                                for e in range(2):
                                    te = t[e * 8:(e + 1) * 8, :]
                                    part[m][r] = te if part[m][r] is None else part[m][r] + te
                    for m in range(2):
                        ra, rb_ = (jnp.sum(v, axis=0, keepdims=True) for v in part[m])
                        gu[m] = gu[m] + jnp.where(subc == 0, ra, rb_)
                g, u = _rb(gu[0]), _rb(gu[1])
                act.append(_rep(_rb(g * jax.nn.sigmoid(g)) * u, 16).astype(bf16))
            if c >= lag:
                wdc = pltpu.bitcast(wd[(c - lag) * FC // 2:(c - lag + 1) * FC // 2, :], bf16)
                d = jnp.dot(act[c - lag], wdc, preferred_element_type=f32)[0:8, :]
                y = d if y is None else y + d
        y = _rb(y)
        ya = _rb(y[0:1, :] * _wide(_rb(jax.nn.sigmoid(score_of(k1[0:1, :]))), D))
        yb = _rb(y[1:2, :] * _wide(_rb(jax.nn.sigmoid(score_of(k2[0:1, :]))), D))

        g1 = pl.multiple_of((i1s >> 4) << 4, 16)
        g2 = pl.multiple_of((i2s >> 4) << 4, 16)
        for t, g0 in enumerate((g1, g2)):
            rid = sub + g0
            x1 = acc[pl.ds(g0, 16), :]
            upd = jnp.where(rid == i1s, ya, 0.0) + jnp.where(rid == i2s, yb, 0.0)
            fix[t] = (x1 + gb * (adaln2(x1, st2_buf[pl.ds(g0, 16), :]) + upd)).astype(bf16)

        pltpu.make_async_copy(o_buf, out_hbm, sem_out.at[0]).wait()

        def cp_fix(t, g0):
            return pltpu.make_async_copy(fix.at[t], out_hbm.at[pl.ds(g0, 16), :], sem_fix.at[t])

        cp_fix(0, g1).start()

        @pl.when(g2 != g1)
        def _():
            cp_fix(1, g2).start()
            cp_fix(1, g2).wait()
        cp_fix(0, g1).wait()

    def looped(*refs):
        one, refs = refs[-1], refs[:-1]
        one[0] = 1

        def body(i, carry):
            kernel(*refs)
            return carry
        lax.fori_loop(0, one[0], body, 0)

    return looped


_CFG = dict(
    G=4, T0=256, TB=1024, TL=256, MCH=256, RB=16, FC=256, PKN=8, RV=160,
    LCA='cc80', LCB2='040g', NHB=16, NL4=8, BQ=3, LCNT='33333333332000',
    LCM='cc0000000000', LCV='000010000000', LCW='00000000000g', LCO='000006bbb0z6',
    LSPLIT=(96, 96, 64), FLAG=1, LKV='00233333333333', LFO='88',
)


def _build(A_x, A_k_cache, A_v_cache, A_wq, A_wo, B_w_r, B_w_gate, B_w_up, B_w_down, c, w_mod,
           **over):
    B, S, D = A_x.shape
    _, H, SK, DH = A_k_cache.shape
    F = B_w_gate.shape[1]
    assert B == 1
    cfg = dict(_CFG, **over)
    T0, TL, G = cfg["T0"], cfg["TL"], cfg["G"]
    MC = (4 * D) // H
    kernel = _make_kernel(S, D, H, DH, SK, F, cfg)
    scratch = [
        pltpu.VMEM((S, D), bf16),
        pltpu.VMEM((S // 2, D), u32),
        pltpu.VMEM((S, D), f32),
        pltpu.VMEM((S, SK), f32),
        pltpu.VMEM((S, 128), f32),
        pltpu.VMEM((TL, SK), f32),
        pltpu.VMEM((TL, 128), f32),
        pltpu.VMEM((TL, SK), f32),
        pltpu.VMEM((TL, 128), f32),
        pltpu.VMEM((TL, SK), f32),
        pltpu.VMEM((TL, 128), f32),
        pltpu.VMEM((S, 256), f32),
        pltpu.VMEM((S, 256), f32),
        pltpu.VMEM((1, S, SK // 4 - 128), f32),
        pltpu.VMEM((4, S // 2, DH), u32),
        pltpu.VMEM((G, S, DH), f32),
        pltpu.VMEM((8, G * DH), f32),
        pltpu.VMEM((4, SK, DH), bf16),
        pltpu.VMEM((4, SK, DH), bf16),
        pltpu.VMEM((D, G * DH), bf16),
        pltpu.VMEM((2, 4, D, 128), bf16),
        pltpu.VMEM((4, 2, DH, D), bf16),
        pltpu.VMEM((G - 1, D, MC), bf16),
        pltpu.VMEM((2, D, D // 2), bf16),
        pltpu.VMEM((D, D), bf16),
        pltpu.VMEM((1, D), bf16),
        pltpu.VMEM((D,), bf16),
        pltpu.VMEM((4, 1, D // 4), f32),
        pltpu.VMEM((D, 128), f32),
        pltpu.VMEM((2, 8, D), f32),
        pltpu.VMEM((H, 1, MC), f32),
        pltpu.VMEM((9, 8, D), f32),
        pltpu.VMEM((F // 128, D // 2, 128), u32),
        pltpu.VMEM((F // 128, D // 2, 128), u32),
        pltpu.VMEM((F // 2, D), u32),
        pltpu.VMEM((2, max(int(max(cfg["LKV"])), 1) * 128, 128), f32),
        pltpu.VMEM((cfg["RV"], DH), f32),
        pltpu.VMEM((cfg["RV"] // 8, DH * 8, 128), f32),
        pltpu.VMEM((DH, D), f32),
        pltpu.VMEM((S, D), bf16),
        pltpu.VMEM((2, 8, 128), i32),
        pltpu.VMEM((2, 16, D), bf16),
        pltpu.SemaphoreType.DMA((sum(_sem_sizes(S, D, cfg)),)),
        pltpu.SMEM((1,), i32),
    ]
    any_spec = pl.BlockSpec(memory_space=pl.ANY)
    out = pl.pallas_call(
        kernel,
        out_shape=jax.ShapeDtypeStruct((S, D), bf16),
        in_specs=[any_spec] * 11,
        out_specs=any_spec,
        scratch_shapes=scratch,
        compiler_params=pltpu.CompilerParams(vmem_limit_bytes=126 * 1024 * 1024,
                                             disable_bounds_checks=True,
                                             disable_semaphore_checks=True),
    )(A_x.reshape(S, D), A_k_cache.reshape(H, SK, DH), A_v_cache.reshape(H, SK, DH),
      A_wq, A_wo, B_w_r, B_w_gate, B_w_up, B_w_down, c, w_mod)
    return out.reshape(B, S, D)


@jax.jit
def pallas_adaLN_cond__mha_block_cached__moe_arch_mod__prompt_kernel(
    A_x: jax.Array,
    A_k_cache: jax.Array,
    A_v_cache: jax.Array,
    A_wq: jax.Array,
    A_wo: jax.Array,
    B_x: jax.Array,
    B_w_r: jax.Array,
    B_w_gate: jax.Array,
    B_w_up: jax.Array,
    B_w_down: jax.Array,
    c: jax.Array,
    w_mod: jax.Array,
):
    del B_x
    return _build(A_x, A_k_cache, A_v_cache, A_wq, A_wo, B_w_r, B_w_gate, B_w_up, B_w_down,
                  c, w_mod)
```

```python
import jax
import jax.numpy as jnp
from jax import lax
import jax.experimental.pallas as pl
import jax.experimental.pallas.tpu as pltpu

f32 = jnp.float32
bf16 = jnp.bfloat16
u32 = jnp.uint32
i32 = jnp.int32

_NT = (((1,), (1,)), ((), ()))
_LOG2E = 1.4426950408889634
_EPS = 1e-5
_IMIN = -2 ** 31


def _rb(v):
    return v.astype(bf16).astype(f32)


def _rep(v, n):
    return v if n == 8 else jnp.tile(v, (n // 8, 1))


def _wide(v, w):
    return jnp.tile(v, (1, w // 128))


def _pack(v):
    return pltpu.bitcast(v.astype(bf16), u32)


def _zero_of(v):
    bits = pltpu.bitcast(v, u32)
    return pltpu.bitcast(lax.shift_right_logical(lax.shift_right_logical(bits, jnp.uint32(31)),
                                                 jnp.uint32(1)), f32)


class _Pace:
    def __init__(self, chunks, counts):
        self.chunks = list(chunks)
        self.counts = [ch if isinstance(ch, int) else int(ch, 36) for ch in counts]
        assert sum(self.counts) == len(self.chunks), (counts, len(self.chunks))

    def done(self, res):
        n = self.counts.pop(0)
        for i in range(n):
            r0 = (i * res.shape[0] // n) // 8 * 8
            self.chunks.pop(0)(_zero_of(res[r0:r0 + 8, 0:128]))


def _mix(*plans):
    plans = [(list(ch), [c if isinstance(c, int) else int(c, 36) for c in cnt]) for ch, cnt in plans]
    for ch, cnt in plans:
        assert sum(cnt) == len(ch), (cnt, len(ch))
    fill, total = [], []
    for r in range(len(plans[0][1])):
        slots = sorted((i / cnt[r], k) for k, (_, cnt) in enumerate(plans)
                       for i in range(cnt[r]))
        fill += [plans[k][0].pop(0) for _, k in slots]
        total.append(len(slots))
    return _Pace(fill, total)


def _tiles(v):
    return [v[:, c * 128:(c + 1) * 128] for c in range(v.shape[1] // 128)]


def _fold(op, parts):
    out = parts[0]
    for p in parts[1:]:
        out = op(out, p)
    return out


def _lane_sum(v):
    return jnp.broadcast_to(jnp.sum(v, axis=-1, keepdims=True), v.shape)


def _row_stats(xf, tok=None, like_bf16=False):
    d = xf.shape[-1]
    ts = _tiles(xf)
    nt = len(ts)
    if tok is not None:
        ts = [ts[0] + tok] + ts[1:]
    mu = _fold(jnp.add, ts) * (1.0 / nt)
    m2 = _fold(jnp.add, [(t - mu) * (t - mu) for t in ts])
    mean = _lane_sum(mu) * (1.0 / 128)
    dm = mu - mean
    var = _lane_sum(m2 + (dm * dm) * float(nt)) * (1.0 / d)
    if not like_bf16:
        return mean, lax.rsqrt(var + _EPS)
    v = _rb(_rb(var) + _EPS)
    y = lax.rsqrt(v)
    sig = _rb(v * y)
    return mean, y * (2.0 - sig * y)


def _sem_sizes(S, D, cfg):
    j0 = S // cfg["T0"]
    return [2, 2 * (D // cfg["MCH"]), j0, 1, 16, 4, 1, 2]


def _make_kernel(S, D, H, DH, SK, F, cfg):
    T0, TL, MCH = cfg["T0"], cfg["TL"], cfg["MCH"]
    J0 = S // T0
    JL = S // TL
    qscale = DH ** -0.5 * _LOG2E
    n_mch = D // MCH
    G = cfg["G"]
    NB = H - G
    MC = (4 * D) // H
    W = 512
    NF = F // 128
    assert MCH == D // 4 and H < 256 and 2 <= G <= 4 and D == 2 * W and MC == DH == 128 and NF <= NB

    def kernel(x_hbm, k_hbm, v_hbm, wq_hbm, wo_hbm, wr_hbm, wg_hbm, wu_hbm, wd_hbm,
               c_hbm, wmod_hbm, out_hbm,
               x_buf, h_buf, acc, s_buf, m_buf, s2_buf, m2_buf, s3_buf, m3_buf, s4_buf, m4_buf,
               st_buf, st2_buf, mp_buf,
               q_ring, qf_buf, bq_buf,
               kb, vb, wq0, w4, wo2, wmx, wca, wsa, c_buf, wr_buf, sc_buf, cb_buf, mod0, modr, modv,
               wg, wu, wd, xc_buf, ov_buf, obx, wof, o_buf, key_buf, fix,
               sems):

        class _Sem:
            def __init__(self, base):
                self.base = base
                self.at = self

            def __getitem__(self, i):
                return sems.at[self.base + i]

        sizes = _sem_sizes(S, D, cfg)
        offs = [sum(sizes[:i]) for i in range(len(sizes))]
        (sem_small, sem_ca, sem_x, sem_sa, sem_first, sem_head,
         sem_out, sem_fix) = (_Sem(o) for o in offs)

        def _mul(a, n):
            v = a * n
            return v if isinstance(a, int) else pl.multiple_of(v, n)

        def view(ref, j, t, n=1):
            return ref.at[pl.ds(_mul(j, t), n * t), :]

        def cp_c():
            return pltpu.make_async_copy(c_hbm, c_buf, sem_small.at[0])

        def cp_wr():
            return pltpu.make_async_copy(wr_hbm, wr_buf, sem_small.at[1])

        def cp_ca(c, i):
            return pltpu.make_async_copy(
                wmod_hbm.at[pl.ds(_mul(i, MCH), MCH), pl.ds(D + c * W, W)], view(wca.at[c], i, MCH),
                sem_ca.at[c * n_mch + i])

        def cp_sa():
            return pltpu.make_async_copy(wmod_hbm.at[:, pl.ds(0, D)], wsa, sem_sa.at[0])

        def cp_x(j):
            return pltpu.make_async_copy(view(x_hbm, j, T0), view(x_buf, j, T0), sem_x.at[j])

        def cp_wq0(c):
            return pltpu.make_async_copy(wq_hbm.at[pl.ds(c * W, W), pl.ds(0, G * DH)],
                                         view(wq0, c, W), sem_first.at[14 + c])

        def cp_k(h, sem=None):
            return pltpu.make_async_copy(k_hbm.at[h], kb.at[h & 3],
                                         sem_head.at[0] if sem is None else sem)

        def cp_v(h, sem=None):
            return pltpu.make_async_copy(v_hbm.at[h], vb.at[h & 3],
                                         sem_head.at[1] if sem is None else sem)

        def cp_wo(h, sem=None):
            return pltpu.make_async_copy(view(wo_hbm, h, DH), wo2.at[h & 3, 0],
                                         sem_head.at[2] if sem is None else sem)

        def _clamp(a, hi):
            return min(a, hi) if isinstance(a, int) else jnp.minimum(a, hi)

        def cols(ref, t):
            return ref.at[:, pl.ds(_mul(t, 128), 128)]

        def cp_wmx(p):
            return pltpu.make_async_copy(cols(wmod_hbm, p + (2 * D) // MC), wmx.at[p - NB - 1],
                                         sem_first.at[4 + p - NB])

        def start_head(h):
            f = _clamp(h, NF - 1)
            for i, src in enumerate((cols(wq_hbm, _clamp(h + G, H - 1)),
                                     cols(wmod_hbm, h + (2 * D) // MC),
                                     cols(wg_hbm, f), cols(wu_hbm, f))):
                pltpu.make_async_copy(src, w4.at[h & 1, i], sem_head.at[3]).start()
            cp_k(h + G - 1).start()
            cp_wo(h + 2).start()
            pltpu.make_async_copy(view(wd_hbm, f, 128), wo2.at[(h + 2) & 3, 1],
                                  sem_head.at[2]).start()
            cp_v(h + 2).start()

        def wait_head(h):
            pltpu.make_async_copy(w4.at[h & 1], w4.at[h & 1], sem_head.at[3]).wait()
            cp_k(h + G - 1).wait()
            pltpu.make_async_copy(wo2.at[(h + 2) & 3], wo2.at[(h + 2) & 3], sem_head.at[2]).wait()
            cp_v(h + 2).wait()

        def pack_chunks(h):
            f = _clamp(h, NF - 1)
            out = []
            for sv, dv in ((w4.at[h & 1, 2], wg.at[f]), (w4.at[h & 1, 3], wu.at[f]),
                           (wo2.at[(h + 2) & 3, 1], view(wd, f, 64))):
                n, w = sv.shape
                step = n // cfg['PKN']

                def chunk(r, sv=sv, dv=dv, step=step, w=w):
                    def fn(tok):
                        z = _rep(_wide(pltpu.bitcast(tok, u32), w), step // 2)
                        dv[r // 2:(r + step) // 2, :] = pltpu.bitcast(sv[r:r + step, :], u32) | z
                    return fn
                out += [chunk(r) for r in range(0, n, step)]
            return out

        def cp_out(j):
            return pltpu.make_async_copy(view(o_buf, j, TL), view(out_hbm, j, TL), sem_out.at[0])

        def ln1_chunks(j, t):
            xv, sv, av = view(x_buf, j, t), view(st_buf, j, t), view(acc, j, t)

            def chunk(off):
                def f(tok=None):
                    av[off:off + 8, :] = jnp.zeros((8, D), f32) if tok is None else _wide(tok, D)
                    mean, inv = _row_stats(xv[off:off + 8, :].astype(f32), tok)
                    sv[off:off + 8, 0:128] = mean
                    sv[off:off + 8, 128:256] = inv
                return f
            return [chunk(off) for off in range(0, xv.shape[0], 8)]

        def ln1_scaled(x, stat, cs, tok=None):
            w = x.shape[1]
            mean = stat[:, 0:128] if tok is None else stat[:, 0:128] + _rep(tok, x.shape[0])
            n = (x.astype(f32) - _wide(mean, w)) * _wide(stat[:, 128:256], w)
            return n * _rep(mod0[1, :, cs], x.shape[0])

        def qproj(h, wv, rec=None):
            q = None
            for c in range(D // W):
                cs = slice(c * W, (c + 1) * W)
                part = jnp.dot(pltpu.bitcast(h_buf[:, cs], bf16), wv[cs, :],
                               preferred_element_type=f32)
                q = part if q is None else q + part
                if rec is not None:
                    rec.done(part)
            q_ring[h & 3] = _pack(q * qscale)

        def q_early(g, q):
            return (q + _rep(bq_buf[:, g * DH:(g + 1) * DH], q.shape[0])) * qscale

        def scores(h, q, sv, mv, rec, partial=False):
            nr = SK // W
            for c in range(nr):
                cs = slice(c * W, (c + 1) * W)
                s = lax.dot_general(q, kb[h & 3, cs, :], _NT, preferred_element_type=f32)
                if partial:
                    t = _tiles(s)
                    mp = jnp.maximum(jnp.maximum(t[0], t[1]), jnp.maximum(t[2], t[3]))
                    if c < nr - 1:
                        z = lax.shift_right_logical(h, 8)
                        mp_buf[z, :, c * 128:(c + 1) * 128] = mp
                sv[:, cs] = s
                if rec is not None:
                    rec.done(s)
            mp = _fold(jnp.maximum, [mp] + _tiles(mp_buf[0]) if partial else _tiles(sv[...]))
            mv[...] = jnp.broadcast_to(jnp.max(mp, axis=-1, keepdims=True), mp.shape)

        def pv(h, sv, mv, rec=None, late=False):
            o = lp = None
            for c in range(SK // W):
                cs = slice(c * W, (c + 1) * W)
                m = mv[...]
                if c >= 2 and sv.shape[0] == S:
                    m = m + _zero_of(lp)
                p = jnp.exp2(sv[:, cs] - _wide(m, W))
                lp = _fold(jnp.add, ([] if lp is None else [lp]) + _tiles(p))
                d = jnp.dot(p.astype(bf16), vb[h & 3, cs, :], preferred_element_type=f32)
                o = d if o is None else o + d
                if rec is not None:
                    rec.done(d)
            if late:
                lp = lp + _zero_of(o)
            l = jnp.sum(lp, axis=-1, keepdims=True)
            r = pl.reciprocal(l, approx=True)
            r = r * (2.0 - l * r)
            return o * r

        def oproj(hos, av, xv=None, rec=None):
            for c in range(D // W):
                cs = slice(c * W, (c + 1) * W)
                a = av[:, cs]
                for h, o in hos:
                    d = jnp.dot(o.astype(bf16), wo2[h & 3, 0, :, cs], preferred_element_type=f32)
                    if rec is not None:
                        rec.done(d)
                    a = a + d
                if xv is not None:
                    a = xv[:, cs].astype(f32) + _rep(modv[0, :, cs], a.shape[0]) * a
                av[:, cs] = a

        RV = cfg["RV"]

        def expand_chunks(h):
            def wchunk(r):
                def f(tok):
                    wof[r:r + 8, :] = wo2[h & 3, 0, r:r + 8, :].astype(f32) + _wide(tok, D)
                return f

            lane = lax.broadcasted_iota(i32, (8, 128), 1)

            def ochunk(g, e0):
                def f(tok):
                    o = ov_buf[g * 8:(g + 1) * 8, :] + tok
                    rs = slice(e0 * 8, (e0 + 32) * 8)
                    cols = jnp.concatenate(
                        [jnp.where(lane == e, o, 0.0) for e in range(e0, e0 + 32)], axis=0)
                    obx[g, rs, :] = _lane_sum(cols)
                return f
            och = [ochunk(g, e0) for g in range(RV // 8) for e0 in range(0, DH, 32)]
            return [wchunk(r) for r in range(0, DH, 8)], och

        def vproj(h):
            def f(tok):
                wrow = [jnp.concatenate(
                    [jnp.broadcast_to(wof[e:e + 1, t * 128:(t + 1) * 128], (8, 128))
                     for t in range(D // 128)], axis=1) for e in range(DH)]
                tok = _wide(tok, D)
                for g in range(RV // 8):
                    rows = slice(S - RV + g * 8, S - RV + g * 8 + 8)
                    a = acc[rows, :] + tok
                    ob = obx[g]
                    for e in range(DH):
                        a = a + _wide(ob[e * 8:(e + 1) * 8, :], D) * wrow[e]
                    tok = _zero_of(a)
                    acc[rows, :] = jnp.where(h > 0, a, 0.0)
            return f

        def matvec(wv, tok=None, step=16):
            n = wv.shape[1]
            part = None if tok is None else _wide(tok, n)
            for r in range(0, D, step):
                t = wv[r:r + step, :].astype(f32) * _wide(cb_buf[r:r + step, :], n)
                for e in range(step // 8):
                    te = t[e * 8:(e + 1) * 8, :]
                    part = te if part is None else part + te
            return _rb(jnp.sum(part, axis=0, keepdims=True))

        def mod_piece(p):
            extra = isinstance(p, int) and p > NB
            modr[p] = matvec(wmx.at[p - NB - 1] if extra else w4.at[p & 1, 1])

        def finish_mod():
            n = D // MC
            ga, sb, cb, gb = (jnp.concatenate([modr[i * n + t] for t in range(n)], axis=-1)
                              for i in range(4))
            cb1 = _rb(1.0 + cb)
            wr = wr_buf[...].astype(f32).reshape(1, D)
            a = cb1 * wr
            a0 = jnp.broadcast_to(jnp.sum(a, axis=-1, keepdims=True), (1, D))
            b0 = jnp.broadcast_to(jnp.sum(sb * wr, axis=-1, keepdims=True), (1, D))
            for i, v in enumerate((ga, sb, cb1, gb, a, gb * cb1, gb * sb, a0, b0)):
                modv[i] = jnp.broadcast_to(v, (8, D))

        def out_rows(x1, mean, inv):
            return (x1 + ((x1 - _wide(mean, D)) * (_wide(inv, D) * modv[5]) + modv[6])).astype(bf16)

        def out_chunks(j):
            x1v, sv, ov = view(acc, j, TL), view(st2_buf, j, TL), view(o_buf, j, TL)

            def chunk(off):
                def f(tok):
                    rs = slice(off, off + 8)
                    ov[rs, :] = out_rows(x1v[rs, :], sv[rs, 0:128] + tok, sv[rs, 128:256] + tok)
                return f
            return [chunk(off) for off in range(0, TL, 8)]

        def epi_chunks(j, x1v, ov, with_out=True):
            sub = lax.broadcasted_iota(i32, (8, 128), 0)
            low = (0xFFFF - j * TL) - sub
            sv = view(st2_buf, j, TL)
            st = {}

            def chunk(off):
                def f(tok=None):
                    if off == 0:
                        st["k1"], st["k2"] = key_buf[0], key_buf[1]
                    x1 = x1v[off:off + 8, :]
                    mean, inv = _row_stats(x1, tok, like_bf16=True)
                    sv[off:off + 8, 0:128] = mean
                    sv[off:off + 8, 128:256] = inv
                    xa = _tiles(x1 * modv[4])
                    if tok is not None:
                        xa[0] = xa[0] + tok
                    ra = _lane_sum(_fold(jnp.add, xa))
                    r = inv * (ra - mean * modv[7, :, 0:128]) + modv[8, :, 0:128]
                    if with_out:
                        ov[off:off + 8, :] = out_rows(x1, mean, inv)
                    bits = pltpu.bitcast(_rb(r) + 0.0, i32)
                    key = jnp.where(bits < 0, bits ^ 0x7FFF0000, bits) | (low - off)
                    st["k2"] = jnp.maximum(st["k2"], jnp.minimum(st["k1"], key))
                    st["k1"] = jnp.maximum(st["k1"], key)
                    if off + 8 == TL:
                        key_buf[0], key_buf[1] = st["k1"], st["k2"]
                return f
            return [chunk(off) for off in range(0, TL, 8)]

        cp_c().start()
        cp_x(0).start()
        for c in range(2):
            cp_wq0(c).start()
            for i in range(n_mch):
                cp_ca(c, i).start()
            if c == 0:
                for j in range(1, J0):
                    cp_x(j).start()
        cp_sa().start()
        for h in range(G - 1):
            cp_k(h, sem_first.at[1 + h]).start()
        early = []
        for h in range(2):
            early += [cp_v(h, sem_first.at[8 + 2 * h]), cp_wo(h, sem_first.at[9 + 2 * h])]
        for cp in early:
            cp.start()
        start_head(0)

        cp_c().wait()
        cf = c_buf[...].astype(f32)
        sc = _rb(cf * jax.nn.sigmoid(cf))
        for t in range(4):
            sc_buf[t] = sc[:, t * (D // 4):(t + 1) * (D // 4)]

        def cb_body(t, carry):
            view(cb_buf, t, D // 4)[...] = jnp.transpose(jnp.broadcast_to(sc_buf[t], (128, D // 4)))
            return carry
        lax.fori_loop(0, 4, cb_body, 0)
        key_buf[...] = jnp.full(key_buf.shape, _IMIN, i32)
        cp_x(0).wait()

        def st0_body(i, carry):
            for ch in ln1_chunks(i, T0 // 4):
                ch()
            return carry
        lax.fori_loop(0, 4, st0_body, 0)

        def ca_half(c, stream):
            def step(i, part):
                scb = jnp.broadcast_to(sc_buf[i], (16, MCH)).astype(bf16)
                return part + jnp.dot(scb, view(wca.at[c], i, MCH)[...],
                                      preferred_element_type=f32)[0:8, :]

            def wait_step(i, part):
                cp_ca(c, i).wait()
                return step(i, part)

            cp_wq0(c).wait()
            part = jnp.zeros((8, W), f32)
            if stream:
                part = lax.fori_loop(0, n_mch, wait_step, part)
            else:
                for i in range(n_mch):
                    cp_ca(c, i).wait()
                for i in range(n_mch):
                    part = step(i, part)
            mod0[1, :, c * W:(c + 1) * W] = _rb(1.0 + _rb(part))

        def q_first(r0, t, c, rec, mid=None):
            rows = pl.ds(r0, t)
            cs = slice(c * W, (c + 1) * W)
            hh = ln1_scaled(x_buf[rows, cs], st_buf[rows, :], cs).astype(bf16)
            for g in range(G):
                if mid is not None and g == mid[0]:
                    mid[1]()
                part = jnp.dot(hh, wq0[cs, g * DH:(g + 1) * DH], preferred_element_type=f32)
                qf_buf[g, rows, :] = part if c == 0 else qf_buf[g, rows, :] + part
                if rec is not None:
                    rec.done(part)

        ca_half(0, True)

        def pa_body(j, carry):
            @pl.when(j + 1 < J0)
            def _():
                cp_x(j + 1).wait()
            jn = jnp.minimum(j + 1, J0 - 1)
            rec = _Pace(ln1_chunks(jn, T0), cfg["LCA"])
            q_first(_mul(j, T0), T0, 0, rec)
            return carry
        lax.fori_loop(0, J0, pa_body, 0)

        TB, RB = cfg["TB"], cfg["RB"]
        ca_half(1, False)

        def pb_body(j, carry):
            q_first(_mul(j, TB // 2), TB // 2, 1, None)
            return carry
        lax.fori_loop(0, 2, pb_body, 0)
        cp_sa().wait()
        cp_k(0, sem_first.at[1]).wait()
        cp_wr().start()
        for p in range(NB + 1, H):
            cp_wmx(p).start()

        def sa_chunk(t):
            def f(tok):
                cs = slice(t * 256, (t + 1) * 256)
                mod0[0, :, cs] = jnp.broadcast_to(matvec(wsa.at[:, cs], tok, 8), (8, 256))
            return f

        def sa_bias():
            bq_buf[...] = jnp.dot(_rep(mod0[0], 16).astype(bf16), wq0[...],
                                  preferred_element_type=f32)[0:8, :]

        def h_chunk(off):
            def f(tok):
                rs, rh = slice(off, off + RB), slice(off // 2, (off + RB) // 2)
                hh = (ln1_scaled(x_buf[rs, :], st_buf[rs, :], slice(0, D), tok)
                      + _rep(mod0[0], RB)).astype(bf16)
                h_buf[rh, :] = pltpu.bitcast(hh, u32)
            return f

        def q_chunk(off):
            def f(tok):
                n = 2 * RB
                rs, rh = slice(off, off + n), slice(off // 2, (off + n) // 2)
                for g in range(1, G):
                    q_ring[g, rh, :] = _pack(q_early(g, qf_buf[g, rs, :] + _rep(tok, n)))
            return f

        hs = [h_chunk(off) for off in range(0, S, RB)]
        qs = [q_chunk(off) for off in range(0, S, 2 * RB)]
        nh = cfg["NHB"]
        rest_chunks = []
        nq, nr = len(qs), len(hs) - nh
        for i, ch in enumerate(hs[nh:]):
            rest_chunks.append(ch)
            while qs and (nq - len(qs)) * nr < (i + 1) * nq:
                rest_chunks.append(qs.pop(0))
        assert not qs
        rec = _Pace([sa_chunk(t) for t in range(D // 256)] + hs[:nh], cfg["LCB2"])
        q_first(TB, S - TB, 1, rec, mid=(cfg["BQ"], sa_bias))
        n4 = len(rest_chunks)
        n3 = n4 - cfg["NL4"]
        cnt = [n3 // 3 + (1 if i < n3 % 3 else 0) for i in range(3)] + [cfg["NL4"]]
        scores(0, q_early(0, qf_buf[0]).astype(bf16), s_buf, m_buf, rec=_Pace(rest_chunks, cnt))

        def main_body(h, carry):
            wch, och = expand_chunks(h)
            rec = _mix((pack_chunks(h), cfg["LCM"]), ([vproj(h)], cfg["LCV"]),
                       (wch, cfg["LCW"]), (och, cfg["LCO"]))
            o = pv(h, s_buf, m_buf, rec=rec)
            ov_buf[...] = _rb(o[S - RV:, :])
            qproj(h + G, w4.at[h & 1, 0], rec=rec)
            start_head(h + 1)
            scores(h + 1, pltpu.bitcast(q_ring[(h + 1) & 3], bf16), s_buf, m_buf, rec=rec,
                   partial=True)
            oproj([(h, o[0:S - RV, :])], acc.at[0:S - RV, :], rec=rec)
            mod_piece(h)
            wait_head(h + 1)
            return carry
        for h in range(1, G - 1):
            cp_k(h, sem_first.at[1 + h]).wait()
        for cp in early:
            cp.wait()
        wait_head(0)
        lax.fori_loop(0, NB, main_body, 0)

        ha = NB
        rest = list(zip(range(NB + 1, H), (s2_buf, s3_buf, s4_buf), (m2_buf, m3_buf, m4_buf)))
        late = []
        for n, h in enumerate(range(NB + 3, H)):
            late += [cp_v(h, sem_first.at[8 + 2 * n]), cp_wo(h, sem_first.at[9 + 2 * n])]
        cp_wr().wait()
        for p in range(NB + 1, H):
            cp_wmx(p).wait()
        oproj([(NB - 1, ov_buf[...])], acc.at[S - RV:, :])
        for cp in late:
            cp.start()

        def l_step(j, do_x, do_y):
            if do_x and do_y:
                aw = view(acc, j - 1, TL, 2)
                ay, ax = aw.at[0:TL, :], aw.at[TL:2 * TL, :]
            elif do_x:
                ax = view(acc, j, TL)
            else:
                ay = view(acc, j - 1, TL)
            rec = None
            if do_y:
                chunks = epi_chunks(j - 1, ay, view(o_buf, j - 1, TL), with_out=do_x)
                os_ = [(h, pv(h, sv, mv, late=not do_x)) for h, sv, mv in rest]
            if do_x:
                oa = pv(ha, view(s_buf, j, TL), view(m_buf, j, TL))
            if do_y and do_x:
                oproj(os_, ay, view(x_buf, j - 1, TL))
            elif do_y:
                xv = view(x_buf, j - 1, TL)
                r0, prev = 0, []
                for n in cfg["LSPLIT"]:
                    rs = slice(r0, r0 + n)
                    nr = len(os_) * (D // W)
                    cnt = [len(prev) // nr + (1 if i < len(prev) % nr else 0) for i in range(nr)]
                    rec = _Pace(prev, cnt)
                    oproj([(h, o[rs]) for h, o in os_], ay.at[rs, :], xv.at[rs, :], rec=rec)
                    prev = chunks[r0 // 8:(r0 + n) // 8]
                    r0 += n
                chunks = prev
            if do_x:
                if do_y:
                    rec = _Pace(chunks, cfg["LCNT"])
                for h, sv, mv in rest:
                    q = pltpu.bitcast(view(q_ring.at[h & 3], j, TL // 2)[...], bf16)
                    scores(h, q, sv, mv, rec=rec)
                oproj([(ha, oa)], ax, rec=rec)
            if do_y:
                if do_x:
                    cp_out(j - 1).start()
                else:
                    for ch in chunks:
                        ch()

        for p in range(NB, H):
            mod_piece(p)
        finish_mod()
        l_step(0, True, False)
        for cp in late:
            cp.wait()

        def pl_body(j, carry):
            l_step(j, True, True)
            return carry
        lax.fori_loop(1, JL, pl_body, 0)
        l_step(JL, False, True)

        k1, k2 = key_buf[0], key_buf[1]
        for sh in (4, 2, 1):
            o1, o2 = pltpu.roll(k1, sh, 0), pltpu.roll(k2, sh, 0)
            k2 = jnp.maximum(jnp.minimum(k1, o1), jnp.maximum(k2, o2))
            k1 = jnp.maximum(k1, o1)

        def score_of(k):
            hi = k & jnp.int32(-65536)
            return pltpu.bitcast(jnp.where(hi < 0, hi ^ 0x7FFF0000, hi), f32)

        i1s = jnp.minimum(0xFFFF - (k1[0, 0] & 0xFFFF), S - 1)
        i2s = jnp.minimum(0xFFFF - (k2[0, 0] & 0xFFFF), S - 1)

        sub = lax.broadcasted_iota(i32, (16, D), 0)
        sb, cb1, gb = (_rep(modv[i], 16) for i in (1, 2, 3))

        def adaln2(x1, stat):
            return (x1 - _wide(stat[:, 0:128], D)) * _wide(stat[:, 128:256], D) * cb1 + sb

        def pick(ref):
            sel = lax.broadcasted_iota(i32, (16, ref.shape[1]), 0) == 0
            return jnp.where(sel, ref[pl.ds(i1s, 1), :], ref[pl.ds(i2s, 1), :])

        xs = adaln2(pick(acc), pick(st2_buf)).astype(bf16)
        FC, lag = cfg["FC"], cfg["FLAG"]
        kvs = [int(ch) for ch in cfg["LKV"]]
        fout = [int(ch, 36) for ch in cfg["LFO"]]
        KV = max(kvs)

        def wrows(ref, a, b, c):
            n = FC // 128
            u = [ref[c * n + t, a // 2:b // 2, :] for t in range(n)]
            return pltpu.bitcast(u[0] if n == 1 else jnp.concatenate(u, axis=1), bf16)

        DV = D - KV * 128
        if KV:
            xf = xs.astype(f32)
            for r in range(2):
                xc_buf[r] = jnp.transpose(jnp.broadcast_to(xf[r:r + 1, DV:], (128, D - DV)))
        subc = lax.broadcasted_iota(i32, (8, FC), 0)
        y = None
        act = []
        outs = out_chunks(JL - 1)
        for c in range(F // FC + lag):
            if c < F // FC:
                dm = D - kvs[c] * 128
                gu = [jnp.dot(xs[:, :dm], wrows(w, 0, dm, c), preferred_element_type=f32)[0:8, :]
                      for w in (wg, wu)]
                for v in gu:
                    for t in range(fout[c] if c < len(fout) else 0):
                        if outs:
                            outs.pop(0)(_zero_of(v[0:8, (t % 2) * 128:(t % 2 + 1) * 128]))
                            if not outs:
                                cp_out(JL - 1).start()
                if dm < D:
                    part = [[None, None], [None, None]]
                    for k in range(dm, D, 16):
                        xcol = [_wide(xc_buf[r, k - DV:k - DV + 16, :], FC) for r in range(2)]
                        for m, w in enumerate((wg, wu)):
                            wv = wrows(w, k, k + 16, c).astype(f32)
                            for r in range(2):
                                t = wv * xcol[r]
                                for e in range(2):
                                    te = t[e * 8:(e + 1) * 8, :]
                                    part[m][r] = te if part[m][r] is None else part[m][r] + te
                    for m in range(2):
                        ra, rb_ = (jnp.sum(v, axis=0, keepdims=True) for v in part[m])
                        gu[m] = gu[m] + jnp.where(subc == 0, ra, rb_)
                g, u = _rb(gu[0]), _rb(gu[1])
                act.append(_rep(_rb(g * jax.nn.sigmoid(g)) * u, 16).astype(bf16))
            if c >= lag:
                wdc = pltpu.bitcast(wd[(c - lag) * FC // 2:(c - lag + 1) * FC // 2, :], bf16)
                d = jnp.dot(act[c - lag], wdc, preferred_element_type=f32)[0:8, :]
                y = d if y is None else y + d
        y = _rb(y)
        ya = _rb(y[0:1, :] * _wide(_rb(jax.nn.sigmoid(score_of(k1[0:1, :]))), D))
        yb = _rb(y[1:2, :] * _wide(_rb(jax.nn.sigmoid(score_of(k2[0:1, :]))), D))

        g1 = pl.multiple_of((i1s >> 4) << 4, 16)
        g2 = pl.multiple_of((i2s >> 4) << 4, 16)
        for t, g0 in enumerate((g1, g2)):
            rid = sub + g0
            x1 = acc[pl.ds(g0, 16), :]
            upd = jnp.where(rid == i1s, ya, 0.0) + jnp.where(rid == i2s, yb, 0.0)
            fix[t] = (x1 + gb * (adaln2(x1, st2_buf[pl.ds(g0, 16), :]) + upd)).astype(bf16)

        pltpu.make_async_copy(o_buf, out_hbm, sem_out.at[0]).wait()

        def cp_fix(t, g0):
            return pltpu.make_async_copy(fix.at[t], out_hbm.at[pl.ds(g0, 16), :], sem_fix.at[t])

        cp_fix(0, g1).start()

        @pl.when(g2 != g1)
        def _():
            cp_fix(1, g2).start()
            cp_fix(1, g2).wait()
        cp_fix(0, g1).wait()

    def looped(*refs):
        one, refs = refs[-1], refs[:-1]
        one[0] = 1

        def body(i, carry):
            kernel(*refs)
            return carry
        lax.fori_loop(0, one[0], body, 0)

    return looped


_CFG = dict(
    G=4, T0=256, TB=1024, TL=256, MCH=256, RB=16, FC=256, PKN=8, RV=160,
    LCA='cc80', LCB2='040g', NHB=16, NL4=8, BQ=3, LCNT='33333333332000',
    LCM='cc0000000000', LCV='000010000000', LCW='00000000000g', LCO='000006bbb0z6',
    LSPLIT=(96, 96, 64), FLAG=1, LKV='00233333333333', LFO='88',
)


def _build(A_x, A_k_cache, A_v_cache, A_wq, A_wo, B_w_r, B_w_gate, B_w_up, B_w_down, c, w_mod,
           **over):
    B, S, D = A_x.shape
    _, H, SK, DH = A_k_cache.shape
    F = B_w_gate.shape[1]
    assert B == 1
    cfg = dict(_CFG, **over)
    T0, TL, G = cfg["T0"], cfg["TL"], cfg["G"]
    MC = (4 * D) // H
    kernel = _make_kernel(S, D, H, DH, SK, F, cfg)
    scratch = [
        pltpu.VMEM((S, D), bf16),
        pltpu.VMEM((S // 2, D), u32),
        pltpu.VMEM((S, D), f32),
        pltpu.VMEM((S, SK), f32),
        pltpu.VMEM((S, 128), f32),
        pltpu.VMEM((TL, SK), f32),
        pltpu.VMEM((TL, 128), f32),
        pltpu.VMEM((TL, SK), f32),
        pltpu.VMEM((TL, 128), f32),
        pltpu.VMEM((TL, SK), f32),
        pltpu.VMEM((TL, 128), f32),
        pltpu.VMEM((S, 256), f32),
        pltpu.VMEM((S, 256), f32),
        pltpu.VMEM((1, S, SK // 4 - 128), f32),
        pltpu.VMEM((4, S // 2, DH), u32),
        pltpu.VMEM((G, S, DH), f32),
        pltpu.VMEM((8, G * DH), f32),
        pltpu.VMEM((4, SK, DH), bf16),
        pltpu.VMEM((4, SK, DH), bf16),
        pltpu.VMEM((D, G * DH), bf16),
        pltpu.VMEM((2, 4, D, 128), bf16),
        pltpu.VMEM((4, 2, DH, D), bf16),
        pltpu.VMEM((G - 1, D, MC), bf16),
        pltpu.VMEM((2, D, D // 2), bf16),
        pltpu.VMEM((D, D), bf16),
        pltpu.VMEM((1, D), bf16),
        pltpu.VMEM((D,), bf16),
        pltpu.VMEM((4, 1, D // 4), f32),
        pltpu.VMEM((D, 128), f32),
        pltpu.VMEM((2, 8, D), f32),
        pltpu.VMEM((H, 1, MC), f32),
        pltpu.VMEM((9, 8, D), f32),
        pltpu.VMEM((F // 128, D // 2, 128), u32),
        pltpu.VMEM((F // 128, D // 2, 128), u32),
        pltpu.VMEM((F // 2, D), u32),
        pltpu.VMEM((2, max(int(max(cfg["LKV"])), 1) * 128, 128), f32),
        pltpu.VMEM((cfg["RV"], DH), f32),
        pltpu.VMEM((cfg["RV"] // 8, DH * 8, 128), f32),
        pltpu.VMEM((DH, D), f32),
        pltpu.VMEM((S, D), bf16),
        pltpu.VMEM((2, 8, 128), i32),
        pltpu.VMEM((2, 16, D), bf16),
        pltpu.SemaphoreType.DMA((sum(_sem_sizes(S, D, cfg)),)),
        pltpu.SMEM((1,), i32),
    ]
    any_spec = pl.BlockSpec(memory_space=pl.ANY)
    out = pl.pallas_call(
        kernel,
        out_shape=jax.ShapeDtypeStruct((S, D), bf16),
        in_specs=[any_spec] * 11,
        out_specs=any_spec,
        scratch_shapes=scratch,
        compiler_params=pltpu.CompilerParams(vmem_limit_bytes=126 * 1024 * 1024,
                                             disable_bounds_checks=True,
                                             disable_semaphore_checks=True),
    )(A_x.reshape(S, D), A_k_cache.reshape(H, SK, DH), A_v_cache.reshape(H, SK, DH),
      A_wq, A_wo, B_w_r, B_w_gate, B_w_up, B_w_down, c, w_mod)
    return out.reshape(B, S, D)


@jax.jit
def pallas_adaLN_cond__mha_block_cached__moe_arch_mod__prompt_kernel(
    A_x: jax.Array,
    A_k_cache: jax.Array,
    A_v_cache: jax.Array,
    A_wq: jax.Array,
    A_wo: jax.Array,
    B_x: jax.Array,
    B_w_r: jax.Array,
    B_w_gate: jax.Array,
    B_w_up: jax.Array,
    B_w_down: jax.Array,
    c: jax.Array,
    w_mod: jax.Array,
):
    del B_x
    return _build(A_x, A_k_cache, A_v_cache, A_wq, A_wo, B_w_r, B_w_gate, B_w_up, B_w_down,
                  c, w_mod)
```

```python
import jax
import jax.numpy as jnp
from jax import lax
import jax.experimental.pallas as pl
import jax.experimental.pallas.tpu as pltpu

f32 = jnp.float32
bf16 = jnp.bfloat16
u32 = jnp.uint32
i32 = jnp.int32

_NT = (((1,), (1,)), ((), ()))
_LOG2E = 1.4426950408889634
_EPS = 1e-5
_IMIN = -2 ** 31


def _rb(v):
    return v.astype(bf16).astype(f32)


def _rep(v, n):
    return v if n == 8 else jnp.tile(v, (n // 8, 1))


def _wide(v, w):
    return jnp.tile(v, (1, w // 128))


def _pack(v):
    return pltpu.bitcast(v.astype(bf16), u32)


def _zero_of(v):
    bits = pltpu.bitcast(v, u32)
    return pltpu.bitcast(lax.shift_right_logical(lax.shift_right_logical(bits, jnp.uint32(31)),
                                                 jnp.uint32(1)), f32)


class _Pace:
    def __init__(self, chunks, counts):
        self.chunks = list(chunks)
        self.counts = [ch if isinstance(ch, int) else int(ch, 36) for ch in counts]
        assert sum(self.counts) == len(self.chunks), (counts, len(self.chunks))

    def done(self, res):
        n = self.counts.pop(0)
        for i in range(n):
            r0 = (i * res.shape[0] // n) // 8 * 8
            self.chunks.pop(0)(_zero_of(res[r0:r0 + 8, 0:128]))


def _mix(*plans):
    plans = [(list(ch), [c if isinstance(c, int) else int(c, 36) for c in cnt]) for ch, cnt in plans]
    for ch, cnt in plans:
        assert sum(cnt) == len(ch), (cnt, len(ch))
    fill, total = [], []
    for r in range(len(plans[0][1])):
        slots = sorted((i / cnt[r], k) for k, (_, cnt) in enumerate(plans)
                       for i in range(cnt[r]))
        fill += [plans[k][0].pop(0) for _, k in slots]
        total.append(len(slots))
    return _Pace(fill, total)


def _tiles(v):
    return [v[:, c * 128:(c + 1) * 128] for c in range(v.shape[1] // 128)]


def _fold(op, parts):
    out = parts[0]
    for p in parts[1:]:
        out = op(out, p)
    return out


def _lane_sum(v):
    return jnp.broadcast_to(jnp.sum(v, axis=-1, keepdims=True), v.shape)


def _row_stats(xf, tok=None, like_bf16=False):
    d = xf.shape[-1]
    ts = _tiles(xf)
    nt = len(ts)
    if tok is not None:
        ts = [ts[0] + tok] + ts[1:]
    mu = _fold(jnp.add, ts) * (1.0 / nt)
    m2 = _fold(jnp.add, [(t - mu) * (t - mu) for t in ts])
    mean = _lane_sum(mu) * (1.0 / 128)
    dm = mu - mean
    var = _lane_sum(m2 + (dm * dm) * float(nt)) * (1.0 / d)
    if not like_bf16:
        return mean, lax.rsqrt(var + _EPS)
    v = _rb(_rb(var) + _EPS)
    y = lax.rsqrt(v)
    sig = _rb(v * y)
    return mean, y * (2.0 - sig * y)


def _sem_sizes(S, D, cfg):
    j0 = S // cfg["T0"]
    return [2, 2 * (D // cfg["MCH"]), j0, 1, 16, 4, 1, 2]


def _make_kernel(S, D, H, DH, SK, F, cfg):
    T0, TL, MCH = cfg["T0"], cfg["TL"], cfg["MCH"]
    J0 = S // T0
    JL = S // TL
    qscale = DH ** -0.5 * _LOG2E
    n_mch = D // MCH
    G = cfg["G"]
    NB = H - G
    MC = (4 * D) // H
    W = 512
    NF = F // 128
    assert MCH == D // 4 and H < 256 and 2 <= G <= 4 and D == 2 * W and MC == DH == 128 and NF <= NB

    def kernel(x_hbm, k_hbm, v_hbm, wq_hbm, wo_hbm, wr_hbm, wg_hbm, wu_hbm, wd_hbm,
               c_hbm, wmod_hbm, out_hbm,
               x_buf, h_buf, acc, s_buf, m_buf, s2_buf, m2_buf, s3_buf, m3_buf, s4_buf, m4_buf,
               st_buf, st2_buf, mp_buf,
               q_ring, qf_buf, bq_buf,
               kb, vb, wq0, w4, wo2, wmx, wca, wsa, c_buf, wr_buf, sc_buf, cb_buf, mod0, modr, modv,
               wg, wu, wd, xc_buf, ov_buf, obx, wof, o_buf, key_buf, fix,
               sems):

        class _Sem:
            def __init__(self, base):
                self.base = base
                self.at = self

            def __getitem__(self, i):
                return sems.at[self.base + i]

        sizes = _sem_sizes(S, D, cfg)
        offs = [sum(sizes[:i]) for i in range(len(sizes))]
        (sem_small, sem_ca, sem_x, sem_sa, sem_first, sem_head,
         sem_out, sem_fix) = (_Sem(o) for o in offs)

        def _mul(a, n):
            v = a * n
            return v if isinstance(a, int) else pl.multiple_of(v, n)

        def view(ref, j, t, n=1):
            return ref.at[pl.ds(_mul(j, t), n * t), :]

        def cp_c():
            return pltpu.make_async_copy(c_hbm, c_buf, sem_small.at[0])

        def cp_wr():
            return pltpu.make_async_copy(wr_hbm, wr_buf, sem_small.at[1])

        def cp_ca(c, i):
            return pltpu.make_async_copy(
                wmod_hbm.at[pl.ds(_mul(i, MCH), MCH), pl.ds(D + c * W, W)], view(wca.at[c], i, MCH),
                sem_ca.at[c * n_mch + i])

        def cp_sa():
            return pltpu.make_async_copy(wmod_hbm.at[:, pl.ds(0, D)], wsa, sem_sa.at[0])

        def cp_x(j):
            return pltpu.make_async_copy(view(x_hbm, j, T0), view(x_buf, j, T0), sem_x.at[j])

        def cp_wq0(c):
            return pltpu.make_async_copy(wq_hbm.at[pl.ds(c * W, W), pl.ds(0, G * DH)],
                                         view(wq0, c, W), sem_first.at[14 + c])

        def cp_k(h, sem=None):
            return pltpu.make_async_copy(k_hbm.at[h], kb.at[h & 3],
                                         sem_head.at[0] if sem is None else sem)

        def cp_v(h, sem=None):
            return pltpu.make_async_copy(v_hbm.at[h], vb.at[h & 3],
                                         sem_head.at[1] if sem is None else sem)

        def cp_wo(h, sem=None):
            return pltpu.make_async_copy(view(wo_hbm, h, DH), wo2.at[h & 3, 0],
                                         sem_head.at[2] if sem is None else sem)

        def _clamp(a, hi):
            return min(a, hi) if isinstance(a, int) else jnp.minimum(a, hi)

        def cols(ref, t):
            return ref.at[:, pl.ds(_mul(t, 128), 128)]

        def cp_wmx(p):
            return pltpu.make_async_copy(cols(wmod_hbm, p + (2 * D) // MC), wmx.at[p - NB - 1],
                                         sem_first.at[4 + p - NB])

        def start_head(h):
            f = _clamp(h, NF - 1)
            for i, src in enumerate((cols(wq_hbm, _clamp(h + G, H - 1)),
                                     cols(wmod_hbm, h + (2 * D) // MC),
                                     cols(wg_hbm, f), cols(wu_hbm, f))):
                pltpu.make_async_copy(src, w4.at[h & 1, i], sem_head.at[3]).start()
            cp_k(h + G - 1).start()
            cp_wo(h + 2).start()
            pltpu.make_async_copy(view(wd_hbm, f, 128), wo2.at[(h + 2) & 3, 1],
                                  sem_head.at[2]).start()
            cp_v(h + 2).start()

        def wait_head(h):
            pltpu.make_async_copy(w4.at[h & 1], w4.at[h & 1], sem_head.at[3]).wait()
            cp_k(h + G - 1).wait()
            pltpu.make_async_copy(wo2.at[(h + 2) & 3], wo2.at[(h + 2) & 3], sem_head.at[2]).wait()
            cp_v(h + 2).wait()

        def pack_chunks(h):
            f = _clamp(h, NF - 1)
            out = []
            for sv, dv in ((w4.at[h & 1, 2], wg.at[f]), (w4.at[h & 1, 3], wu.at[f]),
                           (wo2.at[(h + 2) & 3, 1], view(wd, f, 64))):
                n, w = sv.shape
                step = n // cfg['PKN']

                def chunk(r, sv=sv, dv=dv, step=step, w=w):
                    def fn(tok):
                        z = _rep(_wide(pltpu.bitcast(tok, u32), w), step // 2)
                        dv[r // 2:(r + step) // 2, :] = pltpu.bitcast(sv[r:r + step, :], u32) | z
                    return fn
                out += [chunk(r) for r in range(0, n, step)]
            return out

        def cp_out(j):
            return pltpu.make_async_copy(view(o_buf, j, TL), view(out_hbm, j, TL), sem_out.at[0])

        def ln1_chunks(j, t):
            xv, sv, av = view(x_buf, j, t), view(st_buf, j, t), view(acc, j, t)

            def chunk(off):
                def f(tok=None):
                    av[off:off + 8, :] = jnp.zeros((8, D), f32) if tok is None else _wide(tok, D)
                    mean, inv = _row_stats(xv[off:off + 8, :].astype(f32), tok)
                    sv[off:off + 8, 0:128] = mean
                    sv[off:off + 8, 128:256] = inv
                return f
            return [chunk(off) for off in range(0, xv.shape[0], 8)]

        def ln1_scaled(x, stat, cs, tok=None):
            w = x.shape[1]
            mean = stat[:, 0:128] if tok is None else stat[:, 0:128] + _rep(tok, x.shape[0])
            n = (x.astype(f32) - _wide(mean, w)) * _wide(stat[:, 128:256], w)
            return n * _rep(mod0[1, :, cs], x.shape[0])

        def qproj(h, wv, rec=None):
            q = None
            for c in range(D // W):
                cs = slice(c * W, (c + 1) * W)
                part = jnp.dot(pltpu.bitcast(h_buf[:, cs], bf16), wv[cs, :],
                               preferred_element_type=f32)
                q = part if q is None else q + part
                if rec is not None:
                    rec.done(part)
            q_ring[h & 3] = _pack(q * qscale)

        def q_early(g, q):
            return (q + _rep(bq_buf[:, g * DH:(g + 1) * DH], q.shape[0])) * qscale

        def scores(h, q, sv, mv, rec, partial=False):
            nr = SK // W
            for c in range(nr):
                cs = slice(c * W, (c + 1) * W)
                s = lax.dot_general(q, kb[h & 3, cs, :], _NT, preferred_element_type=f32)
                if partial:
                    t = _tiles(s)
                    mp = jnp.maximum(jnp.maximum(t[0], t[1]), jnp.maximum(t[2], t[3]))
                    if c < nr - 1:
                        z = lax.shift_right_logical(h, 8)
                        mp_buf[z, :, c * 128:(c + 1) * 128] = mp
                sv[:, cs] = s
                if rec is not None:
                    rec.done(s)
            mp = _fold(jnp.maximum, [mp] + _tiles(mp_buf[0]) if partial else _tiles(sv[...]))
            mv[...] = jnp.broadcast_to(jnp.max(mp, axis=-1, keepdims=True), mp.shape)

        def pv(h, sv, mv, rec=None, late=False):
            o = lp = None
            for c in range(SK // W):
                cs = slice(c * W, (c + 1) * W)
                m = mv[...]
                if c >= 2 and sv.shape[0] == S:
                    m = m + _zero_of(lp)
                p = jnp.exp2(sv[:, cs] - _wide(m, W))
                lp = _fold(jnp.add, ([] if lp is None else [lp]) + _tiles(p))
                d = jnp.dot(p.astype(bf16), vb[h & 3, cs, :], preferred_element_type=f32)
                o = d if o is None else o + d
                if rec is not None:
                    rec.done(d)
            if late:
                lp = lp + _zero_of(o)
            l = jnp.sum(lp, axis=-1, keepdims=True)
            r = pl.reciprocal(l, approx=True)
            r = r * (2.0 - l * r)
            return o * r

        def oproj(hos, av, xv=None, rec=None):
            for c in range(D // W):
                cs = slice(c * W, (c + 1) * W)
                a = av[:, cs]
                for h, o in hos:
                    d = jnp.dot(o.astype(bf16), wo2[h & 3, 0, :, cs], preferred_element_type=f32)
                    if rec is not None:
                        rec.done(d)
                    a = a + d
                if xv is not None:
                    a = xv[:, cs].astype(f32) + _rep(modv[0, :, cs], a.shape[0]) * a
                av[:, cs] = a

        RV = cfg["RV"]

        def expand_chunks(h):
            def wchunk(r):
                def f(tok):
                    wof[r:r + 8, :] = wo2[h & 3, 0, r:r + 8, :].astype(f32) + _wide(tok, D)
                return f

            lane = lax.broadcasted_iota(i32, (32, 8, 128), 2)
            col = lax.broadcasted_iota(i32, (32, 8, 128), 0)

            def ochunk(g, e0):
                def f(tok):
                    o = ov_buf[g * 8:(g + 1) * 8, :] + tok
                    rs = slice(e0 * 8, (e0 + 32) * 8)
                    cols = jnp.where(lane == col + e0, o[None], 0.0).reshape(256, 128)
                    obx[g, rs, :] = _lane_sum(cols)
                return f
            och = [ochunk(g, e0) for g in range(RV // 8) for e0 in range(0, DH, 32)]
            return [wchunk(r) for r in range(0, DH, 8)], och

        def vproj(h):
            def f(tok):
                wrow = [jnp.concatenate(
                    [jnp.broadcast_to(wof[e:e + 1, t * 128:(t + 1) * 128], (8, 128))
                     for t in range(D // 128)], axis=1) for e in range(DH)]
                wall = jnp.concatenate(wrow, axis=0)
                tok = _wide(tok, D)
                for g in range(RV // 8):
                    rows = slice(S - RV + g * 8, S - RV + g * 8 + 8)
                    terms = jnp.concatenate([acc[rows, :] + tok, _wide(obx[g], D) * wall], axis=0)
                    a = terms.reshape(DH + 1, 8, D).sum(axis=0)
                    tok = _zero_of(a)
                    acc[rows, :] = jnp.where(h > 0, a, 0.0)
            return f

        def matvec(wv, tok=None, step=16):
            n = wv.shape[1]
            part = None if tok is None else _wide(tok, n)
            for r in range(0, D, step):
                t = wv[r:r + step, :].astype(f32) * _wide(cb_buf[r:r + step, :], n)
                for e in range(step // 8):
                    te = t[e * 8:(e + 1) * 8, :]
                    part = te if part is None else part + te
            return _rb(jnp.sum(part, axis=0, keepdims=True))

        def mod_piece(p):
            extra = isinstance(p, int) and p > NB
            modr[p] = matvec(wmx.at[p - NB - 1] if extra else w4.at[p & 1, 1])

        def finish_mod():
            n = D // MC
            ga, sb, cb, gb = (jnp.concatenate([modr[i * n + t] for t in range(n)], axis=-1)
                              for i in range(4))
            cb1 = _rb(1.0 + cb)
            wr = wr_buf[...].astype(f32).reshape(1, D)
            a = cb1 * wr
            a0 = jnp.broadcast_to(jnp.sum(a, axis=-1, keepdims=True), (1, D))
            b0 = jnp.broadcast_to(jnp.sum(sb * wr, axis=-1, keepdims=True), (1, D))
            for i, v in enumerate((ga, sb, cb1, gb, a, gb * cb1, gb * sb, a0, b0)):
                modv[i] = jnp.broadcast_to(v, (8, D))

        def out_rows(x1, mean, inv):
            return (x1 + ((x1 - _wide(mean, D)) * (_wide(inv, D) * modv[5]) + modv[6])).astype(bf16)

        def out_chunks(j):
            x1v, sv, ov = view(acc, j, TL), view(st2_buf, j, TL), view(o_buf, j, TL)

            def chunk(off):
                def f(tok):
                    rs = slice(off, off + 8)
                    ov[rs, :] = out_rows(x1v[rs, :], sv[rs, 0:128] + tok, sv[rs, 128:256] + tok)
                return f
            return [chunk(off) for off in range(0, TL, 8)]

        def epi_chunks(j, x1v, ov, with_out=True):
            sub = lax.broadcasted_iota(i32, (8, 128), 0)
            low = (0xFFFF - j * TL) - sub
            sv = view(st2_buf, j, TL)
            st = {}

            def chunk(off):
                def f(tok=None):
                    if off == 0:
                        st["k1"], st["k2"] = key_buf[0], key_buf[1]
                    x1 = x1v[off:off + 8, :]
                    mean, inv = _row_stats(x1, tok, like_bf16=True)
                    sv[off:off + 8, 0:128] = mean
                    sv[off:off + 8, 128:256] = inv
                    xa = _tiles(x1 * modv[4])
                    if tok is not None:
                        xa[0] = xa[0] + tok
                    ra = _lane_sum(_fold(jnp.add, xa))
                    r = inv * (ra - mean * modv[7, :, 0:128]) + modv[8, :, 0:128]
                    if with_out:
                        ov[off:off + 8, :] = out_rows(x1, mean, inv)
                    bits = pltpu.bitcast(_rb(r) + 0.0, i32)
                    key = jnp.where(bits < 0, bits ^ 0x7FFF0000, bits) | (low - off)
                    st["k2"] = jnp.maximum(st["k2"], jnp.minimum(st["k1"], key))
                    st["k1"] = jnp.maximum(st["k1"], key)
                    if off + 8 == TL:
                        key_buf[0], key_buf[1] = st["k1"], st["k2"]
                return f
            return [chunk(off) for off in range(0, TL, 8)]

        cp_c().start()
        cp_x(0).start()
        for c in range(2):
            cp_wq0(c).start()
            for i in range(n_mch):
                cp_ca(c, i).start()
            if c == 0:
                for j in range(1, J0):
                    cp_x(j).start()
        cp_sa().start()
        for h in range(G - 1):
            cp_k(h, sem_first.at[1 + h]).start()
        early = []
        for h in range(2):
            early += [cp_v(h, sem_first.at[8 + 2 * h]), cp_wo(h, sem_first.at[9 + 2 * h])]
        for cp in early:
            cp.start()
        start_head(0)

        cp_c().wait()
        cf = c_buf[...].astype(f32)
        sc = _rb(cf * jax.nn.sigmoid(cf))
        for t in range(4):
            sc_buf[t] = sc[:, t * (D // 4):(t + 1) * (D // 4)]

        def cb_body(t, carry):
            view(cb_buf, t, D // 4)[...] = jnp.transpose(jnp.broadcast_to(sc_buf[t], (128, D // 4)))
            return carry
        lax.fori_loop(0, 4, cb_body, 0)
        key_buf[...] = jnp.full(key_buf.shape, _IMIN, i32)
        cp_x(0).wait()

        def st0_body(i, carry):
            for ch in ln1_chunks(i, T0 // 4):
                ch()
            return carry
        lax.fori_loop(0, 4, st0_body, 0)

        def ca_half(c, stream):
            def step(i, part):
                scb = jnp.broadcast_to(sc_buf[i], (16, MCH)).astype(bf16)
                return part + jnp.dot(scb, view(wca.at[c], i, MCH)[...],
                                      preferred_element_type=f32)[0:8, :]

            def wait_step(i, part):
                cp_ca(c, i).wait()
                return step(i, part)

            cp_wq0(c).wait()
            part = jnp.zeros((8, W), f32)
            if stream:
                part = lax.fori_loop(0, n_mch, wait_step, part)
            else:
                for i in range(n_mch):
                    cp_ca(c, i).wait()
                for i in range(n_mch):
                    part = step(i, part)
            mod0[1, :, c * W:(c + 1) * W] = _rb(1.0 + _rb(part))

        def q_first(r0, t, c, rec, mid=None):
            rows = pl.ds(r0, t)
            cs = slice(c * W, (c + 1) * W)
            hh = ln1_scaled(x_buf[rows, cs], st_buf[rows, :], cs).astype(bf16)
            for g in range(G):
                if mid is not None and g == mid[0]:
                    mid[1]()
                part = jnp.dot(hh, wq0[cs, g * DH:(g + 1) * DH], preferred_element_type=f32)
                qf_buf[g, rows, :] = part if c == 0 else qf_buf[g, rows, :] + part
                if rec is not None:
                    rec.done(part)

        ca_half(0, True)

        def pa_body(j, carry):
            @pl.when(j + 1 < J0)
            def _():
                cp_x(j + 1).wait()
            jn = jnp.minimum(j + 1, J0 - 1)
            rec = _Pace(ln1_chunks(jn, T0), cfg["LCA"])
            q_first(_mul(j, T0), T0, 0, rec)
            return carry
        lax.fori_loop(0, J0, pa_body, 0)

        TB, RB = cfg["TB"], cfg["RB"]
        ca_half(1, False)

        def pb_body(j, carry):
            q_first(_mul(j, TB // 2), TB // 2, 1, None)
            return carry
        lax.fori_loop(0, 2, pb_body, 0)
        cp_sa().wait()
        cp_k(0, sem_first.at[1]).wait()
        cp_wr().start()
        for p in range(NB + 1, H):
            cp_wmx(p).start()

        def sa_chunk(t):
            def f(tok):
                cs = slice(t * 256, (t + 1) * 256)
                mod0[0, :, cs] = jnp.broadcast_to(matvec(wsa.at[:, cs], tok, 8), (8, 256))
            return f

        def sa_bias():
            bq_buf[...] = jnp.dot(_rep(mod0[0], 16).astype(bf16), wq0[...],
                                  preferred_element_type=f32)[0:8, :]

        def h_chunk(off):
            def f(tok):
                rs, rh = slice(off, off + RB), slice(off // 2, (off + RB) // 2)
                hh = (ln1_scaled(x_buf[rs, :], st_buf[rs, :], slice(0, D), tok)
                      + _rep(mod0[0], RB)).astype(bf16)
                h_buf[rh, :] = pltpu.bitcast(hh, u32)
            return f

        def q_chunk(off):
            def f(tok):
                n = 2 * RB
                rs, rh = slice(off, off + n), slice(off // 2, (off + n) // 2)
                for g in range(1, G):
                    q_ring[g, rh, :] = _pack(q_early(g, qf_buf[g, rs, :] + _rep(tok, n)))
            return f

        hs = [h_chunk(off) for off in range(0, S, RB)]
        qs = [q_chunk(off) for off in range(0, S, 2 * RB)]
        nh = cfg["NHB"]
        rest_chunks = []
        nq, nr = len(qs), len(hs) - nh
        for i, ch in enumerate(hs[nh:]):
            rest_chunks.append(ch)
            while qs and (nq - len(qs)) * nr < (i + 1) * nq:
                rest_chunks.append(qs.pop(0))
        assert not qs
        rec = _Pace([sa_chunk(t) for t in range(D // 256)] + hs[:nh], cfg["LCB2"])
        q_first(TB, S - TB, 1, rec, mid=(cfg["BQ"], sa_bias))
        n4 = len(rest_chunks)
        n3 = n4 - cfg["NL4"]
        cnt = [n3 // 3 + (1 if i < n3 % 3 else 0) for i in range(3)] + [cfg["NL4"]]
        scores(0, q_early(0, qf_buf[0]).astype(bf16), s_buf, m_buf, rec=_Pace(rest_chunks, cnt))

        def main_body(h, carry):
            wch, och = expand_chunks(h)
            rec = _mix((pack_chunks(h), cfg["LCM"]), ([vproj(h)], cfg["LCV"]),
                       (wch, cfg["LCW"]), (och, cfg["LCO"]))
            o = pv(h, s_buf, m_buf, rec=rec)
            ov_buf[...] = _rb(o[S - RV:, :])
            qproj(h + G, w4.at[h & 1, 0], rec=rec)
            start_head(h + 1)
            scores(h + 1, pltpu.bitcast(q_ring[(h + 1) & 3], bf16), s_buf, m_buf, rec=rec,
                   partial=True)
            oproj([(h, o[0:S - RV, :])], acc.at[0:S - RV, :], rec=rec)
            mod_piece(h)
            wait_head(h + 1)
            return carry
        for h in range(1, G - 1):
            cp_k(h, sem_first.at[1 + h]).wait()
        for cp in early:
            cp.wait()
        wait_head(0)
        lax.fori_loop(0, NB, main_body, 0)

        ha = NB
        rest = list(zip(range(NB + 1, H), (s2_buf, s3_buf, s4_buf), (m2_buf, m3_buf, m4_buf)))
        late = []
        for n, h in enumerate(range(NB + 3, H)):
            late += [cp_v(h, sem_first.at[8 + 2 * n]), cp_wo(h, sem_first.at[9 + 2 * n])]
        cp_wr().wait()
        for p in range(NB + 1, H):
            cp_wmx(p).wait()
        oproj([(NB - 1, ov_buf[...])], acc.at[S - RV:, :])
        for cp in late:
            cp.start()

        def l_step(j, do_x, do_y):
            if do_x and do_y:
                aw = view(acc, j - 1, TL, 2)
                ay, ax = aw.at[0:TL, :], aw.at[TL:2 * TL, :]
            elif do_x:
                ax = view(acc, j, TL)
            else:
                ay = view(acc, j - 1, TL)
            rec = None
            if do_y:
                chunks = epi_chunks(j - 1, ay, view(o_buf, j - 1, TL), with_out=do_x)
                os_ = [(h, pv(h, sv, mv, late=not do_x)) for h, sv, mv in rest]
            if do_x:
                oa = pv(ha, view(s_buf, j, TL), view(m_buf, j, TL))
            if do_y and do_x:
                oproj(os_, ay, view(x_buf, j - 1, TL))
            elif do_y:
                xv = view(x_buf, j - 1, TL)
                r0, prev = 0, []
                for n in cfg["LSPLIT"]:
                    rs = slice(r0, r0 + n)
                    nr = len(os_) * (D // W)
                    cnt = [len(prev) // nr + (1 if i < len(prev) % nr else 0) for i in range(nr)]
                    rec = _Pace(prev, cnt)
                    oproj([(h, o[rs]) for h, o in os_], ay.at[rs, :], xv.at[rs, :], rec=rec)
                    prev = chunks[r0 // 8:(r0 + n) // 8]
                    r0 += n
                chunks = prev
            if do_x:
                if do_y:
                    rec = _Pace(chunks, cfg["LCNT"])
                for h, sv, mv in rest:
                    q = pltpu.bitcast(view(q_ring.at[h & 3], j, TL // 2)[...], bf16)
                    scores(h, q, sv, mv, rec=rec)
                oproj([(ha, oa)], ax, rec=rec)
            if do_y:
                if do_x:
                    cp_out(j - 1).start()
                else:
                    for ch in chunks:
                        ch()

        for p in range(NB, H):
            mod_piece(p)
        finish_mod()
        l_step(0, True, False)
        for cp in late:
            cp.wait()

        def pl_body(j, carry):
            l_step(j, True, True)
            return carry
        lax.fori_loop(1, JL, pl_body, 0)
        l_step(JL, False, True)

        k1, k2 = key_buf[0], key_buf[1]
        for sh in (4, 2, 1):
            o1, o2 = pltpu.roll(k1, sh, 0), pltpu.roll(k2, sh, 0)
            k2 = jnp.maximum(jnp.minimum(k1, o1), jnp.maximum(k2, o2))
            k1 = jnp.maximum(k1, o1)

        def score_of(k):
            hi = k & jnp.int32(-65536)
            return pltpu.bitcast(jnp.where(hi < 0, hi ^ 0x7FFF0000, hi), f32)

        i1s = jnp.minimum(0xFFFF - (k1[0, 0] & 0xFFFF), S - 1)
        i2s = jnp.minimum(0xFFFF - (k2[0, 0] & 0xFFFF), S - 1)

        sub = lax.broadcasted_iota(i32, (16, D), 0)
        sb, cb1, gb = (_rep(modv[i], 16) for i in (1, 2, 3))

        def adaln2(x1, stat):
            return (x1 - _wide(stat[:, 0:128], D)) * _wide(stat[:, 128:256], D) * cb1 + sb

        def pick(ref):
            sel = lax.broadcasted_iota(i32, (16, ref.shape[1]), 0) == 0
            return jnp.where(sel, ref[pl.ds(i1s, 1), :], ref[pl.ds(i2s, 1), :])

        xs = adaln2(pick(acc), pick(st2_buf)).astype(bf16)
        FC, lag = cfg["FC"], cfg["FLAG"]
        kvs = [int(ch) for ch in cfg["LKV"]]
        fout = [int(ch, 36) for ch in cfg["LFO"]]
        KV = max(kvs)

        def wrows(ref, a, b, c):
            n = FC // 128
            u = [ref[c * n + t, a // 2:b // 2, :] for t in range(n)]
            return pltpu.bitcast(u[0] if n == 1 else jnp.concatenate(u, axis=1), bf16)

        DV = D - KV * 128
        if KV:
            xf = xs.astype(f32)
            for r in range(2):
                xc_buf[r] = jnp.transpose(jnp.broadcast_to(xf[r:r + 1, DV:], (128, D - DV)))
        subc = lax.broadcasted_iota(i32, (8, FC), 0)
        y = None
        act = []
        outs = out_chunks(JL - 1)
        for c in range(F // FC + lag):
            if c < F // FC:
                dm = D - kvs[c] * 128
                gu = [jnp.dot(xs[:, :dm], wrows(w, 0, dm, c), preferred_element_type=f32)[0:8, :]
                      for w in (wg, wu)]
                for v in gu:
                    for t in range(fout[c] if c < len(fout) else 0):
                        if outs:
                            outs.pop(0)(_zero_of(v[0:8, (t % 2) * 128:(t % 2 + 1) * 128]))
                            if not outs:
                                cp_out(JL - 1).start()
                if dm < D:
                    part = [[None, None], [None, None]]
                    for k in range(dm, D, 16):
                        xcol = [_wide(xc_buf[r, k - DV:k - DV + 16, :], FC) for r in range(2)]
                        for m, w in enumerate((wg, wu)):
                            wv = wrows(w, k, k + 16, c).astype(f32)
                            for r in range(2):
                                t = wv * xcol[r]
                                for e in range(2):
                                    te = t[e * 8:(e + 1) * 8, :]
                                    part[m][r] = te if part[m][r] is None else part[m][r] + te
                    for m in range(2):
                        ra, rb_ = (jnp.sum(v, axis=0, keepdims=True) for v in part[m])
                        gu[m] = gu[m] + jnp.where(subc == 0, ra, rb_)
                g, u = _rb(gu[0]), _rb(gu[1])
                act.append(_rep(_rb(g * jax.nn.sigmoid(g)) * u, 16).astype(bf16))
            if c >= lag:
                wdc = pltpu.bitcast(wd[(c - lag) * FC // 2:(c - lag + 1) * FC // 2, :], bf16)
                d = jnp.dot(act[c - lag], wdc, preferred_element_type=f32)[0:8, :]
                y = d if y is None else y + d
        y = _rb(y)
        ya = _rb(y[0:1, :] * _wide(_rb(jax.nn.sigmoid(score_of(k1[0:1, :]))), D))
        yb = _rb(y[1:2, :] * _wide(_rb(jax.nn.sigmoid(score_of(k2[0:1, :]))), D))

        g1 = pl.multiple_of((i1s >> 4) << 4, 16)
        g2 = pl.multiple_of((i2s >> 4) << 4, 16)
        for t, g0 in enumerate((g1, g2)):
            rid = sub + g0
            x1 = acc[pl.ds(g0, 16), :]
            upd = jnp.where(rid == i1s, ya, 0.0) + jnp.where(rid == i2s, yb, 0.0)
            fix[t] = (x1 + gb * (adaln2(x1, st2_buf[pl.ds(g0, 16), :]) + upd)).astype(bf16)

        pltpu.make_async_copy(o_buf, out_hbm, sem_out.at[0]).wait()

        def cp_fix(t, g0):
            return pltpu.make_async_copy(fix.at[t], out_hbm.at[pl.ds(g0, 16), :], sem_fix.at[t])

        cp_fix(0, g1).start()

        @pl.when(g2 != g1)
        def _():
            cp_fix(1, g2).start()
            cp_fix(1, g2).wait()
        cp_fix(0, g1).wait()

    def looped(*refs):
        one, refs = refs[-1], refs[:-1]
        one[0] = 1

        def body(i, carry):
            kernel(*refs)
            return carry
        lax.fori_loop(0, one[0], body, 0)

    return looped


_CFG = dict(
    G=4, T0=256, TB=1024, TL=256, MCH=256, RB=16, FC=256, PKN=8, RV=160,
    LCA='cc80', LCB2='040g', NHB=16, NL4=8, BQ=3, LCNT='33333333332000',
    LCM='cc0000000000', LCV='000010000000', LCW='00000000000g', LCO='000006bbb0z6',
    LSPLIT=(96, 96, 64), FLAG=1, LKV='00233333333333', LFO='88',
)


def _build(A_x, A_k_cache, A_v_cache, A_wq, A_wo, B_w_r, B_w_gate, B_w_up, B_w_down, c, w_mod,
           **over):
    B, S, D = A_x.shape
    _, H, SK, DH = A_k_cache.shape
    F = B_w_gate.shape[1]
    assert B == 1
    cfg = dict(_CFG, **over)
    T0, TL, G = cfg["T0"], cfg["TL"], cfg["G"]
    MC = (4 * D) // H
    kernel = _make_kernel(S, D, H, DH, SK, F, cfg)
    scratch = [
        pltpu.VMEM((S, D), bf16),
        pltpu.VMEM((S // 2, D), u32),
        pltpu.VMEM((S, D), f32),
        pltpu.VMEM((S, SK), f32),
        pltpu.VMEM((S, 128), f32),
        pltpu.VMEM((TL, SK), f32),
        pltpu.VMEM((TL, 128), f32),
        pltpu.VMEM((TL, SK), f32),
        pltpu.VMEM((TL, 128), f32),
        pltpu.VMEM((TL, SK), f32),
        pltpu.VMEM((TL, 128), f32),
        pltpu.VMEM((S, 256), f32),
        pltpu.VMEM((S, 256), f32),
        pltpu.VMEM((1, S, SK // 4 - 128), f32),
        pltpu.VMEM((4, S // 2, DH), u32),
        pltpu.VMEM((G, S, DH), f32),
        pltpu.VMEM((8, G * DH), f32),
        pltpu.VMEM((4, SK, DH), bf16),
        pltpu.VMEM((4, SK, DH), bf16),
        pltpu.VMEM((D, G * DH), bf16),
        pltpu.VMEM((2, 4, D, 128), bf16),
        pltpu.VMEM((4, 2, DH, D), bf16),
        pltpu.VMEM((G - 1, D, MC), bf16),
        pltpu.VMEM((2, D, D // 2), bf16),
        pltpu.VMEM((D, D), bf16),
        pltpu.VMEM((1, D), bf16),
        pltpu.VMEM((D,), bf16),
        pltpu.VMEM((4, 1, D // 4), f32),
        pltpu.VMEM((D, 128), f32),
        pltpu.VMEM((2, 8, D), f32),
        pltpu.VMEM((H, 1, MC), f32),
        pltpu.VMEM((9, 8, D), f32),
        pltpu.VMEM((F // 128, D // 2, 128), u32),
        pltpu.VMEM((F // 128, D // 2, 128), u32),
        pltpu.VMEM((F // 2, D), u32),
        pltpu.VMEM((2, max(int(max(cfg["LKV"])), 1) * 128, 128), f32),
        pltpu.VMEM((cfg["RV"], DH), f32),
        pltpu.VMEM((cfg["RV"] // 8, DH * 8, 128), f32),
        pltpu.VMEM((DH, D), f32),
        pltpu.VMEM((S, D), bf16),
        pltpu.VMEM((2, 8, 128), i32),
        pltpu.VMEM((2, 16, D), bf16),
        pltpu.SemaphoreType.DMA((sum(_sem_sizes(S, D, cfg)),)),
        pltpu.SMEM((1,), i32),
    ]
    any_spec = pl.BlockSpec(memory_space=pl.ANY)
    out = pl.pallas_call(
        kernel,
        out_shape=jax.ShapeDtypeStruct((S, D), bf16),
        in_specs=[any_spec] * 11,
        out_specs=any_spec,
        scratch_shapes=scratch,
        compiler_params=pltpu.CompilerParams(vmem_limit_bytes=126 * 1024 * 1024,
                                             disable_bounds_checks=True,
                                             disable_semaphore_checks=True),
    )(A_x.reshape(S, D), A_k_cache.reshape(H, SK, DH), A_v_cache.reshape(H, SK, DH),
      A_wq, A_wo, B_w_r, B_w_gate, B_w_up, B_w_down, c, w_mod)
    return out.reshape(B, S, D)


@jax.jit
def pallas_adaLN_cond__mha_block_cached__moe_arch_mod__prompt_kernel(
    A_x: jax.Array,
    A_k_cache: jax.Array,
    A_v_cache: jax.Array,
    A_wq: jax.Array,
    A_wo: jax.Array,
    B_x: jax.Array,
    B_w_r: jax.Array,
    B_w_gate: jax.Array,
    B_w_up: jax.Array,
    B_w_down: jax.Array,
    c: jax.Array,
    w_mod: jax.Array,
):
    del B_x
    return _build(A_x, A_k_cache, A_v_cache, A_wq, A_wo, B_w_r, B_w_gate, B_w_up, B_w_down,
                  c, w_mod)
```
